```python
import jax
import jax.numpy as jnp

def _softmax(x, axis=-1):
    return jax.nn.softmax(x, axis=axis)

def _gelu(x):
    return jax.nn.gelu(x, approximate=True)

def _silu(x):
    return jax.nn.silu(x)

def _sigmoid(x):
    return jax.nn.sigmoid(x)

def _layernorm(x, axis=-1, eps=1e-05):
    m = jnp.mean(x, axis=axis, keepdims=True)
    v = jnp.var(x, axis=axis, keepdims=True)
    return (x - m) / jnp.sqrt(v + eps)

def _scatter_add(tgt, idx, src, axis=0):
    return tgt.at[idx].add(src)

def _segment_sum(src, seg, n):
    return jax.ops.segment_sum(src, seg, n)

class _Rng:

    def __init__(self, key):
        self._k = key

    def _next(self):
        self._k, sub = jax.random.split(self._k)
        return sub

    def normal(self, shape):
        return jax.random.normal(self._next(), shape, dtype=jnp.bfloat16)

    def randint(self, lo, hi, shape):
        return jax.random.randint(self._next(), shape, lo, hi, dtype=jnp.int32)

    def uniform(self, shape, lo=0.0, hi=1.0):
        return jax.random.uniform(self._next(), shape, jnp.bfloat16, lo, hi)

    def permutation(self, n):
        return jax.random.permutation(self._next(), n)
kernel_name = 'concat_heads__ssm_conv_h3__memory_aug_recurrent_mem_tr__prompt'

def setup_inputs():
    _rng = _Rng(jax.random.key(int.from_bytes(__import__("os").urandom(4), "little")))
    _w = lambda a: (lambda t: t.astype(jnp.bfloat16) if jnp.issubdtype(t.dtype, jnp.floating) else t)(jnp.asarray(a))

    def _A_setup():
        B, S, D = (1, 2048, 1024)
        ks = 4
        return {'q': _w((lambda *s: _rng.normal(s) * 0.05)(B, S, D)), 'k': _w((lambda *s: _rng.normal(s) * 0.05)(B, S, D)), 'v': _w((lambda *s: _rng.normal(s) * 0.05)(B, S, D)), 'shift_k': _w((lambda *s: _rng.normal(s) * 0.05)(D, ks) * 0.5), 'ssm_k': _w((lambda *s: _rng.normal(s) * 0.05)(D, S) * (1.0 / S ** 0.5)), 'ssm_D': _w((lambda *s: _rng.normal(s) * 0.05)(D))}
    _A_in = _A_setup()

    def _B_setup():
        B, S, Dm = (1, 2048, 1024)
        H, Dh = (32, 128)
        M, seg = (8, 32)
        seg = min(seg, S)
        S = S // seg * seg
        return {'x': _w((lambda *s: _rng.normal(s) * 0.05)(B, S, Dm)), 'mem0': _w((lambda *s: _rng.normal(s) * 0.05)(B, M, Dm)), 'Wq': _w((lambda *s: _rng.normal(s) * 0.05)(Dm, H, Dh) * Dm ** (-0.5)), 'Wk': _w((lambda *s: _rng.normal(s) * 0.05)(Dm, H, Dh) * Dm ** (-0.5)), 'Wv': _w((lambda *s: _rng.normal(s) * 0.05)(Dm, H, Dh) * Dm ** (-0.5)), 'Wo': _w((lambda *s: _rng.normal(s) * 0.05)(H, Dh, Dm) * (H * Dh) ** (-0.5)), 'seg_len': seg}
    _B_in = _B_setup()
    return {'A_q': _A_in['q'], 'A_k': _A_in['k'], 'A_v': _A_in['v'], 'A_shift_k': _A_in['shift_k'], 'A_ssm_k': _A_in['ssm_k'], 'A_ssm_D': _A_in['ssm_D'], 'B_x': _B_in['x'], 'B_mem0': _B_in['mem0'], 'B_Wq': _B_in['Wq'], 'B_Wk': _B_in['Wk'], 'B_Wv': _B_in['Wv'], 'B_Wo': _B_in['Wo'], 'B_seg_len': _B_in['seg_len']}

def reference(A_q, A_k, A_v, A_shift_k, A_ssm_k, A_ssm_D, B_x, B_mem0, B_Wq, B_Wk, B_Wv, B_Wo, B_seg_len):

    def _A_ref(q, k, v, shift_k, ssm_k, ssm_D):
        B, S, D = q.shape
        ks = shift_k.shape[-1]
        k_pad = jnp.pad(k, ((0, 0), (ks - 1, 0), (0, 0)))
        k_shift = jnp.zeros_like(k)
        for t in range(ks):
            k_shift = k_shift + k_pad[:, t:t + S, :] * shift_k[:, ks - 1 - t][None, None, :]
        kv = k_shift * v
        L = 2 * S
        kv_pad = jnp.pad(kv, ((0, 0), (0, S), (0, 0)))
        kf_pad = jnp.pad(ssm_k, ((0, 0), (0, S)))
        kv_f = (lambda x, axes=(-2, -1): jnp.fft.rfft2(x.astype(jnp.float32), axes=axes))(kv_pad[:, None, :, :], axes=(1, 2))
        kf_f = (lambda x, axes=(-2, -1): jnp.fft.rfft2(x.astype(jnp.float32), axes=axes))(kf_pad[:, None, :], axes=(1, 2))
        kf_f = (lambda x, *d: x.transpose(*d))(kf_f, 1, 2, 0)
        y_f = kv_f * kf_f[None, :, :, :]
        y = (lambda x, s, axes=(-2, -1): jnp.fft.irfft2(x, s=s, axes=axes).astype(jnp.bfloat16))(y_f, (1, L), axes=(1, 2))[:, 0, :S, :]
        y = y + kv * ssm_D[None, None, :]
        return q * y

    def _B_ref(x, mem0, Wq, Wk, Wv, Wo, seg_len):
        B, S, Dm = x.shape
        H, Dh = (Wq.shape[1], Wq.shape[2])
        M = mem0.shape[1]
        scale = Dh ** (-0.5)
        n_seg = S // seg_len
        L = M + seg_len
        idx = jnp.arange(L)
        mask = (idx[:, None] < M) | (idx[:, None] >= idx[None, :])
        mem = mem0
        outs = []
        for s in range(n_seg):
            xs = x[:, s * seg_len:(s + 1) * seg_len, :].copy()
            h = jnp.concatenate([mem, xs], axis=1)
            q = jnp.einsum('btd,dhe->bhte', h, Wq)
            k = jnp.einsum('btd,dhe->bhte', h, Wk)
            v = jnp.einsum('btd,dhe->bhte', h, Wv)
            scores = jnp.einsum('bhqe,bhke->bhqk', q, k) * scale
            scores = jnp.where(mask[None, None], scores, -1000000000.0)
            p = _softmax(scores, axis=-1)
            o = jnp.einsum('bhqk,bhke->bhqe', p, v)
            o = jnp.einsum('bhte,hed->btd', o, Wo)
            mem = o[:, :M, :].copy()
            outs.append(o[:, M:, :])
        return jnp.concatenate(outs, axis=1)
    a = _A_ref(A_q, A_k, A_v, A_shift_k, A_ssm_k, A_ssm_D)
    b = _B_ref(B_x, B_mem0, B_Wq, B_Wk, B_Wv, B_Wo, B_seg_len)
    return jnp.concatenate([a, b], axis=-1)
```

```python
import functools

import numpy as np
import jax
import jax.numpy as jnp
from jax import lax
import jax.experimental.pallas as pl
import jax.experimental.pallas.tpu as pltpu

F32 = jnp.float32
BF16 = jnp.bfloat16
U32 = jnp.uint32

S = 2048
D = 1024
H = 32
DH = 128
M = 8
SEG = 32
NSEG = S // SEG
NPAIR = H // 2
R = 2 * (M + SEG)
SLAB = 520
KS = 4
C = 128
NC = S // C
NG = D // 128
NB = D // 128


def _dft_constants():
    f = np.concatenate([np.arange(0, C, 2), np.arange(1, C, 2)])
    w = np.pi * (2 * f + 1) / (2 * C)
    t = np.arange(C)
    ang = w[:, None] * t[None, :]
    fwd = np.concatenate([np.cos(ang), -np.sin(ang)], axis=0)
    inv = np.concatenate([np.cos(ang).T, -np.sin(ang).T], axis=1) / C
    return fwd.astype(np.float32), inv.astype(np.float32)


def _mask_fill():
    head = np.concatenate([np.zeros(SEG), np.ones(SEG), np.zeros(M), np.ones(M)])
    blk = np.concatenate([np.arange(M), M + np.arange(M, SEG)])
    lead = M + np.arange(M)
    pos = np.concatenate([blk, blk, lead, lead])
    same = head[:, None] == head[None, :]
    ok = (pos[:, None] < M) | (pos[:, None] >= pos[None, :])
    fill = np.where(same, np.where(ok, 0.0, -1e9), -np.inf)
    return fill.astype(np.float32)


def _dot(a, b):
    return jnp.dot(a, b, preferred_element_type=F32)


def _dot_nt(a, b):
    return lax.dot_general(a, b, (((1,), (1,)), ((), ())), preferred_element_type=F32)


def _kernel(cfg,
            aq_hbm, ak_hbm, av_hbm, sk_ref, ssmk_hbm, ssmd_ref, x_hbm, mem0_ref,
            wq_hbm, wk_hbm, wv_hbm, wo_hbm, fwd_ref, inv_ref, fill_ref,
            out_hbm,
            w_u, wo_u, wstage, wostage, xbuf, xlead, xlead_u, qkvb, ob, obuf, obb,
            abuf, hbuf, kf, kvb, ubuf, gbuf, ybuf, aout, sems):
    w_hbms = (wq_hbm, wk_hbm, wv_hbm)

    def w_copy(c):
        m, g = c // 2, c % 2
        return pltpu.make_async_copy(
            w_hbms[m].at[:, pl.ds(16 * g, 16), :], wstage.at[c % 2], sems.at[c % 2])

    xlead_cp = pltpu.make_async_copy(x_hbm.at[:, pl.ds(0, M), :], xlead, sems.at[2])
    x_cp = pltpu.make_async_copy(x_hbm, xbuf, sems.at[3])
    wo_cp = pltpu.make_async_copy(wo_hbm, wostage, sems.at[4])

    def a_copies(g):
        cps = [pltpu.make_async_copy(r.at[:, pl.ds(g * 128, 128)], abuf.at[t, g], sems.at[5])
               for t, r in enumerate((aq_hbm, ak_hbm, av_hbm))]
        return cps

    h_cp = pltpu.make_async_copy(ssmk_hbm, hbuf, sems.at[6])

    xlead_cp.start()
    w_copy(0).start()
    w_copy(1).start()

    def w_slab(m, h):
        slab = m * H + (h % 2) * NPAIR + h // 2
        return pltpu.bitcast(w_u[pl.ds(slab * SLAB, D // 2), :], BF16)

    if cfg["B"]:
        xlead_cp.wait()

        def pack_lead(t, carry):
            a = xlead[2 * t].astype(F32)
            b = xlead[2 * t + 1].astype(F32)
            v = jnp.concatenate([a, b], axis=0).astype(BF16)
            xlead_u[pl.ds(pl.multiple_of(t * 8, 8), 8), :] = pltpu.bitcast(v, U32)
            return carry
        lax.fori_loop(0, NSEG // 2, pack_lead, 0)

        def relayout(c):
            m, g = c // 2, c % 2

            def body(i, carry):
                a = pltpu.bitcast(wstage[c % 2, 2 * i], U32)
                b = pltpu.bitcast(wstage[c % 2, 2 * i + 1], U32)
                ev = (a & jnp.uint32(0xFFFF)) | (b << 16)
                od = (a >> 16) | (b & jnp.uint32(0xFFFF0000))
                base = (m * H + 8 * g) * SLAB
                w_u[pl.ds(base + i, 8, stride=SLAB), :] = ev
                w_u[pl.ds(base + NPAIR * SLAB + i, 8, stride=SLAB), :] = od
                return carry
            lax.fori_loop(0, D // 2, body, 0, unroll=8)

        def batch_proj(c):
            m, g = c // 2, c % 2

            def body(jl, carry):
                j = 8 * g + jl
                xl = pltpu.bitcast(xlead_u[...], BF16)
                outs = []
                for par in range(2):
                    row = pl.multiple_of((m * H + par * NPAIR + j) * SLAB, 8)
                    w = pltpu.bitcast(w_u[pl.ds(row, D // 2), :], BF16)
                    outs.append(_dot(xl, w).reshape(NSEG, M, DH))
                both = jnp.concatenate(outs, axis=1).astype(BF16)
                qkvb[m * NPAIR + j] = pltpu.bitcast(both, U32)
                return carry
            lax.fori_loop(0, 8, body, 0)

        for c in range(6):
            w_copy(c).wait()
            relayout(c)
            if c + 2 < 6:
                w_copy(c + 2).start()
            if c == 3:
                wo_cp.start()
                x_cp.start()
            batch_proj(c)

        wo_cp.wait()

        def wo_relayout(i, carry):
            r = pl.multiple_of(i * 64, 64)
            blk = wostage[pl.ds(r, 64), :]
            for n in range(NB):
                wo_u[n, pl.ds(pl.multiple_of(i * 32, 32), 32), :] = pltpu.bitcast(
                    blk[:, n * 128:(n + 1) * 128], U32)
            return carry
        lax.fori_loop(0, (H * DH) // 64, wo_relayout, 0)
        x_cp.wait()
    else:
        xlead_cp.wait()
        w_copy(0).wait()
        w_copy(1).wait()

    if cfg["A"]:
        for g in range(NG):
            for cp in a_copies(g):
                cp.start()
        h_cp.start()

    scale = DH ** (-0.5)

    def step(s, mem):
        xs = xbuf[s]
        top = jnp.concatenate([mem, xs[0:16].astype(F32)[8:16]], axis=0).astype(BF16)
        lhs = jnp.concatenate([top, xs[16:32]], axis=0)
        fill = fill_ref[...]
        keep = fill == 0.0

        def proj(j):
            res = []
            for m in range(3):
                a = _dot(lhs, w_slab(m, 2 * j)).astype(BF16)
                b = _dot(lhs, w_slab(m, 2 * j + 1)).astype(BF16)
                lead = pltpu.bitcast(qkvb[m * NPAIR + j, s], BF16)
                res.append(jnp.concatenate([a, b, lead], axis=0))
            return res

        def probs(q, k):
            sc = jnp.where(keep, _dot_nt(q, k) * scale, fill)
            mx = jnp.max(sc, axis=-1, keepdims=True)
            e = jnp.exp(sc - mx)
            l = jnp.sum(e, axis=-1, keepdims=True)
            r = pl.reciprocal(l, approx=True)
            r = r * (2.0 - l * r)
            return (e * r).astype(BF16)

        def attend(j, p, v):
            o = _dot(p, v)
            row = pl.multiple_of(s * M, M)
            ob[2 * j, pl.ds(row, M), :] = o[2 * SEG:2 * SEG + M].astype(BF16)
            ob[2 * j + 1, pl.ds(row, M), :] = o[2 * SEG + M:].astype(BF16)
            return [o[0:SEG].astype(BF16), o[SEG:2 * SEG].astype(BF16)]

        qkv, ps, os_ = {}, {}, []
        l1, l2 = cfg["lag1"], cfg["lag2"]
        for t in range(NPAIR + l2):
            if t < NPAIR:
                qkv[t] = proj(t)
            if 0 <= t - l1 < NPAIR:
                ps[t - l1] = probs(qkv[t - l1][0], qkv[t - l1][1])
            if 0 <= t - l2 < NPAIR:
                os_ += attend(t - l2, ps[t - l2], qkv[t - l2][2])

        ksplit = cfg["ksplit"]
        o1 = jnp.concatenate(os_[:ksplit], axis=1)
        o2 = jnp.concatenate(os_[ksplit:], axis=1)
        acc = []
        for n in range(NB):
            w = pltpu.bitcast(wo_u[n, pl.ds(0, ksplit * 64), :], BF16)
            acc.append(_dot(o1, w))
        for n in range(NB):
            w = pltpu.bitcast(wo_u[n, pl.ds(ksplit * 64, (H - ksplit) * 64), :], BF16)
            acc[n] = acc[n] + _dot(o2, w)
        res = jnp.concatenate(acc, axis=1)
        obuf[s] = res.astype(BF16)
        return res[0:M]

    ob_cp = pltpu.make_async_copy(
        obuf.at[:, pl.ds(M, SEG - M), :],
        out_hbm.at[:, pl.ds(M, SEG - M), pl.ds(D, D)], sems.at[7])

    def obb_cp(n):
        return pltpu.make_async_copy(
            obb.at[n], out_hbm.at[:, pl.ds(0, M), pl.ds(D + n * 128, 128)], sems.at[8])

    if cfg["B"]:
        lax.fori_loop(0, cfg["nstep"], step, mem0_ref[...].astype(F32))
        ob_cp.start()

        def epi(n, carry):
            lhs = jnp.concatenate([ob[h] for h in range(H)], axis=1)
            w = pltpu.bitcast(wo_u[n], BF16)
            obb[n] = _dot(lhs, w).reshape(NSEG, M, 128).astype(BF16)
            return carry
        lax.fori_loop(0, NB, epi, 0)
        for n in range(NB):
            obb_cp(n).start()

    def aout_cp(g):
        return pltpu.make_async_copy(
            aout.at[g], out_hbm.at[:, :, pl.ds(g * 128, 128)], sems.at[9])

    if cfg["A"]:
        for g in range(NG):
            for cp in a_copies(g):
                cp.wait()
        h_cp.wait()
        kf[pl.ds(0, 8), :] = jnp.zeros((8, 128), F32)

        def group(g, carry):
            sk = sk_ref[g].astype(F32)
            dd = ssmd_ref[g].astype(F32)
            fwd = fwd_ref[...]
            inv = inv_ref[...]

            def stage1(i, c):
                r = pl.multiple_of(i * C, C)
                kf[pl.ds(8 + r, C), :] = abuf[1, g, pl.ds(r, C), :].astype(F32)
                ks = kf[pl.ds(8 + r, C), :] * sk[0:1]
                for j in range(1, KS):
                    ks = ks + kf[pl.ds(8 + r - j, C), :] * sk[j:j + 1]
                kv = (ks * abuf[2, g, pl.ds(r, C), :].astype(F32)).astype(BF16)
                kvb[pl.ds(pl.multiple_of(i * (C // 2), C // 2), C // 2), :] = pltpu.bitcast(kv, U32)
                ubuf[i] = _dot(fwd, kv)
                return c
            lax.fori_loop(0, NC, stage1, 0)
            hrows = hbuf[pl.ds(pl.multiple_of(g * 128, 128), 128), :]
            for i in range(NC):
                gbuf[i] = _dot_nt(fwd, hrows[:, i * C:(i + 1) * C])

            def stage2(p, sgn):
                r = pl.multiple_of(p * 16, 16)
                ua = [ubuf[i, pl.ds(r, 16), :] for i in range(NC)]
                ub = [ubuf[i, pl.ds(C + r, 16), :] for i in range(NC)]
                hr = [gbuf[i, pl.ds(r, 16), :] for i in range(NC)]
                hi = [gbuf[i, pl.ds(C + r, 16), :] for i in range(NC)]
                gc = [hr[0]] + [hr[i] - sgn * hi[i - 1] for i in range(1, NC)]
                gd = [hi[0]] + [hi[i] + sgn * hr[i - 1] for i in range(1, NC)]

                def conv(a, b):
                    outs = []
                    for i in range(NC):
                        acc = a[i] * b[0]
                        for j in range(1, i + 1):
                            acc = acc + a[i - j] * b[j]
                        outs.append(acc)
                    return outs
                k1 = conv(gc, [ua[i] + ub[i] for i in range(NC)])
                k2 = conv([gd[i] - gc[i] for i in range(NC)], ua)
                k3 = conv([gd[i] + gc[i] for i in range(NC)], ub)
                q8 = pl.multiple_of(p * 8, 8)
                for i in range(NC):
                    ybuf[i, pl.ds(q8, 8), :] = pltpu.bitcast((k1[i] - k3[i]).astype(BF16), U32)
                    ybuf[i, pl.ds(C // 2 + q8, 8), :] = pltpu.bitcast((k1[i] + k2[i]).astype(BF16), U32)

            def stage2_loop(p, c):
                sgn = jnp.where(p < 4, 1.0, -1.0).astype(F32)
                stage2(p, sgn)
                return c
            lax.fori_loop(0, 8, stage2_loop, 0)

            def stage3(i, c):
                r = pl.multiple_of(i * C, C)
                y = _dot(inv, pltpu.bitcast(ybuf[i], BF16))
                kv = pltpu.bitcast(kvb[pl.ds(pl.multiple_of(i * (C // 2), C // 2), C // 2), :], BF16)
                y = y + kv.astype(F32) * dd
                o = (abuf[0, g, pl.ds(r, C), :].astype(F32) * y).astype(BF16)
                aout[g, pl.ds(pl.multiple_of(i * 4, 4), 4)] = o.reshape(4, SEG, 128)
                return c
            lax.fori_loop(0, NC, stage3, 0)
            return carry
        lax.fori_loop(0, NG, group, 0)
        for g in range(NG):
            aout_cp(g).start()
        for g in range(NG):
            aout_cp(g).wait()

    if cfg["B"]:
        ob_cp.wait()
        for n in range(NB):
            obb_cp(n).wait()


_DEFAULT_CFG = dict(A=True, B=True, nstep=NSEG, lag1=1, lag2=2, ksplit=24)


def _build(cfg):
    fwd_np, inv_np = _dft_constants()
    fill_np = _mask_fill()

    def run(A_q, A_k, A_v, A_shift_k, A_ssm_k, A_ssm_D, B_x, B_mem0, B_Wq, B_Wk, B_Wv, B_Wo):
        sk = A_shift_k.T.reshape(KS, NG, 128).transpose(1, 0, 2)
        dd = A_ssm_D.reshape(NG, 1, 128)
        any_spec = pl.BlockSpec(memory_space=pl.ANY)
        vmem_spec = pl.BlockSpec(memory_space=pltpu.VMEM)
        out = pl.pallas_call(
            functools.partial(_kernel, cfg),
            out_shape=jax.ShapeDtypeStruct((NSEG, SEG, 2 * D), BF16),
            in_specs=[any_spec, any_spec, any_spec, vmem_spec, any_spec, vmem_spec,
                      any_spec, vmem_spec, any_spec, any_spec, any_spec, any_spec,
                      vmem_spec, vmem_spec, vmem_spec],
            out_specs=any_spec,
            scratch_shapes=[
                pltpu.VMEM((3 * H * SLAB, 128), U32),
                pltpu.VMEM((NB, H * DH // 2, 128), U32),
                pltpu.VMEM((2, D, 16, DH), BF16),
                pltpu.VMEM((H * DH, D), BF16),
                pltpu.VMEM((NSEG, SEG, D), BF16),
                pltpu.VMEM((NSEG, M, D), BF16),
                pltpu.VMEM((NSEG * M // 2, D), U32),
                pltpu.VMEM((3 * NPAIR, NSEG, 8, 128), U32),
                pltpu.VMEM((H, NSEG * M, DH), BF16),
                pltpu.VMEM((NSEG, SEG, D), BF16),
                pltpu.VMEM((NB, NSEG, M, 128), BF16),
                pltpu.VMEM((3, NG, S, 128), BF16),
                pltpu.VMEM((D, S), BF16),
                pltpu.VMEM((S + 8, 128), F32),
                pltpu.VMEM((S // 2, 128), U32),
                pltpu.VMEM((NC, 2 * C, 128), F32),
                pltpu.VMEM((NC, 2 * C, 128), F32),
                pltpu.VMEM((NC, C, 128), U32),
                pltpu.VMEM((NG, NSEG, SEG, 128), BF16),
                pltpu.SemaphoreType.DMA((10,)),
            ],
            compiler_params=pltpu.CompilerParams(vmem_limit_bytes=120 * 1024 * 1024),
        )(A_q.reshape(S, D), A_k.reshape(S, D), A_v.reshape(S, D), sk, A_ssm_k, dd,
          B_x.reshape(NSEG, SEG, D), B_mem0.reshape(M, D), B_Wq, B_Wk, B_Wv,
          B_Wo.reshape(H * DH, D),
          jnp.asarray(fwd_np, BF16), jnp.asarray(inv_np, BF16), jnp.asarray(fill_np))
        return out.reshape(1, S, 2 * D)

    return run


@functools.partial(jax.jit, static_argnames=("B_seg_len",))
def pallas_concat_heads__ssm_conv_h3__memory_aug_recurrent_mem_tr__prompt_kernel(
    A_q: jax.Array,
    A_k: jax.Array,
    A_v: jax.Array,
    A_shift_k: jax.Array,
    A_ssm_k: jax.Array,
    A_ssm_D: jax.Array,
    B_x: jax.Array,
    B_mem0: jax.Array,
    B_Wq: jax.Array,
    B_Wk: jax.Array,
    B_Wv: jax.Array,
    B_Wo: jax.Array,
    B_seg_len: int = SEG,
):
    assert B_seg_len == SEG
    return _build(_DEFAULT_CFG)(A_q, A_k, A_v, A_shift_k, A_ssm_k, A_ssm_D, B_x, B_mem0,
                                B_Wq, B_Wk, B_Wv, B_Wo)
```

```python
import functools

import numpy as np
import jax
import jax.numpy as jnp
from jax import lax
import jax.experimental.pallas as pl
import jax.experimental.pallas.tpu as pltpu

F32 = jnp.float32
BF16 = jnp.bfloat16
U32 = jnp.uint32

S = 2048
D = 1024
H = 32
DH = 128
M = 8
SEG = 32
NSEG = S // SEG
NPAIR = H // 2
R = 2 * (M + SEG)
SLAB = 520
KS = 4
C = 128
NC = S // C
NG = D // 128
NB = D // 128


def _dft_constants():
    f = np.concatenate([np.arange(0, C, 2), np.arange(1, C, 2)])
    w = np.pi * (2 * f + 1) / (2 * C)
    t = np.arange(C)
    ang = w[:, None] * t[None, :]
    fwd = np.concatenate([np.cos(ang), -np.sin(ang)], axis=0)
    inv = np.concatenate([np.cos(ang).T, -np.sin(ang).T], axis=1) / C
    return fwd.astype(np.float32), inv.astype(np.float32)


def _mask_fill():
    head = np.concatenate([np.zeros(SEG), np.ones(SEG), np.zeros(M), np.ones(M)])
    blk = np.concatenate([np.arange(M), M + np.arange(M, SEG)])
    lead = M + np.arange(M)
    pos = np.concatenate([blk, blk, lead, lead])
    same = head[:, None] == head[None, :]
    ok = (pos[:, None] < M) | (pos[:, None] >= pos[None, :])
    fill = np.where(same, np.where(ok, 0.0, -1e9), -np.inf)
    return fill.astype(np.float32)


def _dot(a, b):
    return jnp.dot(a, b, preferred_element_type=F32)


def _dot_nt(a, b):
    return lax.dot_general(a, b, (((1,), (1,)), ((), ())), preferred_element_type=F32)


def _kernel(cfg,
            aq_hbm, ak_hbm, av_hbm, sk_ref, ssmk_hbm, ssmd_ref, x_hbm, mem0_ref,
            wq_hbm, wk_hbm, wv_hbm, wo_hbm, fwd_ref, inv_ref, fill_ref,
            out_hbm,
            w_u, wo_u, wstage, wostage, xbuf, xlead, xlead_u, qkvb, ob, obuf, obb,
            abuf, hbuf, kf, kvb, ubuf, gbuf, hlast, aout,
            sem_w, sem_wo, sem_x, sem_h, sem_a, sem_out):
    w_hbms = (wq_hbm, wk_hbm, wv_hbm)
    a_hbms = (aq_hbm, ak_hbm, av_hbm)
    do_a = cfg["A"]

    def w_copy(c, k):
        m, g = c // 2, c % 2
        slot = (c % 2) * 8 + k
        return pltpu.make_async_copy(
            w_hbms[m].at[pl.ds(k * 128, 128), pl.ds(16 * g, 16), :],
            wstage.at[slot], sem_w.at[slot])

    def w_wait(slot):
        pltpu.make_async_copy(wstage.at[slot], wstage.at[slot], sem_w.at[slot]).wait()

    def wo_copy(k):
        return pltpu.make_async_copy(
            wo_hbm.at[pl.ds(k * 512, 512), :], wostage.at[k], sem_wo.at[k])

    xlead_cp = pltpu.make_async_copy(x_hbm.at[:, pl.ds(0, M), :], xlead, sem_x.at[0])
    x_cp = pltpu.make_async_copy(
        x_hbm.at[:, pl.ds(M, SEG - M), :], xbuf.at[:, pl.ds(M, SEG - M), :], sem_x.at[1])

    def h_copy(c):
        return pltpu.make_async_copy(
            ssmk_hbm.at[:, pl.ds(c * C, C)], hbuf.at[c], sem_h.at[0])

    def a_copy(t, g):
        return pltpu.make_async_copy(
            a_hbms[t].at[:, pl.ds(g * 128, 128)], abuf.at[g, t], sem_a.at[g])

    xlead_cp.start()
    for c in range(2):
        for k in range(8):
            w_copy(c, k).start()

    def relayout_piece(c, k, slot, dpairs=None):
        base = ((c // 2) * H + 8 * (c % 2)) * SLAB + k * 64
        for i in range(64):
            a = pltpu.bitcast(wstage[slot, 2 * i], U32)
            b = pltpu.bitcast(wstage[slot, 2 * i + 1], U32)
            ev = (a & jnp.uint32(0xFFFF)) | (b << 16)
            od = (a >> 16) | (b & jnp.uint32(0xFFFF0000))
            w_u[pl.ds(base + i, 8, stride=SLAB), :] = ev
            w_u[pl.ds(base + NPAIR * SLAB + i, 8, stride=SLAB), :] = od

    def batch_pair(it):
        m = it // NPAIR
        j = it % NPAIR
        xl = pltpu.bitcast(xlead_u[...], BF16)
        outs = []
        for par in range(2):
            row = pl.multiple_of((m * H + par * NPAIR + j) * SLAB, 8)
            w = pltpu.bitcast(w_u[pl.ds(row, D // 2), :], BF16)
            outs.append(_dot(xl, w).reshape(NSEG, M, DH))
        both = jnp.concatenate(outs, axis=1).astype(BF16)
        qkvb[it] = pltpu.bitcast(both, U32)

    xlead_cp.wait()

    def pack_lead(t, carry):
        a = xlead[2 * t].astype(F32)
        b = xlead[2 * t + 1].astype(F32)
        v = jnp.concatenate([a, b], axis=0).astype(BF16)
        xlead_u[pl.ds(pl.multiple_of(t * 8, 8), 8), :] = pltpu.bitcast(v, U32)
        return carry
    lax.fori_loop(0, NSEG // 2, pack_lead, 0)

    if do_a:
        kf[pl.ds(0, 8), :] = jnp.zeros((8, 128), F32)
        for b in range(2):
            gbuf[b, pl.ds(0, 7)] = jnp.zeros((7, 2 * C, 128), F32)

    def first_chunk(k, carry):
        w_wait(k)
        relayout_piece(0, k, k)
        return carry
    lax.fori_loop(0, 8, first_chunk, 0)

    PP = cfg["pp"]
    IPC = 8 // PP

    def issue(c):
        if c + 2 < 6:
            for k in range(8):
                w_copy(c + 2, k).start()
        if c < 2:
            for k in range(4 * c, 4 * c + 4):
                wo_copy(k).start()
        if c == 2:
            x_cp.start()
        if do_a and c == 3:
            for cc in range(NC):
                h_copy(cc).start()
        if do_a and c == 4:
            for g in range(NG):
                for t in (1, 2, 0):
                    a_copy(t, g).start()

    def pro_body(it, carry):
        for c in range(5):
            @pl.when(it == c * IPC)
            def _():
                issue(c)
        cn = it // IPC + 1
        for u in range(PP):
            k = (it % IPC) * PP + u
            w_wait((cn % 2) * 8 + k)
        for u in range(PP):
            k = (it % IPC) * PP + u
            batch_pair(it * PP + u)
            relayout_piece(cn, k, (cn % 2) * 8 + k)
        return carry
    lax.fori_loop(0, 5 * IPC, pro_body, 0)

    def pro_last(it, carry):
        for u in range(PP):
            k = it * PP + u
            pltpu.make_async_copy(wostage.at[k], wostage.at[k], sem_wo.at[k]).wait()
        for u in range(PP):
            k = it * PP + u
            batch_pair(40 + k)
            for r in range(8):
                blk = wostage[k, pl.ds(r * 64, 64), :]
                row = pl.multiple_of(k * 256 + r * 32, 32)
                for n in range(NB):
                    wo_u[n, pl.ds(row, 32), :] = pltpu.bitcast(blk[:, n * 128:(n + 1) * 128], U32)
        return carry
    lax.fori_loop(0, IPC, pro_last, 0)
    x_cp.wait()
    if do_a:
        pltpu.make_async_copy(hbuf, hbuf, sem_h.at[0]).wait()

    def a_stage1_pre(g, p):
        sk = sk_ref[g].astype(F32)
        r = pl.multiple_of(p * 2 * C, 2 * C)
        kf[pl.ds(8 + r, 2 * C), :] = abuf[g, 1, pl.ds(r, 2 * C), :].astype(F32)
        ks = kf[pl.ds(8 + r, 2 * C), :] * sk[0:1]
        for j in range(1, KS):
            ks = ks + kf[pl.ds(8 + r - j, 2 * C), :] * sk[j:j + 1]
        kv = (ks * abuf[g, 2, pl.ds(r, 2 * C), :].astype(F32)).astype(BF16)
        kvb[g % 2, pl.ds(pl.multiple_of(p * C, C), C), :] = pltpu.bitcast(kv, U32)
        return kv

    def a_stage1_u(g, p, kv):
        fwd = fwd_ref[...]
        for u in range(2):
            ubuf[g % 2, 2 * p + u] = _dot(fwd, kv[u * C:(u + 1) * C])

    def a_stage1_h(g, p):
        fwd = fwd_ref[...]
        rows = pl.ds(pl.multiple_of(g * 128, 128), 128)
        hs = [_dot_nt(fwd, hbuf[2 * p + u, rows, :]) for u in range(2)]
        prev = jnp.where(p == 0, 0.0, hlast[...])
        hlast[...] = hs[1]
        hc = C // 2
        for u, (cur, prv) in enumerate(((hs[0], prev), (hs[1], hs[0]))):
            gbuf[g % 2, 7 + 2 * p + u] = jnp.concatenate([
                cur[0:hc] - prv[C:C + hc], cur[hc:C] + prv[C + hc:],
                cur[C:C + hc] + prv[0:hc], cur[C + hc:] - prv[hc:C]], axis=0)

    def a_stage2(gp, p):
        b = gp % 2
        RB = cfg["rb"]
        chain = cfg["chain"]
        never = p > 100
        re = [[], []]
        im = [[], []]
        last = None
        for r in range(0, C, RB):
            gr = [gbuf[b, 7 + p + 8 - j, pl.ds(r, RB), :] for j in range(NC)]
            gi = [gbuf[b, 7 + p + 8 - j, pl.ds(C + r, RB), :] for j in range(NC)]
            ur = [ubuf[b, j, pl.ds(r, RB), :] for j in range(NC)]
            ui = [ubuf[b, j, pl.ds(C + r, RB), :] for j in range(NC)]
            for o, (nt, off) in enumerate(((8, 8), (16, 0))):
                if chain == 0:
                    ar = ai = None
                    for j in range(nt):
                        tr = gr[j + off] * ur[j] - gi[j + off] * ui[j]
                        ti = gr[j + off] * ui[j] + gi[j + off] * ur[j]
                        ar = tr if ar is None else ar + tr
                        ai = ti if ai is None else ai + ti
                else:
                    ar = gr[off] * ur[0]
                    ai = gr[off] * ui[0]
                    if last is not None:
                        ar = jnp.where(never, last[0], ar)
                        ai = jnp.where(never, last[1], ai)
                    ar = ar - gi[off] * ui[0]
                    ai = ai + gi[off] * ur[0]
                    for j in range(1, nt):
                        ar = ar + gr[j + off] * ur[j]
                        ai = ai + gr[j + off] * ui[j]
                        ar = ar - gi[j + off] * ui[j]
                        ai = ai + gi[j + off] * ur[j]
                    last = (ar, ai)
                re[o].append(ar)
                im[o].append(ai)
        return [jnp.concatenate(re[o] + im[o], axis=0).astype(BF16) for o in range(2)]

    def a_stage3(gp, gq, p, ys):
        inv = inv_ref[...]
        dd = ssmd_ref[gq].astype(F32)
        for o in range(2):
            i = p + 8 * o
            y = _dot(inv, ys[o])
            kv = pltpu.bitcast(
                kvb[gp % 2, pl.ds(pl.multiple_of(i * (C // 2), C // 2), C // 2), :], BF16)
            y = y + kv.astype(F32) * dd
            q = abuf[gq, 0, pl.ds(pl.multiple_of(i * C, C), C), :]
            res = (q.astype(F32) * y).astype(BF16)
            aout[gq, pl.ds(pl.multiple_of(i * 4, 4), 4)] = res.reshape(4, SEG, 128)

    scale = DH ** (-0.5)

    def w_slab(m, h):
        slab = m * H + (h % 2) * NPAIR + h // 2
        return pltpu.bitcast(w_u[pl.ds(slab * SLAB, D // 2), :], BF16)

    def step(s, mem):
        g = s // 8
        p = s % 8
        if do_a:
            @pl.when(p == 0)
            def _():
                pltpu.make_async_copy(abuf.at[g], abuf.at[g], sem_a.at[g]).wait()

        x1 = xbuf[s, pl.ds(M, M), :].astype(F32)
        top = jnp.concatenate([mem, x1], axis=0).astype(BF16)
        lhs = jnp.concatenate([top, xbuf[s, pl.ds(16, 16), :]], axis=0)
        fill = fill_ref[...]
        keep = fill == 0.0

        def proj(m, j):
            a = _dot(lhs, w_slab(m, 2 * j)).astype(BF16)
            b = _dot(lhs, w_slab(m, 2 * j + 1)).astype(BF16)
            lead = pltpu.bitcast(qkvb[m * NPAIR + j, s], BF16)
            return jnp.concatenate([a, b, lead], axis=0)

        def probs(q, k):
            sc = jnp.where(keep, _dot_nt(q, k) * scale, fill)
            mx = jnp.max(sc, axis=-1, keepdims=True)
            e = jnp.exp(sc - mx)
            l = jnp.sum(e, axis=-1, keepdims=True)
            r = pl.reciprocal(l, approx=True)
            r = r * (2.0 - l * r)
            return (e * r).astype(BF16)

        def attend(j, p_, v):
            o = _dot(p_, v)
            row = pl.multiple_of(s * M, M)
            ob[2 * j, pl.ds(row, M), :] = o[2 * SEG:2 * SEG + M].astype(BF16)
            ob[2 * j + 1, pl.ds(row, M), :] = o[2 * SEG + M:].astype(BF16)
            return [o[0:SEG].astype(BF16), o[SEG:2 * SEG].astype(BF16)]

        qkv, ps, os_ = {}, {}, []
        acc = [None] * NB
        st = {}

        def wo(h0, h1, ns):
            o = jnp.concatenate(os_[h0:h1], axis=1)
            for n in ns:
                w = pltpu.bitcast(wo_u[n, pl.ds(h0 * 64, (h1 - h0) * 64), :], BF16)
                d = _dot(o, w)
                acc[n] = d if acc[n] is None else d + acc[n]

        gp = g + 1
        gq = jnp.maximum(g - 1, 0)
        for item in _make_order(cfg["order"]):
            kind = item[0]
            if kind == "P":
                qkv[item[1], item[2]] = proj(item[1], item[2])
            elif kind == "S":
                j = item[1]
                ps[j] = probs(qkv[0, j], qkv[1, j])
            elif kind == "V":
                j = item[1]
                os_ += attend(j, ps[j], qkv[2, j])
            elif kind == "W":
                wo(item[1], item[2], item[3])
            elif not do_a:
                pass
            elif kind == "A1":
                st["kv"] = a_stage1_pre(g, p)
            elif kind == "AU":
                a_stage1_u(g, p, st["kv"])
            elif kind == "AH":
                a_stage1_h(g, p)
            elif kind == "A2":
                st["ys"] = a_stage2(gp, p)
            elif kind == "A3":
                a_stage3(gp, gq, p, st["ys"])
        res = jnp.concatenate(acc, axis=1)
        obuf[s] = res.astype(BF16)
        return res[0:M]

    lax.fori_loop(0, cfg["nstep"], step, mem0_ref[...].astype(F32))

    ob_cp = pltpu.make_async_copy(
        obuf.at[:, pl.ds(M, SEG - M), :],
        out_hbm.at[:, pl.ds(M, SEG - M), pl.ds(D, D)], sem_out.at[0])

    def obb_cp(n):
        return pltpu.make_async_copy(
            obb.at[n], out_hbm.at[:, pl.ds(0, M), pl.ds(D + n * 128, 128)], sem_out.at[1])

    def aout_cp(g):
        return pltpu.make_async_copy(
            aout.at[g], out_hbm.at[:, :, pl.ds(g * 128, 128)], sem_out.at[2])

    ob_cp.start()
    if do_a:
        for g in range(NG - 1):
            aout_cp(g).start()

    EP = cfg["ep"]

    def epi(it, carry):
        lhs = jnp.concatenate([ob[h] for h in range(H)], axis=1)
        for u in range(EP):
            n = it * EP + u
            if do_a:
                ys = a_stage2(NG - 1, n)
            w = pltpu.bitcast(wo_u[n], BF16)
            obb[n] = _dot(lhs, w).reshape(NSEG, M, 128).astype(BF16)
            if do_a:
                a_stage3(NG - 1, NG - 1, n, ys)
        return carry
    lax.fori_loop(0, NB // EP, epi, 0)
    for n in range(NB):
        obb_cp(n).start()
    if do_a:
        aout_cp(NG - 1).start()
        for g in range(NG):
            aout_cp(g).wait()
    ob_cp.wait()
    for n in range(NB):
        obb_cp(n).wait()


def _make_order(kind):
    alln = tuple(range(NB))
    if kind == 1:
        order = [("A1",), ("AH",)]
        for t in range(NPAIR):
            order += [("P", 0, t), ("P", 1, t), ("P", 2, t)]
            if t >= 1:
                order.append(("S", t - 1))
            if t >= 2:
                order.append(("V", t - 2))
            if t == 1:
                order += [("AU",), ("A2",)]
        order += [("W", 0, 24, (0, 1)), ("S", 15), ("V", 14), ("W", 0, 24, (2, 3)), ("A3",), ("V", 15),
                  ("W", 0, 24, (4, 5, 6, 7)), ("W", 24, 32, alln)]
    elif kind == 2:
        order = [("A1",), ("AH",)]
        for t in range(NPAIR):
            order.append(("P", 0, t))
            if t >= 1:
                order.append(("S", t - 1))
            order += [("P", 1, t), ("P", 2, t)]
            if t >= 2:
                order.append(("V", t - 2))
            if t == 1:
                order += [("AU",), ("A2",)]
        order += [("W", 0, 24, (0,)), ("S", 15), ("W", 0, 24, (1,)), ("V", 14), ("W", 0, 24, (2, 3)),
                  ("A3",), ("V", 15), ("W", 0, 24, (4, 5, 6, 7)), ("W", 24, 32, alln)]
    elif kind == 3:
        order = [("A1",), ("AH",)]
        for t in range(NPAIR):
            order.append(("P", 0, t))
            if t >= 1:
                order.append(("P", 2, t - 1))
                order.append(("S", t - 1))
            order.append(("P", 1, t))
            if t >= 2:
                order.append(("V", t - 2))
            if t == 1:
                order += [("AU",), ("A2",)]
        order += [("P", 2, 15), ("W", 0, 24, (0,)), ("S", 15), ("W", 0, 24, (1,)), ("V", 14), ("W", 0, 24, (2, 3)),
                  ("A3",), ("V", 15), ("W", 0, 24, (4, 5, 6, 7)), ("W", 24, 32, alln)]
    return order


_DEFAULT_CFG = dict(A=True, nstep=NSEG, order=3, pp=2, ep=1, rb=16, chain=1)


def _build(cfg):
    fwd_np, inv_np = _dft_constants()
    fill_np = _mask_fill()

    def run(A_q, A_k, A_v, A_shift_k, A_ssm_k, A_ssm_D, B_x, B_mem0, B_Wq, B_Wk, B_Wv, B_Wo):
        sk = A_shift_k.T.reshape(KS, NG, 128).transpose(1, 0, 2)
        dd = A_ssm_D.reshape(NG, 1, 128)
        any_spec = pl.BlockSpec(memory_space=pl.ANY)
        vmem_spec = pl.BlockSpec(memory_space=pltpu.VMEM)
        out = pl.pallas_call(
            functools.partial(_kernel, cfg),
            out_shape=jax.ShapeDtypeStruct((NSEG, SEG, 2 * D), BF16),
            in_specs=[any_spec, any_spec, any_spec, vmem_spec, any_spec, vmem_spec,
                      any_spec, vmem_spec, any_spec, any_spec, any_spec, any_spec,
                      vmem_spec, vmem_spec, vmem_spec],
            out_specs=any_spec,
            scratch_shapes=[
                pltpu.VMEM((3 * H * SLAB, 128), U32),
                pltpu.VMEM((NB, H * DH // 2, 128), U32),
                pltpu.VMEM((16, 128, 16, DH), BF16),
                pltpu.VMEM((8, 512, D), BF16),
                pltpu.VMEM((NSEG, SEG, D), BF16),
                pltpu.VMEM((NSEG, M, D), BF16),
                pltpu.VMEM((NSEG * M // 2, D), U32),
                pltpu.VMEM((3 * NPAIR, NSEG, 8, 128), U32),
                pltpu.VMEM((H, NSEG * M, DH), BF16),
                pltpu.VMEM((NSEG, SEG, D), BF16),
                pltpu.VMEM((NB, NSEG, M, 128), BF16),
                pltpu.VMEM((NG, 3, S, 128), BF16),
                pltpu.VMEM((NC, D, C), BF16),
                pltpu.VMEM((S + 8, 128), F32),
                pltpu.VMEM((2, S // 2, 128), U32),
                pltpu.VMEM((2, NC, 2 * C, 128), F32),
                pltpu.VMEM((2, NC + 7, 2 * C, 128), F32),
                pltpu.VMEM((2 * C, 128), F32),
                pltpu.VMEM((NG, NSEG, SEG, 128), BF16),
                pltpu.SemaphoreType.DMA((16,)),
                pltpu.SemaphoreType.DMA((8,)),
                pltpu.SemaphoreType.DMA((2,)),
                pltpu.SemaphoreType.DMA((1,)),
                pltpu.SemaphoreType.DMA((NG,)),
                pltpu.SemaphoreType.DMA((3,)),
            ],
            compiler_params=pltpu.CompilerParams(vmem_limit_bytes=124 * 1024 * 1024),
        )(A_q.reshape(S, D), A_k.reshape(S, D), A_v.reshape(S, D), sk, A_ssm_k, dd,
          B_x.reshape(NSEG, SEG, D), B_mem0.reshape(M, D), B_Wq, B_Wk, B_Wv,
          B_Wo.reshape(H * DH, D),
          jnp.asarray(fwd_np, BF16), jnp.asarray(inv_np, BF16), jnp.asarray(fill_np))
        return out.reshape(1, S, 2 * D)

    return run


@functools.partial(jax.jit, static_argnames=("B_seg_len",))
def pallas_concat_heads__ssm_conv_h3__memory_aug_recurrent_mem_tr__prompt_kernel(
    A_q: jax.Array,
    A_k: jax.Array,
    A_v: jax.Array,
    A_shift_k: jax.Array,
    A_ssm_k: jax.Array,
    A_ssm_D: jax.Array,
    B_x: jax.Array,
    B_mem0: jax.Array,
    B_Wq: jax.Array,
    B_Wk: jax.Array,
    B_Wv: jax.Array,
    B_Wo: jax.Array,
    B_seg_len: int = SEG,
):
    assert B_seg_len == SEG
    return _build(_DEFAULT_CFG)(A_q, A_k, A_v, A_shift_k, A_ssm_k, A_ssm_D, B_x, B_mem0,
                                B_Wq, B_Wk, B_Wv, B_Wo)
```

```python
import functools

import numpy as np
import jax
import jax.numpy as jnp
from jax import lax
import jax.experimental.pallas as pl
import jax.experimental.pallas.tpu as pltpu

F32 = jnp.float32
BF16 = jnp.bfloat16
U32 = jnp.uint32

S = 2048
D = 1024
H = 32
DH = 128
M = 8
SEG = 32
NSEG = S // SEG
NPAIR = H // 2
R = 2 * (M + SEG)
SLAB = 520
KS = 4
C = 128
NC = S // C
NG = D // 128
KQ = D // 4
KPAD = 32
NB = D // 128


def _dft_constants():
    f = np.concatenate([np.arange(0, C, 2), np.arange(1, C, 2)])
    w = np.pi * (2 * f + 1) / (2 * C)
    t = np.arange(C)
    ang = w[:, None] * t[None, :]
    fwd = np.concatenate([np.cos(ang), -np.sin(ang)], axis=0)
    inv = np.concatenate([np.cos(ang).T, -np.sin(ang).T], axis=1) / C
    return fwd.astype(np.float32), inv.astype(np.float32)


def _mask_fill():
    head = np.concatenate([np.zeros(SEG), np.ones(SEG), np.zeros(M), np.ones(M)])
    blk = np.concatenate([np.arange(M), M + np.arange(M, SEG)])
    lead = M + np.arange(M)
    pos = np.concatenate([blk, blk, lead, lead])
    same = head[:, None] == head[None, :]
    ok = (pos[:, None] < M) | (pos[:, None] >= pos[None, :])
    fill = np.where(same, np.where(ok, 0.0, -1e9), -np.inf)
    return fill.astype(np.float32)


def _dot(a, b):
    return jnp.dot(a, b, preferred_element_type=F32)


def _dot_nt(a, b):
    return lax.dot_general(a, b, (((1,), (1,)), ((), ())), preferred_element_type=F32)


def _kernel(cfg,
            aq_hbm, ak_hbm, av_hbm, sk_hbm, ssmk_hbm, ssmd_hbm, x_hbm, mem0_hbm,
            wq_hbm, wk_hbm, wv_hbm, wo_hbm, fwd_hbm, inv_hbm, fill_hbm,
            out_hbm,
            w_u, wo_u, wstage, wostage, xbuf, xlead, xlead_u, qkvb, ob, obuf, obb,
            abuf, hbuf, kf, kvb, ubuf, gbuf, hlast, aout, ystage,
            fwd_ref, inv_ref, fill_ref, taps, mem0_ref, sk_ref, ssmd_ref,
            sems):
    import contextlib
    scope = jax.named_scope if cfg.get("scopes") else (lambda name: contextlib.nullcontext())
    SW, SWO, SXL, SX, SH, SA, SO, SS = 0, 16, 24, 28, 29, 30, 38, 42
    w_hbms = (wq_hbm, wk_hbm, wv_hbm)
    a_hbms = (aq_hbm, ak_hbm, av_hbm)

    def w_copy(c, k):
        m, g = c // 2, c % 2
        slot = (c % 2) * 8 + k
        return pltpu.make_async_copy(
            w_hbms[m].at[pl.ds(k * 128, 128), pl.ds(16 * g, 16), :],
            wstage.at[slot], sems.at[SW + slot])

    def self_wait(ref, sem):
        pltpu.make_async_copy(ref, ref, sems.at[sem]).wait()

    def wo_copy(k):
        return pltpu.make_async_copy(
            wo_hbm.at[pl.ds(k * 512, 512), :], wostage.at[k], sems.at[SWO + k])

    def xlead_copy(q):
        return pltpu.make_async_copy(
            x_hbm.at[:, pl.ds(0, M), pl.ds(q * KQ, KQ)], xlead.at[q], sems.at[SXL + q])

    x_cp = pltpu.make_async_copy(
        x_hbm.at[:, pl.ds(M, SEG - M), :], xbuf.at[:, pl.ds(M, SEG - M), :], sems.at[SX])

    def h_copy(c):
        return pltpu.make_async_copy(
            ssmk_hbm.at[:, pl.ds(c * C, C)], hbuf.at[c], sems.at[SH])

    def a_copy(t, g):
        return pltpu.make_async_copy(
            a_hbms[t].at[:, pl.ds(g * 128, 128)], abuf.at[g, t], sems.at[SA + g])

    small = [pltpu.make_async_copy(src, dst, sems.at[SS + i]) for i, (src, dst) in enumerate((
        (fwd_hbm, fwd_ref), (inv_hbm, inv_ref), (fill_hbm, fill_ref),
        (mem0_hbm, mem0_ref), (sk_hbm, sk_ref), (ssmd_hbm, ssmd_ref)))]

    for q in range(4):
        xlead_copy(q).start()
        w_copy(0, 2 * q).start()
        w_copy(0, 2 * q + 1).start()
    for k in range(8):
        w_copy(1, k).start()

    kf[pl.ds(0, KPAD), :] = jnp.zeros((KPAD, 128), F32)
    for b in range(2):
        gbuf[b, pl.ds(0, 7)] = jnp.zeros((7, 2 * C, 128), F32)

    def relayout_piece(c, k):
        slot = (c % 2) * 8 + k
        base = ((c // 2) * H + 8 * (c % 2)) * SLAB + k * 64
        for i in range(64):
            a = pltpu.bitcast(wstage[slot, 2 * i], U32)
            b = pltpu.bitcast(wstage[slot, 2 * i + 1], U32)
            ev = (a & jnp.uint32(0xFFFF)) | (b << 16)
            od = (a >> 16) | (b & jnp.uint32(0xFFFF0000))
            w_u[pl.ds(base + i, 8, stride=SLAB), :] = ev
            w_u[pl.ds(base + NPAIR * SLAB + i, 8, stride=SLAB), :] = od

    def store_pair(it, outs):
        both = jnp.concatenate([o.reshape(NSEG, M, DH) for o in outs], axis=1)
        qkvb[it] = pltpu.bitcast(both.astype(BF16), U32)

    def batch_pair(it):
        m = it // NPAIR
        j = it % NPAIR
        xl = jnp.concatenate([pltpu.bitcast(xlead_u[q], BF16) for q in range(4)], axis=1)
        outs = []
        for par in range(2):
            row = pl.multiple_of((m * H + par * NPAIR + j) * SLAB, 8)
            w = pltpu.bitcast(w_u[pl.ds(row, D // 2), :], BF16)
            outs.append(_dot(xl, w))
        store_pair(it, outs)

    def quarter_prep(q):
        self_wait(xlead.at[q], SXL + q)
        for u in range(2):
            self_wait(wstage.at[2 * q + u], SW + 2 * q + u)
        xq = xlead[q].astype(F32).reshape(NSEG * M, KQ).astype(BF16)
        xlead_u[q] = pltpu.bitcast(xq, U32)
        for u in range(2):
            relayout_piece(0, 2 * q + u)

    def quarter_dot(q, par, j):
        row = pl.multiple_of((par * NPAIR + j) * SLAB + q * (KQ // 2), 8)
        w = pltpu.bitcast(w_u[pl.ds(row, KQ // 2), :], BF16)
        return _dot(pltpu.bitcast(xlead_u[q], BF16), w)

    def facc_get(hh):
        return jnp.concatenate([ubuf[0, hh], ubuf[1, hh]], axis=0)

    def quarter(q, carry):
        quarter_prep(q)
        for u in range(2):
            w_copy(2, 2 * q + u).start()
        for j in range(8):
            for par in range(2):
                hh = 2 * j + par
                d = quarter_dot(q, par, j) + jnp.where(q == 0, 0.0, facc_get(hh))
                ubuf[0, hh] = d[0:2 * C]
                ubuf[1, hh] = d[2 * C:]
        return carry
    with scope("quarters"):
        lax.fori_loop(0, 3, quarter, 0)
        quarter_prep(3)
        for u in range(2):
            w_copy(2, 6 + u).start()

    def quarter_last(it, carry):
        for u in range(4):
            self_wait(wstage.at[8 + 4 * it + u], SW + 8 + 4 * it + u)
        for u in range(4):
            j = 4 * it + u
            store_pair(j, [quarter_dot(3, par, j) + facc_get(2 * j + par) for par in range(2)])
            relayout_piece(1, j)
        return carry
    with scope("quarter_last"):
        lax.fori_loop(0, 2, quarter_last, 0)

    PP = cfg["pp"]
    IPC = 8 // PP

    def issue(c):
        if c + 2 < 6:
            for k in range(8):
                w_copy(c + 2, k).start()
        if c < 3:
            for k in range(4 * (c - 1), 4 * c):
                wo_copy(k).start()
        if c == 1:
            for cp in small:
                cp.start()
        if c == 3:
            x_cp.start()
        if c == 4:
            for cc in range(NC):
                h_copy(cc).start()
            for g in range(NG):
                for t in (1, 2, 0):
                    a_copy(t, g).start()

    def pro_body(it, carry):
        for c in range(1, 5):
            @pl.when(it == c * IPC)
            def _():
                issue(c)
        cn = it // IPC + 1
        for u in range(PP):
            slot = (cn % 2) * 8 + (it % IPC) * PP + u
            self_wait(wstage.at[slot], SW + slot)
        for u in range(PP):
            batch_pair(it * PP + u)
            relayout_piece(cn, (it % IPC) * PP + u)
        return carry
    with scope("pro_body"):
        lax.fori_loop(IPC, 5 * IPC, pro_body, 0)

    for cp in small:
        cp.wait()
    for g in range(NG):
        sk = sk_ref[g].astype(F32)
        for j in range(KS):
            taps[g, j] = jnp.broadcast_to(sk[j:j + 1], (8, 128))
        taps[g, KS] = jnp.broadcast_to(ssmd_ref[...].astype(F32)[g:g + 1], (8, 128))

    def pro_last(it, carry):
        for u in range(PP):
            k = it * PP + u
            self_wait(wostage.at[k], SWO + k)
        for u in range(PP):
            k = it * PP + u
            batch_pair(40 + k)
            for r in range(8):
                blk = wostage[k, pl.ds(r * 64, 64), :]
                row = pl.multiple_of(k * 256 + r * 32, 32)
                for n in range(NB):
                    wo_u[n, pl.ds(row, 32), :] = pltpu.bitcast(blk[:, n * 128:(n + 1) * 128], U32)
        return carry
    with scope("pro_last"):
        lax.fori_loop(0, IPC, pro_last, 0)
    with scope("xh_wait"):
        x_cp.wait()
        self_wait(hbuf, SH)

    def rep(x, rows):
        return x if rows == 8 else jnp.concatenate([x] * (rows // 8), axis=0)

    def a_stage1_pre(g, p):
        r = pl.multiple_of(p * 2 * C, 2 * C)
        never = p > 100
        kf[pl.ds(KPAD + r, 2 * C), :] = abuf[g, 1, pl.ds(r, 2 * C), :].astype(F32)
        RB = cfg["rb1"]
        sk = [rep(taps[g, j], RB) for j in range(KS)]
        parts = []
        for b in range(0, 2 * C, RB):
            ks = kf[pl.ds(KPAD + r + b, RB), :] * sk[0]
            if parts and cfg["chain1"]:
                ks = jnp.where(never, parts[-1], ks)
            for j in range(1, KS):
                ks = ks + kf[pl.ds(KPAD + r + b - j, RB), :] * sk[j]
            v16 = abuf[g, 2, pl.ds(pl.multiple_of(r + (b // 16) * 16, 16), max(RB, 16)), :].astype(F32)
            v = v16 if RB >= 16 else v16[b % 16:b % 16 + RB]
            parts.append(ks * v)
        kv = jnp.concatenate(parts, axis=0).astype(BF16)
        kvb[g % 2, pl.ds(pl.multiple_of(p * C, C), C), :] = pltpu.bitcast(kv, U32)
        return kv

    def a_stage1_u(g, p, kv):
        fwd = pltpu.bitcast(fwd_ref[...], BF16)
        for u in range(2):
            ubuf[g % 2, 2 * p + u] = _dot(fwd, kv[u * C:(u + 1) * C])

    def a_stage1_h(g, p):
        fwd = pltpu.bitcast(fwd_ref[...], BF16)
        rows = pl.ds(pl.multiple_of(g * 128, 128), 128)
        hs = [_dot_nt(fwd, hbuf[2 * p + u, rows, :]) for u in range(2)]
        prev = jnp.where(p == 0, 0.0, hlast[...])
        hlast[...] = hs[1]
        hc = C // 2
        for u, (cur, prv) in enumerate(((hs[0], prev), (hs[1], hs[0]))):
            gbuf[g % 2, 7 + 2 * p + u] = jnp.concatenate([
                cur[0:hc] - prv[C:C + hc], cur[hc:C] + prv[C + hc:],
                cur[C:C + hc] + prv[0:hc], cur[C + hc:] - prv[hc:C]], axis=0)

    def a_stage2(gp, p, slot, chain):
        b = gp % 2
        RB = cfg["rb"]
        never = p > 100
        re = [[], []]
        im = [[], []]
        last = None
        for r in range(0, C, RB):
            gr = [gbuf[b, 7 + p + 8 - j, pl.ds(r, RB), :] for j in range(NC)]
            gi = [gbuf[b, 7 + p + 8 - j, pl.ds(C + r, RB), :] for j in range(NC)]
            ur = [ubuf[b, j, pl.ds(r, RB), :] for j in range(NC)]
            ui = [ubuf[b, j, pl.ds(C + r, RB), :] for j in range(NC)]
            for o, (nt, off) in enumerate(((8, 8), (16, 0))):
                if chain == 1:
                    ar = gr[off] * ur[0]
                    ai = gr[off] * ui[0]
                    if last is not None:
                        ar = jnp.where(never, last[0], ar)
                        ai = jnp.where(never, last[1], ai)
                    ar = ar - gi[off] * ui[0]
                    ai = ai + gi[off] * ur[0]
                    for j in range(1, nt):
                        ar = ar + gr[j + off] * ur[j]
                        ai = ai + gr[j + off] * ui[j]
                        ar = ar - gi[j + off] * ui[j]
                        ai = ai + gi[j + off] * ur[j]
                    last = (ar, ai)
                else:
                    ar = gr[off] * ur[0]
                    if last is not None:
                        ar = jnp.where(never, last, ar)
                    ar = ar - gi[off] * ui[0]
                    for j in range(1, nt):
                        ar = ar + gr[j + off] * ur[j]
                        ar = ar - gi[j + off] * ui[j]
                    ai = jnp.where(never, ar, gr[off] * ui[0])
                    ai = ai + gi[off] * ur[0]
                    for j in range(1, nt):
                        ai = ai + gr[j + off] * ui[j]
                        ai = ai + gi[j + off] * ur[j]
                    last = ai
                re[o].append(ar)
                im[o].append(ai)
                if (r + RB) % 16 == 0:
                    k = 16 // RB
                    r0 = (r + RB - 16) // 2
                    ystage[slot, o, pl.ds(r0, 8), :] = pltpu.bitcast(
                        jnp.concatenate(re[o][-k:], axis=0).astype(BF16), U32)
                    ystage[slot, o, pl.ds(C // 2 + r0, 8), :] = pltpu.bitcast(
                        jnp.concatenate(im[o][-k:], axis=0).astype(BF16), U32)

    def a_stage3(gp, gq, p, slot):
        inv = pltpu.bitcast(inv_ref[...], BF16)
        dd = rep(taps[gq, KS], C)
        for o in range(2):
            i = p + 8 * o
            y = _dot(inv, pltpu.bitcast(ystage[slot, o], BF16))
            kv = pltpu.bitcast(
                kvb[gp % 2, pl.ds(pl.multiple_of(i * (C // 2), C // 2), C // 2), :], BF16)
            y = y + kv.astype(F32) * dd
            q = abuf[gq, 0, pl.ds(pl.multiple_of(i * C, C), C), :]
            res = (q.astype(F32) * y).astype(BF16)
            aout[gq, pl.ds(pl.multiple_of(i * 4, 4), 4)] = res.reshape(4, SEG, 128)

    scale = DH ** (-0.5)

    def w_slab(m, h):
        slab = m * H + (h % 2) * NPAIR + h // 2
        return pltpu.bitcast(w_u[pl.ds(slab * SLAB, D // 2), :], BF16)

    class Step:
        def __init__(self, s, u):
            self.s = s
            self.slot = u % 2
            self.g = s // 8
            self.p = s % 8
            self.qkv, self.ps, self.os = {}, {}, []
            self.acc = [None] * NB

        def start(self, mem):
            s = self.s
            x1 = xbuf[s, pl.ds(M, M), :].astype(F32)
            top = jnp.concatenate([mem, x1], axis=0).astype(BF16)
            self.lhs = jnp.concatenate([top, xbuf[s, pl.ds(16, 16), :]], axis=0)

        def proj(self, m, j):
            a = _dot(self.lhs, w_slab(m, 2 * j)).astype(BF16)
            b = _dot(self.lhs, w_slab(m, 2 * j + 1)).astype(BF16)
            lead = pltpu.bitcast(qkvb[m * NPAIR + j, self.s], BF16)
            self.qkv[m, j] = jnp.concatenate([a, b, lead], axis=0)

        def probs(self, j):
            fill = fill_ref[pl.ds(0, R), pl.ds(0, R)]
            sc = jnp.where(fill == 0.0, _dot_nt(self.qkv[0, j], self.qkv[1, j]) * scale, fill)
            mx = jnp.max(sc, axis=-1, keepdims=True)
            e = jnp.exp(sc - mx)
            l = jnp.sum(e, axis=-1, keepdims=True)
            r = pl.reciprocal(l, approx=True)
            r = r * (2.0 - l * r)
            self.ps[j] = (e * r).astype(BF16)

        def attend(self, j):
            o = _dot(self.ps[j], self.qkv[2, j])
            row = pl.multiple_of(self.s * M, M)
            ob[2 * j, pl.ds(row, M), :] = o[2 * SEG:2 * SEG + M].astype(BF16)
            ob[2 * j + 1, pl.ds(row, M), :] = o[2 * SEG + M:].astype(BF16)
            self.os += [o[0:SEG].astype(BF16), o[SEG:2 * SEG].astype(BF16)]

        def wo(self, h0, h1, ns):
            o = jnp.concatenate(self.os[h0:h1], axis=1)
            for n in ns:
                w = pltpu.bitcast(wo_u[n, pl.ds(h0 * 64, (h1 - h0) * 64), :], BF16)
                d = _dot(o, w)
                self.acc[n] = d if self.acc[n] is None else d + self.acc[n]

        def finish(self):
            res = jnp.concatenate(self.acc, axis=1)
            obuf[self.s] = res.astype(BF16)
            return res[0:M]

        def run(self, item):
            kind = item[0]
            g, p = self.g, self.p
            if kind == "P":
                self.proj(item[1], item[2])
            elif kind == "S":
                self.probs(item[1])
            elif kind == "V":
                self.attend(item[1])
            elif kind == "W":
                self.wo(item[1], item[2], item[3])
            elif kind == "A1":
                self.kv = a_stage1_pre(g, p)
            elif kind == "AU":
                a_stage1_u(g, p, self.kv)
            elif kind == "AH":
                a_stage1_h(g, p)
            elif kind == "A2":
                a_stage2(g + 1, p, self.slot, cfg["chain"])
            elif kind == "A3":
                a_stage3(g + 1, jnp.maximum(g - 1, 0), p, self.slot)

    U, order = _make_order(cfg["order"])

    def steps(i, mem):
        s0 = i * U

        @pl.when(s0 % 8 == 0)
        def _():
            self_wait(abuf.at[s0 // 8], SA + s0 // 8)
        st = [Step(s0 + u, u) for u in range(U)]
        for u, item in order:
            if item[0] == "start":
                st[u].start(mem)
            elif item[0] == "finish":
                mem = st[u].finish()
            else:
                st[u].run(item)
        return mem

    with scope("steps"):
        lax.fori_loop(0, NSEG // U, steps, mem0_ref[...].astype(F32))

    ob_cp = pltpu.make_async_copy(
        obuf.at[:, pl.ds(M, SEG - M), :],
        out_hbm.at[:, pl.ds(M, SEG - M), pl.ds(D, D)], sems.at[SO])
    ob_cp.start()
    for g in range(NG - 1):
        pltpu.make_async_copy(
            aout.at[g], out_hbm.at[:, :, pl.ds(g * 128, 128)], sems.at[SO + 1]).start()

    EP = cfg["ep"]
    GL = NG - 1
    HS = cfg["ep_split"]

    def epi(it, carry):
        def part(n, h0, h1):
            lhs = jnp.concatenate([ob[h] for h in range(h0, h1)], axis=1)
            return _dot(lhs, pltpu.bitcast(wo_u[n, pl.ds(h0 * 64, (h1 - h0) * 64), :], BF16))
        for u in range(EP):
            n = it * EP + u
            a_stage2(GL, n, u % 2, cfg["ep_chain"])
            d = part(n, 0, HS)
            a_stage3(GL, GL, n, u % 2)
            d = part(n, HS, H) + d
            obb[n] = d.reshape(NSEG, M, 128).astype(BF16)
        for u in range(EP):
            n = it * EP + u
            col = pl.multiple_of(D + n * 128, 128)
            pltpu.make_async_copy(
                obb.at[n], out_hbm.at[:, pl.ds(0, M), pl.ds(col, 128)], sems.at[SO + 2]).start()
        for o in range(2):
            rows = pl.ds((it * EP + 8 * o) * 4, 4 * EP)
            pltpu.make_async_copy(
                aout.at[GL, rows], out_hbm.at[rows, :, pl.ds(GL * 128, 128)], sems.at[SO + 1]).start()
        return carry
    with scope("epi"):
        lax.fori_loop(0, NB // EP, epi, 0)
    ob_cp.wait()
    self_wait(aout, SO + 1)
    self_wait(obb, SO + 2)


def _b_order(u, extra):
    alln = tuple(range(NB))
    out = list(extra.get("pre", [])) + [(u, ("start",))]
    for t in range(NPAIR):
        out.append((u, ("P", 0, t)))
        if t >= 1:
            out += [(u, ("P", 2, t - 1)), (u, ("S", t - 1))]
        out.append((u, ("P", 1, t)))
        if t >= 2:
            out.append((u, ("V", t - 2)))
        out += extra.get(t, [])
    out += [(u, x) for x in (("P", 2, 15), ("W", 0, 24, (0,)), ("S", 15), ("W", 0, 24, (1,)), ("V", 14),
                             ("W", 0, 24, (2, 3)))]
    out += extra.get("tail", [])
    out += [(u, x) for x in (("V", 15), ("W", 0, 24, (4, 5, 6, 7)), ("W", 24, 32, alln), ("finish",))]
    return out


def _make_order(kind):
    def A(u, *names):
        return [(u, (n,)) for n in names]
    if kind == 3:
        return 1, _b_order(0, {"pre": A(0, "A1", "AH"), 1: A(0, "AU", "A2"), "tail": A(0, "A3")})
    if kind == 7:
        return 1, _b_order(0, {"pre": A(0, "A2", "A1"), "tail": A(0, "A3", "AH", "AU")})
    if kind == 8:
        return 1, _b_order(0, {"pre": A(0, "A2", "A1"), 10: A(0, "A3", "AH", "AU")})
    if kind == 9:
        return 1, _b_order(0, {"pre": A(0, "A2", "A1"), 10: A(0, "A3", "AU", "AH")})
    if kind in (20, 21, 40):
        U = kind // 10
        out = []
        for u in range(U):
            ex = {"pre": []}
            if u > 0:
                ex["pre"] += A(u - 1, "A3", "AH", "AU") if kind != 21 else A(u - 1, "A3", "AU", "AH")
            ex["pre"] += A(u, "A2", "A1")
            if u == U - 1:
                ex["tail"] = A(u, "A3", "AH", "AU")
            out += _b_order(u, ex)
        return U, out
    raise ValueError(kind)


_DEFAULT_CFG = dict(order=3, pp=4, ep=2, ep_split=24, ep_chain=1, rb=8, chain=1, rb1=16, chain1=1)


def _pack_rows(x):
    b = np.asarray(x, dtype=jnp.bfloat16).view(np.uint16).astype(np.uint32)
    return b[0::2] | (b[1::2] << 16)


def _build(cfg):
    fwd_np, inv_np = _dft_constants()
    fill_np = np.zeros((96, 128), np.float32)
    fill_np[:R, :R] = _mask_fill()

    def run(A_q, A_k, A_v, A_shift_k, A_ssm_k, A_ssm_D, B_x, B_mem0, B_Wq, B_Wk, B_Wv, B_Wo):
        sk = A_shift_k.T.reshape(KS, NG, 128).transpose(1, 0, 2)
        any_spec = pl.BlockSpec(memory_space=pl.ANY)
        out = pl.pallas_call(
            functools.partial(_kernel, cfg),
            out_shape=jax.ShapeDtypeStruct((NSEG, SEG, 2 * D), BF16),
            in_specs=[any_spec] * 15,
            out_specs=any_spec,
            scratch_shapes=[
                pltpu.VMEM((3 * H * SLAB, 128), U32),
                pltpu.VMEM((NB, H * DH // 2, 128), U32),
                pltpu.VMEM((16, 128, 16, DH), BF16),
                pltpu.VMEM((8, 512, D), BF16),
                pltpu.VMEM((NSEG, SEG, D), BF16),
                pltpu.VMEM((4, NSEG, M, KQ), BF16),
                pltpu.VMEM((4, NSEG * M // 2, KQ), U32),
                pltpu.VMEM((3 * NPAIR, NSEG, 8, 128), U32),
                pltpu.VMEM((H, NSEG * M, DH), BF16),
                pltpu.VMEM((NSEG, SEG, D), BF16),
                pltpu.VMEM((NB, NSEG, M, 128), BF16),
                pltpu.VMEM((NG, 3, S, 128), BF16),
                pltpu.VMEM((NC, D, C), BF16),
                pltpu.VMEM((S + KPAD, 128), F32),
                pltpu.VMEM((2, S // 2, 128), U32),
                pltpu.VMEM((2, NC, 2 * C, 128), F32),
                pltpu.VMEM((2, NC + 7, 2 * C, 128), F32),
                pltpu.VMEM((2 * C, 128), F32),
                pltpu.VMEM((NG, NSEG, SEG, 128), BF16),
                pltpu.VMEM((2, 2, C, 128), U32),
                pltpu.VMEM((C, C), U32),
                pltpu.VMEM((C // 2, 2 * C), U32),
                pltpu.VMEM((96, 128), F32),
                pltpu.VMEM((NG, 8, 8, 128), F32),
                pltpu.VMEM((M, D), BF16),
                pltpu.VMEM((NG, KS, 128), BF16),
                pltpu.VMEM((NG, 128), BF16),
                pltpu.SemaphoreType.DMA((48,)),
            ],
            compiler_params=pltpu.CompilerParams(vmem_limit_bytes=124 * 1024 * 1024),
        )(A_q.reshape(S, D), A_k.reshape(S, D), A_v.reshape(S, D), sk, A_ssm_k,
          A_ssm_D.reshape(NG, 128), B_x.reshape(NSEG, SEG, D), B_mem0.reshape(M, D),
          B_Wq, B_Wk, B_Wv, B_Wo.reshape(H * DH, D),
          jnp.asarray(_pack_rows(fwd_np)), jnp.asarray(_pack_rows(inv_np)), jnp.asarray(fill_np))
        return out.reshape(1, S, 2 * D)

    return run


@functools.partial(jax.jit, static_argnames=("B_seg_len",))
def pallas_concat_heads__ssm_conv_h3__memory_aug_recurrent_mem_tr__prompt_kernel(
    A_q: jax.Array,
    A_k: jax.Array,
    A_v: jax.Array,
    A_shift_k: jax.Array,
    A_ssm_k: jax.Array,
    A_ssm_D: jax.Array,
    B_x: jax.Array,
    B_mem0: jax.Array,
    B_Wq: jax.Array,
    B_Wk: jax.Array,
    B_Wv: jax.Array,
    B_Wo: jax.Array,
    B_seg_len: int = SEG,
):
    assert B_seg_len == SEG
    return _build(_DEFAULT_CFG)(A_q, A_k, A_v, A_shift_k, A_ssm_k, A_ssm_D, B_x, B_mem0,
                                B_Wq, B_Wk, B_Wv, B_Wo)
```

```python
import functools

import numpy as np
import jax
import jax.numpy as jnp
from jax import lax
import jax.experimental.pallas as pl
import jax.experimental.pallas.tpu as pltpu

F32 = jnp.float32
BF16 = jnp.bfloat16
U32 = jnp.uint32

S = 2048
D = 1024
H = 32
DH = 128
M = 8
SEG = 32
NSEG = S // SEG
NPAIR = H // 2
R = 2 * (M + SEG)
SLAB = 520
KS = 4
C = 128
NC = S // C
NG = D // 128
KQ = D // 4
KPAD = 32
NB = D // 128


def _dft_constants():
    fe = np.arange(0, C, 2)
    f = np.concatenate([fe, C - 1 - fe])
    t = np.arange(C)
    ang = (np.pi * (2 * f + 1) / (2 * C))[:, None] * t[None, :]
    fwd = np.concatenate([np.cos(ang), -np.sin(ang)], axis=0)
    a = ang[:C // 2]
    inv = np.stack([np.cos(a), -np.sin(a)], axis=1).reshape(C, C).T / C
    inv = np.concatenate([inv[0::2], inv[1::2]], axis=0)
    return fwd.astype(np.float32), inv.astype(np.float32)


def _mask_fill():
    blk = np.concatenate([np.arange(M), M + np.arange(M, SEG)])
    lead = M + np.arange(M)
    qhead = np.concatenate([np.zeros(SEG), np.ones(SEG), np.zeros(M), np.ones(M)])
    qpos = np.concatenate([blk, blk, lead, lead])
    khead = np.arange(R) % 2
    kpos = np.concatenate([blk, lead])[np.arange(R) // 2]
    same = qhead[:, None] == khead[None, :]
    ok = (qpos[:, None] < M) | (qpos[:, None] >= kpos[None, :])
    fill = np.where(same, np.where(ok, 0.0, -1e9), -np.inf)
    return fill.astype(np.float32)


def _pack(lo, hi):
    return pltpu.pack_elementwise([lo, hi], packed_dtype=BF16)


def _unpack(w, index):
    return pltpu.unpack_elementwise(w, index=index, packed_dtype=BF16, unpacked_dtype=F32)


def _dot(a, b):
    return jnp.dot(a, b, preferred_element_type=F32)


def _dot_nt(a, b):
    return lax.dot_general(a, b, (((1,), (1,)), ((), ())), preferred_element_type=F32)


def _kernel(cfg,
            aq_hbm, ak_hbm, av_hbm, sk_hbm, ssmk_hbm, ssmd_hbm, x_hbm, mem0_hbm,
            wq_hbm, wk_hbm, wv_hbm, wo_hbm, fwd_hbm, inv_hbm, fill_hbm,
            out_hbm,
            w_u, wo_u, wstage, wostage, xbuf, xlead, xlead_u, qkvb, ob, obuf, obb,
            abuf, hbuf, kf, kvb, ubuf, gbuf, hlast, aout, ystage,
            fwd_ref, inv_ref, fill_ref, taps, mem0_ref, sk_ref, ssmd_ref,
            sems):
    import contextlib
    scope = jax.named_scope if cfg.get("scopes") else (lambda name: contextlib.nullcontext())
    SW, SWO, SXL, SX, SH, SA, SO, SS = 0, 16, 24, 28, 29, 30, 38, 42
    w_hbms = (wq_hbm, wk_hbm, wv_hbm)
    a_hbms = (aq_hbm, ak_hbm, av_hbm)

    def w_copy(c, k):
        m, g = c // 2, c % 2
        slot = (c % 2) * 8 + k
        return pltpu.make_async_copy(
            w_hbms[m].at[pl.ds(k * 128, 128), pl.ds(16 * g, 16), :],
            wstage.at[slot], sems.at[SW + slot])

    def self_wait(ref, sem):
        pltpu.make_async_copy(ref, ref, sems.at[sem]).wait()

    def wo_copy(k):
        return pltpu.make_async_copy(
            wo_hbm.at[pl.ds(k * 512, 512), :], wostage.at[k], sems.at[SWO + k])

    def xlead_copy(q):
        return pltpu.make_async_copy(
            x_hbm.at[:, pl.ds(0, M), pl.ds(q * KQ, KQ)], xlead.at[q], sems.at[SXL + q])

    x_cp = pltpu.make_async_copy(
        x_hbm.at[:, pl.ds(M, SEG - M), :], xbuf.at[:, pl.ds(M, SEG - M), :], sems.at[SX])

    def h_copy(c):
        return pltpu.make_async_copy(
            ssmk_hbm.at[:, pl.ds(c * C, C)], hbuf.at[c], sems.at[SH])

    def a_copy(t, g):
        return pltpu.make_async_copy(
            a_hbms[t].at[:, pl.ds(g * 128, 128)], abuf.at[g, t], sems.at[SA + g])

    small = [pltpu.make_async_copy(src, dst, sems.at[SS + i]) for i, (src, dst) in enumerate((
        (fwd_hbm, fwd_ref), (inv_hbm, inv_ref), (fill_hbm, fill_ref),
        (mem0_hbm, mem0_ref), (sk_hbm, sk_ref), (ssmd_hbm, ssmd_ref)))]

    for q in range(4):
        xlead_copy(q).start()
        w_copy(0, 2 * q).start()
        w_copy(0, 2 * q + 1).start()
    for k in range(8):
        w_copy(1, k).start()

    kf[pl.ds(0, KPAD), :] = jnp.zeros((KPAD, 128), U32)
    for b in range(2):
        gbuf[b, pl.ds(0, 7)] = jnp.zeros((7, 2 * C, 128), F32)

    def relayout_piece(c, k):
        slot = (c % 2) * 8 + k
        base = ((c // 2) * H + 8 * (c % 2)) * SLAB + k * 64
        for i in range(64):
            a = pltpu.bitcast(wstage[slot, 2 * i], U32)
            b = pltpu.bitcast(wstage[slot, 2 * i + 1], U32)
            ev = (a & jnp.uint32(0xFFFF)) | (b << 16)
            od = (a >> 16) | (b & jnp.uint32(0xFFFF0000))
            w_u[pl.ds(base + i, 8, stride=SLAB), :] = ev
            w_u[pl.ds(base + NPAIR * SLAB + i, 8, stride=SLAB), :] = od

    def store_pair(it, outs):
        qkvb[it] = _pack(outs[0], outs[1]).reshape(NSEG, M, DH)

    def batch_pair(it):
        m = it // NPAIR
        j = it % NPAIR
        xl = jnp.concatenate([pltpu.bitcast(xlead_u[q], BF16) for q in range(4)], axis=1)
        outs = []
        for par in range(2):
            row = pl.multiple_of((m * H + par * NPAIR + j) * SLAB, 8)
            w = pltpu.bitcast(w_u[pl.ds(row, D // 2), :], BF16)
            outs.append(_dot(xl, w))
        store_pair(it, outs)

    def quarter_prep(q):
        self_wait(xlead.at[q], SXL + q)
        for u in range(2):
            self_wait(wstage.at[2 * q + u], SW + 2 * q + u)
        xq = xlead[q].astype(F32).reshape(NSEG * M, KQ).astype(BF16)
        xlead_u[q] = pltpu.bitcast(xq, U32)
        for u in range(2):
            relayout_piece(0, 2 * q + u)

    def quarter_dot(q, par, j):
        row = pl.multiple_of((par * NPAIR + j) * SLAB + q * (KQ // 2), 8)
        w = pltpu.bitcast(w_u[pl.ds(row, KQ // 2), :], BF16)
        return _dot(pltpu.bitcast(xlead_u[q], BF16), w)

    def facc_get(hh):
        return jnp.concatenate([ubuf[0, hh], ubuf[1, hh]], axis=0)

    def quarter(q, carry):
        quarter_prep(q)
        for u in range(2):
            w_copy(2, 2 * q + u).start()
        for j in range(8):
            for par in range(2):
                hh = 2 * j + par
                d = quarter_dot(q, par, j) + jnp.where(q == 0, 0.0, facc_get(hh))
                ubuf[0, hh] = d[0:2 * C]
                ubuf[1, hh] = d[2 * C:]
        return carry
    with scope("quarters"):
        lax.fori_loop(0, 3, quarter, 0)
        quarter_prep(3)
        for u in range(2):
            w_copy(2, 6 + u).start()

    def quarter_last(it, carry):
        for u in range(4):
            self_wait(wstage.at[8 + 4 * it + u], SW + 8 + 4 * it + u)
        for u in range(4):
            j = 4 * it + u
            store_pair(j, [quarter_dot(3, par, j) + facc_get(2 * j + par) for par in range(2)])
            relayout_piece(1, j)
        return carry
    with scope("quarter_last"):
        lax.fori_loop(0, 2, quarter_last, 0)

    PP = cfg["pp"]
    IPC = 8 // PP

    def issue(c):
        if c + 2 < 6:
            for k in range(8):
                w_copy(c + 2, k).start()
        if c < 3:
            for k in range(4 * (c - 1), 4 * c):
                wo_copy(k).start()
        if c == 1:
            for cp in small:
                cp.start()
        if c == 3:
            x_cp.start()
        if c == 4:
            for cc in range(NC):
                h_copy(cc).start()
            for g in range(NG):
                for t in (1, 2, 0):
                    a_copy(t, g).start()

    def pro_body(it, carry):
        for c in range(1, 5):
            @pl.when(it == c * IPC)
            def _():
                issue(c)
        cn = it // IPC + 1
        for u in range(PP):
            slot = (cn % 2) * 8 + (it % IPC) * PP + u
            self_wait(wstage.at[slot], SW + slot)
        for u in range(PP):
            batch_pair(it * PP + u)
            relayout_piece(cn, (it % IPC) * PP + u)
        return carry
    with scope("pro_body"):
        lax.fori_loop(IPC, 5 * IPC, pro_body, 0)

    for cp in small:
        cp.wait()
    for g in range(NG):
        sk = sk_ref[g].astype(F32)
        for j in range(KS):
            taps[g, j] = jnp.broadcast_to(sk[j:j + 1], (8, 128))
        taps[g, KS] = jnp.broadcast_to(ssmd_ref[...].astype(F32)[g:g + 1], (8, 128))

    def pro_last(it, carry):
        for u in range(PP):
            k = it * PP + u
            self_wait(wostage.at[k], SWO + k)
        for u in range(PP):
            k = it * PP + u
            batch_pair(40 + k)
            for r in range(8):
                blk = wostage[k, pl.ds(r * 64, 64), :]
                row = pl.multiple_of(k * 256 + r * 32, 32)
                for n in range(NB):
                    wo_u[n, pl.ds(row, 32), :] = pltpu.bitcast(blk[:, n * 128:(n + 1) * 128], U32)
        return carry
    with scope("pro_last"):
        lax.fori_loop(0, IPC, pro_last, 0)
    with scope("xh_wait"):
        x_cp.wait()
        self_wait(hbuf, SH)

    def rep(x, rows):
        return x if rows == 8 else jnp.concatenate([x] * (rows // 8), axis=0)

    def a_stage1_pre(g, p, never, par=None):
        par = g % 2 if par is None else par
        r = p * C if isinstance(p, int) else pl.multiple_of(p * C, C)
        r2 = 2 * r if isinstance(p, int) else pl.multiple_of(2 * r, 2 * C)
        kw = pltpu.bitcast(abuf[g, 1, pl.ds(r2, 2 * C), :], U32)
        vw = pltpu.bitcast(abuf[g, 2, pl.ds(r2, 2 * C), :], U32)
        kf[pl.ds(KPAD + r, C), :] = kw
        t = [taps[g, j] for j in range(KS)]
        parts = []
        last = None
        for b in range(0, C, 8):
            w1 = kf[pl.ds(KPAD + r + b - 1, 8), :]
            w2 = kf[pl.ds(KPAD + r + b - 2, 8), :]
            e0, o0 = _unpack(kw[b:b + 8], 0), _unpack(kw[b:b + 8], 1)
            e1, o1 = _unpack(w1, 0), _unpack(w1, 1)
            o2 = _unpack(w2, 1)
            ke = e0 * t[0]
            ko = o0 * t[0]
            if last is not None and cfg["chain1"] and never is not None:
                ke = jnp.where(never, last[0], ke)
                ko = jnp.where(never, last[1], ko)
            ke = ke + o1 * t[1] + e1 * t[2] + o2 * t[3]
            ko = ko + e0 * t[1] + o1 * t[2] + e1 * t[3]
            last = (ke * _unpack(vw[b:b + 8], 0), ko * _unpack(vw[b:b + 8], 1))
            parts.append(_pack(*last))
        kv = jnp.concatenate(parts, axis=0)
        kvb[par, pl.ds(r, C), :] = kv
        return kv

    def a_stage1_u(g, p, kv):
        fwd = pltpu.bitcast(fwd_ref[...], BF16)
        if kv is None:
            kv = kvb[g % 2, pl.ds(pl.multiple_of(p * C, C), C), :]
        for u in range(2):
            w = pltpu.bitcast(kv[u * C // 2:(u + 1) * C // 2], BF16)
            if cfg["split_u"]:
                for hf in range(2):
                    ubuf[g % 2, 2 * p + u, pl.ds(hf * C, C), :] = _dot(fwd[hf * C:(hf + 1) * C], w)
            else:
                ubuf[g % 2, 2 * p + u] = _dot(fwd, w)

    def a_stage1_h(g, p):
        fwd = pltpu.bitcast(fwd_ref[...], BF16)
        rows = pl.ds(pl.multiple_of(g * 128, 128), 128)
        if cfg["split_h"]:
            hs = [jnp.concatenate([_dot_nt(fwd[hf * C:(hf + 1) * C], hbuf[2 * p + u, rows, :])
                                   for hf in range(2)], axis=0) for u in range(2)]
        else:
            hs = [_dot_nt(fwd, hbuf[2 * p + u, rows, :]) for u in range(2)]
        prev = jnp.where(p == 0, 0.0, hlast[...])
        hlast[...] = hs[1]
        hc = C // 2
        for u, (cur, prv) in enumerate(((hs[0], prev), (hs[1], hs[0]))):
            gbuf[g % 2, 7 + 2 * p + u] = jnp.concatenate([
                cur[0:hc] - prv[C:C + hc], cur[hc:C] + prv[C + hc:],
                cur[C:C + hc] + prv[0:hc], cur[C + hc:] - prv[hc:C]], axis=0)

    def a_stage2(gp, p, slot, chain, never):
        b = gp % 2
        RB = 8
        re = [[], []]
        im = [[], []]
        last = None
        for r in [r0 + blk for r0 in range(0, C // 2, RB) for blk in (0, C // 2)]:
            gr = [gbuf[b, 7 + p + 8 - j, pl.ds(r, RB), :] for j in range(NC)]
            gi = [gbuf[b, 7 + p + 8 - j, pl.ds(C + r, RB), :] for j in range(NC)]
            ur = [ubuf[b, j, pl.ds(r, RB), :] for j in range(NC)]
            ui = [ubuf[b, j, pl.ds(C + r, RB), :] for j in range(NC)]
            for o, (nt, off) in enumerate(((8, 8), (16, 0))):
                if chain == 1:
                    ar = gr[off] * ur[0]
                    ai = gr[off] * ui[0]
                    if last is not None:
                        ar = jnp.where(never, last[0], ar)
                        ai = jnp.where(never, last[1], ai)
                    ar = ar - gi[off] * ui[0]
                    ai = ai + gi[off] * ur[0]
                    for j in range(1, nt):
                        ar = ar + gr[j + off] * ur[j]
                        ai = ai + gr[j + off] * ui[j]
                        ar = ar - gi[j + off] * ui[j]
                        ai = ai + gi[j + off] * ur[j]
                    last = (ar, ai)
                else:
                    ar = gr[off] * ur[0]
                    if last is not None:
                        ar = jnp.where(never, last, ar)
                    ar = ar - gi[off] * ui[0]
                    for j in range(1, nt):
                        ar = ar + gr[j + off] * ur[j]
                        ar = ar - gi[j + off] * ui[j]
                    ai = jnp.where(never, ar, gr[off] * ui[0])
                    ai = ai + gi[off] * ur[0]
                    for j in range(1, nt):
                        ai = ai + gr[j + off] * ui[j]
                        ai = ai + gi[j + off] * ur[j]
                    last = ai
                re[o].append(ar)
                im[o].append(ai)
                if r >= C // 2:
                    rows = pl.ds(r - C // 2, RB)
                    ystage[slot, o, 0, rows, :] = _pack(re[o][-2] + ar, im[o][-2] - ai)
                    ystage[slot, o, 1, rows, :] = _pack(re[o][-2] - ar, im[o][-2] + ai)
        return list(last) if chain == 1 else [last]

    def a_stage3(gp, gq, p, slot):
        inv = pltpu.bitcast(inv_ref[...], BF16)
        dd = rep(taps[gq, KS], C // 2)
        for o in range(2):
            i = p + 8 * o
            kvw = kvb[gp % 2, pl.ds(pl.multiple_of(i * (C // 2), C // 2), C // 2), :]
            qw = pltpu.bitcast(abuf[gq, 0, pl.ds(pl.multiple_of(i * C, C), C), :], U32)
            res = []
            for e in range(2):
                y = _dot(inv[e * (C // 2):(e + 1) * (C // 2)], pltpu.bitcast(ystage[slot, o, e], BF16))
                res.append(_unpack(qw, e) * (y + _unpack(kvw, e) * dd))
            out = pltpu.bitcast(_pack(res[0], res[1]), BF16)
            aout[gq, pl.ds(pl.multiple_of(i * 4, 4), 4)] = out.reshape(4, SEG, 128)

    scale = DH ** (-0.5)

    def w_slab(m, h):
        slab = m * H + (h % 2) * NPAIR + h // 2
        return pltpu.bitcast(w_u[pl.ds(slab * SLAB, D // 2), :], BF16)

    class Step:
        def __init__(self, s, u):
            self.s = s
            self.slot = u % 2
            self.g = s // 8
            self.p = s % 8
            self.qkv, self.ps, self.os = {}, {}, []
            self.acc = [None] * NB
            self.ocat = {}
            self.ties = []

        def start(self, mem):
            x = xbuf[self.s, pl.ds(M, SEG - M), :].astype(F32)
            self.lhs = jnp.concatenate([mem, x], axis=0).astype(BF16)

        def proj(self, m, j):
            a = _dot(self.lhs, w_slab(m, 2 * j))
            b = _dot(self.lhs, w_slab(m, 2 * j + 1))
            lead = qkvb[m * NPAIR + j, self.s]
            if m == 0:
                r = jnp.concatenate([a, b, _unpack(lead, 0), _unpack(lead, 1)], axis=0).astype(BF16)
            else:
                r = pltpu.bitcast(jnp.concatenate([_pack(a, b), lead], axis=0), BF16)
            self.qkv[m, j] = r

        def probs(self, j):
            fill = fill_ref[pl.ds(0, R), pl.ds(0, R)]
            sc = jnp.where(fill == 0.0, _dot_nt(self.qkv[0, j], self.qkv[1, j]) * scale, fill)
            mx = jnp.max(sc, axis=-1, keepdims=True)
            e = jnp.exp(sc - mx)
            l = jnp.sum(e, axis=-1, keepdims=True)
            r = pl.reciprocal(l, approx=True)
            r = r * (2.0 - l * r)
            self.ps[j] = (e * r).astype(BF16)

        def attend(self, j):
            o = _dot(self.ps[j], self.qkv[2, j])
            row = pl.multiple_of(self.s * M, M)
            ob[2 * j, pl.ds(row, M), :] = o[2 * SEG:2 * SEG + M].astype(BF16)
            ob[2 * j + 1, pl.ds(row, M), :] = o[2 * SEG + M:].astype(BF16)
            self.os += [o[0:SEG], o[SEG:2 * SEG]]

        def wo(self, h0, h1, ns):
            if (h0, h1) not in self.ocat:
                self.ocat[h0, h1] = jnp.concatenate(self.os[h0:h1], axis=1).astype(BF16)
            o = self.ocat[h0, h1]
            for n in ns:
                w = wo_u[n, pl.ds(h0 * 64, (h1 - h0) * 64), :]
                if cfg["tie"] == n + 1 + (NB if h1 == H else 0):
                    parts = [jnp.where(self.s > 1000, pltpu.bitcast(t, U32), w[8 * i:8 * i + 8])
                             for i, t in enumerate(self.ties)]
                    w = jnp.concatenate(parts + [w[8 * len(parts):]], axis=0)
                d = _dot(o, pltpu.bitcast(w, BF16))
                self.acc[n] = d if self.acc[n] is None else d + self.acc[n]

        def finish(self):
            res = jnp.concatenate(self.acc, axis=1)
            obuf[self.s] = res.astype(BF16)
            return res[0:M]

        def run(self, item):
            kind = item[0]
            g, p = self.g, self.p
            never = (self.s if cfg["real_chain"] else p) > 1000
            if kind == "P":
                self.proj(item[1], item[2])
            elif kind == "S":
                self.probs(item[1])
            elif kind == "V":
                self.attend(item[1])
            elif kind == "W":
                self.wo(item[1], item[2], item[3])
            elif kind == "A1":
                self.kv = a_stage1_pre(g, p, never)
            elif kind == "AU":
                a_stage1_u(g, p, self.kv)
            elif kind == "AH":
                a_stage1_h(g, p)
            elif kind == "A2":
                a_stage2(g + 1, p, self.slot, cfg["chain"], never)
            elif kind == "A3":
                a_stage3(g + 1, jnp.maximum(g - 1, 0), p, self.slot)
            elif kind == "N1":
                gn = (self.s + 1) // 8
                kv = a_stage1_pre(jnp.minimum(gn, NG - 1), (self.s + 1) % 8, never, gn % 2)
                if cfg["tie"]:
                    self.ties.append(pltpu.bitcast(kv[C - 8:C], F32))
            elif kind == "N2":
                tails = a_stage2((self.s + 1) // 8 + 1, (self.s + 1) % 8, 0, cfg["chain"], never)
                if cfg["tie"]:
                    self.ties += tails
            elif kind == "PU":
                a_stage1_u(g, p, None)
            elif kind == "P3":
                a_stage3(g + 1, jnp.maximum(g - 1, 0), p, 0)

    U, order = _make_order(cfg["order"])
    pipe = any(item[0] == "N1" for _, item in order)
    pipe2 = any(item[0] == "N2" for _, item in order)
    if pipe:
        self_wait(abuf.at[0], SA)
        a_stage1_pre(0, 0, None)

    def steps(i, mem):
        s0 = i * U
        sw = s0 + U if pipe else s0

        @pl.when(jnp.logical_and(sw % 8 == 0, sw < NSEG))
        def _():
            self_wait(abuf.at[sw // 8], SA + sw // 8)
        st = [Step(s0 + u, u) for u in range(U)]
        for u, item in order:
            if item[0] == "start":
                st[u].start(mem)
            elif item[0] == "finish":
                mem = st[u].finish()
            else:
                st[u].run(item)
        return mem

    with scope("steps"):
        lax.fori_loop(0, NSEG // U, steps, mem0_ref[...].astype(F32))

    ob_cp = pltpu.make_async_copy(
        obuf.at[:, pl.ds(M, SEG - M), :],
        out_hbm.at[:, pl.ds(M, SEG - M), pl.ds(D, D)], sems.at[SO])
    ob_cp.start()
    for g in range(NG - 1):
        pltpu.make_async_copy(
            aout.at[g], out_hbm.at[:, :, pl.ds(g * 128, 128)], sems.at[SO + 1]).start()

    EP = cfg["ep"]
    GL = NG - 1
    HS = cfg["ep_split"]

    def epi(it, carry):
        def part(n, h0, h1):
            lhs = jnp.concatenate([ob[h] for h in range(h0, h1)], axis=1)
            return _dot(lhs, pltpu.bitcast(wo_u[n, pl.ds(h0 * 64, (h1 - h0) * 64), :], BF16))
        for u in range(EP):
            n = it * EP + u
            if pipe2:
                a_stage3(GL, GL, n, 0)
                a_stage2(GL, jnp.minimum(n + 1, 7), 0, cfg["ep_chain"], it > 1000)
                d = part(n, 0, H)
            else:
                a_stage2(GL, n, u % 2, cfg["ep_chain"], it > 1000)
                d = part(n, 0, HS)
                a_stage3(GL, GL, n, u % 2)
                d = part(n, HS, H) + d
            obb[n] = d.reshape(NSEG, M, 128).astype(BF16)
        for u in range(EP):
            n = it * EP + u
            col = pl.multiple_of(D + n * 128, 128)
            pltpu.make_async_copy(
                obb.at[n], out_hbm.at[:, pl.ds(0, M), pl.ds(col, 128)], sems.at[SO + 2]).start()
        for o in range(2):
            rows = pl.ds((it * EP + 8 * o) * 4, 4 * EP)
            pltpu.make_async_copy(
                aout.at[GL, rows], out_hbm.at[rows, :, pl.ds(GL * 128, 128)], sems.at[SO + 1]).start()
        return carry
    with scope("epi"):
        lax.fori_loop(0, NB // EP, epi, 0)
    ob_cp.wait()
    self_wait(aout, SO + 1)
    self_wait(obb, SO + 2)


def _b_order(u, extra, o):
    ks = o.get("ks", 24)
    tmpl = [(x[0], int(x[1:])) for x in o.get("tmpl", "q0 v1 S1 k0 V2").split()]
    out = list(extra.get("pre", [])) + [(u, ("start",))]
    nw = 0
    for t in range(NPAIR + max(l for _, l in tmpl)):
        for kind, lag in tmpl:
            j = t - lag
            if j < 0:
                continue
            if j >= NPAIR:
                if kind in "qkv" and nw < NB:
                    out.append((u, ("W", 0, ks, (nw,))))
                    nw += 1
                continue
            out.append((u, ("P", "qkv".index(kind), j) if kind in "qkv" else (kind, j)))
        out += extra.get(t, [])
    out += extra.get("tail", [])
    out += [(u, ("W", 0, ks, tuple(range(nw, NB))))]
    out += extra.get("tail2", [])
    out += [(u, ("W", ks, H, tuple(range(NB))))]
    out += extra.get("end", [])
    out += [(u, ("finish",))]
    out += extra.get("post", [])
    return out


def _make_order(o):
    out = []
    U = len(o["a"])
    for u, d in enumerate(o["a"]):
        ex = {}
        for k, names in d.items():
            k = int(k) if k.isdigit() else k
            ex[k] = [(u - 1, (n[1:],)) if n.startswith("-") else (u, (n,)) for n in names]
        out += _b_order(u, ex, o)
    return U, out


_DEFAULT_CFG = dict(order=dict(a=[{"pre": ["A1"], "0": ["AH"], "5": ["AU", "A2"], "17": ["A3"]}],
                               tmpl="q0 S1 k0 v1 V2", ks=24),
                    pp=4, ep=2, ep_split=24, ep_chain=1, chain=1, chain1=1, real_chain=1,
                    split_u=0, split_h=0, tie=0)


def _pack_rows(x):
    b = np.asarray(x, dtype=jnp.bfloat16).view(np.uint16).astype(np.uint32)
    return b[0::2] | (b[1::2] << 16)


def _build(cfg):
    fwd_np, inv_np = _dft_constants()
    fill_np = np.zeros((96, 128), np.float32)
    fill_np[:R, :R] = _mask_fill()

    def run(A_q, A_k, A_v, A_shift_k, A_ssm_k, A_ssm_D, B_x, B_mem0, B_Wq, B_Wk, B_Wv, B_Wo):
        sk = A_shift_k.T.reshape(KS, NG, 128).transpose(1, 0, 2)
        any_spec = pl.BlockSpec(memory_space=pl.ANY)
        out = pl.pallas_call(
            functools.partial(_kernel, cfg),
            out_shape=jax.ShapeDtypeStruct((NSEG, SEG, 2 * D), BF16),
            in_specs=[any_spec] * 15,
            out_specs=any_spec,
            scratch_shapes=[
                pltpu.VMEM((3 * H * SLAB + 544, 128), U32),
                pltpu.VMEM((NB, H * DH // 2, 128), U32),
                pltpu.VMEM((16, 128, 16, DH), BF16),
                pltpu.VMEM((8, 512, D), BF16),
                pltpu.VMEM((NSEG, SEG, D), BF16),
                pltpu.VMEM((4, NSEG, M, KQ), BF16),
                pltpu.VMEM((4, NSEG * M // 2, KQ), U32),
                pltpu.VMEM((3 * NPAIR, NSEG, 8, 128), U32),
                pltpu.VMEM((H, NSEG * M, DH), BF16),
                pltpu.VMEM((NSEG, SEG, D), BF16),
                pltpu.VMEM((NB, NSEG, M, 128), BF16),
                pltpu.VMEM((NG, 3, S, 128), BF16),
                pltpu.VMEM((NC, D, C), BF16),
                pltpu.VMEM((S // 2 + KPAD, 128), U32),
                pltpu.VMEM((2, S // 2, 128), U32),
                pltpu.VMEM((2, NC, 2 * C, 128), F32),
                pltpu.VMEM((2, NC + 7, 2 * C, 128), F32),
                pltpu.VMEM((2 * C, 128), F32),
                pltpu.VMEM((NG, NSEG, SEG, 128), BF16),
                pltpu.VMEM((2, 2, 2, C // 2, 128), U32),
                pltpu.VMEM((C, C), U32),
                pltpu.VMEM((C // 2, C), U32),
                pltpu.VMEM((96, 128), F32),
                pltpu.VMEM((NG, 8, 8, 128), F32),
                pltpu.VMEM((M, D), BF16),
                pltpu.VMEM((NG, KS, 128), BF16),
                pltpu.VMEM((NG, 128), BF16),
                pltpu.SemaphoreType.DMA((48,)),
            ],
            compiler_params=pltpu.CompilerParams(vmem_limit_bytes=124 * 1024 * 1024),
        )(A_q.reshape(S, D), A_k.reshape(S, D), A_v.reshape(S, D), sk, A_ssm_k,
          A_ssm_D.reshape(NG, 128), B_x.reshape(NSEG, SEG, D), B_mem0.reshape(M, D),
          B_Wq, B_Wk, B_Wv, B_Wo.reshape(H * DH, D),
          jnp.asarray(_pack_rows(fwd_np)), jnp.asarray(_pack_rows(inv_np)), jnp.asarray(fill_np))
        return out.reshape(1, S, 2 * D)

    return run


@functools.partial(jax.jit, static_argnames=("B_seg_len",))
def pallas_concat_heads__ssm_conv_h3__memory_aug_recurrent_mem_tr__prompt_kernel(
    A_q: jax.Array,
    A_k: jax.Array,
    A_v: jax.Array,
    A_shift_k: jax.Array,
    A_ssm_k: jax.Array,
    A_ssm_D: jax.Array,
    B_x: jax.Array,
    B_mem0: jax.Array,
    B_Wq: jax.Array,
    B_Wk: jax.Array,
    B_Wv: jax.Array,
    B_Wo: jax.Array,
    B_seg_len: int = SEG,
):
    assert B_seg_len == SEG
    return _build(_DEFAULT_CFG)(A_q, A_k, A_v, A_shift_k, A_ssm_k, A_ssm_D, B_x, B_mem0,
                                B_Wq, B_Wk, B_Wv, B_Wo)
```

```python
import functools

import numpy as np
import jax
import jax.numpy as jnp
from jax import lax
import jax.experimental.pallas as pl
import jax.experimental.pallas.tpu as pltpu

F32 = jnp.float32
BF16 = jnp.bfloat16
U32 = jnp.uint32

S = 2048
D = 1024
H = 32
DH = 128
M = 8
SEG = 32
NSEG = S // SEG
NPAIR = H // 2
R = 2 * (M + SEG)
SLAB = 520
KS = 4
C = 128
NC = S // C
NG = D // 128
KQ = D // 4
KPAD = 32
NB = D // 128


def _dft_constants():
    fe = np.arange(0, C, 2)
    f = np.concatenate([fe, C - 1 - fe])
    t = np.arange(C)
    ang = (np.pi * (2 * f + 1) / (2 * C))[:, None] * t[None, :]
    fwd = np.concatenate([np.cos(ang), -np.sin(ang)], axis=0)
    a = ang[:C // 2]
    inv = np.stack([np.cos(a), -np.sin(a)], axis=1).reshape(C, C).T / C
    inv = np.concatenate([inv[0::2], inv[1::2]], axis=0)
    return fwd.astype(np.float32), inv.astype(np.float32)


def _mask_fill():
    blk = np.concatenate([np.arange(M), M + np.arange(M, SEG)])
    lead = M + np.arange(M)
    qhead = np.concatenate([np.zeros(SEG), np.ones(SEG), np.zeros(M), np.ones(M)])
    qpos = np.concatenate([blk, blk, lead, lead])
    khead = np.arange(R) % 2
    kpos = np.concatenate([blk, lead])[np.arange(R) // 2]
    same = qhead[:, None] == khead[None, :]
    ok = (qpos[:, None] < M) | (qpos[:, None] >= kpos[None, :])
    fill = np.where(same, np.where(ok, 0.0, -1e9), -np.inf)
    return fill.astype(np.float32)


def _pack(lo, hi):
    return pltpu.pack_elementwise([lo, hi], packed_dtype=BF16)


def _unpack(w, index):
    return pltpu.unpack_elementwise(w, index=index, packed_dtype=BF16, unpacked_dtype=F32)


def _dot(a, b):
    return jnp.dot(a, b, preferred_element_type=F32)


def _dot_nt(a, b):
    return lax.dot_general(a, b, (((1,), (1,)), ((), ())), preferred_element_type=F32)


def _kernel(cfg,
            aq_hbm, ak_hbm, av_hbm, sk_hbm, ssmk_hbm, ssmd_hbm, x_hbm, mem0_hbm,
            wq_hbm, wk_hbm, wv_hbm, wo_hbm, fwd_hbm, inv_hbm, fill_hbm,
            out_hbm,
            w_u, wo_u, wstage, wostage, xbuf, xlead, xlead_u, qkvb, ob, obuf, obb,
            abuf, hbuf, kf, kvb, ubuf, gbuf, hlast, aout, ystage,
            fwd_ref, inv_ref, fill_ref, taps, mem0_ref, sk_ref, ssmd_ref,
            sems):
    import contextlib
    scope = jax.named_scope if cfg.get("scopes") else (lambda name: contextlib.nullcontext())
    SW, SWO, SXL, SX, SH, SA, SO, SS = 0, 16, 24, 28, 29, 30, 38, 42
    only = cfg.get("only")

    def loop(name, lo, hi, body, init):
        if only is not None and name not in only:
            return init
        with scope(name):
            return lax.fori_loop(lo, hi, body, init)
    w_hbms = (wq_hbm, wk_hbm, wv_hbm)
    a_hbms = (aq_hbm, ak_hbm, av_hbm)

    def w_copy(c, k):
        m, g = c // 2, c % 2
        slot = (c % 2) * 8 + k
        return pltpu.make_async_copy(
            w_hbms[m].at[pl.ds(k * 128, 128), pl.ds(16 * g, 16), :],
            wstage.at[slot], sems.at[SW + slot])

    def self_wait(ref, sem):
        pltpu.make_async_copy(ref, ref, sems.at[sem]).wait()

    def wo_copy(k):
        return pltpu.make_async_copy(
            wo_hbm.at[pl.ds(k * 512, 512), :], wostage.at[k], sems.at[SWO + k])

    def xlead_copy(q):
        return pltpu.make_async_copy(
            x_hbm.at[:, pl.ds(0, M), pl.ds(q * KQ, KQ)], xlead.at[q], sems.at[SXL + q])

    x_cp = pltpu.make_async_copy(
        x_hbm.at[:, pl.ds(M, SEG - M), :], xbuf.at[:, pl.ds(M, SEG - M), :], sems.at[SX])

    def h_copy(c):
        return pltpu.make_async_copy(
            ssmk_hbm.at[:, pl.ds(c * C, C)], hbuf.at[c], sems.at[SH])

    def a_copy(t, g):
        return pltpu.make_async_copy(
            a_hbms[t].at[:, pl.ds(g * 128, 128)], abuf.at[g, t], sems.at[SA + g])

    small = [pltpu.make_async_copy(src, dst, sems.at[SS + i]) for i, (src, dst) in enumerate((
        (fwd_hbm, fwd_ref), (inv_hbm, inv_ref), (fill_hbm, fill_ref),
        (mem0_hbm, mem0_ref), (sk_hbm, sk_ref), (ssmd_hbm, ssmd_ref)))]

    for q in range(4):
        xlead_copy(q).start()
        w_copy(0, 2 * q).start()
        w_copy(0, 2 * q + 1).start()
    for k in range(8):
        w_copy(1, k).start()

    kf[pl.ds(0, KPAD), :] = jnp.zeros((KPAD, 128), U32)
    for b in range(2):
        gbuf[b, pl.ds(0, 7)] = jnp.zeros((7, 2 * C, 128), F32)

    def relayout_piece(c, k):
        slot = (c % 2) * 8 + k
        base = ((c // 2) * H + 8 * (c % 2)) * SLAB + k * 64
        for i in range(64):
            a = pltpu.bitcast(wstage[slot, 2 * i], U32)
            b = pltpu.bitcast(wstage[slot, 2 * i + 1], U32)
            ev = (a & jnp.uint32(0xFFFF)) | (b << 16)
            od = (a >> 16) | (b & jnp.uint32(0xFFFF0000))
            w_u[pl.ds(base + i, 8, stride=SLAB), :] = ev
            w_u[pl.ds(base + NPAIR * SLAB + i, 8, stride=SLAB), :] = od

    def store_pair(it, outs):
        qkvb[it] = _pack(outs[0], outs[1]).reshape(NSEG, M, DH)

    def batch_pair(it):
        m = it // NPAIR
        j = it % NPAIR
        xl = jnp.concatenate([pltpu.bitcast(xlead_u[q], BF16) for q in range(4)], axis=1)
        outs = []
        for par in range(2):
            row = pl.multiple_of((m * H + par * NPAIR + j) * SLAB, 8)
            w = pltpu.bitcast(w_u[pl.ds(row, D // 2), :], BF16)
            outs.append(_dot(xl, w))
        store_pair(it, outs)

    def quarter_prep(q):
        self_wait(xlead.at[q], SXL + q)
        for u in range(2):
            self_wait(wstage.at[2 * q + u], SW + 2 * q + u)
        xq = xlead[q].astype(F32).reshape(NSEG * M, KQ).astype(BF16)
        xlead_u[q] = pltpu.bitcast(xq, U32)
        for u in range(2):
            relayout_piece(0, 2 * q + u)

    def quarter_dot(q, par, j):
        row = pl.multiple_of((par * NPAIR + j) * SLAB + q * (KQ // 2), 8)
        w = pltpu.bitcast(w_u[pl.ds(row, KQ // 2), :], BF16)
        return _dot(pltpu.bitcast(xlead_u[q], BF16), w)

    def facc_get(hh):
        return jnp.concatenate([ubuf[0, hh], ubuf[1, hh]], axis=0)

    def quarter(q, carry):
        quarter_prep(q)
        for u in range(2):
            w_copy(2, 2 * q + u).start()
        for j in range(8):
            for par in range(2):
                hh = 2 * j + par
                d = quarter_dot(q, par, j) + jnp.where(q == 0, 0.0, facc_get(hh))
                ubuf[0, hh] = d[0:2 * C]
                ubuf[1, hh] = d[2 * C:]
        return carry
    loop("quarters", 0, 3, quarter, 0)
    quarter_prep(3)
    for u in range(2):
        w_copy(2, 6 + u).start()

    def quarter_last(it, carry):
        for u in range(4):
            self_wait(wstage.at[8 + 4 * it + u], SW + 8 + 4 * it + u)
        for u in range(4):
            j = 4 * it + u
            store_pair(j, [quarter_dot(3, par, j) + facc_get(2 * j + par) for par in range(2)])
            relayout_piece(1, j)
        return carry
    loop("quarter_last", 0, 2, quarter_last, 0)

    PP = cfg["pp"]
    IPC = 8 // PP

    def issue(c):
        if c + 2 < 6:
            for k in range(8):
                w_copy(c + 2, k).start()
        if c < 3:
            for k in range(4 * (c - 1), 4 * c):
                wo_copy(k).start()
        if c == 1:
            for cp in small:
                cp.start()
        if c == 3:
            x_cp.start()
        if c == 4:
            for cc in range(NC):
                h_copy(cc).start()
            for g in range(NG):
                for t in (1, 2, 0):
                    a_copy(t, g).start()

    def pro_body(it, carry):
        for c in range(1, 5):
            @pl.when(it == c * IPC)
            def _():
                issue(c)
        cn = it // IPC + 1
        for u in range(PP):
            slot = (cn % 2) * 8 + (it % IPC) * PP + u
            self_wait(wstage.at[slot], SW + slot)
        for u in range(PP):
            batch_pair(it * PP + u)
            relayout_piece(cn, (it % IPC) * PP + u)
        return carry
    loop("pro_body", IPC, 5 * IPC, pro_body, 0)

    for cp in small:
        cp.wait()
    for g in range(NG):
        sk = sk_ref[g].astype(F32)
        for j in range(KS):
            taps[g, j] = jnp.broadcast_to(sk[j:j + 1], (8, 128))
        taps[g, KS] = jnp.broadcast_to(ssmd_ref[...].astype(F32)[g:g + 1], (8, 128))

    def pro_last(it, carry):
        for u in range(PP):
            k = it * PP + u
            self_wait(wostage.at[k], SWO + k)
        for u in range(PP):
            k = it * PP + u
            batch_pair(40 + k)
            for r in range(8):
                blk = wostage[k, pl.ds(r * 64, 64), :]
                row = pl.multiple_of(k * 256 + r * 32, 32)
                for n in range(NB):
                    wo_u[n, pl.ds(row, 32), :] = pltpu.bitcast(blk[:, n * 128:(n + 1) * 128], U32)
        return carry
    loop("pro_last", 0, IPC, pro_last, 0)
    with scope("xh_wait"):
        x_cp.wait()
        self_wait(hbuf, SH)

    def rep(x, rows):
        return x if rows == 8 else jnp.concatenate([x] * (rows // 8), axis=0)

    def a_stage1_pre(g, p, never, par=None):
        par = g % 2 if par is None else par
        r = p * C if isinstance(p, int) else pl.multiple_of(p * C, C)
        r2 = 2 * r if isinstance(p, int) else pl.multiple_of(2 * r, 2 * C)
        kw = pltpu.bitcast(abuf[g, 1, pl.ds(r2, 2 * C), :], U32)
        vw = pltpu.bitcast(abuf[g, 2, pl.ds(r2, 2 * C), :], U32)
        kf[pl.ds(KPAD + r, C), :] = kw
        t = [taps[g, j] for j in range(KS)]
        parts = {}
        last = None
        mode = cfg["chain1"] if never is not None else 0
        blocks = list(range(0, C, 8))
        if cfg.get("rev1"):
            blocks = [b + h for b in range(C // 2 - 8, -8, -8) for h in (0, C // 2)]
        for b in blocks:
            w0 = kw[b:b + 8]
            w1 = kf[pl.ds(KPAD + r + b - 1, 8), :]
            w2 = kf[pl.ds(KPAD + r + b - 2, 8), :]
            if last is not None and mode == 3:
                w0 = jnp.where(never, last, w0)
                w1 = jnp.where(never, last, w1)
            e0, o0 = _unpack(w0, 0), _unpack(w0, 1)
            e1, o1 = _unpack(w1, 0), _unpack(w1, 1)
            o2 = _unpack(w2, 1)
            ke = e0 * t[0]
            ko = o0 * t[0]
            if last is not None and mode == 1:
                ke = jnp.where(never, last[0], ke)
                ko = jnp.where(never, last[1], ko)
            if last is not None and mode == 2:
                ke = jnp.where(never, last[1], ke)
            ke = (ke + o1 * t[1] + e1 * t[2] + o2 * t[3]) * _unpack(vw[b:b + 8], 0)
            if mode >= 2:
                ko = jnp.where(never, ke, ko)
            ko = (ko + e0 * t[1] + o1 * t[2] + e1 * t[3]) * _unpack(vw[b:b + 8], 1)
            parts[b] = _pack(ke, ko)
            last = parts[b] if mode == 3 else (ke, ko)
        parts = [parts[b] for b in range(0, C, 8)]
        kv = jnp.concatenate(parts, axis=0)
        kvb[par, pl.ds(r, C), :] = kv
        return kv

    def a_stage1_u(g, p, kv):
        fwd = pltpu.bitcast(fwd_ref[...], BF16)
        if kv is None:
            kv = kvb[g % 2, pl.ds(pl.multiple_of(p * C, C), C), :]
        for u in range(2):
            w = pltpu.bitcast(kv[u * C // 2:(u + 1) * C // 2], BF16)
            if cfg["split_u"]:
                for hf in range(2):
                    ubuf[g % 2, 2 * p + u, pl.ds(hf * C, C), :] = _dot(fwd[hf * C:(hf + 1) * C], w)
            else:
                ubuf[g % 2, 2 * p + u] = _dot(fwd, w)

    def a_stage1_h(g, p):
        fwd = pltpu.bitcast(fwd_ref[...], BF16)
        rows = pl.ds(pl.multiple_of(g * 128, 128), 128)
        if cfg["split_h"]:
            hs = [jnp.concatenate([_dot_nt(fwd[hf * C:(hf + 1) * C], hbuf[2 * p + u, rows, :])
                                   for hf in range(2)], axis=0) for u in range(2)]
        else:
            hs = [_dot_nt(fwd, hbuf[2 * p + u, rows, :]) for u in range(2)]
        prev = jnp.where(p == 0, 0.0, hlast[...])
        hlast[...] = hs[1]
        hc = C // 2
        for u, (cur, prv) in enumerate(((hs[0], prev), (hs[1], hs[0]))):
            gbuf[g % 2, 7 + 2 * p + u] = jnp.concatenate([
                cur[0:hc] - prv[C:C + hc], cur[hc:C] + prv[C + hc:],
                cur[C:C + hc] + prv[0:hc], cur[C + hc:] - prv[hc:C]], axis=0)

    def a_stage2(gp, p, slot, chain, never):
        b = gp % 2
        RB = 8
        re = [[], []]
        im = [[], []]
        last = None
        for r in [r0 + blk for r0 in range(0, C // 2, RB) for blk in (0, C // 2)]:
            gr = [gbuf[b, 7 + p + 8 - j, pl.ds(r, RB), :] for j in range(NC)]
            gi = [gbuf[b, 7 + p + 8 - j, pl.ds(C + r, RB), :] for j in range(NC)]
            ur = [ubuf[b, j, pl.ds(r, RB), :] for j in range(NC)]
            ui = [ubuf[b, j, pl.ds(C + r, RB), :] for j in range(NC)]
            for o, (nt, off) in enumerate(((8, 8), (16, 0))):
                if chain == 1:
                    ar = gr[off] * ur[0]
                    ai = gr[off] * ui[0]
                    if last is not None:
                        ar = jnp.where(never, last[0], ar)
                        ai = jnp.where(never, last[1], ai)
                    ar = ar - gi[off] * ui[0]
                    ai = ai + gi[off] * ur[0]
                    for j in range(1, nt):
                        ar = ar + gr[j + off] * ur[j]
                        ai = ai + gr[j + off] * ui[j]
                        ar = ar - gi[j + off] * ui[j]
                        ai = ai + gi[j + off] * ur[j]
                    last = (ar, ai)
                else:
                    ar = gr[off] * ur[0]
                    if last is not None:
                        ar = jnp.where(never, last, ar)
                    ar = ar - gi[off] * ui[0]
                    for j in range(1, nt):
                        ar = ar + gr[j + off] * ur[j]
                        ar = ar - gi[j + off] * ui[j]
                    ai = jnp.where(never, ar, gr[off] * ui[0])
                    ai = ai + gi[off] * ur[0]
                    for j in range(1, nt):
                        ai = ai + gr[j + off] * ui[j]
                        ai = ai + gi[j + off] * ur[j]
                    last = ai
                re[o].append(ar)
                im[o].append(ai)
                if r >= C // 2:
                    rows = pl.ds(r - C // 2, RB)
                    ystage[slot, o, 0, rows, :] = _pack(re[o][-2] + ar, im[o][-2] - ai)
                    ystage[slot, o, 1, rows, :] = _pack(re[o][-2] - ar, im[o][-2] + ai)
        return list(last) if chain == 1 else [last]

    def a_stage3(gp, gq, p, slot):
        inv = pltpu.bitcast(inv_ref[...], BF16)
        dd = rep(taps[gq, KS], C // 2)
        for o in range(2):
            i = p + 8 * o
            kvw = kvb[gp % 2, pl.ds(pl.multiple_of(i * (C // 2), C // 2), C // 2), :]
            qw = pltpu.bitcast(abuf[gq, 0, pl.ds(pl.multiple_of(i * C, C), C), :], U32)
            res = []
            for e in range(2):
                y = _dot(inv[e * (C // 2):(e + 1) * (C // 2)], pltpu.bitcast(ystage[slot, o, e], BF16))
                res.append(_unpack(qw, e) * (y + _unpack(kvw, e) * dd))
            out = pltpu.bitcast(_pack(res[0], res[1]), BF16)
            aout[gq, pl.ds(pl.multiple_of(i * 4, 4), 4)] = out.reshape(4, SEG, 128)

    scale = DH ** (-0.5)

    def w_slab(m, h, z):
        slab = m * H + (h % 2) * NPAIR + h // 2
        row = slab * SLAB if z is None else pl.multiple_of(z + slab * SLAB, 8)
        return pltpu.bitcast(w_u[pl.ds(row, D // 2), :], BF16)

    class Step:
        def __init__(self, s, u):
            self.s = s
            self.slot = u % 2
            self.z = None if (u == 0 or not cfg.get("zoff")) else pl.multiple_of(jnp.where(s > 1000 + u, 32, 0), 32)
            self.g = s // 8
            self.p = s % 8
            self.qkv, self.ps, self.os = {}, {}, []
            self.acc = [None] * NB
            self.ocat = {}
            self.early = {}
            self.ties = []

        def start(self, mem):
            x = xbuf[self.s, pl.ds(M, SEG - M), :].astype(F32)
            self.lhsf = jnp.concatenate([mem, x], axis=0)
            self.lhs = self.lhsf.astype(BF16)

        def proj_early(self, m, j, k):
            self.early[m, j] = (k, [_dot(self.lhsf[:, :k].astype(BF16), w_slab(m, 2 * j + e, self.z)[:k])
                                    for e in range(2)])

        def proj(self, m, j):
            if (m, j) in self.early:
                k, part = self.early[m, j]
                a, b = [_dot(self.lhsf[:, k:].astype(BF16), w_slab(m, 2 * j + e, self.z)[k:]) + part[e]
                        for e in range(2)]
            else:
                a = _dot(self.lhs, w_slab(m, 2 * j, self.z))
                b = _dot(self.lhs, w_slab(m, 2 * j + 1, self.z))
            lead = qkvb[m * NPAIR + j, self.s]
            if m == 0:
                r = jnp.concatenate([a, b, _unpack(lead, 0), _unpack(lead, 1)], axis=0).astype(BF16)
            else:
                r = pltpu.bitcast(jnp.concatenate([_pack(a, b), lead], axis=0), BF16)
            self.qkv[m, j] = r

        def probs(self, j):
            fill = fill_ref[pl.ds(0, R), pl.ds(0, R)]
            sc = jnp.where(fill == 0.0, _dot_nt(self.qkv[0, j], self.qkv[1, j]) * scale, fill)
            mx = jnp.max(sc, axis=-1, keepdims=True)
            e = jnp.exp(sc - mx)
            l = jnp.sum(e, axis=-1, keepdims=True)
            r = pl.reciprocal(l, approx=True)
            r = r * (2.0 - l * r)
            self.ps[j] = (e * r).astype(BF16)

        def attend(self, j):
            o = _dot(self.ps[j], self.qkv[2, j])
            row = pl.multiple_of(self.s * M, M)
            ob[2 * j, pl.ds(row, M), :] = o[2 * SEG:2 * SEG + M].astype(BF16)
            ob[2 * j + 1, pl.ds(row, M), :] = o[2 * SEG + M:].astype(BF16)
            self.os += [o[0:SEG], o[SEG:2 * SEG]]

        def wo(self, h0, h1, ns):
            if (h0, h1) not in self.ocat:
                self.ocat[h0, h1] = jnp.concatenate(self.os[h0:h1], axis=1).astype(BF16)
            o = self.ocat[h0, h1]
            for n in ns:
                row = h0 * 64 if self.z is None else pl.multiple_of(self.z + h0 * 64, 32)
                w = wo_u[n, pl.ds(row, (h1 - h0) * 64), :]
                if cfg["tie"] == n + 1 + (NB if h1 == H else 0):
                    parts = [jnp.where(self.s > 1000, pltpu.bitcast(t, U32), w[8 * i:8 * i + 8])
                             for i, t in enumerate(self.ties)]
                    w = jnp.concatenate(parts + [w[8 * len(parts):]], axis=0)
                d = _dot(o, pltpu.bitcast(w, BF16))
                self.acc[n] = d if self.acc[n] is None else d + self.acc[n]

        def finish(self):
            res = jnp.concatenate(self.acc, axis=1)
            obuf[self.s] = res.astype(BF16)
            return res[0:M]

        def run(self, item):
            kind = item[0]
            g, p = self.g, self.p
            never = (self.s if cfg["real_chain"] else p) > 1000
            if kind == "P":
                self.proj(item[1], item[2])
            elif kind == "E":
                self.proj_early(item[1], item[2], item[3])
            elif kind == "S":
                self.probs(item[1])
            elif kind == "V":
                self.attend(item[1])
            elif kind == "W":
                self.wo(item[1], item[2], item[3])
            elif kind == "A1":
                self.kv = a_stage1_pre(g, p, never)
            elif kind == "AU":
                a_stage1_u(g, p, self.kv)
            elif kind == "AH":
                a_stage1_h(g, p)
            elif kind == "A2":
                a_stage2(g + 1, p, self.slot, cfg["chain"], never)
            elif kind == "A3":
                a_stage3(g + 1, jnp.maximum(g - 1, 0), p, self.slot)
            elif kind == "N1":
                gn = (self.s + 1) // 8
                kv = a_stage1_pre(jnp.minimum(gn, NG - 1), (self.s + 1) % 8, never, gn % 2)
                if cfg["tie"]:
                    self.ties.append(pltpu.bitcast(kv[C - 8:C], F32))
            elif kind == "N2":
                tails = a_stage2((self.s + 1) // 8 + 1, (self.s + 1) % 8, 0, cfg["chain"], never)
                if cfg["tie"]:
                    self.ties += tails
            elif kind == "PU":
                a_stage1_u(g, p, None)
            elif kind == "P3":
                a_stage3(g + 1, jnp.maximum(g - 1, 0), p, 0)

    U, order = _make_order(cfg["order"])
    pipe = any(item[0] == "N1" for _, item in order)
    pipe2 = any(item[0] == "N2" for _, item in order)
    if pipe:
        self_wait(abuf.at[0], SA)
        a_stage1_pre(0, 0, None)

    def steps(i, mem):
        s0 = i * U
        sw = s0 + U if pipe else s0

        @pl.when(jnp.logical_and(sw % 8 == 0, sw < NSEG))
        def _():
            self_wait(abuf.at[sw // 8], SA + sw // 8)
        st = [Step(s0 + u, u) for u in range(U)]
        for u, item in order:
            if item[0] == "start":
                st[u].start(mem)
            elif item[0] == "finish":
                mem = st[u].finish()
            else:
                st[u].run(item)
        return mem

    loop("steps", 0, NSEG // U, steps, mem0_ref[...].astype(F32))

    ob_cp = pltpu.make_async_copy(
        obuf.at[:, pl.ds(M, SEG - M), :],
        out_hbm.at[:, pl.ds(M, SEG - M), pl.ds(D, D)], sems.at[SO])
    ob_cp.start()
    for g in range(NG - 1):
        pltpu.make_async_copy(
            aout.at[g], out_hbm.at[:, :, pl.ds(g * 128, 128)], sems.at[SO + 1]).start()

    EP = cfg["ep"]
    GL = NG - 1
    HS = cfg["ep_split"]

    def epi(it, carry):
        def part(n, h0, h1):
            lhs = jnp.concatenate([ob[h] for h in range(h0, h1)], axis=1)
            return _dot(lhs, pltpu.bitcast(wo_u[n, pl.ds(h0 * 64, (h1 - h0) * 64), :], BF16))
        for u in range(EP):
            n = it * EP + u
            if pipe2:
                a_stage3(GL, GL, n, 0)
                a_stage2(GL, jnp.minimum(n + 1, 7), 0, cfg["ep_chain"], it > 1000)
                d = part(n, 0, H)
            else:
                a_stage2(GL, n, u % 2, cfg["ep_chain"], it > 1000)
                d = part(n, 0, HS)
                a_stage3(GL, GL, n, u % 2)
                d = part(n, HS, H) + d
            obb[n] = d.reshape(NSEG, M, 128).astype(BF16)
        for u in range(EP):
            n = it * EP + u
            col = pl.multiple_of(D + n * 128, 128)
            pltpu.make_async_copy(
                obb.at[n], out_hbm.at[:, pl.ds(0, M), pl.ds(col, 128)], sems.at[SO + 2]).start()
        for o in range(2):
            rows = pl.ds((it * EP + 8 * o) * 4, 4 * EP)
            pltpu.make_async_copy(
                aout.at[GL, rows], out_hbm.at[rows, :, pl.ds(GL * 128, 128)], sems.at[SO + 1]).start()
        return carry
    loop("epi", 0, NB // EP, epi, 0)
    ob_cp.wait()
    self_wait(aout, SO + 1)
    self_wait(obb, SO + 2)


def _b_order(u, extra, o):
    ks = o.get("ks", 24)
    tmpl = [(x[0], int(x[1:])) for x in o.get("tmpl", "q0 v1 S1 k0 V2").split()]
    out = list(extra.get("pre", [])) + [(u, ("start",))]
    if u > 0:
        first = [(kind, t - lag) for t in range(3) for kind, lag in tmpl if kind in "qkv" and t >= lag]
        out += [(u, ("E", "qkv".index(kind), j, o.get("ek", 768))) for kind, j in first[:o.get("ne", 2)]]
    nw = 0
    for t in range(NPAIR + max(l for _, l in tmpl)):
        for kind, lag in tmpl:
            j = t - lag
            if j < 0:
                continue
            if j >= NPAIR:
                if kind in "qkv" and nw < NB:
                    out.append((u, ("W", 0, ks, (nw,))))
                    nw += 1
                continue
            out.append((u, ("P", "qkv".index(kind), j) if kind in "qkv" else (kind, j)))
        out += extra.get(t, [])
    out += extra.get("tail", [])
    out += [(u, ("W", 0, ks, tuple(range(nw, NB))))]
    out += extra.get("tail2", [])
    out += [(u, ("W", ks, H, tuple(range(NB))))]
    out += extra.get("end", [])
    out += [(u, ("finish",))]
    out += extra.get("post", [])
    return out


def _make_order(o):
    out = []
    U = len(o["a"])
    for u, d in enumerate(o["a"]):
        ex = {}
        for k, names in d.items():
            k = int(k) if k.isdigit() else k
            ex[k] = [(u - n.count("-") + n.count("+"), (n.lstrip("+-"),)) for n in names]
        out += _b_order(u, ex, o)
    return U, out


_DEFAULT_CFG = dict(
    order=dict(a=[{"pre": ["A1", "+A1"], "0": ["AH"], "2": ["AU"], "4": ["+AU", "A2"], "16": ["A3"]},
                  {"1": ["AH", "A2"], "14": ["A3"]}],
               tmpl="q0 v1 S1 k0 V2", ks=16, ne=2, ek=768),
    pp=4, ep=2, ep_split=24, ep_chain=1, chain=1, chain1=2, real_chain=1,
    split_u=0, split_h=0, tie=0)


def _pack_rows(x):
    b = np.asarray(x, dtype=jnp.bfloat16).view(np.uint16).astype(np.uint32)
    return b[0::2] | (b[1::2] << 16)


def _build(cfg):
    fwd_np, inv_np = _dft_constants()
    fill_np = np.zeros((96, 128), np.float32)
    fill_np[:R, :R] = _mask_fill()

    def run(A_q, A_k, A_v, A_shift_k, A_ssm_k, A_ssm_D, B_x, B_mem0, B_Wq, B_Wk, B_Wv, B_Wo):
        sk = A_shift_k.T.reshape(KS, NG, 128).transpose(1, 0, 2)
        any_spec = pl.BlockSpec(memory_space=pl.ANY)
        out = pl.pallas_call(
            functools.partial(_kernel, cfg),
            out_shape=jax.ShapeDtypeStruct((NSEG, SEG, 2 * D), BF16),
            in_specs=[any_spec] * 15,
            out_specs=any_spec,
            scratch_shapes=[
                pltpu.VMEM((3 * H * SLAB + 544, 128), U32),
                pltpu.VMEM((NB, H * DH // 2, 128), U32),
                pltpu.VMEM((16, 128, 16, DH), BF16),
                pltpu.VMEM((8, 512, D), BF16),
                pltpu.VMEM((NSEG, SEG, D), BF16),
                pltpu.VMEM((4, NSEG, M, KQ), BF16),
                pltpu.VMEM((4, NSEG * M // 2, KQ), U32),
                pltpu.VMEM((3 * NPAIR, NSEG, 8, 128), U32),
                pltpu.VMEM((H, NSEG * M, DH), BF16),
                pltpu.VMEM((NSEG, SEG, D), BF16),
                pltpu.VMEM((NB, NSEG, M, 128), BF16),
                pltpu.VMEM((NG, 3, S, 128), BF16),
                pltpu.VMEM((NC, D, C), BF16),
                pltpu.VMEM((S // 2 + KPAD, 128), U32),
                pltpu.VMEM((2, S // 2, 128), U32),
                pltpu.VMEM((2, NC, 2 * C, 128), F32),
                pltpu.VMEM((2, NC + 7, 2 * C, 128), F32),
                pltpu.VMEM((2 * C, 128), F32),
                pltpu.VMEM((NG, NSEG, SEG, 128), BF16),
                pltpu.VMEM((2, 2, 2, C // 2, 128), U32),
                pltpu.VMEM((C, C), U32),
                pltpu.VMEM((C // 2, C), U32),
                pltpu.VMEM((96, 128), F32),
                pltpu.VMEM((NG, 8, 8, 128), F32),
                pltpu.VMEM((M, D), BF16),
                pltpu.VMEM((NG, KS, 128), BF16),
                pltpu.VMEM((NG, 128), BF16),
                pltpu.SemaphoreType.DMA((48,)),
            ],
            compiler_params=pltpu.CompilerParams(vmem_limit_bytes=124 * 1024 * 1024),
        )(A_q.reshape(S, D), A_k.reshape(S, D), A_v.reshape(S, D), sk, A_ssm_k,
          A_ssm_D.reshape(NG, 128), B_x.reshape(NSEG, SEG, D), B_mem0.reshape(M, D),
          B_Wq, B_Wk, B_Wv, B_Wo.reshape(H * DH, D),
          jnp.asarray(_pack_rows(fwd_np)), jnp.asarray(_pack_rows(inv_np)), jnp.asarray(fill_np))
        return out.reshape(1, S, 2 * D)

    return run


@functools.partial(jax.jit, static_argnames=("B_seg_len",))
def pallas_concat_heads__ssm_conv_h3__memory_aug_recurrent_mem_tr__prompt_kernel(
    A_q: jax.Array,
    A_k: jax.Array,
    A_v: jax.Array,
    A_shift_k: jax.Array,
    A_ssm_k: jax.Array,
    A_ssm_D: jax.Array,
    B_x: jax.Array,
    B_mem0: jax.Array,
    B_Wq: jax.Array,
    B_Wk: jax.Array,
    B_Wv: jax.Array,
    B_Wo: jax.Array,
    B_seg_len: int = SEG,
):
    assert B_seg_len == SEG
    return _build(_DEFAULT_CFG)(A_q, A_k, A_v, A_shift_k, A_ssm_k, A_ssm_D, B_x, B_mem0,
                                B_Wq, B_Wk, B_Wv, B_Wo)
```

```python
import functools

import numpy as np
import jax
import jax.numpy as jnp
from jax import lax
import jax.experimental.pallas as pl
import jax.experimental.pallas.tpu as pltpu

F32 = jnp.float32
BF16 = jnp.bfloat16
U32 = jnp.uint32

S = 2048
D = 1024
H = 32
DH = 128
M = 8
SEG = 32
NSEG = S // SEG
NPAIR = H // 2
R = 2 * (M + SEG)
SLAB = 520
KS = 4
C = 128
NC = S // C
NG = D // 128
KQ = D // 4
KPAD = 32
NB = D // 128


def _dft_constants():
    fe = np.arange(0, C, 2)
    f = np.concatenate([fe, C - 1 - fe])
    t = np.arange(C)
    ang = (np.pi * (2 * f + 1) / (2 * C))[:, None] * t[None, :]
    fwd = np.concatenate([np.cos(ang), -np.sin(ang)], axis=0)
    a = ang[:C // 2]
    inv = np.stack([np.cos(a), -np.sin(a)], axis=1).reshape(C, C).T / C
    inv = np.concatenate([inv[0::2], inv[1::2]], axis=0)
    return fwd.astype(np.float32), inv.astype(np.float32)


def _mask_fill():
    blk = np.concatenate([np.arange(M), M + np.arange(M, SEG)])
    lead = M + np.arange(M)
    qhead = np.concatenate([np.zeros(SEG), np.ones(SEG), np.zeros(M), np.ones(M)])
    qpos = np.concatenate([blk, blk, lead, lead])
    khead = np.arange(R) % 2
    kpos = np.concatenate([blk, lead])[np.arange(R) // 2]
    same = qhead[:, None] == khead[None, :]
    ok = (qpos[:, None] < M) | (qpos[:, None] >= kpos[None, :])
    fill = np.where(same, np.where(ok, 0.0, -1e9), -np.inf)
    return fill.astype(np.float32)


def _pack(lo, hi):
    return pltpu.pack_elementwise([lo, hi], packed_dtype=BF16)


def _unpack(w, index):
    return pltpu.unpack_elementwise(w, index=index, packed_dtype=BF16, unpacked_dtype=F32)


def _dot(a, b):
    return jnp.dot(a, b, preferred_element_type=F32)


def _dot_nt(a, b):
    return lax.dot_general(a, b, (((1,), (1,)), ((), ())), preferred_element_type=F32)


def _kernel(cfg,
            aq_hbm, ak_hbm, av_hbm, sk_hbm, ssmk_hbm, ssmd_hbm, x_hbm, mem0_hbm,
            wq_hbm, wk_hbm, wv_hbm, wo_hbm, fwd_hbm, inv_hbm, fill_hbm,
            out_hbm,
            w_a, w_b, wo_u, wstage, wostage, xbuf, xlead, xlead_u, xs_u, qkvb, ob, obuf, obb,
            abuf, hbuf, kf, kvb, ubuf, gbuf, hlast, aout, ystage,
            fwd_ref, inv_ref, fill_ref, taps, mem0_ref, sk_ref, ssmd_ref,
            sems):
    import contextlib
    scope = jax.named_scope if cfg.get("scopes") else (lambda name: contextlib.nullcontext())
    SW, SWO, SXL, SX, SH, SA, SO, SS = 0, 16, 24, 28, 29, 30, 38, 42
    only = cfg.get("only")

    def loop(name, lo, hi, body, init):
        if only is not None and name not in only:
            return init
        if cfg.get("scopes") == 2:
            def body2(i, c):
                with scope(name + "_it"):
                    return body(i, c)
            return lax.fori_loop(lo, hi, body2, init)
        with scope(name):
            return lax.fori_loop(lo, hi, body, init)
    w_hbms = (wq_hbm, wk_hbm, wv_hbm)
    a_hbms = (aq_hbm, ak_hbm, av_hbm)

    def w_copy(c, k):
        m, g = c // 2, c % 2
        slot = (c % 2) * 8 + k
        return pltpu.make_async_copy(
            w_hbms[m].at[pl.ds(k * 128, 128), pl.ds(16 * g, 16), :],
            wstage.at[slot], sems.at[SW + slot])

    def self_wait(ref, sem):
        pltpu.make_async_copy(ref, ref, sems.at[sem]).wait()

    def wo_copy(k):
        return pltpu.make_async_copy(
            wo_hbm.at[pl.ds(k * 512, 512), :], wostage.at[k], sems.at[SWO + k])

    def xlead_copy(q):
        return pltpu.make_async_copy(
            x_hbm.at[:, pl.ds(0, M), pl.ds(q * KQ, KQ)], xlead.at[q], sems.at[SXL + q])

    x_cp = pltpu.make_async_copy(
        x_hbm.at[:, pl.ds(M, SEG - M), :], xbuf.at[:, pl.ds(M, SEG - M), :], sems.at[SX])

    def h_copy(c):
        return pltpu.make_async_copy(
            ssmk_hbm.at[:, pl.ds(c * C, C)], hbuf.at[c], sems.at[SH])

    def a_copy(t, g):
        return pltpu.make_async_copy(
            a_hbms[t].at[:, pl.ds(g * 128, 128)], abuf.at[g, t], sems.at[SA + g])

    small = [pltpu.make_async_copy(src, dst, sems.at[SS + i]) for i, (src, dst) in enumerate((
        (fwd_hbm, fwd_ref), (inv_hbm, inv_ref), (fill_hbm, fill_ref),
        (mem0_hbm, mem0_ref), (sk_hbm, sk_ref), (ssmd_hbm, ssmd_ref.at[0])))]

    for q in range(4):
        xlead_copy(q).start()
        w_copy(0, 2 * q).start()
        w_copy(0, 2 * q + 1).start()
        for k in {0: (), 1: (0, 1), 2: (2, 3), 3: (4, 5, 6, 7)}[q]:
            w_copy(1, k).start()

    kf[pl.ds(0, KPAD), :] = jnp.zeros((KPAD, 128), U32)
    for b in range(2):
        gbuf[b, pl.ds(0, 7)] = jnp.zeros((7, 2 * C, 128), F32)

    w_parts = (w_a, w_b)

    def slab_row(m, par, jl):
        return (m * 16 + par * 8 + jl) * SLAB

    def gated(x, i, n, gates):
        if gates is None or not cfg["gate"]:
            return x
        never, vals = gates
        v = vals[(i * len(vals) * 3) // (n * 4)]
        return jnp.where(never, pltpu.bitcast(v, U32), x)

    def vregs(*mats):
        return [m_[r:r + 8] for m_ in mats for r in range(0, m_.shape[0], 8)]

    def relayout_piece(c, k, gates=None, slot=None):
        slot = (c % 2) * 8 + k if slot is None else slot
        dst = w_parts[c % 2]
        base = slab_row(c // 2, 0, 0) + k * 64
        for i in range(64):
            a = gated(pltpu.bitcast(wstage[slot, 2 * i], U32), i, 64, gates)
            b = pltpu.bitcast(wstage[slot, 2 * i + 1], U32)
            ev = (a & jnp.uint32(0xFFFF)) | (b << 16)
            od = (a >> 16) | (b & jnp.uint32(0xFFFF0000))
            dst[pl.ds(base + i, 8, stride=SLAB), :] = ev
            dst[pl.ds(base + 8 * SLAB + i, 8, stride=SLAB), :] = od

    def comb(x, y, sign):
        f = (lambda a, b: a + b) if sign > 0 else (lambda a, b: a - b)
        return _pack(f(_unpack(x, 0), _unpack(y, 0)), f(_unpack(x, 1), _unpack(y, 1)))

    HR = NSEG * M // 4

    def batch_pair(c, jl):
        m, g = c // 2, c % 2
        it = m * NPAIR + 8 * g + jl
        rows = [pl.multiple_of(slab_row(m, par, jl), 8) for par in range(2)]
        if not cfg["strassen"]:
            xl = jnp.concatenate([pltpu.bitcast(xlead_u[q], BF16) for q in range(4)], axis=1)
            outs = [_dot(xl, pltpu.bitcast(w_parts[g][pl.ds(r, D // 2), :], BF16)) for r in rows]
            qkvb[:, it] = _pack(outs[0], outs[1]).reshape(NSEG, M, DH)
            return vregs(*outs)
        def blk(kh, par):
            return w_parts[g][pl.ds(rows[par] + kh * (D // 4), D // 4), :]

        def mm(a, b):
            return _dot(pltpu.bitcast(jnp.concatenate(a, axis=1), BF16), pltpu.bitcast(b, BF16))

        def xs(f):
            return [xs_u[f, q] for q in range(2)]
        a11 = [xlead_u[q, pl.ds(0, HR), :] for q in (0, 1)]
        a22 = [xlead_u[q, pl.ds(HR, HR), :] for q in (2, 3)]
        m5 = mm(xs(2), blk(1, 1))
        m1 = mm(xs(0), comb(blk(0, 0), blk(1, 1), 1))
        m4 = mm(a22, comb(blk(1, 0), blk(0, 0), -1))
        c11 = mm(xs(4), comb(blk(1, 0), blk(1, 1), 1)) + (m1 + m4 - m5)
        m3 = mm(a11, comb(blk(0, 1), blk(1, 1), -1))
        qkvb[pl.ds(0, NSEG // 2), it] = _pack(c11, m3 + m5).reshape(NSEG // 2, M, DH)
        m2 = mm(xs(1), blk(0, 0))
        c22 = mm(xs(3), comb(blk(0, 0), blk(0, 1), 1)) + (m1 - m2 + m3)
        qkvb[pl.ds(NSEG // 2, NSEG // 2), it] = _pack(m2 + m4, c22).reshape(NSEG // 2, M, DH)
        return vregs(m5, m1, m4, c11, m3, m2, c22)

    def quarter_prep(q):
        self_wait(xlead.at[q], SXL + q)
        for u in range(2):
            self_wait(wstage.at[2 * q + u], SW + 2 * q + u)
        xq = xlead[q].astype(F32).reshape(NSEG * M, KQ).astype(BF16)
        xlead_u[q] = pltpu.bitcast(xq, U32)
        for u in range(2):
            relayout_piece(0, 2 * q + u)

    def quarter_dot(q, par, j):
        row = slab_row(0, par, j) + q * (KQ // 2)
        row = row if isinstance(row, int) else pl.multiple_of(row, 8)
        w = pltpu.bitcast(w_a[pl.ds(row, KQ // 2), :], BF16)
        return _dot(pltpu.bitcast(xlead_u[q], BF16), w)

    def facc_get(hh):
        return jnp.concatenate([ubuf[0, hh], ubuf[1, hh]], axis=0)

    def quarter(q, carry):
        quarter_prep(q)

        @pl.when(q > 0)
        def _():
            for u in range(2):
                self_wait(wstage.at[6 + 2 * q + u], SW + 6 + 2 * q + u)
        outs = []
        for j in range(8):
            for par in range(2):
                hh = 2 * j + par
                d = quarter_dot(q, par, j) + jnp.where(q == 0, 0.0, facc_get(hh))
                ubuf[0, hh] = d[0:2 * C]
                ubuf[1, hh] = d[2 * C:]
                outs.append(d)
        for u in range(2):
            k = jnp.maximum(2 * q - 2, 0) + u
            relayout_piece(1, k, (q > 1000, vregs(*outs[8 * u:8 * u + 8])),
                           slot=jnp.where(q == 0, u, 8 + k))
        return carry
    loop("quarters", 0, 3, quarter, 0)
    quarter_prep(3)

    def quarter_last(it, carry):
        @pl.when(it == 0)
        def _():
            for k in range(8):
                w_copy(2, k).start()
        for u in range(2):
            self_wait(wstage.at[12 + 2 * it + u], SW + 12 + 2 * it + u)
        res = []
        for u in range(4):
            j = 4 * it + u
            outs = [quarter_dot(3, par, j) + facc_get(2 * j + par) for par in range(2)]
            qkvb[:, j] = _pack(outs[0], outs[1]).reshape(NSEG, M, DH)
            res += outs
        for u in range(2):
            relayout_piece(1, 4 + 2 * it + u, (it > 1000, vregs(*res[4 * u:4 * u + 4])))
        if cfg["strassen"]:
            gates = (it > 1000, vregs(*res))
            for r in range(0, HR, 8):
                for cb in range(2):
                    cols = pl.ds(cb * 128, 128)
                    i = 2 * (r // 8) + cb
                    a11 = gated(xlead_u[it, pl.ds(r, 8), cols], i, HR // 4, gates)
                    a22 = gated(xlead_u[2 + it, pl.ds(HR + r, 8), cols], i, HR // 4, gates)
                    a21, a12 = xlead_u[it, pl.ds(HR + r, 8), cols], xlead_u[2 + it, pl.ds(r, 8), cols]
                    for f, (x, y, sg) in enumerate(((a11, a22, 1), (a21, a22, 1), (a11, a12, 1),
                                                    (a21, a11, -1), (a12, a22, -1))):
                        xs_u[f, it, pl.ds(r, 8), cols] = comb(x, y, sg)
        return carry
    loop("quarter_last", 0, 2, quarter_last, 0)

    PP = cfg["pp"]

    def issue(c):
        if c + 2 < 6:
            for k in range(8):
                w_copy(c + 2, k).start()
        if c < 3:
            for k in range(4 * (c - 1), 4 * c):
                wo_copy(k).start()
        if c == 1:
            for cp in small:
                cp.start()
        if c == 3:
            x_cp.start()
        if c == 4:
            for cc in range(NC):
                h_copy(cc).start()
            for g in range(NG):
                for t in (1, 2, 0):
                    a_copy(t, g).start()

    def wo_relayout(k, gates):
        for r in range(32):
            blk = pltpu.bitcast(wostage[k, pl.ds(r * 16, 16), :], U32)
            row = pl.multiple_of(k * 256 + r * 8, 8)
            for n in range(NB):
                wo_u[n, pl.ds(row, 8), :] = gated(blk[:, n * 128:(n + 1) * 128], r * NB + n, 32 * NB, gates)

    def chunk_body(c, pp, it, carry):
        for u in range(pp):
            k = it * pp + u
            if c < 5:
                slot = ((c + 1) % 2) * 8 + k
                self_wait(wstage.at[slot], SW + slot)
            else:
                self_wait(wostage.at[k], SWO + k)
        for u in range(pp):
            k = it * pp + u
            gates = (it > 1000, batch_pair(c, k))
            if c < 5:
                relayout_piece(c + 1, k, gates)
            else:
                wo_relayout(k, gates)
        if c == 5:
            for gg in range(pp):
                g = it * pp + gg
                sk = sk_ref[g].astype(F32)
                for j in range(KS):
                    taps[g, j] = jnp.broadcast_to(sk[j:j + 1], (8, 128))
            dd = ssmd_ref[0].astype(F32)
            for g in range(NG):
                taps[g, KS] = jnp.broadcast_to(dd[g:g + 1], (8, 128))
        return carry

    for c in range(1, 6):
        issue(c)
        if c == 5:
            for cp in small:
                cp.wait()
        pp = cfg["pp1"] if c == 1 else PP
        loop("chunk%d" % c, 0, 8 // pp, functools.partial(chunk_body, c, pp), 0)
    with scope("xh_wait"):
        x_cp.wait()
        self_wait(hbuf, SH)

    def rep(x, rows):
        return x if rows == 8 else jnp.concatenate([x] * (rows // 8), axis=0)

    def a_stage1_pre(g, p, never, par=None):
        par = g % 2 if par is None else par
        r = p * C if isinstance(p, int) else pl.multiple_of(p * C, C)
        r2 = 2 * r if isinstance(p, int) else pl.multiple_of(2 * r, 2 * C)
        kw = pltpu.bitcast(abuf[g, 1, pl.ds(r2, 2 * C), :], U32)
        vw = pltpu.bitcast(abuf[g, 2, pl.ds(r2, 2 * C), :], U32)
        kf[pl.ds(KPAD + r, C), :] = kw
        t = [taps[g, j] for j in range(KS)]
        parts = {}
        last = None
        mode = cfg["chain1"] if never is not None else 0
        blocks = list(range(0, C, 8))
        if cfg.get("rev1"):
            blocks = [b + h for b in range(C // 2 - 8, -8, -8) for h in (0, C // 2)]
        for b in blocks:
            w0 = kw[b:b + 8]
            w1 = kf[pl.ds(KPAD + r + b - 1, 8), :]
            w2 = kf[pl.ds(KPAD + r + b - 2, 8), :]
            if last is not None and mode == 3:
                w0 = jnp.where(never, last, w0)
                w1 = jnp.where(never, last, w1)
            e0, o0 = _unpack(w0, 0), _unpack(w0, 1)
            e1, o1 = _unpack(w1, 0), _unpack(w1, 1)
            o2 = _unpack(w2, 1)
            ke = e0 * t[0]
            ko = o0 * t[0]
            if last is not None and mode == 1:
                ke = jnp.where(never, last[0], ke)
                ko = jnp.where(never, last[1], ko)
            if last is not None and mode == 2:
                ke = jnp.where(never, last[1], ke)
            ke = (ke + o1 * t[1] + e1 * t[2] + o2 * t[3]) * _unpack(vw[b:b + 8], 0)
            if mode >= 2:
                ko = jnp.where(never, ke, ko)
            ko = (ko + e0 * t[1] + o1 * t[2] + e1 * t[3]) * _unpack(vw[b:b + 8], 1)
            parts[b] = _pack(ke, ko)
            last = parts[b] if mode == 3 else (ke, ko)
        parts = [parts[b] for b in range(0, C, 8)]
        kv = jnp.concatenate(parts, axis=0)
        kvb[par, pl.ds(r, C), :] = kv
        return kv

    def a_stage1_u(g, p, kv):
        fwd = pltpu.bitcast(fwd_ref[...], BF16)
        if kv is None:
            kv = kvb[g % 2, pl.ds(pl.multiple_of(p * C, C), C), :]
        for u in range(2):
            w = pltpu.bitcast(kv[u * C // 2:(u + 1) * C // 2], BF16)
            if cfg["split_u"]:
                for hf in range(2):
                    ubuf[g % 2, 2 * p + u, pl.ds(hf * C, C), :] = _dot(fwd[hf * C:(hf + 1) * C], w)
            else:
                ubuf[g % 2, 2 * p + u] = _dot(fwd, w)

    def a_stage1_h(g, p):
        fwd = pltpu.bitcast(fwd_ref[...], BF16)
        rows = pl.ds(pl.multiple_of(g * 128, 128), 128)
        if cfg["split_h"]:
            hs = [jnp.concatenate([_dot_nt(fwd[hf * C:(hf + 1) * C], hbuf[2 * p + u, rows, :])
                                   for hf in range(2)], axis=0) for u in range(2)]
        else:
            hs = [_dot_nt(fwd, hbuf[2 * p + u, rows, :]) for u in range(2)]
        prev = jnp.where(p == 0, 0.0, hlast[...])
        hlast[...] = hs[1]
        hc = C // 2
        for u, (cur, prv) in enumerate(((hs[0], prev), (hs[1], hs[0]))):
            gbuf[g % 2, 7 + 2 * p + u] = jnp.concatenate([
                cur[0:hc] - prv[C:C + hc], cur[hc:C] + prv[C + hc:],
                cur[C:C + hc] + prv[0:hc], cur[C + hc:] - prv[hc:C]], axis=0)

    def a_stage2(gp, p, slot, chain, never):
        b = gp % 2
        RB = 8
        re = [[], []]
        im = [[], []]
        last = None
        for r in [r0 + blk for r0 in range(0, C // 2, RB) for blk in (0, C // 2)]:
            gr = [gbuf[b, 7 + p + 8 - j, pl.ds(r, RB), :] for j in range(NC)]
            gi = [gbuf[b, 7 + p + 8 - j, pl.ds(C + r, RB), :] for j in range(NC)]
            ur = [ubuf[b, j, pl.ds(r, RB), :] for j in range(NC)]
            ui = [ubuf[b, j, pl.ds(C + r, RB), :] for j in range(NC)]
            for o, (nt, off) in enumerate(((8, 8), (16, 0))):
                if chain == 1:
                    ar = gr[off] * ur[0]
                    ai = gr[off] * ui[0]
                    if last is not None:
                        ar = jnp.where(never, last[0], ar)
                        ai = jnp.where(never, last[1], ai)
                    ar = ar - gi[off] * ui[0]
                    ai = ai + gi[off] * ur[0]
                    for j in range(1, nt):
                        ar = ar + gr[j + off] * ur[j]
                        ai = ai + gr[j + off] * ui[j]
                        ar = ar - gi[j + off] * ui[j]
                        ai = ai + gi[j + off] * ur[j]
                    last = (ar, ai)
                else:
                    ar = gr[off] * ur[0]
                    if last is not None:
                        ar = jnp.where(never, last, ar)
                    ar = ar - gi[off] * ui[0]
                    for j in range(1, nt):
                        ar = ar + gr[j + off] * ur[j]
                        ar = ar - gi[j + off] * ui[j]
                    ai = jnp.where(never, ar, gr[off] * ui[0])
                    ai = ai + gi[off] * ur[0]
                    for j in range(1, nt):
                        ai = ai + gr[j + off] * ui[j]
                        ai = ai + gi[j + off] * ur[j]
                    last = ai
                re[o].append(ar)
                im[o].append(ai)
                if r >= C // 2:
                    rows = pl.ds(r - C // 2, RB)
                    ystage[slot, o, 0, rows, :] = _pack(re[o][-2] + ar, im[o][-2] - ai)
                    ystage[slot, o, 1, rows, :] = _pack(re[o][-2] - ar, im[o][-2] + ai)
        return list(last) if chain == 1 else [last]

    def a_stage3(gp, gq, p, slot):
        inv = pltpu.bitcast(inv_ref[...], BF16)
        dd = rep(taps[gq, KS], C // 2)
        for o in range(2):
            i = p + 8 * o
            kvw = kvb[gp % 2, pl.ds(pl.multiple_of(i * (C // 2), C // 2), C // 2), :]
            qw = pltpu.bitcast(abuf[gq, 0, pl.ds(pl.multiple_of(i * C, C), C), :], U32)
            res = []
            for e in range(2):
                y = _dot(inv[e * (C // 2):(e + 1) * (C // 2)], pltpu.bitcast(ystage[slot, o, e], BF16))
                res.append(_unpack(qw, e) * (y + _unpack(kvw, e) * dd))
            out = pltpu.bitcast(_pack(res[0], res[1]), BF16)
            aout[gq, pl.ds(pl.multiple_of(i * 4, 4), 4)] = out.reshape(4, SEG, 128)

    scale = DH ** (-0.5)

    def w_slab(m, h, z):
        j = h // 2
        row = slab_row(m, h % 2, j % 8)
        row = row if z is None else pl.multiple_of(z + row, 8)
        return pltpu.bitcast(w_parts[j // 8][pl.ds(row, D // 2), :], BF16)

    class Step:
        def __init__(self, s, u):
            self.s = s
            self.slot = u % 2
            self.z = None if (u == 0 or not cfg.get("zoff")) else pl.multiple_of(jnp.where(s > 1000 + u, 32, 0), 32)
            self.g = s // 8
            self.p = s % 8
            self.qkv, self.ps, self.os = {}, {}, []
            self.acc = [None] * NB
            self.ocat = {}
            self.early = {}
            self.ties = []

        def start(self, mem):
            x = xbuf[self.s, pl.ds(M, SEG - M), :].astype(F32)
            self.lhsf = jnp.concatenate([mem, x], axis=0)
            self.lhs = self.lhsf.astype(BF16)

        def proj_early(self, m, j, k):
            self.early[m, j] = (k, [_dot(self.lhsf[:, :k].astype(BF16), w_slab(m, 2 * j + e, self.z)[:k])
                                    for e in range(2)])

        def proj(self, m, j):
            if (m, j) in self.early:
                k, part = self.early[m, j]
                a, b = [_dot(self.lhsf[:, k:].astype(BF16), w_slab(m, 2 * j + e, self.z)[k:]) + part[e]
                        for e in range(2)]
            else:
                a = _dot(self.lhs, w_slab(m, 2 * j, self.z))
                b = _dot(self.lhs, w_slab(m, 2 * j + 1, self.z))
            lead = qkvb[self.s, m * NPAIR + j]
            if m == 0:
                r = jnp.concatenate([a, b, _unpack(lead, 0), _unpack(lead, 1)], axis=0).astype(BF16)
            else:
                r = pltpu.bitcast(jnp.concatenate([_pack(a, b), lead], axis=0), BF16)
            self.qkv[m, j] = r

        def probs(self, j):
            fill = fill_ref[pl.ds(0, R), pl.ds(0, R)]
            sc = jnp.where(fill == 0.0, _dot_nt(self.qkv[0, j], self.qkv[1, j]) * scale, fill)
            mx = jnp.max(sc, axis=-1, keepdims=True)
            e = jnp.exp(sc - mx)
            l = jnp.sum(e, axis=-1, keepdims=True)
            r = pl.reciprocal(l, approx=True)
            r = r * (2.0 - l * r)
            self.ps[j] = (e * r).astype(BF16)

        def attend(self, j):
            o = _dot(self.ps[j], self.qkv[2, j])
            row = pl.multiple_of(self.s * M, M)
            ob[2 * j, pl.ds(row, M), :] = o[2 * SEG:2 * SEG + M].astype(BF16)
            ob[2 * j + 1, pl.ds(row, M), :] = o[2 * SEG + M:].astype(BF16)
            self.os += [o[0:SEG], o[SEG:2 * SEG]]

        def wo(self, h0, h1, ns):
            if (h0, h1) not in self.ocat:
                self.ocat[h0, h1] = jnp.concatenate(self.os[h0:h1], axis=1).astype(BF16)
            o = self.ocat[h0, h1]
            for n in ns:
                row = h0 * 64 if self.z is None else pl.multiple_of(self.z + h0 * 64, 32)
                w = wo_u[n, pl.ds(row, (h1 - h0) * 64), :]
                if cfg["tie"] == n + 1 + (NB if h1 == H else 0):
                    parts = [jnp.where(self.s > 1000, pltpu.bitcast(t, U32), w[8 * i:8 * i + 8])
                             for i, t in enumerate(self.ties)]
                    w = jnp.concatenate(parts + [w[8 * len(parts):]], axis=0)
                d = _dot(o, pltpu.bitcast(w, BF16))
                self.acc[n] = d if self.acc[n] is None else d + self.acc[n]

        def finish(self):
            res = jnp.concatenate(self.acc, axis=1)
            obuf[self.s] = res.astype(BF16)
            return res[0:M]

        def run(self, item):
            kind = item[0]
            g, p = self.g, self.p
            never = (self.s if cfg["real_chain"] else p) > 1000
            if kind == "P":
                self.proj(item[1], item[2])
            elif kind == "E":
                self.proj_early(item[1], item[2], item[3])
            elif kind == "S":
                self.probs(item[1])
            elif kind == "V":
                self.attend(item[1])
            elif kind == "W":
                self.wo(item[1], item[2], item[3])
            elif kind == "A1":
                self.kv = a_stage1_pre(g, p, never)
            elif kind == "AU":
                a_stage1_u(g, p, self.kv)
            elif kind == "AH":
                a_stage1_h(g, p)
            elif kind == "A2":
                a_stage2(g + 1, p, self.slot, cfg["chain"], never)
            elif kind == "A3":
                a_stage3(g + 1, jnp.maximum(g - 1, 0), p, self.slot)
            elif kind == "N1":
                gn = (self.s + 1) // 8
                kv = a_stage1_pre(jnp.minimum(gn, NG - 1), (self.s + 1) % 8, never, gn % 2)
                if cfg["tie"]:
                    self.ties.append(pltpu.bitcast(kv[C - 8:C], F32))
            elif kind == "N2":
                tails = a_stage2((self.s + 1) // 8 + 1, (self.s + 1) % 8, 0, cfg["chain"], never)
                if cfg["tie"]:
                    self.ties += tails
            elif kind == "PU":
                a_stage1_u(g, p, None)
            elif kind == "P3":
                a_stage3(g + 1, jnp.maximum(g - 1, 0), p, 0)

    U, order = _make_order(cfg["order"])
    pipe = any(item[0] == "N1" for _, item in order)
    pipe2 = any(item[0] == "N2" for _, item in order)
    if pipe:
        self_wait(abuf.at[0], SA)
        a_stage1_pre(0, 0, None)

    def steps(i, mem):
        s0 = i * U
        sw = s0 + U if pipe else s0

        @pl.when(jnp.logical_and(sw % 8 == 0, sw < NSEG))
        def _():
            self_wait(abuf.at[sw // 8], SA + sw // 8)
        st = [Step(s0 + u, u) for u in range(U)]
        for u, item in order:
            if item[0] == "start":
                st[u].start(mem)
            elif item[0] == "finish":
                mem = st[u].finish()
            else:
                st[u].run(item)
        return mem

    loop("steps", 0, NSEG // U, steps, mem0_ref[...].astype(F32))

    ob_cp = pltpu.make_async_copy(
        obuf.at[:, pl.ds(M, SEG - M), :],
        out_hbm.at[:, pl.ds(M, SEG - M), pl.ds(D, D)], sems.at[SO])
    ob_cp.start()
    for g in range(NG - 1):
        pltpu.make_async_copy(
            aout.at[g], out_hbm.at[:, :, pl.ds(g * 128, 128)], sems.at[SO + 1]).start()

    EP = cfg["ep"]
    GL = NG - 1
    HS = cfg["ep_split"]

    def epi(it, carry):
        def part(n, h0, h1):
            lhs = jnp.concatenate([ob[h] for h in range(h0, h1)], axis=1)
            return _dot(lhs, pltpu.bitcast(wo_u[n, pl.ds(h0 * 64, (h1 - h0) * 64), :], BF16))
        for u in range(EP):
            n = it * EP + u
            if pipe2:
                a_stage3(GL, GL, n, 0)
                a_stage2(GL, jnp.minimum(n + 1, 7), 0, cfg["ep_chain"], it > 1000)
                d = part(n, 0, H)
            else:
                a_stage2(GL, n, u % 2, cfg["ep_chain"], it > 1000)
                d = part(n, 0, HS)
                a_stage3(GL, GL, n, u % 2)
                d = part(n, HS, H) + d
            obb[n] = d.reshape(NSEG, M, 128).astype(BF16)
        for u in range(EP):
            n = it * EP + u
            col = pl.multiple_of(D + n * 128, 128)
            pltpu.make_async_copy(
                obb.at[n], out_hbm.at[:, pl.ds(0, M), pl.ds(col, 128)], sems.at[SO + 2]).start()
        for o in range(2):
            rows = pl.ds((it * EP + 8 * o) * 4, 4 * EP)
            pltpu.make_async_copy(
                aout.at[GL, rows], out_hbm.at[rows, :, pl.ds(GL * 128, 128)], sems.at[SO + 1]).start()
        return carry
    loop("epi", 0, NB // EP, epi, 0)
    ob_cp.wait()
    self_wait(aout, SO + 1)
    self_wait(obb, SO + 2)


def _b_order(u, extra, o):
    ks = o.get("ks", 24)
    tmpl = [(x[0], int(x[1:])) for x in o.get("tmpl", "q0 v1 S1 k0 V2").split()]
    out = list(extra.get("pre", [])) + [(u, ("start",))]
    if u > 0:
        first = [(kind, t - lag) for t in range(3) for kind, lag in tmpl if kind in "qkv" and t >= lag]
        out += [(u, ("E", "qkv".index(kind), j, o.get("ek", 768))) for kind, j in first[:o.get("ne", 2)]]
    nw = 0
    for t in range(NPAIR + max(l for _, l in tmpl)):
        for kind, lag in tmpl:
            j = t - lag
            if j < 0:
                continue
            if j >= NPAIR:
                if kind in "qkv" and nw < NB:
                    out.append((u, ("W", 0, ks, (nw,))))
                    nw += 1
                continue
            out.append((u, ("P", "qkv".index(kind), j) if kind in "qkv" else (kind, j)))
        out += extra.get(t, [])
    out += extra.get("tail", [])
    out += [(u, ("W", 0, ks, tuple(range(nw, NB))))]
    out += extra.get("tail2", [])
    out += [(u, ("W", ks, H, tuple(range(NB))))]
    out += extra.get("end", [])
    out += [(u, ("finish",))]
    out += extra.get("post", [])
    return out


def _make_order(o):
    out = []
    U = len(o["a"])
    for u, d in enumerate(o["a"]):
        ex = {}
        for k, names in d.items():
            k = int(k) if k.isdigit() else k
            ex[k] = [(u - n.count("-") + n.count("+"), (n.lstrip("+-"),)) for n in names]
        out += _b_order(u, ex, o)
    return U, out


_DEFAULT_CFG = dict(
    order=dict(a=[{"pre": ["A1", "+A1"], "0": ["AH"], "2": ["AU"], "4": ["+AU", "A2"], "16": ["A3"]},
                  {"1": ["AH", "A2"], "14": ["A3"]}],
               tmpl="q0 v1 S1 k0 V2", ks=16, ne=2, ek=768),
    pp=4, ep=2, ep_split=24, ep_chain=1, chain=1, chain1=2, real_chain=1,
    split_u=0, split_h=0, tie=0, strassen=1, gate=1, pp1=2, nobc=0)


def _pack_rows(x):
    b = np.asarray(x, dtype=jnp.bfloat16).view(np.uint16).astype(np.uint32)
    return b[0::2] | (b[1::2] << 16)


def _build(cfg):
    fwd_np, inv_np = _dft_constants()
    fill_np = np.zeros((96, 128), np.float32)
    fill_np[:R, :R] = _mask_fill()

    def run(A_q, A_k, A_v, A_shift_k, A_ssm_k, A_ssm_D, B_x, B_mem0, B_Wq, B_Wk, B_Wv, B_Wo):
        sk = A_shift_k.T.reshape(KS, NG, 128).transpose(1, 0, 2)
        any_spec = pl.BlockSpec(memory_space=pl.ANY)
        out = pl.pallas_call(
            functools.partial(_kernel, cfg),
            out_shape=jax.ShapeDtypeStruct((NSEG, SEG, 2 * D), BF16),
            in_specs=[any_spec] * 15,
            out_specs=any_spec,
            scratch_shapes=[
                pltpu.VMEM((48 * SLAB + 544, 128), U32),
                pltpu.VMEM((48 * SLAB + 544, 128), U32),
                pltpu.VMEM((NB, H * DH // 2, 128), U32),
                pltpu.VMEM((16, 128, 16, DH), BF16),
                pltpu.VMEM((8, 512, D), BF16),
                pltpu.VMEM((NSEG, SEG, D), BF16),
                pltpu.VMEM((4, NSEG, M, KQ), BF16),
                pltpu.VMEM((4, NSEG * M // 2, KQ), U32),
                pltpu.VMEM((5, 2, NSEG * M // 4, KQ), U32),
                pltpu.VMEM((NSEG, 3 * NPAIR, 8, 128), U32),
                pltpu.VMEM((H, NSEG * M, DH), BF16),
                pltpu.VMEM((NSEG, SEG, D), BF16),
                pltpu.VMEM((NB, NSEG, M, 128), BF16),
                pltpu.VMEM((NG, 3, S, 128), BF16),
                pltpu.VMEM((NC, D, C), BF16),
                pltpu.VMEM((S // 2 + KPAD, 128), U32),
                pltpu.VMEM((2, S // 2, 128), U32),
                pltpu.VMEM((2, NC, 2 * C, 128), F32),
                pltpu.VMEM((2, NC + 7, 2 * C, 128), F32),
                pltpu.VMEM((2 * C, 128), F32),
                pltpu.VMEM((NG, NSEG, SEG, 128), BF16),
                pltpu.VMEM((2, 2, 2, C // 2, 128), U32),
                pltpu.VMEM((C, C), U32),
                pltpu.VMEM((C // 2, C), U32),
                pltpu.VMEM((96, 128), F32),
                pltpu.VMEM((NG, 8, 8, 128), F32),
                pltpu.VMEM((M, D), BF16),
                pltpu.VMEM((NG, KS, 128), BF16),
                pltpu.VMEM((4, NG, 128), BF16),
                pltpu.SemaphoreType.DMA((48,)),
            ],
            compiler_params=pltpu.CompilerParams(vmem_limit_bytes=124 * 1024 * 1024,
                                                 disable_bounds_checks=bool(cfg["nobc"])),
        )(A_q.reshape(S, D), A_k.reshape(S, D), A_v.reshape(S, D), sk, A_ssm_k,
          A_ssm_D.reshape(NG, 128), B_x.reshape(NSEG, SEG, D), B_mem0.reshape(M, D),
          B_Wq, B_Wk, B_Wv, B_Wo.reshape(H * DH, D),
          jnp.asarray(_pack_rows(fwd_np)), jnp.asarray(_pack_rows(inv_np)), jnp.asarray(fill_np))
        return out.reshape(1, S, 2 * D)

    return run


@functools.partial(jax.jit, static_argnames=("B_seg_len",))
def pallas_concat_heads__ssm_conv_h3__memory_aug_recurrent_mem_tr__prompt_kernel(
    A_q: jax.Array,
    A_k: jax.Array,
    A_v: jax.Array,
    A_shift_k: jax.Array,
    A_ssm_k: jax.Array,
    A_ssm_D: jax.Array,
    B_x: jax.Array,
    B_mem0: jax.Array,
    B_Wq: jax.Array,
    B_Wk: jax.Array,
    B_Wv: jax.Array,
    B_Wo: jax.Array,
    B_seg_len: int = SEG,
):
    assert B_seg_len == SEG
    return _build(_DEFAULT_CFG)(A_q, A_k, A_v, A_shift_k, A_ssm_k, A_ssm_D, B_x, B_mem0,
                                B_Wq, B_Wk, B_Wv, B_Wo)
```

```python
import functools

import numpy as np
import jax
import jax.numpy as jnp
from jax import lax
import jax.experimental.pallas as pl
import jax.experimental.pallas.tpu as pltpu

F32 = jnp.float32
BF16 = jnp.bfloat16
U32 = jnp.uint32

S = 2048
D = 1024
H = 32
DH = 128
M = 8
SEG = 32
NSEG = S // SEG
NPAIR = H // 2
R = 2 * (M + SEG)
SLAB = 520
KS = 4
C = 128
NC = S // C
NG = D // 128
KQ = D // 4
SPEC = 2 * C + 32
OFF = (0, C + 8, 16, C + 24)
NB = D // 128


def _dft_constants():
    fe = np.arange(0, C, 2)
    f = np.concatenate([fe, C - 1 - fe])
    t = np.arange(C)
    ang = (np.pi * (2 * f + 1) / (2 * C))[:, None] * t[None, :]
    fwd = np.concatenate([np.cos(ang), -np.sin(ang)], axis=0)
    a = ang[:C // 2]
    inv = np.stack([np.cos(a), -np.sin(a)], axis=1).reshape(C, C).T / C
    inv = np.concatenate([inv[0::2], inv[1::2]], axis=0)
    return fwd.astype(np.float32), inv.astype(np.float32)


def _mask_fill():
    blk = np.concatenate([np.arange(M), M + np.arange(M, SEG)])
    lead = M + np.arange(M)
    qhead = np.concatenate([np.zeros(SEG), np.ones(SEG), np.zeros(M), np.ones(M)])
    qpos = np.concatenate([blk, blk, lead, lead])
    khead = np.arange(R) % 2
    kpos = np.concatenate([blk, lead])[np.arange(R) // 2]
    same = qhead[:, None] == khead[None, :]
    ok = (qpos[:, None] < M) | (qpos[:, None] >= kpos[None, :])
    fill = np.where(same, np.where(ok, 0.0, -1e9), -np.inf)
    return fill.astype(np.float32)


def _pack(lo, hi):
    return pltpu.pack_elementwise([lo, hi], packed_dtype=BF16)


def _unpack(w, index):
    return pltpu.unpack_elementwise(w, index=index, packed_dtype=BF16, unpacked_dtype=F32)


def _dot(a, b):
    return jnp.dot(a, b, preferred_element_type=F32)


def _dot_nt(a, b):
    return lax.dot_general(a, b, (((1,), (1,)), ((), ())), preferred_element_type=F32)


def _kernel(cfg,
            aq_hbm, ak_hbm, av_hbm, sk_hbm, ssmk_hbm, ssmd_hbm, x_hbm, mem0_hbm,
            wq_hbm, wk_hbm, wv_hbm, wo_hbm, fwd_hbm, inv_hbm, fill_hbm,
            out_hbm,
            w_a, w_b, wo_u, wstage, wostage, xbuf, xlead, xlead_u, xs_u, qkvb, ob, obuf, obb,
            abuf, hbuf, kvb, ubuf, gbuf, hlast, aout, ystage,
            fwd_ref, inv_ref, fill_ref, taps, mem0_ref, sk_ref, ssmd_ref,
            sems):
    import contextlib
    scope = jax.named_scope if cfg.get("scopes") else (lambda name: contextlib.nullcontext())
    SW, SWO, SXL, SX, SH, SA, SO, SS = 0, 16, 24, 28, 29, 30, 38, 42
    only = cfg.get("only")

    def loop(name, lo, hi, body, init):
        if only is not None and name not in only:
            return init
        if cfg.get("scopes") == 2:
            def body2(i, c):
                with scope(name + "_it"):
                    return body(i, c)
            return lax.fori_loop(lo, hi, body2, init)
        with scope(name):
            return lax.fori_loop(lo, hi, body, init)
    w_hbms = (wq_hbm, wk_hbm, wv_hbm)
    a_hbms = (aq_hbm, ak_hbm, av_hbm)

    def w_copy(c, k):
        m, g = c // 2, c % 2
        slot = (c % 2) * 8 + k
        return pltpu.make_async_copy(
            w_hbms[m].at[pl.ds(k * 128, 128), pl.ds(16 * g, 16), :],
            wstage.at[slot], sems.at[SW + slot])

    def self_wait(ref, sem):
        pltpu.make_async_copy(ref, ref, sems.at[sem]).wait()

    def wo_copy(k):
        return pltpu.make_async_copy(
            wo_hbm.at[pl.ds(k * 512, 512), :], wostage.at[k], sems.at[SWO + k])

    def xlead_copy(q):
        return pltpu.make_async_copy(
            x_hbm.at[:, pl.ds(0, M), pl.ds(q * KQ, KQ)], xlead.at[q], sems.at[SXL + q])

    x_cp = pltpu.make_async_copy(
        x_hbm.at[:, pl.ds(M, SEG - M), :], xbuf.at[:, pl.ds(M, SEG - M), :], sems.at[SX])

    def h_copy(c):
        return pltpu.make_async_copy(
            ssmk_hbm.at[:, pl.ds(c * C, C)], hbuf.at[c], sems.at[SH])

    def a_copy(t, g):
        return pltpu.make_async_copy(
            a_hbms[t].at[:, pl.ds(g * 128, 128)], abuf.at[g, t], sems.at[SA + g])

    small = [pltpu.make_async_copy(src, dst, sems.at[SS + i]) for i, (src, dst) in enumerate((
        (fwd_hbm, fwd_ref), (inv_hbm, inv_ref), (fill_hbm, fill_ref),
        (mem0_hbm, mem0_ref), (sk_hbm, sk_ref), (ssmd_hbm, ssmd_ref.at[0])))]

    for q in range(4):
        xlead_copy(q).start()
        w_copy(0, 2 * q).start()
        w_copy(0, 2 * q + 1).start()
        for k in {0: (), 1: (0, 1), 2: (2, 3), 3: (4, 5, 6, 7)}[q]:
            w_copy(1, k).start()

    for b in range(2):
        gbuf[b, pl.ds(0, 7)] = jnp.zeros((7, SPEC, 128), F32)

    w_parts = (w_a, w_b)

    def slab_row(m, par, jl):
        return (m * 16 + par * 8 + jl) * SLAB

    def gated(x, i, n, gates):
        if gates is None or not cfg["gate"]:
            return x
        never, vals = gates
        v = vals[(i * len(vals) * 3) // (n * 4)]
        return jnp.where(never, pltpu.bitcast(v, U32), x)

    def vregs(*mats):
        return [m_[r:r + 8] for m_ in mats for r in range(0, m_.shape[0], 8)]

    def relayout_piece(c, k, gates=None, slot=None):
        slot = (c % 2) * 8 + k if slot is None else slot
        dst = w_parts[c % 2]
        base = slab_row(c // 2, 0, 0) + k * 64
        for i in range(64):
            a = gated(pltpu.bitcast(wstage[slot, 2 * i], U32), i, 64, gates)
            b = pltpu.bitcast(wstage[slot, 2 * i + 1], U32)
            ev = (a & jnp.uint32(0xFFFF)) | (b << 16)
            od = (a >> 16) | (b & jnp.uint32(0xFFFF0000))
            dst[pl.ds(base + i, 8, stride=SLAB), :] = ev
            dst[pl.ds(base + 8 * SLAB + i, 8, stride=SLAB), :] = od

    def comb(x, y, sign):
        f = (lambda a, b: a + b) if sign > 0 else (lambda a, b: a - b)
        return _pack(f(_unpack(x, 0), _unpack(y, 0)), f(_unpack(x, 1), _unpack(y, 1)))

    HR = NSEG * M // 4

    def batch_pair(c, jl):
        m, g = c // 2, c % 2
        it = m * NPAIR + 8 * g + jl
        rows = [pl.multiple_of(slab_row(m, par, jl), 8) for par in range(2)]
        if not cfg["strassen"]:
            xl = jnp.concatenate([pltpu.bitcast(xlead_u[q], BF16) for q in range(4)], axis=1)
            outs = [_dot(xl, pltpu.bitcast(w_parts[g][pl.ds(r, D // 2), :], BF16)) for r in rows]
            qkvb[:, it] = _pack(outs[0], outs[1]).reshape(NSEG, M, DH)
            return vregs(*outs)
        def blk(kh, par):
            return w_parts[g][pl.ds(rows[par] + kh * (D // 4), D // 4), :]

        def mm(a, b):
            return _dot(pltpu.bitcast(jnp.concatenate(a, axis=1), BF16), pltpu.bitcast(b, BF16))

        def xs(f):
            return [xs_u[f, q] for q in range(2)]
        a11 = [xlead_u[q, pl.ds(0, HR), :] for q in (0, 1)]
        a22 = [xlead_u[q, pl.ds(HR, HR), :] for q in (2, 3)]
        m5 = mm(xs(2), blk(1, 1))
        m1 = mm(xs(0), comb(blk(0, 0), blk(1, 1), 1))
        m4 = mm(a22, comb(blk(1, 0), blk(0, 0), -1))
        c11 = mm(xs(4), comb(blk(1, 0), blk(1, 1), 1)) + (m1 + m4 - m5)
        m3 = mm(a11, comb(blk(0, 1), blk(1, 1), -1))
        qkvb[pl.ds(0, NSEG // 2), it] = _pack(c11, m3 + m5).reshape(NSEG // 2, M, DH)
        m2 = mm(xs(1), blk(0, 0))
        c22 = mm(xs(3), comb(blk(0, 0), blk(0, 1), 1)) + (m1 - m2 + m3)
        qkvb[pl.ds(NSEG // 2, NSEG // 2), it] = _pack(m2 + m4, c22).reshape(NSEG // 2, M, DH)
        return vregs(m5, m1, m4, c11, m3, m2, c22)

    def quarter_prep(q):
        self_wait(xlead.at[q], SXL + q)
        for u in range(2):
            self_wait(wstage.at[2 * q + u], SW + 2 * q + u)
        xq = xlead[q].astype(F32).reshape(NSEG * M, KQ).astype(BF16)
        xlead_u[q] = pltpu.bitcast(xq, U32)
        for u in range(2):
            relayout_piece(0, 2 * q + u)

    def quarter_dot(q, par, j):
        row = slab_row(0, par, j) + q * (KQ // 2)
        row = row if isinstance(row, int) else pl.multiple_of(row, 8)
        w = pltpu.bitcast(w_a[pl.ds(row, KQ // 2), :], BF16)
        return _dot(pltpu.bitcast(xlead_u[q], BF16), w)

    def facc_get(hh):
        return jnp.concatenate([ubuf[b, hh, pl.ds(0, 2 * C), :] for b in range(2)], axis=0)

    def quarter(q, carry):
        quarter_prep(q)

        @pl.when(q > 0)
        def _():
            for u in range(2):
                self_wait(wstage.at[6 + 2 * q + u], SW + 6 + 2 * q + u)
        outs = []
        for j in range(8):
            for par in range(2):
                hh = 2 * j + par
                d = quarter_dot(q, par, j) + jnp.where(q == 0, 0.0, facc_get(hh))
                ubuf[0, hh, pl.ds(0, 2 * C), :] = d[0:2 * C]
                ubuf[1, hh, pl.ds(0, 2 * C), :] = d[2 * C:]
                outs.append(d)
        for u in range(2):
            k = jnp.maximum(2 * q - 2, 0) + u
            relayout_piece(1, k, (q > 1000, vregs(*outs[8 * u:8 * u + 8])),
                           slot=jnp.where(q == 0, u, 8 + k))
        return carry
    loop("quarters", 0, 3, quarter, 0)
    quarter_prep(3)

    def quarter_last(it, carry):
        @pl.when(it == 0)
        def _():
            for k in range(8):
                w_copy(2, k).start()
        for u in range(2):
            self_wait(wstage.at[12 + 2 * it + u], SW + 12 + 2 * it + u)
        res = []
        for u in range(4):
            j = 4 * it + u
            outs = [quarter_dot(3, par, j) + facc_get(2 * j + par) for par in range(2)]
            qkvb[:, j] = _pack(outs[0], outs[1]).reshape(NSEG, M, DH)
            res += outs
        for u in range(2):
            relayout_piece(1, 4 + 2 * it + u, (it > 1000, vregs(*res[4 * u:4 * u + 4])))
        if cfg["strassen"]:
            gates = (it > 1000, vregs(*res))
            for r in range(0, HR, 8):
                for cb in range(2):
                    cols = pl.ds(cb * 128, 128)
                    i = 2 * (r // 8) + cb
                    a11 = gated(xlead_u[it, pl.ds(r, 8), cols], i, HR // 4, gates)
                    a22 = gated(xlead_u[2 + it, pl.ds(HR + r, 8), cols], i, HR // 4, gates)
                    a21, a12 = xlead_u[it, pl.ds(HR + r, 8), cols], xlead_u[2 + it, pl.ds(r, 8), cols]
                    for f, (x, y, sg) in enumerate(((a11, a22, 1), (a21, a22, 1), (a11, a12, 1),
                                                    (a21, a11, -1), (a12, a22, -1))):
                        xs_u[f, it, pl.ds(r, 8), cols] = comb(x, y, sg)
        return carry
    loop("quarter_last", 0, 2, quarter_last, 0)

    PP = cfg["pp"]

    def issue(c):
        if c + 2 < 6:
            for k in range(8):
                w_copy(c + 2, k).start()
        if c < 3:
            for k in range(4 * (c - 1), 4 * c):
                wo_copy(k).start()
        if c == 1:
            for cp in small:
                cp.start()
        if c == 3:
            x_cp.start()
        if c == 4:
            for cc in range(NC):
                h_copy(cc).start()
            for g in range(NG):
                for t in (1, 2, 0):
                    a_copy(t, g).start()

    def wo_relayout(k, gates):
        for r in range(32):
            blk = pltpu.bitcast(wostage[k, pl.ds(r * 16, 16), :], U32)
            row = pl.multiple_of(k * 256 + r * 8, 8)
            for n in range(NB):
                wo_u[n, pl.ds(row, 8), :] = gated(blk[:, n * 128:(n + 1) * 128], r * NB + n, 32 * NB, gates)

    def chunk_body(c, pp, it, carry):
        for u in range(pp):
            k = it * pp + u
            if c < 5:
                slot = ((c + 1) % 2) * 8 + k
                self_wait(wstage.at[slot], SW + slot)
            else:
                self_wait(wostage.at[k], SWO + k)
        for u in range(pp):
            k = it * pp + u
            gates = (it > 1000, batch_pair(c, k))
            if c < 5:
                relayout_piece(c + 1, k, gates)
            else:
                wo_relayout(k, gates)
        if c == 5:
            for gg in range(pp):
                g = it * pp + gg
                sk = sk_ref[g].astype(F32)
                for j in range(KS):
                    taps[g, j] = jnp.broadcast_to(sk[j:j + 1], (8, 128))
            dd = ssmd_ref[0].astype(F32)
            for g in range(NG):
                taps[g, KS] = jnp.broadcast_to(dd[g:g + 1], (8, 128))
        return carry

    for c in range(1, 6):
        issue(c)
        if c == 5:
            for cp in small:
                cp.wait()
        pp = cfg["pp1"] if c == 1 else PP
        loop("chunk%d" % c, 0, 8 // pp, functools.partial(chunk_body, c, pp), 0)
    with scope("xh_wait"):
        x_cp.wait()
        self_wait(hbuf, SH)

    def rep(x, rows):
        return x if rows == 8 else jnp.concatenate([x] * (rows // 8), axis=0)

    def a_stage1_pre(g, p, never, par=None):
        par = g % 2 if par is None else par
        r = p * C if isinstance(p, int) else pl.multiple_of(p * C, C)
        r2 = 2 * r if isinstance(p, int) else pl.multiple_of(2 * r, 2 * C)
        kw = pltpu.bitcast(abuf[g, 1, pl.ds(r2, 2 * C), :], U32)
        vw = pltpu.bitcast(abuf[g, 2, pl.ds(r2, 2 * C), :], U32)
        if isinstance(p, int):
            assert p == 0
            halo = jnp.zeros((8, 128), U32)
        else:
            rh = pl.multiple_of(jnp.maximum(r2 - 16, 0), 16)
            halo = jnp.where(p == 0, jnp.uint32(0), pltpu.bitcast(abuf[g, 1, pl.ds(rh, 16), :], U32))
        sub = lax.broadcasted_iota(jnp.int32, (8, 128), 0)
        blk = [halo] + [kw[b:b + 8] for b in range(0, C, 8)]
        rolled = {sh: [pltpu.roll(x, sh, 0) for x in blk] for sh in (1, 2)}

        def shifted(b, sh):
            return jnp.where(sub < sh, rolled[sh][b // 8], rolled[sh][b // 8 + 1])
        t = [taps[g, j] for j in range(KS)]
        parts = {}
        last = None
        mode = cfg["chain1"] if never is not None else 0
        blocks = list(range(0, C, 8))
        if cfg.get("rev1"):
            blocks = [b + h for b in range(C // 2 - 8, -8, -8) for h in (0, C // 2)]
        for b in blocks:
            w0 = kw[b:b + 8]
            w1 = shifted(b, 1)
            w2 = shifted(b, 2)
            if last is not None and mode == 3:
                w0 = jnp.where(never, last, w0)
                w1 = jnp.where(never, last, w1)
            e0, o0 = _unpack(w0, 0), _unpack(w0, 1)
            e1, o1 = _unpack(w1, 0), _unpack(w1, 1)
            o2 = _unpack(w2, 1)
            ke = e0 * t[0]
            ko = o0 * t[0]
            if last is not None and mode == 1:
                ke = jnp.where(never, last[0], ke)
                ko = jnp.where(never, last[1], ko)
            if last is not None and mode == 2:
                ke = jnp.where(never, last[1], ke)
            ke = (ke + o1 * t[1] + e1 * t[2] + o2 * t[3]) * _unpack(vw[b:b + 8], 0)
            if mode >= 2:
                ko = jnp.where(never, ke, ko)
            ko = (ko + e0 * t[1] + o1 * t[2] + e1 * t[3]) * _unpack(vw[b:b + 8], 1)
            parts[b] = _pack(ke, ko)
            last = parts[b] if mode == 3 else (ke, ko)
        parts = [parts[b] for b in range(0, C, 8)]
        kv = jnp.concatenate(parts, axis=0)
        kvb[par, pl.ds(r, C), :] = kv
        return kv

    def a_stage1_u(g, p, kv):
        fwd = pltpu.bitcast(fwd_ref[...], BF16)
        if kv is None:
            kv = kvb[g % 2, pl.ds(pl.multiple_of(p * C, C), C), :]
        for u in range(2):
            w = pltpu.bitcast(kv[u * C // 2:(u + 1) * C // 2], BF16)
            if cfg["split_u"]:
                for hf in range(2):
                    ubuf[g % 2, 2 * p + u, pl.ds(OFF[hf], C), :] = _dot(fwd[hf * C:(hf + 1) * C], w)
            else:
                d = _dot(fwd, w)
                for hf in range(2):
                    ubuf[g % 2, 2 * p + u, pl.ds(OFF[hf], C), :] = d[hf * C:(hf + 1) * C]

    def a_stage1_h(g, p):
        fwd = pltpu.bitcast(fwd_ref[...], BF16)
        rows = pl.ds(pl.multiple_of(g * 128, 128), 128)
        if cfg["split_h"]:
            hs = [jnp.concatenate([_dot_nt(fwd[hf * C:(hf + 1) * C], hbuf[2 * p + u, rows, :])
                                   for hf in range(2)], axis=0) for u in range(2)]
        else:
            hs = [_dot_nt(fwd, hbuf[2 * p + u, rows, :]) for u in range(2)]
        prev = jnp.where(p == 0, 0.0, hlast[...])
        hlast[...] = hs[1]
        hc = C // 2
        for u, (cur, prv) in enumerate(((hs[0], prev), (hs[1], hs[0]))):
            gbuf[g % 2, 7 + 2 * p + u, pl.ds(OFF[2], C), :] = jnp.concatenate(
                [cur[0:hc] - prv[C:C + hc], cur[hc:C] + prv[C + hc:]], axis=0)
            gbuf[g % 2, 7 + 2 * p + u, pl.ds(OFF[3], C), :] = jnp.concatenate(
                [cur[C:C + hc] + prv[0:hc], cur[C + hc:] - prv[hc:C]], axis=0)

    def a_stage2(gp, p, slot, chain, never):
        b = gp % 2
        RB = 8
        re = [[], []]
        im = [[], []]
        last = None
        for r in [r0 + blk for r0 in range(0, C // 2, RB) for blk in (0, C // 2)]:
            gr = [gbuf[b, 7 + p + 8 - j, pl.ds(OFF[2] + r, RB), :] for j in range(NC)]
            gi = [gbuf[b, 7 + p + 8 - j, pl.ds(OFF[3] + r, RB), :] for j in range(NC)]
            ur = [ubuf[b, j, pl.ds(OFF[0] + r, RB), :] for j in range(NC)]
            ui = [ubuf[b, j, pl.ds(OFF[1] + r, RB), :] for j in range(NC)]
            for o, (nt, off) in enumerate(((8, 8), (16, 0))):
                if chain == 1:
                    ar = gr[off] * ur[0]
                    ai = gr[off] * ui[0]
                    if last is not None:
                        ar = jnp.where(never, last[0], ar)
                        ai = jnp.where(never, last[1], ai)
                    ar = ar - gi[off] * ui[0]
                    ai = ai + gi[off] * ur[0]
                    for j in range(1, nt):
                        ar = ar + gr[j + off] * ur[j]
                        ai = ai + gr[j + off] * ui[j]
                        ar = ar - gi[j + off] * ui[j]
                        ai = ai + gi[j + off] * ur[j]
                    last = (ar, ai)
                else:
                    ar = gr[off] * ur[0]
                    if last is not None:
                        ar = jnp.where(never, last, ar)
                    ar = ar - gi[off] * ui[0]
                    for j in range(1, nt):
                        ar = ar + gr[j + off] * ur[j]
                        ar = ar - gi[j + off] * ui[j]
                    ai = jnp.where(never, ar, gr[off] * ui[0])
                    ai = ai + gi[off] * ur[0]
                    for j in range(1, nt):
                        ai = ai + gr[j + off] * ui[j]
                        ai = ai + gi[j + off] * ur[j]
                    last = ai
                re[o].append(ar)
                im[o].append(ai)
                if r >= C // 2:
                    rows = pl.ds(r - C // 2, RB)
                    ystage[slot, o, 0, rows, :] = _pack(re[o][-2] + ar, im[o][-2] - ai)
                    ystage[slot, o, 1, rows, :] = _pack(re[o][-2] - ar, im[o][-2] + ai)
        return list(last) if chain == 1 else [last]

    def a_stage3(gp, gq, p, slot):
        inv = pltpu.bitcast(inv_ref[...], BF16)
        dd = rep(taps[gq, KS], C // 2)
        for o in range(2):
            i = p + 8 * o
            kvw = kvb[gp % 2, pl.ds(pl.multiple_of(i * (C // 2), C // 2), C // 2), :]
            qw = pltpu.bitcast(abuf[gq, 0, pl.ds(pl.multiple_of(i * C, C), C), :], U32)
            res = []
            for e in range(2):
                y = _dot(inv[e * (C // 2):(e + 1) * (C // 2)], pltpu.bitcast(ystage[slot, o, e], BF16))
                res.append(_unpack(qw, e) * (y + _unpack(kvw, e) * dd))
            out = pltpu.bitcast(_pack(res[0], res[1]), BF16)
            aout[gq, pl.ds(pl.multiple_of(i * 4, 4), 4)] = out.reshape(4, SEG, 128)

    scale = DH ** (-0.5)

    def w_slab(m, h, z):
        j = h // 2
        row = slab_row(m, h % 2, j % 8)
        row = row if z is None else pl.multiple_of(z + row, 8)
        return pltpu.bitcast(w_parts[j // 8][pl.ds(row, D // 2), :], BF16)

    class Step:
        def __init__(self, s, u):
            self.s = s
            self.slot = u % 2
            self.z = None if (u == 0 or not cfg.get("zoff")) else pl.multiple_of(jnp.where(s > 1000 + u, 32, 0), 32)
            self.g = s // 8
            self.p = s % 8
            self.qkv, self.ps, self.os = {}, {}, []
            self.acc = [None] * NB
            self.ocat = {}
            self.early = {}
            self.ties = []

        def start(self, mem):
            x = xbuf[self.s, pl.ds(M, SEG - M), :].astype(F32)
            self.lhsf = jnp.concatenate([mem, x], axis=0)
            self.lhs = self.lhsf.astype(BF16)

        def proj_early(self, m, j, k):
            self.early[m, j] = (k, [_dot(self.lhsf[:, :k].astype(BF16), w_slab(m, 2 * j + e, self.z)[:k])
                                    for e in range(2)])

        def proj(self, m, j):
            if (m, j) in self.early:
                k, part = self.early[m, j]
                a, b = [_dot(self.lhsf[:, k:].astype(BF16), w_slab(m, 2 * j + e, self.z)[k:]) + part[e]
                        for e in range(2)]
            else:
                a = _dot(self.lhs, w_slab(m, 2 * j, self.z))
                b = _dot(self.lhs, w_slab(m, 2 * j + 1, self.z))
            lead = qkvb[self.s, m * NPAIR + j]
            if m == 0:
                r = jnp.concatenate([a, b, _unpack(lead, 0), _unpack(lead, 1)], axis=0).astype(BF16)
            else:
                r = pltpu.bitcast(jnp.concatenate([_pack(a, b), lead], axis=0), BF16)
            self.qkv[m, j] = r

        def probs(self, j):
            fill = fill_ref[pl.ds(0, R), pl.ds(0, R)]
            sc = jnp.where(fill == 0.0, _dot_nt(self.qkv[0, j], self.qkv[1, j]) * scale, fill)
            mx = jnp.max(sc, axis=-1, keepdims=True)
            e = jnp.exp(sc - mx)
            l = jnp.sum(e, axis=-1, keepdims=True)
            r = pl.reciprocal(l, approx=True)
            r = r * (2.0 - l * r)
            self.ps[j] = (e * r).astype(BF16)

        def attend(self, j):
            o = _dot(self.ps[j], self.qkv[2, j])
            row = pl.multiple_of(self.s * M, M)
            ob[2 * j, pl.ds(row, M), :] = o[2 * SEG:2 * SEG + M].astype(BF16)
            ob[2 * j + 1, pl.ds(row, M), :] = o[2 * SEG + M:].astype(BF16)
            self.os += [o[0:SEG], o[SEG:2 * SEG]]

        def wo(self, h0, h1, ns):
            if (h0, h1) not in self.ocat:
                self.ocat[h0, h1] = jnp.concatenate(self.os[h0:h1], axis=1).astype(BF16)
            o = self.ocat[h0, h1]
            for n in ns:
                row = h0 * 64 if self.z is None else pl.multiple_of(self.z + h0 * 64, 32)
                w = wo_u[n, pl.ds(row, (h1 - h0) * 64), :]
                if cfg["tie"] == n + 1 + (NB if h1 == H else 0):
                    parts = [jnp.where(self.s > 1000, pltpu.bitcast(t, U32), w[8 * i:8 * i + 8])
                             for i, t in enumerate(self.ties)]
                    w = jnp.concatenate(parts + [w[8 * len(parts):]], axis=0)
                d = _dot(o, pltpu.bitcast(w, BF16))
                self.acc[n] = d if self.acc[n] is None else d + self.acc[n]

        def finish(self):
            res = jnp.concatenate(self.acc, axis=1)
            obuf[self.s] = res.astype(BF16)
            return res[0:M]

        def run(self, item):
            kind = item[0]
            g, p = self.g, self.p
            never = (self.s if cfg["real_chain"] else p) > 1000
            if kind == "P":
                self.proj(item[1], item[2])
            elif kind == "E":
                self.proj_early(item[1], item[2], item[3])
            elif kind == "S":
                self.probs(item[1])
            elif kind == "V":
                self.attend(item[1])
            elif kind == "W":
                self.wo(item[1], item[2], item[3])
            elif kind == "A1":
                self.kv = a_stage1_pre(g, p, never)
            elif kind == "AU":
                a_stage1_u(g, p, self.kv)
            elif kind == "AH":
                a_stage1_h(g, p)
            elif kind == "A2":
                a_stage2(g + 1, p, self.slot, cfg["chain"], never)
            elif kind == "A3":
                a_stage3(g + 1, jnp.maximum(g - 1, 0), p, self.slot)
            elif kind == "N1":
                gn = (self.s + 1) // 8
                kv = a_stage1_pre(jnp.minimum(gn, NG - 1), (self.s + 1) % 8, never, gn % 2)
                if cfg["tie"]:
                    self.ties.append(pltpu.bitcast(kv[C - 8:C], F32))
            elif kind == "N2":
                tails = a_stage2((self.s + 1) // 8 + 1, (self.s + 1) % 8, 0, cfg["chain"], never)
                if cfg["tie"]:
                    self.ties += tails
            elif kind == "PU":
                a_stage1_u(g, p, None)
            elif kind == "P3":
                a_stage3(g + 1, jnp.maximum(g - 1, 0), p, 0)

    U, order = _make_order(cfg["order"])
    pipe = any(item[0] == "N1" for _, item in order)
    pipe2 = any(item[0] == "N2" for _, item in order)
    if pipe:
        self_wait(abuf.at[0], SA)
        a_stage1_pre(0, 0, None)

    def steps(i, mem):
        s0 = i * U
        sw = s0 + U if pipe else s0

        @pl.when(jnp.logical_and(sw % 8 == 0, sw < NSEG))
        def _():
            self_wait(abuf.at[sw // 8], SA + sw // 8)
        st = [Step(s0 + u, u) for u in range(U)]
        for u, item in order:
            if item[0] == "start":
                st[u].start(mem)
            elif item[0] == "finish":
                mem = st[u].finish()
            else:
                st[u].run(item)
        return mem

    loop("steps", 0, NSEG // U, steps, mem0_ref[...].astype(F32))

    ob_cp = pltpu.make_async_copy(
        obuf.at[:, pl.ds(M, SEG - M), :],
        out_hbm.at[:, pl.ds(M, SEG - M), pl.ds(D, D)], sems.at[SO])
    ob_cp.start()
    for g in range(NG - 1):
        pltpu.make_async_copy(
            aout.at[g], out_hbm.at[:, :, pl.ds(g * 128, 128)], sems.at[SO + 1]).start()

    EP = cfg["ep"]
    GL = NG - 1
    HS = cfg["ep_split"]

    def epi(it, carry):
        def part(n, h0, h1):
            lhs = jnp.concatenate([ob[h] for h in range(h0, h1)], axis=1)
            return _dot(lhs, pltpu.bitcast(wo_u[n, pl.ds(h0 * 64, (h1 - h0) * 64), :], BF16))
        for u in range(EP):
            n = it * EP + u
            if pipe2:
                a_stage3(GL, GL, n, 0)
                a_stage2(GL, jnp.minimum(n + 1, 7), 0, cfg["ep_chain"], it > 1000)
                d = part(n, 0, H)
            else:
                a_stage2(GL, n, u % 2, cfg["ep_chain"], it > 1000)
                d = part(n, 0, HS)
                a_stage3(GL, GL, n, u % 2)
                d = part(n, HS, H) + d
            obb[n] = d.reshape(NSEG, M, 128).astype(BF16)
        for u in range(EP):
            n = it * EP + u
            col = pl.multiple_of(D + n * 128, 128)
            pltpu.make_async_copy(
                obb.at[n], out_hbm.at[:, pl.ds(0, M), pl.ds(col, 128)], sems.at[SO + 2]).start()
        for o in range(2):
            rows = pl.ds((it * EP + 8 * o) * 4, 4 * EP)
            pltpu.make_async_copy(
                aout.at[GL, rows], out_hbm.at[rows, :, pl.ds(GL * 128, 128)], sems.at[SO + 1]).start()
        return carry
    loop("epi", 0, NB // EP, epi, 0)
    ob_cp.wait()
    self_wait(aout, SO + 1)
    self_wait(obb, SO + 2)


def _b_order(u, extra, o):
    ks = o.get("ks", 24)
    tmpl = [(x[0], int(x[1:])) for x in o.get("tmpl", "q0 v1 S1 k0 V2").split()]
    out = list(extra.get("pre", [])) + [(u, ("start",))]
    if u > 0:
        first = [(kind, t - lag) for t in range(3) for kind, lag in tmpl if kind in "qkv" and t >= lag]
        out += [(u, ("E", "qkv".index(kind), j, o.get("ek", 768))) for kind, j in first[:o.get("ne", 2)]]
    nw = 0
    for t in range(NPAIR + max(l for _, l in tmpl)):
        for kind, lag in tmpl:
            j = t - lag
            if j < 0:
                continue
            if j >= NPAIR:
                if kind in "qkv" and nw < NB:
                    out.append((u, ("W", 0, ks, (nw,))))
                    nw += 1
                continue
            out.append((u, ("P", "qkv".index(kind), j) if kind in "qkv" else (kind, j)))
        out += extra.get(t, [])
    out += extra.get("tail", [])
    out += [(u, ("W", 0, ks, tuple(range(nw, NB))))]
    out += extra.get("tail2", [])
    out += [(u, ("W", ks, H, tuple(range(NB))))]
    out += extra.get("end", [])
    out += [(u, ("finish",))]
    out += extra.get("post", [])
    return out


def _make_order(o):
    out = []
    U = len(o["a"])
    for u, d in enumerate(o["a"]):
        ex = {}
        for k, names in d.items():
            k = int(k) if k.isdigit() else k
            ex[k] = [(u - n.count("-") + n.count("+"), (n.lstrip("+-"),)) for n in names]
        out += _b_order(u, ex, o)
    return U, out


_DEFAULT_CFG = dict(
    order=dict(a=[{"pre": ["A1", "+A1"], "0": ["AH"], "2": ["AU"], "4": ["+AU", "A2"], "16": ["A3"]},
                  {"1": ["AH", "A2"], "14": ["A3"]}],
               tmpl="q0 v1 S1 k0 V2", ks=16, ne=2, ek=768),
    pp=4, ep=2, ep_split=24, ep_chain=1, chain=1, chain1=2, real_chain=1,
    split_u=0, split_h=0, tie=0, strassen=1, gate=1, pp1=2, nobc=0)


def _pack_rows(x):
    b = np.asarray(x, dtype=jnp.bfloat16).view(np.uint16).astype(np.uint32)
    return b[0::2] | (b[1::2] << 16)


def _build(cfg):
    fwd_np, inv_np = _dft_constants()
    fill_np = np.zeros((96, 128), np.float32)
    fill_np[:R, :R] = _mask_fill()

    def run(A_q, A_k, A_v, A_shift_k, A_ssm_k, A_ssm_D, B_x, B_mem0, B_Wq, B_Wk, B_Wv, B_Wo):
        sk = A_shift_k.T.reshape(KS, NG, 128).transpose(1, 0, 2)
        any_spec = pl.BlockSpec(memory_space=pl.ANY)
        out = pl.pallas_call(
            functools.partial(_kernel, cfg),
            out_shape=jax.ShapeDtypeStruct((NSEG, SEG, 2 * D), BF16),
            in_specs=[any_spec] * 15,
            out_specs=any_spec,
            scratch_shapes=[
                pltpu.VMEM((48 * SLAB + 544, 128), U32),
                pltpu.VMEM((48 * SLAB + 544, 128), U32),
                pltpu.VMEM((NB, H * DH // 2, 128), U32),
                pltpu.VMEM((16, 128, 16, DH), BF16),
                pltpu.VMEM((8, 512, D), BF16),
                pltpu.VMEM((NSEG, SEG, D), BF16),
                pltpu.VMEM((4, NSEG, M, KQ), BF16),
                pltpu.VMEM((4, NSEG * M // 2, KQ), U32),
                pltpu.VMEM((5, 2, NSEG * M // 4, KQ), U32),
                pltpu.VMEM((NSEG, 3 * NPAIR, 8, 128), U32),
                pltpu.VMEM((H, NSEG * M, DH), BF16),
                pltpu.VMEM((NSEG, SEG, D), BF16),
                pltpu.VMEM((NB, NSEG, M, 128), BF16),
                pltpu.VMEM((NG, 3, S, 128), BF16),
                pltpu.VMEM((NC, D, C), BF16),
                pltpu.VMEM((2, S // 2, 128), U32),
                pltpu.VMEM((2, NC, SPEC, 128), F32),
                pltpu.VMEM((2, NC + 7, SPEC, 128), F32),
                pltpu.VMEM((2 * C, 128), F32),
                pltpu.VMEM((NG, NSEG, SEG, 128), BF16),
                pltpu.VMEM((2, 2, 2, C // 2, 128), U32),
                pltpu.VMEM((C, C), U32),
                pltpu.VMEM((C // 2, C), U32),
                pltpu.VMEM((96, 128), F32),
                pltpu.VMEM((NG, 8, 8, 128), F32),
                pltpu.VMEM((M, D), BF16),
                pltpu.VMEM((NG, KS, 128), BF16),
                pltpu.VMEM((4, NG, 128), BF16),
                pltpu.SemaphoreType.DMA((48,)),
            ],
            compiler_params=pltpu.CompilerParams(vmem_limit_bytes=124 * 1024 * 1024,
                                                 disable_bounds_checks=bool(cfg["nobc"])),
        )(A_q.reshape(S, D), A_k.reshape(S, D), A_v.reshape(S, D), sk, A_ssm_k,
          A_ssm_D.reshape(NG, 128), B_x.reshape(NSEG, SEG, D), B_mem0.reshape(M, D),
          B_Wq, B_Wk, B_Wv, B_Wo.reshape(H * DH, D),
          jnp.asarray(_pack_rows(fwd_np)), jnp.asarray(_pack_rows(inv_np)), jnp.asarray(fill_np))
        return out.reshape(1, S, 2 * D)

    return run


@functools.partial(jax.jit, static_argnames=("B_seg_len",))
def pallas_concat_heads__ssm_conv_h3__memory_aug_recurrent_mem_tr__prompt_kernel(
    A_q: jax.Array,
    A_k: jax.Array,
    A_v: jax.Array,
    A_shift_k: jax.Array,
    A_ssm_k: jax.Array,
    A_ssm_D: jax.Array,
    B_x: jax.Array,
    B_mem0: jax.Array,
    B_Wq: jax.Array,
    B_Wk: jax.Array,
    B_Wv: jax.Array,
    B_Wo: jax.Array,
    B_seg_len: int = SEG,
):
    assert B_seg_len == SEG
    return _build(_DEFAULT_CFG)(A_q, A_k, A_v, A_shift_k, A_ssm_k, A_ssm_D, B_x, B_mem0,
                                B_Wq, B_Wk, B_Wv, B_Wo)
```

```python
import functools

import numpy as np
import jax
import jax.numpy as jnp
from jax import lax
import jax.experimental.pallas as pl
import jax.experimental.pallas.tpu as pltpu

F32 = jnp.float32
BF16 = jnp.bfloat16
U32 = jnp.uint32

S = 2048
D = 1024
H = 32
DH = 128
M = 8
SEG = 32
NSEG = S // SEG
NPAIR = H // 2
R = 2 * (M + SEG)
SLAB = 520
KS = 4
C = 128
NC = S // C
NG = D // 128
KQ = D // 4
SPEC = 2 * C + 32
OFF = (0, C + 8, 16, C + 24)
NB = D // 128


def _dft_constants():
    fe = np.arange(0, C, 2)
    f = np.concatenate([fe, C - 1 - fe])
    t = np.arange(C)
    ang = (np.pi * (2 * f + 1) / (2 * C))[:, None] * t[None, :]
    fwd = np.concatenate([np.cos(ang), -np.sin(ang)], axis=0)
    a = ang[:C // 2]
    inv = np.stack([np.cos(a), -np.sin(a)], axis=1).reshape(C, C).T / C
    inv = np.concatenate([inv[0::2], inv[1::2]], axis=0)
    return fwd.astype(np.float32), inv.astype(np.float32)


def _mask_fill():
    blk = np.concatenate([np.arange(M), M + np.arange(M, SEG)])
    lead = M + np.arange(M)
    qhead = np.concatenate([np.zeros(SEG), np.ones(SEG), np.zeros(M), np.ones(M)])
    qpos = np.concatenate([blk, blk, lead, lead])
    khead = np.arange(R) % 2
    kpos = np.concatenate([blk, lead])[np.arange(R) // 2]
    same = qhead[:, None] == khead[None, :]
    ok = (qpos[:, None] < M) | (qpos[:, None] >= kpos[None, :])
    fill = np.where(same, np.where(ok, 0.0, -1e9), -np.inf)
    return fill.astype(np.float32)


def _pack(lo, hi):
    return pltpu.pack_elementwise([lo, hi], packed_dtype=BF16)


def _unpack(w, index):
    return pltpu.unpack_elementwise(w, index=index, packed_dtype=BF16, unpacked_dtype=F32)


def _dot(a, b):
    return jnp.dot(a, b, preferred_element_type=F32)


def _dot_nt(a, b):
    return lax.dot_general(a, b, (((1,), (1,)), ((), ())), preferred_element_type=F32)


def _kernel(cfg,
            aq_hbm, ak_hbm, av_hbm, sk_hbm, ssmk_hbm, ssmd_hbm, x_hbm, mem0_hbm,
            wq_hbm, wk_hbm, wv_hbm, wo_hbm, fwd_hbm, inv_hbm, fill_hbm,
            out_hbm,
            w_a, w_b, wo_u, wstage, wostage, xbuf, xlead, xlead_u, xs_u, qkvb, ob, obuf, obb,
            abuf, hbuf, kvb, ubuf, gbuf, hlast, aout, ystage,
            fwd_ref, inv_ref, fill_ref, taps, mem0_ref, sk_ref, ssmd_ref,
            sems):
    import contextlib
    scope = jax.named_scope if cfg.get("scopes") else (lambda name: contextlib.nullcontext())
    SW, SWO, SXL, SX, SH, SA, SO, SS = 0, 16, 24, 28, 29, 30, 38, 42
    only = cfg.get("only")

    def loop(name, lo, hi, body, init):
        if only is not None and name not in only:
            return init
        if cfg.get("scopes") == 2:
            def body2(i, c):
                with scope(name + "_it"):
                    return body(i, c)
            return lax.fori_loop(lo, hi, body2, init)
        with scope(name):
            return lax.fori_loop(lo, hi, body, init)
    w_hbms = (wq_hbm, wk_hbm, wv_hbm)
    a_hbms = (aq_hbm, ak_hbm, av_hbm)

    def w_copy(c, k):
        m, g = c // 2, c % 2
        slot = (c % 2) * 8 + k
        return pltpu.make_async_copy(
            w_hbms[m].at[pl.ds(k * 128, 128), pl.ds(16 * g, 16), :],
            wstage.at[slot], sems.at[SW + slot])

    def self_wait(ref, sem):
        pltpu.make_async_copy(ref, ref, sems.at[sem]).wait()

    def wo_copy(k):
        return pltpu.make_async_copy(
            wo_hbm.at[pl.ds(k * 512, 512), :], wostage.at[k], sems.at[SWO + k])

    def xlead_copy(q):
        return pltpu.make_async_copy(
            x_hbm.at[:, pl.ds(0, M), pl.ds(q * KQ, KQ)], xlead.at[q], sems.at[SXL + q])

    x_cp = pltpu.make_async_copy(
        x_hbm.at[:, pl.ds(M, SEG - M), :], xbuf.at[:, pl.ds(M, SEG - M), :], sems.at[SX])

    def h_copy(c):
        return pltpu.make_async_copy(
            ssmk_hbm.at[:, pl.ds(c * C, C)], hbuf.at[c], sems.at[SH])

    def a_copy(t, g):
        return pltpu.make_async_copy(
            a_hbms[t].at[:, pl.ds(g * 128, 128)], abuf.at[g, t], sems.at[SA + g])

    small = [pltpu.make_async_copy(src, dst, sems.at[SS + i]) for i, (src, dst) in enumerate((
        (fwd_hbm, fwd_ref), (inv_hbm, inv_ref), (fill_hbm, fill_ref),
        (mem0_hbm, mem0_ref), (sk_hbm, sk_ref), (ssmd_hbm, ssmd_ref.at[0])))]

    for q in range(4):
        xlead_copy(q).start()
        w_copy(0, 2 * q).start()
        w_copy(0, 2 * q + 1).start()
        for k in {0: (), 1: (0, 1), 2: (2, 3), 3: (4, 5, 6, 7)}[q]:
            w_copy(1, k).start()

    for b in range(2):
        gbuf[b, pl.ds(0, 7)] = jnp.zeros((7, SPEC, 128), F32)

    w_parts = (w_a, w_b)

    def slab_row(m, par, jl):
        return (m * 16 + par * 8 + jl) * SLAB

    def gated(x, i, n, gates):
        if gates is None or not cfg["gate"]:
            return x
        never, vals = gates
        v = vals[(i * len(vals) * 3) // (n * 4)]
        return jnp.where(never, pltpu.bitcast(v, U32), x)

    def vregs(*mats):
        return [m_[r:r + 8] for m_ in mats for r in range(0, m_.shape[0], 8)]

    def relayout_piece(c, k, gates=None, slot=None):
        slot = (c % 2) * 8 + k if slot is None else slot
        dst = w_parts[c % 2]
        base = slab_row(c // 2, 0, 0) + k * 64
        for i in range(64):
            a = gated(pltpu.bitcast(wstage[slot, 2 * i], U32), i, 64, gates)
            b = pltpu.bitcast(wstage[slot, 2 * i + 1], U32)
            ev = (a & jnp.uint32(0xFFFF)) | (b << 16)
            od = (a >> 16) | (b & jnp.uint32(0xFFFF0000))
            dst[pl.ds(base + i, 8, stride=SLAB), :] = ev
            dst[pl.ds(base + 8 * SLAB + i, 8, stride=SLAB), :] = od

    def comb(x, y, sign):
        f = (lambda a, b: a + b) if sign > 0 else (lambda a, b: a - b)
        return _pack(f(_unpack(x, 0), _unpack(y, 0)), f(_unpack(x, 1), _unpack(y, 1)))

    HR = NSEG * M // 4

    def batch_pair(c, jl):
        m, g = c // 2, c % 2
        it = m * NPAIR + 8 * g + jl
        rows = [pl.multiple_of(slab_row(m, par, jl), 8) for par in range(2)]
        if not cfg["strassen"]:
            xl = jnp.concatenate([pltpu.bitcast(xlead_u[q], BF16) for q in range(4)], axis=1)
            outs = [_dot(xl, pltpu.bitcast(w_parts[g][pl.ds(r, D // 2), :], BF16)) for r in rows]
            qkvb[:, it] = _pack(outs[0], outs[1]).reshape(NSEG, M, DH)
            return vregs(*outs)
        def blk(kh, par):
            return w_parts[g][pl.ds(rows[par] + kh * (D // 4), D // 4), :]

        def mm(a, b):
            return _dot(pltpu.bitcast(jnp.concatenate(a, axis=1), BF16), pltpu.bitcast(b, BF16))

        def xs(f):
            return [xs_u[f, q] for q in range(2)]
        a11 = [xlead_u[q, pl.ds(0, HR), :] for q in (0, 1)]
        a22 = [xlead_u[q, pl.ds(HR, HR), :] for q in (2, 3)]
        m5 = mm(xs(2), blk(1, 1))
        m1 = mm(xs(0), comb(blk(0, 0), blk(1, 1), 1))
        m4 = mm(a22, comb(blk(1, 0), blk(0, 0), -1))
        c11 = mm(xs(4), comb(blk(1, 0), blk(1, 1), 1)) + (m1 + m4 - m5)
        m3 = mm(a11, comb(blk(0, 1), blk(1, 1), -1))
        qkvb[pl.ds(0, NSEG // 2), it] = _pack(c11, m3 + m5).reshape(NSEG // 2, M, DH)
        m2 = mm(xs(1), blk(0, 0))
        c22 = mm(xs(3), comb(blk(0, 0), blk(0, 1), 1)) + (m1 - m2 + m3)
        qkvb[pl.ds(NSEG // 2, NSEG // 2), it] = _pack(m2 + m4, c22).reshape(NSEG // 2, M, DH)
        return vregs(m5, m1, m4, c11, m3, m2, c22)

    def quarter_prep(q):
        self_wait(xlead.at[q], SXL + q)
        for u in range(2):
            self_wait(wstage.at[2 * q + u], SW + 2 * q + u)
        xq = xlead[q].astype(F32).reshape(NSEG * M, KQ).astype(BF16)
        xlead_u[q] = pltpu.bitcast(xq, U32)
        for u in range(2):
            relayout_piece(0, 2 * q + u)

    def quarter_dot(q, par, j):
        row = slab_row(0, par, j) + q * (KQ // 2)
        row = row if isinstance(row, int) else pl.multiple_of(row, 8)
        w = pltpu.bitcast(w_a[pl.ds(row, KQ // 2), :], BF16)
        return _dot(pltpu.bitcast(xlead_u[q], BF16), w)

    def facc_get(hh):
        return jnp.concatenate([ubuf[b, hh, pl.ds(0, 2 * C), :] for b in range(2)], axis=0)

    def quarter(q, carry):
        quarter_prep(q)

        @pl.when(q > 0)
        def _():
            for u in range(2):
                self_wait(wstage.at[6 + 2 * q + u], SW + 6 + 2 * q + u)
        outs = []
        for j in range(8):
            for par in range(2):
                hh = 2 * j + par
                d = quarter_dot(q, par, j) + jnp.where(q == 0, 0.0, facc_get(hh))
                ubuf[0, hh, pl.ds(0, 2 * C), :] = d[0:2 * C]
                ubuf[1, hh, pl.ds(0, 2 * C), :] = d[2 * C:]
                outs.append(d)
        for u in range(2):
            k = jnp.maximum(2 * q - 2, 0) + u
            relayout_piece(1, k, (q > 1000, vregs(*outs[8 * u:8 * u + 8])),
                           slot=jnp.where(q == 0, u, 8 + k))
        return carry
    loop("quarters", 0, 3, quarter, 0)
    quarter_prep(3)

    def quarter_last(it, carry):
        @pl.when(it == 0)
        def _():
            for k in range(8):
                w_copy(2, k).start()
        for u in range(2):
            self_wait(wstage.at[12 + 2 * it + u], SW + 12 + 2 * it + u)
        res = []
        for u in range(4):
            j = 4 * it + u
            outs = [quarter_dot(3, par, j) + facc_get(2 * j + par) for par in range(2)]
            qkvb[:, j] = _pack(outs[0], outs[1]).reshape(NSEG, M, DH)
            res += outs
        for u in range(2):
            relayout_piece(1, 4 + 2 * it + u, (it > 1000, vregs(*res[4 * u:4 * u + 4])))
        if cfg["strassen"]:
            gates = (it > 1000, vregs(*res))
            for r in range(0, HR, 8):
                for cb in range(2):
                    cols = pl.ds(cb * 128, 128)
                    i = 2 * (r // 8) + cb
                    a11 = gated(xlead_u[it, pl.ds(r, 8), cols], i, HR // 4, gates)
                    a22 = gated(xlead_u[2 + it, pl.ds(HR + r, 8), cols], i, HR // 4, gates)
                    a21, a12 = xlead_u[it, pl.ds(HR + r, 8), cols], xlead_u[2 + it, pl.ds(r, 8), cols]
                    for f, (x, y, sg) in enumerate(((a11, a22, 1), (a21, a22, 1), (a11, a12, 1),
                                                    (a21, a11, -1), (a12, a22, -1))):
                        xs_u[f, it, pl.ds(r, 8), cols] = comb(x, y, sg)
        return carry
    loop("quarter_last", 0, 2, quarter_last, 0)

    PP = cfg["pp"]

    def issue(c):
        if c + 2 < 6:
            for k in range(8):
                w_copy(c + 2, k).start()
        if c < 3:
            for k in range(4 * (c - 1), 4 * c):
                wo_copy(k).start()
        if c == 1:
            for cp in small:
                cp.start()
        if c == 3:
            x_cp.start()
        if c == 4:
            for cc in range(NC):
                h_copy(cc).start()
            for g in range(NG):
                for t in (1, 2, 0):
                    a_copy(t, g).start()

    def wo_relayout(k, gates):
        for r in range(32):
            blk = pltpu.bitcast(wostage[k, pl.ds(r * 16, 16), :], U32)
            row = pl.multiple_of(k * 256 + r * 8, 8)
            for n in range(NB):
                wo_u[n, pl.ds(row, 8), :] = gated(blk[:, n * 128:(n + 1) * 128], r * NB + n, 32 * NB, gates)

    def chunk_body(c, pp, it, carry):
        for u in range(pp):
            k = it * pp + u
            if c < 5:
                slot = ((c + 1) % 2) * 8 + k
                self_wait(wstage.at[slot], SW + slot)
            else:
                self_wait(wostage.at[k], SWO + k)
        for u in range(pp):
            k = it * pp + u
            gates = (it > 1000, batch_pair(c, k))
            if c < 5:
                relayout_piece(c + 1, k, gates)
            else:
                wo_relayout(k, gates)
        if c == 5:
            for gg in range(pp):
                g = it * pp + gg
                sk = sk_ref[g].astype(F32)
                for j in range(KS):
                    taps[g, j] = jnp.broadcast_to(sk[j:j + 1], (8, 128))
            dd = ssmd_ref[0].astype(F32)
            for g in range(NG):
                taps[g, KS] = jnp.broadcast_to(dd[g:g + 1], (8, 128))
        return carry

    for c in range(1, 6):
        issue(c)
        if c == 5:
            for cp in small:
                cp.wait()
        pp = cfg["pp1"] if c == 1 else PP
        loop("chunk%d" % c, 0, 8 // pp, functools.partial(chunk_body, c, pp), 0)
    with scope("xh_wait"):
        x_cp.wait()
        self_wait(hbuf, SH)

    def rep(x, rows):
        return x if rows == 8 else jnp.concatenate([x] * (rows // 8), axis=0)

    def a_stage1_pre(g, p, never, par=None):
        par = g % 2 if par is None else par
        r = p * C if isinstance(p, int) else pl.multiple_of(p * C, C)
        r2 = 2 * r if isinstance(p, int) else pl.multiple_of(2 * r, 2 * C)
        kw = pltpu.bitcast(abuf[g, 1, pl.ds(r2, 2 * C), :], U32)
        vw = pltpu.bitcast(abuf[g, 2, pl.ds(r2, 2 * C), :], U32)
        if isinstance(p, int):
            assert p == 0
            halo = jnp.zeros((8, 128), U32)
        else:
            rh = pl.multiple_of(jnp.maximum(r2 - 16, 0), 16)
            halo = jnp.where(p == 0, jnp.uint32(0), pltpu.bitcast(abuf[g, 1, pl.ds(rh, 16), :], U32))
        sub = lax.broadcasted_iota(jnp.int32, (8, 128), 0)
        blk = [halo] + [kw[b:b + 8] for b in range(0, C, 8)]
        rolled = {sh: [pltpu.roll(x, sh, 0) for x in blk] for sh in (1, 2)}

        def shifted(b, sh):
            return jnp.where(sub < sh, rolled[sh][b // 8], rolled[sh][b // 8 + 1])
        t = [taps[g, j] for j in range(KS)]
        parts = {}
        last = None
        mode = cfg["chain1"] if never is not None else 0
        blocks = list(range(0, C, 8))
        if cfg.get("rev1"):
            blocks = [b + h for b in range(C // 2 - 8, -8, -8) for h in (0, C // 2)]
        for b in blocks:
            w0 = kw[b:b + 8]
            w1 = shifted(b, 1)
            w2 = shifted(b, 2)
            if last is not None and mode == 3:
                w0 = jnp.where(never, last, w0)
                w1 = jnp.where(never, last, w1)
            e0, o0 = _unpack(w0, 0), _unpack(w0, 1)
            e1, o1 = _unpack(w1, 0), _unpack(w1, 1)
            o2 = _unpack(w2, 1)
            ke = e0 * t[0]
            ko = o0 * t[0]
            if last is not None and mode == 1:
                ke = jnp.where(never, last[0], ke)
                ko = jnp.where(never, last[1], ko)
            if last is not None and mode == 2:
                ke = jnp.where(never, last[1], ke)
            ke = (ke + o1 * t[1] + e1 * t[2] + o2 * t[3]) * _unpack(vw[b:b + 8], 0)
            if mode >= 2:
                ko = jnp.where(never, ke, ko)
            ko = (ko + e0 * t[1] + o1 * t[2] + e1 * t[3]) * _unpack(vw[b:b + 8], 1)
            parts[b] = _pack(ke, ko)
            last = parts[b] if mode == 3 else (ke, ko)
        parts = [parts[b] for b in range(0, C, 8)]
        kv = jnp.concatenate(parts, axis=0)
        kvb[par, pl.ds(r, C), :] = kv
        return kv

    def a_stage1_u(g, p, kv):
        fwd = pltpu.bitcast(fwd_ref[...], BF16)
        if kv is None:
            kv = kvb[g % 2, pl.ds(pl.multiple_of(p * C, C), C), :]
        for u in range(2):
            w = pltpu.bitcast(kv[u * C // 2:(u + 1) * C // 2], BF16)
            if cfg["split_u"]:
                for hf in range(2):
                    ubuf[g % 2, 2 * p + u, pl.ds(OFF[hf], C), :] = _dot(fwd[hf * C:(hf + 1) * C], w)
            else:
                d = _dot(fwd, w)
                for hf in range(2):
                    ubuf[g % 2, 2 * p + u, pl.ds(OFF[hf], C), :] = d[hf * C:(hf + 1) * C]

    def a_stage1_h(g, p):
        fwd = pltpu.bitcast(fwd_ref[...], BF16)
        rows = pl.ds(pl.multiple_of(g * 128, 128), 128)
        if cfg["split_h"]:
            hs = [jnp.concatenate([_dot_nt(fwd[hf * C:(hf + 1) * C], hbuf[2 * p + u, rows, :])
                                   for hf in range(2)], axis=0) for u in range(2)]
        else:
            hs = [_dot_nt(fwd, hbuf[2 * p + u, rows, :]) for u in range(2)]
        prev = jnp.where(p == 0, 0.0, hlast[...])
        hlast[...] = hs[1]
        hc = C // 2
        for u, (cur, prv) in enumerate(((hs[0], prev), (hs[1], hs[0]))):
            gbuf[g % 2, 7 + 2 * p + u, pl.ds(OFF[2], C), :] = jnp.concatenate(
                [cur[0:hc] - prv[C:C + hc], cur[hc:C] + prv[C + hc:]], axis=0)
            gbuf[g % 2, 7 + 2 * p + u, pl.ds(OFF[3], C), :] = jnp.concatenate(
                [cur[C:C + hc] + prv[0:hc], cur[C + hc:] - prv[hc:C]], axis=0)

    def a_stage2(gp, p, slot, chain, never):
        b = gp % 2
        RB = 8
        re = [[], []]
        im = [[], []]
        last = None
        for r in [r0 + blk for r0 in range(0, C // 2, RB) for blk in (0, C // 2)]:
            gr = [gbuf[b, 7 + p + 8 - j, pl.ds(OFF[2] + r, RB), :] for j in range(NC)]
            gi = [gbuf[b, 7 + p + 8 - j, pl.ds(OFF[3] + r, RB), :] for j in range(NC)]
            ur = [ubuf[b, j, pl.ds(OFF[0] + r, RB), :] for j in range(NC)]
            ui = [ubuf[b, j, pl.ds(OFF[1] + r, RB), :] for j in range(NC)]
            for o, (nt, off) in enumerate(((8, 8), (16, 0))):
                if chain == 1:
                    ar = gr[off] * ur[0]
                    ai = gr[off] * ui[0]
                    if last is not None:
                        ar = jnp.where(never, last[0], ar)
                        ai = jnp.where(never, last[1], ai)
                    ar = ar - gi[off] * ui[0]
                    ai = ai + gi[off] * ur[0]
                    for j in range(1, nt):
                        ar = ar + gr[j + off] * ur[j]
                        ai = ai + gr[j + off] * ui[j]
                        ar = ar - gi[j + off] * ui[j]
                        ai = ai + gi[j + off] * ur[j]
                    last = (ar, ai)
                else:
                    ar = gr[off] * ur[0]
                    if last is not None:
                        ar = jnp.where(never, last, ar)
                    ar = ar - gi[off] * ui[0]
                    for j in range(1, nt):
                        ar = ar + gr[j + off] * ur[j]
                        ar = ar - gi[j + off] * ui[j]
                    ai = jnp.where(never, ar, gr[off] * ui[0])
                    ai = ai + gi[off] * ur[0]
                    for j in range(1, nt):
                        ai = ai + gr[j + off] * ui[j]
                        ai = ai + gi[j + off] * ur[j]
                    last = ai
                re[o].append(ar)
                im[o].append(ai)
                if r >= C // 2:
                    rows = pl.ds(r - C // 2, RB)
                    ystage[slot, o, 0, rows, :] = _pack(re[o][-2] + ar, im[o][-2] - ai)
                    ystage[slot, o, 1, rows, :] = _pack(re[o][-2] - ar, im[o][-2] + ai)
        return list(last) if chain == 1 else [last]

    def a_stage3(gp, gq, p, slot):
        inv = pltpu.bitcast(inv_ref[...], BF16)
        dd = rep(taps[gq, KS], C // 2)
        for o in range(2):
            i = p + 8 * o
            kvw = kvb[gp % 2, pl.ds(pl.multiple_of(i * (C // 2), C // 2), C // 2), :]
            qw = pltpu.bitcast(abuf[gq, 0, pl.ds(pl.multiple_of(i * C, C), C), :], U32)
            res = []
            for e in range(2):
                y = _dot(inv[e * (C // 2):(e + 1) * (C // 2)], pltpu.bitcast(ystage[slot, o, e], BF16))
                res.append(_unpack(qw, e) * (y + _unpack(kvw, e) * dd))
            out = pltpu.bitcast(_pack(res[0], res[1]), BF16)
            aout[gq, pl.ds(pl.multiple_of(i * 4, 4), 4)] = out.reshape(4, SEG, 128)

    scale = DH ** (-0.5)

    def w_slab(m, h, z):
        j = h // 2
        row = slab_row(m, h % 2, j % 8)
        row = row if z is None else pl.multiple_of(z + row, 8)
        return pltpu.bitcast(w_parts[j // 8][pl.ds(row, D // 2), :], BF16)

    class Step:
        def __init__(self, s, u):
            self.s = s
            self.slot = u % 2
            self.z = None if (u == 0 or not cfg.get("zoff")) else pl.multiple_of(jnp.where(s > 1000 + u, 32, 0), 32)
            self.g = s // 8
            self.p = s % 8
            self.qkv, self.ps, self.os = {}, {}, []
            self.acc = [None] * NB
            self.ocat = {}
            self.lead = {}
            self.prev = None
            self.early = {}
            self.ties = []

        def start(self, mem):
            x = xbuf[self.s, pl.ds(M, SEG - M), :].astype(F32)
            self.lhsf = jnp.concatenate([mem, x], axis=0)
            self.lhs = self.lhsf.astype(BF16)

        def proj_early(self, m, j, k):
            self.early[m, j] = (k, [_dot(self.lhsf[:, :k].astype(BF16), w_slab(m, 2 * j + e, self.z)[:k])
                                    for e in range(2)])

        def proj(self, m, j):
            if (m, j) in self.early:
                k, part = self.early[m, j]
                a, b = [_dot(self.lhsf[:, k:].astype(BF16), w_slab(m, 2 * j + e, self.z)[k:]) + part[e]
                        for e in range(2)]
            else:
                a = _dot(self.lhs, w_slab(m, 2 * j, self.z))
                b = _dot(self.lhs, w_slab(m, 2 * j + 1, self.z))
            lead = qkvb[self.s, m * NPAIR + j]
            if m == 0:
                r = jnp.concatenate([a, b, _unpack(lead, 0), _unpack(lead, 1)], axis=0).astype(BF16)
            else:
                r = pltpu.bitcast(jnp.concatenate([_pack(a, b), lead], axis=0), BF16)
            self.qkv[m, j] = r

        def probs(self, j):
            fill = fill_ref[pl.ds(0, R), pl.ds(0, R)]
            sc = jnp.where(fill == 0.0, _dot_nt(self.qkv[0, j], self.qkv[1, j]) * scale, fill)
            mx = jnp.max(sc, axis=-1, keepdims=True)
            e = jnp.exp(sc - mx)
            l = jnp.sum(e, axis=-1, keepdims=True)
            r = pl.reciprocal(l, approx=True)
            r = r * (2.0 - l * r)
            self.ps[j] = (e * r).astype(BF16)

        def attend(self, j):
            o = _dot(self.ps[j], self.qkv[2, j])
            la, lb = o[2 * SEG:2 * SEG + M], o[2 * SEG + M:]
            if cfg["strassen_e"]:
                rows = pl.ds(pl.multiple_of((self.s // 2) * M, M), M)
                if self.prev is None:
                    self.lead[j] = (la, lb)
                    forms = {2: la + lb, 5: la}
                else:
                    a11, a12 = self.prev.lead[j]
                    forms = {0: a11 + lb, 1: la + lb, 3: la - a11, 4: a12 - lb, 6: lb}
                for f, v in forms.items():
                    ob[f * NPAIR + j, rows, :] = v.astype(BF16)
            else:
                rows = pl.ds(pl.multiple_of(self.s * M, M), M)
                ob[2 * j, rows, :] = la.astype(BF16)
                ob[2 * j + 1, rows, :] = lb.astype(BF16)
            self.os += [o[0:SEG], o[SEG:2 * SEG]]

        def wo(self, h0, h1, ns):
            if (h0, h1) not in self.ocat:
                self.ocat[h0, h1] = jnp.concatenate(self.os[h0:h1], axis=1).astype(BF16)
            o = self.ocat[h0, h1]
            for n in ns:
                row = h0 * 64 if self.z is None else pl.multiple_of(self.z + h0 * 64, 32)
                w = wo_u[n, pl.ds(row, (h1 - h0) * 64), :]
                if cfg["tie"] == n + 1 + (NB if h1 == H else 0):
                    parts = [jnp.where(self.s > 1000, pltpu.bitcast(t, U32), w[8 * i:8 * i + 8])
                             for i, t in enumerate(self.ties)]
                    w = jnp.concatenate(parts + [w[8 * len(parts):]], axis=0)
                d = _dot(o, pltpu.bitcast(w, BF16))
                self.acc[n] = d if self.acc[n] is None else d + self.acc[n]

        def finish(self):
            res = jnp.concatenate(self.acc, axis=1)
            obuf[self.s] = res.astype(BF16)
            return res[0:M]

        def run(self, item):
            kind = item[0]
            g, p = self.g, self.p
            never = (self.s if cfg["real_chain"] else p) > 1000
            if kind == "P":
                self.proj(item[1], item[2])
            elif kind == "E":
                self.proj_early(item[1], item[2], item[3])
            elif kind == "S":
                self.probs(item[1])
            elif kind == "V":
                self.attend(item[1])
            elif kind == "W":
                self.wo(item[1], item[2], item[3])
            elif kind == "A1":
                self.kv = a_stage1_pre(g, p, never)
            elif kind == "AU":
                a_stage1_u(g, p, self.kv)
            elif kind == "AH":
                a_stage1_h(g, p)
            elif kind == "A2":
                a_stage2(g + 1, p, self.slot, cfg["chain"], never)
            elif kind == "A3":
                a_stage3(g + 1, jnp.maximum(g - 1, 0), p, self.slot)
            elif kind == "N1":
                gn = (self.s + 1) // 8
                kv = a_stage1_pre(jnp.minimum(gn, NG - 1), (self.s + 1) % 8, never, gn % 2)
                if cfg["tie"]:
                    self.ties.append(pltpu.bitcast(kv[C - 8:C], F32))
            elif kind == "N2":
                tails = a_stage2((self.s + 1) // 8 + 1, (self.s + 1) % 8, 0, cfg["chain"], never)
                if cfg["tie"]:
                    self.ties += tails
            elif kind == "PU":
                a_stage1_u(g, p, None)
            elif kind == "P3":
                a_stage3(g + 1, jnp.maximum(g - 1, 0), p, 0)

    U, order = _make_order(cfg["order"])
    pipe = any(item[0] == "N1" for _, item in order)
    pipe2 = any(item[0] == "N2" for _, item in order)
    if pipe:
        self_wait(abuf.at[0], SA)
        a_stage1_pre(0, 0, None)

    def steps(i, mem):
        s0 = i * U
        sw = s0 + U if pipe else s0

        @pl.when(jnp.logical_and(sw % 8 == 0, sw < NSEG))
        def _():
            self_wait(abuf.at[sw // 8], SA + sw // 8)
        st = [Step(s0 + u, u) for u in range(U)]
        for u in range(1, U, 2):
            st[u].prev = st[u - 1]
        for u, item in order:
            if item[0] == "start":
                st[u].start(mem)
            elif item[0] == "finish":
                mem = st[u].finish()
            else:
                st[u].run(item)
        return mem

    loop("steps", 0, NSEG // U, steps, mem0_ref[...].astype(F32))

    ob_cp = pltpu.make_async_copy(
        obuf.at[:, pl.ds(M, SEG - M), :],
        out_hbm.at[:, pl.ds(M, SEG - M), pl.ds(D, D)], sems.at[SO])
    ob_cp.start()
    for g in range(NG - 1):
        pltpu.make_async_copy(
            aout.at[g], out_hbm.at[:, :, pl.ds(g * 128, 128)], sems.at[SO + 1]).start()

    EP = cfg["ep"]
    GL = NG - 1
    HS = cfg["ep_split"]

    def epi_strassen(it):
        never = it > 1000
        ns = [2 * it, 2 * it + 1]

        def blk(hp, u):
            return [wo_u[ns[u], pl.ds((2 * j + hp) * 64, 64), :] for j in range(NPAIR)]

        def mm(f, bs):
            lhs = jnp.concatenate([ob[f * NPAIR + j] for j in range(NPAIR)], axis=1)
            return _dot(lhs, pltpu.bitcast(jnp.concatenate(bs, axis=0), BF16))

        def cb(x, y, sign):
            return [comb(a, b, sign) for a, b in zip(x, y)]

        def put(u, par, c):
            for i in range(NSEG // 2):
                obb[ns[u], 2 * i + par] = c[M * i:M * i + M].astype(BF16)
        sched = cfg["ep_sched"]

        def hook(k):
            for u in range(2):
                if sched[u] == k:
                    a_stage3(GL, GL, ns[u], u)
        for u in range(2):
            a_stage2(GL, ns[u], u, cfg["ep_chain"], never)
        m5 = mm(2, blk(1, 1))
        m1 = mm(0, cb(blk(0, 0), blk(1, 1), 1))
        hook(2)
        m4 = mm(6, cb(blk(1, 0), blk(0, 0), -1))
        hook(3)
        put(0, 0, mm(4, cb(blk(1, 0), blk(1, 1), 1)) + (m1 + m4 - m5))
        hook(4)
        m3 = mm(5, cb(blk(0, 1), blk(1, 1), -1))
        put(1, 0, m3 + m5)
        hook(5)
        m2 = mm(1, blk(0, 0))
        put(0, 1, m2 + m4)
        hook(6)
        put(1, 1, mm(3, cb(blk(0, 0), blk(0, 1), 1)) + (m1 - m2 + m3))

    def epi(it, carry):
        def part(n, h0, h1):
            lhs = jnp.concatenate([ob[h] for h in range(h0, h1)], axis=1)
            return _dot(lhs, pltpu.bitcast(wo_u[n, pl.ds(h0 * 64, (h1 - h0) * 64), :], BF16))
        if cfg["strassen_e"]:
            assert EP == 2 and U % 2 == 0 and not pipe2
            epi_strassen(it)
        for u in range(0 if cfg["strassen_e"] else EP):
            n = it * EP + u
            if pipe2:
                a_stage3(GL, GL, n, 0)
                a_stage2(GL, jnp.minimum(n + 1, 7), 0, cfg["ep_chain"], it > 1000)
                d = part(n, 0, H)
            else:
                a_stage2(GL, n, u % 2, cfg["ep_chain"], it > 1000)
                d = part(n, 0, HS)
                a_stage3(GL, GL, n, u % 2)
                d = part(n, HS, H) + d
            obb[n] = d.reshape(NSEG, M, 128).astype(BF16)
        for u in range(EP):
            n = it * EP + u
            col = pl.multiple_of(D + n * 128, 128)
            pltpu.make_async_copy(
                obb.at[n], out_hbm.at[:, pl.ds(0, M), pl.ds(col, 128)], sems.at[SO + 2]).start()
        for o in range(2):
            rows = pl.ds((it * EP + 8 * o) * 4, 4 * EP)
            pltpu.make_async_copy(
                aout.at[GL, rows], out_hbm.at[rows, :, pl.ds(GL * 128, 128)], sems.at[SO + 1]).start()
        return carry
    loop("epi", 0, NB // EP, epi, 0)
    ob_cp.wait()
    self_wait(aout, SO + 1)
    self_wait(obb, SO + 2)


def _b_order(u, extra, o):
    ks = o.get("ks", 24)
    tmpl = [(x[0], int(x[1:])) for x in o.get("tmpl", "q0 v1 S1 k0 V2").split()]
    out = list(extra.get("pre", [])) + [(u, ("start",))]
    if u > 0:
        first = [(kind, t - lag) for t in range(3) for kind, lag in tmpl if kind in "qkv" and t >= lag]
        out += [(u, ("E", "qkv".index(kind), j, o.get("ek", 768))) for kind, j in first[:o.get("ne", 2)]]
    nw = 0
    for t in range(NPAIR + max(l for _, l in tmpl)):
        for kind, lag in tmpl:
            j = t - lag
            if j < 0:
                continue
            if j >= NPAIR:
                if kind in "qkv" and nw < NB:
                    out.append((u, ("W", 0, ks, (nw,))))
                    nw += 1
                continue
            out.append((u, ("P", "qkv".index(kind), j) if kind in "qkv" else (kind, j)))
        out += extra.get(t, [])
    out += extra.get("tail", [])
    out += [(u, ("W", 0, ks, tuple(range(nw, NB))))]
    out += extra.get("tail2", [])
    out += [(u, ("W", ks, H, tuple(range(NB))))]
    out += extra.get("end", [])
    out += [(u, ("finish",))]
    out += extra.get("post", [])
    return out


def _make_order(o):
    out = []
    U = len(o["a"])
    for u, d in enumerate(o["a"]):
        ex = {}
        for k, names in d.items():
            k = int(k) if k.isdigit() else k
            ex[k] = [(u - n.count("-") + n.count("+"), (n.lstrip("+-"),)) for n in names]
        out += _b_order(u, ex, o)
    return U, out


_DEFAULT_CFG = dict(
    order=dict(a=[{"pre": ["A1", "+A1"], "0": ["AH"], "2": ["AU"], "4": ["+AU", "A2"], "16": ["A3"]},
                  {"1": ["AH", "A2"], "14": ["A3"]}],
               tmpl="q0 v1 S1 k0 V2", ks=16, ne=2, ek=768),
    pp=4, ep=2, ep_split=24, ep_chain=1, chain=1, chain1=2, real_chain=1,
    split_u=0, split_h=0, tie=0, strassen=1, gate=1, pp1=2, nobc=0,
    strassen_e=1, ep_sched=(3, 6))


def _pack_rows(x):
    b = np.asarray(x, dtype=jnp.bfloat16).view(np.uint16).astype(np.uint32)
    return b[0::2] | (b[1::2] << 16)


def _build(cfg):
    fwd_np, inv_np = _dft_constants()
    fill_np = np.zeros((96, 128), np.float32)
    fill_np[:R, :R] = _mask_fill()

    def run(A_q, A_k, A_v, A_shift_k, A_ssm_k, A_ssm_D, B_x, B_mem0, B_Wq, B_Wk, B_Wv, B_Wo):
        sk = A_shift_k.T.reshape(KS, NG, 128).transpose(1, 0, 2)
        any_spec = pl.BlockSpec(memory_space=pl.ANY)
        out = pl.pallas_call(
            functools.partial(_kernel, cfg),
            out_shape=jax.ShapeDtypeStruct((NSEG, SEG, 2 * D), BF16),
            in_specs=[any_spec] * 15,
            out_specs=any_spec,
            scratch_shapes=[
                pltpu.VMEM((48 * SLAB + 544, 128), U32),
                pltpu.VMEM((48 * SLAB + 544, 128), U32),
                pltpu.VMEM((NB, H * DH // 2, 128), U32),
                pltpu.VMEM((16, 128, 16, DH), BF16),
                pltpu.VMEM((8, 512, D), BF16),
                pltpu.VMEM((NSEG, SEG, D), BF16),
                pltpu.VMEM((4, NSEG, M, KQ), BF16),
                pltpu.VMEM((4, NSEG * M // 2, KQ), U32),
                pltpu.VMEM((5, 2, NSEG * M // 4, KQ), U32),
                pltpu.VMEM((NSEG, 3 * NPAIR, 8, 128), U32),
                (pltpu.VMEM((7 * NPAIR, NSEG * M // 2, DH), BF16) if cfg["strassen_e"]
                 else pltpu.VMEM((H, NSEG * M, DH), BF16)),
                pltpu.VMEM((NSEG, SEG, D), BF16),
                pltpu.VMEM((NB, NSEG, M, 128), BF16),
                pltpu.VMEM((NG, 3, S, 128), BF16),
                pltpu.VMEM((NC, D, C), BF16),
                pltpu.VMEM((2, S // 2, 128), U32),
                pltpu.VMEM((2, NC, SPEC, 128), F32),
                pltpu.VMEM((2, NC + 7, SPEC, 128), F32),
                pltpu.VMEM((2 * C, 128), F32),
                pltpu.VMEM((NG, NSEG, SEG, 128), BF16),
                pltpu.VMEM((2, 2, 2, C // 2, 128), U32),
                pltpu.VMEM((C, C), U32),
                pltpu.VMEM((C // 2, C), U32),
                pltpu.VMEM((96, 128), F32),
                pltpu.VMEM((NG, 8, 8, 128), F32),
                pltpu.VMEM((M, D), BF16),
                pltpu.VMEM((NG, KS, 128), BF16),
                pltpu.VMEM((4, NG, 128), BF16),
                pltpu.SemaphoreType.DMA((48,)),
            ],
            compiler_params=pltpu.CompilerParams(vmem_limit_bytes=124 * 1024 * 1024,
                                                 disable_bounds_checks=bool(cfg["nobc"])),
        )(A_q.reshape(S, D), A_k.reshape(S, D), A_v.reshape(S, D), sk, A_ssm_k,
          A_ssm_D.reshape(NG, 128), B_x.reshape(NSEG, SEG, D), B_mem0.reshape(M, D),
          B_Wq, B_Wk, B_Wv, B_Wo.reshape(H * DH, D),
          jnp.asarray(_pack_rows(fwd_np)), jnp.asarray(_pack_rows(inv_np)), jnp.asarray(fill_np))
        return out.reshape(1, S, 2 * D)

    return run


@functools.partial(jax.jit, static_argnames=("B_seg_len",))
def pallas_concat_heads__ssm_conv_h3__memory_aug_recurrent_mem_tr__prompt_kernel(
    A_q: jax.Array,
    A_k: jax.Array,
    A_v: jax.Array,
    A_shift_k: jax.Array,
    A_ssm_k: jax.Array,
    A_ssm_D: jax.Array,
    B_x: jax.Array,
    B_mem0: jax.Array,
    B_Wq: jax.Array,
    B_Wk: jax.Array,
    B_Wv: jax.Array,
    B_Wo: jax.Array,
    B_seg_len: int = SEG,
):
    assert B_seg_len == SEG
    return _build(_DEFAULT_CFG)(A_q, A_k, A_v, A_shift_k, A_ssm_k, A_ssm_D, B_x, B_mem0,
                                B_Wq, B_Wk, B_Wv, B_Wo)
```

```python
import functools

import numpy as np
import jax
import jax.numpy as jnp
from jax import lax
import jax.experimental.pallas as pl
import jax.experimental.pallas.tpu as pltpu

F32 = jnp.float32
BF16 = jnp.bfloat16
U32 = jnp.uint32

S = 2048
D = 1024
H = 32
DH = 128
M = 8
SEG = 32
NSEG = S // SEG
NPAIR = H // 2
R = 2 * (M + SEG)
SLAB = 520
KS = 4
C = 128
NC = S // C
NG = D // 128
KQ = D // 4
SPEC = 2 * C + 32
OFF = (0, C + 8, 16, C + 24)
NB = D // 128


def _dft_constants():
    fe = np.arange(0, C, 2)
    f = np.concatenate([fe, C - 1 - fe])
    t = np.arange(C)
    ang = (np.pi * (2 * f + 1) / (2 * C))[:, None] * t[None, :]
    fwd = np.concatenate([np.cos(ang), -np.sin(ang)], axis=0)
    a = ang[:C // 2]
    inv = np.stack([np.cos(a), -np.sin(a)], axis=1).reshape(C, C).T / C
    inv = np.concatenate([inv[0::2], inv[1::2]], axis=0)
    return fwd.astype(np.float32), inv.astype(np.float32)


def _mask_fill():
    blk = np.concatenate([np.arange(M), M + np.arange(M, SEG)])
    lead = M + np.arange(M)
    qhead = np.concatenate([np.zeros(SEG), np.ones(SEG), np.zeros(M), np.ones(M)])
    qpos = np.concatenate([blk, blk, lead, lead])
    khead = np.arange(R) % 2
    kpos = np.concatenate([blk, lead])[np.arange(R) // 2]
    same = qhead[:, None] == khead[None, :]
    ok = (qpos[:, None] < M) | (qpos[:, None] >= kpos[None, :])
    fill = np.where(same, np.where(ok, 0.0, -1e9), -np.inf)
    return fill.astype(np.float32)


def _pack(lo, hi):
    return pltpu.pack_elementwise([lo, hi], packed_dtype=BF16)


def _unpack(w, index):
    return pltpu.unpack_elementwise(w, index=index, packed_dtype=BF16, unpacked_dtype=F32)


def _dot(a, b):
    return jnp.dot(a, b, preferred_element_type=F32)


def _dot_nt(a, b):
    return lax.dot_general(a, b, (((1,), (1,)), ((), ())), preferred_element_type=F32)


def _kernel(cfg,
            aq_hbm, ak_hbm, av_hbm, sk_hbm, ssmk_hbm, ssmd_hbm, x_hbm, mem0_hbm,
            wq_hbm, wk_hbm, wv_hbm, wo_hbm, fwd_hbm, inv_hbm, fill_hbm,
            out_hbm,
            w_a, w_b, wo_u, wstage, wostage, xbuf, xlead, xlead_u, xs_u, qkvb, ob, obuf, obb,
            abuf, hbuf, kvb, ubuf, gbuf, hlast, aout, ystage,
            fwd_ref, inv_ref, fill_ref, taps, mem0_ref, sk_ref, ssmd_ref,
            sems):
    import contextlib
    scope = jax.named_scope if cfg.get("scopes") else (lambda name: contextlib.nullcontext())
    SW, SWO, SXL, SX, SH, SA, SO, SS = 0, 16, 24, 28, 29, 30, 38, 42
    only = cfg.get("only")

    def loop(name, lo, hi, body, init):
        if only is not None and name not in only:
            return init
        if cfg.get("scopes") == 2:
            def body2(i, c):
                with scope(name + "_it"):
                    return body(i, c)
            return lax.fori_loop(lo, hi, body2, init)
        with scope(name):
            return lax.fori_loop(lo, hi, body, init)
    w_hbms = (wq_hbm, wk_hbm, wv_hbm)
    a_hbms = (aq_hbm, ak_hbm, av_hbm)

    def w_copy(c, k):
        m, g = c // 2, c % 2
        slot = (c % 2) * 8 + k
        return pltpu.make_async_copy(
            w_hbms[m].at[pl.ds(k * 128, 128), pl.ds(16 * g, 16), :],
            wstage.at[slot], sems.at[SW + slot])

    def self_wait(ref, sem):
        pltpu.make_async_copy(ref, ref, sems.at[sem]).wait()

    def wo_copy(k):
        return pltpu.make_async_copy(
            wo_hbm.at[pl.ds(k * 512, 512), :], wostage.at[k], sems.at[SWO + k])

    def xlead_copy(q):
        return pltpu.make_async_copy(
            x_hbm.at[:, pl.ds(0, M), pl.ds(q * KQ, KQ)], xlead.at[q], sems.at[SXL + q])

    x_cp = pltpu.make_async_copy(
        x_hbm.at[:, pl.ds(M, SEG - M), :], xbuf.at[:, pl.ds(M, SEG - M), :], sems.at[SX])

    def h_copy(c):
        return pltpu.make_async_copy(
            ssmk_hbm.at[:, pl.ds(c * C, C)], hbuf.at[c], sems.at[SH])

    def a_copy(t, g):
        return pltpu.make_async_copy(
            a_hbms[t].at[:, pl.ds(g * 128, 128)], abuf.at[g, t], sems.at[SA + g])

    small = [pltpu.make_async_copy(src, dst, sems.at[SS + i]) for i, (src, dst) in enumerate((
        (fwd_hbm, fwd_ref), (inv_hbm, inv_ref), (fill_hbm, fill_ref),
        (mem0_hbm, mem0_ref), (sk_hbm, sk_ref), (ssmd_hbm, ssmd_ref.at[0])))]

    for q in range(4):
        xlead_copy(q).start()
        w_copy(0, 2 * q).start()
        w_copy(0, 2 * q + 1).start()
        for k in {0: (), 1: (0, 1), 2: (2, 3), 3: (4, 5, 6, 7)}[q]:
            w_copy(1, k).start()

    for b in range(2):
        gbuf[b, pl.ds(0, 7)] = jnp.zeros((7, SPEC, 128), F32)

    w_parts = (w_a, w_b)

    def slab_row(m, par, jl):
        return (m * 16 + par * 8 + jl) * SLAB

    def gated(x, i, n, gates):
        if gates is None or not cfg["gate"]:
            return x
        never, vals = gates
        v = vals[(i * len(vals) * 3) // (n * 4)]
        return jnp.where(never, pltpu.bitcast(v, U32), x)

    def vregs(*mats):
        return [m_[r:r + 8] for m_ in mats for r in range(0, m_.shape[0], 8)]

    def relayout_piece(c, k, gates=None, slot=None):
        slot = (c % 2) * 8 + k if slot is None else slot
        dst = w_parts[c % 2]
        base = slab_row(c // 2, 0, 0) + k * 64
        for i in range(64):
            a = gated(pltpu.bitcast(wstage[slot, 2 * i], U32), i, 64, gates)
            b = pltpu.bitcast(wstage[slot, 2 * i + 1], U32)
            ev = (a & jnp.uint32(0xFFFF)) | (b << 16)
            od = (a >> 16) | (b & jnp.uint32(0xFFFF0000))
            dst[pl.ds(base + i, 8, stride=SLAB), :] = ev
            dst[pl.ds(base + 8 * SLAB + i, 8, stride=SLAB), :] = od

    def comb(x, y, sign):
        f = (lambda a, b: a + b) if sign > 0 else (lambda a, b: a - b)
        return _pack(f(_unpack(x, 0), _unpack(y, 0)), f(_unpack(x, 1), _unpack(y, 1)))

    HR = NSEG * M // 4

    def batch_pair(c, jl):
        m, g = c // 2, c % 2
        it = m * NPAIR + 8 * g + jl
        rows = [pl.multiple_of(slab_row(m, par, jl), 8) for par in range(2)]
        if not cfg["strassen"]:
            xl = jnp.concatenate([pltpu.bitcast(xlead_u[q], BF16) for q in range(4)], axis=1)
            outs = [_dot(xl, pltpu.bitcast(w_parts[g][pl.ds(r, D // 2), :], BF16)) for r in rows]
            qkvb[:, it] = _pack(outs[0], outs[1]).reshape(NSEG, M, DH)
            return vregs(*outs)
        def blk(kh, par):
            return w_parts[g][pl.ds(rows[par] + kh * (D // 4), D // 4), :]

        def mm(a, b):
            return _dot(pltpu.bitcast(jnp.concatenate(a, axis=1), BF16), pltpu.bitcast(b, BF16))

        def xs(f):
            return [xs_u[f, q] for q in range(2)]
        a11 = [xlead_u[q, pl.ds(0, HR), :] for q in (0, 1)]
        a22 = [xlead_u[q, pl.ds(HR, HR), :] for q in (2, 3)]
        m5 = mm(xs(2), blk(1, 1))
        m1 = mm(xs(0), comb(blk(0, 0), blk(1, 1), 1))
        m4 = mm(a22, comb(blk(1, 0), blk(0, 0), -1))
        c11 = mm(xs(4), comb(blk(1, 0), blk(1, 1), 1)) + (m1 + m4 - m5)
        m3 = mm(a11, comb(blk(0, 1), blk(1, 1), -1))
        qkvb[pl.ds(0, NSEG // 2), it] = _pack(c11, m3 + m5).reshape(NSEG // 2, M, DH)
        m2 = mm(xs(1), blk(0, 0))
        c22 = mm(xs(3), comb(blk(0, 0), blk(0, 1), 1)) + (m1 - m2 + m3)
        qkvb[pl.ds(NSEG // 2, NSEG // 2), it] = _pack(m2 + m4, c22).reshape(NSEG // 2, M, DH)
        return vregs(m5, m1, m4, c11, m3, m2, c22)

    def quarter_prep(q):
        self_wait(xlead.at[q], SXL + q)
        for u in range(2):
            self_wait(wstage.at[2 * q + u], SW + 2 * q + u)
        xq = xlead[q].astype(F32).reshape(NSEG * M, KQ).astype(BF16)
        xlead_u[q] = pltpu.bitcast(xq, U32)
        for u in range(2):
            relayout_piece(0, 2 * q + u)

    def quarter_dot(q, par, j):
        row = slab_row(0, par, j) + q * (KQ // 2)
        row = row if isinstance(row, int) else pl.multiple_of(row, 8)
        w = pltpu.bitcast(w_a[pl.ds(row, KQ // 2), :], BF16)
        return _dot(pltpu.bitcast(xlead_u[q], BF16), w)

    def facc_get(hh):
        return jnp.concatenate([ubuf[b, hh, pl.ds(0, 2 * C), :] for b in range(2)], axis=0)

    def quarter(q, carry):
        quarter_prep(q)

        @pl.when(q > 0)
        def _():
            for u in range(2):
                self_wait(wstage.at[6 + 2 * q + u], SW + 6 + 2 * q + u)
        outs = []
        for j in range(8):
            for par in range(2):
                hh = 2 * j + par
                d = quarter_dot(q, par, j) + jnp.where(q == 0, 0.0, facc_get(hh))
                ubuf[0, hh, pl.ds(0, 2 * C), :] = d[0:2 * C]
                ubuf[1, hh, pl.ds(0, 2 * C), :] = d[2 * C:]
                outs.append(d)
        for u in range(2):
            k = jnp.maximum(2 * q - 2, 0) + u
            relayout_piece(1, k, (q > 1000, vregs(*outs[8 * u:8 * u + 8])),
                           slot=jnp.where(q == 0, u, 8 + k))
        return carry
    loop("quarters", 0, 3, quarter, 0)
    quarter_prep(3)

    def quarter_last(it, carry):
        @pl.when(it == 0)
        def _():
            for k in range(8):
                w_copy(2, k).start()
        for u in range(2):
            self_wait(wstage.at[12 + 2 * it + u], SW + 12 + 2 * it + u)
        res = []
        for u in range(4):
            j = 4 * it + u
            outs = [quarter_dot(3, par, j) + facc_get(2 * j + par) for par in range(2)]
            qkvb[:, j] = _pack(outs[0], outs[1]).reshape(NSEG, M, DH)
            res += outs
        for u in range(2):
            relayout_piece(1, 4 + 2 * it + u, (it > 1000, vregs(*res[4 * u:4 * u + 4])))
        if cfg["strassen"]:
            gates = (it > 1000, vregs(*res))
            for r in range(0, HR, 8):
                for cb in range(2):
                    cols = pl.ds(cb * 128, 128)
                    i = 2 * (r // 8) + cb
                    a11 = gated(xlead_u[it, pl.ds(r, 8), cols], i, HR // 4, gates)
                    a22 = gated(xlead_u[2 + it, pl.ds(HR + r, 8), cols], i, HR // 4, gates)
                    a21, a12 = xlead_u[it, pl.ds(HR + r, 8), cols], xlead_u[2 + it, pl.ds(r, 8), cols]
                    for f, (x, y, sg) in enumerate(((a11, a22, 1), (a21, a22, 1), (a11, a12, 1),
                                                    (a21, a11, -1), (a12, a22, -1))):
                        xs_u[f, it, pl.ds(r, 8), cols] = comb(x, y, sg)
        return carry
    loop("quarter_last", 0, 2, quarter_last, 0)

    PP = cfg["pp"]

    def issue(c):
        if c + 2 < 6:
            for k in range(8):
                w_copy(c + 2, k).start()
        if c < 3:
            for k in range(4 * (c - 1), 4 * c):
                wo_copy(k).start()
        if c == 1:
            for cp in small:
                cp.start()
        if c == 3:
            x_cp.start()
        if c == 4:
            for cc in range(NC):
                h_copy(cc).start()
            for g in range(NG):
                for t in (1, 2, 0):
                    a_copy(t, g).start()

    def wo_relayout(k, gates):
        for r in range(32):
            blk = pltpu.bitcast(wostage[k, pl.ds(r * 16, 16), :], U32)
            row = pl.multiple_of(k * 256 + r * 8, 8)
            for n in range(NB):
                wo_u[n, pl.ds(row, 8), :] = gated(blk[:, n * 128:(n + 1) * 128], r * NB + n, 32 * NB, gates)

    def chunk_body(c, pp, it, carry):
        for u in range(pp):
            k = it * pp + u
            if c < 5:
                slot = ((c + 1) % 2) * 8 + k
                self_wait(wstage.at[slot], SW + slot)
            else:
                self_wait(wostage.at[k], SWO + k)
        for u in range(pp):
            k = it * pp + u
            gates = (it > 1000, batch_pair(c, k))
            if c < 5:
                relayout_piece(c + 1, k, gates)
            else:
                wo_relayout(k, gates)
        if c == 5:
            for gg in range(pp):
                g = it * pp + gg
                sk = sk_ref[g].astype(F32)
                for j in range(KS):
                    taps[g, j] = jnp.broadcast_to(sk[j:j + 1], (8, 128))
            dd = ssmd_ref[0].astype(F32)
            for g in range(NG):
                taps[g, KS] = jnp.broadcast_to(dd[g:g + 1], (8, 128))
        return carry

    for c in range(1, 6):
        issue(c)
        if c == 5:
            for cp in small:
                cp.wait()
        pp = cfg["pp1"] if c == 1 else PP
        loop("chunk%d" % c, 0, 8 // pp, functools.partial(chunk_body, c, pp), 0)
    with scope("xh_wait"):
        x_cp.wait()
        self_wait(hbuf, SH)

    def rep(x, rows):
        return x if rows == 8 else jnp.concatenate([x] * (rows // 8), axis=0)

    def a_stage1_pre(g, p, never, par=None, gates=None):
        par = g % 2 if par is None else par
        r = p * C if isinstance(p, int) else pl.multiple_of(p * C, C)
        r2 = 2 * r if isinstance(p, int) else pl.multiple_of(2 * r, 2 * C)
        kw = pltpu.bitcast(abuf[g, 1, pl.ds(r2, 2 * C), :], U32)
        vw = pltpu.bitcast(abuf[g, 2, pl.ds(r2, 2 * C), :], U32)
        if isinstance(p, int):
            assert p == 0
            halo = jnp.zeros((8, 128), U32)
        else:
            rh = pl.multiple_of(jnp.maximum(r2 - 16, 0), 16)
            halo = jnp.where(p == 0, jnp.uint32(0), pltpu.bitcast(abuf[g, 1, pl.ds(rh, 16), :], U32))
        sub = lax.broadcasted_iota(jnp.int32, (8, 128), 0)
        cur = [kw[b:b + 8] for b in range(0, C, 8)]
        if gates is not None:
            cur = [jnp.where(never, pltpu.bitcast(gates[(i * len(gates)) // len(cur)], U32), x)
                   for i, x in enumerate(cur)]
        blk = [halo] + cur
        rolled = {sh: [pltpu.roll(x, sh, 0) for x in blk] for sh in (1, 2)}

        def shifted(b, sh):
            return jnp.where(sub < sh, rolled[sh][b // 8], rolled[sh][b // 8 + 1])
        t = [taps[g, j] for j in range(KS)]
        parts = {}
        last = None
        mode = cfg["chain1"] if (never is not None and gates is None) else 0
        blocks = list(range(0, C, 8))
        if cfg.get("rev1"):
            blocks = [b + h for b in range(C // 2 - 8, -8, -8) for h in (0, C // 2)]
        for b in blocks:
            w0 = cur[b // 8]
            w1 = shifted(b, 1)
            w2 = shifted(b, 2)
            if last is not None and mode == 3:
                w0 = jnp.where(never, last, w0)
                w1 = jnp.where(never, last, w1)
            e0, o0 = _unpack(w0, 0), _unpack(w0, 1)
            e1, o1 = _unpack(w1, 0), _unpack(w1, 1)
            o2 = _unpack(w2, 1)
            ke = e0 * t[0]
            ko = o0 * t[0]
            if last is not None and mode == 1:
                ke = jnp.where(never, last[0], ke)
                ko = jnp.where(never, last[1], ko)
            if last is not None and mode == 2:
                ke = jnp.where(never, last[1], ke)
            ke = (ke + o1 * t[1] + e1 * t[2] + o2 * t[3]) * _unpack(vw[b:b + 8], 0)
            if mode >= 2:
                ko = jnp.where(never, ke, ko)
            ko = (ko + e0 * t[1] + o1 * t[2] + e1 * t[3]) * _unpack(vw[b:b + 8], 1)
            parts[b] = _pack(ke, ko)
            last = parts[b] if mode == 3 else (ke, ko)
        parts = [parts[b] for b in range(0, C, 8)]
        kv = jnp.concatenate(parts, axis=0)
        kvb[par, pl.ds(r, C), :] = kv
        return kv

    def a_stage1_u(g, p, kv):
        fwd = pltpu.bitcast(fwd_ref[...], BF16)
        if kv is None:
            kv = kvb[g % 2, pl.ds(pl.multiple_of(p * C, C), C), :]
        for u in range(2):
            w = pltpu.bitcast(kv[u * C // 2:(u + 1) * C // 2], BF16)
            if cfg["split_u"]:
                for hf in range(2):
                    ubuf[g % 2, 2 * p + u, pl.ds(OFF[hf], C), :] = _dot(fwd[hf * C:(hf + 1) * C], w)
            else:
                d = _dot(fwd, w)
                for hf in range(2):
                    ubuf[g % 2, 2 * p + u, pl.ds(OFF[hf], C), :] = d[hf * C:(hf + 1) * C]

    def a_stage1_h(g, p):
        fwd = pltpu.bitcast(fwd_ref[...], BF16)
        rows = pl.ds(pl.multiple_of(g * 128, 128), 128)
        if cfg["split_h"]:
            hs = [jnp.concatenate([_dot_nt(fwd[hf * C:(hf + 1) * C], hbuf[2 * p + u, rows, :])
                                   for hf in range(2)], axis=0) for u in range(2)]
        else:
            hs = [_dot_nt(fwd, hbuf[2 * p + u, rows, :]) for u in range(2)]
        prev = jnp.where(p == 0, 0.0, hlast[...])
        hlast[...] = hs[1]
        hc = C // 2
        for u, (cur, prv) in enumerate(((hs[0], prev), (hs[1], hs[0]))):
            gbuf[g % 2, 7 + 2 * p + u, pl.ds(OFF[2], C), :] = jnp.concatenate(
                [cur[0:hc] - prv[C:C + hc], cur[hc:C] + prv[C + hc:]], axis=0)
            gbuf[g % 2, 7 + 2 * p + u, pl.ds(OFF[3], C), :] = jnp.concatenate(
                [cur[C:C + hc] + prv[0:hc], cur[C + hc:] - prv[hc:C]], axis=0)

    def a_stage2(gp, p, slot, chain, never, gates=None, last=None):
        b = gp % 2
        RB = 8
        re = [[], []]
        im = [[], []]
        done = 0
        for r in [r0 + blk for r0 in range(0, C // 2, RB) for blk in (0, C // 2)]:
            gr = [gbuf[b, 7 + p + 8 - j, pl.ds(OFF[2] + r, RB), :] for j in range(NC)]
            gi = [gbuf[b, 7 + p + 8 - j, pl.ds(OFF[3] + r, RB), :] for j in range(NC)]
            ur = [ubuf[b, j, pl.ds(OFF[0] + r, RB), :] for j in range(NC)]
            ui = [ubuf[b, j, pl.ds(OFF[1] + r, RB), :] for j in range(NC)]
            for o, (nt, off) in enumerate(((8, 8), (16, 0))):
                if gates is not None:
                    gs = cfg["gate_terms"]
                    ar = ai = None
                    for j in range(nt):
                        g0 = gr[j + off]
                        if j % gs == 0:
                            gt = gates[(done * len(gates)) // (24 * 16)]
                            g0 = jnp.where(never, gt, g0)
                        done += 1
                        tr, ti = g0 * ur[j], g0 * ui[j]
                        ar = tr if ar is None else ar + tr
                        ai = ti if ai is None else ai + ti
                        ar = ar - gi[j + off] * ui[j]
                        ai = ai + gi[j + off] * ur[j]
                    last = (ar, ai)
                elif chain == 1:
                    ar = gr[off] * ur[0]
                    ai = gr[off] * ui[0]
                    if last is not None:
                        ar = jnp.where(never, last[0], ar)
                        ai = jnp.where(never, last[1], ai)
                    ar = ar - gi[off] * ui[0]
                    ai = ai + gi[off] * ur[0]
                    for j in range(1, nt):
                        ar = ar + gr[j + off] * ur[j]
                        ai = ai + gr[j + off] * ui[j]
                        ar = ar - gi[j + off] * ui[j]
                        ai = ai + gi[j + off] * ur[j]
                    last = (ar, ai)
                else:
                    ar = gr[off] * ur[0]
                    if last is not None:
                        ar = jnp.where(never, last, ar)
                    ar = ar - gi[off] * ui[0]
                    for j in range(1, nt):
                        ar = ar + gr[j + off] * ur[j]
                        ar = ar - gi[j + off] * ui[j]
                    ai = jnp.where(never, ar, gr[off] * ui[0])
                    ai = ai + gi[off] * ur[0]
                    for j in range(1, nt):
                        ai = ai + gr[j + off] * ui[j]
                        ai = ai + gi[j + off] * ur[j]
                    last = ai
                re[o].append(ar)
                im[o].append(ai)
                if r >= C // 2:
                    rows = pl.ds(r - C // 2, RB)
                    ev = _pack(re[o][-2] + ar, im[o][-2] - ai)
                    od = _pack(re[o][-2] - ar, im[o][-2] + ai)
                    ystage[slot, o, 0, rows, :] = ev
                    ystage[slot, o, 1, rows, :] = od
                    if cfg["chain_pack"] and chain == 1:
                        last = (pltpu.bitcast(ev, F32), pltpu.bitcast(od, F32))
        return list(last) if isinstance(last, tuple) else [last]

    def a_stage3(gp, gq, p, slot):
        inv = pltpu.bitcast(inv_ref[...], BF16)
        dd = rep(taps[gq, KS], C // 2)
        for o in range(2):
            i = p + 8 * o
            kvw = kvb[gp % 2, pl.ds(pl.multiple_of(i * (C // 2), C // 2), C // 2), :]
            qw = pltpu.bitcast(abuf[gq, 0, pl.ds(pl.multiple_of(i * C, C), C), :], U32)
            res = []
            for e in range(2):
                y = _dot(inv[e * (C // 2):(e + 1) * (C // 2)], pltpu.bitcast(ystage[slot, o, e], BF16))
                res.append(_unpack(qw, e) * (y + _unpack(kvw, e) * dd))
            out = pltpu.bitcast(_pack(res[0], res[1]), BF16)
            aout[gq, pl.ds(pl.multiple_of(i * 4, 4), 4)] = out.reshape(4, SEG, 128)

    scale = DH ** (-0.5)

    def w_slab(m, h, z):
        j = h // 2
        row = slab_row(m, h % 2, j % 8)
        row = row if z is None else pl.multiple_of(z + row, 8)
        return pltpu.bitcast(w_parts[j // 8][pl.ds(row, D // 2), :], BF16)

    shared = {}

    class Step:
        def __init__(self, s, u):
            self.s = s
            self.slot = u
            self.z = None if (u == 0 or not cfg.get("zoff")) else pl.multiple_of(jnp.where(s > 1000 + u, 32, 0), 32)
            self.g = s // 8
            self.p = s % 8
            self.qkv, self.ps, self.os = {}, {}, []
            self.acc = [None] * NB
            self.ocat = {}
            self.gates = []
            self.lead = {}
            self.prev = None
            self.early = {}
            self.ties = []

        def start(self, mem):
            x = xbuf[self.s, pl.ds(M, SEG - M), :].astype(F32)
            self.lhsf = jnp.concatenate([mem, x], axis=0)
            self.lhs = self.lhsf.astype(BF16)

        def proj_early(self, m, j, k):
            self.early[m, j] = (k, [_dot(self.lhsf[:, :k].astype(BF16), w_slab(m, 2 * j + e, self.z)[:k])
                                    for e in range(2)])

        def proj(self, m, j):
            if (m, j) in self.early:
                k, part = self.early[m, j]
                a, b = [_dot(self.lhsf[:, k:].astype(BF16), w_slab(m, 2 * j + e, self.z)[k:]) + part[e]
                        for e in range(2)]
            else:
                a = _dot(self.lhs, w_slab(m, 2 * j, self.z))
                b = _dot(self.lhs, w_slab(m, 2 * j + 1, self.z))
            self.gates += vregs(a, b)
            lead = qkvb[self.s, m * NPAIR + j]
            if m == 0:
                r = jnp.concatenate([a, b, _unpack(lead, 0), _unpack(lead, 1)], axis=0).astype(BF16)
            else:
                r = pltpu.bitcast(jnp.concatenate([_pack(a, b), lead], axis=0), BF16)
            self.qkv[m, j] = r

        def probs(self, j):
            fill = fill_ref[pl.ds(0, R), pl.ds(0, R)]
            sc = jnp.where(fill == 0.0, _dot_nt(self.qkv[0, j], self.qkv[1, j]) * scale, fill)
            mx = jnp.max(sc, axis=-1, keepdims=True)
            e = jnp.exp(sc - mx)
            l = jnp.sum(e, axis=-1, keepdims=True)
            r = pl.reciprocal(l, approx=True)
            r = r * (2.0 - l * r)
            self.ps[j] = (e * r).astype(BF16)

        def attend(self, j):
            o = _dot(self.ps[j], self.qkv[2, j])
            la, lb = o[2 * SEG:2 * SEG + M], o[2 * SEG + M:]
            if cfg["strassen_e"]:
                rows = pl.ds(pl.multiple_of((self.s // 2) * M, M), M)
                if self.prev is None:
                    self.lead[j] = (la, lb)
                    forms = {2: la + lb, 5: la}
                else:
                    a11, a12 = self.prev.lead[j]
                    forms = {0: a11 + lb, 1: la + lb, 3: la - a11, 4: a12 - lb, 6: lb}
                for f, v in forms.items():
                    ob[f * NPAIR + j, rows, :] = v.astype(BF16)
            else:
                rows = pl.ds(pl.multiple_of(self.s * M, M), M)
                ob[2 * j, rows, :] = la.astype(BF16)
                ob[2 * j + 1, rows, :] = lb.astype(BF16)
            self.os += [o[0:SEG], o[SEG:2 * SEG]]

        def wo(self, h0, h1, ns):
            if (h0, h1) not in self.ocat:
                self.ocat[h0, h1] = jnp.concatenate(self.os[h0:h1], axis=1).astype(BF16)
            o = self.ocat[h0, h1]
            for n in ns:
                row = h0 * 64 if self.z is None else pl.multiple_of(self.z + h0 * 64, 32)
                w = wo_u[n, pl.ds(row, (h1 - h0) * 64), :]
                if cfg["tie"] == n + 1 + (NB if h1 == H else 0):
                    parts = [jnp.where(self.s > 1000, pltpu.bitcast(t, U32), w[8 * i:8 * i + 8])
                             for i, t in enumerate(self.ties)]
                    w = jnp.concatenate(parts + [w[8 * len(parts):]], axis=0)
                d = _dot(o, pltpu.bitcast(w, BF16))
                self.acc[n] = d if self.acc[n] is None else d + self.acc[n]
                self.gates += [v for v in vregs(self.acc[n]) for _ in range((h1 - h0) // 8)]

        def finish(self):
            res = jnp.concatenate(self.acc, axis=1)
            obuf[self.s] = res.astype(BF16)
            return res[0:M]

        def run(self, item):
            kind = item[0]
            g, p = self.g, self.p
            never = (self.s if cfg["real_chain"] else p) > 1000
            if kind == "P":
                self.proj(item[1], item[2])
            elif kind == "E":
                self.proj_early(item[1], item[2], item[3])
            elif kind == "S":
                self.probs(item[1])
            elif kind == "V":
                self.attend(item[1])
            elif kind == "W":
                self.wo(item[1], item[2], item[3])
            elif kind == "A1":
                self.kv = a_stage1_pre(g, p, never)
            elif kind == "AU":
                a_stage1_u(g, p, self.kv)
            elif kind == "AH":
                a_stage1_h(g, p)
            elif kind == "A2":
                tail = a_stage2(g + 1, p, self.slot, cfg["chain"], never, last=shared.get("a2"))
                if cfg["chain_a2"]:
                    shared["a2"] = tuple(tail)
            elif kind == "A3":
                a_stage3(g + 1, jnp.maximum(g - 1, 0), p, self.slot)
            elif kind == "N1":
                gn = (self.s + 1) // 8
                kv = a_stage1_pre(jnp.minimum(gn, NG - 1), (self.s + 1) % 8, never, gn % 2)
                if cfg["tie"]:
                    self.ties.append(pltpu.bitcast(kv[C - 8:C], F32))
            elif kind == "N2":
                tails = a_stage2((self.s + 1) // 8 + 1, (self.s + 1) % 8, 0, cfg["chain"], never)
                if cfg["tie"]:
                    self.ties += tails
            elif kind in ("G1", "G2"):
                t = self.s + U
                lo, hi = cfg["g1" if kind == "G1" else "g2"]
                gates = self.gates[(lo * len(self.gates)) // 100:(hi * len(self.gates)) // 100]
                if kind == "G1":
                    a_stage1_pre(jnp.minimum(t // 8, NG - 1), t % 8, never, (t // 8) % 2, gates)
                else:
                    a_stage2(t // 8 + 1, t % 8, self.slot, None, never, gates)
            elif kind == "PU":
                a_stage1_u(g, p, None)
            elif kind == "P3":
                a_stage3(g + 1, jnp.maximum(g - 1, 0), p, 0)

    U, order = _make_order(cfg["order"])
    pipe = any(item[0] == "N1" for _, item in order)
    pipe2 = any(item[0] == "N2" for _, item in order)
    if pipe:
        self_wait(abuf.at[0], SA)
        a_stage1_pre(0, 0, None)

    def steps(i, mem):
        s0 = i * U
        sw = s0 + U if pipe else s0

        @pl.when(jnp.logical_and(sw % 8 == 0, sw < NSEG))
        def _():
            self_wait(abuf.at[sw // 8], SA + sw // 8)
        shared.clear()
        st = [Step(s0 + u, u) for u in range(U)]
        for u in range(1, U, 2):
            st[u].prev = st[u - 1]
        for u, item in order:
            if item[0] == "start":
                st[u].start(mem)
            elif item[0] == "finish":
                mem = st[u].finish()
            else:
                st[u].run(item)
        return mem

    loop("steps", 0, NSEG // U, steps, mem0_ref[...].astype(F32))

    ob_cp = pltpu.make_async_copy(
        obuf.at[:, pl.ds(M, SEG - M), :],
        out_hbm.at[:, pl.ds(M, SEG - M), pl.ds(D, D)], sems.at[SO])
    ob_cp.start()
    for g in range(NG - 1):
        pltpu.make_async_copy(
            aout.at[g], out_hbm.at[:, :, pl.ds(g * 128, 128)], sems.at[SO + 1]).start()

    EP = cfg["ep"]
    GL = NG - 1
    HS = cfg["ep_split"]

    def epi_strassen(it):
        never = it > 1000
        ns = [2 * it, 2 * it + 1]

        def blk(hp, u):
            return [wo_u[ns[u], pl.ds((2 * j + hp) * 64, 64), :] for j in range(NPAIR)]

        def mm(f, bs):
            lhs = jnp.concatenate([ob[f * NPAIR + j] for j in range(NPAIR)], axis=1)
            return _dot(lhs, pltpu.bitcast(jnp.concatenate(bs, axis=0), BF16))

        def cb(x, y, sign):
            return [comb(a, b, sign) for a, b in zip(x, y)]

        def put(u, par, c):
            for i in range(NSEG // 2):
                obb[ns[u], 2 * i + par] = c[M * i:M * i + M].astype(BF16)
        sched = cfg["ep_sched"]

        def hook(k):
            for u in range(2):
                if sched[u] == k:
                    a_stage3(GL, GL, ns[u], u)
        for u in range(2):
            a_stage2(GL, ns[u], u, cfg["ep_chain"], never)
        m5 = mm(2, blk(1, 1))
        m1 = mm(0, cb(blk(0, 0), blk(1, 1), 1))
        hook(2)
        m4 = mm(6, cb(blk(1, 0), blk(0, 0), -1))
        hook(3)
        put(0, 0, mm(4, cb(blk(1, 0), blk(1, 1), 1)) + (m1 + m4 - m5))
        hook(4)
        m3 = mm(5, cb(blk(0, 1), blk(1, 1), -1))
        put(1, 0, m3 + m5)
        hook(5)
        m2 = mm(1, blk(0, 0))
        put(0, 1, m2 + m4)
        hook(6)
        put(1, 1, mm(3, cb(blk(0, 0), blk(0, 1), 1)) + (m1 - m2 + m3))

    def epi(it, carry):
        def part(n, h0, h1):
            lhs = jnp.concatenate([ob[h] for h in range(h0, h1)], axis=1)
            return _dot(lhs, pltpu.bitcast(wo_u[n, pl.ds(h0 * 64, (h1 - h0) * 64), :], BF16))
        if cfg["strassen_e"]:
            assert EP == 2 and U % 2 == 0 and not pipe2
            epi_strassen(it)
        for u in range(0 if cfg["strassen_e"] else EP):
            n = it * EP + u
            if pipe2:
                a_stage3(GL, GL, n, 0)
                a_stage2(GL, jnp.minimum(n + 1, 7), 0, cfg["ep_chain"], it > 1000)
                d = part(n, 0, H)
            else:
                a_stage2(GL, n, u % 2, cfg["ep_chain"], it > 1000)
                d = part(n, 0, HS)
                a_stage3(GL, GL, n, u % 2)
                d = part(n, HS, H) + d
            obb[n] = d.reshape(NSEG, M, 128).astype(BF16)
        for u in range(EP):
            n = it * EP + u
            col = pl.multiple_of(D + n * 128, 128)
            pltpu.make_async_copy(
                obb.at[n], out_hbm.at[:, pl.ds(0, M), pl.ds(col, 128)], sems.at[SO + 2]).start()
        for o in range(2):
            rows = pl.ds((it * EP + 8 * o) * 4, 4 * EP)
            pltpu.make_async_copy(
                aout.at[GL, rows], out_hbm.at[rows, :, pl.ds(GL * 128, 128)], sems.at[SO + 1]).start()
        return carry
    loop("epi", 0, NB // EP, epi, 0)
    ob_cp.wait()
    self_wait(aout, SO + 1)
    self_wait(obb, SO + 2)


def _b_order(u, extra, o):
    ks = o.get("ks", 24)
    tmpl = [(x[0], int(x[1:])) for x in o.get("tmpl", "q0 v1 S1 k0 V2").split()]
    out = list(extra.get("pre", [])) + [(u, ("start",))]
    if u > 0:
        first = [(kind, t - lag) for t in range(3) for kind, lag in tmpl if kind in "qkv" and t >= lag]
        out += [(u, ("E", "qkv".index(kind), j, o.get("ek", 768))) for kind, j in first[:o.get("ne", 2)]]
    nw = 0
    for t in range(NPAIR + max(l for _, l in tmpl)):
        for kind, lag in tmpl:
            j = t - lag
            if j < 0:
                continue
            if j >= NPAIR:
                if kind in "qkv" and nw < NB:
                    out.append((u, ("W", 0, ks, (nw,))))
                    nw += 1
                continue
            out.append((u, ("P", "qkv".index(kind), j) if kind in "qkv" else (kind, j)))
        out += extra.get(t, [])
    out += extra.get("tail", [])
    out += [(u, ("W", 0, ks, tuple(range(nw, NB))))]
    out += extra.get("tail2", [])
    out += [(u, ("W", ks, H, tuple(range(NB))))]
    out += extra.get("end", [])
    out += [(u, ("finish",))]
    out += extra.get("post", [])
    return out


def _make_order(o):
    out = []
    U = len(o["a"])
    for u, d in enumerate(o["a"]):
        ex = {}
        for k, names in d.items():
            k = int(k) if k.isdigit() else k
            ex[k] = [(u - n.count("-") + n.count("+"), (n.lstrip("+-"),)) for n in names]
        out += _b_order(u, ex, o)
    return U, out


_DEFAULT_CFG = dict(
    order=dict(a=[{"pre": ["A1", "+A1"], "0": ["AH"], "2": ["AU"], "4": ["+AU"], "6": ["+AH", "A2", "+A2"]},
                  {"tail2": ["-A3", "A3"]}],
               tmpl="q0 v1 S1 k0 V2", ks=16, ne=2, ek=768),
    pp=4, ep=2, ep_split=24, ep_chain=1, chain=1, chain1=2, real_chain=1,
    split_u=0, split_h=0, tie=0, strassen=1, gate=1, pp1=2, nobc=1,
    strassen_e=1, ep_sched=(4, 6), g1=(85, 97), g2=(5, 85), gate_terms=8,
    chain_pack=0, chain_a2=0)


def _pack_rows(x):
    b = np.asarray(x, dtype=jnp.bfloat16).view(np.uint16).astype(np.uint32)
    return b[0::2] | (b[1::2] << 16)


def _build(cfg):
    fwd_np, inv_np = _dft_constants()
    fill_np = np.zeros((96, 128), np.float32)
    fill_np[:R, :R] = _mask_fill()

    def run(A_q, A_k, A_v, A_shift_k, A_ssm_k, A_ssm_D, B_x, B_mem0, B_Wq, B_Wk, B_Wv, B_Wo):
        sk = A_shift_k.T.reshape(KS, NG, 128).transpose(1, 0, 2)
        any_spec = pl.BlockSpec(memory_space=pl.ANY)
        out = pl.pallas_call(
            functools.partial(_kernel, cfg),
            out_shape=jax.ShapeDtypeStruct((NSEG, SEG, 2 * D), BF16),
            in_specs=[any_spec] * 15,
            out_specs=any_spec,
            scratch_shapes=[
                pltpu.VMEM((48 * SLAB + 544, 128), U32),
                pltpu.VMEM((48 * SLAB + 544, 128), U32),
                pltpu.VMEM((NB, H * DH // 2, 128), U32),
                pltpu.VMEM((16, 128, 16, DH), BF16),
                pltpu.VMEM((8, 512, D), BF16),
                pltpu.VMEM((NSEG, SEG, D), BF16),
                pltpu.VMEM((4, NSEG, M, KQ), BF16),
                pltpu.VMEM((4, NSEG * M // 2, KQ), U32),
                pltpu.VMEM((5, 2, NSEG * M // 4, KQ), U32),
                pltpu.VMEM((NSEG, 3 * NPAIR, 8, 128), U32),
                (pltpu.VMEM((7 * NPAIR, NSEG * M // 2, DH), BF16) if cfg["strassen_e"]
                 else pltpu.VMEM((H, NSEG * M, DH), BF16)),
                pltpu.VMEM((NSEG, SEG, D), BF16),
                pltpu.VMEM((NB, NSEG, M, 128), BF16),
                pltpu.VMEM((NG, 3, S, 128), BF16),
                pltpu.VMEM((NC, D, C), BF16),
                pltpu.VMEM((2, S // 2, 128), U32),
                pltpu.VMEM((2, NC, SPEC, 128), F32),
                pltpu.VMEM((2, NC + 7, SPEC, 128), F32),
                pltpu.VMEM((2 * C, 128), F32),
                pltpu.VMEM((NG, NSEG, SEG, 128), BF16),
                pltpu.VMEM((4, 2, 2, C // 2, 128), U32),
                pltpu.VMEM((C, C), U32),
                pltpu.VMEM((C // 2, C), U32),
                pltpu.VMEM((96, 128), F32),
                pltpu.VMEM((NG, 8, 8, 128), F32),
                pltpu.VMEM((M, D), BF16),
                pltpu.VMEM((NG, KS, 128), BF16),
                pltpu.VMEM((4, NG, 128), BF16),
                pltpu.SemaphoreType.DMA((48,)),
            ],
            compiler_params=pltpu.CompilerParams(vmem_limit_bytes=124 * 1024 * 1024,
                                                 disable_bounds_checks=bool(cfg["nobc"])),
        )(A_q.reshape(S, D), A_k.reshape(S, D), A_v.reshape(S, D), sk, A_ssm_k,
          A_ssm_D.reshape(NG, 128), B_x.reshape(NSEG, SEG, D), B_mem0.reshape(M, D),
          B_Wq, B_Wk, B_Wv, B_Wo.reshape(H * DH, D),
          jnp.asarray(_pack_rows(fwd_np)), jnp.asarray(_pack_rows(inv_np)), jnp.asarray(fill_np))
        return out.reshape(1, S, 2 * D)

    return run


@functools.partial(jax.jit, static_argnames=("B_seg_len",))
def pallas_concat_heads__ssm_conv_h3__memory_aug_recurrent_mem_tr__prompt_kernel(
    A_q: jax.Array,
    A_k: jax.Array,
    A_v: jax.Array,
    A_shift_k: jax.Array,
    A_ssm_k: jax.Array,
    A_ssm_D: jax.Array,
    B_x: jax.Array,
    B_mem0: jax.Array,
    B_Wq: jax.Array,
    B_Wk: jax.Array,
    B_Wv: jax.Array,
    B_Wo: jax.Array,
    B_seg_len: int = SEG,
):
    assert B_seg_len == SEG
    return _build(_DEFAULT_CFG)(A_q, A_k, A_v, A_shift_k, A_ssm_k, A_ssm_D, B_x, B_mem0,
                                B_Wq, B_Wk, B_Wv, B_Wo)
```

```python
import functools

import numpy as np
import jax
import jax.numpy as jnp
from jax import lax
import jax.experimental.pallas as pl
import jax.experimental.pallas.tpu as pltpu

F32 = jnp.float32
BF16 = jnp.bfloat16
U32 = jnp.uint32

S = 2048
D = 1024
H = 32
DH = 128
M = 8
SEG = 32
NSEG = S // SEG
NPAIR = H // 2
R = 2 * (M + SEG)
SLAB = 520
KS = 4
C = 128
NC = S // C
NG = D // 128
KQ = D // 4
SPEC = 2 * C + 32
OFF = (0, C + 8, 16, C + 24)
NB = D // 128


def _dft_constants():
    fe = np.arange(0, C, 2)
    f = np.concatenate([fe, C - 1 - fe])
    t = np.arange(C)
    ang = (np.pi * (2 * f + 1) / (2 * C))[:, None] * t[None, :]
    fwd = np.concatenate([np.cos(ang), -np.sin(ang)], axis=0)
    a = ang[:C // 2]
    inv = np.stack([np.cos(a), -np.sin(a)], axis=1).reshape(C, C).T / C
    inv = np.concatenate([inv[0::2], inv[1::2]], axis=0)
    return fwd.astype(np.float32), inv.astype(np.float32)


def _mask_fill():
    blk = np.concatenate([np.arange(M), M + np.arange(M, SEG)])
    lead = M + np.arange(M)
    qhead = np.concatenate([np.zeros(SEG), np.ones(SEG), np.zeros(M), np.ones(M)])
    qpos = np.concatenate([blk, blk, lead, lead])
    khead = np.arange(R) % 2
    kpos = np.concatenate([blk, lead])[np.arange(R) // 2]
    same = qhead[:, None] == khead[None, :]
    ok = (qpos[:, None] < M) | (qpos[:, None] >= kpos[None, :])
    fill = np.where(same, np.where(ok, 0.0, -1e9), -np.inf)
    return fill.astype(np.float32)


def _pack(lo, hi):
    return pltpu.pack_elementwise([lo, hi], packed_dtype=BF16)


def _unpack(w, index):
    return pltpu.unpack_elementwise(w, index=index, packed_dtype=BF16, unpacked_dtype=F32)


def _dot(a, b):
    return jnp.dot(a, b, preferred_element_type=F32)


def _dot_nt(a, b):
    return lax.dot_general(a, b, (((1,), (1,)), ((), ())), preferred_element_type=F32)


def _kernel(cfg,
            aq_hbm, ak_hbm, av_hbm, sk_hbm, ssmk_hbm, ssmd_hbm, x_hbm, mem0_hbm,
            wq_hbm, wk_hbm, wv_hbm, wo_hbm, fwd_hbm, inv_hbm, fill_hbm,
            out_hbm,
            w_a, w_b, wo_u, wstage, wostage, xbuf, xlead, xlead_u, xs_u, qkvb, ob, obuf, obb,
            abuf, hbuf, kvb, ubuf, gbuf, hlast, aout, ystage,
            fwd_ref, inv_ref, fill_ref, taps, mem0_ref, sk_ref, ssmd_ref,
            sems):
    import contextlib
    scope = jax.named_scope if cfg.get("scopes") else (lambda name: contextlib.nullcontext())
    SW, SWO, SXL, SX, SH, SA, SO, SS = 0, 16, 24, 28, 36, 44, 52, 56
    U, order = _make_order(cfg["order"])
    HW = 2 * C * U
    only = cfg.get("only")

    def loop(name, lo, hi, body, init):
        if only is not None and name not in only:
            return init
        if cfg.get("scopes") == 2:
            def body2(i, c):
                with scope(name + "_it"):
                    return body(i, c)
            return lax.fori_loop(lo, hi, body2, init)
        with scope(name):
            return lax.fori_loop(lo, hi, body, init)
    w_hbms = (wq_hbm, wk_hbm, wv_hbm)
    a_hbms = (aq_hbm, ak_hbm, av_hbm)

    def w_copy(c, k):
        m, g = c // 2, c % 2
        slot = (c % 2) * 8 + k
        return pltpu.make_async_copy(
            w_hbms[m].at[pl.ds(k * 128, 128), pl.ds(16 * g, 16), :],
            wstage.at[slot], sems.at[SW + slot])

    def self_wait(ref, sem):
        pltpu.make_async_copy(ref, ref, sems.at[sem]).wait()

    def wo_copy(k):
        return pltpu.make_async_copy(
            wo_hbm.at[pl.ds(k * 512, 512), :], wostage.at[k], sems.at[SWO + k])

    def xlead_copy(q):
        return pltpu.make_async_copy(
            x_hbm.at[:, pl.ds(0, M), pl.ds(q * KQ, KQ)], xlead.at[q], sems.at[SXL + q])

    def x_copy(g):
        segs = pl.ds(g * 8, 8)
        return pltpu.make_async_copy(
            x_hbm.at[segs, pl.ds(M, SEG - M), :], xbuf.at[segs, pl.ds(M, SEG - M), :], sems.at[SX + g])

    def h_copy(g, part):
        return pltpu.make_async_copy(
            ssmk_hbm.at[pl.ds(g * 128, 128), pl.ds(part * HW, HW)], hbuf.at[g, part], sems.at[SH + g])

    def a_copy(t, g):
        return pltpu.make_async_copy(
            a_hbms[t].at[:, pl.ds(g * 128, 128)], abuf.at[g, t], sems.at[SA + g])

    def group_start(g):
        x_copy(g).start()
        for t in (1, 2):
            a_copy(t, g).start()
        for part in range(S // HW):
            h_copy(g, part).start()
        a_copy(0, g).start()

    def group_wait(g):
        x_copy(g).wait()
        self_wait(hbuf.at[g], SH + g)
        self_wait(abuf.at[g], SA + g)

    small = [pltpu.make_async_copy(src, dst, sems.at[SS + i]) for i, (src, dst) in enumerate((
        (fwd_hbm, fwd_ref), (inv_hbm, inv_ref), (fill_hbm, fill_ref),
        (mem0_hbm, mem0_ref), (sk_hbm, sk_ref), (ssmd_hbm, ssmd_ref.at[0])))]

    for q in range(4):
        xlead_copy(q).start()
        w_copy(0, 2 * q).start()
        w_copy(0, 2 * q + 1).start()
        for k in ({2: (0, 1), 3: (2, 3, 4, 5, 6, 7)} if cfg["up"] == 2 else
                  {q: (2 * q, 2 * q + 1)}).get(q, ()):
            w_copy(1, k).start()

    def zero_pad(i, carry):
        gbuf[i // 7, i % 7] = jnp.zeros((SPEC, 128), F32)
        return carry
    lax.fori_loop(0, 14, zero_pad, 0)

    w_parts = (w_a, w_b)

    def slab_row(m, par, jl):
        return (m * 16 + par * 8 + jl) * SLAB

    def gated(x, i, n, gates):
        if gates is None or not cfg["gate"]:
            return x
        never, vals = gates
        v = vals[(i * len(vals) * 3) // (n * 4)]
        return jnp.where(never, pltpu.bitcast(v, U32), x)

    def vregs(*mats):
        return [m_[r:r + 8] for m_ in mats for r in range(0, m_.shape[0], 8)]

    def relayout_piece(m, g, k, gates=None, slot=None):
        slot = g * 8 + k if slot is None else slot
        dst = w_parts[g]
        base = slab_row(m, 0, 0) + k * 64
        for i in range(64):
            a = gated(pltpu.bitcast(wstage[slot, 2 * i], U32), i, 64, gates)
            b = pltpu.bitcast(wstage[slot, 2 * i + 1], U32)
            ev = (a & jnp.uint32(0xFFFF)) | (b << 16)
            od = (a >> 16) | (b & jnp.uint32(0xFFFF0000))
            dst[pl.ds(base + i, 8, stride=SLAB), :] = ev
            dst[pl.ds(base + 8 * SLAB + i, 8, stride=SLAB), :] = od

    def comb(x, y, sign):
        f = (lambda a, b: a + b) if sign > 0 else (lambda a, b: a - b)
        return _pack(f(_unpack(x, 0), _unpack(y, 0)), f(_unpack(x, 1), _unpack(y, 1)))

    HR = NSEG * M // 4

    def batch_pair(m, g, jl):
        it = m * NPAIR + 8 * g + jl
        rows = [pl.multiple_of(slab_row(m, par, jl), 8) for par in range(2)]
        if not cfg["strassen"]:
            xl = jnp.concatenate([pltpu.bitcast(xlead_u[q], BF16) for q in range(4)], axis=1)
            outs = [_dot(xl, pltpu.bitcast(w_parts[g][pl.ds(r, D // 2), :], BF16)) for r in rows]
            qkvb[:, it] = _pack(outs[0], outs[1]).reshape(NSEG, M, DH)
            return vregs(*outs)
        def blk(kh, par):
            return w_parts[g][pl.ds(rows[par] + kh * (D // 4), D // 4), :]

        def mm(a, b):
            return _dot(pltpu.bitcast(jnp.concatenate(a, axis=1), BF16), pltpu.bitcast(b, BF16))

        def xs(f):
            return [xs_u[f, q] for q in range(2)]
        a11 = [xlead_u[q, pl.ds(0, HR), :] for q in (0, 1)]
        a22 = [xlead_u[q, pl.ds(HR, HR), :] for q in (2, 3)]
        m5 = mm(xs(2), blk(1, 1))
        m1 = mm(xs(0), comb(blk(0, 0), blk(1, 1), 1))
        m4 = mm(a22, comb(blk(1, 0), blk(0, 0), -1))
        c11 = mm(xs(4), comb(blk(1, 0), blk(1, 1), 1)) + (m1 + m4 - m5)
        m3 = mm(a11, comb(blk(0, 1), blk(1, 1), -1))
        qkvb[pl.ds(0, NSEG // 2), it] = _pack(c11, m3 + m5).reshape(NSEG // 2, M, DH)
        m2 = mm(xs(1), blk(0, 0))
        c22 = mm(xs(3), comb(blk(0, 0), blk(0, 1), 1)) + (m1 - m2 + m3)
        qkvb[pl.ds(NSEG // 2, NSEG // 2), it] = _pack(m2 + m4, c22).reshape(NSEG // 2, M, DH)
        return vregs(m5, m1, m4, c11, m3, m2, c22)

    def unit(n, carry):
        q, half = n // 2, n % 2
        never = n > 1000
        UP = cfg["up"]
        n0 = 8 - 8 // UP

        @pl.when(half == 0)
        def _():
            self_wait(xlead.at[q], SXL + q)
            for u in range(2):
                self_wait(wstage.at[2 * q + u], SW + 2 * q + u)
            xq = xlead[q].astype(F32).reshape(NSEG * M, KQ).astype(BF16)
            xlead_u[q] = pltpu.bitcast(xq, U32)
            for u in range(2):
                relayout_piece(0, 0, 2 * q + u)

        @pl.when(n == 6)
        def _():
            for k in range(8):
                w_copy(2, k).start()

        @pl.when(n >= n0)
        def _():
            for u in range(UP):
                slot = 8 + (n - n0) * UP + u
                self_wait(wstage.at[slot], SW + slot)
        res = []
        xq = pltpu.bitcast(xlead_u[q], BF16)
        for u in range(4):
            jl = 4 * half + u
            outs = []
            for par in range(2):
                hh = 2 * jl + par
                row = pl.multiple_of(slab_row(0, par, jl) + q * (KQ // 2), 8)
                w = pltpu.bitcast(w_a[pl.ds(row, KQ // 2), :], BF16)
                old = jnp.concatenate([ubuf[b, hh, pl.ds(0, 2 * C), :] for b in range(2)], axis=0)
                d = _dot(xq, w) + jnp.where(q == 0, 0.0, old)
                ubuf[0, hh, pl.ds(0, 2 * C), :] = d[0:2 * C]
                ubuf[1, hh, pl.ds(0, 2 * C), :] = d[2 * C:]
                outs.append(d)
            qkvb[:, jl] = _pack(outs[0], outs[1]).reshape(NSEG, M, DH)
            res += outs
        for u in range(UP):
            k = jnp.maximum(n - n0, 0) * UP + u
            nv = 8 // UP
            relayout_piece(0, 1, k, (never, vregs(*res[nv * u:nv * u + nv])),
                           slot=jnp.where(n < n0, u, 8 + k))
        if cfg["strassen"]:
            gates = (never, vregs(*res))
            for r in range(0, HR, 8):
                for cb in range(2):
                    cols = pl.ds(cb * 128, 128)
                    i = 2 * (r // 8) + cb
                    a11 = gated(xlead_u[half, pl.ds(r, 8), cols], i, HR // 4, gates)
                    a22 = gated(xlead_u[2 + half, pl.ds(HR + r, 8), cols], i, HR // 4, gates)
                    a21 = xlead_u[half, pl.ds(HR + r, 8), cols]
                    a12 = xlead_u[2 + half, pl.ds(r, 8), cols]
                    for f, (x, y, sg) in enumerate(((a11, a22, 1), (a21, a22, 1), (a11, a12, 1),
                                                    (a21, a11, -1), (a12, a22, -1))):
                        xs_u[f, half, pl.ds(r, 8), cols] = comb(x, y, sg)
        return carry
    loop("units", 0, 8, unit, 0)

    PP = cfg["pp"]

    def issue(c):
        if c + 2 < 6:
            for k in range(8):
                w_copy(c + 2, k).start()
        for k in cfg["wo_issue"].get(c, ()):
            wo_copy(k).start()
        if c == 1:
            for cp in small:
                cp.start()
        for g in cfg["g_issue"].get(c, ()):
            group_start(g)

    def wo_relayout(src_slot, hp, gates):
        r0 = (hp % 2) * 256
        for r in range(16):
            blk = pltpu.bitcast(wostage[src_slot, pl.ds(pl.multiple_of(r0 + r * 16, 16), 16), :], U32)
            row = pl.multiple_of(hp * 128 + r * 8, 8)
            for n in range(NB):
                wo_u[n, pl.ds(row, 8), :] = gated(blk[:, n * 128:(n + 1) * 128], r * NB + n, 16 * NB, gates)

    def chunk_body(c, g, it, carry):
        @pl.when(c < 5)
        def _():
            for u in range(PP):
                slot = (1 - g) * 8 + it * PP + u
                self_wait(wstage.at[slot], SW + slot)

        @pl.when(c >= 4)
        def _():
            for u in range(PP // 2):
                k = (c - 4) * 4 + it * (PP // 2) + u
                self_wait(wostage.at[k], SWO + k)
        for u in range(PP):
            k = it * PP + u
            gates = (it > 1000, batch_pair(c // 2, g, k))
            relayout_piece(jnp.minimum((c + 1) // 2, 2), 1 - g, k, gates)
            hp = jnp.maximum(c - 4, 0) * 8 + k
            wo_relayout(jnp.where(c >= 4, hp // 2, 8), hp, gates)
        return carry

    def chunk_pair(mm, carry):
        for g, c in ((1, 2 * mm + 1), (0, 2 * mm + 2)):
            for cs in range(2 - g, 6, 2):
                pl.when(c == cs)(functools.partial(issue, cs))

            @pl.when(c < 6)
            def _():
                loop("chunk", 0, 8 // PP, functools.partial(chunk_body, c, g), 0)
        return carry
    lax.fori_loop(0, 3, chunk_pair, 0)

    for cp in small:
        cp.wait()
    dd = ssmd_ref[0].astype(F32)
    for g in range(NG):
        sk = sk_ref[g].astype(F32)
        for j in range(KS):
            taps[g, j] = jnp.broadcast_to(sk[j:j + 1], (8, 128))
        taps[g, KS] = jnp.broadcast_to(dd[g:g + 1], (8, 128))

    def rep(x, rows):
        return x if rows == 8 else jnp.concatenate([x] * (rows // 8), axis=0)

    def a_stage1_pre(g, p, never, par=None, gates=None):
        par = g % 2 if par is None else par
        r = p * C if isinstance(p, int) else pl.multiple_of(p * C, C)
        r2 = 2 * r if isinstance(p, int) else pl.multiple_of(2 * r, 2 * C)
        kw = pltpu.bitcast(abuf[g, 1, pl.ds(r2, 2 * C), :], U32)
        vw = pltpu.bitcast(abuf[g, 2, pl.ds(r2, 2 * C), :], U32)
        if isinstance(p, int):
            assert p == 0
            halo = jnp.zeros((8, 128), U32)
        else:
            rh = pl.multiple_of(jnp.maximum(r2 - 16, 0), 16)
            halo = jnp.where(p == 0, jnp.uint32(0), pltpu.bitcast(abuf[g, 1, pl.ds(rh, 16), :], U32))
        sub = lax.broadcasted_iota(jnp.int32, (8, 128), 0)
        cur = [kw[b:b + 8] for b in range(0, C, 8)]
        if gates is not None:
            cur = [jnp.where(never, pltpu.bitcast(gates[(i * len(gates)) // len(cur)], U32), x)
                   for i, x in enumerate(cur)]
        blk = [halo] + cur
        rolled = {sh: [pltpu.roll(x, sh, 0) for x in blk] for sh in (1, 2)}

        def shifted(b, sh):
            return jnp.where(sub < sh, rolled[sh][b // 8], rolled[sh][b // 8 + 1])
        t = [taps[g, j] for j in range(KS)]
        parts = {}
        last = None
        mode = cfg["chain1"] if (never is not None and gates is None) else 0
        blocks = list(range(0, C, 8))
        if cfg.get("rev1"):
            blocks = [b + h for b in range(C // 2 - 8, -8, -8) for h in (0, C // 2)]
        for b in blocks:
            w0 = cur[b // 8]
            w1 = shifted(b, 1)
            w2 = shifted(b, 2)
            if last is not None and mode == 3:
                w0 = jnp.where(never, last, w0)
                w1 = jnp.where(never, last, w1)
            e0, o0 = _unpack(w0, 0), _unpack(w0, 1)
            e1, o1 = _unpack(w1, 0), _unpack(w1, 1)
            o2 = _unpack(w2, 1)
            ke = e0 * t[0]
            ko = o0 * t[0]
            if last is not None and mode == 1:
                ke = jnp.where(never, last[0], ke)
                ko = jnp.where(never, last[1], ko)
            if last is not None and mode == 2:
                ke = jnp.where(never, last[1], ke)
            ke = (ke + o1 * t[1] + e1 * t[2] + o2 * t[3]) * _unpack(vw[b:b + 8], 0)
            if mode >= 2:
                ko = jnp.where(never, ke, ko)
            ko = (ko + e0 * t[1] + o1 * t[2] + e1 * t[3]) * _unpack(vw[b:b + 8], 1)
            parts[b] = _pack(ke, ko)
            last = parts[b] if mode == 3 else (ke, ko)
        parts = [parts[b] for b in range(0, C, 8)]
        kv = jnp.concatenate(parts, axis=0)
        kvb[par, pl.ds(r, C), :] = kv
        return kv

    def a_stage1_u(g, p, kv):
        fwd = pltpu.bitcast(fwd_ref[...], BF16)
        if kv is None:
            kv = kvb[g % 2, pl.ds(pl.multiple_of(p * C, C), C), :]
        for u in range(2):
            w = pltpu.bitcast(kv[u * C // 2:(u + 1) * C // 2], BF16)
            if cfg["split_u"]:
                for hf in range(2):
                    ubuf[g % 2, 2 * p + u, pl.ds(OFF[hf], C), :] = _dot(fwd[hf * C:(hf + 1) * C], w)
            else:
                d = _dot(fwd, w)
                for hf in range(2):
                    ubuf[g % 2, 2 * p + u, pl.ds(OFF[hf], C), :] = d[hf * C:(hf + 1) * C]

    def a_stage1_h(g, p, sub):
        fwd = pltpu.bitcast(fwd_ref[...], BF16)
        hc = [hbuf[g, p // U, :, pl.ds((2 * sub + u) * C, C)] for u in range(2)]
        if cfg["split_h"]:
            hs = [jnp.concatenate([_dot_nt(fwd[hf * C:(hf + 1) * C], hc[u])
                                   for hf in range(2)], axis=0) for u in range(2)]
        else:
            hs = [_dot_nt(fwd, hc[u]) for u in range(2)]
        prev = jnp.where(p == 0, 0.0, hlast[...])
        hlast[...] = hs[1]
        hc = C // 2
        for u, (cur, prv) in enumerate(((hs[0], prev), (hs[1], hs[0]))):
            gbuf[g % 2, 7 + 2 * p + u, pl.ds(OFF[2], C), :] = jnp.concatenate(
                [cur[0:hc] - prv[C:C + hc], cur[hc:C] + prv[C + hc:]], axis=0)
            gbuf[g % 2, 7 + 2 * p + u, pl.ds(OFF[3], C), :] = jnp.concatenate(
                [cur[C:C + hc] + prv[0:hc], cur[C + hc:] - prv[hc:C]], axis=0)

    def a_stage2(gp, p, slot, chain, never, gates=None, last=None):
        b = gp % 2
        RB = 8
        re = [[], []]
        im = [[], []]
        done = 0
        for r in [r0 + blk for r0 in range(0, C // 2, RB) for blk in (0, C // 2)]:
            gr = [gbuf[b, 7 + p + 8 - j, pl.ds(OFF[2] + r, RB), :] for j in range(NC)]
            gi = [gbuf[b, 7 + p + 8 - j, pl.ds(OFF[3] + r, RB), :] for j in range(NC)]
            ur = [ubuf[b, j, pl.ds(OFF[0] + r, RB), :] for j in range(NC)]
            ui = [ubuf[b, j, pl.ds(OFF[1] + r, RB), :] for j in range(NC)]
            for o, (nt, off) in enumerate(((8, 8), (16, 0))):
                if gates is not None:
                    gs = cfg["gate_terms"]
                    ar = ai = None
                    for j in range(nt):
                        g0 = gr[j + off]
                        if j % gs == 0:
                            gt = gates[(done * len(gates)) // (24 * 16)]
                            g0 = jnp.where(never, gt, g0)
                        done += 1
                        tr, ti = g0 * ur[j], g0 * ui[j]
                        ar = tr if ar is None else ar + tr
                        ai = ti if ai is None else ai + ti
                        ar = ar - gi[j + off] * ui[j]
                        ai = ai + gi[j + off] * ur[j]
                    last = (ar, ai)
                elif chain == 1:
                    ar = gr[off] * ur[0]
                    ai = gr[off] * ui[0]
                    if last is not None:
                        ar = jnp.where(never, last[0], ar)
                        ai = jnp.where(never, last[1], ai)
                    ar = ar - gi[off] * ui[0]
                    ai = ai + gi[off] * ur[0]
                    for j in range(1, nt):
                        ar = ar + gr[j + off] * ur[j]
                        ai = ai + gr[j + off] * ui[j]
                        ar = ar - gi[j + off] * ui[j]
                        ai = ai + gi[j + off] * ur[j]
                    last = (ar, ai)
                else:
                    ar = gr[off] * ur[0]
                    if last is not None:
                        ar = jnp.where(never, last, ar)
                    ar = ar - gi[off] * ui[0]
                    for j in range(1, nt):
                        ar = ar + gr[j + off] * ur[j]
                        ar = ar - gi[j + off] * ui[j]
                    ai = jnp.where(never, ar, gr[off] * ui[0])
                    ai = ai + gi[off] * ur[0]
                    for j in range(1, nt):
                        ai = ai + gr[j + off] * ui[j]
                        ai = ai + gi[j + off] * ur[j]
                    last = ai
                re[o].append(ar)
                im[o].append(ai)
                if r >= C // 2:
                    rows = pl.ds(r - C // 2, RB)
                    ev = _pack(re[o][-2] + ar, im[o][-2] - ai)
                    od = _pack(re[o][-2] - ar, im[o][-2] + ai)
                    ystage[slot, o, 0, rows, :] = ev
                    ystage[slot, o, 1, rows, :] = od
                    if cfg["chain_pack"] and chain == 1:
                        last = (pltpu.bitcast(ev, F32), pltpu.bitcast(od, F32))
        return list(last) if isinstance(last, tuple) else [last]

    def a_stage3(gp, gq, p, slot):
        inv = pltpu.bitcast(inv_ref[...], BF16)
        dd = rep(taps[gq, KS], C // 2)
        for o in range(2):
            i = p + 8 * o
            kvw = kvb[gp % 2, pl.ds(pl.multiple_of(i * (C // 2), C // 2), C // 2), :]
            qw = pltpu.bitcast(abuf[gq, 0, pl.ds(pl.multiple_of(i * C, C), C), :], U32)
            res = []
            for e in range(2):
                y = _dot(inv[e * (C // 2):(e + 1) * (C // 2)], pltpu.bitcast(ystage[slot, o, e], BF16))
                res.append(_unpack(qw, e) * (y + _unpack(kvw, e) * dd))
            out = pltpu.bitcast(_pack(res[0], res[1]), BF16)
            aout[gq, pl.ds(pl.multiple_of(i * 4, 4), 4)] = out.reshape(4, SEG, 128)

    scale = DH ** (-0.5)

    def w_slab(m, h, z):
        j = h // 2
        row = slab_row(m, h % 2, j % 8)
        row = row if z is None else pl.multiple_of(z + row, 8)
        return pltpu.bitcast(w_parts[j // 8][pl.ds(row, D // 2), :], BF16)

    shared = {}

    class Step:
        def __init__(self, s, u):
            self.s = s
            self.slot = u
            self.z = None if (u == 0 or not cfg.get("zoff")) else pl.multiple_of(jnp.where(s > 1000 + u, 32, 0), 32)
            self.g = s // 8
            self.p = s % 8
            self.qkv, self.ps, self.os = {}, {}, []
            self.acc = [None] * NB
            self.ocat = {}
            self.gates = []
            self.lead = {}
            self.prev = None
            self.early = {}
            self.ties = []

        def start(self, mem):
            x = xbuf[self.s, pl.ds(M, SEG - M), :].astype(F32)
            self.lhsf = jnp.concatenate([mem, x], axis=0)
            self.lhs = self.lhsf.astype(BF16)

        def proj_early(self, m, j, k):
            self.early[m, j] = (k, [_dot(self.lhsf[:, :k].astype(BF16), w_slab(m, 2 * j + e, self.z)[:k])
                                    for e in range(2)])

        def proj(self, m, j):
            if (m, j) in self.early:
                k, part = self.early[m, j]
                a, b = [_dot(self.lhsf[:, k:].astype(BF16), w_slab(m, 2 * j + e, self.z)[k:]) + part[e]
                        for e in range(2)]
            else:
                a = _dot(self.lhs, w_slab(m, 2 * j, self.z))
                b = _dot(self.lhs, w_slab(m, 2 * j + 1, self.z))
            self.gates += vregs(a, b)
            lead = qkvb[self.s, m * NPAIR + j]
            if m == 0:
                r = jnp.concatenate([a, b, _unpack(lead, 0), _unpack(lead, 1)], axis=0).astype(BF16)
            else:
                r = pltpu.bitcast(jnp.concatenate([_pack(a, b), lead], axis=0), BF16)
            self.qkv[m, j] = r

        def probs(self, j):
            fill = fill_ref[pl.ds(0, R), pl.ds(0, R)]
            sc = jnp.where(fill == 0.0, _dot_nt(self.qkv[0, j], self.qkv[1, j]) * scale, fill)
            mx = jnp.max(sc, axis=-1, keepdims=True)
            e = jnp.exp(sc - mx)
            l = jnp.sum(e, axis=-1, keepdims=True)
            r = pl.reciprocal(l, approx=True)
            r = r * (2.0 - l * r)
            self.ps[j] = (e * r).astype(BF16)

        def attend(self, j):
            o = _dot(self.ps[j], self.qkv[2, j])
            la, lb = o[2 * SEG:2 * SEG + M], o[2 * SEG + M:]
            if cfg["strassen_e"]:
                rows = pl.ds(pl.multiple_of((self.s // 2) * M, M), M)
                if self.prev is None:
                    self.lead[j] = (la, lb)
                    forms = {2: la + lb, 5: la}
                else:
                    a11, a12 = self.prev.lead[j]
                    forms = {0: a11 + lb, 1: la + lb, 3: la - a11, 4: a12 - lb, 6: lb}
                for f, v in forms.items():
                    ob[f * NPAIR + j, rows, :] = v.astype(BF16)
            else:
                rows = pl.ds(pl.multiple_of(self.s * M, M), M)
                ob[2 * j, rows, :] = la.astype(BF16)
                ob[2 * j + 1, rows, :] = lb.astype(BF16)
            self.os += [o[0:SEG], o[SEG:2 * SEG]]

        def wo(self, h0, h1, ns):
            if (h0, h1) not in self.ocat:
                self.ocat[h0, h1] = jnp.concatenate(self.os[h0:h1], axis=1).astype(BF16)
            o = self.ocat[h0, h1]
            for n in ns:
                row = h0 * 64 if self.z is None else pl.multiple_of(self.z + h0 * 64, 32)
                w = wo_u[n, pl.ds(row, (h1 - h0) * 64), :]
                if cfg["tie"] == n + 1 + (NB if h1 == H else 0):
                    parts = [jnp.where(self.s > 1000, pltpu.bitcast(t, U32), w[8 * i:8 * i + 8])
                             for i, t in enumerate(self.ties)]
                    w = jnp.concatenate(parts + [w[8 * len(parts):]], axis=0)
                d = _dot(o, pltpu.bitcast(w, BF16))
                self.acc[n] = d if self.acc[n] is None else d + self.acc[n]
                self.gates += [v for v in vregs(self.acc[n]) for _ in range((h1 - h0) // 8)]

        def finish(self):
            res = jnp.concatenate(self.acc, axis=1)
            obuf[self.s] = res.astype(BF16)
            return res[0:M]

        def run(self, item):
            kind = item[0]
            g, p = self.g, self.p
            never = (self.s if cfg["real_chain"] else p) > 1000
            if kind == "P":
                self.proj(item[1], item[2])
            elif kind == "E":
                self.proj_early(item[1], item[2], item[3])
            elif kind == "S":
                self.probs(item[1])
            elif kind == "V":
                self.attend(item[1])
            elif kind == "W":
                self.wo(item[1], item[2], item[3])
            elif kind == "A1":
                self.kv = a_stage1_pre(g, p, never)
            elif kind == "AU":
                a_stage1_u(g, p, self.kv)
            elif kind == "AH":
                a_stage1_h(g, p, self.slot)
            elif kind == "A2":
                tail = a_stage2(g + 1, p, self.slot, cfg["chain"], never, last=shared.get("a2"))
                if cfg["chain_a2"]:
                    shared["a2"] = tuple(tail)
            elif kind == "A3":
                a_stage3(g + 1, jnp.maximum(g - 1, 0), p, self.slot)
            elif kind == "N1":
                gn = (self.s + 1) // 8
                kv = a_stage1_pre(jnp.minimum(gn, NG - 1), (self.s + 1) % 8, never, gn % 2)
                if cfg["tie"]:
                    self.ties.append(pltpu.bitcast(kv[C - 8:C], F32))
            elif kind == "N2":
                tails = a_stage2((self.s + 1) // 8 + 1, (self.s + 1) % 8, 0, cfg["chain"], never)
                if cfg["tie"]:
                    self.ties += tails
            elif kind in ("G1", "G2"):
                t = self.s + U
                lo, hi = cfg["g1" if kind == "G1" else "g2"]
                gates = self.gates[(lo * len(self.gates)) // 100:(hi * len(self.gates)) // 100]
                if kind == "G1":
                    a_stage1_pre(jnp.minimum(t // 8, NG - 1), t % 8, never, (t // 8) % 2, gates)
                else:
                    a_stage2(t // 8 + 1, t % 8, self.slot, None, never, gates)
            elif kind == "PU":
                a_stage1_u(g, p, None)
            elif kind == "P3":
                a_stage3(g + 1, jnp.maximum(g - 1, 0), p, 0)

    pipe2 = False

    def steps(i, mem):
        s0 = i * U

        @pl.when(s0 % 8 == 0)
        def _():
            group_wait(s0 // 8)
        shared.clear()
        st = [Step(s0 + u, u) for u in range(U)]
        for u in range(1, U, 2):
            st[u].prev = st[u - 1]
        for u, item in order:
            if item[0] == "start":
                st[u].start(mem)
            elif item[0] == "finish":
                mem = st[u].finish()
            else:
                st[u].run(item)
        return mem

    loop("steps", 0, NSEG // U, steps, mem0_ref[...].astype(F32))

    ob_cp = pltpu.make_async_copy(
        obuf.at[:, pl.ds(M, SEG - M), :],
        out_hbm.at[:, pl.ds(M, SEG - M), pl.ds(D, D)], sems.at[SO])
    ob_cp.start()
    for g in range(NG - 1):
        pltpu.make_async_copy(
            aout.at[g], out_hbm.at[:, :, pl.ds(g * 128, 128)], sems.at[SO + 1]).start()

    EP = cfg["ep"]
    GL = NG - 1
    HS = cfg["ep_split"]

    def epi_strassen(it):
        never = it > 1000
        ns = [2 * it, 2 * it + 1]

        def blk(hp, u):
            return [wo_u[ns[u], pl.ds((2 * j + hp) * 64, 64), :] for j in range(NPAIR)]

        def mm(f, bs):
            lhs = jnp.concatenate([ob[f * NPAIR + j] for j in range(NPAIR)], axis=1)
            return _dot(lhs, pltpu.bitcast(jnp.concatenate(bs, axis=0), BF16))

        def cb(x, y, sign):
            return [comb(a, b, sign) for a, b in zip(x, y)]

        def put(u, par, c):
            for i in range(NSEG // 2):
                obb[ns[u], 2 * i + par] = c[M * i:M * i + M].astype(BF16)
        sched = cfg["ep_sched"]

        def hook(k):
            for u in range(2):
                if sched[u] == k:
                    a_stage3(GL, GL, ns[u], u)
        for u in range(2):
            a_stage2(GL, ns[u], u, cfg["ep_chain"], never)
        m5 = mm(2, blk(1, 1))
        m1 = mm(0, cb(blk(0, 0), blk(1, 1), 1))
        hook(2)
        m4 = mm(6, cb(blk(1, 0), blk(0, 0), -1))
        hook(3)
        put(0, 0, mm(4, cb(blk(1, 0), blk(1, 1), 1)) + (m1 + m4 - m5))
        hook(4)
        m3 = mm(5, cb(blk(0, 1), blk(1, 1), -1))
        put(1, 0, m3 + m5)
        hook(5)
        m2 = mm(1, blk(0, 0))
        put(0, 1, m2 + m4)
        hook(6)
        put(1, 1, mm(3, cb(blk(0, 0), blk(0, 1), 1)) + (m1 - m2 + m3))

    def epi(it, carry):
        def part(n, h0, h1):
            lhs = jnp.concatenate([ob[h] for h in range(h0, h1)], axis=1)
            return _dot(lhs, pltpu.bitcast(wo_u[n, pl.ds(h0 * 64, (h1 - h0) * 64), :], BF16))
        if cfg["strassen_e"]:
            assert EP == 2 and U % 2 == 0 and not pipe2
            epi_strassen(it)
        for u in range(0 if cfg["strassen_e"] else EP):
            n = it * EP + u
            if pipe2:
                a_stage3(GL, GL, n, 0)
                a_stage2(GL, jnp.minimum(n + 1, 7), 0, cfg["ep_chain"], it > 1000)
                d = part(n, 0, H)
            else:
                a_stage2(GL, n, u % 2, cfg["ep_chain"], it > 1000)
                d = part(n, 0, HS)
                a_stage3(GL, GL, n, u % 2)
                d = part(n, HS, H) + d
            obb[n] = d.reshape(NSEG, M, 128).astype(BF16)
        for u in range(EP):
            n = it * EP + u
            col = pl.multiple_of(D + n * 128, 128)
            pltpu.make_async_copy(
                obb.at[n], out_hbm.at[:, pl.ds(0, M), pl.ds(col, 128)], sems.at[SO + 2]).start()
        for o in range(2):
            rows = pl.ds((it * EP + 8 * o) * 4, 4 * EP)
            pltpu.make_async_copy(
                aout.at[GL, rows], out_hbm.at[rows, :, pl.ds(GL * 128, 128)], sems.at[SO + 1]).start()
        return carry
    loop("epi", 0, NB // EP, epi, 0)
    ob_cp.wait()
    self_wait(aout, SO + 1)
    self_wait(obb, SO + 2)


def _b_order(u, extra, o):
    ks = o.get("ks", 24)
    tmpl = [(x[0], int(x[1:])) for x in o.get("tmpl", "q0 v1 S1 k0 V2").split()]
    out = list(extra.get("pre", [])) + [(u, ("start",))]
    if u > 0:
        first = [(kind, t - lag) for t in range(3) for kind, lag in tmpl if kind in "qkv" and t >= lag]
        out += [(u, ("E", "qkv".index(kind), j, o.get("ek", 768))) for kind, j in first[:o.get("ne", 2)]]
    nw = 0
    for t in range(NPAIR + max(l for _, l in tmpl)):
        for kind, lag in tmpl:
            j = t - lag
            if j < 0:
                continue
            if j >= NPAIR:
                if kind in "qkv" and nw < NB:
                    out.append((u, ("W", 0, ks, (nw,))))
                    nw += 1
                continue
            out.append((u, ("P", "qkv".index(kind), j) if kind in "qkv" else (kind, j)))
        out += extra.get(t, [])
    out += extra.get("tail", [])
    out += [(u, ("W", 0, ks, tuple(range(nw, NB))))]
    out += extra.get("tail2", [])
    out += [(u, ("W", ks, H, tuple(range(NB))))]
    out += extra.get("end", [])
    out += [(u, ("finish",))]
    out += extra.get("post", [])
    return out


def _make_order(o):
    out = []
    U = len(o["a"])
    for u, d in enumerate(o["a"]):
        ex = {}
        for k, names in d.items():
            k = int(k) if k.isdigit() else k
            ex[k] = [(u - n.count("-") + n.count("+"), (n.lstrip("+-"),)) for n in names]
        out += _b_order(u, ex, o)
    return U, out


_DEFAULT_CFG = dict(
    order=dict(a=[{"pre": ["A1", "+A1", "++A1", "+++A1"], "0": ["AH"], "2": ["AU"], "4": ["+AU"], "6": ["+AH"],
                   "8": ["++AU"], "10": ["++AH"], "12": ["+++AU"],
                   "14": ["+++AH", "A2", "+A2", "++A2", "+++A2"]},
                  {}, {}, {"tail2": ["---A3", "--A3", "-A3", "A3"]}],
               tmpl="q0 v1 S1 k0 V2", ks=16, ne=2, ek=768),
    wo_issue={1: (0, 1), 2: (2, 3, 4), 3: (5, 6, 7)}, g_issue={4: (0,), 5: (1, 2, 3, 4, 5, 6, 7)},
    pp=4, ep=2, ep_split=24, ep_chain=1, chain=1, chain1=2, real_chain=1,
    split_u=0, split_h=0, tie=0, strassen=1, gate=1, up=2, nobc=1,
    strassen_e=1, ep_sched=(4, 6), g1=(85, 97), g2=(5, 85), gate_terms=8,
    chain_pack=1, chain_a2=1)


def _pack_rows(x):
    b = np.asarray(x, dtype=jnp.bfloat16).view(np.uint16).astype(np.uint32)
    return b[0::2] | (b[1::2] << 16)


def _build(cfg):
    fwd_np, inv_np = _dft_constants()
    fill_np = np.zeros((96, 128), np.float32)
    fill_np[:R, :R] = _mask_fill()
    nsub = len(cfg["order"]["a"])

    def run(A_q, A_k, A_v, A_shift_k, A_ssm_k, A_ssm_D, B_x, B_mem0, B_Wq, B_Wk, B_Wv, B_Wo):
        sk = A_shift_k.T.reshape(KS, NG, 128).transpose(1, 0, 2)
        any_spec = pl.BlockSpec(memory_space=pl.ANY)
        out = pl.pallas_call(
            functools.partial(_kernel, cfg),
            out_shape=jax.ShapeDtypeStruct((NSEG, SEG, 2 * D), BF16),
            in_specs=[any_spec] * 15,
            out_specs=any_spec,
            scratch_shapes=[
                pltpu.VMEM((48 * SLAB + 544, 128), U32),
                pltpu.VMEM((48 * SLAB + 544, 128), U32),
                pltpu.VMEM((NB, H * DH // 2, 128), U32),
                pltpu.VMEM((16, 128, 16, DH), BF16),
                pltpu.VMEM((9, 512, D), BF16),
                pltpu.VMEM((NSEG, SEG, D), BF16),
                pltpu.VMEM((4, NSEG, M, KQ), BF16),
                pltpu.VMEM((4, NSEG * M // 2, KQ), U32),
                pltpu.VMEM((5, 2, NSEG * M // 4, KQ), U32),
                pltpu.VMEM((NSEG, 3 * NPAIR, 8, 128), U32),
                (pltpu.VMEM((7 * NPAIR, NSEG * M // 2, DH), BF16) if cfg["strassen_e"]
                 else pltpu.VMEM((H, NSEG * M, DH), BF16)),
                pltpu.VMEM((NSEG, SEG, D), BF16),
                pltpu.VMEM((NB, NSEG, M, 128), BF16),
                pltpu.VMEM((NG, 3, S, 128), BF16),
                pltpu.VMEM((NG, NC // (2 * nsub), 128, 2 * C * nsub), BF16),
                pltpu.VMEM((2, S // 2, 128), U32),
                pltpu.VMEM((2, NC, SPEC, 128), F32),
                pltpu.VMEM((2, NC + 7, SPEC, 128), F32),
                pltpu.VMEM((2 * C, 128), F32),
                pltpu.VMEM((NG, NSEG, SEG, 128), BF16),
                pltpu.VMEM((max(nsub, 2), 2, 2, C // 2, 128), U32),
                pltpu.VMEM((C, C), U32),
                pltpu.VMEM((C // 2, C), U32),
                pltpu.VMEM((96, 128), F32),
                pltpu.VMEM((NG, 8, 8, 128), F32),
                pltpu.VMEM((M, D), BF16),
                pltpu.VMEM((NG, KS, 128), BF16),
                pltpu.VMEM((4, NG, 128), BF16),
                pltpu.SemaphoreType.DMA((62,)),
            ],
            compiler_params=pltpu.CompilerParams(vmem_limit_bytes=124 * 1024 * 1024,
                                                 disable_bounds_checks=bool(cfg["nobc"])),
        )(A_q.reshape(S, D), A_k.reshape(S, D), A_v.reshape(S, D), sk, A_ssm_k,
          A_ssm_D.reshape(NG, 128), B_x.reshape(NSEG, SEG, D), B_mem0.reshape(M, D),
          B_Wq, B_Wk, B_Wv, B_Wo.reshape(H * DH, D),
          jnp.asarray(_pack_rows(fwd_np)), jnp.asarray(_pack_rows(inv_np)), jnp.asarray(fill_np))
        return out.reshape(1, S, 2 * D)

    return run


@functools.partial(jax.jit, static_argnames=("B_seg_len",))
def pallas_concat_heads__ssm_conv_h3__memory_aug_recurrent_mem_tr__prompt_kernel(
    A_q: jax.Array,
    A_k: jax.Array,
    A_v: jax.Array,
    A_shift_k: jax.Array,
    A_ssm_k: jax.Array,
    A_ssm_D: jax.Array,
    B_x: jax.Array,
    B_mem0: jax.Array,
    B_Wq: jax.Array,
    B_Wk: jax.Array,
    B_Wv: jax.Array,
    B_Wo: jax.Array,
    B_seg_len: int = SEG,
):
    assert B_seg_len == SEG
    return _build(_DEFAULT_CFG)(A_q, A_k, A_v, A_shift_k, A_ssm_k, A_ssm_D, B_x, B_mem0,
                                B_Wq, B_Wk, B_Wv, B_Wo)
```

```python
import functools

import numpy as np
import jax
import jax.numpy as jnp
from jax import lax
import jax.experimental.pallas as pl
import jax.experimental.pallas.tpu as pltpu

F32 = jnp.float32
BF16 = jnp.bfloat16
U32 = jnp.uint32

S = 2048
D = 1024
H = 32
DH = 128
M = 8
SEG = 32
NSEG = S // SEG
U = 4
NPAIR = H // 2
R = 2 * (M + SEG)
SLAB = 520
KS = 4
NG = D // 128
KQ = D // 4
NB = D // 128
PP = 4
HR = NSEG * M // 4

TAF, TAI, TB, TC, TD, TE, NT = 0, 16, 32, 64, 192, 256, 512
WX, WT, WY, WK, NW = 0, 512, 1024, 1280, 1408


def _twiddles():
    tw = np.zeros((2, NT, 8), np.float64)

    def put(j, idx, z):
        tw[j, idx] = np.real(z)
        tw[j, idx + 1] = np.imag(z)
    s = np.arange(8)
    tau = 2j * np.pi
    for j in range(2):
        lx = 1j * np.pi * (1 + 4 * j) / 4096
        for d in range(8):
            put(j, TAF + 2 * d, np.exp(lx * 256 * d))
            put(j, TAI + 2 * d, np.exp(lx * 256 * d) / 2048)
        for r in range(4):
            for k in range(4):
                put(j, TB + 8 * k + 2 * r, np.exp((lx * 64 + tau * k / 16) * r))
            for k in range(16):
                put(j, TC + 8 * k + 2 * r, np.exp((lx * 16 + tau * k / 64) * r))
            for kb in range(8):
                put(j, TD + 8 * kb + 2 * r, np.exp((lx * 4 + tau * (s + 8 * kb) / 256) * r))
                for k3 in range(4):
                    put(j, TE + 8 * (4 * kb + k3) + 2 * r,
                        np.exp((lx + tau * (s + 8 * kb + 64 * k3) / 1024) * r))
    return np.ascontiguousarray(np.broadcast_to(tw[..., None], (2, NT, 8, 128))).astype(np.float32)


def _mask_fill():
    blk = np.concatenate([np.arange(M), M + np.arange(M, SEG)])
    lead = M + np.arange(M)
    qhead = np.concatenate([np.zeros(SEG), np.ones(SEG), np.zeros(M), np.ones(M)])
    qpos = np.concatenate([blk, blk, lead, lead])
    khead = np.arange(R) % 2
    kpos = np.concatenate([blk, lead])[np.arange(R) // 2]
    same = qhead[:, None] == khead[None, :]
    ok = (qpos[:, None] < M) | (qpos[:, None] >= kpos[None, :])
    fill = np.where(same, np.where(ok, 0.0, -1e9), -np.inf)
    return fill.astype(np.float32)


def _pack(lo, hi):
    return pltpu.pack_elementwise([lo, hi], packed_dtype=BF16)


def _unpack(w, index):
    return pltpu.unpack_elementwise(w, index=index, packed_dtype=BF16, unpacked_dtype=F32)


def _dot(a, b):
    return jnp.dot(a, b, preferred_element_type=F32)


def _dot_nt(a, b):
    return lax.dot_general(a, b, (((1,), (1,)), ((), ())), preferred_element_type=F32)


def _cadd(a, b):
    return (a[0] + b[0], a[1] + b[1])


def _csub(a, b):
    return (a[0] - b[0], a[1] - b[1])


def _cmul(a, w):
    return (a[0] * w[0] - a[1] * w[1], a[0] * w[1] + a[1] * w[0])


def _cmulc(a, w):
    return (a[0] * w[0] + a[1] * w[1], a[1] * w[0] - a[0] * w[1])


def _bfly_i(b, d, sg):
    p = (b[0] - d[1], b[1] + d[0])
    q = (b[0] + d[1], b[1] - d[0])
    return (p, q) if sg > 0 else (q, p)


def _dft4(x, sg):
    a, b = _cadd(x[0], x[2]), _csub(x[0], x[2])
    c, d = _cadd(x[1], x[3]), _csub(x[1], x[3])
    p, q = _bfly_i(b, d, sg)
    return [_cadd(a, c), p, _csub(a, c), q]


def _kernel(cfg,
            aq_hbm, ak_hbm, av_hbm, sk_hbm, ssmk_hbm, ssmd_hbm, x_hbm, mem0_hbm,
            wq_hbm, wk_hbm, wv_hbm, wo_hbm, tw_hbm, fill_hbm,
            out_hbm,
            w_a, w_b, wo_u, wstage, wostage, xbuf, xlead, xlead_u, xs_u, qkvb, ob, obuf, obb,
            abuf, hbuf, ht, kvb, wk, tw, aout, lst,
            fill_ref, taps, mem0_ref, sk_ref, ssmd_ref,
            sems):
    import contextlib
    scope = jax.named_scope if cfg.get("scopes") else (lambda name: contextlib.nullcontext())
    SW, SWO, SXL, SX, SH, SA, ST, SO, SS = 0, 16, 24, 28, 36, 44, 46, 48, 52
    only = cfg.get("only")

    def loop(name, lo, hi, body, init):
        if only is not None and name not in only:
            return init
        if cfg.get("scopes") == 2:
            def body2(i, c):
                with scope(name + "_it"):
                    return body(i, c)
            return lax.fori_loop(lo, hi, body2, init)
        with scope(name):
            return lax.fori_loop(lo, hi, body, init)
    w_hbms = (wq_hbm, wk_hbm, wv_hbm)
    a_hbms = (aq_hbm, ak_hbm, av_hbm)

    def w_copy(c, k):
        m, g = c // 2, c % 2
        slot = (c % 2) * 8 + k
        return pltpu.make_async_copy(
            w_hbms[m].at[pl.ds(k * 128, 128), pl.ds(16 * g, 16), :],
            wstage.at[slot], sems.at[SW + slot])

    def self_wait(ref, sem):
        pltpu.make_async_copy(ref, ref, sems.at[sem]).wait()

    def late_start(k):
        pltpu.make_async_copy(
            wo_hbm.at[pl.ds(k * 512, 512), :], wostage.at[k], sems.at[SWO + k]).start()
        for part in range(2):
            pltpu.make_async_copy(
                ssmk_hbm.at[pl.ds(k * 128, 128), pl.ds(part * (S // 2), S // 2)],
                hbuf.at[k, part], sems.at[SH + k]).start()

    def xlead_copy(q):
        return pltpu.make_async_copy(
            x_hbm.at[:, pl.ds(0, M), pl.ds(q * KQ, KQ)], xlead.at[q], sems.at[SXL + q])

    def x_copy(g):
        segs = pl.ds(g * 8, 8)
        return pltpu.make_async_copy(
            x_hbm.at[segs, pl.ds(M, SEG - M), :], xbuf.at[segs, pl.ds(M, SEG - M), :], sems.at[SX + g])

    def a_start(g):
        col = g * 128 if isinstance(g, int) else pl.multiple_of(g * 128, 128)
        for t in (1, 2, 0):
            pltpu.make_async_copy(
                a_hbms[t].at[:, pl.ds(col, 128)], abuf.at[g % 2, t], sems.at[SA + g % 2]).start()

    def tw_copy(j):
        return pltpu.make_async_copy(tw_hbm.at[j], tw.at[j], sems.at[ST + j])

    small = [pltpu.make_async_copy(src, dst, sems.at[SS + i]) for i, (src, dst) in enumerate((
        (fill_hbm, fill_ref), (mem0_hbm, mem0_ref), (sk_hbm, sk_ref), (ssmd_hbm, ssmd_ref.at[0])))]

    for q in range(4):
        xlead_copy(q).start()
        w_copy(0, 2 * q).start()
        w_copy(0, 2 * q + 1).start()
        for k in {2: (0, 1), 3: (2, 3, 4, 5, 6, 7)}.get(q, ()):
            w_copy(1, k).start()

    w_parts = (w_a, w_b)

    def slab_row(m, par, jl):
        return (m * 16 + par * 8 + jl) * SLAB

    def gated(x, i, n, gates):
        if gates is None:
            return x
        never, vals = gates
        v = vals[(i * len(vals) * 3) // (n * 4)]
        return jnp.where(never, pltpu.bitcast(v, U32), x)

    def vregs(*mats):
        return [m_[r:r + 8] for m_ in mats for r in range(0, m_.shape[0], 8)]

    def relayout_piece(m, g, k, gates=None, slot=None):
        slot = g * 8 + k if slot is None else slot
        dst = w_parts[g]
        base = slab_row(m, 0, 0) + k * 64
        for i in range(64):
            a = gated(pltpu.bitcast(wstage[slot, 2 * i], U32), i, 64, gates)
            b = pltpu.bitcast(wstage[slot, 2 * i + 1], U32)
            ev = (a & jnp.uint32(0xFFFF)) | (b << 16)
            od = (a >> 16) | (b & jnp.uint32(0xFFFF0000))
            dst[pl.ds(base + i, 8, stride=SLAB), :] = ev
            dst[pl.ds(base + 8 * SLAB + i, 8, stride=SLAB), :] = od

    def comb(x, y, sign):
        f = (lambda a, b: a + b) if sign > 0 else (lambda a, b: a - b)
        return _pack(f(_unpack(x, 0), _unpack(y, 0)), f(_unpack(x, 1), _unpack(y, 1)))

    def batch_pair(m, g, jl):
        it = m * NPAIR + 8 * g + jl
        rows = [pl.multiple_of(slab_row(m, par, jl), 8) for par in range(2)]

        def blk(kh, par):
            return w_parts[g][pl.ds(rows[par] + kh * (D // 4), D // 4), :]

        def mm(a, b):
            return _dot(pltpu.bitcast(jnp.concatenate(a, axis=1), BF16), pltpu.bitcast(b, BF16))

        def xs(f):
            return [xs_u[f, q] for q in range(2)]
        a11 = [xlead_u[q, pl.ds(0, HR), :] for q in (0, 1)]
        a22 = [xlead_u[q, pl.ds(HR, HR), :] for q in (2, 3)]
        m5 = mm(xs(2), blk(1, 1))
        m1 = mm(xs(0), comb(blk(0, 0), blk(1, 1), 1))
        m4 = mm(a22, comb(blk(1, 0), blk(0, 0), -1))
        c11 = mm(xs(4), comb(blk(1, 0), blk(1, 1), 1)) + (m1 + m4 - m5)
        m3 = mm(a11, comb(blk(0, 1), blk(1, 1), -1))
        qkvb[pl.ds(0, NSEG // 2), it] = _pack(c11, m3 + m5).reshape(NSEG // 2, M, DH)
        m2 = mm(xs(1), blk(0, 0))
        c22 = mm(xs(3), comb(blk(0, 0), blk(0, 1), 1)) + (m1 - m2 + m3)
        qkvb[pl.ds(NSEG // 2, NSEG // 2), it] = _pack(m2 + m4, c22).reshape(NSEG // 2, M, DH)
        return vregs(m5, m1, m4, c11, m3, m2, c22)

    def unit(n, carry):
        q, half = n // 2, n % 2
        never = n > 1000

        @pl.when(half == 0)
        def _():
            self_wait(xlead.at[q], SXL + q)
            for u in range(2):
                self_wait(wstage.at[2 * q + u], SW + 2 * q + u)
            xq = xlead[q].astype(F32).reshape(NSEG * M, KQ).astype(BF16)
            xlead_u[q] = pltpu.bitcast(xq, U32)
            for u in range(2):
                relayout_piece(0, 0, 2 * q + u)

        @pl.when(n == 6)
        def _():
            for k in range(8):
                w_copy(2, k).start()

        @pl.when(n >= 4)
        def _():
            for u in range(2):
                self_wait(wstage.at[2 * n + u], SW + 2 * n + u)
        res = []
        xq = pltpu.bitcast(xlead_u[q], BF16)
        for u in range(4):
            jl = 4 * half + u
            outs = []
            for par in range(2):
                acc = pl.ds(pl.multiple_of((2 * jl + par) * (NSEG * M), NSEG * M), NSEG * M)
                row = pl.multiple_of(slab_row(0, par, jl) + q * (KQ // 2), 8)
                w = pltpu.bitcast(w_a[pl.ds(row, KQ // 2), :], BF16)
                d = _dot(xq, w) + jnp.where(q == 0, 0.0, wk[acc, :])
                wk[acc, :] = d
                outs.append(d)
            qkvb[:, jl] = _pack(outs[0], outs[1]).reshape(NSEG, M, DH)
            res += outs
        for u in range(2):
            k = jnp.maximum(n - 4, 0) * 2 + u
            relayout_piece(0, 1, k, (never, vregs(*res[4 * u:4 * u + 4])),
                           slot=jnp.where(n < 4, u, 8 + k))
        gates = (never, vregs(*res))
        for r in range(0, HR, 8):
            for cb in range(2):
                cols = pl.ds(cb * 128, 128)
                i = 2 * (r // 8) + cb
                a11 = gated(xlead_u[half, pl.ds(r, 8), cols], i, HR // 4, gates)
                a22 = gated(xlead_u[2 + half, pl.ds(HR + r, 8), cols], i, HR // 4, gates)
                a21 = xlead_u[half, pl.ds(HR + r, 8), cols]
                a12 = xlead_u[2 + half, pl.ds(r, 8), cols]
                for f, (x, y, sg) in enumerate(((a11, a22, 1), (a21, a22, 1), (a11, a12, 1),
                                                (a21, a11, -1), (a12, a22, -1))):
                    xs_u[f, half, pl.ds(r, 8), cols] = comb(x, y, sg)
        return carry
    loop("units", 0, 8, unit, 0)

    def issue(c):
        if c + 2 < 6:
            for k in range(8):
                w_copy(c + 2, k).start()
        for k in {1: (0, 1), 2: (2, 3), 3: (4, 5, 6, 7)}.get(c, ()):
            late_start(k)
        if c == 1:
            for cp in small:
                cp.start()
        if c == 4:
            x_copy(0).start()
            a_start(0)
            tw_copy(0).start()
        if c == 5:
            tw_copy(1).start()
            a_start(1)
            for g in range(1, NG):
                x_copy(g).start()

    def late_relayout(src, hp, gates):
        half = hp % 2
        for r in range(16):
            blk = pltpu.bitcast(
                wostage[src, pl.ds(pl.multiple_of(half * 256 + r * 16, 16), 16), :], U32)
            row = pl.multiple_of(hp * 128 + r * 8, 8)
            for n in range(NB):
                wo_u[n, pl.ds(row, 8), :] = gated(blk[:, n * 128:(n + 1) * 128], r * NB + n, 16 * NB, gates)
        for t in range(8):
            tile = pltpu.bitcast(hbuf[src, half, :, pl.ds(t * 128, 128)], U32)
            tile = jnp.concatenate([gated(tile[0:8], t, 8, gates), tile[8:]], axis=0)
            row = pl.multiple_of(hp * 512 + t * 64, 64)
            ht[pl.ds(row, 64), :] = pltpu.bitcast(pltpu.bitcast(tile, BF16).T, U32)

    def chunk_body(c, g, it, carry):
        @pl.when(c < 5)
        def _():
            for u in range(PP):
                slot = (1 - g) * 8 + it * PP + u
                self_wait(wstage.at[slot], SW + slot)

        @pl.when(c >= 4)
        def _():
            for u in range(PP // 2):
                k = (c - 4) * 4 + it * (PP // 2) + u
                self_wait(wostage.at[k], SWO + k)
                self_wait(hbuf.at[k], SH + k)
        for u in range(PP):
            k = it * PP + u
            gates = (it > 1000, batch_pair(c // 2, g, k))
            relayout_piece(jnp.minimum((c + 1) // 2, 2), 1 - g, k, gates)
            hp = jnp.maximum(c - 4, 0) * 8 + k
            late_relayout(jnp.where(c >= 4, hp // 2, 8), hp, gates)
        return carry

    def chunk_pair(mm, carry):
        for g, c in ((1, 2 * mm + 1), (0, 2 * mm + 2)):
            for cs in range(2 - g, 6, 2):
                pl.when(c == cs)(functools.partial(issue, cs))

            @pl.when(c < 6)
            def _():
                loop("chunk", 0, 8 // PP, functools.partial(chunk_body, c, g), 0)
        return carry
    lax.fori_loop(0, 3, chunk_pair, 0)

    for cp in small:
        cp.wait()
    dd = ssmd_ref[0].astype(F32)
    for g in range(NG):
        sk = sk_ref[g].astype(F32)
        for j in range(KS):
            taps[g, j] = jnp.broadcast_to(sk[j:j + 1], (8, 128))
        taps[g, KS] = jnp.broadcast_to(dd[g:g + 1], (8, 128))

    def part_a(i, gates, kick=None):
        g, j = i // 2, i % 2
        sl = g % 2
        never = i > 1000
        nevers = [i > 3000, i > 4000]
        state = dict(last=None, done=0)
        total = 128 * 26 + 64 * 46 + (8 + 3) * 32 * 34 + 32 * 58 + 32 * 96
        zz = pl.multiple_of(jnp.where(never, 32, 0), 32)
        z = zz if cfg["a_dyn"] else 0
        zk = zz if cfg["a_dynk"] else 0
        zs = [pl.multiple_of(jnp.where(i > 2000 + e, 32, 0), 32) for e in range(2)]
        state["z"] = z
        state["unit"] = 0

        def token():
            return wk[pl.ds(state["z"] + 8 * NW, 8), :]

        def next_unit():
            if cfg["a_mem"]:
                state["unit"] += 1
                state["z"] = zs[state["unit"] % 2]
                for _ in range(cfg["a_delay"]):
                    t = token()
                    wk[pl.ds(state["z"] + 8 * NW, 8), :] = t
                    state["unit"] += 1
                    state["z"] = zs[state["unit"] % 2]

        def begin(xs, ops, ng=1):
            xs = list(xs)
            srcs = []
            if state["last"] is not None and cfg["a_chain"]:
                srcs.append(state["last"])
            if gates is not None:
                srcs.append(gates[min(state["done"] * len(gates) // total, len(gates) - 1)])
            state["done"] += ops
            ng = min(ng, len(xs))
            for t, src in enumerate(srcs):
                for e in range(ng if t == len(srcs) - 1 else 1):
                    x = xs[e]
                    xs[e] = jnp.where(never, src if src.dtype == x.dtype else pltpu.bitcast(src, x.dtype), x)
            return xs

        def ld(v):
            return wk[pl.ds(state["z"] + 8 * v, 8), :]

        def st(v, x):
            wk[pl.ds(state["z"] + 8 * v, 8), :] = x

        def st_t(v, s, x):
            wk[pl.ds(state["z"] + 8 * v + s, 8, stride=8), :] = x

        def twid(idx):
            return (tw[j, idx], tw[j, idx + 1])

        def natural(w, hh):
            return pltpu.bitcast(w, BF16).astype(F32)[8 * hh:8 * hh + 8]

        def kv_st(v, x):
            if cfg["a_mem"]:
                st(WK + v, pltpu.bitcast(x, F32))
            else:
                kvb[pl.ds(zk + 8 * v, 8), :] = x

        def kv_ld(v):
            if cfg["a_mem"]:
                return pltpu.bitcast(ld(WK + v), U32)
            return kvb[pl.ds(zk + 8 * v, 8), :]

        def pass_kv():
            sub = lax.broadcasted_iota(jnp.int32, (8, 128), 0)
            t = [taps[g, a] for a in range(KS)]
            prev = {sh: jnp.zeros((8, 128), U32) for sh in (1, 2)}
            for v in range(S // 16):
                w0 = pltpu.bitcast(abuf[sl, 1, pl.ds(16 * v, 16), :], U32)
                vw = pltpu.bitcast(abuf[sl, 2, pl.ds(16 * v, 16), :], U32)
                if cfg["a_mem"]:
                    w0 = jnp.where(never, pltpu.bitcast(token(), U32), w0)
                w0, = begin([w0], 26)
                cur = {sh: pltpu.roll(w0, sh, 0) for sh in (1, 2)}
                w1, w2 = [jnp.where(sub < sh, prev[sh], cur[sh]) for sh in (1, 2)]
                prev = cur
                e0, o0, e1, o1, o2 = (_unpack(w0, 0), _unpack(w0, 1), _unpack(w1, 0),
                                      _unpack(w1, 1), _unpack(w2, 1))
                ke = (e0 * t[0] + o1 * t[1] + e1 * t[2] + o2 * t[3]) * _unpack(vw, 0)
                ko = (o0 * t[0] + e0 * t[1] + o1 * t[2] + e1 * t[3]) * _unpack(vw, 1)
                kv = _pack(ke, ko)
                kv_st(v, kv)
                next_unit()
                state["last"] = kv

        def merge(vals):
            g_ = vals[-1]
            if cfg["a_merge"]:
                seq = list(vals[:-1])[:cfg["a_merge"]] + [vals[e % len(vals)] for e in range(cfg["a_pad"])]
                for e, v in enumerate(seq):
                    g_ = jnp.maximum(v, g_) if cfg["a_mop"] else jnp.where(nevers[e % 2], v, g_)
            state["last"] = g_

        def pairs(flat):
            return [(flat[2 * e], flat[2 * e + 1]) for e in range(len(flat) // 2)]

        def fwd4(locs, t0):
            if cfg["a_stag"]:
                k = cfg["a_stag"]
                v = [(ld(locs[0][0]), ld(locs[0][1]))]
                v += [tuple(begin([ld(x) for x in locs[r]], ops, k)) for r, ops in ((2, 10), (1, 6), (3, 18))]
                v = [v[0], v[2], v[1], v[3]]
            else:
                v = pairs(begin([ld(x) for loc in locs[::-1] for x in loc], 34, cfg["a_g4"]))[::-1]
            return _dft4([v[0]] + [_cmul(v[r], twid(t0 + 2 * r)) for r in range(1, 4)], +1)

        def inv4(v, t0):
            o = _dft4(v, -1)
            if cfg["a_stag"]:
                state["done"] -= 12
                o[1] = tuple(begin(o[1], 6, cfg["a_stag"]))
                o[3] = tuple(begin(o[3], 6, cfg["a_stag"]))
            return [o[0]] + [_cmulc(o[r], twid(t0 + 2 * r)) for r in range(1, 4)]

        def ld4(locs, ops):
            return pairs(begin([ld(x) for loc in locs for x in loc], ops, cfg["a_g4i"]))

        def put4(locs, o):
            for loc, x in zip(locs, o):
                st(loc[0], x[0])
                st(loc[1], x[1])
            merge([x for c in o for x in c])
            next_unit()

        def xloc(sig, n):
            return (WX + 256 * sig + 2 * n, WX + 256 * sig + 2 * n + 1)

        def tloc(base, kb, l):
            v = base + 32 * kb + 16 * (l // 8) + l % 8
            return (v, v + 8)

        def put4_t(dsts, o):
            for (blk, slot), x in zip(dsts, o):
                st_t(blk, slot, x[0])
                st_t(blk + 8, slot, x[1])
            merge([x for c in o for x in c])
            next_unit()

        def forward(sig, src):
            for n in range(32):
                ws = begin([src(n // 2 + 16 * d) for d in range(8)], 46, cfg["a_ga"])
                if cfg["a_mem"] and sig == 1:
                    tk = pltpu.bitcast(token(), U32)
                    ws = [jnp.where(never, tk, w) if d < cfg["a_ga"] else w for d, w in enumerate(ws)]
                x = [natural(w, n % 2) for w in ws]
                cs = []
                for d in range(4):
                    a, b = twid(TAF + 2 * d), twid(TAF + 2 * (d + 4))
                    if d == 0:
                        s_ = x[4] * b[0]
                        cs.append((x[0] + s_, s_))
                    else:
                        cs.append((x[d] * a[0] + x[d + 4] * b[0], x[d] * a[1] + x[d + 4] * b[1]))
                put4([xloc(sig, n + 32 * k0) for k0 in range(4)], _dft4(cs, +1))
            for k0 in range(4):
                for n in range(8):
                    locs = [xloc(sig, n + 8 * r + 32 * k0) for r in range(4)]
                    put4(locs, fwd4(locs, TB + 8 * k0))
            tb = WT + 256 * sig
            for k0 in range(4):
                for k1 in range(4):
                    k = k0 + 4 * k1
                    for a in range(2):
                        o = fwd4([xloc(sig, a + 2 * r + 8 * k1 + 32 * k0) for r in range(4)], TC + 8 * k)
                        put4_t([(tb + 32 * ((k + 16 * k2) // 8) + 16 * a, k % 8) for k2 in range(4)], o)
            for kb in range(8):
                for e in range(4):
                    locs = [tloc(tb, kb, e + 4 * r) for r in range(4)]
                    put4(locs, fwd4(locs, TD + 8 * kb))

        def pass_e(sig):
            for kb in range(8):
                for k3 in range(4):
                    locs = [tloc(WT + 256 * sig, kb, r + 4 * k3) for r in range(4)]
                    t0 = TE + 8 * (4 * kb + k3)
                    o = fwd4(locs, t0)
                    if sig == 0:
                        hs = ld4([tloc(WT + 256, kb, r + 4 * k3) for r in range(4)], 58)
                        o = inv4([_cmul(a, b) for a, b in zip(o, hs)], t0)
                    put4(locs, o)

        def inverse():
            zb = WX + 256
            for kb in range(8):
                for e in range(4):
                    o = inv4(ld4([tloc(WT, kb, e + 4 * r) for r in range(4)], 34), TD + 8 * kb)
                    put4_t([(zb + 32 * kb + 16 * ((e + 4 * f) // 8), (e + 4 * f) % 8) for f in range(4)], o)
            for k0 in range(4):
                for k1 in range(4):
                    k = k0 + 4 * k1
                    for a in range(2):
                        v = ld4([tloc(zb, (k + 16 * r) // 8, 8 * a + k % 8) for r in range(4)], 34)
                        put4([xloc(0, a + 2 * b + 8 * k1 + 32 * k0) for b in range(4)], inv4(v, TC + 8 * k))
            for k0 in range(4):
                for n in range(8):
                    locs = [xloc(0, n + 8 * r + 32 * k0) for r in range(4)]
                    put4(locs, inv4(ld4(locs, 34), TB + 8 * k0))
            dskip = taps[g, KS]
            for n0 in range(32):
                cs = _dft4(ld4([xloc(0, n0 + 32 * r) for r in range(4)], 16), -1)
                outs = []
                for d in [dd_ + 4 * hh for dd_ in range(4) for hh in range(2)]:
                    n = n0 + 32 * d
                    a = twid(TAI + 2 * d)
                    if d < 4:
                        k = cfg["a_fine"]
                        if k and d % k == 0 and d > 0:
                            cs[d:d + k] = pairs(begin([x for c in cs[d:d + k] for x in c], 0, 99))
                        state["done"] += 20
                    c = cs[d % 4]
                    y = c[0] * a[0] if d == 0 else c[0] * a[0] + c[1] * a[1]
                    kv = natural(kv_ld(n // 2), n % 2)
                    y = y + jnp.where(j == 0, kv * dskip, ld(WY + n))
                    st(WY + n, y)
                    res = abuf[sl, 0, pl.ds(8 * n, 8), :].astype(F32) * y
                    aout[g, n // 4, pl.ds(8 * (n % 4), 8), :] = res.astype(BF16)
                    outs.append(res)
                    state["last"] = res
                merge(outs)
                next_unit()

        if kick is not None:
            mode, val = kick
            if mode == 1:
                state["last"] = val
            else:
                lst[jnp.where(never, 1, 0), pl.ds(0, 8), pl.ds(0, 128)] = pltpu.bitcast(val, U32)
                state["last"] = lst[jnp.where(nevers[0], 0, 1), pl.ds(0, 8), pl.ds(0, 128)]
        pass_kv()
        forward(1, lambda v: ht[pl.ds(pl.multiple_of(g * (S // 2), S // 2) + 8 * v, 8), :])
        pass_e(1)
        forward(0, kv_ld)
        pass_e(0)
        inverse()
        assert state["done"] == total, state["done"]
        return token() if cfg["a_mem"] else state["last"]

    scale = DH ** (-0.5)

    def w_slab(m, h):
        j = h // 2
        return pltpu.bitcast(w_parts[j // 8][pl.ds(slab_row(m, h % 2, j % 8), D // 2), :], BF16)

    def pick(vs, sel):
        return [vs[e] for e in sel]

    class Step:
        def __init__(self, s, u, prev, gates):
            self.s = s
            self.u = u
            self.prev = prev
            self.gates = gates
            self.qkv, self.ps, self.os = {}, {}, []
            self.acc = [None] * NB
            self.ocat, self.lead, self.early = {}, {}, {}
            self.tie = None

        def start(self, mem):
            x = xbuf[self.s, pl.ds(M, SEG - M), :].astype(F32)
            self.lhsf = jnp.concatenate([mem, x], axis=0)
            self.lhs_v = self.lhsf.astype(BF16)
            self.lhs_h = [self.lhsf[:, :D // 2].astype(BF16), self.lhsf[:, D // 2:].astype(BF16)]
            if cfg["lhs_mem"]:
                self.lslot = jnp.where(self.s > 1000, U, self.u)
                lst[self.lslot] = pltpu.bitcast(self.lhsf.astype(BF16), U32)

        @property
        def lhs(self):
            if cfg["lhs_mem"]:
                return pltpu.bitcast(lst[self.lslot], BF16)
            return self.lhs_v

        def proj_early(self, m, j, k):
            self.early[m, j] = (k, [_dot(self.lhsf[:, :k].astype(BF16), w_slab(m, 2 * j + e)[:k])
                                    for e in range(2)])

        def proj(self, m, j):
            if (m, j) in self.early:
                k, part = self.early[m, j]
                a, b = [_dot(self.lhsf[:, k:].astype(BF16), w_slab(m, 2 * j + e)[k:]) + part[e]
                        for e in range(2)]
                self.gates += vregs(a, b)
            elif cfg["psplit"]:
                res = []
                for e in range(2):
                    w = w_slab(m, 2 * j + e)
                    d0 = _dot(self.lhs_h[0], w[:D // 2])
                    d1 = _dot(self.lhs_h[1], w[D // 2:]) + d0
                    self.gates += vregs(d0, d1)
                    res.append(d1)
                a, b = res
            else:
                a = _dot(self.lhs, w_slab(m, 2 * j))
                b = _dot(self.lhs, w_slab(m, 2 * j + 1))
                self.gates += [v for x in (a, b) for v in pick(vregs(x), cfg["wq"])]
            lead = qkvb[self.s, m * NPAIR + j]
            if m == 0:
                r = jnp.concatenate([a, b, _unpack(lead, 0), _unpack(lead, 1)], axis=0).astype(BF16)
            else:
                r = pltpu.bitcast(jnp.concatenate([_pack(a, b), lead], axis=0), BF16)
            self.qkv[m, j] = r

        def probs(self, j):
            fill = fill_ref[pl.ds(0, R), pl.ds(0, R)]
            sc = jnp.where(fill == 0.0, _dot_nt(self.qkv[0, j], self.qkv[1, j]) * scale, fill)
            mx = jnp.max(sc, axis=-1, keepdims=True)
            e = jnp.exp(sc - mx)
            l = jnp.sum(e, axis=-1, keepdims=True)
            r = pl.reciprocal(l, approx=True)
            r = r * (2.0 - l * r)
            self.ps[j] = (e * r).astype(BF16)

        def attend(self, j):
            o = _dot(self.ps[j], self.qkv[2, j])
            la, lb = o[2 * SEG:2 * SEG + M], o[2 * SEG + M:]
            rows = pl.ds(pl.multiple_of((self.s // 2) * M, M), M)
            if self.prev is None:
                self.lead[j] = (la, lb)
                forms = {2: la + lb, 5: la}
            else:
                a11, a12 = self.prev.lead[j]
                forms = {0: a11 + lb, 1: la + lb, 3: la - a11, 4: a12 - lb, 6: lb}
            for f, v in forms.items():
                ob[f * NPAIR + j, rows, :] = v.astype(BF16)
            self.os += [o[0:SEG], o[SEG:2 * SEG]]

        def wo(self, h0, h1, ns):
            hs = cfg["wsplit"]
            for n in ns:
                for h in range(h0, h1, hs):
                    he = min(h + hs, h1)
                    if h not in self.ocat:
                        self.ocat[h] = jnp.concatenate(self.os[h:he], axis=1).astype(BF16)
                    w = wo_u[n, pl.ds(h * 64, (he - h) * 64), :]
                    if self.tie is not None and n == cfg["tie_n"] and h == h0:
                        w = jnp.concatenate(
                            [jnp.where(self.s > 1000, pltpu.bitcast(self.tie, U32), w[0:8]), w[8:]], axis=0)
                    d = _dot(self.ocat[h], pltpu.bitcast(w, BF16))
                    self.acc[n] = d if self.acc[n] is None else d + self.acc[n]
                    self.gates += pick(vregs(self.acc[n]), cfg["ww"])

        def finish(self):
            res = jnp.concatenate(self.acc, axis=1)
            obuf[self.s] = res.astype(BF16)
            return res[0:M]

    def steps(i, mem):
        g = i // 2

        @pl.when(i % 2 == 0)
        def _():
            x_copy(g).wait()
            self_wait(abuf.at[g % 2], SA + g % 2)

            @pl.when(jnp.logical_and(g >= 1, g < NG - 1))
            def _():
                a_start(g + 1)

        @pl.when(i < 2)
        def _():
            self_wait(tw.at[i], ST + i)
        gates = []
        prev = None
        for u in range(U):
            st = Step(i * U + u, u, prev if u % 2 else None, gates)
            prev = st
            for item in _step_order(u, cfg):
                kind = item[0]
                if kind == "start":
                    st.start(mem)
                elif kind == "finish":
                    mem = st.finish()
                elif kind == "A":
                    if cfg["a"]:
                        lo, hi = cfg["a_span"]
                        gs = gates[lo * len(gates) // 100:hi * len(gates) // 100] if cfg["a_pace"] else None
                        kick = (cfg["a_kick"], gates[lo * len(gates) // 100]) if cfg["a_kick"] else None
                        tail = part_a(i, gs, kick)
                        st.tie = tail if cfg["a_tie"] else None
                else:
                    dict(P=st.proj, E=st.proj_early, S=st.probs, V=st.attend, W=st.wo)[kind](*item[1:])
        return mem

    loop("steps", 0, NSEG // U, steps, mem0_ref[...].astype(F32))

    ob_cp = pltpu.make_async_copy(
        obuf.at[:, pl.ds(M, SEG - M), :],
        out_hbm.at[:, pl.ds(M, SEG - M), pl.ds(D, D)], sems.at[SO])
    ob_cp.start()
    for g in range(NG):
        pltpu.make_async_copy(
            aout.at[g], out_hbm.at[:, :, pl.ds(g * 128, 128)], sems.at[SO + 1]).start()

    def epi(it, carry):
        ns = [2 * it, 2 * it + 1]

        def blk(hp, u):
            return [wo_u[ns[u], pl.ds((2 * j + hp) * 64, 64), :] for j in range(NPAIR)]

        def mm(f, bs):
            lhs = jnp.concatenate([ob[f * NPAIR + j] for j in range(NPAIR)], axis=1)
            return _dot(lhs, pltpu.bitcast(jnp.concatenate(bs, axis=0), BF16))

        def cb(x, y, sign):
            return [comb(a, b, sign) for a, b in zip(x, y)]

        def put(u, par, c):
            for i in range(NSEG // 2):
                obb[ns[u], 2 * i + par] = c[M * i:M * i + M].astype(BF16)
        m5 = mm(2, blk(1, 1))
        m1 = mm(0, cb(blk(0, 0), blk(1, 1), 1))
        m4 = mm(6, cb(blk(1, 0), blk(0, 0), -1))
        put(0, 0, mm(4, cb(blk(1, 0), blk(1, 1), 1)) + (m1 + m4 - m5))
        m3 = mm(5, cb(blk(0, 1), blk(1, 1), -1))
        put(1, 0, m3 + m5)
        m2 = mm(1, blk(0, 0))
        put(0, 1, m2 + m4)
        put(1, 1, mm(3, cb(blk(0, 0), blk(0, 1), 1)) + (m1 - m2 + m3))
        for n in ns:
            col = pl.multiple_of(D + n * 128, 128)
            pltpu.make_async_copy(
                obb.at[n], out_hbm.at[:, pl.ds(0, M), pl.ds(col, 128)], sems.at[SO + 2]).start()
        return carry
    loop("epi", 0, NB // 2, epi, 0)
    ob_cp.wait()
    self_wait(aout, SO + 1)
    self_wait(obb, SO + 2)


def _step_order(u, cfg):
    ks = cfg["ks"]
    tmpl = [(x[0], int(x[1:])) for x in cfg["tmpl"].split()]
    vlag = dict(tmpl)["V"]
    out = [("start",)]
    if u > 0:
        first = [(kind, t - lag) for t in range(3) for kind, lag in tmpl if kind in "qkv" and t >= lag]
        out += [("E", "qkv".index(kind), j, cfg["ek"]) for kind, j in first[:cfg["ne"]]]
    early = [(h, n) for h in range(0, ks, 8) for n in range(NB)] if cfg["wint"] else \
        [(h, n) for n in range(NB) for h in range(0, ks, 8)]
    keep = cfg["wkeep"]
    for t in range(NPAIR + max(l for _, l in tmpl)):
        for kind, lag in tmpl:
            j = t - lag
            if j < 0:
                continue
            if j >= NPAIR:
                if kind in "qkv":
                    for _ in range(cfg["wfill"]):
                        if early:
                            h, n = early.pop(0)
                            out.append(("W", h, h + 8, (n,)))
                continue
            out.append(("P", "qkv".index(kind), j) if kind in "qkv" else (kind, j))
            if kind in cfg["wint_after"] and cfg["wint"] and len(early) > keep \
                    and early[0][0] // 2 + 3 + vlag + 1 <= t:
                h, n = early.pop(0)
                out.append(("W", h, h + 8, (n,)))
    out += [("W", h, h + 8, (n,)) for h, n in early]
    if u == U - 1 and cfg["a_tie"]:
        out.append(("A",))
    out += [("W", ks, H, tuple(range(NB))), ("finish",)]
    if u == U - 1 and not cfg["a_tie"]:
        out.append(("A",))
    return out


_DEFAULT_CFG = dict(tmpl="q0 v1 S1 k0 V2", ks=16, ne=2, ek=768, wsplit=8, wint=0, wkeep=10, wfill=2, wint_after="qk",
                    a=1, a_tie=1, tie_n=7, a_chain=1, a_pace=0, a_span=(5, 98),
                    a_dyn=0, a_dynk=0, psplit=0, a_stag=0, a_mem=0, a_delay=0, a_merge=7, a_pad=0, a_kick=2, a_mop=1, wq=(0, 1, 2, 3), ww=(0, 1, 2, 3), a_fine=1, lhs_mem=0, a_g4=1, a_g4i=1, a_ga=8)


def _build(cfg):
    tw_np = _twiddles()
    fill_np = np.zeros((96, 128), np.float32)
    fill_np[:R, :R] = _mask_fill()

    def run(A_q, A_k, A_v, A_shift_k, A_ssm_k, A_ssm_D, B_x, B_mem0, B_Wq, B_Wk, B_Wv, B_Wo):
        sk = A_shift_k.T.reshape(KS, NG, 128).transpose(1, 0, 2)
        any_spec = pl.BlockSpec(memory_space=pl.ANY)
        out = pl.pallas_call(
            functools.partial(_kernel, cfg),
            out_shape=jax.ShapeDtypeStruct((NSEG, SEG, 2 * D), BF16),
            in_specs=[any_spec] * 14,
            out_specs=any_spec,
            scratch_shapes=[
                pltpu.VMEM((48 * SLAB + 544, 128), U32),
                pltpu.VMEM((48 * SLAB + 544, 128), U32),
                pltpu.VMEM((NB, H * DH // 2, 128), U32),
                pltpu.VMEM((16, 128, 16, DH), BF16),
                pltpu.VMEM((9, 512, D), BF16),
                pltpu.VMEM((NSEG, SEG, D), BF16),
                pltpu.VMEM((4, NSEG, M, KQ), BF16),
                pltpu.VMEM((4, NSEG * M // 2, KQ), U32),
                pltpu.VMEM((5, 2, HR, KQ), U32),
                pltpu.VMEM((NSEG, 3 * NPAIR, 8, 128), U32),
                pltpu.VMEM((7 * NPAIR, NSEG * M // 2, DH), BF16),
                pltpu.VMEM((NSEG, SEG, D), BF16),
                pltpu.VMEM((NB, NSEG, M, 128), BF16),
                pltpu.VMEM((2, 3, S, 128), BF16),
                pltpu.VMEM((NG + 1, 2, 128, S // 2), BF16),
                pltpu.VMEM((NG * S // 2, 128), U32),
                pltpu.VMEM((S // 2 + 32, 128), U32),
                pltpu.VMEM((8 * NW + 64, 128), F32),
                pltpu.VMEM((2, NT, 8, 128), F32),
                pltpu.VMEM((NG, NSEG, SEG, 128), BF16),
                pltpu.VMEM((U + 1, SEG // 2, D), U32),
                pltpu.VMEM((96, 128), F32),
                pltpu.VMEM((NG, 8, 8, 128), F32),
                pltpu.VMEM((M, D), BF16),
                pltpu.VMEM((NG, KS, 128), BF16),
                pltpu.VMEM((4, NG, 128), BF16),
                pltpu.SemaphoreType.DMA((56,)),
            ],
            compiler_params=pltpu.CompilerParams(vmem_limit_bytes=124 * 1024 * 1024,
                                                 disable_bounds_checks=True),
        )(A_q.reshape(S, D), A_k.reshape(S, D), A_v.reshape(S, D), sk, A_ssm_k,
          A_ssm_D.reshape(NG, 128), B_x.reshape(NSEG, SEG, D), B_mem0.reshape(M, D),
          B_Wq, B_Wk, B_Wv, B_Wo.reshape(H * DH, D),
          jnp.asarray(tw_np), jnp.asarray(fill_np))
        return out.reshape(1, S, 2 * D)

    return run


@functools.partial(jax.jit, static_argnames=("B_seg_len",))
def pallas_concat_heads__ssm_conv_h3__memory_aug_recurrent_mem_tr__prompt_kernel(
    A_q: jax.Array,
    A_k: jax.Array,
    A_v: jax.Array,
    A_shift_k: jax.Array,
    A_ssm_k: jax.Array,
    A_ssm_D: jax.Array,
    B_x: jax.Array,
    B_mem0: jax.Array,
    B_Wq: jax.Array,
    B_Wk: jax.Array,
    B_Wv: jax.Array,
    B_Wo: jax.Array,
    B_seg_len: int = SEG,
):
    assert B_seg_len == SEG
    return _build(_DEFAULT_CFG)(A_q, A_k, A_v, A_shift_k, A_ssm_k, A_ssm_D, B_x, B_mem0,
                                B_Wq, B_Wk, B_Wv, B_Wo)
```

```python
import functools

import numpy as np
import jax
import jax.numpy as jnp
from jax import lax
import jax.experimental.pallas as pl
import jax.experimental.pallas.tpu as pltpu

F32 = jnp.float32
BF16 = jnp.bfloat16
U32 = jnp.uint32

S = 2048
D = 1024
H = 32
DH = 128
M = 8
SEG = 32
NSEG = S // SEG
U = 4
NPAIR = H // 2
R = 2 * (M + SEG)
SLAB = 520
KS = 4
NG = D // 128
KQ = D // 4
NB = D // 128
PP = 4
HR = NSEG * M // 4

TAF, TAI, TB, TC, TD, TE, NT = 0, 16, 32, 64, 192, 256, 512
WX, WS, WY, NW = 0, 512, 1024, 1280
LOG2E = 1.4426950408889634


def _twiddles():
    tw = np.zeros((2, NT, 8), np.float64)

    def put(j, idx, z):
        tw[j, idx] = np.real(z)
        tw[j, idx + 1] = np.imag(z)
    s = np.arange(8)
    tau = 2j * np.pi
    for j in range(2):
        lx = 1j * np.pi * (1 + 4 * j) / 4096
        for d in range(8):
            put(j, TAF + 2 * d, np.exp(lx * 256 * d))
            put(j, TAI + 2 * d, np.exp(lx * 256 * d) / 2048)
        for r in range(4):
            for k in range(4):
                put(j, TB + 8 * k + 2 * r, np.exp((lx * 64 + tau * k / 16) * r))
            for k in range(16):
                put(j, TC + 8 * k + 2 * r, np.exp((lx * 16 + tau * k / 64) * r))
            for kb in range(8):
                put(j, TD + 8 * kb + 2 * r, np.exp((lx * 4 + tau * (s + 8 * kb) / 256) * r))
                for k3 in range(4):
                    put(j, TE + 8 * (4 * kb + k3) + 2 * r,
                        np.exp((lx + tau * (s + 8 * kb + 64 * k3) / 1024) * r))
    return np.ascontiguousarray(np.broadcast_to(tw[..., None], (2, NT, 8, 128))).astype(np.float32)


def _mask_fill():
    blk = np.concatenate([np.arange(M), M + np.arange(M, SEG)])
    lead = M + np.arange(M)
    qhead = np.concatenate([np.zeros(SEG), np.ones(SEG), np.zeros(M), np.ones(M)])
    qpos = np.concatenate([blk, blk, lead, lead])
    khead = np.arange(R) % 2
    kpos = np.concatenate([blk, lead])[np.arange(R) // 2]
    same = qhead[:, None] == khead[None, :]
    ok = (qpos[:, None] < M) | (qpos[:, None] >= kpos[None, :])
    fill = np.where(same, np.where(ok, 0.0, -1e9), -np.inf)
    return fill.astype(np.float32)


def _pack(lo, hi):
    return pltpu.pack_elementwise([lo, hi], packed_dtype=BF16)


def _unpack(w, index):
    return pltpu.unpack_elementwise(w, index=index, packed_dtype=BF16, unpacked_dtype=F32)


def _dot(a, b):
    return jnp.dot(a, b, preferred_element_type=F32)


def _dot_nt(a, b):
    return lax.dot_general(a, b, (((1,), (1,)), ((), ())), preferred_element_type=F32)


def _cadd(a, b):
    return (a[0] + b[0], a[1] + b[1])


def _csub(a, b):
    return (a[0] - b[0], a[1] - b[1])


def _cmul(a, w):
    return (a[0] * w[0] - a[1] * w[1], a[0] * w[1] + a[1] * w[0])


def _cmulc(a, w):
    return (a[0] * w[0] + a[1] * w[1], a[1] * w[0] - a[0] * w[1])


def _bfly_i(b, d, sg):
    p = (b[0] - d[1], b[1] + d[0])
    q = (b[0] + d[1], b[1] - d[0])
    return (p, q) if sg > 0 else (q, p)


def _dft4(x, sg):
    a, b = _cadd(x[0], x[2]), _csub(x[0], x[2])
    c, d = _cadd(x[1], x[3]), _csub(x[1], x[3])
    p, q = _bfly_i(b, d, sg)
    return [_cadd(a, c), p, _csub(a, c), q]


def _kernel(cfg,
            aq_hbm, ak_hbm, av_hbm, sk_hbm, ssmk_hbm, ssmd_hbm, x_hbm, mem0_hbm,
            wq_hbm, wk_hbm, wv_hbm, wo_hbm, tw_hbm, fill_hbm,
            out_hbm,
            w_a, w_b, wo_u, wstage, wostage, xbuf, xlead, xlead_u, xs_u, qkvb, ob, obuf, obb,
            abuf, hbuf, ht, kvb, wk, tw, aout, kickbuf,
            fill_ref, taps, mem0_ref, sk_ref, ssmd_ref,
            sems):
    import contextlib
    scope = jax.named_scope if cfg.get("scopes") else (lambda name: contextlib.nullcontext())
    SW, SWO, SXL, SX, SH, SA, ST, SO, SS = 0, 16, 24, 28, 36, 44, 46, 48, 52
    only = cfg.get("only")

    def loop(name, lo, hi, body, init):
        if only is not None and name not in only:
            return init
        if cfg.get("scopes") == 2:
            def body2(i, c):
                with scope(name + "_it"):
                    return body(i, c)
            return lax.fori_loop(lo, hi, body2, init)
        with scope(name):
            return lax.fori_loop(lo, hi, body, init)
    w_hbms = (wq_hbm, wk_hbm, wv_hbm)
    a_hbms = (aq_hbm, ak_hbm, av_hbm)

    def w_copy(c, k):
        m, g = c // 2, c % 2
        slot = (c % 2) * 8 + k
        return pltpu.make_async_copy(
            w_hbms[m].at[pl.ds(k * 128, 128), pl.ds(16 * g, 16), :],
            wstage.at[slot], sems.at[SW + slot])

    def self_wait(ref, sem):
        pltpu.make_async_copy(ref, ref, sems.at[sem]).wait()

    def late_start(k):
        pltpu.make_async_copy(
            wo_hbm.at[pl.ds(k * 512, 512), :], wostage.at[k], sems.at[SWO + k]).start()
        for part in range(2):
            pltpu.make_async_copy(
                ssmk_hbm.at[pl.ds(k * 128, 128), pl.ds(part * (S // 2), S // 2)],
                hbuf.at[k, part], sems.at[SH + k]).start()

    def xlead_copy(q):
        return pltpu.make_async_copy(
            x_hbm.at[:, pl.ds(0, M), pl.ds(q * KQ, KQ)], xlead.at[q], sems.at[SXL + q])

    def x_copy(g):
        segs = pl.ds(g * 8, 8)
        return pltpu.make_async_copy(
            x_hbm.at[segs, pl.ds(M, SEG - M), :], xbuf.at[segs, pl.ds(M, SEG - M), :], sems.at[SX + g])

    def a_start(g):
        col = g * 128 if isinstance(g, int) else pl.multiple_of(g * 128, 128)
        for t in (1, 2, 0):
            pltpu.make_async_copy(
                a_hbms[t].at[:, pl.ds(col, 128)], abuf.at[g % 2, t], sems.at[SA + g % 2]).start()

    def tw_copy(j):
        return pltpu.make_async_copy(tw_hbm.at[j], tw.at[j], sems.at[ST + j])

    small = [pltpu.make_async_copy(src, dst, sems.at[SS + i]) for i, (src, dst) in enumerate((
        (fill_hbm, fill_ref), (mem0_hbm, mem0_ref), (sk_hbm, sk_ref), (ssmd_hbm, ssmd_ref.at[0])))]

    for q in range(4):
        xlead_copy(q).start()
        w_copy(0, 2 * q).start()
        w_copy(0, 2 * q + 1).start()
        for k in {2: (0, 1), 3: (2, 3, 4, 5, 6, 7)}.get(q, ()):
            w_copy(1, k).start()

    w_parts = (w_a, w_b)

    def slab_row(m, par, jl):
        return (m * 16 + par * 8 + jl) * SLAB

    def gated(x, i, n, gates):
        if gates is None:
            return x
        never, vals = gates
        v = vals[(i * len(vals) * 3) // (n * 4)]
        return jnp.where(never, pltpu.bitcast(v, U32), x)

    def vregs(*mats):
        return [m_[r:r + 8] for m_ in mats for r in range(0, m_.shape[0], 8)]

    def relayout_piece(m, g, k, gates=None, slot=None):
        slot = g * 8 + k if slot is None else slot
        dst = w_parts[g]
        base = slab_row(m, 0, 0) + k * 64
        for i in range(64):
            a = gated(pltpu.bitcast(wstage[slot, 2 * i], U32), i, 64, gates)
            b = pltpu.bitcast(wstage[slot, 2 * i + 1], U32)
            ev = (a & jnp.uint32(0xFFFF)) | (b << 16)
            od = (a >> 16) | (b & jnp.uint32(0xFFFF0000))
            dst[pl.ds(base + i, 8, stride=SLAB), :] = ev
            dst[pl.ds(base + 8 * SLAB + i, 8, stride=SLAB), :] = od

    def comb(x, y, sign):
        f = (lambda a, b: a + b) if sign > 0 else (lambda a, b: a - b)
        return _pack(f(_unpack(x, 0), _unpack(y, 0)), f(_unpack(x, 1), _unpack(y, 1)))

    def batch_pair(m, g, jl):
        it = m * NPAIR + 8 * g + jl
        rows = [pl.multiple_of(slab_row(m, par, jl), 8) for par in range(2)]

        def blk(kh, par):
            return w_parts[g][pl.ds(rows[par] + kh * (D // 4), D // 4), :]

        def mm(a, b):
            return _dot(pltpu.bitcast(jnp.concatenate(a, axis=1), BF16), pltpu.bitcast(b, BF16))

        def xs(f):
            return [xs_u[f, q] for q in range(2)]
        a11 = [xlead_u[q, pl.ds(0, HR), :] for q in (0, 1)]
        a22 = [xlead_u[q, pl.ds(HR, HR), :] for q in (2, 3)]
        m5 = mm(xs(2), blk(1, 1))
        m1 = mm(xs(0), comb(blk(0, 0), blk(1, 1), 1))
        m4 = mm(a22, comb(blk(1, 0), blk(0, 0), -1))
        c11 = mm(xs(4), comb(blk(1, 0), blk(1, 1), 1)) + (m1 + m4 - m5)
        m3 = mm(a11, comb(blk(0, 1), blk(1, 1), -1))
        qkvb[pl.ds(0, NSEG // 2), it] = _pack(c11, m3 + m5).reshape(NSEG // 2, M, DH)
        m2 = mm(xs(1), blk(0, 0))
        c22 = mm(xs(3), comb(blk(0, 0), blk(0, 1), 1)) + (m1 - m2 + m3)
        qkvb[pl.ds(NSEG // 2, NSEG // 2), it] = _pack(m2 + m4, c22).reshape(NSEG // 2, M, DH)
        return vregs(m5, m1, m4, c11, m3, m2, c22)

    def unit(n, carry):
        q, half = n // 2, n % 2
        never = n > 1000

        @pl.when(half == 0)
        def _():
            self_wait(xlead.at[q], SXL + q)
            for u in range(2):
                self_wait(wstage.at[2 * q + u], SW + 2 * q + u)
            xq = xlead[q].astype(F32).reshape(NSEG * M, KQ).astype(BF16)
            xlead_u[q] = pltpu.bitcast(xq, U32)
            for u in range(2):
                relayout_piece(0, 0, 2 * q + u)

        @pl.when(n == 6)
        def _():
            for k in range(8):
                w_copy(2, k).start()

        @pl.when(n >= 4)
        def _():
            for u in range(2):
                self_wait(wstage.at[2 * n + u], SW + 2 * n + u)
        res = []
        xq = pltpu.bitcast(xlead_u[q], BF16)
        for u in range(4):
            jl = 4 * half + u
            outs = []
            for par in range(2):
                acc = pl.ds(pl.multiple_of((2 * jl + par) * (NSEG * M), NSEG * M), NSEG * M)
                row = pl.multiple_of(slab_row(0, par, jl) + q * (KQ // 2), 8)
                w = pltpu.bitcast(w_a[pl.ds(row, KQ // 2), :], BF16)
                d = _dot(xq, w) + jnp.where(q == 0, 0.0, wk[acc, :])
                wk[acc, :] = d
                outs.append(d)
            qkvb[:, jl] = _pack(outs[0], outs[1]).reshape(NSEG, M, DH)
            res += outs
        for u in range(2):
            k = jnp.maximum(n - 4, 0) * 2 + u
            relayout_piece(0, 1, k, (never, vregs(*res[4 * u:4 * u + 4])),
                           slot=jnp.where(n < 4, u, 8 + k))
        gates = (never, vregs(*res))
        for r in range(0, HR, 8):
            for cb in range(2):
                cols = pl.ds(cb * 128, 128)
                i = 2 * (r // 8) + cb
                a11 = gated(xlead_u[half, pl.ds(r, 8), cols], i, HR // 4, gates)
                a22 = gated(xlead_u[2 + half, pl.ds(HR + r, 8), cols], i, HR // 4, gates)
                a21 = xlead_u[half, pl.ds(HR + r, 8), cols]
                a12 = xlead_u[2 + half, pl.ds(r, 8), cols]
                for f, (x, y, sg) in enumerate(((a11, a22, 1), (a21, a22, 1), (a11, a12, 1),
                                                (a21, a11, -1), (a12, a22, -1))):
                    xs_u[f, half, pl.ds(r, 8), cols] = comb(x, y, sg)
        return carry
    loop("units", 0, 8, unit, 0)

    def issue(c):
        if c + 2 < 6:
            for k in range(8):
                w_copy(c + 2, k).start()
        for k in {1: (0, 1), 2: (2, 3), 3: (4, 5, 6, 7)}.get(c, ()):
            late_start(k)
        if c == 1:
            for cp in small:
                cp.start()
        if c == 4:
            x_copy(0).start()
            a_start(0)
            tw_copy(0).start()
        if c == 5:
            tw_copy(1).start()
            a_start(1)
            for g in range(1, NG):
                x_copy(g).start()

    def late_relayout(src, hp, gates):
        half = hp % 2
        for r in range(16):
            blk = pltpu.bitcast(
                wostage[src, pl.ds(pl.multiple_of(half * 256 + r * 16, 16), 16), :], U32)
            row = pl.multiple_of(hp * 128 + r * 8, 8)
            for n in range(NB):
                wo_u[n, pl.ds(row, 8), :] = gated(blk[:, n * 128:(n + 1) * 128], r * NB + n, 16 * NB, gates)
        for t in range(8):
            tile = pltpu.bitcast(hbuf[src, half, :, pl.ds(t * 128, 128)], U32)
            tile = jnp.concatenate([gated(tile[0:8], t, 8, gates), tile[8:]], axis=0)
            row = pl.multiple_of(hp * 512 + t * 64, 64)
            ht[pl.ds(row, 64), :] = pltpu.bitcast(pltpu.bitcast(tile, BF16).T, U32)

    def chunk_body(c, g, it, carry):
        @pl.when(c < 5)
        def _():
            for u in range(PP):
                slot = (1 - g) * 8 + it * PP + u
                self_wait(wstage.at[slot], SW + slot)

        @pl.when(c >= 4)
        def _():
            for u in range(PP // 2):
                k = (c - 4) * 4 + it * (PP // 2) + u
                self_wait(wostage.at[k], SWO + k)
                self_wait(hbuf.at[k], SH + k)
        for u in range(PP):
            k = it * PP + u
            gates = (it > 1000, batch_pair(c // 2, g, k))
            relayout_piece(jnp.minimum((c + 1) // 2, 2), 1 - g, k, gates)
            hp = jnp.maximum(c - 4, 0) * 8 + k
            late_relayout(jnp.where(c >= 4, hp // 2, 8), hp, gates)
        return carry

    def chunk_pair(mm, carry):
        for g, c in ((1, 2 * mm + 1), (0, 2 * mm + 2)):
            for cs in range(2 - g, 6, 2):
                pl.when(c == cs)(functools.partial(issue, cs))

            @pl.when(c < 6)
            def _():
                loop("chunk", 0, 8 // PP, functools.partial(chunk_body, c, g), 0)
        return carry
    lax.fori_loop(0, 3, chunk_pair, 0)

    for cp in small:
        cp.wait()
    dd = ssmd_ref[0].astype(F32)
    for g in range(NG):
        sk = sk_ref[g].astype(F32)
        for j in range(KS):
            taps[g, j] = jnp.broadcast_to(sk[j:j + 1], (8, 128))
        taps[g, KS] = jnp.broadcast_to(dd[g:g + 1], (8, 128))

    def part_a(i, kick):
        g, j = i // 2, i % 2
        sl = g % 2
        never = i > 1000
        z = pl.multiple_of(jnp.where(never, 32, 0), 32) if cfg["a_dyn"] else 0
        sub = lax.broadcasted_iota(jnp.int32, (8, 128), 0)
        kickbuf[jnp.where(never, 1, 0)] = kick
        chain = [kickbuf[jnp.where(i > 2000, 0, 1)]]

        def begin(xs, ng):
            xs = list(xs)
            for e in range(min(ng, len(xs))):
                c = chain[0]
                c = c if c.dtype == xs[e].dtype else pltpu.bitcast(c, xs[e].dtype)
                xs[e] = jnp.where(never, c, xs[e])
            return xs

        def merge(vals):
            c = vals[-1]
            for v in list(vals[:-1])[:cfg["a_merge"]] + list(vals[:cfg["a_pad"]]):
                c = jnp.maximum(v, c)
            chain[0] = c

        def ld(v):
            if isinstance(v, tuple):
                blk, ri, r = v
                base = 8 * WS + 256 * blk + 16 * ri + 32 * r
                lo = wk[pl.ds(base, 8), :]
                if r == 0:
                    return lo
                return pltpu.roll(jnp.where(sub >= r, lo, wk[pl.ds(base + 8, 8), :]), 8 - r, 0)
            return wk[pl.ds(z + 8 * v, 8), :]

        def st(v, x):
            wk[pl.ds(z + 8 * v, 8), :] = x

        def twid(idx):
            return (tw[j, idx], tw[j, idx + 1])

        def natural(w, hh):
            return pltpu.bitcast(w, BF16).astype(F32)[8 * hh:8 * hh + 8]

        def pairs(flat):
            return [(flat[2 * e], flat[2 * e + 1]) for e in range(len(flat) // 2)]

        def fwd4(locs, t0):
            v = pairs(begin([ld(x) for loc in locs[::-1] for x in loc], cfg["a_g4"]))[::-1]
            return _dft4([v[0]] + [_cmul(v[r], twid(t0 + 2 * r)) for r in range(1, 4)], +1)

        def inv4(v, t0):
            o = _dft4(v, -1)
            return [o[0]] + [_cmulc(o[r], twid(t0 + 2 * r)) for r in range(1, 4)]

        def ld4(locs):
            return pairs(begin([ld(x) for loc in locs for x in loc], cfg["a_g4i"]))

        def put4(locs, o):
            for loc, x in zip(locs, o):
                st(loc[0], x[0])
                st(loc[1], x[1])
            merge([x for c in o for x in c])

        def put4_t(dsts, o):
            for (blk, slot), x in zip(dsts, o):
                for ri in range(2):
                    wk[pl.ds(8 * WS + 256 * blk + 16 * ri + slot, 8, stride=33), :] = x[ri]
            merge([x for c in o for x in c])

        def xloc(sig, n):
            return (WX + 256 * sig + 2 * n, WX + 256 * sig + 2 * n + 1)

        def sloc(kb, l):
            return ((2 * kb + l // 8, 0, l % 8), (2 * kb + l // 8, 1, l % 8))

        def pass_kv():
            t = [taps[g, a] for a in range(KS)]
            prev = {sh: jnp.zeros((8, 128), U32) for sh in (1, 2)}
            for v in range(S // 16):
                w0, = begin([pltpu.bitcast(abuf[sl, 1, pl.ds(16 * v, 16), :], U32)], 1)
                vw = pltpu.bitcast(abuf[sl, 2, pl.ds(16 * v, 16), :], U32)
                cur = {sh: pltpu.roll(w0, sh, 0) for sh in (1, 2)}
                w1, w2 = [jnp.where(sub < sh, prev[sh], cur[sh]) for sh in (1, 2)]
                prev = cur
                e0, o0, e1, o1, o2 = (_unpack(w0, 0), _unpack(w0, 1), _unpack(w1, 0),
                                      _unpack(w1, 1), _unpack(w2, 1))
                ke = (e0 * t[0] + o1 * t[1] + e1 * t[2] + o2 * t[3]) * _unpack(vw, 0)
                ko = (o0 * t[0] + e0 * t[1] + o1 * t[2] + e1 * t[3]) * _unpack(vw, 1)
                chain[0] = _pack(ke, ko)
                kvb[pl.ds(8 * v, 8), :] = chain[0]

        def forward(sig, src):
            for n in range(32):
                x = [natural(w, n % 2) for w in begin([src(n // 2 + 16 * d) for d in range(8)], 8)]
                cs = []
                for d in range(4):
                    a, b = twid(TAF + 2 * d), twid(TAF + 2 * (d + 4))
                    if d == 0:
                        s_ = x[4] * b[0]
                        cs.append((x[0] + s_, s_))
                    else:
                        cs.append((x[d] * a[0] + x[d + 4] * b[0], x[d] * a[1] + x[d + 4] * b[1]))
                put4([xloc(sig, n + 32 * k0) for k0 in range(4)], _dft4(cs, +1))
            for k0 in range(4):
                for n in range(8):
                    locs = [xloc(sig, n + 8 * r + 32 * k0) for r in range(4)]
                    put4(locs, fwd4(locs, TB + 8 * k0))
            for k0 in range(4):
                for k1 in range(4):
                    k = k0 + 4 * k1
                    for a in range(2):
                        o = fwd4([xloc(sig, a + 2 * r + 8 * k1 + 32 * k0) for r in range(4)], TC + 8 * k)
                        put4_t([(2 * ((k + 16 * k2) // 8) + a, k % 8) for k2 in range(4)], o)
            for kb in range(8):
                for e in range(4):
                    o = fwd4([sloc(kb, e + 4 * r) for r in range(4)], TD + 8 * kb)
                    put4([xloc(sig, 16 * kb + e + 4 * r) for r in range(4)], o)
            for kb in range(8):
                for k3 in range(4):
                    locs = [xloc(sig, 16 * kb + r + 4 * k3) for r in range(4)]
                    t0 = TE + 8 * (4 * kb + k3)
                    o = fwd4(locs, t0)
                    if sig == 0:
                        hs = ld4([xloc(1, 16 * kb + r + 4 * k3) for r in range(4)])
                        o = inv4([_cmul(a, b) for a, b in zip(o, hs)], t0)
                    put4(locs, o)

        def inverse():
            for kb in range(8):
                for e in range(4):
                    o = inv4(ld4([xloc(0, 16 * kb + e + 4 * r) for r in range(4)]), TD + 8 * kb)
                    put4_t([(2 * kb + (e + 4 * f) // 8, (e + 4 * f) % 8) for f in range(4)], o)
            for k0 in range(4):
                for k1 in range(4):
                    k = k0 + 4 * k1
                    for a in range(2):
                        v = ld4([sloc((k + 16 * r) // 8, 8 * a + k % 8) for r in range(4)])
                        put4([xloc(0, a + 2 * b + 8 * k1 + 32 * k0) for b in range(4)], inv4(v, TC + 8 * k))
            for k0 in range(4):
                for n in range(8):
                    locs = [xloc(0, n + 8 * r + 32 * k0) for r in range(4)]
                    put4(locs, inv4(ld4(locs), TB + 8 * k0))
            dskip = taps[g, KS]
            for n0 in range(32):
                cs = _dft4(ld4([xloc(0, n0 + 32 * r) for r in range(4)]), -1)
                outs = []
                for d in [d0 + 4 * hh for d0 in range(4) for hh in range(2)]:
                    n = n0 + 32 * d
                    a = twid(TAI + 2 * d)
                    if 0 < d < 4 and cfg["a_fine"]:
                        cs[d] = tuple(begin(cs[d], 2))
                    c = cs[d % 4]
                    y = c[0] * a[0] if d == 0 else c[0] * a[0] + c[1] * a[1]
                    kv = natural(kvb[pl.ds(8 * (n // 2), 8), :], n % 2)
                    y = y + jnp.where(j == 0, kv * dskip, ld(WY + n))
                    st(WY + n, y)
                    chain[0] = abuf[sl, 0, pl.ds(8 * n, 8), :].astype(F32) * y
                    aout[g, n // 4, pl.ds(8 * (n % 4), 8), :] = chain[0].astype(BF16)
                    outs.append(chain[0])
                merge(outs)

        def filt(v):
            return ht[pl.ds(pl.multiple_of(g * (S // 2), S // 2) + 8 * v, 8), :]
        if cfg["a_hfirst"]:
            forward(1, filt)
            pass_kv()
        else:
            pass_kv()
            forward(1, filt)
        forward(0, lambda v: kvb[pl.ds(8 * v, 8), :])
        inverse()
        return chain[0]

    scale = DH ** (-0.5)

    def w_slab(m, h):
        j = h // 2
        return pltpu.bitcast(w_parts[j // 8][pl.ds(slab_row(m, h % 2, j % 8), D // 2), :], BF16)

    class Step:
        def __init__(self, s, prev, mem):
            self.s = s
            self.prev = prev
            self.qkv, self.ps, self.os = {}, {}, []
            self.acc = [None] * NB
            self.ocat, self.lead, self.early, self.marks = {}, {}, {}, {}
            self.tie = None
            x = xbuf[s, pl.ds(M, SEG - M), :].astype(F32)
            self.lhsf = jnp.concatenate([mem, x], axis=0)
            self.lhs = self.lhsf.astype(BF16)

        def proj_early(self, m, j, k):
            self.early[m, j] = (k, [_dot(self.lhsf[:, :k].astype(BF16), w_slab(m, 2 * j + e)[:k])
                                    for e in range(2)])

        def proj(self, m, j):
            if (m, j) in self.early:
                k, part = self.early[m, j]
                a, b = [_dot(self.lhsf[:, k:].astype(BF16), w_slab(m, 2 * j + e)[k:]) + part[e]
                        for e in range(2)]
            else:
                a = _dot(self.lhs, w_slab(m, 2 * j))
                b = _dot(self.lhs, w_slab(m, 2 * j + 1))
            self.marks[m, j] = a[0:8]
            lead = qkvb[self.s, m * NPAIR + j]
            if m == 0:
                r = jnp.concatenate([a, b, _unpack(lead, 0), _unpack(lead, 1)], axis=0).astype(BF16)
            else:
                r = pltpu.bitcast(jnp.concatenate([_pack(a, b), lead], axis=0), BF16)
            self.qkv[m, j] = r

        def probs(self, j):
            fill = fill_ref[pl.ds(0, R), pl.ds(0, R)]
            qk = _dot_nt(self.qkv[0, j], self.qkv[1, j])
            if cfg["exp2"]:
                sc = jnp.where(fill == 0.0, qk, fill)
                e = jnp.exp2((sc - jnp.max(sc, axis=-1, keepdims=True)) * (scale * LOG2E))
            else:
                sc = jnp.where(fill == 0.0, qk * scale, fill)
                e = jnp.exp(sc - jnp.max(sc, axis=-1, keepdims=True))
            l = jnp.sum(e, axis=-1, keepdims=True)
            r = pl.reciprocal(l, approx=True)
            r = r * (2.0 - l * r)
            self.ps[j] = (e * r).astype(BF16)

        def attend(self, j):
            o = _dot(self.ps[j], self.qkv[2, j])
            la, lb = o[2 * SEG:2 * SEG + M], o[2 * SEG + M:]
            rows = pl.ds(pl.multiple_of((self.s // 2) * M, M), M)
            if self.prev is None:
                self.lead[j] = (la, lb)
                forms = {2: la + lb, 5: la}
            else:
                a11, a12 = self.prev.lead[j]
                forms = {0: a11 + lb, 1: la + lb, 3: la - a11, 4: a12 - lb, 6: lb}
            for f, v in forms.items():
                ob[f * NPAIR + j, rows, :] = v.astype(BF16)
            self.os += [o[0:SEG], o[SEG:2 * SEG]]

        def wo(self, h0, h1, n):
            if h0 not in self.ocat:
                self.ocat[h0] = jnp.concatenate(self.os[h0:h1], axis=1).astype(BF16)
            w = wo_u[n, pl.ds(h0 * 64, (h1 - h0) * 64), :]
            if self.tie is not None:
                w = jnp.concatenate(
                    [jnp.where(self.s > 1000, pltpu.bitcast(self.tie, U32), w[0:8]), w[8:]], axis=0)
                self.tie = None
            d = _dot(self.ocat[h0], pltpu.bitcast(w, BF16))
            self.acc[n] = d if self.acc[n] is None else d + self.acc[n]

        def finish(self):
            res = jnp.concatenate(self.acc, axis=1)
            obuf[self.s] = res.astype(BF16)
            return res[0:M]

    def steps(i, mem):
        g = i // 2

        @pl.when(i % 2 == 0)
        def _():
            x_copy(g).wait()
            self_wait(abuf.at[g % 2], SA + g % 2)

            @pl.when(jnp.logical_and(g >= 1, g < NG - 1))
            def _():
                a_start(g + 1)

        @pl.when(i < 2)
        def _():
            self_wait(tw.at[i], ST + i)
        sts = []
        for u in range(U):
            st = Step(i * U + u, sts[-1] if u % 2 else None, mem)
            sts.append(st)
            for item in _step_order(u, cfg):
                if item[0] == "A":
                    if cfg["a"]:
                        ku, km, kj = cfg["kick"]
                        st.tie = part_a(i, sts[ku].marks[km, kj])
                else:
                    dict(P=st.proj, E=st.proj_early, S=st.probs, V=st.attend, W=st.wo)[item[0]](*item[1:])
            mem = st.finish()
        return mem

    loop("steps", 0, NSEG // U, steps, mem0_ref[...].astype(F32))

    ob_cp = pltpu.make_async_copy(
        obuf.at[:, pl.ds(M, SEG - M), :],
        out_hbm.at[:, pl.ds(M, SEG - M), pl.ds(D, D)], sems.at[SO])
    ob_cp.start()
    for g in range(NG):
        pltpu.make_async_copy(
            aout.at[g], out_hbm.at[:, :, pl.ds(g * 128, 128)], sems.at[SO + 1]).start()

    def epi(it, carry):
        ns = [2 * it, 2 * it + 1]

        def blk(hp, u):
            return [wo_u[ns[u], pl.ds((2 * j + hp) * 64, 64), :] for j in range(NPAIR)]

        def mm(f, bs):
            lhs = jnp.concatenate([ob[f * NPAIR + j] for j in range(NPAIR)], axis=1)
            return _dot(lhs, pltpu.bitcast(jnp.concatenate(bs, axis=0), BF16))

        def cb(x, y, sign):
            return [comb(a, b, sign) for a, b in zip(x, y)]

        def put(u, par, c):
            for i in range(NSEG // 2):
                obb[ns[u], 2 * i + par] = c[M * i:M * i + M].astype(BF16)
        m5 = mm(2, blk(1, 1))
        m1 = mm(0, cb(blk(0, 0), blk(1, 1), 1))
        m4 = mm(6, cb(blk(1, 0), blk(0, 0), -1))
        put(0, 0, mm(4, cb(blk(1, 0), blk(1, 1), 1)) + (m1 + m4 - m5))
        m3 = mm(5, cb(blk(0, 1), blk(1, 1), -1))
        put(1, 0, m3 + m5)
        m2 = mm(1, blk(0, 0))
        put(0, 1, m2 + m4)
        put(1, 1, mm(3, cb(blk(0, 0), blk(0, 1), 1)) + (m1 - m2 + m3))
        for n in ns:
            col = pl.multiple_of(D + n * 128, 128)
            pltpu.make_async_copy(
                obb.at[n], out_hbm.at[:, pl.ds(0, M), pl.ds(col, 128)], sems.at[SO + 2]).start()
        return carry
    loop("epi", 0, NB // 2, epi, 0)
    ob_cp.wait()
    self_wait(aout, SO + 1)
    self_wait(obb, SO + 2)


def _step_order(u, cfg):
    ks = cfg["ks"]
    tmpl = [(x[0], int(x[1:])) for x in cfg["tmpl"].split()]
    out = []
    if u > 0:
        first = [(kind, t - lag) for t in range(3) for kind, lag in tmpl if kind in "qkv" and t >= lag]
        out += [("E", "qkv".index(kind), j, cfg["ek"]) for kind, j in first[:cfg["ne"]]]
    nw = 0
    for t in range(NPAIR + max(l for _, l in tmpl)):
        for kind, lag in tmpl:
            j = t - lag
            if j < 0:
                continue
            if j >= NPAIR:
                if kind in "qkv" and nw < NB:
                    out.append(("W", 0, ks, nw))
                    nw += 1
                continue
            out.append(("P", "qkv".index(kind), j) if kind in "qkv" else (kind, j))
    out += [("W", 0, ks, n) for n in range(nw, NB)]
    for n in range(NB):
        if u == U - 1 and n == cfg["tie_n"]:
            out.append(("A",))
        out.append(("W", ks, H, n))
    return out


_DEFAULT_CFG = dict(tmpl="k0 v1 S1 q0 V2", ks=16, ne=2, ek=640, exp2=0,
                    a=1, tie_n=7, kick=(0, 0, 2), a_dyn=0, a_merge=5, a_pad=0, a_fine=1,
                    a_g4=8, a_g4i=4, a_hfirst=0)


def _build(cfg):
    tw_np = _twiddles()
    fill_np = np.zeros((96, 128), np.float32)
    fill_np[:R, :R] = _mask_fill() * (DH ** 0.5 if cfg["exp2"] else 1.0)

    def run(A_q, A_k, A_v, A_shift_k, A_ssm_k, A_ssm_D, B_x, B_mem0, B_Wq, B_Wk, B_Wv, B_Wo):
        sk = A_shift_k.T.reshape(KS, NG, 128).transpose(1, 0, 2)
        any_spec = pl.BlockSpec(memory_space=pl.ANY)
        out = pl.pallas_call(
            functools.partial(_kernel, cfg),
            out_shape=jax.ShapeDtypeStruct((NSEG, SEG, 2 * D), BF16),
            in_specs=[any_spec] * 14,
            out_specs=any_spec,
            scratch_shapes=[
                pltpu.VMEM((48 * SLAB + 544, 128), U32),
                pltpu.VMEM((48 * SLAB + 544, 128), U32),
                pltpu.VMEM((NB, H * DH // 2, 128), U32),
                pltpu.VMEM((16, 128, 16, DH), BF16),
                pltpu.VMEM((9, 512, D), BF16),
                pltpu.VMEM((NSEG, SEG, D), BF16),
                pltpu.VMEM((4, NSEG, M, KQ), BF16),
                pltpu.VMEM((4, NSEG * M // 2, KQ), U32),
                pltpu.VMEM((5, 2, HR, KQ), U32),
                pltpu.VMEM((NSEG, 3 * NPAIR, 8, 128), U32),
                pltpu.VMEM((7 * NPAIR, NSEG * M // 2, DH), BF16),
                pltpu.VMEM((NSEG, SEG, D), BF16),
                pltpu.VMEM((NB, NSEG, M, 128), BF16),
                pltpu.VMEM((2, 3, S, 128), BF16),
                pltpu.VMEM((NG + 1, 2, 128, S // 2), BF16),
                pltpu.VMEM((NG * S // 2, 128), U32),
                pltpu.VMEM((S // 2, 128), U32),
                pltpu.VMEM((8 * NW + 32, 128), F32),
                pltpu.VMEM((2, NT, 8, 128), F32),
                pltpu.VMEM((NG, NSEG, SEG, 128), BF16),
                pltpu.VMEM((4, 8, 128), F32),
                pltpu.VMEM((96, 128), F32),
                pltpu.VMEM((NG, 8, 8, 128), F32),
                pltpu.VMEM((M, D), BF16),
                pltpu.VMEM((NG, KS, 128), BF16),
                pltpu.VMEM((4, NG, 128), BF16),
                pltpu.SemaphoreType.DMA((56,)),
            ],
            compiler_params=pltpu.CompilerParams(vmem_limit_bytes=124 * 1024 * 1024,
                                                 disable_bounds_checks=True),
        )(A_q.reshape(S, D), A_k.reshape(S, D), A_v.reshape(S, D), sk, A_ssm_k,
          A_ssm_D.reshape(NG, 128), B_x.reshape(NSEG, SEG, D), B_mem0.reshape(M, D),
          B_Wq, B_Wk, B_Wv, B_Wo.reshape(H * DH, D),
          jnp.asarray(tw_np), jnp.asarray(fill_np))
        return out.reshape(1, S, 2 * D)

    return run


@functools.partial(jax.jit, static_argnames=("B_seg_len",))
def pallas_concat_heads__ssm_conv_h3__memory_aug_recurrent_mem_tr__prompt_kernel(
    A_q: jax.Array,
    A_k: jax.Array,
    A_v: jax.Array,
    A_shift_k: jax.Array,
    A_ssm_k: jax.Array,
    A_ssm_D: jax.Array,
    B_x: jax.Array,
    B_mem0: jax.Array,
    B_Wq: jax.Array,
    B_Wk: jax.Array,
    B_Wv: jax.Array,
    B_Wo: jax.Array,
    B_seg_len: int = SEG,
):
    assert B_seg_len == SEG
    return _build(_DEFAULT_CFG)(A_q, A_k, A_v, A_shift_k, A_ssm_k, A_ssm_D, B_x, B_mem0,
                                B_Wq, B_Wk, B_Wv, B_Wo)
```

```python
import functools

import numpy as np
import jax
import jax.numpy as jnp
from jax import lax
import jax.experimental.pallas as pl
import jax.experimental.pallas.tpu as pltpu

F32 = jnp.float32
BF16 = jnp.bfloat16
U32 = jnp.uint32

S = 2048
D = 1024
H = 32
DH = 128
M = 8
SEG = 32
NSEG = S // SEG
U = 4
NPAIR = H // 2
R = 2 * (M + SEG)
SLAB = 520
KS = 4
NG = D // 128
KQ = D // 4
NB = D // 128
PP = 4
HR = NSEG * M // 4

TAF, TAI, TB, TC, TD, TE, NT = 0, 16, 32, 64, 192, 256, 512
WX, WS, WY, NW = 0, 512, 1024, 1280
LOG2E = 1.4426950408889634


def _twiddles():
    tw = np.zeros((2, NT, 8), np.float64)

    def put(j, idx, z):
        tw[j, idx] = np.real(z)
        tw[j, idx + 1] = np.imag(z)
    s = np.arange(8)
    tau = 2j * np.pi
    for j in range(2):
        lx = 1j * np.pi * (1 + 4 * j) / 4096
        for d in range(8):
            put(j, TAF + 2 * d, np.exp(lx * 256 * d))
            put(j, TAI + 2 * d, np.exp(lx * 256 * d) / 2048)
        for r in range(4):
            for k in range(4):
                put(j, TB + 8 * k + 2 * r, np.exp((lx * 64 + tau * k / 16) * r))
            for k in range(16):
                put(j, TC + 8 * k + 2 * r, np.exp((lx * 16 + tau * k / 64) * r))
            for kb in range(8):
                put(j, TD + 8 * kb + 2 * r, np.exp((lx * 4 + tau * (s + 8 * kb) / 256) * r))
                for k3 in range(4):
                    put(j, TE + 8 * (4 * kb + k3) + 2 * r,
                        np.exp((lx + tau * (s + 8 * kb + 64 * k3) / 1024) * r))
    return np.ascontiguousarray(np.broadcast_to(tw[..., None], (2, NT, 8, 128))).astype(np.float32)


def _mask_fill():
    blk = np.concatenate([np.arange(M), M + np.arange(M, SEG)])
    lead = M + np.arange(M)
    qhead = np.concatenate([np.zeros(SEG), np.ones(SEG), np.zeros(M), np.ones(M)])
    qpos = np.concatenate([blk, blk, lead, lead])
    khead = np.arange(R) % 2
    kpos = np.concatenate([blk, lead])[np.arange(R) // 2]
    same = qhead[:, None] == khead[None, :]
    ok = (qpos[:, None] < M) | (qpos[:, None] >= kpos[None, :])
    fill = np.where(same, np.where(ok, 0.0, -1e9), -np.inf)
    return fill.astype(np.float32)


def _pack(lo, hi):
    return pltpu.pack_elementwise([lo, hi], packed_dtype=BF16)


def _unpack(w, index):
    return pltpu.unpack_elementwise(w, index=index, packed_dtype=BF16, unpacked_dtype=F32)


def _dot(a, b):
    return jnp.dot(a, b, preferred_element_type=F32)


def _dot_nt(a, b):
    return lax.dot_general(a, b, (((1,), (1,)), ((), ())), preferred_element_type=F32)


def _cadd(a, b):
    return (a[0] + b[0], a[1] + b[1])


def _csub(a, b):
    return (a[0] - b[0], a[1] - b[1])


def _cmul(a, w):
    return (a[0] * w[0] - a[1] * w[1], a[0] * w[1] + a[1] * w[0])


def _cmulc(a, w):
    return (a[0] * w[0] + a[1] * w[1], a[1] * w[0] - a[0] * w[1])


def _bfly_i(b, d, sg):
    p = (b[0] - d[1], b[1] + d[0])
    q = (b[0] + d[1], b[1] - d[0])
    return (p, q) if sg > 0 else (q, p)


def _dft4(x, sg):
    a, b = _cadd(x[0], x[2]), _csub(x[0], x[2])
    c, d = _cadd(x[1], x[3]), _csub(x[1], x[3])
    p, q = _bfly_i(b, d, sg)
    return [_cadd(a, c), p, _csub(a, c), q]


def _kernel(cfg,
            aq_hbm, ak_hbm, av_hbm, sk_hbm, ssmk_hbm, ssmd_hbm, x_hbm, mem0_hbm,
            wq_hbm, wk_hbm, wv_hbm, wo_hbm, tw_hbm, fill_hbm,
            out_hbm,
            w_a, w_b, wo_u, wstage, wostage, xbuf, xlead, xlead_u, xs_u, qkvb, ob, obuf, obb,
            abuf, hbuf, ht, kvb, wk, tw, aout, kickbuf,
            fill_ref, taps, mem0_ref, sk_ref, ssmd_ref,
            sems):
    import contextlib
    scope = jax.named_scope if cfg.get("scopes") else (lambda name: contextlib.nullcontext())
    SW, SWO, SXL, SX, SH, SA, ST, SO, SS = 0, 16, 24, 28, 36, 44, 46, 48, 52
    only = cfg.get("only")

    def loop(name, lo, hi, body, init):
        if only is not None and name not in only:
            return init
        if cfg.get("scopes") == 2:
            def body2(i, c):
                with scope(name + "_it"):
                    return body(i, c)
            return lax.fori_loop(lo, hi, body2, init)
        with scope(name):
            return lax.fori_loop(lo, hi, body, init)
    w_hbms = (wq_hbm, wk_hbm, wv_hbm)
    a_hbms = (aq_hbm, ak_hbm, av_hbm)

    def w_copy(c, k):
        m, g = c // 2, c % 2
        slot = (c % 2) * 8 + k
        return pltpu.make_async_copy(
            w_hbms[m].at[pl.ds(k * 128, 128), pl.ds(16 * g, 16), :],
            wstage.at[slot], sems.at[SW + slot])

    def self_wait(ref, sem):
        pltpu.make_async_copy(ref, ref, sems.at[sem]).wait()

    def late_start(k):
        pltpu.make_async_copy(
            wo_hbm.at[pl.ds(k * 512, 512), :], wostage.at[k], sems.at[SWO + k]).start()
        for part in range(2):
            pltpu.make_async_copy(
                ssmk_hbm.at[pl.ds(k * 128, 128), pl.ds(part * (S // 2), S // 2)],
                hbuf.at[k, part], sems.at[SH + k]).start()

    def xlead_copy(q):
        return pltpu.make_async_copy(
            x_hbm.at[:, pl.ds(0, M), pl.ds(q * KQ, KQ)], xlead.at[q], sems.at[SXL + q])

    def x_copy(g):
        segs = pl.ds(g * 8, 8)
        return pltpu.make_async_copy(
            x_hbm.at[segs, pl.ds(M, SEG - M), :], xbuf.at[segs, pl.ds(M, SEG - M), :], sems.at[SX + g])

    def a_start(g):
        col = g * 128 if isinstance(g, int) else pl.multiple_of(g * 128, 128)
        for t in (1, 2, 0):
            pltpu.make_async_copy(
                a_hbms[t].at[:, pl.ds(col, 128)], abuf.at[g % 2, t], sems.at[SA + g % 2]).start()

    def tw_copy(j):
        return pltpu.make_async_copy(tw_hbm.at[j], tw.at[j], sems.at[ST + j])

    small = [pltpu.make_async_copy(src, dst, sems.at[SS + i]) for i, (src, dst) in enumerate((
        (fill_hbm, fill_ref), (mem0_hbm, mem0_ref), (sk_hbm, sk_ref), (ssmd_hbm, ssmd_ref.at[0])))]

    for q in range(4):
        xlead_copy(q).start()
        w_copy(0, 2 * q).start()
        w_copy(0, 2 * q + 1).start()
        for k in {2: (0, 1), 3: (2, 3, 4, 5, 6, 7)}.get(q, ()):
            w_copy(1, k).start()

    w_parts = (w_a, w_b)

    def slab_row(m, par, jl):
        return (m * 16 + par * 8 + jl) * SLAB

    def gated(x, i, n, gates):
        if gates is None:
            return x
        never, vals = gates
        v = vals[(i * len(vals) * 3) // (n * 4)]
        return jnp.where(never, pltpu.bitcast(v, U32), x)

    def vregs(*mats):
        return [m_[r:r + 8] for m_ in mats for r in range(0, m_.shape[0], 8)]

    def relayout_piece(m, g, k, gates=None, slot=None):
        slot = g * 8 + k if slot is None else slot
        dst = w_parts[g]
        base = slab_row(m, 0, 0) + k * 64
        for i in range(64):
            a = gated(pltpu.bitcast(wstage[slot, 2 * i], U32), i, 64, gates)
            b = pltpu.bitcast(wstage[slot, 2 * i + 1], U32)
            ev = (a & jnp.uint32(0xFFFF)) | (b << 16)
            od = (a >> 16) | (b & jnp.uint32(0xFFFF0000))
            dst[pl.ds(base + i, 8, stride=SLAB), :] = ev
            dst[pl.ds(base + 8 * SLAB + i, 8, stride=SLAB), :] = od

    def comb(x, y, sign):
        f = (lambda a, b: a + b) if sign > 0 else (lambda a, b: a - b)
        return _pack(f(_unpack(x, 0), _unpack(y, 0)), f(_unpack(x, 1), _unpack(y, 1)))

    def batch_pair(m, g, jl):
        it = m * NPAIR + 8 * g + jl
        rows = [pl.multiple_of(slab_row(m, par, jl), 8) for par in range(2)]

        def blk(kh, par):
            return w_parts[g][pl.ds(rows[par] + kh * (D // 4), D // 4), :]

        def mm(a, b):
            return _dot(pltpu.bitcast(jnp.concatenate(a, axis=1), BF16), pltpu.bitcast(b, BF16))

        def xs(f):
            return [xs_u[f, q] for q in range(2)]
        a11 = [xlead_u[q, pl.ds(0, HR), :] for q in (0, 1)]
        a22 = [xlead_u[q, pl.ds(HR, HR), :] for q in (2, 3)]
        m5 = mm(xs(2), blk(1, 1))
        m1 = mm(xs(0), comb(blk(0, 0), blk(1, 1), 1))
        m4 = mm(a22, comb(blk(1, 0), blk(0, 0), -1))
        c11 = mm(xs(4), comb(blk(1, 0), blk(1, 1), 1)) + (m1 + m4 - m5)
        m3 = mm(a11, comb(blk(0, 1), blk(1, 1), -1))
        qkvb[pl.ds(0, NSEG // 2), it] = _pack(c11, m3 + m5).reshape(NSEG // 2, M, DH)
        m2 = mm(xs(1), blk(0, 0))
        c22 = mm(xs(3), comb(blk(0, 0), blk(0, 1), 1)) + (m1 - m2 + m3)
        qkvb[pl.ds(NSEG // 2, NSEG // 2), it] = _pack(m2 + m4, c22).reshape(NSEG // 2, M, DH)
        return vregs(m5, m1, m4, c11, m3, m2, c22)

    def unit(n, carry):
        q, half = n // 2, n % 2
        never = n > 1000

        @pl.when(half == 0)
        def _():
            self_wait(xlead.at[q], SXL + q)
            for u in range(2):
                self_wait(wstage.at[2 * q + u], SW + 2 * q + u)
            xq = xlead[q].astype(F32).reshape(NSEG * M, KQ).astype(BF16)
            xlead_u[q] = pltpu.bitcast(xq, U32)
            for u in range(2):
                relayout_piece(0, 0, 2 * q + u)

        @pl.when(n == 6)
        def _():
            for k in range(8):
                w_copy(2, k).start()

        @pl.when(n >= 4)
        def _():
            for u in range(2):
                self_wait(wstage.at[2 * n + u], SW + 2 * n + u)
        res = []
        xq = pltpu.bitcast(xlead_u[q], BF16)
        for u in range(4):
            jl = 4 * half + u
            outs = []
            for par in range(2):
                acc = pl.ds(pl.multiple_of((2 * jl + par) * (NSEG * M), NSEG * M), NSEG * M)
                row = pl.multiple_of(slab_row(0, par, jl) + q * (KQ // 2), 8)
                w = pltpu.bitcast(w_a[pl.ds(row, KQ // 2), :], BF16)
                d = _dot(xq, w) + jnp.where(q == 0, 0.0, wk[acc, :])
                wk[acc, :] = d
                outs.append(d)
            qkvb[:, jl] = _pack(outs[0], outs[1]).reshape(NSEG, M, DH)
            res += outs
        for u in range(2):
            k = jnp.maximum(n - 4, 0) * 2 + u
            relayout_piece(0, 1, k, (never, vregs(*res[4 * u:4 * u + 4])),
                           slot=jnp.where(n < 4, u, 8 + k))
        gates = (never, vregs(*res))
        for r in range(0, HR, 8):
            for cb in range(2):
                cols = pl.ds(cb * 128, 128)
                i = 2 * (r // 8) + cb
                a11 = gated(xlead_u[half, pl.ds(r, 8), cols], i, HR // 4, gates)
                a22 = gated(xlead_u[2 + half, pl.ds(HR + r, 8), cols], i, HR // 4, gates)
                a21 = xlead_u[half, pl.ds(HR + r, 8), cols]
                a12 = xlead_u[2 + half, pl.ds(r, 8), cols]
                for f, (x, y, sg) in enumerate(((a11, a22, 1), (a21, a22, 1), (a11, a12, 1),
                                                (a21, a11, -1), (a12, a22, -1))):
                    xs_u[f, half, pl.ds(r, 8), cols] = comb(x, y, sg)
        return carry
    loop("units", 0, 8, unit, 0)

    def issue(c):
        if c + 2 < 6:
            for k in range(8):
                w_copy(c + 2, k).start()
        for k in {1: (0, 1), 2: (2, 3), 3: (4, 5, 6, 7)}.get(c, ()):
            late_start(k)
        if c == 1:
            for cp in small:
                cp.start()
        if c == 4:
            x_copy(0).start()
            a_start(0)
            tw_copy(0).start()
            tw_copy(1).start()
        if c == 5:
            a_start(1)
            for g in range(1, NG):
                x_copy(g).start()

    def late_relayout(src, hp, gates):
        half = hp % 2
        for r in range(16):
            blk = pltpu.bitcast(
                wostage[src, pl.ds(pl.multiple_of(half * 256 + r * 16, 16), 16), :], U32)
            row = pl.multiple_of(hp * 128 + r * 8, 8)
            for n in range(NB):
                wo_u[n, pl.ds(row, 8), :] = gated(blk[:, n * 128:(n + 1) * 128], r * NB + n, 16 * NB, gates)
        for t in range(8):
            tile = pltpu.bitcast(hbuf[src, half, :, pl.ds(t * 128, 128)], U32)
            tile = jnp.concatenate([gated(tile[0:8], t, 8, gates), tile[8:]], axis=0)
            row = pl.multiple_of(hp * 512 + t * 64, 64)
            ht[pl.ds(row, 64), :] = pltpu.bitcast(pltpu.bitcast(tile, BF16).T, U32)

    def chunk_body(c, g, it, carry):
        @pl.when(c < 5)
        def _():
            for u in range(PP):
                slot = (1 - g) * 8 + it * PP + u
                self_wait(wstage.at[slot], SW + slot)

        @pl.when(c >= 4)
        def _():
            for u in range(PP // 2):
                k = (c - 4) * 4 + it * (PP // 2) + u
                self_wait(wostage.at[k], SWO + k)
                self_wait(hbuf.at[k], SH + k)
        for u in range(PP):
            k = it * PP + u
            gates = (it > 1000, batch_pair(c // 2, g, k))
            relayout_piece(jnp.minimum((c + 1) // 2, 2), 1 - g, k, gates)
            hp = jnp.maximum(c - 4, 0) * 8 + k
            late_relayout(jnp.where(c >= 4, hp // 2, 8), hp, gates)
        return carry

    def chunk_pair(mm, carry):
        for g, c in ((1, 2 * mm + 1), (0, 2 * mm + 2)):
            for cs in range(2 - g, 6, 2):
                pl.when(c == cs)(functools.partial(issue, cs))

            @pl.when(c < 6)
            def _():
                loop("chunk", 0, 8 // PP, functools.partial(chunk_body, c, g), 0)
        return carry
    lax.fori_loop(0, 3, chunk_pair, 0)

    for cp in small:
        cp.wait()
    dd = ssmd_ref[0].astype(F32)
    for g in range(NG):
        sk = sk_ref[g].astype(F32)
        for j in range(KS):
            taps[g, j] = jnp.broadcast_to(sk[j:j + 1], (8, 128))
        taps[g, KS] = jnp.broadcast_to(dd[g:g + 1], (8, 128))

    def part_a(i, kick):
        g, j = i // 2, i % 2
        sl = g % 2
        never = i > 1000
        z = pl.multiple_of(jnp.where(never, 32, 0), 32) if cfg["a_dyn"] else 0
        sub = lax.broadcasted_iota(jnp.int32, (8, 128), 0)
        kickbuf[jnp.where(never, 1, 0)] = kick
        chain = [kickbuf[jnp.where(i > 2000, 0, 1)]]

        def begin(xs, ng):
            xs = list(xs)
            for e in range(min(ng, len(xs))):
                c = chain[0]
                c = c if c.dtype == xs[e].dtype else pltpu.bitcast(c, xs[e].dtype)
                xs[e] = jnp.where(never, c, xs[e])
            return xs

        def merge(vals):
            c = vals[-1]
            for v in list(vals[:-1])[:cfg["a_merge"]] + list(vals[:cfg["a_pad"]]):
                c = jnp.maximum(v, c)
            chain[0] = c

        def ld(v):
            if isinstance(v, tuple):
                blk, ri, r = v
                base = 8 * WS + 256 * blk + 16 * ri + 32 * r
                if cfg["skew2"]:
                    base += 8 * (blk % 2)
                lo = wk[pl.ds(base, 8), :]
                if r == 0:
                    return lo
                if cfg["skew2"]:
                    return pltpu.roll(lo, 8 - r, 0)
                return pltpu.roll(jnp.where(sub >= r, lo, wk[pl.ds(base + 8, 8), :]), 8 - r, 0)
            return wk[pl.ds(z + 8 * v, 8), :]

        def st(v, x):
            wk[pl.ds(z + 8 * v, 8), :] = x

        def twid(idx):
            return (tw[j, idx], tw[j, idx + 1])

        def natural(w, hh):
            return pltpu.bitcast(w, BF16).astype(F32)[8 * hh:8 * hh + 8]

        def pairs(flat):
            return [(flat[2 * e], flat[2 * e + 1]) for e in range(len(flat) // 2)]

        def fwd4(locs, t0):
            v = pairs(begin([ld(x) for loc in locs[::-1] for x in loc], cfg["a_g4"]))[::-1]
            return _dft4([v[0]] + [_cmul(v[r], twid(t0 + 2 * r)) for r in range(1, 4)], +1)

        def inv4(v, t0):
            o = _dft4(v, -1)
            return [o[0]] + [_cmulc(o[r], twid(t0 + 2 * r)) for r in range(1, 4)]

        def ld4(locs):
            return pairs(begin([ld(x) for loc in locs for x in loc], cfg["a_g4i"]))

        def put4(locs, o):
            for loc, x in zip(locs, o):
                st(loc[0], x[0])
                st(loc[1], x[1])
            merge([x for c in o for x in c])

        def put4_t(dsts, o):
            for (blk, slot), x in zip(dsts, o):
                for ri in range(2):
                    base = 8 * WS + 256 * blk + 16 * ri + slot
                    if cfg["skew2"]:
                        base += 8 * (blk % 2)
                        wk[pl.ds(base, 8 - slot, stride=33), :] = x[ri][0:8 - slot]
                        if slot:
                            wk[pl.ds(base - 8 + 33 * (8 - slot), slot, stride=33), :] = x[ri][8 - slot:8]
                    else:
                        wk[pl.ds(base, 8, stride=33), :] = x[ri]
            merge([x for c in o for x in c])

        def xloc(sig, n):
            return (WX + 256 * sig + 2 * n, WX + 256 * sig + 2 * n + 1)

        def sloc(kb, l):
            return ((2 * kb + l // 8, 0, l % 8), (2 * kb + l // 8, 1, l % 8))

        def pass_kv():
            t = [taps[g, a] for a in range(KS)]
            prev = {sh: jnp.zeros((8, 128), U32) for sh in (1, 2)}
            for v in range(S // 16):
                w0, = begin([pltpu.bitcast(abuf[sl, 1, pl.ds(16 * v, 16), :], U32)], 1)
                vw = pltpu.bitcast(abuf[sl, 2, pl.ds(16 * v, 16), :], U32)
                cur = {sh: pltpu.roll(w0, sh, 0) for sh in (1, 2)}
                w1, w2 = [jnp.where(sub < sh, prev[sh], cur[sh]) for sh in (1, 2)]
                prev = cur
                e0, o0, e1, o1, o2 = (_unpack(w0, 0), _unpack(w0, 1), _unpack(w1, 0),
                                      _unpack(w1, 1), _unpack(w2, 1))
                ke = (e0 * t[0] + o1 * t[1] + e1 * t[2] + o2 * t[3]) * _unpack(vw, 0)
                ko = (o0 * t[0] + e0 * t[1] + o1 * t[2] + e1 * t[3]) * _unpack(vw, 1)
                chain[0] = _pack(ke, ko)
                kvb[pl.ds(8 * v, 8), :] = chain[0]

        def forward(sig, src):
            for n in range(32):
                x = [natural(w, n % 2) for w in begin([src(n // 2 + 16 * d) for d in range(8)], 8)]
                cs = []
                for d in range(4):
                    a, b = twid(TAF + 2 * d), twid(TAF + 2 * (d + 4))
                    if d == 0:
                        s_ = x[4] * b[0]
                        cs.append((x[0] + s_, s_))
                    else:
                        cs.append((x[d] * a[0] + x[d + 4] * b[0], x[d] * a[1] + x[d + 4] * b[1]))
                put4([xloc(sig, n + 32 * k0) for k0 in range(4)], _dft4(cs, +1))
            for k0 in range(4):
                for n in range(8):
                    locs = [xloc(sig, n + 8 * r + 32 * k0) for r in range(4)]
                    put4(locs, fwd4(locs, TB + 8 * k0))
            for k0 in range(4):
                for k1 in range(4):
                    k = k0 + 4 * k1
                    for a in range(2):
                        o = fwd4([xloc(sig, a + 2 * r + 8 * k1 + 32 * k0) for r in range(4)], TC + 8 * k)
                        put4_t([(2 * ((k + 16 * k2) // 8) + a, k % 8) for k2 in range(4)], o)
            for kb in range(8):
                for e in range(4):
                    o = fwd4([sloc(kb, e + 4 * r) for r in range(4)], TD + 8 * kb)
                    put4([xloc(sig, 16 * kb + e + 4 * r) for r in range(4)], o)
            for kb in range(8):
                for k3 in range(4):
                    locs = [xloc(sig, 16 * kb + r + 4 * k3) for r in range(4)]
                    t0 = TE + 8 * (4 * kb + k3)
                    o = fwd4(locs, t0)
                    if sig == 0:
                        hs = ld4([xloc(1, 16 * kb + r + 4 * k3) for r in range(4)])
                        o = inv4([_cmul(a, b) for a, b in zip(o, hs)], t0)
                    put4(locs, o)

        def inverse():
            for kb in range(8):
                for e in range(4):
                    o = inv4(ld4([xloc(0, 16 * kb + e + 4 * r) for r in range(4)]), TD + 8 * kb)
                    put4_t([(2 * kb + (e + 4 * f) // 8, (e + 4 * f) % 8) for f in range(4)], o)
            for k0 in range(4):
                for k1 in range(4):
                    k = k0 + 4 * k1
                    for a in range(2):
                        v = ld4([sloc((k + 16 * r) // 8, 8 * a + k % 8) for r in range(4)])
                        put4([xloc(0, a + 2 * b + 8 * k1 + 32 * k0) for b in range(4)], inv4(v, TC + 8 * k))
            for k0 in range(4):
                for n in range(8):
                    locs = [xloc(0, n + 8 * r + 32 * k0) for r in range(4)]
                    put4(locs, inv4(ld4(locs), TB + 8 * k0))
            dskip = taps[g, KS]
            for n0 in range(32):
                cs = _dft4(ld4([xloc(0, n0 + 32 * r) for r in range(4)]), -1)
                outs = []
                for d in [d0 + 4 * hh for d0 in range(4) for hh in range(2)]:
                    n = n0 + 32 * d
                    a = twid(TAI + 2 * d)
                    if 0 < d < 4 and cfg["a_fine"]:
                        cs[d] = tuple(begin(cs[d], 2))
                    c = cs[d % 4]
                    y = c[0] * a[0] if d == 0 else c[0] * a[0] + c[1] * a[1]
                    kv = natural(kvb[pl.ds(8 * (n // 2), 8), :], n % 2)
                    y = y + jnp.where(j == 0, kv * dskip, ld(WY + n))
                    st(WY + n, y)
                    chain[0] = abuf[sl, 0, pl.ds(8 * n, 8), :].astype(F32) * y
                    aout[g, n // 4, pl.ds(8 * (n % 4), 8), :] = chain[0].astype(BF16)
                    outs.append(chain[0])
                merge(outs)

        def filt(v):
            return ht[pl.ds(pl.multiple_of(g * (S // 2), S // 2) + 8 * v, 8), :]
        if cfg["a_hfirst"]:
            forward(1, filt)
            pass_kv()
        else:
            pass_kv()
            forward(1, filt)
        forward(0, lambda v: kvb[pl.ds(8 * v, 8), :])
        inverse()
        return chain[0]

    scale = DH ** (-0.5)

    def w_slab(m, h):
        j = h // 2
        return pltpu.bitcast(w_parts[j // 8][pl.ds(slab_row(m, h % 2, j % 8), D // 2), :], BF16)

    class Step:
        def __init__(self, s, prev, mem):
            self.s = s
            self.prev = prev
            self.qkv, self.ps, self.os = {}, {}, []
            self.acc = [None] * NB
            self.ocat, self.lead, self.early, self.marks = {}, {}, {}, {}
            self.tie = None
            x = xbuf[s, pl.ds(M, SEG - M), :].astype(F32)
            self.lhsf = jnp.concatenate([mem, x], axis=0)
            self.lhs = self.lhsf.astype(BF16)

        def proj_early(self, m, j, k):
            self.early[m, j] = (k, [_dot(self.lhsf[:, :k].astype(BF16), w_slab(m, 2 * j + e)[:k])
                                    for e in range(2)])

        def proj(self, m, j):
            if (m, j) in self.early:
                k, part = self.early[m, j]
                a, b = [_dot(self.lhsf[:, k:].astype(BF16), w_slab(m, 2 * j + e)[k:]) + part[e]
                        for e in range(2)]
            else:
                a = _dot(self.lhs, w_slab(m, 2 * j))
                b = _dot(self.lhs, w_slab(m, 2 * j + 1))
            self.marks[m, j] = a[0:8]
            lead = qkvb[self.s, m * NPAIR + j]
            if m == 0:
                r = jnp.concatenate([a, b, _unpack(lead, 0), _unpack(lead, 1)], axis=0).astype(BF16)
            else:
                r = pltpu.bitcast(jnp.concatenate([_pack(a, b), lead], axis=0), BF16)
            self.qkv[m, j] = r

        def probs(self, j):
            fill = fill_ref[pl.ds(0, R), pl.ds(0, R)]
            qk = _dot_nt(self.qkv[0, j], self.qkv[1, j])
            if cfg["exp2"]:
                sc = jnp.where(fill == 0.0, qk, fill)
                e = jnp.exp2((sc - jnp.max(sc, axis=-1, keepdims=True)) * (scale * LOG2E))
            else:
                sc = jnp.where(fill == 0.0, qk * scale, fill)
                e = jnp.exp(sc - jnp.max(sc, axis=-1, keepdims=True))
            l = jnp.sum(e, axis=-1, keepdims=True)
            r = pl.reciprocal(l, approx=True)
            r = r * (2.0 - l * r)
            self.ps[j] = (e * r).astype(BF16)

        def attend(self, j):
            o = _dot(self.ps[j], self.qkv[2, j])
            la, lb = o[2 * SEG:2 * SEG + M], o[2 * SEG + M:]
            rows = pl.ds(pl.multiple_of((self.s // 2) * M, M), M)
            if self.prev is None:
                self.lead[j] = (la, lb)
                forms = {2: la + lb, 5: la}
            else:
                a11, a12 = self.prev.lead[j]
                forms = {0: a11 + lb, 1: la + lb, 3: la - a11, 4: a12 - lb, 6: lb}
            for f, v in forms.items():
                ob[f * NPAIR + j, rows, :] = v.astype(BF16)
            self.os += [o[0:SEG], o[SEG:2 * SEG]]

        def wo(self, h0, h1, n):
            if h0 not in self.ocat:
                self.ocat[h0] = jnp.concatenate(self.os[h0:h1], axis=1).astype(BF16)
            w = wo_u[n, pl.ds(h0 * 64, (h1 - h0) * 64), :]
            if self.tie is not None:
                w = jnp.concatenate(
                    [jnp.where(self.s > 1000, pltpu.bitcast(self.tie, U32), w[0:8]), w[8:]], axis=0)
                self.tie = None
            d = _dot(self.ocat[h0], pltpu.bitcast(w, BF16))
            self.acc[n] = d if self.acc[n] is None else d + self.acc[n]

        def finish(self):
            res = jnp.concatenate(self.acc, axis=1)
            obuf[self.s] = res.astype(BF16)
            return res[0:M]

    def steps(i, mem):
        sts = []
        for u in range(U):
            st = Step(i * U + u, sts[-1] if u % 2 else None, mem)
            sts.append(st)
            for item in _step_order(u, cfg):
                if item[0] == "A":
                    if cfg["a"]:
                        ku, km, kj = cfg["kick"]
                        st.tie = part_a(i, sts[ku].marks[km, kj])
                else:
                    dict(P=st.proj, E=st.proj_early, S=st.probs, V=st.attend, W=st.wo)[item[0]](*item[1:])
            mem = st.finish()
        return mem

    def group(g, mem):
        x_copy(g).wait()
        self_wait(abuf.at[g % 2], SA + g % 2)

        @pl.when(jnp.logical_and(g >= 1, g < NG - 1))
        def _():
            a_start(g + 1)
        return loop("steps", 2 * g, 2 * g + 2, steps, mem)

    for j in range(2):
        tw_copy(j).wait()
    lax.fori_loop(0, NG, group, mem0_ref[...].astype(F32))

    ob_cp = pltpu.make_async_copy(
        obuf.at[:, pl.ds(M, SEG - M), :],
        out_hbm.at[:, pl.ds(M, SEG - M), pl.ds(D, D)], sems.at[SO])
    ob_cp.start()
    for g in range(NG):
        pltpu.make_async_copy(
            aout.at[g], out_hbm.at[:, :, pl.ds(g * 128, 128)], sems.at[SO + 1]).start()

    def epi(it, carry):
        ns = [2 * it, 2 * it + 1]

        def blk(hp, u):
            return [wo_u[ns[u], pl.ds((2 * j + hp) * 64, 64), :] for j in range(NPAIR)]

        def mm(f, bs):
            lhs = jnp.concatenate([ob[f * NPAIR + j] for j in range(NPAIR)], axis=1)
            return _dot(lhs, pltpu.bitcast(jnp.concatenate(bs, axis=0), BF16))

        def cb(x, y, sign):
            return [comb(a, b, sign) for a, b in zip(x, y)]

        def put(u, par, c):
            for i in range(NSEG // 2):
                obb[ns[u], 2 * i + par] = c[M * i:M * i + M].astype(BF16)
        m5 = mm(2, blk(1, 1))
        m1 = mm(0, cb(blk(0, 0), blk(1, 1), 1))
        m4 = mm(6, cb(blk(1, 0), blk(0, 0), -1))
        put(0, 0, mm(4, cb(blk(1, 0), blk(1, 1), 1)) + (m1 + m4 - m5))
        m3 = mm(5, cb(blk(0, 1), blk(1, 1), -1))
        put(1, 0, m3 + m5)
        m2 = mm(1, blk(0, 0))
        put(0, 1, m2 + m4)

        def send(n):
            col = pl.multiple_of(D + n * 128, 128)
            pltpu.make_async_copy(
                obb.at[n], out_hbm.at[:, pl.ds(0, M), pl.ds(col, 128)], sems.at[SO + 2]).start()
        send(ns[0])
        put(1, 1, mm(3, cb(blk(0, 0), blk(0, 1), 1)) + (m1 - m2 + m3))
        send(ns[1])
        return carry
    loop("epi", 0, NB // 2, epi, 0)
    ob_cp.wait()
    self_wait(aout, SO + 1)
    self_wait(obb, SO + 2)


def _step_order(u, cfg):
    ks = cfg["ks"]
    tmpl = [(x[0], int(x[1:])) for x in cfg["tmpl"].split()]
    out = []
    if u > 0:
        first = [(kind, t - lag) for t in range(3) for kind, lag in tmpl if kind in "qkv" and t >= lag]
        out += [("E", "qkv".index(kind), j, cfg["ek"]) for kind, j in first[:cfg["ne"]]]
    nw = 0
    for t in range(NPAIR + max(l for _, l in tmpl)):
        for kind, lag in tmpl:
            j = t - lag
            if j < 0:
                continue
            if j >= NPAIR:
                if kind in "qkv" and nw < NB:
                    out.append(("W", 0, ks, nw))
                    nw += 1
                continue
            out.append(("P", "qkv".index(kind), j) if kind in "qkv" else (kind, j))
    out += [("W", 0, ks, n) for n in range(nw, NB)]
    for n in range(NB):
        if u == U - 1 and n == cfg["tie_n"]:
            out.append(("A",))
        out.append(("W", ks, H, n))
    return out


_DEFAULT_CFG = dict(tmpl="k0 v1 S1 q0 V2", ks=16, ne=2, ek=640, exp2=0,
                    a=1, tie_n=7, kick=(0, 1, 1), skew2=0, a_dyn=0, a_merge=5, a_pad=0, a_fine=1,
                    a_g4=8, a_g4i=4, a_hfirst=0)


def _build(cfg):
    tw_np = _twiddles()
    fill_np = np.zeros((96, 128), np.float32)
    fill_np[:R, :R] = _mask_fill() * (DH ** 0.5 if cfg["exp2"] else 1.0)

    def run(A_q, A_k, A_v, A_shift_k, A_ssm_k, A_ssm_D, B_x, B_mem0, B_Wq, B_Wk, B_Wv, B_Wo):
        sk = A_shift_k.T.reshape(KS, NG, 128).transpose(1, 0, 2)
        any_spec = pl.BlockSpec(memory_space=pl.ANY)
        out = pl.pallas_call(
            functools.partial(_kernel, cfg),
            out_shape=jax.ShapeDtypeStruct((NSEG, SEG, 2 * D), BF16),
            in_specs=[any_spec] * 14,
            out_specs=any_spec,
            scratch_shapes=[
                pltpu.VMEM((48 * SLAB + 544, 128), U32),
                pltpu.VMEM((48 * SLAB + 544, 128), U32),
                pltpu.VMEM((NB, H * DH // 2, 128), U32),
                pltpu.VMEM((16, 128, 16, DH), BF16),
                pltpu.VMEM((9, 512, D), BF16),
                pltpu.VMEM((NSEG, SEG, D), BF16),
                pltpu.VMEM((4, NSEG, M, KQ), BF16),
                pltpu.VMEM((4, NSEG * M // 2, KQ), U32),
                pltpu.VMEM((5, 2, HR, KQ), U32),
                pltpu.VMEM((NSEG, 3 * NPAIR, 8, 128), U32),
                pltpu.VMEM((7 * NPAIR, NSEG * M // 2, DH), BF16),
                pltpu.VMEM((NSEG, SEG, D), BF16),
                pltpu.VMEM((NB, NSEG, M, 128), BF16),
                pltpu.VMEM((2, 3, S, 128), BF16),
                pltpu.VMEM((NG + 1, 2, 128, S // 2), BF16),
                pltpu.VMEM((NG * S // 2, 128), U32),
                pltpu.VMEM((S // 2, 128), U32),
                pltpu.VMEM((8 * NW + 32, 128), F32),
                pltpu.VMEM((2, NT, 8, 128), F32),
                pltpu.VMEM((NG, NSEG, SEG, 128), BF16),
                pltpu.VMEM((4, 8, 128), F32),
                pltpu.VMEM((96, 128), F32),
                pltpu.VMEM((NG, 8, 8, 128), F32),
                pltpu.VMEM((M, D), BF16),
                pltpu.VMEM((NG, KS, 128), BF16),
                pltpu.VMEM((4, NG, 128), BF16),
                pltpu.SemaphoreType.DMA((56,)),
            ],
            compiler_params=pltpu.CompilerParams(vmem_limit_bytes=124 * 1024 * 1024,
                                                 disable_bounds_checks=True),
        )(A_q.reshape(S, D), A_k.reshape(S, D), A_v.reshape(S, D), sk, A_ssm_k,
          A_ssm_D.reshape(NG, 128), B_x.reshape(NSEG, SEG, D), B_mem0.reshape(M, D),
          B_Wq, B_Wk, B_Wv, B_Wo.reshape(H * DH, D),
          jnp.asarray(tw_np), jnp.asarray(fill_np))
        return out.reshape(1, S, 2 * D)

    return run


@functools.partial(jax.jit, static_argnames=("B_seg_len",))
def pallas_concat_heads__ssm_conv_h3__memory_aug_recurrent_mem_tr__prompt_kernel(
    A_q: jax.Array,
    A_k: jax.Array,
    A_v: jax.Array,
    A_shift_k: jax.Array,
    A_ssm_k: jax.Array,
    A_ssm_D: jax.Array,
    B_x: jax.Array,
    B_mem0: jax.Array,
    B_Wq: jax.Array,
    B_Wk: jax.Array,
    B_Wv: jax.Array,
    B_Wo: jax.Array,
    B_seg_len: int = SEG,
):
    assert B_seg_len == SEG
    return _build(_DEFAULT_CFG)(A_q, A_k, A_v, A_shift_k, A_ssm_k, A_ssm_D, B_x, B_mem0,
                                B_Wq, B_Wk, B_Wv, B_Wo)
```

```python
import functools

import numpy as np
import jax
import jax.numpy as jnp
from jax import lax
import jax.experimental.pallas as pl
import jax.experimental.pallas.tpu as pltpu

F32 = jnp.float32
BF16 = jnp.bfloat16
U32 = jnp.uint32

S = 2048
D = 1024
H = 32
DH = 128
M = 8
SEG = 32
NSEG = S // SEG
U = 4
NPAIR = H // 2
R = 2 * (M + SEG)
SLAB = 520
KS = 4
NG = D // 128
KQ = D // 4
NB = D // 128
HR = NSEG * M // 4

TAF, TAI, TB, TC, TD, TE, NT = 0, 16, 32, 64, 192, 256, 512
WX, WS, WY, NW = 0, 512, 1024, 1280
LOG2E = 1.4426950408889634


def _twiddles():
    tw = np.zeros((2, NT, 8), np.float64)

    def put(j, idx, z):
        tw[j, idx] = np.real(z)
        tw[j, idx + 1] = np.imag(z)
    s = np.arange(8)
    tau = 2j * np.pi
    for j in range(2):
        lx = 1j * np.pi * (1 + 4 * j) / 4096
        for d in range(8):
            put(j, TAF + 2 * d, np.exp(lx * 256 * d))
            put(j, TAI + 2 * d, np.exp(lx * 256 * d) / 2048)
        for r in range(4):
            for k in range(4):
                put(j, TB + 8 * k + 2 * r, np.exp((lx * 64 + tau * k / 16) * r))
            for k in range(16):
                put(j, TC + 8 * k + 2 * r, np.exp((lx * 16 + tau * k / 64) * r))
            for kb in range(8):
                put(j, TD + 8 * kb + 2 * r, np.exp((lx * 4 + tau * (s + 8 * kb) / 256) * r))
                for k3 in range(4):
                    put(j, TE + 8 * (4 * kb + k3) + 2 * r,
                        np.exp((lx + tau * (s + 8 * kb + 64 * k3) / 1024) * r))
    return np.ascontiguousarray(np.broadcast_to(tw[..., None], (2, NT, 8, 128))).astype(np.float32)


def _mask_fill():
    blk = np.concatenate([np.arange(M), M + np.arange(M, SEG)])
    lead = M + np.arange(M)
    qhead = np.concatenate([np.zeros(SEG), np.ones(SEG), np.zeros(M), np.ones(M)])
    qpos = np.concatenate([blk, blk, lead, lead])
    khead = np.arange(R) % 2
    kpos = np.concatenate([blk, lead])[np.arange(R) // 2]
    same = qhead[:, None] == khead[None, :]
    ok = (qpos[:, None] < M) | (qpos[:, None] >= kpos[None, :])
    fill = np.where(same, np.where(ok, 0.0, -1e9), -np.inf)
    return fill.astype(np.float32)


def _pack(lo, hi):
    return pltpu.pack_elementwise([lo, hi], packed_dtype=BF16)


def _unpack(w, index):
    return pltpu.unpack_elementwise(w, index=index, packed_dtype=BF16, unpacked_dtype=F32)


def _dot(a, b):
    return jnp.dot(a, b, preferred_element_type=F32)


def _dot_nt(a, b):
    return lax.dot_general(a, b, (((1,), (1,)), ((), ())), preferred_element_type=F32)


def _cadd(a, b):
    return (a[0] + b[0], a[1] + b[1])


def _csub(a, b):
    return (a[0] - b[0], a[1] - b[1])


def _cmul(a, w):
    return (a[0] * w[0] - a[1] * w[1], a[0] * w[1] + a[1] * w[0])


def _cmulc(a, w):
    return (a[0] * w[0] + a[1] * w[1], a[1] * w[0] - a[0] * w[1])


def _bfly_i(b, d, sg):
    p = (b[0] - d[1], b[1] + d[0])
    q = (b[0] + d[1], b[1] - d[0])
    return (p, q) if sg > 0 else (q, p)


def _dft4(x, sg):
    a, b = _cadd(x[0], x[2]), _csub(x[0], x[2])
    c, d = _cadd(x[1], x[3]), _csub(x[1], x[3])
    p, q = _bfly_i(b, d, sg)
    return [_cadd(a, c), p, _csub(a, c), q]


def _kernel(cfg,
            aq_hbm, ak_hbm, av_hbm, sk_hbm, ssmk_hbm, ssmd_hbm, x_hbm, mem0_hbm,
            wq_hbm, wk_hbm, wv_hbm, wo_hbm, tw_hbm, fill_hbm,
            out_hbm,
            w_a, w_b, wo_u, wstage, wostage, xbuf, xlead, xlead_u, xs_u, qkvb, ob, obuf, obb,
            abuf, hbuf, ht, kvb, wk, tw, aout, kickbuf,
            fill_ref, taps, mem0_ref, sk_ref, ssmd_ref,
            sems):
    import contextlib
    scope = jax.named_scope if cfg.get("scopes") else (lambda name: contextlib.nullcontext())
    SW, SWO, SXL, SX, SH, SA, ST, SO, SS = 0, 16, 24, 28, 36, 44, 46, 48, 52
    only = cfg.get("only")

    def loop(name, lo, hi, body, init):
        if only is not None and name not in only:
            return init
        if cfg.get("scopes") == 2:
            def body2(i, c):
                with scope(name + "_it"):
                    return body(i, c)
            return lax.fori_loop(lo, hi, body2, init)
        with scope(name):
            return lax.fori_loop(lo, hi, body, init)
    w_hbms = (wq_hbm, wk_hbm, wv_hbm)
    a_hbms = (aq_hbm, ak_hbm, av_hbm)

    def w_copy(u, q=None):
        rows = pl.ds(0, D) if q is None else pl.ds(q * KQ, KQ)
        sem = SW + 8 + u % 4 if q is None else SW + 4 * u + q
        return pltpu.make_async_copy(
            w_hbms[u // 4].at[rows, pl.ds(8 * (u % 4), 8), :], wstage.at[u % 4, rows], sems.at[sem])

    def self_wait(ref, sem):
        pltpu.make_async_copy(ref, ref, sems.at[sem]).wait()

    def late_start(k):
        pltpu.make_async_copy(
            wo_hbm.at[pl.ds(k * 512, 512), :], wostage.at[k], sems.at[SWO + k]).start()
        for part in range(2):
            pltpu.make_async_copy(
                ssmk_hbm.at[pl.ds(k * 128, 128), pl.ds(part * (S // 2), S // 2)],
                hbuf.at[k, part], sems.at[SH + k]).start()

    def xlead_copy(q):
        return pltpu.make_async_copy(
            x_hbm.at[:, pl.ds(0, M), pl.ds(q * KQ, KQ)], xlead.at[q], sems.at[SXL + q])

    def x_copy(g):
        segs = pl.ds(g * 8, 8)
        return pltpu.make_async_copy(
            x_hbm.at[segs, pl.ds(M, SEG - M), :], xbuf.at[segs, pl.ds(M, SEG - M), :], sems.at[SX + g])

    def a_start(g):
        col = g * 128 if isinstance(g, int) else pl.multiple_of(g * 128, 128)
        for t in (1, 2, 0):
            pltpu.make_async_copy(
                a_hbms[t].at[:, pl.ds(col, 128)], abuf.at[g % 2, t], sems.at[SA + g % 2]).start()

    def tw_copy(j):
        return pltpu.make_async_copy(tw_hbm.at[j], tw.at[j], sems.at[ST + j])

    small = [pltpu.make_async_copy(src, dst, sems.at[SS + i]) for i, (src, dst) in enumerate((
        (fill_hbm, fill_ref), (mem0_hbm, mem0_ref), (sk_hbm, sk_ref), (ssmd_hbm, ssmd_ref.at[0])))]

    for q in range(4):
        xlead_copy(q).start()
        w_copy(0, q).start()
        if q > 0:
            w_copy(1, q - 1).start()
    w_copy(1, 3).start()
    w_copy(2).start()
    w_copy(3).start()

    w_parts = (w_a, w_b)

    def slab_row(u, par, jl):
        return ((u // 2) * 8 + par * 4 + jl) * SLAB

    def gated(x, i, n, gates):
        if gates is None:
            return x
        never, vals = gates
        v = vals[(i * len(vals) * 3) // (n * 4)]
        return jnp.where(never, pltpu.bitcast(v, U32), x)

    def vregs(*mats):
        return [m_[r:r + 8] for m_ in mats for r in range(0, m_.shape[0], 8)]

    def relayout(u, g, q, gates=None, src=None):
        slot, qs = (u % 4, q) if src is None else src
        low = lax.broadcasted_iota(jnp.int32, (8, 128), 0) < 4
        keep = jnp.where(low, jnp.uint32(0xFFFF), jnp.uint32(0xFFFF0000))
        shl = jnp.where(low, jnp.uint32(16), jnp.uint32(0))
        base = slab_row(u, 0, 0) + q * (KQ // 2)
        for i in range(KQ // 2):
            x = wstage[slot, pl.ds(qs * KQ + 2 * i, 2)].reshape(16, DH)
            x = gated(pltpu.bitcast(x, U32), i, KQ // 2, gates)
            y = pltpu.roll(x, 4, 0)
            w_parts[g][pl.ds(base + i, 8, stride=SLAB), :] = (x & keep) | ((y << shl) >> (16 - shl))

    def comb(x, y, sign):
        f = (lambda a, b: a + b) if sign > 0 else (lambda a, b: a - b)
        return _pack(f(_unpack(x, 0), _unpack(y, 0)), f(_unpack(x, 1), _unpack(y, 1)))

    def batch_pair(u, g, jl):
        it = 4 * u + jl
        rows = [pl.multiple_of(slab_row(u, par, jl), 8) for par in range(2)]

        def blk(kh, par):
            return w_parts[g][pl.ds(rows[par] + kh * (D // 4), D // 4), :]

        def mm(a, b):
            return _dot(pltpu.bitcast(jnp.concatenate(a, axis=1), BF16), pltpu.bitcast(b, BF16))

        def xs(f):
            return [xs_u[f, q] for q in range(2)]
        a11 = [xlead_u[q, pl.ds(0, HR), :] for q in (0, 1)]
        a22 = [xlead_u[q, pl.ds(HR, HR), :] for q in (2, 3)]
        m5 = mm(xs(2), blk(1, 1))
        m1 = mm(xs(0), comb(blk(0, 0), blk(1, 1), 1))
        m4 = mm(a22, comb(blk(1, 0), blk(0, 0), -1))
        c11 = mm(xs(4), comb(blk(1, 0), blk(1, 1), 1)) + (m1 + m4 - m5)
        m3 = mm(a11, comb(blk(0, 1), blk(1, 1), -1))
        qkvb[pl.ds(0, NSEG // 2), it] = _pack(c11, m3 + m5).reshape(NSEG // 2, M, DH)
        m2 = mm(xs(1), blk(0, 0))
        c22 = mm(xs(3), comb(blk(0, 0), blk(0, 1), 1)) + (m1 - m2 + m3)
        qkvb[pl.ds(NSEG // 2, NSEG // 2), it] = _pack(m2 + m4, c22).reshape(NSEG // 2, M, DH)
        return vregs(m5, m1, m4, c11, m3, m2, c22)

    def quarter_wait(u, q):
        self_wait(wstage.at[u, pl.ds(pl.multiple_of(q * KQ, KQ), KQ)], SW + 4 * u + q)

    def first_unit(q, carry):
        never = q > 1000
        half = q % 2
        self_wait(xlead.at[q], SXL + q)
        quarter_wait(0, q)
        xq = xlead[q].astype(F32).reshape(NSEG * M, KQ).astype(BF16)
        xlead_u[q] = pltpu.bitcast(xq, U32)
        relayout(0, 0, q)

        @pl.when(q > 0)
        def _():
            quarter_wait(1, q - 1)
        res = []
        xq = pltpu.bitcast(xlead_u[q], BF16)
        for jl in range(4):
            outs = []
            for par in range(2):
                acc = pl.ds((2 * jl + par) * (NSEG * M), NSEG * M)
                row = pl.multiple_of(slab_row(0, par, jl) + q * (KQ // 2), 8)
                w = pltpu.bitcast(w_a[pl.ds(row, KQ // 2), :], BF16)
                d = _dot(xq, w) + jnp.where(q == 0, 0.0, wk[acc, :])
                wk[acc, :] = d
                outs.append(d)
            qkvb[:, jl] = _pack(outs[0], outs[1]).reshape(NSEG, M, DH)
            res += outs
        gates = (never, vregs(*res))
        qn = jnp.maximum(q - 1, 0)
        relayout(1, 1, qn, gates, src=(jnp.minimum(q, 1), qn))
        for r in range(0, HR, 8):
            for cb in range(2):
                cols = pl.ds(cb * 128, 128)
                i = 2 * (r // 8) + cb
                a11 = gated(xlead_u[half, pl.ds(r, 8), cols], i, HR // 4, gates)
                a22 = gated(xlead_u[2 + half, pl.ds(HR + r, 8), cols], i, HR // 4, gates)
                a21 = xlead_u[half, pl.ds(HR + r, 8), cols]
                a12 = xlead_u[2 + half, pl.ds(r, 8), cols]
                for f, (x, y, sg) in enumerate(((a11, a22, 1), (a21, a22, 1), (a11, a12, 1),
                                                (a21, a11, -1), (a12, a22, -1))):
                    xs_u[f, half, pl.ds(r, 8), cols] = comb(x, y, sg)
        return carry
    loop("units", 0, 4, first_unit, 0)
    w_copy(1, 3).wait()
    relayout(1, 1, 3)

    def issue(u):
        for un in {2: (4, 5, 6)}.get(u, (u + 4,) if 2 < u < 8 else ()):
            w_copy(un).start()
        for k in cfg["late"].get(u, ()):
            late_start(k)
        if u == 1:
            for cp in small:
                cp.start()
        if u == 8:
            x_copy(0).start()
            a_start(0)
            tw_copy(0).start()
            tw_copy(1).start()
        if u == 10:
            a_start(1)
            for g in range(1, NG):
                x_copy(g).start()

    def late_relayout(src, hp, gates):
        half = hp % 2
        for r in range(16):
            blk = pltpu.bitcast(
                wostage[src, pl.ds(pl.multiple_of(half * 256 + r * 16, 16), 16), :], U32)
            row = pl.multiple_of(hp * 128 + r * 8, 8)
            for n in range(NB):
                wo_u[n, pl.ds(row, 8), :] = gated(blk[:, n * 128:(n + 1) * 128], r * NB + n, 16 * NB, gates)
        for t in range(8):
            tile = pltpu.bitcast(hbuf[src, half, :, pl.ds(t * 128, 128)], U32)
            tile = jnp.concatenate([gated(tile[0:8], t, 8, gates), tile[8:]], axis=0)
            row = pl.multiple_of(hp * 512 + t * 64, 64)
            ht[pl.ds(row, 64), :] = pltpu.bitcast(pltpu.bitcast(tile, BF16).T, U32)

    def unit_body(u, g):
        real = jnp.logical_and(u > 1, u < 11)

        @pl.when(real)
        def _():
            self_wait(wstage.at[(u + 1) % 4], SW + 8 + (u + 1) % 4)

        @pl.when(u >= 8)
        def _():
            for e in range(2):
                k = (u - 8) * 2 + e
                self_wait(wostage.at[k], SWO + k)
                self_wait(hbuf.at[k], SH + k)
        with scope("unit"):
            if only is None or "chunk" in only:
                for jl in range(4):
                    gates = (u > 1000, batch_pair(u, g, jl))
                    relayout(jnp.where(real, u + 1, u - 1), 1 - g, jl, gates)
                    hp = jnp.maximum(u - 8, 0) * 4 + jl
                    late_relayout(jnp.where(u >= 8, hp // 2, 8), hp, gates)

    def unit_pair(mm, carry):
        for g, u in ((1, 2 * mm + 1), (0, 2 * mm + 2)):
            if g == 0:
                @pl.when(u == 2)
                def _():
                    w_copy(2).wait()

                    def body(q, c):
                        relayout(2, 0, q)
                        return c
                    lax.fori_loop(0, 4, body, 0)
            for us in range(2 - g, 11, 2):
                pl.when(u == us)(functools.partial(issue, us))
            pl.when(u < 12)(functools.partial(unit_body, u, g))
        return carry
    lax.fori_loop(0, 6, unit_pair, 0)

    for cp in small:
        cp.wait()
    dd = ssmd_ref[0].astype(F32)
    for g in range(NG):
        sk = sk_ref[g].astype(F32)
        for j in range(KS):
            taps[g, j] = jnp.broadcast_to(sk[j:j + 1], (8, 128))
        taps[g, KS] = jnp.broadcast_to(dd[g:g + 1], (8, 128))

    def part_a(i, kick):
        g, j = i // 2, i % 2
        sl = g % 2
        never = i > 1000
        z = pl.multiple_of(jnp.where(never, 32, 0), 32) if cfg["a_dyn"] else 0
        sub = lax.broadcasted_iota(jnp.int32, (8, 128), 0)
        kickbuf[jnp.where(never, 1, 0)] = kick
        chain = [kickbuf[jnp.where(i > 2000, 0, 1)]]

        def begin(xs, ng):
            xs = list(xs)
            for e in range(min(ng, len(xs))):
                c = chain[0]
                c = c if c.dtype == xs[e].dtype else pltpu.bitcast(c, xs[e].dtype)
                xs[e] = jnp.where(never, c, xs[e])
            return xs

        def merge(vals):
            c = vals[-1]
            for v in list(vals[:-1])[:cfg["a_merge"]] + list(vals[:cfg["a_pad"]]):
                c = jnp.maximum(v, c)
            chain[0] = c

        def ld(v):
            if isinstance(v, tuple):
                blk, ri, r = v
                base = 8 * WS + 256 * blk + 16 * ri + 32 * r
                if cfg["skew2"]:
                    base += 8 * (blk % 2)
                lo = wk[pl.ds(base, 8), :]
                if r == 0:
                    return lo
                if cfg["skew2"]:
                    return pltpu.roll(lo, 8 - r, 0)
                return pltpu.roll(jnp.where(sub >= r, lo, wk[pl.ds(base + 8, 8), :]), 8 - r, 0)
            return wk[pl.ds(z + 8 * v, 8), :]

        def st(v, x):
            wk[pl.ds(z + 8 * v, 8), :] = x

        def twid(idx):
            return (tw[j, idx], tw[j, idx + 1])

        def natural(w, hh):
            return pltpu.bitcast(w, BF16).astype(F32)[8 * hh:8 * hh + 8]

        def pairs(flat):
            return [(flat[2 * e], flat[2 * e + 1]) for e in range(len(flat) // 2)]

        def fwd4(locs, t0):
            v = pairs(begin([ld(x) for loc in locs[::-1] for x in loc], cfg["a_g4"]))[::-1]
            return _dft4([v[0]] + [_cmul(v[r], twid(t0 + 2 * r)) for r in range(1, 4)], +1)

        def inv4(v, t0):
            o = _dft4(v, -1)
            return [o[0]] + [_cmulc(o[r], twid(t0 + 2 * r)) for r in range(1, 4)]

        def ld4(locs):
            return pairs(begin([ld(x) for loc in locs for x in loc], cfg["a_g4i"]))

        def put4(locs, o):
            for loc, x in zip(locs, o):
                st(loc[0], x[0])
                st(loc[1], x[1])
            merge([x for c in o for x in c])

        def put4_t(dsts, o):
            for (blk, slot), x in zip(dsts, o):
                for ri in range(2):
                    base = 8 * WS + 256 * blk + 16 * ri + slot
                    if cfg["skew2"]:
                        base += 8 * (blk % 2)
                        wk[pl.ds(base, 8 - slot, stride=33), :] = x[ri][0:8 - slot]
                        if slot:
                            wk[pl.ds(base - 8 + 33 * (8 - slot), slot, stride=33), :] = x[ri][8 - slot:8]
                    else:
                        wk[pl.ds(base, 8, stride=33), :] = x[ri]
            merge([x for c in o for x in c])

        def xloc(sig, n):
            return (WX + 256 * sig + 2 * n, WX + 256 * sig + 2 * n + 1)

        def sloc(kb, l):
            return ((2 * kb + l // 8, 0, l % 8), (2 * kb + l // 8, 1, l % 8))

        def pass_kv():
            t = [taps[g, a] for a in range(KS)]
            prev = {sh: jnp.zeros((8, 128), U32) for sh in (1, 2)}
            for v in range(S // 16):
                w0, = begin([pltpu.bitcast(abuf[sl, 1, pl.ds(16 * v, 16), :], U32)], 1)
                vw = pltpu.bitcast(abuf[sl, 2, pl.ds(16 * v, 16), :], U32)
                cur = {sh: pltpu.roll(w0, sh, 0) for sh in (1, 2)}
                w1, w2 = [jnp.where(sub < sh, prev[sh], cur[sh]) for sh in (1, 2)]
                prev = cur
                e0, o0, e1, o1, o2 = (_unpack(w0, 0), _unpack(w0, 1), _unpack(w1, 0),
                                      _unpack(w1, 1), _unpack(w2, 1))
                ke = (e0 * t[0] + o1 * t[1] + e1 * t[2] + o2 * t[3]) * _unpack(vw, 0)
                ko = (o0 * t[0] + e0 * t[1] + o1 * t[2] + e1 * t[3]) * _unpack(vw, 1)
                chain[0] = _pack(ke, ko)
                kvb[pl.ds(8 * v, 8), :] = chain[0]

        def forward(sig, src):
            for n in range(32):
                x = [natural(w, n % 2) for w in begin([src(n // 2 + 16 * d) for d in range(8)], 8)]
                cs = []
                for d in range(4):
                    a, b = twid(TAF + 2 * d), twid(TAF + 2 * (d + 4))
                    if d == 0:
                        s_ = x[4] * b[0]
                        cs.append((x[0] + s_, s_))
                    else:
                        cs.append((x[d] * a[0] + x[d + 4] * b[0], x[d] * a[1] + x[d + 4] * b[1]))
                put4([xloc(sig, n + 32 * k0) for k0 in range(4)], _dft4(cs, +1))
            for k0 in range(4):
                for n in range(8):
                    locs = [xloc(sig, n + 8 * r + 32 * k0) for r in range(4)]
                    put4(locs, fwd4(locs, TB + 8 * k0))
            for k0 in range(4):
                for k1 in range(4):
                    k = k0 + 4 * k1
                    for a in range(2):
                        o = fwd4([xloc(sig, a + 2 * r + 8 * k1 + 32 * k0) for r in range(4)], TC + 8 * k)
                        put4_t([(2 * ((k + 16 * k2) // 8) + a, k % 8) for k2 in range(4)], o)
            for kb in range(8):
                for e in range(4):
                    o = fwd4([sloc(kb, e + 4 * r) for r in range(4)], TD + 8 * kb)
                    put4([xloc(sig, 16 * kb + e + 4 * r) for r in range(4)], o)
            for kb in range(8):
                for k3 in range(4):
                    locs = [xloc(sig, 16 * kb + r + 4 * k3) for r in range(4)]
                    t0 = TE + 8 * (4 * kb + k3)
                    o = fwd4(locs, t0)
                    if sig == 0:
                        hs = ld4([xloc(1, 16 * kb + r + 4 * k3) for r in range(4)])
                        o = inv4([_cmul(a, b) for a, b in zip(o, hs)], t0)
                    put4(locs, o)

        def inverse():
            for kb in range(8):
                for e in range(4):
                    o = inv4(ld4([xloc(0, 16 * kb + e + 4 * r) for r in range(4)]), TD + 8 * kb)
                    put4_t([(2 * kb + (e + 4 * f) // 8, (e + 4 * f) % 8) for f in range(4)], o)
            for k0 in range(4):
                for k1 in range(4):
                    k = k0 + 4 * k1
                    for a in range(2):
                        v = ld4([sloc((k + 16 * r) // 8, 8 * a + k % 8) for r in range(4)])
                        put4([xloc(0, a + 2 * b + 8 * k1 + 32 * k0) for b in range(4)], inv4(v, TC + 8 * k))
            for k0 in range(4):
                for n in range(8):
                    locs = [xloc(0, n + 8 * r + 32 * k0) for r in range(4)]
                    put4(locs, inv4(ld4(locs), TB + 8 * k0))
            dskip = taps[g, KS]
            for n0 in range(32):
                cs = _dft4(ld4([xloc(0, n0 + 32 * r) for r in range(4)]), -1)
                outs = []
                for d in [d0 + 4 * hh for d0 in range(4) for hh in range(2)]:
                    n = n0 + 32 * d
                    a = twid(TAI + 2 * d)
                    if 0 < d < 4 and cfg["a_fine"]:
                        cs[d] = tuple(begin(cs[d], 2))
                    c = cs[d % 4]
                    y = c[0] * a[0] if d == 0 else c[0] * a[0] + c[1] * a[1]
                    kv = natural(kvb[pl.ds(8 * (n // 2), 8), :], n % 2)
                    y = y + jnp.where(j == 0, kv * dskip, ld(WY + n))
                    st(WY + n, y)
                    chain[0] = abuf[sl, 0, pl.ds(8 * n, 8), :].astype(F32) * y
                    aout[g, n // 4, pl.ds(8 * (n % 4), 8), :] = chain[0].astype(BF16)
                    outs.append(chain[0])
                merge(outs)

        def filt(v):
            return ht[pl.ds(pl.multiple_of(g * (S // 2), S // 2) + 8 * v, 8), :]
        if cfg["a_hfirst"]:
            forward(1, filt)
            pass_kv()
        else:
            pass_kv()
            forward(1, filt)
        forward(0, lambda v: kvb[pl.ds(8 * v, 8), :])
        inverse()
        return chain[0]

    scale = DH ** (-0.5)

    def w_slab(m, h):
        u = 4 * m + h // 8
        return pltpu.bitcast(w_parts[u % 2][pl.ds(slab_row(u, h % 2, (h // 2) % 4), D // 2), :], BF16)

    class Step:
        def __init__(self, s, prev, mem):
            self.s = s
            self.prev = prev
            self.qkv, self.ps, self.os = {}, {}, []
            self.acc = [None] * NB
            self.ocat, self.lead, self.early, self.marks = {}, {}, {}, {}
            self.tie = None
            x = xbuf[s, pl.ds(M, SEG - M), :].astype(F32)
            self.lhsf = jnp.concatenate([mem, x], axis=0)
            self.lhs = self.lhsf.astype(BF16)

        def proj_early(self, m, j, k):
            self.early[m, j] = (k, [_dot(self.lhsf[:, :k].astype(BF16), w_slab(m, 2 * j + e)[:k])
                                    for e in range(2)])

        def proj(self, m, j):
            if (m, j) in self.early:
                k, part = self.early[m, j]
                a, b = [_dot(self.lhsf[:, k:].astype(BF16), w_slab(m, 2 * j + e)[k:]) + part[e]
                        for e in range(2)]
            else:
                a = _dot(self.lhs, w_slab(m, 2 * j))
                b = _dot(self.lhs, w_slab(m, 2 * j + 1))
            self.marks[m, j] = a[0:8]
            lead = qkvb[self.s, m * NPAIR + j]
            if m == 0:
                r = jnp.concatenate([a, b, _unpack(lead, 0), _unpack(lead, 1)], axis=0).astype(BF16)
            else:
                r = pltpu.bitcast(jnp.concatenate([_pack(a, b), lead], axis=0), BF16)
            self.qkv[m, j] = r

        def probs(self, j):
            fill = fill_ref[pl.ds(0, R), pl.ds(0, R)]
            qk = _dot_nt(self.qkv[0, j], self.qkv[1, j])
            if cfg["exp2"]:
                sc = jnp.where(fill == 0.0, qk, fill)
                e = jnp.exp2((sc - jnp.max(sc, axis=-1, keepdims=True)) * (scale * LOG2E))
            else:
                sc = jnp.where(fill == 0.0, qk * scale, fill)
                e = jnp.exp(sc - jnp.max(sc, axis=-1, keepdims=True))
            l = jnp.sum(e, axis=-1, keepdims=True)
            r = pl.reciprocal(l, approx=True)
            r = r * (2.0 - l * r)
            self.ps[j] = (e * r).astype(BF16)

        def attend(self, j):
            o = _dot(self.ps[j], self.qkv[2, j])
            la, lb = o[2 * SEG:2 * SEG + M], o[2 * SEG + M:]
            rows = pl.ds(pl.multiple_of((self.s // 2) * M, M), M)
            if self.prev is None:
                self.lead[j] = (la, lb)
                forms = {2: la + lb, 5: la}
            else:
                a11, a12 = self.prev.lead[j]
                forms = {0: a11 + lb, 1: la + lb, 3: la - a11, 4: a12 - lb, 6: lb}
            for f, v in forms.items():
                ob[f * NPAIR + j, rows, :] = v.astype(BF16)
            self.os += [o[0:SEG], o[SEG:2 * SEG]]

        def wo(self, h0, h1, n):
            if h0 not in self.ocat:
                self.ocat[h0] = jnp.concatenate(self.os[h0:h1], axis=1).astype(BF16)
            w = wo_u[n, pl.ds(h0 * 64, (h1 - h0) * 64), :]
            if self.tie is not None:
                w = jnp.concatenate(
                    [jnp.where(self.s > 1000, pltpu.bitcast(self.tie, U32), w[0:8]), w[8:]], axis=0)
                self.tie = None
            d = _dot(self.ocat[h0], pltpu.bitcast(w, BF16))
            self.acc[n] = d if self.acc[n] is None else d + self.acc[n]

        def finish(self):
            res = jnp.concatenate(self.acc, axis=1)
            obuf[self.s] = res.astype(BF16)
            return res[0:M]

    def steps(i, mem):
        sts = []
        for u in range(U):
            st = Step(i * U + u, sts[-1] if u % 2 else None, mem)
            sts.append(st)
            for item in _step_order(u, cfg):
                if item[0] == "A":
                    if cfg["a"]:
                        ku, km, kj = cfg["kick"]
                        st.tie = part_a(i, sts[ku].marks[km, kj])
                else:
                    dict(P=st.proj, E=st.proj_early, S=st.probs, V=st.attend, W=st.wo)[item[0]](*item[1:])
            mem = st.finish()
        return mem

    def group(g, mem):
        x_copy(g).wait()
        self_wait(abuf.at[g % 2], SA + g % 2)

        @pl.when(jnp.logical_and(g >= 1, g < NG - 1))
        def _():
            a_start(g + 1)
        return loop("steps", 2 * g, 2 * g + 2, steps, mem)

    for j in range(2):
        tw_copy(j).wait()
    lax.fori_loop(0, NG, group, mem0_ref[...].astype(F32))

    ob_cp = pltpu.make_async_copy(
        obuf.at[:, pl.ds(M, SEG - M), :],
        out_hbm.at[:, pl.ds(M, SEG - M), pl.ds(D, D)], sems.at[SO])
    ob_cp.start()
    for g in range(NG):
        pltpu.make_async_copy(
            aout.at[g], out_hbm.at[:, :, pl.ds(g * 128, 128)], sems.at[SO + 1]).start()

    def epi(it, carry):
        ns = [2 * it, 2 * it + 1]

        def blk(hp, u):
            return [wo_u[ns[u], pl.ds((2 * j + hp) * 64, 64), :] for j in range(NPAIR)]

        def mm(f, bs):
            lhs = jnp.concatenate([ob[f * NPAIR + j] for j in range(NPAIR)], axis=1)
            return _dot(lhs, pltpu.bitcast(jnp.concatenate(bs, axis=0), BF16))

        def cb(x, y, sign):
            return [comb(a, b, sign) for a, b in zip(x, y)]

        def put(u, par, c):
            for i in range(NSEG // 2):
                obb[ns[u], 2 * i + par] = c[M * i:M * i + M].astype(BF16)
        m5 = mm(2, blk(1, 1))
        m1 = mm(0, cb(blk(0, 0), blk(1, 1), 1))
        m4 = mm(6, cb(blk(1, 0), blk(0, 0), -1))
        put(0, 0, mm(4, cb(blk(1, 0), blk(1, 1), 1)) + (m1 + m4 - m5))
        m3 = mm(5, cb(blk(0, 1), blk(1, 1), -1))
        put(1, 0, m3 + m5)
        m2 = mm(1, blk(0, 0))
        put(0, 1, m2 + m4)

        def send(n):
            col = pl.multiple_of(D + n * 128, 128)
            pltpu.make_async_copy(
                obb.at[n], out_hbm.at[:, pl.ds(0, M), pl.ds(col, 128)], sems.at[SO + 2]).start()
        send(ns[0])
        put(1, 1, mm(3, cb(blk(0, 0), blk(0, 1), 1)) + (m1 - m2 + m3))
        send(ns[1])
        return carry
    loop("epi", 0, NB // 2, epi, 0)
    ob_cp.wait()
    self_wait(aout, SO + 1)
    self_wait(obb, SO + 2)


def _step_order(u, cfg):
    ks = cfg["ks"]
    tmpl = [(x[0], int(x[1:])) for x in cfg["tmpl"].split()]
    out = []
    if u > 0:
        first = [(kind, t - lag) for t in range(3) for kind, lag in tmpl if kind in "qkv" and t >= lag]
        out += [("E", "qkv".index(kind), j, cfg["ek"]) for kind, j in first[:cfg["ne"]]]
    nw = 0
    for t in range(NPAIR + max(l for _, l in tmpl)):
        for kind, lag in tmpl:
            j = t - lag
            if j < 0:
                continue
            if j >= NPAIR:
                if kind in "qkv" and nw < NB:
                    out.append(("W", 0, ks, nw))
                    nw += 1
                continue
            out.append(("P", "qkv".index(kind), j) if kind in "qkv" else (kind, j))
    out += [("W", 0, ks, n) for n in range(nw, NB)]
    for n in range(NB):
        if u == U - 1 and n == cfg["tie_n"]:
            out.append(("A",))
        out.append(("W", ks, H, n))
    return out


_DEFAULT_CFG = dict(tmpl="k0 v1 S1 q0 V2", ks=16, ne=2, ek=640, exp2=0,
                    a=1, tie_n=7, kick=(0, 1, 1), skew2=0, a_dyn=0, a_merge=5, a_pad=0, a_fine=1,
                    a_g4=8, a_g4i=4, a_hfirst=0,
                    late={1: (0,), 3: (1,), 4: (2,), 5: (3,), 6: (4, 5), 7: (6, 7)})


def _build(cfg):
    tw_np = _twiddles()
    fill_np = np.zeros((96, 128), np.float32)
    fill_np[:R, :R] = _mask_fill() * (DH ** 0.5 if cfg["exp2"] else 1.0)

    def run(A_q, A_k, A_v, A_shift_k, A_ssm_k, A_ssm_D, B_x, B_mem0, B_Wq, B_Wk, B_Wv, B_Wo):
        sk = A_shift_k.T.reshape(KS, NG, 128).transpose(1, 0, 2)
        any_spec = pl.BlockSpec(memory_space=pl.ANY)
        out = pl.pallas_call(
            functools.partial(_kernel, cfg),
            out_shape=jax.ShapeDtypeStruct((NSEG, SEG, 2 * D), BF16),
            in_specs=[any_spec] * 14,
            out_specs=any_spec,
            scratch_shapes=[
                pltpu.VMEM((48 * SLAB + 544, 128), U32),
                pltpu.VMEM((48 * SLAB + 544, 128), U32),
                pltpu.VMEM((NB, H * DH // 2, 128), U32),
                pltpu.VMEM((4, D, 8, DH), BF16),
                pltpu.VMEM((9, 512, D), BF16),
                pltpu.VMEM((NSEG, SEG, D), BF16),
                pltpu.VMEM((4, NSEG, M, KQ), BF16),
                pltpu.VMEM((4, NSEG * M // 2, KQ), U32),
                pltpu.VMEM((5, 2, HR, KQ), U32),
                pltpu.VMEM((NSEG, 3 * NPAIR, 8, 128), U32),
                pltpu.VMEM((7 * NPAIR, NSEG * M // 2, DH), BF16),
                pltpu.VMEM((NSEG, SEG, D), BF16),
                pltpu.VMEM((NB, NSEG, M, 128), BF16),
                pltpu.VMEM((2, 3, S, 128), BF16),
                pltpu.VMEM((NG + 1, 2, 128, S // 2), BF16),
                pltpu.VMEM((NG * S // 2, 128), U32),
                pltpu.VMEM((S // 2, 128), U32),
                pltpu.VMEM((8 * NW + 32, 128), F32),
                pltpu.VMEM((2, NT, 8, 128), F32),
                pltpu.VMEM((NG, NSEG, SEG, 128), BF16),
                pltpu.VMEM((4, 8, 128), F32),
                pltpu.VMEM((96, 128), F32),
                pltpu.VMEM((NG, 8, 8, 128), F32),
                pltpu.VMEM((M, D), BF16),
                pltpu.VMEM((NG, KS, 128), BF16),
                pltpu.VMEM((4, NG, 128), BF16),
                pltpu.SemaphoreType.DMA((56,)),
            ],
            compiler_params=pltpu.CompilerParams(vmem_limit_bytes=124 * 1024 * 1024,
                                                 disable_bounds_checks=True),
        )(A_q.reshape(S, D), A_k.reshape(S, D), A_v.reshape(S, D), sk, A_ssm_k,
          A_ssm_D.reshape(NG, 128), B_x.reshape(NSEG, SEG, D), B_mem0.reshape(M, D),
          B_Wq, B_Wk, B_Wv, B_Wo.reshape(H * DH, D),
          jnp.asarray(tw_np), jnp.asarray(fill_np))
        return out.reshape(1, S, 2 * D)

    return run


@functools.partial(jax.jit, static_argnames=("B_seg_len",))
def pallas_concat_heads__ssm_conv_h3__memory_aug_recurrent_mem_tr__prompt_kernel(
    A_q: jax.Array,
    A_k: jax.Array,
    A_v: jax.Array,
    A_shift_k: jax.Array,
    A_ssm_k: jax.Array,
    A_ssm_D: jax.Array,
    B_x: jax.Array,
    B_mem0: jax.Array,
    B_Wq: jax.Array,
    B_Wk: jax.Array,
    B_Wv: jax.Array,
    B_Wo: jax.Array,
    B_seg_len: int = SEG,
):
    assert B_seg_len == SEG
    return _build(_DEFAULT_CFG)(A_q, A_k, A_v, A_shift_k, A_ssm_k, A_ssm_D, B_x, B_mem0,
                                B_Wq, B_Wk, B_Wv, B_Wo)
```

```python
import functools

import numpy as np
import jax
import jax.numpy as jnp
from jax import lax
import jax.experimental.pallas as pl
import jax.experimental.pallas.tpu as pltpu

F32 = jnp.float32
BF16 = jnp.bfloat16
U32 = jnp.uint32

S = 2048
D = 1024
H = 32
DH = 128
M = 8
SEG = 32
NSEG = S // SEG
U = 4
NPAIR = H // 2
R = 2 * (M + SEG)
SLAB = 520
KS = 4
NG = D // 128
KQ = D // 4
NB = D // 128
HR = NSEG * M // 4

TAF, TAI, TB, TC, TD, TE, NT = 0, 16, 32, 64, 192, 256, 512
WX, WS, WY, NW = 0, 512, 1024, 1280
LOG2E = 1.4426950408889634


def _twiddles():
    tw = np.zeros((2, NT, 8), np.float64)

    def put(j, idx, z):
        tw[j, idx] = np.real(z)
        tw[j, idx + 1] = np.imag(z)
    s = np.arange(8)
    tau = 2j * np.pi
    for j in range(2):
        lx = 1j * np.pi * (1 + 4 * j) / 4096
        for d in range(8):
            put(j, TAF + 2 * d, np.exp(lx * 256 * d))
            put(j, TAI + 2 * d, np.exp(lx * 256 * d) / 2048)
        for r in range(4):
            for k in range(4):
                put(j, TB + 8 * k + 2 * r, np.exp((lx * 64 + tau * k / 16) * r))
            for k in range(16):
                put(j, TC + 8 * k + 2 * r, np.exp((lx * 16 + tau * k / 64) * r))
            for kb in range(8):
                put(j, TD + 8 * kb + 2 * r, np.exp((lx * 4 + tau * (s + 8 * kb) / 256) * r))
                for k3 in range(4):
                    put(j, TE + 8 * (4 * kb + k3) + 2 * r,
                        np.exp((lx + tau * (s + 8 * kb + 64 * k3) / 1024) * r))
    return np.ascontiguousarray(np.broadcast_to(tw[..., None], (2, NT, 8, 128))).astype(np.float32)


def _mask_fill():
    blk = np.concatenate([np.arange(M), M + np.arange(M, SEG)])
    lead = M + np.arange(M)
    qhead = np.concatenate([np.zeros(SEG), np.ones(SEG), np.zeros(M), np.ones(M)])
    qpos = np.concatenate([blk, blk, lead, lead])
    khead = np.arange(R) % 2
    kpos = np.concatenate([blk, lead])[np.arange(R) // 2]
    same = qhead[:, None] == khead[None, :]
    ok = (qpos[:, None] < M) | (qpos[:, None] >= kpos[None, :])
    fill = np.where(same, np.where(ok, 0.0, -1e9), -np.inf)
    return fill.astype(np.float32)


def _pack(lo, hi):
    return pltpu.pack_elementwise([lo, hi], packed_dtype=BF16)


def _unpack(w, index):
    return pltpu.unpack_elementwise(w, index=index, packed_dtype=BF16, unpacked_dtype=F32)


def _dot(a, b):
    return jnp.dot(a, b, preferred_element_type=F32)


def _dot_nt(a, b):
    return lax.dot_general(a, b, (((1,), (1,)), ((), ())), preferred_element_type=F32)


def _cadd(a, b):
    return (a[0] + b[0], a[1] + b[1])


def _csub(a, b):
    return (a[0] - b[0], a[1] - b[1])


def _cmul(a, w):
    return (a[0] * w[0] - a[1] * w[1], a[0] * w[1] + a[1] * w[0])


def _cmulc(a, w):
    return (a[0] * w[0] + a[1] * w[1], a[1] * w[0] - a[0] * w[1])


def _bfly_i(b, d, sg):
    p = (b[0] - d[1], b[1] + d[0])
    q = (b[0] + d[1], b[1] - d[0])
    return (p, q) if sg > 0 else (q, p)


def _dft4(x, sg):
    a, b = _cadd(x[0], x[2]), _csub(x[0], x[2])
    c, d = _cadd(x[1], x[3]), _csub(x[1], x[3])
    p, q = _bfly_i(b, d, sg)
    return [_cadd(a, c), p, _csub(a, c), q]


def _kernel(cfg,
            aq_hbm, ak_hbm, av_hbm, sk_hbm, ssmk_hbm, ssmd_hbm, x_hbm, mem0_hbm,
            wq_hbm, wk_hbm, wv_hbm, wo_hbm, tw_hbm, fill_hbm,
            out_hbm,
            w_a, w_b, wo_u, wstage, wostage, xbuf, xlead, xlead_u, xs_u, qkvb, ob, obuf, obb,
            abuf, hbuf, ht, kvb, wk, tw, aout, kickbuf,
            fill_ref, taps, mem0_ref, sk_ref, ssmd_ref,
            sems):
    import contextlib
    scope = jax.named_scope if cfg.get("scopes") else (lambda name: contextlib.nullcontext())
    SW, SWO, SXL, SX, SH, SA, ST, SO, SS = 0, 16, 24, 28, 36, 44, 46, 48, 52
    only = cfg.get("only")

    def loop(name, lo, hi, body, init):
        if only is not None and name not in only:
            return init
        if cfg.get("scopes") == 2:
            def body2(i, c):
                with scope(name + "_it"):
                    return body(i, c)
            return lax.fori_loop(lo, hi, body2, init)
        with scope(name):
            return lax.fori_loop(lo, hi, body, init)
    w_hbms = (wq_hbm, wk_hbm, wv_hbm)
    a_hbms = (aq_hbm, ak_hbm, av_hbm)

    def w_copy(m, hq, q=None):
        rows = pl.ds(0, D) if q is None else pl.ds(q * KQ, KQ)
        sem = SW + 8 + hq if q is None else SW + 4 * hq + q
        heads = 8 * hq if isinstance(hq, int) else pl.multiple_of(8 * hq, 8)
        return pltpu.make_async_copy(
            w_hbms[m].at[rows, pl.ds(heads, 8), :], wstage.at[hq, rows], sems.at[sem])

    def self_wait(ref, sem):
        pltpu.make_async_copy(ref, ref, sems.at[sem]).wait()

    def late_start(k):
        pltpu.make_async_copy(
            wo_hbm.at[pl.ds(pl.multiple_of(k * 512, 512), 512), :], wostage.at[k],
            sems.at[SWO + k]).start()
        pltpu.make_async_copy(
            ssmk_hbm.at[pl.ds(pl.multiple_of(k * 128, 128), 128), :], hbuf.at[k],
            sems.at[SH + k]).start()

    def xlead_copy(q):
        return pltpu.make_async_copy(
            x_hbm.at[:, pl.ds(0, M), pl.ds(q * KQ, KQ)], xlead.at[q], sems.at[SXL + q])

    def x_copy(g):
        segs = pl.ds(g * 8, 8)
        return pltpu.make_async_copy(
            x_hbm.at[segs, pl.ds(M, SEG - M), :], xbuf.at[segs, pl.ds(M, SEG - M), :], sems.at[SX + g])

    def a_start(g):
        col = g * 128 if isinstance(g, int) else pl.multiple_of(g * 128, 128)
        for t in (1, 2, 0):
            pltpu.make_async_copy(
                a_hbms[t].at[:, pl.ds(col, 128)], abuf.at[g & 1, t], sems.at[SA + (g & 1)]).start()

    tw_cp = pltpu.make_async_copy(tw_hbm, tw, sems.at[ST])

    small = [pltpu.make_async_copy(src, dst, sems.at[SS + i]) for i, (src, dst) in enumerate((
        (fill_hbm, fill_ref), (mem0_hbm, mem0_ref), (sk_hbm, sk_ref), (ssmd_hbm, ssmd_ref.at[0])))]

    for q in range(4):
        xlead_copy(q).start()
        w_copy(0, 0, q).start()
        if q > 0:
            w_copy(0, 1, q - 1).start()
    w_copy(0, 1, 3).start()
    w_copy(0, 2).start()
    w_copy(0, 3).start()
    for cp in small:
        cp.start()

    w_parts = (w_a, w_b)

    def slab_row(u, par, jl):
        return ((u >> 1) * 8 + par * 4 + jl) * SLAB

    def gated(x, i, n, gates):
        if gates is None:
            return x
        never, vals = gates
        v = vals[(i * len(vals) * 3) // (n * 4)]
        return jnp.where(never, pltpu.bitcast(v, U32), x)

    def vregs(*mats):
        return [m_[r:r + 8] for m_ in mats for r in range(0, m_.shape[0], 8)]

    def relayout(u, g, q, gates=None, src=None):
        slot, qs = (u & 3, q) if src is None else src
        low = lax.broadcasted_iota(jnp.int32, (8, 128), 0) < 4
        keep = jnp.where(low, jnp.uint32(0xFFFF), jnp.uint32(0xFFFF0000))
        shl = jnp.where(low, jnp.uint32(16), jnp.uint32(0))
        base = slab_row(u, 0, 0) + q * (KQ // 2)
        for i in range(KQ // 2):
            x = wstage[slot, pl.ds(qs * KQ + 2 * i, 2)].reshape(16, DH)
            x = gated(pltpu.bitcast(x, U32), i, KQ // 2, gates)
            y = pltpu.roll(x, 4, 0)
            w_parts[g][pl.ds(base + i, 8, stride=SLAB), :] = (x & keep) | ((y << shl) >> (16 - shl))

    def comb(x, y, sign):
        f = (lambda a, b: a + b) if sign > 0 else (lambda a, b: a - b)
        return _pack(f(_unpack(x, 0), _unpack(y, 0)), f(_unpack(x, 1), _unpack(y, 1)))

    def batch_pair(u, g, jl):
        it = 4 * u + jl
        rows = [pl.multiple_of(slab_row(u, par, jl), 8) for par in range(2)]

        def blk(kh, par):
            return w_parts[g][pl.ds(rows[par] + kh * (D // 4), D // 4), :]

        def mm(a, b):
            return _dot(pltpu.bitcast(jnp.concatenate(a, axis=1), BF16), pltpu.bitcast(b, BF16))

        def xs(f):
            return [xs_u[f, q] for q in range(2)]
        a11 = [xlead_u[q, pl.ds(0, HR), :] for q in (0, 1)]
        a22 = [xlead_u[q, pl.ds(HR, HR), :] for q in (2, 3)]
        m5 = mm(xs(2), blk(1, 1))
        m1 = mm(xs(0), comb(blk(0, 0), blk(1, 1), 1))
        m4 = mm(a22, comb(blk(1, 0), blk(0, 0), -1))
        c11 = mm(xs(4), comb(blk(1, 0), blk(1, 1), 1)) + (m1 + m4 - m5)
        m3 = mm(a11, comb(blk(0, 1), blk(1, 1), -1))
        qkvb[pl.ds(0, NSEG // 2), it] = _pack(c11, m3 + m5).reshape(NSEG // 2, M, DH)
        m2 = mm(xs(1), blk(0, 0))
        c22 = mm(xs(3), comb(blk(0, 0), blk(0, 1), 1)) + (m1 - m2 + m3)
        qkvb[pl.ds(NSEG // 2, NSEG // 2), it] = _pack(m2 + m4, c22).reshape(NSEG // 2, M, DH)
        return vregs(m5, m1, m4, c11, m3, m2, c22)

    def quarter_wait(u, q):
        self_wait(wstage.at[u, pl.ds(pl.multiple_of(q * KQ, KQ), KQ)], SW + 4 * u + q)

    def first_unit(q, carry):
        never = q > 1000
        half = q & 1
        self_wait(xlead.at[q], SXL + q)
        quarter_wait(0, q)
        xq = xlead[q].astype(F32).reshape(NSEG * M, KQ).astype(BF16)
        xlead_u[q] = pltpu.bitcast(xq, U32)
        relayout(0, 0, q)

        @pl.when(q > 0)
        def _():
            quarter_wait(1, q - 1)
        res = []
        xq = pltpu.bitcast(xlead_u[q], BF16)
        for jl in range(4):
            outs = []
            for par in range(2):
                acc = pl.ds((2 * jl + par) * (NSEG * M), NSEG * M)
                row = pl.multiple_of(slab_row(0, par, jl) + q * (KQ // 2), 8)
                w = pltpu.bitcast(w_a[pl.ds(row, KQ // 2), :], BF16)
                d = _dot(xq, w) + jnp.where(q == 0, 0.0, wk[acc, :])
                wk[acc, :] = d
                outs.append(d)
            qkvb[:, jl] = _pack(outs[0], outs[1]).reshape(NSEG, M, DH)
            res += outs
        gates = (never, vregs(*res))
        qn = jnp.maximum(q - 1, 0)
        relayout(1, 1, qn, gates, src=(jnp.minimum(q, 1), qn))
        for r in range(0, HR, 8):
            for cb in range(2):
                cols = pl.ds(cb * 128, 128)
                i = 2 * (r // 8) + cb
                a11 = gated(xlead_u[half, pl.ds(r, 8), cols], i, HR // 4, gates)
                a22 = gated(xlead_u[2 + half, pl.ds(HR + r, 8), cols], i, HR // 4, gates)
                a21 = xlead_u[half, pl.ds(HR + r, 8), cols]
                a12 = xlead_u[2 + half, pl.ds(r, 8), cols]
                for f, (x, y, sg) in enumerate(((a11, a22, 1), (a21, a22, 1), (a11, a12, 1),
                                                (a21, a11, -1), (a12, a22, -1))):
                    xs_u[f, half, pl.ds(r, 8), cols] = comb(x, y, sg)
        return carry
    loop("units", 0, 4, first_unit, 0)
    w_copy(0, 1, 3).wait()
    relayout(1, 1, 3)

    def late_relayout(src, hp, half, gates):
        for r in range(16):
            blk = pltpu.bitcast(wostage[src, pl.ds(half * 256 + r * 16, 16), :], U32)
            row = pl.multiple_of(hp * 128 + r * 8, 8)
            for n in range(NB):
                wo_u[n, pl.ds(row, 8), :] = gated(blk[:, n * 128:(n + 1) * 128], r * NB + n, 16 * NB, gates)
        for t in range(8):
            tile = pltpu.bitcast(hbuf[src, :, pl.ds((8 * half + t) * 128, 128)], U32)
            tile = jnp.concatenate([gated(tile[0:8], t, 8, gates), tile[8:]], axis=0)
            row = pl.multiple_of(hp * 512 + t * 64, 64)
            ht[pl.ds(row, 64), :] = pltpu.bitcast(pltpu.bitcast(tile, BF16).T, U32)

    def unit_body(u, g):
        @pl.when(jnp.logical_and(u > 1, u < 11))
        def _():
            self_wait(wstage.at[(u + 1) & 3], SW + 8 + ((u + 1) & 3))

        @pl.when(u >= 8)
        def _():
            for e in range(2):
                k = (u - 8) * 2 + e
                self_wait(wostage.at[k], SWO + k)
                self_wait(hbuf.at[k], SH + k)
        for m in (1, 2):
            @pl.when((u + 3) >> 2 == m)
            def _():
                w_copy(m, (u + 3) & 3).start()

        @pl.when(u <= 8)
        def _():
            late_start(u - 1)
        if g == 1:
            @pl.when(u == 9)
            def _():
                x_copy(0).start()
                a_start(0)
                tw_cp.start()
        if only is None or "chunk" in only:
            for jl in range(4):
                gates = (u > 1000, batch_pair(u, g, jl))
                un = jnp.where(u < 11, u + 1, u - 1)
                relayout(un, 1 - g, jl, gates, src=(jnp.where(u == 1, 1, un & 3), jl))
                k = jnp.maximum(u - 8, 0) * 2 + jl // 2
                late_relayout(jnp.where(u >= 8, k, 8), 2 * k + jl % 2, jl % 2, gates)

    def unit_pair(mm, carry):
        with scope("unit"):
            unit_body(2 * mm + 1, 1)

        @pl.when(mm == 0)
        def _():
            w_copy(0, 2).wait()

            def body(q, c):
                relayout(2, 0, q)
                return c
            lax.fori_loop(0, 4, body, 0)

        @pl.when(mm < 5)
        def _():
            with scope("unit"):
                unit_body(2 * mm + 2, 0)
        return carry
    lax.fori_loop(0, 6, unit_pair, 0)

    a_start(1)
    for g in range(1, NG):
        x_copy(g).start()
    for cp in small:
        cp.wait()
    dd = ssmd_ref[0].astype(F32)
    for g in range(NG):
        sk = sk_ref[g].astype(F32)
        for j in range(KS):
            taps[g, j] = jnp.broadcast_to(sk[j:j + 1], (8, 128))
        taps[g, KS] = jnp.broadcast_to(dd[g:g + 1], (8, 128))

    def part_a(i, kick):
        g, j = i >> 1, i & 1
        sl = g & 1
        never = i > 1000
        z = pl.multiple_of(jnp.where(never, 32, 0), 32) if cfg["a_dyn"] else 0
        sub = lax.broadcasted_iota(jnp.int32, (8, 128), 0)
        kickbuf[jnp.where(never, 1, 0)] = kick
        chain = [kickbuf[jnp.where(i > 2000, 0, 1)]]

        def begin(xs, ng):
            xs = list(xs)
            for e in range(min(ng, len(xs))):
                c = chain[0]
                c = c if c.dtype == xs[e].dtype else pltpu.bitcast(c, xs[e].dtype)
                xs[e] = jnp.where(never, c, xs[e])
            return xs

        def merge(vals):
            c = vals[-1]
            for v in list(vals[:-1])[:cfg["a_merge"]] + list(vals[:cfg["a_pad"]]):
                c = jnp.maximum(v, c)
            chain[0] = c

        def ld(v):
            if isinstance(v, tuple):
                blk, ri, r = v
                base = 8 * WS + 256 * blk + 16 * ri + 32 * r
                if cfg["skew2"]:
                    base += 8 * (blk % 2)
                lo = wk[pl.ds(base, 8), :]
                if r == 0:
                    return lo
                if cfg["skew2"]:
                    return pltpu.roll(lo, 8 - r, 0)
                return pltpu.roll(jnp.where(sub >= r, lo, wk[pl.ds(base + 8, 8), :]), 8 - r, 0)
            return wk[pl.ds(z + 8 * v, 8), :]

        def st(v, x):
            wk[pl.ds(z + 8 * v, 8), :] = x

        def twid(idx):
            return (tw[j, idx], tw[j, idx + 1])

        def natural(w, hh):
            return pltpu.bitcast(w, BF16).astype(F32)[8 * hh:8 * hh + 8]

        def pairs(flat):
            return [(flat[2 * e], flat[2 * e + 1]) for e in range(len(flat) // 2)]

        def fwd4(locs, t0):
            v = pairs(begin([ld(x) for loc in locs[::-1] for x in loc], cfg["a_g4"]))[::-1]
            return _dft4([v[0]] + [_cmul(v[r], twid(t0 + 2 * r)) for r in range(1, 4)], +1)

        def inv4(v, t0):
            o = _dft4(v, -1)
            return [o[0]] + [_cmulc(o[r], twid(t0 + 2 * r)) for r in range(1, 4)]

        def ld4(locs):
            return pairs(begin([ld(x) for loc in locs for x in loc], cfg["a_g4i"]))

        def put4(locs, o):
            for loc, x in zip(locs, o):
                st(loc[0], x[0])
                st(loc[1], x[1])
            merge([x for c in o for x in c])

        def put4_t(dsts, o):
            for (blk, slot), x in zip(dsts, o):
                for ri in range(2):
                    base = 8 * WS + 256 * blk + 16 * ri + slot
                    if cfg["skew2"]:
                        base += 8 * (blk % 2)
                        wk[pl.ds(base, 8 - slot, stride=33), :] = x[ri][0:8 - slot]
                        if slot:
                            wk[pl.ds(base - 8 + 33 * (8 - slot), slot, stride=33), :] = x[ri][8 - slot:8]
                    else:
                        wk[pl.ds(base, 8, stride=33), :] = x[ri]
            merge([x for c in o for x in c])

        def xloc(sig, n):
            return (WX + 256 * sig + 2 * n, WX + 256 * sig + 2 * n + 1)

        def sloc(kb, l):
            return ((2 * kb + l // 8, 0, l % 8), (2 * kb + l // 8, 1, l % 8))

        def pass_kv():
            t = [taps[g, a] for a in range(KS)]
            prev = {sh: jnp.zeros((8, 128), U32) for sh in (1, 2)}
            for v in range(S // 16):
                w0, = begin([pltpu.bitcast(abuf[sl, 1, pl.ds(16 * v, 16), :], U32)], 1)
                vw = pltpu.bitcast(abuf[sl, 2, pl.ds(16 * v, 16), :], U32)
                cur = {sh: pltpu.roll(w0, sh, 0) for sh in (1, 2)}
                w1, w2 = [jnp.where(sub < sh, prev[sh], cur[sh]) for sh in (1, 2)]
                prev = cur
                e0, o0, e1, o1, o2 = (_unpack(w0, 0), _unpack(w0, 1), _unpack(w1, 0),
                                      _unpack(w1, 1), _unpack(w2, 1))
                ke = (e0 * t[0] + o1 * t[1] + e1 * t[2] + o2 * t[3]) * _unpack(vw, 0)
                ko = (o0 * t[0] + e0 * t[1] + o1 * t[2] + e1 * t[3]) * _unpack(vw, 1)
                chain[0] = _pack(ke, ko)
                kvb[pl.ds(8 * v, 8), :] = chain[0]

        def forward(sig, src):
            for n in range(32):
                x = [natural(w, n % 2) for w in begin([src(n // 2 + 16 * d) for d in range(8)], 8)]
                cs = []
                for d in range(4):
                    a, b = twid(TAF + 2 * d), twid(TAF + 2 * (d + 4))
                    if d == 0:
                        s_ = x[4] * b[0]
                        cs.append((x[0] + s_, s_))
                    else:
                        cs.append((x[d] * a[0] + x[d + 4] * b[0], x[d] * a[1] + x[d + 4] * b[1]))
                put4([xloc(sig, n + 32 * k0) for k0 in range(4)], _dft4(cs, +1))
            for k0 in range(4):
                for n in range(8):
                    locs = [xloc(sig, n + 8 * r + 32 * k0) for r in range(4)]
                    put4(locs, fwd4(locs, TB + 8 * k0))
            for k0 in range(4):
                for k1 in range(4):
                    k = k0 + 4 * k1
                    for a in range(2):
                        o = fwd4([xloc(sig, a + 2 * r + 8 * k1 + 32 * k0) for r in range(4)], TC + 8 * k)
                        put4_t([(2 * ((k + 16 * k2) // 8) + a, k % 8) for k2 in range(4)], o)
            for kb in range(8):
                for e in range(4):
                    o = fwd4([sloc(kb, e + 4 * r) for r in range(4)], TD + 8 * kb)
                    put4([xloc(sig, 16 * kb + e + 4 * r) for r in range(4)], o)
            for kb in range(8):
                for k3 in range(4):
                    locs = [xloc(sig, 16 * kb + r + 4 * k3) for r in range(4)]
                    t0 = TE + 8 * (4 * kb + k3)
                    o = fwd4(locs, t0)
                    if sig == 0:
                        hs = ld4([xloc(1, 16 * kb + r + 4 * k3) for r in range(4)])
                        o = inv4([_cmul(a, b) for a, b in zip(o, hs)], t0)
                    put4(locs, o)

        def inverse():
            for kb in range(8):
                for e in range(4):
                    o = inv4(ld4([xloc(0, 16 * kb + e + 4 * r) for r in range(4)]), TD + 8 * kb)
                    put4_t([(2 * kb + (e + 4 * f) // 8, (e + 4 * f) % 8) for f in range(4)], o)
            for k0 in range(4):
                for k1 in range(4):
                    k = k0 + 4 * k1
                    for a in range(2):
                        v = ld4([sloc((k + 16 * r) // 8, 8 * a + k % 8) for r in range(4)])
                        put4([xloc(0, a + 2 * b + 8 * k1 + 32 * k0) for b in range(4)], inv4(v, TC + 8 * k))
            for k0 in range(4):
                for n in range(8):
                    locs = [xloc(0, n + 8 * r + 32 * k0) for r in range(4)]
                    put4(locs, inv4(ld4(locs), TB + 8 * k0))
            dskip = taps[g, KS]
            for n0 in range(32):
                cs = _dft4(ld4([xloc(0, n0 + 32 * r) for r in range(4)]), -1)
                outs = []
                for d in [d0 + 4 * hh for d0 in range(4) for hh in range(2)]:
                    n = n0 + 32 * d
                    a = twid(TAI + 2 * d)
                    if 0 < d < 4 and cfg["a_fine"]:
                        cs[d] = tuple(begin(cs[d], 2))
                    c = cs[d % 4]
                    y = c[0] * a[0] if d == 0 else c[0] * a[0] + c[1] * a[1]
                    kv = natural(kvb[pl.ds(8 * (n // 2), 8), :], n % 2)
                    y = y + jnp.where(j == 0, kv * dskip, ld(WY + n))
                    st(WY + n, y)
                    chain[0] = abuf[sl, 0, pl.ds(8 * n, 8), :].astype(F32) * y
                    aout[g, n // 4, pl.ds(8 * (n % 4), 8), :] = chain[0].astype(BF16)
                    outs.append(chain[0])
                merge(outs)

        def filt(v):
            return ht[pl.ds(pl.multiple_of(g * (S // 2), S // 2) + 8 * v, 8), :]
        if cfg["a_hfirst"]:
            forward(1, filt)
            pass_kv()
        else:
            pass_kv()
            forward(1, filt)
        forward(0, lambda v: kvb[pl.ds(8 * v, 8), :])
        inverse()
        return chain[0]

    scale = DH ** (-0.5)

    def w_slab(m, h):
        u = 4 * m + h // 8
        return pltpu.bitcast(w_parts[u % 2][pl.ds(slab_row(u, h % 2, (h // 2) % 4), D // 2), :], BF16)

    class Step:
        def __init__(self, s, prev, mem):
            self.s = s
            self.prev = prev
            self.qkv, self.ps, self.os = {}, {}, []
            self.acc = [None] * NB
            self.ocat, self.lead, self.early, self.marks = {}, {}, {}, {}
            self.tie = None
            x = xbuf[s, pl.ds(M, SEG - M), :].astype(F32)
            self.lhsf = jnp.concatenate([mem, x], axis=0)
            self.lhs = self.lhsf.astype(BF16)

        def proj_early(self, m, j, k):
            self.early[m, j] = (k, [_dot(self.lhsf[:, :k].astype(BF16), w_slab(m, 2 * j + e)[:k])
                                    for e in range(2)])

        def proj(self, m, j):
            if (m, j) in self.early:
                k, part = self.early[m, j]
                a, b = [_dot(self.lhsf[:, k:].astype(BF16), w_slab(m, 2 * j + e)[k:]) + part[e]
                        for e in range(2)]
            else:
                a = _dot(self.lhs, w_slab(m, 2 * j))
                b = _dot(self.lhs, w_slab(m, 2 * j + 1))
            self.marks[m, j] = a[0:8]
            lead = qkvb[self.s, m * NPAIR + j]
            if m == 0:
                r = jnp.concatenate([a, b, _unpack(lead, 0), _unpack(lead, 1)], axis=0).astype(BF16)
            else:
                r = pltpu.bitcast(jnp.concatenate([_pack(a, b), lead], axis=0), BF16)
            self.qkv[m, j] = r

        def probs(self, j):
            fill = fill_ref[pl.ds(0, R), pl.ds(0, R)]
            qk = _dot_nt(self.qkv[0, j], self.qkv[1, j])
            if cfg["exp2"]:
                sc = jnp.where(fill == 0.0, qk, fill)
                e = jnp.exp2((sc - jnp.max(sc, axis=-1, keepdims=True)) * (scale * LOG2E))
            else:
                sc = jnp.where(fill == 0.0, qk * scale, fill)
                e = jnp.exp(sc - jnp.max(sc, axis=-1, keepdims=True))
            l = jnp.sum(e, axis=-1, keepdims=True)
            r = pl.reciprocal(l, approx=True)
            r = r * (2.0 - l * r)
            self.ps[j] = (e * r).astype(BF16)

        def attend(self, j):
            o = _dot(self.ps[j], self.qkv[2, j])
            la, lb = o[2 * SEG:2 * SEG + M], o[2 * SEG + M:]
            rows = pl.ds(pl.multiple_of((self.s >> 1) * M, M), M)
            if self.prev is None:
                self.lead[j] = (la, lb)
                forms = {2: la + lb, 5: la}
            else:
                a11, a12 = self.prev.lead[j]
                forms = {0: a11 + lb, 1: la + lb, 3: la - a11, 4: a12 - lb, 6: lb}
            for f, v in forms.items():
                ob[f * NPAIR + j, rows, :] = v.astype(BF16)
            self.os += [o[0:SEG], o[SEG:2 * SEG]]

        def wo(self, h0, h1, n):
            if h0 not in self.ocat:
                self.ocat[h0] = jnp.concatenate(self.os[h0:h1], axis=1).astype(BF16)
            w = wo_u[n, pl.ds(h0 * 64, (h1 - h0) * 64), :]
            if self.tie is not None:
                w = jnp.concatenate(
                    [jnp.where(self.s > 1000, pltpu.bitcast(self.tie, U32), w[0:8]), w[8:]], axis=0)
                self.tie = None
            d = _dot(self.ocat[h0], pltpu.bitcast(w, BF16))
            self.acc[n] = d if self.acc[n] is None else d + self.acc[n]

        def finish(self):
            res = jnp.concatenate(self.acc, axis=1)
            obuf[self.s] = res.astype(BF16)
            return res[0:M]

    def steps(i, mem):
        sts = []
        for u in range(U):
            st = Step(i * U + u, sts[-1] if u % 2 else None, mem)
            sts.append(st)
            for item in _step_order(u, cfg):
                if item[0] == "A":
                    if cfg["a"]:
                        ku, km, kj = cfg["kick"]
                        st.tie = part_a(i, sts[ku].marks[km, kj])
                else:
                    dict(P=st.proj, E=st.proj_early, S=st.probs, V=st.attend, W=st.wo)[item[0]](*item[1:])
            mem = st.finish()
        return mem

    def group(g, mem):
        x_copy(g).wait()
        self_wait(abuf.at[g & 1], SA + (g & 1))

        @pl.when(jnp.logical_and(g >= 1, g < NG - 1))
        def _():
            a_start(g + 1)
        return loop("steps", 2 * g, 2 * g + 2, steps, mem)

    tw_cp.wait()
    lax.fori_loop(0, NG, group, mem0_ref[...].astype(F32))

    ob_cp = pltpu.make_async_copy(
        obuf.at[:, pl.ds(M, SEG - M), :],
        out_hbm.at[:, pl.ds(M, SEG - M), pl.ds(D, D)], sems.at[SO])
    ob_cp.start()
    for g in range(NG):
        pltpu.make_async_copy(
            aout.at[g], out_hbm.at[:, :, pl.ds(g * 128, 128)], sems.at[SO + 1]).start()

    def epi(it, carry):
        ns = [2 * it, 2 * it + 1]

        def blk(hp, u):
            return [wo_u[ns[u], pl.ds((2 * j + hp) * 64, 64), :] for j in range(NPAIR)]

        def mm(f, bs):
            lhs = jnp.concatenate([ob[f * NPAIR + j] for j in range(NPAIR)], axis=1)
            return _dot(lhs, pltpu.bitcast(jnp.concatenate(bs, axis=0), BF16))

        def cb(x, y, sign):
            return [comb(a, b, sign) for a, b in zip(x, y)]

        def put(u, par, c):
            for i in range(NSEG // 2):
                obb[ns[u], 2 * i + par] = c[M * i:M * i + M].astype(BF16)
        m5 = mm(2, blk(1, 1))
        m1 = mm(0, cb(blk(0, 0), blk(1, 1), 1))
        m4 = mm(6, cb(blk(1, 0), blk(0, 0), -1))
        put(0, 0, mm(4, cb(blk(1, 0), blk(1, 1), 1)) + (m1 + m4 - m5))
        m3 = mm(5, cb(blk(0, 1), blk(1, 1), -1))
        put(1, 0, m3 + m5)
        m2 = mm(1, blk(0, 0))
        put(0, 1, m2 + m4)

        def send(n):
            col = pl.multiple_of(D + n * 128, 128)
            pltpu.make_async_copy(
                obb.at[n], out_hbm.at[:, pl.ds(0, M), pl.ds(col, 128)], sems.at[SO + 2]).start()
        send(ns[0])
        put(1, 1, mm(3, cb(blk(0, 0), blk(0, 1), 1)) + (m1 - m2 + m3))
        send(ns[1])
        return carry
    loop("epi", 0, NB // 2, epi, 0)
    ob_cp.wait()
    self_wait(aout, SO + 1)
    self_wait(obb, SO + 2)


def _step_order(u, cfg):
    ks = cfg["ks"]
    tmpl = [(x[0], int(x[1:])) for x in cfg["tmpl"].split()]
    out = []
    if u > 0:
        first = [(kind, t - lag) for t in range(3) for kind, lag in tmpl if kind in "qkv" and t >= lag]
        out += [("E", "qkv".index(kind), j, cfg["ek"]) for kind, j in first[:cfg["ne"]]]
    nw = 0
    for t in range(NPAIR + max(l for _, l in tmpl)):
        for kind, lag in tmpl:
            j = t - lag
            if j < 0:
                continue
            if j >= NPAIR:
                if kind in "qkv" and nw < NB:
                    out.append(("W", 0, ks, nw))
                    nw += 1
                continue
            out.append(("P", "qkv".index(kind), j) if kind in "qkv" else (kind, j))
    out += [("W", 0, ks, n) for n in range(nw, NB)]
    for n in range(NB):
        if u == U - 1 and n == cfg["tie_n"]:
            out.append(("A",))
        out.append(("W", ks, H, n))
    return out


_DEFAULT_CFG = dict(tmpl="k0 v1 S1 q0 V2", ks=16, ne=2, ek=640, exp2=0,
                    a=1, tie_n=7, kick=(0, 1, 1), skew2=0, a_dyn=0, a_merge=5, a_pad=0, a_fine=1,
                    a_g4=8, a_g4i=4, a_hfirst=0)


def _build(cfg):
    tw_np = _twiddles()
    fill_np = np.zeros((96, 128), np.float32)
    fill_np[:R, :R] = _mask_fill() * (DH ** 0.5 if cfg["exp2"] else 1.0)

    def run(A_q, A_k, A_v, A_shift_k, A_ssm_k, A_ssm_D, B_x, B_mem0, B_Wq, B_Wk, B_Wv, B_Wo):
        sk = A_shift_k.T.reshape(KS, NG, 128).transpose(1, 0, 2)
        any_spec = pl.BlockSpec(memory_space=pl.ANY)
        out = pl.pallas_call(
            functools.partial(_kernel, cfg),
            out_shape=jax.ShapeDtypeStruct((NSEG, SEG, 2 * D), BF16),
            in_specs=[any_spec] * 14,
            out_specs=any_spec,
            scratch_shapes=[
                pltpu.VMEM((48 * SLAB + 544, 128), U32),
                pltpu.VMEM((48 * SLAB + 544, 128), U32),
                pltpu.VMEM((NB, H * DH // 2, 128), U32),
                pltpu.VMEM((4, D, 8, DH), BF16),
                pltpu.VMEM((9, 512, D), BF16),
                pltpu.VMEM((NSEG, SEG, D), BF16),
                pltpu.VMEM((4, NSEG, M, KQ), BF16),
                pltpu.VMEM((4, NSEG * M // 2, KQ), U32),
                pltpu.VMEM((5, 2, HR, KQ), U32),
                pltpu.VMEM((NSEG, 3 * NPAIR, 8, 128), U32),
                pltpu.VMEM((7 * NPAIR, NSEG * M // 2, DH), BF16),
                pltpu.VMEM((NSEG, SEG, D), BF16),
                pltpu.VMEM((NB, NSEG, M, 128), BF16),
                pltpu.VMEM((2, 3, S, 128), BF16),
                pltpu.VMEM((NG + 1, 128, S), BF16),
                pltpu.VMEM((NG * S // 2, 128), U32),
                pltpu.VMEM((S // 2, 128), U32),
                pltpu.VMEM((8 * NW + 32, 128), F32),
                pltpu.VMEM((2, NT, 8, 128), F32),
                pltpu.VMEM((NG, NSEG, SEG, 128), BF16),
                pltpu.VMEM((4, 8, 128), F32),
                pltpu.VMEM((96, 128), F32),
                pltpu.VMEM((NG, 8, 8, 128), F32),
                pltpu.VMEM((M, D), BF16),
                pltpu.VMEM((NG, KS, 128), BF16),
                pltpu.VMEM((4, NG, 128), BF16),
                pltpu.SemaphoreType.DMA((56,)),
            ],
            compiler_params=pltpu.CompilerParams(vmem_limit_bytes=124 * 1024 * 1024,
                                                 disable_bounds_checks=True),
        )(A_q.reshape(S, D), A_k.reshape(S, D), A_v.reshape(S, D), sk, A_ssm_k,
          A_ssm_D.reshape(NG, 128), B_x.reshape(NSEG, SEG, D), B_mem0.reshape(M, D),
          B_Wq, B_Wk, B_Wv, B_Wo.reshape(H * DH, D),
          jnp.asarray(tw_np), jnp.asarray(fill_np))
        return out.reshape(1, S, 2 * D)

    return run


@functools.partial(jax.jit, static_argnames=("B_seg_len",))
def pallas_concat_heads__ssm_conv_h3__memory_aug_recurrent_mem_tr__prompt_kernel(
    A_q: jax.Array,
    A_k: jax.Array,
    A_v: jax.Array,
    A_shift_k: jax.Array,
    A_ssm_k: jax.Array,
    A_ssm_D: jax.Array,
    B_x: jax.Array,
    B_mem0: jax.Array,
    B_Wq: jax.Array,
    B_Wk: jax.Array,
    B_Wv: jax.Array,
    B_Wo: jax.Array,
    B_seg_len: int = SEG,
):
    assert B_seg_len == SEG
    return _build(_DEFAULT_CFG)(A_q, A_k, A_v, A_shift_k, A_ssm_k, A_ssm_D, B_x, B_mem0,
                                B_Wq, B_Wk, B_Wv, B_Wo)
```

```python
import functools

import numpy as np
import jax
import jax.numpy as jnp
from jax import lax
import jax.experimental.pallas as pl
import jax.experimental.pallas.tpu as pltpu

F32 = jnp.float32
BF16 = jnp.bfloat16
U32 = jnp.uint32

S = 2048
D = 1024
H = 32
DH = 128
M = 8
SEG = 32
NSEG = S // SEG
U = 4
NPAIR = H // 2
R = 2 * (M + SEG)
SLAB = 520
KS = 4
NG = D // 128
KQ = D // 4
NB = D // 128
HR = NSEG * M // 4

TAF, TAI, TB, TC, TD, TE, NT = 0, 16, 32, 64, 192, 256, 512
WX, WS, WY, WK, NW = 0, 512, 1024, 1280, 1536
LOG2E = 1.4426950408889634


def _twiddles():
    tw = np.zeros((2, NT, 8), np.float64)

    def put(j, idx, z):
        tw[j, idx] = np.real(z)
        tw[j, idx + 1] = np.imag(z)
    s = np.arange(8)
    tau = 2j * np.pi
    for j in range(2):
        lx = 1j * np.pi * (1 + 4 * j) / 4096
        for d in range(8):
            put(j, TAF + 2 * d, np.exp(lx * 256 * d))
            put(j, TAI + 2 * d, np.exp(lx * 256 * d) / 2048)
        for r in range(4):
            for k in range(4):
                put(j, TB + 8 * k + 2 * r, np.exp((lx * 64 + tau * k / 16) * r))
            for k in range(16):
                put(j, TC + 8 * k + 2 * r, np.exp((lx * 16 + tau * k / 64) * r))
            for kb in range(8):
                put(j, TD + 8 * kb + 2 * r, np.exp((lx * 4 + tau * (s + 8 * kb) / 256) * r))
                for k3 in range(4):
                    put(j, TE + 8 * (4 * kb + k3) + 2 * r,
                        np.exp((lx + tau * (s + 8 * kb + 64 * k3) / 1024) * r))
    return np.ascontiguousarray(np.broadcast_to(tw[..., None], (2, NT, 8, 128))).astype(np.float32)


def _mask_fill():
    blk = np.concatenate([np.arange(M), M + np.arange(M, SEG)])
    lead = M + np.arange(M)
    head = np.concatenate([np.zeros(SEG), np.ones(SEG), np.zeros(M), np.ones(M)])
    pos = np.concatenate([blk, blk, lead, lead])
    same = head[:, None] == head[None, :]
    ok = (pos[:, None] < M) | (pos[:, None] >= pos[None, :])
    fill = np.where(same, np.where(ok, 0.0, -1e9), -np.inf)
    return fill.astype(np.float32)


def _widen(w):
    return pltpu.bitcast(w, BF16).astype(F32)


def _narrow(x):
    return pltpu.bitcast(x.astype(BF16), U32)


def _dot(a, b):
    return jnp.dot(a, b, preferred_element_type=F32)


def _dot_nt(a, b):
    return lax.dot_general(a, b, (((1,), (1,)), ((), ())), preferred_element_type=F32)


def _cadd(a, b):
    return (a[0] + b[0], a[1] + b[1])


def _csub(a, b):
    return (a[0] - b[0], a[1] - b[1])


def _cmul(a, w):
    return (a[0] * w[0] - a[1] * w[1], a[0] * w[1] + a[1] * w[0])


def _cmulc(a, w):
    return (a[0] * w[0] + a[1] * w[1], a[1] * w[0] - a[0] * w[1])


def _bfly_i(b, d, sg):
    p = (b[0] - d[1], b[1] + d[0])
    q = (b[0] + d[1], b[1] - d[0])
    return (p, q) if sg > 0 else (q, p)


def _dft4(x, sg):
    a, b = _cadd(x[0], x[2]), _csub(x[0], x[2])
    c, d = _cadd(x[1], x[3]), _csub(x[1], x[3])
    p, q = _bfly_i(b, d, sg)
    return [_cadd(a, c), p, _csub(a, c), q]


def _kernel(cfg,
            aq_hbm, ak_hbm, av_hbm, sk_hbm, ssmk_hbm, ssmd_hbm, x_hbm, mem0_hbm,
            wq_hbm, wk_hbm, wv_hbm, wo_hbm, tw_hbm, fill_hbm,
            out_hbm,
            w_a, w_b, wo_u, wstage, wostage, xbuf, xlead, xlead_u, xs_u, qkvb, ob, obuf, obb,
            abuf, hbuf, ht, wk, tw, aout, kickbuf,
            fill_ref, taps, mem0_ref, sk_ref, ssmd_ref,
            sems):
    import contextlib
    scope = jax.named_scope if cfg.get("scopes") else (lambda name: contextlib.nullcontext())
    SW, SWO, SXL, SX, SH, SA, ST, SO, SS = 0, 16, 24, 28, 36, 44, 46, 48, 52
    only = cfg.get("only")

    def loop(name, lo, hi, body, init):
        if only is not None and name not in only:
            return init
        if cfg.get("scopes") == 2:
            def body2(i, c):
                with scope(name + "_it"):
                    return body(i, c)
            return lax.fori_loop(lo, hi, body2, init)
        with scope(name):
            return lax.fori_loop(lo, hi, body, init)
    w_hbms = (wq_hbm, wk_hbm, wv_hbm)
    a_hbms = (aq_hbm, ak_hbm, av_hbm)

    def w_copy(m, hq, q=None):
        rows = pl.ds(0, D) if q is None else pl.ds(q * KQ, KQ)
        sem = SW + 8 + hq if q is None else SW + 4 * hq + q
        heads = 8 * hq if isinstance(hq, int) else pl.multiple_of(8 * hq, 8)
        return pltpu.make_async_copy(
            w_hbms[m].at[rows, pl.ds(heads, 8), :], wstage.at[hq, rows], sems.at[sem])

    def self_wait(ref, sem):
        pltpu.make_async_copy(ref, ref, sems.at[sem]).wait()

    def late_start(k):
        pltpu.make_async_copy(
            wo_hbm.at[pl.ds(pl.multiple_of(k * 512, 512), 512), :], wostage.at[k],
            sems.at[SWO + k]).start()
        pltpu.make_async_copy(
            ssmk_hbm.at[pl.ds(pl.multiple_of(k * 128, 128), 128), :], hbuf.at[k],
            sems.at[SH + k]).start()

    def xlead_copy(q):
        return pltpu.make_async_copy(
            x_hbm.at[:, pl.ds(0, M), pl.ds(q * KQ, KQ)], xlead.at[q], sems.at[SXL + q])

    def x_copy(g):
        segs = pl.ds(g * 8, 8)
        return pltpu.make_async_copy(
            x_hbm.at[segs, pl.ds(M, SEG - M), :], xbuf.at[segs, pl.ds(M, SEG - M), :], sems.at[SX + g])

    def a_start(g):
        col = g * 128 if isinstance(g, int) else pl.multiple_of(g * 128, 128)
        for t in (1, 2, 0):
            pltpu.make_async_copy(
                a_hbms[t].at[:, pl.ds(col, 128)], abuf.at[g & 1, t], sems.at[SA + (g & 1)]).start()

    tw_cp = pltpu.make_async_copy(tw_hbm, tw, sems.at[ST])

    small = [pltpu.make_async_copy(src, dst, sems.at[SS + i]) for i, (src, dst) in enumerate((
        (fill_hbm, fill_ref), (mem0_hbm, mem0_ref), (sk_hbm, sk_ref), (ssmd_hbm, ssmd_ref.at[0])))]

    for q in range(4):
        xlead_copy(q).start()
        w_copy(0, 0, q).start()
        if q > 0:
            w_copy(0, 1, q - 1).start()
    w_copy(0, 1, 3).start()
    w_copy(0, 2).start()
    w_copy(0, 3).start()
    for cp in small:
        cp.start()

    w_parts = (w_a, w_b)

    def slab_row(u, par, jl):
        return ((u >> 1) * 8 + par * 4 + jl) * SLAB

    def gated(x, i, n, gates):
        if gates is None:
            return x
        never, vals = gates
        v = vals[(i * len(vals) * 3) // (n * 4)]
        return jnp.where(never, pltpu.bitcast(v, U32), x)

    def vregs(*mats):
        return [m_[r:r + 8] for m_ in mats for r in range(0, m_.shape[0], 8)]

    def relayout(u, g, q, gates=None, src=None):
        slot, qs = (u & 3, q) if src is None else src
        low = lax.broadcasted_iota(jnp.int32, (8, 128), 0) < 4
        keep = jnp.where(low, jnp.uint32(0xFFFF), jnp.uint32(0xFFFF0000))
        shl = jnp.where(low, jnp.uint32(16), jnp.uint32(0))
        base = slab_row(u, 0, 0) + q * (KQ // 2)
        for i in range(KQ // 2):
            x = wstage[slot, pl.ds(qs * KQ + 2 * i, 2)].reshape(16, DH)
            x = gated(pltpu.bitcast(x, U32), i, KQ // 2, gates)
            y = pltpu.roll(x, 4, 0)
            w_parts[g][pl.ds(base + i, 8, stride=SLAB), :] = (x & keep) | ((y << shl) >> (16 - shl))

    def comb(x, y, sign):
        return _widen(x) + _widen(y) if sign > 0 else _widen(x) - _widen(y)

    def as_bf16(b):
        return pltpu.bitcast(b, BF16) if b.dtype == U32 else b.astype(BF16)

    def put_lead(segs, n, it, a, b):
        both = jnp.concatenate([a.reshape(n, M, DH), b.reshape(n, M, DH)], axis=1)
        qkvb[segs, it] = _narrow(both)

    def batch_pair(u, g, jl):
        it = 4 * u + jl
        rows = [pl.multiple_of(slab_row(u, par, jl), 8) for par in range(2)]

        def blk(kh, par):
            return w_parts[g][pl.ds(rows[par] + kh * (D // 4), D // 4), :]

        def mm(a, b):
            return _dot(pltpu.bitcast(jnp.concatenate(a, axis=1), BF16), as_bf16(b))

        def xs(f):
            return [xs_u[f, q] for q in range(2)]
        a11 = [xlead_u[q, pl.ds(0, HR), :] for q in (0, 1)]
        a22 = [xlead_u[q, pl.ds(HR, HR), :] for q in (2, 3)]
        m5 = mm(xs(2), blk(1, 1))
        m1 = mm(xs(0), comb(blk(0, 0), blk(1, 1), 1))
        m4 = mm(a22, comb(blk(1, 0), blk(0, 0), -1))
        c11 = mm(xs(4), comb(blk(1, 0), blk(1, 1), 1)) + (m1 + m4 - m5)
        m3 = mm(a11, comb(blk(0, 1), blk(1, 1), -1))
        put_lead(pl.ds(0, NSEG // 2), NSEG // 2, it, c11, m3 + m5)
        m2 = mm(xs(1), blk(0, 0))
        c22 = mm(xs(3), comb(blk(0, 0), blk(0, 1), 1)) + (m1 - m2 + m3)
        put_lead(pl.ds(NSEG // 2, NSEG // 2), NSEG // 2, it, m2 + m4, c22)
        return vregs(m5, m1, m4, c11, m3, m2, c22)

    def quarter_wait(u, q):
        self_wait(wstage.at[u, pl.ds(pl.multiple_of(q * KQ, KQ), KQ)], SW + 4 * u + q)

    def first_unit(q, carry):
        never = q > 1000
        half = q & 1
        self_wait(xlead.at[q], SXL + q)
        quarter_wait(0, q)
        xlead_u[q] = _narrow(xlead[q].astype(F32).reshape(NSEG * M, KQ))
        relayout(0, 0, q)

        @pl.when(q > 0)
        def _():
            quarter_wait(1, q - 1)
        res = []
        xq = pltpu.bitcast(xlead_u[q], BF16)
        for jl in range(4):
            outs = []
            for par in range(2):
                acc = pl.ds((2 * jl + par) * (NSEG * M), NSEG * M)
                row = pl.multiple_of(slab_row(0, par, jl) + q * (KQ // 2), 8)
                w = pltpu.bitcast(w_a[pl.ds(row, KQ // 2), :], BF16)
                d = _dot(xq, w) + jnp.where(q == 0, 0.0, wk[acc, :])
                wk[acc, :] = d
                outs.append(d)
            put_lead(pl.ds(0, NSEG), NSEG, jl, outs[0], outs[1])
            res += outs
        gates = (never, vregs(*res))
        qn = jnp.maximum(q - 1, 0)
        relayout(1, 1, qn, gates, src=(jnp.minimum(q, 1), qn))
        for r in range(0, HR, 8):
            for cb in range(2):
                cols = pl.ds(cb * 128, 128)
                i = 2 * (r // 8) + cb
                a11 = gated(xlead_u[half, pl.ds(r, 8), cols], i, HR // 4, gates)
                a22 = gated(xlead_u[2 + half, pl.ds(HR + r, 8), cols], i, HR // 4, gates)
                a21 = xlead_u[half, pl.ds(HR + r, 8), cols]
                a12 = xlead_u[2 + half, pl.ds(r, 8), cols]
                for f, (x, y, sg) in enumerate(((a11, a22, 1), (a21, a22, 1), (a11, a12, 1),
                                                (a21, a11, -1), (a12, a22, -1))):
                    xs_u[f, half, pl.ds(r, 8), cols] = _narrow(comb(x, y, sg))
        return carry
    loop("units", 0, 4, first_unit, 0)
    w_copy(0, 1, 3).wait()
    relayout(1, 1, 3)

    def late_relayout(src, hp, half, gates):
        for r in range(16):
            blk = pltpu.bitcast(wostage[src, pl.ds(half * 256 + r * 16, 16), :], U32)
            row = pl.multiple_of(hp * 128 + r * 8, 8)
            for n in range(NB):
                wo_u[n, pl.ds(row, 8), :] = gated(blk[:, n * 128:(n + 1) * 128], r * NB + n, 16 * NB, gates)
        for t in range(8):
            tile = pltpu.bitcast(hbuf[src, :, pl.ds((8 * half + t) * 128, 128)], U32)
            tile = jnp.concatenate([gated(tile[0:8], t, 8, gates), tile[8:]], axis=0)
            row = pl.multiple_of(hp * 512 + t * 64, 64)
            ht[pl.ds(row, 64), :] = pltpu.bitcast(pltpu.bitcast(tile, BF16).T, U32)

    def unit_body(u, g):
        @pl.when(jnp.logical_and(u > 1, u < 11))
        def _():
            self_wait(wstage.at[(u + 1) & 3], SW + 8 + ((u + 1) & 3))

        @pl.when(u >= 8)
        def _():
            for e in range(2):
                k = (u - 8) * 2 + e
                self_wait(wostage.at[k], SWO + k)
                self_wait(hbuf.at[k], SH + k)
        for m in (1, 2):
            @pl.when((u + 3) >> 2 == m)
            def _():
                w_copy(m, (u + 3) & 3).start()

        @pl.when(u <= 8)
        def _():
            late_start(u - 1)
        if g == 1:
            @pl.when(u == 9)
            def _():
                x_copy(0).start()
                a_start(0)
                tw_cp.start()
        if only is None or "chunk" in only:
            for jl in range(4):
                gates = (u > 1000, batch_pair(u, g, jl))
                un = jnp.where(u < 11, u + 1, u - 1)
                relayout(un, 1 - g, jl, gates, src=(jnp.where(u == 1, 1, un & 3), jl))
                k = jnp.maximum(u - 8, 0) * 2 + jl // 2
                late_relayout(jnp.where(u >= 8, k, 8), 2 * k + jl % 2, jl % 2, gates)

    def unit_pair(mm, carry):
        with scope("unit"):
            unit_body(2 * mm + 1, 1)

        @pl.when(mm == 0)
        def _():
            w_copy(0, 2).wait()

            def body(q, c):
                relayout(2, 0, q)
                return c
            lax.fori_loop(0, 4, body, 0)

        @pl.when(mm < 5)
        def _():
            with scope("unit"):
                unit_body(2 * mm + 2, 0)
        return carry
    lax.fori_loop(0, 6, unit_pair, 0)

    a_start(1)
    for g in range(1, NG):
        x_copy(g).start()
    for cp in small:
        cp.wait()
    dd = ssmd_ref[0].astype(F32)
    for g in range(NG):
        sk = sk_ref[g].astype(F32)
        for j in range(KS):
            taps[g, j] = jnp.broadcast_to(sk[j:j + 1], (8, 128))
        taps[g, KS] = jnp.broadcast_to(dd[g:g + 1], (8, 128))

    def part_a(i, kick):
        g, j = i >> 1, i & 1
        sl = g & 1
        never = i > 1000
        z = pl.multiple_of(jnp.where(never, 32, 0), 32) if cfg["a_dyn"] else 0
        sub = lax.broadcasted_iota(jnp.int32, (8, 128), 0)
        kickbuf[jnp.where(never, 1, 0)] = kick
        chain = [kickbuf[jnp.where(i > 2000, 0, 1)]]

        def begin(xs, ng):
            xs = list(xs)
            for e in range(min(ng, len(xs))):
                c = chain[0]
                c = c if c.dtype == xs[e].dtype else pltpu.bitcast(c, xs[e].dtype)
                xs[e] = jnp.where(never, c, xs[e])
            return xs

        def merge(vals):
            c = vals[-1]
            for v in list(vals[:-1])[:cfg["a_merge"]] + list(vals[:cfg["a_pad"]]):
                c = jnp.maximum(v, c)
            chain[0] = c

        def ld(v):
            if isinstance(v, tuple):
                blk, ri, r = v
                base = 8 * WS + 256 * blk + 16 * ri + 32 * r
                if cfg["skew2"]:
                    base += 8 * (blk % 2)
                lo = wk[pl.ds(base, 8), :]
                if r == 0:
                    return lo
                if cfg["skew2"]:
                    return pltpu.roll(lo, 8 - r, 0)
                return pltpu.roll(jnp.where(sub >= r, lo, wk[pl.ds(base + 8, 8), :]), 8 - r, 0)
            return wk[pl.ds(z + 8 * v, 8), :]

        def st(v, x):
            wk[pl.ds(z + 8 * v, 8), :] = x

        def twid(idx):
            return (tw[j, idx], tw[j, idx + 1])

        def pairs(flat):
            return [(flat[2 * e], flat[2 * e + 1]) for e in range(len(flat) // 2)]

        def fwd4(locs, t0):
            v = pairs(begin([ld(x) for loc in locs[::-1] for x in loc], cfg["a_g4"]))[::-1]
            return _dft4([v[0]] + [_cmul(v[r], twid(t0 + 2 * r)) for r in range(1, 4)], +1)

        def inv4(v, t0):
            o = _dft4(v, -1)
            return [o[0]] + [_cmulc(o[r], twid(t0 + 2 * r)) for r in range(1, 4)]

        def ld4(locs):
            return pairs(begin([ld(x) for loc in locs for x in loc], cfg["a_g4i"]))

        def put4(locs, o):
            for loc, x in zip(locs, o):
                st(loc[0], x[0])
                st(loc[1], x[1])
            merge([x for c in o for x in c])

        def put4_t(dsts, o):
            for (blk, slot), x in zip(dsts, o):
                for ri in range(2):
                    base = 8 * WS + 256 * blk + 16 * ri + slot
                    if cfg["skew2"]:
                        base += 8 * (blk % 2)
                        wk[pl.ds(base, 8 - slot, stride=33), :] = x[ri][0:8 - slot]
                        if slot:
                            wk[pl.ds(base - 8 + 33 * (8 - slot), slot, stride=33), :] = x[ri][8 - slot:8]
                    else:
                        wk[pl.ds(base, 8, stride=33), :] = x[ri]
            merge([x for c in o for x in c])

        def xloc(sig, n):
            return (WX + 256 * sig + 2 * n, WX + 256 * sig + 2 * n + 1)

        def sloc(kb, l):
            return ((2 * kb + l // 8, 0, l % 8), (2 * kb + l // 8, 1, l % 8))

        def pass_kv():
            t = [taps[g, a] for a in range(KS)]
            prev = [None] + [jnp.zeros((8, 128), F32)] * (KS - 1)
            for v in range(S // 16):
                w, = begin([pltpu.bitcast(abuf[sl, 1, pl.ds(16 * v, 16), :], U32)], 1)
                k2 = _widen(w)
                v2 = abuf[sl, 2, pl.ds(16 * v, 16), :].astype(F32)
                outs = []
                for hh in range(2):
                    x = k2[8 * hh:8 * hh + 8]
                    cur = [None] + [pltpu.roll(x, a, 0) for a in range(1, KS)]
                    ks = x * t[0]
                    for a in range(1, KS):
                        ks = ks + jnp.where(sub < a, prev[a], cur[a]) * t[a]
                    prev = cur
                    kv = (ks * v2[8 * hh:8 * hh + 8]).astype(BF16).astype(F32)
                    st(WK + 2 * v + hh, kv)
                    outs.append(kv)
                merge(outs)

        def forward(sig, src):
            for n in range(32):
                x = src(n)
                cs = []
                for d in range(4):
                    a, b = twid(TAF + 2 * d), twid(TAF + 2 * (d + 4))
                    if d == 0:
                        s_ = x[4] * b[0]
                        cs.append((x[0] + s_, s_))
                    else:
                        cs.append((x[d] * a[0] + x[d + 4] * b[0], x[d] * a[1] + x[d + 4] * b[1]))
                put4([xloc(sig, n + 32 * k0) for k0 in range(4)], _dft4(cs, +1))
            for k0 in range(4):
                for n in range(8):
                    locs = [xloc(sig, n + 8 * r + 32 * k0) for r in range(4)]
                    put4(locs, fwd4(locs, TB + 8 * k0))
            for k0 in range(4):
                for k1 in range(4):
                    k = k0 + 4 * k1
                    for a in range(2):
                        o = fwd4([xloc(sig, a + 2 * r + 8 * k1 + 32 * k0) for r in range(4)], TC + 8 * k)
                        put4_t([(2 * ((k + 16 * k2) // 8) + a, k % 8) for k2 in range(4)], o)
            for kb in range(8):
                for e in range(4):
                    o = fwd4([sloc(kb, e + 4 * r) for r in range(4)], TD + 8 * kb)
                    put4([xloc(sig, 16 * kb + e + 4 * r) for r in range(4)], o)
            for kb in range(8):
                for k3 in range(4):
                    locs = [xloc(sig, 16 * kb + r + 4 * k3) for r in range(4)]
                    t0 = TE + 8 * (4 * kb + k3)
                    o = fwd4(locs, t0)
                    if sig == 0:
                        hs = ld4([xloc(1, 16 * kb + r + 4 * k3) for r in range(4)])
                        o = inv4([_cmul(a, b) for a, b in zip(o, hs)], t0)
                    put4(locs, o)

        def inverse():
            for kb in range(8):
                for e in range(4):
                    o = inv4(ld4([xloc(0, 16 * kb + e + 4 * r) for r in range(4)]), TD + 8 * kb)
                    put4_t([(2 * kb + (e + 4 * f) // 8, (e + 4 * f) % 8) for f in range(4)], o)
            for k0 in range(4):
                for k1 in range(4):
                    k = k0 + 4 * k1
                    for a in range(2):
                        v = ld4([sloc((k + 16 * r) // 8, 8 * a + k % 8) for r in range(4)])
                        put4([xloc(0, a + 2 * b + 8 * k1 + 32 * k0) for b in range(4)], inv4(v, TC + 8 * k))
            for k0 in range(4):
                for n in range(8):
                    locs = [xloc(0, n + 8 * r + 32 * k0) for r in range(4)]
                    put4(locs, inv4(ld4(locs), TB + 8 * k0))
            dskip = taps[g, KS]
            for n0 in range(32):
                cs = _dft4(ld4([xloc(0, n0 + 32 * r) for r in range(4)]), -1)
                outs = []
                for d in [d0 + 4 * hh for d0 in range(4) for hh in range(2)]:
                    n = n0 + 32 * d
                    a = twid(TAI + 2 * d)
                    if 0 < d < 4 and cfg["a_fine"]:
                        cs[d] = tuple(begin(cs[d], 2))
                    c = cs[d % 4]
                    y = c[0] * a[0] if d == 0 else c[0] * a[0] + c[1] * a[1]
                    y = y + jnp.where(j == 0, ld(WK + n) * dskip, ld(WY + n))
                    st(WY + n, y)
                    chain[0] = abuf[sl, 0, pl.ds(8 * n, 8), :].astype(F32) * y
                    aout[g, n // 4, pl.ds(8 * (n % 4), 8), :] = chain[0].astype(BF16)
                    outs.append(chain[0])
                merge(outs)

        def filt(n):
            base = pl.multiple_of(g * (S // 2), S // 2)
            ws = begin([ht[pl.ds(base + 8 * (n // 2 + 16 * d), 8), :] for d in range(8)], 8)
            return [_widen(w)[8 * (n % 2):8 * (n % 2) + 8] for w in ws]
        pass_kv()
        forward(1, filt)
        forward(0, lambda n: begin([ld(WK + n + 32 * d) for d in range(8)], 8))
        inverse()
        return chain[0]

    scale = DH ** (-0.5)

    def w_slab(m, h):
        u = 4 * m + h // 8
        return pltpu.bitcast(w_parts[u % 2][pl.ds(slab_row(u, h % 2, (h // 2) % 4), D // 2), :], BF16)

    class Step:
        def __init__(self, s, prev, mem):
            self.s = s
            self.prev = prev
            self.qkv, self.ps, self.os = {}, {}, []
            self.acc = [None] * NB
            self.ocat, self.lead, self.early, self.marks, self.heads = {}, {}, {}, {}, {}
            self.tie = None
            x = xbuf[s, pl.ds(M, SEG - M), :].astype(F32)
            self.lhsf = jnp.concatenate([mem, x], axis=0)
            self.lhs = self.lhsf.astype(BF16)

        def proj_early(self, m, h, k):
            self.early[m, h] = (k, _dot(self.lhsf[:, :k].astype(BF16), w_slab(m, h)[:k]))

        def proj(self, m, h):
            if (m, h) in self.early:
                k, part = self.early[m, h]
                d = _dot(self.lhsf[:, k:].astype(BF16), w_slab(m, h)[k:]) + part
            else:
                d = _dot(self.lhs, w_slab(m, h))
            self.heads[m, h] = d
            j = h // 2
            if (m, h ^ 1) not in self.heads:
                return
            a, b = self.heads[m, 2 * j], self.heads[m, 2 * j + 1]
            self.marks[m, j] = a[0:8]
            lead = _widen(qkvb[self.s, m * NPAIR + j])
            self.qkv[m, j] = jnp.concatenate([a, b, lead], axis=0).astype(BF16)

        def probs(self, j):
            fill = fill_ref[pl.ds(0, R), pl.ds(0, R)]
            qk = _dot_nt(self.qkv[0, j], self.qkv[1, j])
            if cfg["exp2"]:
                sc = jnp.where(fill == 0.0, qk, fill)
                e = jnp.exp2((sc - jnp.max(sc, axis=-1, keepdims=True)) * (scale * LOG2E))
            else:
                sc = jnp.where(fill == 0.0, qk * scale, fill)
                e = jnp.exp(sc - jnp.max(sc, axis=-1, keepdims=True))
            l = jnp.sum(e, axis=-1, keepdims=True)
            r = pl.reciprocal(l, approx=True)
            r = r * (2.0 - l * r)
            self.ps[j] = (e * r).astype(BF16)

        def attend(self, j):
            o = _dot(self.ps[j], self.qkv[2, j])
            la, lb = o[2 * SEG:2 * SEG + M], o[2 * SEG + M:]
            rows = pl.ds(pl.multiple_of((self.s >> 1) * M, M), M)
            if self.prev is None:
                self.lead[j] = (la, lb)
                forms = {2: la + lb, 5: la}
            else:
                a11, a12 = self.prev.lead[j]
                forms = {0: a11 + lb, 1: la + lb, 3: la - a11, 4: a12 - lb, 6: lb}
            for f, v in forms.items():
                ob[f * NPAIR + j, rows, :] = v.astype(BF16)
            self.os += [o[0:SEG], o[SEG:2 * SEG]]

        def wo(self, h0, h1, n):
            if h0 not in self.ocat:
                self.ocat[h0] = jnp.concatenate(self.os[h0:h1], axis=1).astype(BF16)
            w = wo_u[n, pl.ds(h0 * 64, (h1 - h0) * 64), :]
            if self.tie is not None:
                w = jnp.concatenate(
                    [jnp.where(self.s > 1000, pltpu.bitcast(self.tie, U32), w[0:8]), w[8:]], axis=0)
                self.tie = None
            d = _dot(self.ocat[h0], pltpu.bitcast(w, BF16))
            self.acc[n] = d if self.acc[n] is None else d + self.acc[n]

        def finish(self):
            res = jnp.concatenate(self.acc, axis=1)
            obuf[self.s] = res.astype(BF16)
            return res[0:M]

    def steps(i, mem):
        sts = []
        for u in range(U):
            st = Step(i * U + u, sts[-1] if u % 2 else None, mem)
            sts.append(st)
            for item in _step_order(u, cfg):
                if item[0] == "A":
                    if cfg["a"]:
                        ku, km, kj = cfg["kick"]
                        st.tie = part_a(i, sts[ku].marks[km, kj])
                else:
                    dict(P=st.proj, E=st.proj_early, S=st.probs, V=st.attend, W=st.wo)[item[0]](*item[1:])
            mem = st.finish()
        return mem

    def group(g, mem):
        x_copy(g).wait()
        self_wait(abuf.at[g & 1], SA + (g & 1))

        @pl.when(jnp.logical_and(g >= 1, g < NG - 1))
        def _():
            a_start(g + 1)
        return loop("steps", 0, 2, lambda j, m_: steps(2 * g + j, m_), mem)

    tw_cp.wait()
    lax.fori_loop(0, NG, group, mem0_ref[...].astype(F32))

    ob_cp = pltpu.make_async_copy(
        obuf.at[:, pl.ds(M, SEG - M), :],
        out_hbm.at[:, pl.ds(M, SEG - M), pl.ds(D, D)], sems.at[SO])
    ob_cp.start()
    for g in range(NG):
        pltpu.make_async_copy(
            aout.at[g], out_hbm.at[:, :, pl.ds(g * 128, 128)], sems.at[SO + 1]).start()

    def epi(it, carry):
        ns = [2 * it, 2 * it + 1]

        def blk(hp, u):
            return [wo_u[ns[u], pl.ds((2 * j + hp) * 64, 64), :] for j in range(NPAIR)]

        def mm(f, bs):
            lhs = jnp.concatenate([ob[f * NPAIR + j] for j in range(NPAIR)], axis=1)
            return _dot(lhs, as_bf16(jnp.concatenate(bs, axis=0)))

        def cb(x, y, sign):
            return [comb(a, b, sign) for a, b in zip(x, y)]

        def put(u, par, c):
            for i in range(NSEG // 2):
                obb[ns[u], 2 * i + par] = c[M * i:M * i + M].astype(BF16)
        m5 = mm(2, blk(1, 1))
        m1 = mm(0, cb(blk(0, 0), blk(1, 1), 1))
        m4 = mm(6, cb(blk(1, 0), blk(0, 0), -1))
        put(0, 0, mm(4, cb(blk(1, 0), blk(1, 1), 1)) + (m1 + m4 - m5))
        m3 = mm(5, cb(blk(0, 1), blk(1, 1), -1))
        put(1, 0, m3 + m5)
        m2 = mm(1, blk(0, 0))
        put(0, 1, m2 + m4)

        def send(n):
            col = pl.multiple_of(D + n * 128, 128)
            pltpu.make_async_copy(
                obb.at[n], out_hbm.at[:, pl.ds(0, M), pl.ds(col, 128)], sems.at[SO + 2]).start()
        send(ns[0])
        put(1, 1, mm(3, cb(blk(0, 0), blk(0, 1), 1)) + (m1 - m2 + m3))
        send(ns[1])
        return carry
    loop("epi", 0, NB // 2, epi, 0)
    ob_cp.wait()
    self_wait(aout, SO + 1)
    self_wait(obb, SO + 2)


def _step_order(u, cfg):
    ks = cfg["ks"]
    per = cfg["period"]
    tmpl = []
    for x in cfg["tmpl"].split():
        kind, lag = x[:-1], int(x[-1])
        tmpl += [(kind + "a", lag), (kind + "b", lag)] if kind in ("q", "k", "v") else [(kind, lag)]

    def proj(kind, j):
        return ("qkv".index(kind[0]), 2 * j + "ab".index(kind[1]))
    out = []
    nw = 0
    for t in range(per - 1, NPAIR + per + max(l for _, l in tmpl), per):
        for kind, lag in tmpl:
            j = t - lag
            if j < 0:
                continue
            if j >= NPAIR:
                if kind[1:] == "a" and nw < NB:
                    out.append(("W", 0, ks, nw))
                    nw += 1
                continue
            out.append(("P",) + proj(kind, j) if len(kind) == 2 else (kind, j))
    if u > 0:
        first = [x[1:] for x in out if x[0] == "P"][:cfg["ne"]]
        out = [("E",) + x + (cfg["ek"],) for x in first] + out
    out += [("W", 0, ks, n) for n in range(nw, NB)]
    for n in range(NB):
        if u == U - 1 and n == cfg["tie_n"]:
            out.append(("A",))
        out.append(("W", ks, H, n))
    return out


_DEFAULT_CFG = dict(tmpl="V3 k0 v1 S1 q0", ks=24, ne=3, ek=640, period=1, exp2=0,
                    a=1, tie_n=7, kick=(0, 1, 1), skew2=0, a_dyn=0, a_merge=5, a_pad=0, a_fine=1,
                    a_g4=8, a_g4i=4)


def _build(cfg):
    tw_np = _twiddles()
    fill_np = np.zeros((96, 128), np.float32)
    fill_np[:R, :R] = _mask_fill() * (DH ** 0.5 if cfg["exp2"] else 1.0)

    def run(A_q, A_k, A_v, A_shift_k, A_ssm_k, A_ssm_D, B_x, B_mem0, B_Wq, B_Wk, B_Wv, B_Wo):
        sk = A_shift_k.T.reshape(KS, NG, 128).transpose(1, 0, 2)
        any_spec = pl.BlockSpec(memory_space=pl.ANY)
        out = pl.pallas_call(
            functools.partial(_kernel, cfg),
            out_shape=jax.ShapeDtypeStruct((NSEG, SEG, 2 * D), BF16),
            in_specs=[any_spec] * 14,
            out_specs=any_spec,
            scratch_shapes=[
                pltpu.VMEM((48 * SLAB + 544, 128), U32),
                pltpu.VMEM((48 * SLAB + 544, 128), U32),
                pltpu.VMEM((NB, H * DH // 2, 128), U32),
                pltpu.VMEM((4, D, 8, DH), BF16),
                pltpu.VMEM((9, 512, D), BF16),
                pltpu.VMEM((NSEG, SEG, D), BF16),
                pltpu.VMEM((4, NSEG, M, KQ), BF16),
                pltpu.VMEM((4, NSEG * M // 2, KQ), U32),
                pltpu.VMEM((5, 2, HR, KQ), U32),
                pltpu.VMEM((NSEG, 3 * NPAIR, 8, 128), U32),
                pltpu.VMEM((7 * NPAIR, NSEG * M // 2, DH), BF16),
                pltpu.VMEM((NSEG, SEG, D), BF16),
                pltpu.VMEM((NB, NSEG, M, 128), BF16),
                pltpu.VMEM((2, 3, S, 128), BF16),
                pltpu.VMEM((NG + 1, 128, S), BF16),
                pltpu.VMEM((NG * S // 2, 128), U32),
                pltpu.VMEM((8 * NW + 32, 128), F32),
                pltpu.VMEM((2, NT, 8, 128), F32),
                pltpu.VMEM((NG, NSEG, SEG, 128), BF16),
                pltpu.VMEM((4, 8, 128), F32),
                pltpu.VMEM((96, 128), F32),
                pltpu.VMEM((NG, 8, 8, 128), F32),
                pltpu.VMEM((M, D), BF16),
                pltpu.VMEM((NG, KS, 128), BF16),
                pltpu.VMEM((4, NG, 128), BF16),
                pltpu.SemaphoreType.DMA((56,)),
            ],
            compiler_params=pltpu.CompilerParams(vmem_limit_bytes=124 * 1024 * 1024,
                                                 disable_bounds_checks=True),
        )(A_q.reshape(S, D), A_k.reshape(S, D), A_v.reshape(S, D), sk, A_ssm_k,
          A_ssm_D.reshape(NG, 128), B_x.reshape(NSEG, SEG, D), B_mem0.reshape(M, D),
          B_Wq, B_Wk, B_Wv, B_Wo.reshape(H * DH, D),
          jnp.asarray(tw_np), jnp.asarray(fill_np))
        return out.reshape(1, S, 2 * D)

    return run


@functools.partial(jax.jit, static_argnames=("B_seg_len",))
def pallas_concat_heads__ssm_conv_h3__memory_aug_recurrent_mem_tr__prompt_kernel(
    A_q: jax.Array,
    A_k: jax.Array,
    A_v: jax.Array,
    A_shift_k: jax.Array,
    A_ssm_k: jax.Array,
    A_ssm_D: jax.Array,
    B_x: jax.Array,
    B_mem0: jax.Array,
    B_Wq: jax.Array,
    B_Wk: jax.Array,
    B_Wv: jax.Array,
    B_Wo: jax.Array,
    B_seg_len: int = SEG,
):
    assert B_seg_len == SEG
    return _build(_DEFAULT_CFG)(A_q, A_k, A_v, A_shift_k, A_ssm_k, A_ssm_D, B_x, B_mem0,
                                B_Wq, B_Wk, B_Wv, B_Wo)
```

```python
import functools

import numpy as np
import jax
import jax.numpy as jnp
from jax import lax
import jax.experimental.pallas as pl
import jax.experimental.pallas.tpu as pltpu

F32 = jnp.float32
BF16 = jnp.bfloat16
U32 = jnp.uint32

S = 2048
D = 1024
H = 32
DH = 128
M = 8
SEG = 32
NSEG = S // SEG
U = 4
NPAIR = H // 2
R = 2 * (M + SEG)
SLAB = 520
KS = 4
NG = D // 128
KQ = D // 4
NB = D // 128
HR = NSEG * M // 4

TAF, TAI, TB, TC, TD, TE, NT = 0, 16, 32, 64, 192, 256, 512
WX, WS, WY, WK, NW = 0, 512, 1024, 1280, 1536
LOG2E = 1.4426950408889634


def _twiddles():
    tw = np.zeros((2, NT, 8), np.float64)

    def put(j, idx, z):
        tw[j, idx] = np.real(z)
        tw[j, idx + 1] = np.imag(z)
    s = np.arange(8)
    tau = 2j * np.pi
    for j in range(2):
        lx = 1j * np.pi * (1 + 4 * j) / 4096
        for d in range(8):
            put(j, TAF + 2 * d, np.exp(lx * 256 * d))
            put(j, TAI + 2 * d, np.exp(lx * 256 * d) / 2048)
        for r in range(4):
            for k in range(4):
                put(j, TB + 8 * k + 2 * r, np.exp((lx * 64 + tau * k / 16) * r))
            for k in range(16):
                put(j, TC + 8 * k + 2 * r, np.exp((lx * 16 + tau * k / 64) * r))
            for kb in range(8):
                put(j, TD + 8 * kb + 2 * r, np.exp((lx * 4 + tau * (s + 8 * kb) / 256) * r))
                for k3 in range(4):
                    put(j, TE + 8 * (4 * kb + k3) + 2 * r,
                        np.exp((lx + tau * (s + 8 * kb + 64 * k3) / 1024) * r))
    return np.ascontiguousarray(np.broadcast_to(tw[..., None], (2, NT, 8, 128))).astype(np.float32)


def _mask_fill():
    blk = np.concatenate([np.arange(M), M + np.arange(M, SEG)])
    lead = M + np.arange(M)
    head = np.concatenate([np.zeros(SEG), np.ones(SEG), np.zeros(M), np.ones(M)])
    pos = np.concatenate([blk, blk, lead, lead])
    same = head[:, None] == head[None, :]
    ok = (pos[:, None] < M) | (pos[:, None] >= pos[None, :])
    fill = np.where(same, np.where(ok, 0.0, -1e9), -np.inf)
    return fill.astype(np.float32)


def _widen(w):
    return pltpu.bitcast(w, BF16).astype(F32)


def _narrow(x):
    return pltpu.bitcast(x.astype(BF16), U32)


def _dot(a, b):
    return jnp.dot(a, b, preferred_element_type=F32)


def _dot_nt(a, b):
    return lax.dot_general(a, b, (((1,), (1,)), ((), ())), preferred_element_type=F32)


def _cadd(a, b):
    return (a[0] + b[0], a[1] + b[1])


def _csub(a, b):
    return (a[0] - b[0], a[1] - b[1])


def _cmul(a, w):
    return (a[0] * w[0] - a[1] * w[1], a[0] * w[1] + a[1] * w[0])


def _cmulc(a, w):
    return (a[0] * w[0] + a[1] * w[1], a[1] * w[0] - a[0] * w[1])


def _bfly_i(b, d, sg):
    p = (b[0] - d[1], b[1] + d[0])
    q = (b[0] + d[1], b[1] - d[0])
    return (p, q) if sg > 0 else (q, p)


def _dft4(x, sg):
    a, b = _cadd(x[0], x[2]), _csub(x[0], x[2])
    c, d = _cadd(x[1], x[3]), _csub(x[1], x[3])
    p, q = _bfly_i(b, d, sg)
    return [_cadd(a, c), p, _csub(a, c), q]


def _kernel(cfg,
            aq_hbm, ak_hbm, av_hbm, sk_hbm, ssmk_hbm, ssmd_hbm, x_hbm, mem0_hbm,
            wq_hbm, wk_hbm, wv_hbm, wo_hbm, tw_hbm, fill_hbm,
            out_hbm,
            w_a, w_b, wo_u, wstage, wostage, xbuf, xlead, xlead_u, xs_u, qkvb, ob, obuf, obb,
            abuf, hbuf, ht, wk, tw, aout, kickbuf,
            fill_ref, taps, mem0_ref, sk_ref, ssmd_ref,
            sems):
    import contextlib
    scope = jax.named_scope if cfg.get("scopes") else (lambda name: contextlib.nullcontext())
    SW, SWO, SXL, SX, SH, SA, ST, SO, SS = 0, 16, 24, 28, 36, 44, 46, 48, 52
    only = cfg.get("only")

    def loop(name, lo, hi, body, init):
        if only is not None and name not in only:
            return init
        if cfg.get("scopes") == 2:
            def body2(i, c):
                with scope(name + "_it"):
                    return body(i, c)
            return lax.fori_loop(lo, hi, body2, init)
        with scope(name):
            return lax.fori_loop(lo, hi, body, init)
    w_hbms = (wq_hbm, wk_hbm, wv_hbm)
    a_hbms = (aq_hbm, ak_hbm, av_hbm)

    def aligned(x, n):
        return x if isinstance(x, int) else pl.multiple_of(x, n)

    def w_copy(m, hq, q=None):
        rows = pl.ds(0, D) if q is None else pl.ds(q * KQ, KQ)
        sem = SW + 12 + hq if q is None else SW + 4 * hq + q
        heads = aligned(8 * hq, 8)
        return pltpu.make_async_copy(
            w_hbms[m].at[rows, pl.ds(heads, 8), :], wstage.at[hq, rows], sems.at[sem])

    def self_wait(ref, sem):
        pltpu.make_async_copy(ref, ref, sems.at[sem]).wait()

    def late_start(k):
        pltpu.make_async_copy(
            wo_hbm.at[pl.ds(aligned(k * 512, 512), 512), :], wostage.at[k],
            sems.at[SWO + k]).start()
        pltpu.make_async_copy(
            ssmk_hbm.at[pl.ds(aligned(k * 128, 128), 128), :], hbuf.at[k],
            sems.at[SH + k]).start()

    def xlead_copy(q):
        return pltpu.make_async_copy(
            x_hbm.at[:, pl.ds(0, M), pl.ds(q * KQ, KQ)], xlead.at[q], sems.at[SXL + q])

    def x_copy(g):
        segs = pl.ds(g * 8, 8)
        return pltpu.make_async_copy(
            x_hbm.at[segs, pl.ds(M, SEG - M), :], xbuf.at[segs, pl.ds(M, SEG - M), :], sems.at[SX + g])

    def a_start(g):
        col = aligned(g * 128, 128)
        for t in (1, 2, 0):
            pltpu.make_async_copy(
                a_hbms[t].at[:, pl.ds(col, 128)], abuf.at[g & 1, t], sems.at[SA + (g & 1)]).start()

    tw_cp = pltpu.make_async_copy(tw_hbm, tw, sems.at[ST])

    small = [pltpu.make_async_copy(src, dst, sems.at[SS + i]) for i, (src, dst) in enumerate((
        (fill_hbm, fill_ref), (mem0_hbm, mem0_ref), (sk_hbm, sk_ref), (ssmd_hbm, ssmd_ref.at[0])))]

    for q in range(4):
        xlead_copy(q).start()
        w_copy(0, 0, q).start()
        if q > 0:
            w_copy(0, 1, q - 1).start()
    w_copy(0, 1, 3).start()
    for q in range(4):
        w_copy(0, 2, q).start()
    w_copy(0, 3).start()
    for cp in small:
        cp.start()

    w_parts = (w_a, w_b)

    def slab_row(u, par, jl):
        return ((u >> 1) * 8 + par * 4 + jl) * SLAB

    def gated(x, i, n, gates):
        if gates is None:
            return x
        never, vals = gates
        v = vals[(i * len(vals) * 3) // (n * 4)]
        return jnp.where(never, pltpu.bitcast(v, U32), x)

    def vregs(*mats):
        return [m_[r:r + 8] for m_ in mats for r in range(0, m_.shape[0], 8)]

    def relayout(u, g, q, gates=None, src=None):
        slot, qs = (u & 3, q) if src is None else src
        low = lax.broadcasted_iota(jnp.int32, (8, 128), 0) < 4
        keep = jnp.where(low, jnp.uint32(0xFFFF), jnp.uint32(0xFFFF0000))
        shl = jnp.where(low, jnp.uint32(16), jnp.uint32(0))
        base = slab_row(u, 0, 0) + q * (KQ // 2)
        for i in range(KQ // 2):
            x = wstage[slot, pl.ds(qs * KQ + 2 * i, 2)].reshape(16, DH)
            x = gated(pltpu.bitcast(x, U32), i, KQ // 2, gates)
            y = pltpu.roll(x, 4, 0)
            w_parts[g][pl.ds(base + i, 8, stride=SLAB), :] = (x & keep) | ((y << shl) >> (16 - shl))

    def comb(x, y, sign):
        return _widen(x) + _widen(y) if sign > 0 else _widen(x) - _widen(y)

    def as_bf16(b):
        return pltpu.bitcast(b, BF16) if b.dtype == U32 else b.astype(BF16)

    def put_lead(segs, n, it, a, b):
        both = jnp.concatenate([a.reshape(n, M, DH), b.reshape(n, M, DH)], axis=1)
        qkvb[segs, it] = _narrow(both)

    def batch_pair(u, g, jl):
        it = 4 * u + jl
        rows = [pl.multiple_of(slab_row(u, par, jl), 8) for par in range(2)]

        def blk(kh, par):
            return w_parts[g][pl.ds(rows[par] + kh * (D // 4), D // 4), :]

        def mm(a, b):
            return _dot(pltpu.bitcast(jnp.concatenate(a, axis=1), BF16), as_bf16(b))

        def xs(f):
            return [xs_u[f, q] for q in range(2)]
        a11 = [xlead_u[q, pl.ds(0, HR), :] for q in (0, 1)]
        a22 = [xlead_u[q, pl.ds(HR, HR), :] for q in (2, 3)]
        m5 = mm(xs(2), blk(1, 1))
        m1 = mm(xs(0), comb(blk(0, 0), blk(1, 1), 1))
        m4 = mm(a22, comb(blk(1, 0), blk(0, 0), -1))
        c11 = mm(xs(4), comb(blk(1, 0), blk(1, 1), 1)) + (m1 + m4 - m5)
        m3 = mm(a11, comb(blk(0, 1), blk(1, 1), -1))
        put_lead(pl.ds(0, NSEG // 2), NSEG // 2, it, c11, m3 + m5)
        m2 = mm(xs(1), blk(0, 0))
        c22 = mm(xs(3), comb(blk(0, 0), blk(0, 1), 1)) + (m1 - m2 + m3)
        put_lead(pl.ds(NSEG // 2, NSEG // 2), NSEG // 2, it, m2 + m4, c22)
        return vregs(m5, m1, m4, c11, m3, m2, c22)

    def quarter_wait(u, q):
        self_wait(wstage.at[u, pl.ds(pl.multiple_of(q * KQ, KQ), KQ)], SW + 4 * u + q)

    def first_unit(q, carry):
        never = q > 1000
        half = q & 1
        self_wait(xlead.at[q], SXL + q)
        quarter_wait(0, q)
        xlead_u[q] = _narrow(xlead[q].astype(F32).reshape(NSEG * M, KQ))
        relayout(0, 0, q)

        @pl.when(q > 0)
        def _():
            quarter_wait(1, q - 1)
        res = []
        xq = pltpu.bitcast(xlead_u[q], BF16)
        for jl in range(4):
            outs = []
            for par in range(2):
                acc = pl.ds((2 * jl + par) * (NSEG * M), NSEG * M)
                row = pl.multiple_of(slab_row(0, par, jl) + q * (KQ // 2), 8)
                w = pltpu.bitcast(w_a[pl.ds(row, KQ // 2), :], BF16)
                d = _dot(xq, w) + jnp.where(q == 0, 0.0, wk[acc, :])
                wk[acc, :] = d
                outs.append(d)
            put_lead(pl.ds(0, NSEG), NSEG, jl, outs[0], outs[1])
            res += outs
        gates = (never, vregs(*res))
        qn = jnp.maximum(q - 1, 0)
        relayout(1, 1, qn, gates, src=(jnp.minimum(q, 1), qn))
        for r in range(0, HR, 8):
            for cb in range(2):
                cols = pl.ds(cb * 128, 128)
                i = 2 * (r // 8) + cb
                a11 = gated(xlead_u[half, pl.ds(r, 8), cols], i, HR // 4, gates)
                a22 = gated(xlead_u[2 + half, pl.ds(HR + r, 8), cols], i, HR // 4, gates)
                a21 = xlead_u[half, pl.ds(HR + r, 8), cols]
                a12 = xlead_u[2 + half, pl.ds(r, 8), cols]
                for f, (x, y, sg) in enumerate(((a11, a22, 1), (a21, a22, 1), (a11, a12, 1),
                                                (a21, a11, -1), (a12, a22, -1))):
                    xs_u[f, half, pl.ds(r, 8), cols] = _narrow(comb(x, y, sg))
        return carry
    loop("units", 0, 4, first_unit, 0)
    w_copy(1, 0).start()
    late_start(0)
    w_copy(0, 1, 3).wait()
    relayout(1, 1, 3)

    def second_unit(jl, carry):
        quarter_wait(2, jl)
        relayout(2, 0, jl, (jl > 1000, batch_pair(1, 1, jl)))
        return carry
    loop("units", 0, 4, second_unit, 0)

    def late_relayout(src, hp, half, gates):
        for r in range(16):
            blk = pltpu.bitcast(wostage[src, pl.ds(half * 256 + r * 16, 16), :], U32)
            row = pl.multiple_of(hp * 128 + r * 8, 8)
            for n in range(NB):
                wo_u[n, pl.ds(row, 8), :] = gated(blk[:, n * 128:(n + 1) * 128], r * NB + n, 16 * NB, gates)
        for t in range(8):
            tile = pltpu.bitcast(hbuf[src, :, pl.ds((8 * half + t) * 128, 128)], U32)
            tile = jnp.concatenate([gated(tile[0:8], t, 8, gates), tile[8:]], axis=0)
            row = pl.multiple_of(hp * 512 + t * 64, 64)
            ht[pl.ds(row, 64), :] = pltpu.bitcast(pltpu.bitcast(tile, BF16).T, U32)

    def unit_body(u, g):
        @pl.when(u < 11)
        def _():
            self_wait(wstage.at[(u + 1) & 3], SW + 12 + ((u + 1) & 3))

        @pl.when(u >= 8)
        def _():
            for e in range(2):
                k = (u - 8) * 2 + e
                self_wait(wostage.at[k], SWO + k)
                self_wait(hbuf.at[k], SH + k)
        for m in (1, 2):
            @pl.when((u + 3) >> 2 == m)
            def _():
                w_copy(m, (u + 3) & 3).start()

        @pl.when(u <= 8)
        def _():
            late_start(u - 1)
        if g == 1:
            @pl.when(u == 9)
            def _():
                x_copy(0).start()
                a_start(0)
                tw_cp.start()
        if only is None or "chunk" in only:
            for jl in range(4):
                gates = (u > 1000, batch_pair(u, g, jl))
                relayout(jnp.where(u < 11, u + 1, u - 1), 1 - g, jl, gates)
                k = jnp.maximum(u - 8, 0) * 2 + jl // 2
                late_relayout(jnp.where(u >= 8, k, 8), 2 * k + jl % 2, jl % 2, gates)

    def unit_pair(mm, carry):
        for g in range(2):
            with scope("unit"):
                unit_body(2 * mm + g, g)
        return carry
    lax.fori_loop(1, 6, unit_pair, 0)

    a_start(1)
    for g in range(1, NG):
        x_copy(g).start()
    for cp in small:
        cp.wait()
    dd = ssmd_ref[0].astype(F32)
    for g in range(NG):
        sk = sk_ref[g].astype(F32)
        for j in range(KS):
            taps[g, j] = jnp.broadcast_to(sk[j:j + 1], (8, 128))
        taps[g, KS] = jnp.broadcast_to(dd[g:g + 1], (8, 128))

    def part_a(i, kick):
        g, j = i >> 1, i & 1
        sl = g & 1
        never = i > 1000
        z = pl.multiple_of(jnp.where(never, 32, 0), 32) if cfg["a_dyn"] else 0
        sub = lax.broadcasted_iota(jnp.int32, (8, 128), 0)
        kickbuf[jnp.where(never, 1, 0)] = kick
        chain = [kickbuf[jnp.where(i > 2000, 0, 1)]]

        def begin(xs, ng):
            xs = list(xs)
            for e in range(min(ng, len(xs))):
                c = chain[0]
                c = c if c.dtype == xs[e].dtype else pltpu.bitcast(c, xs[e].dtype)
                xs[e] = jnp.where(never, c, xs[e])
            return xs

        def merge(vals):
            c = vals[-1]
            for v in list(vals[:-1])[:cfg["a_merge"]] + list(vals[:cfg["a_pad"]]):
                c = jnp.maximum(v, c)
            chain[0] = c

        def ld(v):
            if isinstance(v, tuple):
                blk, ri, r = v
                base = 8 * WS + 256 * blk + 16 * ri + 32 * r
                if cfg["skew2"]:
                    base += 8 * (blk % 2)
                lo = wk[pl.ds(base, 8), :]
                if r == 0:
                    return lo
                if cfg["skew2"]:
                    return pltpu.roll(lo, 8 - r, 0)
                return pltpu.roll(jnp.where(sub >= r, lo, wk[pl.ds(base + 8, 8), :]), 8 - r, 0)
            return wk[pl.ds(z + 8 * v, 8), :]

        def st(v, x):
            wk[pl.ds(z + 8 * v, 8), :] = x

        def twid(idx):
            return (tw[j, idx], tw[j, idx + 1])

        def pairs(flat):
            return [(flat[2 * e], flat[2 * e + 1]) for e in range(len(flat) // 2)]

        def fwd4(locs, t0):
            v = pairs(begin([ld(x) for loc in locs[::-1] for x in loc], cfg["a_g4"]))[::-1]
            return _dft4([v[0]] + [_cmul(v[r], twid(t0 + 2 * r)) for r in range(1, 4)], +1)

        def inv4(v, t0):
            o = _dft4(v, -1)
            return [o[0]] + [_cmulc(o[r], twid(t0 + 2 * r)) for r in range(1, 4)]

        def ld4(locs):
            return pairs(begin([ld(x) for loc in locs for x in loc], cfg["a_g4i"]))

        def put4(locs, o):
            for loc, x in zip(locs, o):
                st(loc[0], x[0])
                st(loc[1], x[1])
            merge([x for c in o for x in c])

        def put4_t(dsts, o):
            for (blk, slot), x in zip(dsts, o):
                for ri in range(2):
                    base = 8 * WS + 256 * blk + 16 * ri + slot
                    if cfg["skew2"]:
                        base += 8 * (blk % 2)
                        wk[pl.ds(base, 8 - slot, stride=33), :] = x[ri][0:8 - slot]
                        if slot:
                            wk[pl.ds(base - 8 + 33 * (8 - slot), slot, stride=33), :] = x[ri][8 - slot:8]
                    else:
                        wk[pl.ds(base, 8, stride=33), :] = x[ri]
            merge([x for c in o for x in c])

        def xloc(sig, n):
            return (WX + 256 * sig + 2 * n, WX + 256 * sig + 2 * n + 1)

        def sloc(kb, l):
            return ((2 * kb + l // 8, 0, l % 8), (2 * kb + l // 8, 1, l % 8))

        def pass_kv():
            t = [taps[g, a] for a in range(KS)]
            prev = [None] + [jnp.zeros((8, 128), F32)] * (KS - 1)
            for v in range(S // 16):
                w, = begin([pltpu.bitcast(abuf[sl, 1, pl.ds(16 * v, 16), :], U32)], 1)
                k2 = _widen(w)
                v2 = abuf[sl, 2, pl.ds(16 * v, 16), :].astype(F32)
                outs = []
                for hh in range(2):
                    x = k2[8 * hh:8 * hh + 8]
                    cur = [None] + [pltpu.roll(x, a, 0) for a in range(1, KS)]
                    ks = x * t[0]
                    for a in range(1, KS):
                        ks = ks + jnp.where(sub < a, prev[a], cur[a]) * t[a]
                    prev = cur
                    kv = (ks * v2[8 * hh:8 * hh + 8]).astype(BF16).astype(F32)
                    st(WK + 2 * v + hh, kv)
                    outs.append(kv)
                merge(outs)

        def forward(sig, src):
            for n in range(32):
                x = src(n)
                cs = []
                for d in range(4):
                    a, b = twid(TAF + 2 * d), twid(TAF + 2 * (d + 4))
                    if d == 0:
                        s_ = x[4] * b[0]
                        cs.append((x[0] + s_, s_))
                    else:
                        cs.append((x[d] * a[0] + x[d + 4] * b[0], x[d] * a[1] + x[d + 4] * b[1]))
                put4([xloc(sig, n + 32 * k0) for k0 in range(4)], _dft4(cs, +1))
            for k0 in range(4):
                for n in range(8):
                    locs = [xloc(sig, n + 8 * r + 32 * k0) for r in range(4)]
                    put4(locs, fwd4(locs, TB + 8 * k0))
            for k0 in range(4):
                for k1 in range(4):
                    k = k0 + 4 * k1
                    for a in range(2):
                        o = fwd4([xloc(sig, a + 2 * r + 8 * k1 + 32 * k0) for r in range(4)], TC + 8 * k)
                        put4_t([(2 * ((k + 16 * k2) // 8) + a, k % 8) for k2 in range(4)], o)
            for kb in range(8):
                for e in range(4):
                    o = fwd4([sloc(kb, e + 4 * r) for r in range(4)], TD + 8 * kb)
                    put4([xloc(sig, 16 * kb + e + 4 * r) for r in range(4)], o)
            for kb in range(8):
                for k3 in range(4):
                    locs = [xloc(sig, 16 * kb + r + 4 * k3) for r in range(4)]
                    t0 = TE + 8 * (4 * kb + k3)
                    o = fwd4(locs, t0)
                    if sig == 0:
                        hs = ld4([xloc(1, 16 * kb + r + 4 * k3) for r in range(4)])
                        o = inv4([_cmul(a, b) for a, b in zip(o, hs)], t0)
                    put4(locs, o)

        def inverse():
            for kb in range(8):
                for e in range(4):
                    o = inv4(ld4([xloc(0, 16 * kb + e + 4 * r) for r in range(4)]), TD + 8 * kb)
                    put4_t([(2 * kb + (e + 4 * f) // 8, (e + 4 * f) % 8) for f in range(4)], o)
            for k0 in range(4):
                for k1 in range(4):
                    k = k0 + 4 * k1
                    for a in range(2):
                        v = ld4([sloc((k + 16 * r) // 8, 8 * a + k % 8) for r in range(4)])
                        put4([xloc(0, a + 2 * b + 8 * k1 + 32 * k0) for b in range(4)], inv4(v, TC + 8 * k))
            for k0 in range(4):
                for n in range(8):
                    locs = [xloc(0, n + 8 * r + 32 * k0) for r in range(4)]
                    put4(locs, inv4(ld4(locs), TB + 8 * k0))
            dskip = taps[g, KS]
            for n0 in range(32):
                cs = _dft4(ld4([xloc(0, n0 + 32 * r) for r in range(4)]), -1)
                outs = []
                for d in [d0 + 4 * hh for d0 in range(4) for hh in range(2)]:
                    n = n0 + 32 * d
                    a = twid(TAI + 2 * d)
                    if 0 < d < 4 and cfg["a_fine"]:
                        cs[d] = tuple(begin(cs[d], 2))
                    c = cs[d % 4]
                    y = c[0] * a[0] if d == 0 else c[0] * a[0] + c[1] * a[1]
                    y = y + jnp.where(j == 0, ld(WK + n) * dskip, ld(WY + n))
                    st(WY + n, y)
                    chain[0] = abuf[sl, 0, pl.ds(8 * n, 8), :].astype(F32) * y
                    aout[g, n // 4, pl.ds(8 * (n % 4), 8), :] = chain[0].astype(BF16)
                    outs.append(chain[0])
                merge(outs)

        def filt(n):
            base = pl.multiple_of(g * (S // 2), S // 2)
            ws = begin([ht[pl.ds(base + 8 * (n // 2 + 16 * d), 8), :] for d in range(8)], 8)
            return [_widen(w)[8 * (n % 2):8 * (n % 2) + 8] for w in ws]
        pass_kv()
        forward(1, filt)
        forward(0, lambda n: begin([ld(WK + n + 32 * d) for d in range(8)], 8))
        inverse()
        return chain[0]

    scale = DH ** (-0.5)

    def w_slab(m, h):
        u = 4 * m + h // 8
        return pltpu.bitcast(w_parts[u % 2][pl.ds(slab_row(u, h % 2, (h // 2) % 4), D // 2), :], BF16)

    class Step:
        def __init__(self, s, prev, mem):
            self.s = s
            self.prev = prev
            self.qkv, self.ps, self.os = {}, {}, []
            self.acc = [None] * NB
            self.ocat, self.lead, self.early, self.marks, self.heads = {}, {}, {}, {}, {}
            self.tie = None
            x = xbuf[s, pl.ds(M, SEG - M), :].astype(F32)
            self.lhsf = jnp.concatenate([mem, x], axis=0)
            self.lhs = self.lhsf.astype(BF16)

        def proj_early(self, m, h, k):
            self.early[m, h] = (k, _dot(self.lhsf[:, :k].astype(BF16), w_slab(m, h)[:k]))

        def proj(self, m, h):
            if (m, h) in self.early:
                k, part = self.early[m, h]
                d = _dot(self.lhsf[:, k:].astype(BF16), w_slab(m, h)[k:]) + part
            else:
                d = _dot(self.lhs, w_slab(m, h))
            self.heads[m, h] = d
            j = h // 2
            if (m, h ^ 1) not in self.heads:
                return
            a, b = self.heads[m, 2 * j], self.heads[m, 2 * j + 1]
            self.marks[m, j] = a[0:8]
            lead = _widen(qkvb[self.s, m * NPAIR + j])
            self.qkv[m, j] = jnp.concatenate([a, b, lead], axis=0).astype(BF16)

        def probs(self, j):
            fill = fill_ref[pl.ds(0, R), pl.ds(0, R)]
            qk = _dot_nt(self.qkv[0, j], self.qkv[1, j])
            if cfg["exp2"]:
                sc = jnp.where(fill == 0.0, qk, fill)
                e = jnp.exp2((sc - jnp.max(sc, axis=-1, keepdims=True)) * (scale * LOG2E))
            else:
                sc = jnp.where(fill == 0.0, qk * scale, fill)
                e = jnp.exp(sc - jnp.max(sc, axis=-1, keepdims=True))
            l = jnp.sum(e, axis=-1, keepdims=True)
            r = pl.reciprocal(l, approx=True)
            r = r * (2.0 - l * r)
            self.ps[j] = (e * r).astype(BF16)

        def attend(self, j):
            o = _dot(self.ps[j], self.qkv[2, j])
            la, lb = o[2 * SEG:2 * SEG + M], o[2 * SEG + M:]
            rows = pl.ds(pl.multiple_of((self.s >> 1) * M, M), M)
            if self.prev is None:
                self.lead[j] = (la, lb)
                forms = {2: la + lb, 5: la}
            else:
                a11, a12 = self.prev.lead[j]
                forms = {0: a11 + lb, 1: la + lb, 3: la - a11, 4: a12 - lb, 6: lb}
            for f, v in forms.items():
                ob[f * NPAIR + j, rows, :] = v.astype(BF16)
            self.os += [o[0:SEG], o[SEG:2 * SEG]]

        def wo(self, h0, h1, n):
            if h0 not in self.ocat:
                self.ocat[h0] = jnp.concatenate(self.os[h0:h1], axis=1).astype(BF16)
            w = wo_u[n, pl.ds(h0 * 64, (h1 - h0) * 64), :]
            if self.tie is not None:
                w = jnp.concatenate(
                    [jnp.where(self.s > 1000, pltpu.bitcast(self.tie, U32), w[0:8]), w[8:]], axis=0)
                self.tie = None
            d = _dot(self.ocat[h0], pltpu.bitcast(w, BF16))
            self.acc[n] = d if self.acc[n] is None else d + self.acc[n]

        def finish(self):
            res = jnp.concatenate(self.acc, axis=1)
            obuf[self.s] = res.astype(BF16)
            return res[0:M]

    def steps(i, mem):
        sts = []
        for u in range(U):
            st = Step(i * U + u, sts[-1] if u % 2 else None, mem)
            sts.append(st)
            for item in _step_order(u, cfg):
                if item[0] == "A":
                    if cfg["a"]:
                        ku, km, kj = cfg["kick"]
                        st.tie = part_a(i, sts[ku].marks[km, kj])
                else:
                    dict(P=st.proj, E=st.proj_early, S=st.probs, V=st.attend, W=st.wo)[item[0]](*item[1:])
            mem = st.finish()
        return mem

    def group(g, mem):
        x_copy(g).wait()
        self_wait(abuf.at[g & 1], SA + (g & 1))

        @pl.when(jnp.logical_and(g >= 1, g < NG - 1))
        def _():
            a_start(g + 1)
        return loop("steps", 0, 2, lambda j, m_: steps(2 * g + j, m_), mem)

    tw_cp.wait()
    lax.fori_loop(0, NG, group, mem0_ref[...].astype(F32))

    ob_cp = pltpu.make_async_copy(
        obuf.at[:, pl.ds(M, SEG - M), :],
        out_hbm.at[:, pl.ds(M, SEG - M), pl.ds(D, D)], sems.at[SO])
    ob_cp.start()
    for g in range(NG):
        pltpu.make_async_copy(
            aout.at[g], out_hbm.at[:, :, pl.ds(g * 128, 128)], sems.at[SO + 1]).start()

    def epi(it, carry):
        ns = [2 * it, 2 * it + 1]

        def blk(hp, u):
            return [wo_u[ns[u], pl.ds((2 * j + hp) * 64, 64), :] for j in range(NPAIR)]

        def mm(f, bs):
            lhs = jnp.concatenate([ob[f * NPAIR + j] for j in range(NPAIR)], axis=1)
            return _dot(lhs, as_bf16(jnp.concatenate(bs, axis=0)))

        def cb(x, y, sign):
            return [comb(a, b, sign) for a, b in zip(x, y)]

        def put(u, par, c):
            for i in range(NSEG // 2):
                obb[ns[u], 2 * i + par] = c[M * i:M * i + M].astype(BF16)
        m5 = mm(2, blk(1, 1))
        m1 = mm(0, cb(blk(0, 0), blk(1, 1), 1))
        m4 = mm(6, cb(blk(1, 0), blk(0, 0), -1))
        put(0, 0, mm(4, cb(blk(1, 0), blk(1, 1), 1)) + (m1 + m4 - m5))
        m3 = mm(5, cb(blk(0, 1), blk(1, 1), -1))
        put(1, 0, m3 + m5)
        m2 = mm(1, blk(0, 0))
        put(0, 1, m2 + m4)

        def send(n):
            col = pl.multiple_of(D + n * 128, 128)
            pltpu.make_async_copy(
                obb.at[n], out_hbm.at[:, pl.ds(0, M), pl.ds(col, 128)], sems.at[SO + 2]).start()
        send(ns[0])
        put(1, 1, mm(3, cb(blk(0, 0), blk(0, 1), 1)) + (m1 - m2 + m3))
        send(ns[1])
        return carry
    loop("epi", 0, NB // 2, epi, 0)
    ob_cp.wait()
    self_wait(aout, SO + 1)
    self_wait(obb, SO + 2)


def _step_order(u, cfg):
    ks = cfg["ks"]
    per = cfg["period"]
    tmpl = []
    for x in cfg["tmpl"].split():
        kind, lag = x[:-1], int(x[-1])
        tmpl += [(kind + "a", lag), (kind + "b", lag)] if kind in ("q", "k", "v") else [(kind, lag)]

    def proj(kind, j):
        return ("qkv".index(kind[0]), 2 * j + "ab".index(kind[1]))
    out = []
    nw = 0
    for t in range(per - 1, NPAIR + per + max(l for _, l in tmpl), per):
        for kind, lag in tmpl:
            j = t - lag
            if j < 0:
                continue
            if j >= NPAIR:
                if kind[1:] == "a" and nw < NB:
                    out.append(("W", 0, ks, nw))
                    nw += 1
                continue
            out.append(("P",) + proj(kind, j) if len(kind) == 2 else (kind, j))
    if u > 0:
        first = [x[1:] for x in out if x[0] == "P"][:cfg["ne"]]
        out = [("E",) + x + (cfg["ek"],) for x in first] + out
    out += [("W", 0, ks, n) for n in range(nw, NB)]
    for n in range(NB):
        if u == U - 1 and n == cfg["tie_n"]:
            out.append(("A",))
        out.append(("W", ks, H, n))
    return out


_DEFAULT_CFG = dict(tmpl="V3 ka0 kb0 va1 S1 qa0 qb0 vb1", ks=16, ne=5, ek=768, period=1, exp2=0,
                    a=1, tie_n=7, kick=(0, 0, 0), skew2=0, a_dyn=0, a_merge=5, a_pad=0, a_fine=1,
                    a_g4=8, a_g4i=2)


def _build(cfg):
    tw_np = _twiddles()
    fill_np = np.zeros((96, 128), np.float32)
    fill_np[:R, :R] = _mask_fill() * (DH ** 0.5 if cfg["exp2"] else 1.0)

    def run(A_q, A_k, A_v, A_shift_k, A_ssm_k, A_ssm_D, B_x, B_mem0, B_Wq, B_Wk, B_Wv, B_Wo):
        sk = A_shift_k.T.reshape(KS, NG, 128).transpose(1, 0, 2)
        any_spec = pl.BlockSpec(memory_space=pl.ANY)
        out = pl.pallas_call(
            functools.partial(_kernel, cfg),
            out_shape=jax.ShapeDtypeStruct((NSEG, SEG, 2 * D), BF16),
            in_specs=[any_spec] * 14,
            out_specs=any_spec,
            scratch_shapes=[
                pltpu.VMEM((48 * SLAB + 544, 128), U32),
                pltpu.VMEM((48 * SLAB + 544, 128), U32),
                pltpu.VMEM((NB, H * DH // 2, 128), U32),
                pltpu.VMEM((4, D, 8, DH), BF16),
                pltpu.VMEM((9, 512, D), BF16),
                pltpu.VMEM((NSEG, SEG, D), BF16),
                pltpu.VMEM((4, NSEG, M, KQ), BF16),
                pltpu.VMEM((4, NSEG * M // 2, KQ), U32),
                pltpu.VMEM((5, 2, HR, KQ), U32),
                pltpu.VMEM((NSEG, 3 * NPAIR, 8, 128), U32),
                pltpu.VMEM((7 * NPAIR, NSEG * M // 2, DH), BF16),
                pltpu.VMEM((NSEG, SEG, D), BF16),
                pltpu.VMEM((NB, NSEG, M, 128), BF16),
                pltpu.VMEM((2, 3, S, 128), BF16),
                pltpu.VMEM((NG + 1, 128, S), BF16),
                pltpu.VMEM((NG * S // 2, 128), U32),
                pltpu.VMEM((8 * NW + 32, 128), F32),
                pltpu.VMEM((2, NT, 8, 128), F32),
                pltpu.VMEM((NG, NSEG, SEG, 128), BF16),
                pltpu.VMEM((4, 8, 128), F32),
                pltpu.VMEM((96, 128), F32),
                pltpu.VMEM((NG, 8, 8, 128), F32),
                pltpu.VMEM((M, D), BF16),
                pltpu.VMEM((NG, KS, 128), BF16),
                pltpu.VMEM((4, NG, 128), BF16),
                pltpu.SemaphoreType.DMA((56,)),
            ],
            compiler_params=pltpu.CompilerParams(vmem_limit_bytes=124 * 1024 * 1024,
                                                 disable_bounds_checks=True),
        )(A_q.reshape(S, D), A_k.reshape(S, D), A_v.reshape(S, D), sk, A_ssm_k,
          A_ssm_D.reshape(NG, 128), B_x.reshape(NSEG, SEG, D), B_mem0.reshape(M, D),
          B_Wq, B_Wk, B_Wv, B_Wo.reshape(H * DH, D),
          jnp.asarray(tw_np), jnp.asarray(fill_np))
        return out.reshape(1, S, 2 * D)

    return run


@functools.partial(jax.jit, static_argnames=("B_seg_len",))
def pallas_concat_heads__ssm_conv_h3__memory_aug_recurrent_mem_tr__prompt_kernel(
    A_q: jax.Array,
    A_k: jax.Array,
    A_v: jax.Array,
    A_shift_k: jax.Array,
    A_ssm_k: jax.Array,
    A_ssm_D: jax.Array,
    B_x: jax.Array,
    B_mem0: jax.Array,
    B_Wq: jax.Array,
    B_Wk: jax.Array,
    B_Wv: jax.Array,
    B_Wo: jax.Array,
    B_seg_len: int = SEG,
):
    assert B_seg_len == SEG
    return _build(_DEFAULT_CFG)(A_q, A_k, A_v, A_shift_k, A_ssm_k, A_ssm_D, B_x, B_mem0,
                                B_Wq, B_Wk, B_Wv, B_Wo)
```

```python
import functools

import numpy as np
import jax
import jax.numpy as jnp
from jax import lax
import jax.experimental.pallas as pl
import jax.experimental.pallas.tpu as pltpu

F32 = jnp.float32
BF16 = jnp.bfloat16
U32 = jnp.uint32

S = 2048
D = 1024
H = 32
DH = 128
M = 8
SEG = 32
NSEG = S // SEG
U = 4
NPAIR = H // 2
R = 2 * (M + SEG)
SLAB = 520
KS = 4
NG = D // 128
KQ = D // 4
NB = D // 128
HR = NSEG * M // 4

TAF, TAI, TB, TC, TD, TE, NT = 0, 16, 32, 64, 192, 256, 512
WX, WS, WY, WK, NW = 0, 512, 1024, 1280, 1536


def _twiddles():
    tw = np.zeros((2, NT, 8), np.float64)

    def put(j, idx, z):
        tw[j, idx] = np.real(z)
        tw[j, idx + 1] = np.imag(z)
    s = np.arange(8)
    tau = 2j * np.pi
    for j in range(2):
        lx = 1j * np.pi * (1 + 4 * j) / 4096
        for d in range(8):
            put(j, TAF + 2 * d, np.exp(lx * 256 * d))
            put(j, TAI + 2 * d, np.exp(lx * 256 * d) / 2048)
        for r in range(4):
            for k in range(4):
                put(j, TB + 8 * k + 2 * r, np.exp((lx * 64 + tau * k / 16) * r))
            for k in range(16):
                put(j, TC + 8 * k + 2 * r, np.exp((lx * 16 + tau * k / 64) * r))
            for kb in range(8):
                put(j, TD + 8 * kb + 2 * r, np.exp((lx * 4 + tau * (s + 8 * kb) / 256) * r))
                for k3 in range(4):
                    put(j, TE + 8 * (4 * kb + k3) + 2 * r,
                        np.exp((lx + tau * (s + 8 * kb + 64 * k3) / 1024) * r))
    return np.ascontiguousarray(np.broadcast_to(tw[..., None], (2, NT, 8, 128))).astype(np.float32)


def _mask_fill():
    blk = np.concatenate([np.arange(M), M + np.arange(M, SEG)])
    lead = M + np.arange(M)
    head = np.concatenate([np.zeros(SEG), np.ones(SEG), np.zeros(M), np.ones(M)])
    pos = np.concatenate([blk, blk, lead, lead])
    same = head[:, None] == head[None, :]
    ok = (pos[:, None] < M) | (pos[:, None] >= pos[None, :])
    fill = np.where(same, np.where(ok, 0.0, -1e9), -np.inf)
    return fill.astype(np.float32)


def _widen(w):
    return pltpu.bitcast(w, BF16).astype(F32)


def _narrow(x):
    return pltpu.bitcast(x.astype(BF16), U32)


def _dot(a, b):
    return jnp.dot(a, b, preferred_element_type=F32)


def _dot_nt(a, b):
    return lax.dot_general(a, b, (((1,), (1,)), ((), ())), preferred_element_type=F32)


def _cadd(a, b):
    return (a[0] + b[0], a[1] + b[1])


def _csub(a, b):
    return (a[0] - b[0], a[1] - b[1])


def _cmul(a, w):
    return (a[0] * w[0] - a[1] * w[1], a[0] * w[1] + a[1] * w[0])


def _cmulc(a, w):
    return (a[0] * w[0] + a[1] * w[1], a[1] * w[0] - a[0] * w[1])


def _bfly_i(b, d, sg):
    p = (b[0] - d[1], b[1] + d[0])
    q = (b[0] + d[1], b[1] - d[0])
    return (p, q) if sg > 0 else (q, p)


def _dft4(x, sg):
    a, b = _cadd(x[0], x[2]), _csub(x[0], x[2])
    c, d = _cadd(x[1], x[3]), _csub(x[1], x[3])
    p, q = _bfly_i(b, d, sg)
    return [_cadd(a, c), p, _csub(a, c), q]


def _kernel(cfg,
            aq_hbm, ak_hbm, av_hbm, sk_hbm, ssmk_hbm, ssmd_hbm, x_hbm, mem0_hbm,
            wq_hbm, wk_hbm, wv_hbm, wo_hbm, tw_hbm, fill_hbm,
            out_hbm,
            w_a, w_b, wo_u, wstage, wostage, xbuf, xlead, xlead_u, xs_u, qkvb, ob, obuf, obb,
            abuf, hbuf, ht, wk, tw, aout, kickbuf,
            fill_ref, taps, mem0_ref, sk_ref, ssmd_ref,
            sems):
    SW, SWO, SXL, SX, SH, SA, ST, SO, SS = 0, 16, 24, 28, 36, 44, 46, 48, 52
    w_hbms = (wq_hbm, wk_hbm, wv_hbm)
    a_hbms = (aq_hbm, ak_hbm, av_hbm)

    def aligned(x, n):
        return x if isinstance(x, int) else pl.multiple_of(x, n)

    def w_copy(m, hq, q=None):
        rows = pl.ds(0, D) if q is None else pl.ds(q * KQ, KQ)
        sem = SW + 12 + hq if q is None else SW + 4 * hq + q
        heads = aligned(8 * hq, 8)
        return pltpu.make_async_copy(
            w_hbms[m].at[rows, pl.ds(heads, 8), :], wstage.at[hq, rows], sems.at[sem])

    def self_wait(ref, sem):
        pltpu.make_async_copy(ref, ref, sems.at[sem]).wait()

    def late_start(k):
        pltpu.make_async_copy(
            wo_hbm.at[pl.ds(aligned(k * 512, 512), 512), :], wostage.at[k],
            sems.at[SWO + k]).start()
        pltpu.make_async_copy(
            ssmk_hbm.at[pl.ds(aligned(k * 128, 128), 128), :], hbuf.at[k],
            sems.at[SH + k]).start()

    def xlead_copy(q):
        return pltpu.make_async_copy(
            x_hbm.at[:, pl.ds(0, M), pl.ds(q * KQ, KQ)], xlead.at[q], sems.at[SXL + q])

    def x_copy(g):
        segs = pl.ds(g * 8, 8)
        return pltpu.make_async_copy(
            x_hbm.at[segs, pl.ds(M, SEG - M), :], xbuf.at[segs, pl.ds(M, SEG - M), :], sems.at[SX + g])

    def a_start(g):
        col = aligned(g * 128, 128)
        for t in (1, 2, 0):
            pltpu.make_async_copy(
                a_hbms[t].at[:, pl.ds(col, 128)], abuf.at[g & 1, t], sems.at[SA + (g & 1)]).start()

    tw_cp = pltpu.make_async_copy(tw_hbm, tw, sems.at[ST])

    small = [pltpu.make_async_copy(src, dst, sems.at[SS + i]) for i, (src, dst) in enumerate((
        (fill_hbm, fill_ref), (mem0_hbm, mem0_ref), (sk_hbm, sk_ref), (ssmd_hbm, ssmd_ref.at[0])))]

    for q in range(4):
        xlead_copy(q).start()
        w_copy(0, 0, q).start()
        if q > 0:
            w_copy(0, 1, q - 1).start()
    w_copy(0, 1, 3).start()
    for q in range(4):
        w_copy(0, 2, q).start()
    w_copy(0, 3).start()
    for cp in small:
        cp.start()

    w_parts = (w_a, w_b)

    def slab_row(u, par, jl):
        return ((u >> 1) * 8 + par * 4 + jl) * SLAB

    def gated(x, i, n, gates):
        if gates is None:
            return x
        never, vals = gates
        v = vals[(i * len(vals) * 3) // (n * 4)]
        return jnp.where(never, pltpu.bitcast(v, U32), x)

    def vregs(*mats):
        return [m_[r:r + 8] for m_ in mats for r in range(0, m_.shape[0], 8)]

    def relayout(u, g, q, gates=None, src=None):
        slot, qs = (u & 3, q) if src is None else src
        low = lax.broadcasted_iota(jnp.int32, (8, 128), 0) < 4
        keep = jnp.where(low, jnp.uint32(0xFFFF), jnp.uint32(0xFFFF0000))
        shl = jnp.where(low, jnp.uint32(16), jnp.uint32(0))
        base = slab_row(u, 0, 0) + q * (KQ // 2)
        for i in range(KQ // 2):
            x = wstage[slot, pl.ds(qs * KQ + 2 * i, 2)].reshape(16, DH)
            x = gated(pltpu.bitcast(x, U32), i, KQ // 2, gates)
            y = pltpu.roll(x, 4, 0)
            w_parts[g][pl.ds(base + i, 8, stride=SLAB), :] = (x & keep) | ((y << shl) >> (16 - shl))

    def comb(x, y, sign):
        return _widen(x) + _widen(y) if sign > 0 else _widen(x) - _widen(y)

    def as_bf16(b):
        return pltpu.bitcast(b, BF16) if b.dtype == U32 else b.astype(BF16)

    def put_lead(segs, n, it, a, b):
        both = jnp.concatenate([a.reshape(n, M, DH), b.reshape(n, M, DH)], axis=1)
        qkvb[segs, it] = _narrow(both)

    def batch_pair(u, g, jl):
        it = 4 * u + jl
        rows = [pl.multiple_of(slab_row(u, par, jl), 8) for par in range(2)]

        def blk(kh, par):
            return w_parts[g][pl.ds(rows[par] + kh * (D // 4), D // 4), :]

        def mm(a, b):
            return _dot(pltpu.bitcast(jnp.concatenate(a, axis=1), BF16), as_bf16(b))

        def xs(f):
            return [xs_u[f, q] for q in range(2)]
        a11 = [xlead_u[q, pl.ds(0, HR), :] for q in (0, 1)]
        a22 = [xlead_u[q, pl.ds(HR, HR), :] for q in (2, 3)]
        m5 = mm(xs(2), blk(1, 1))
        m1 = mm(xs(0), comb(blk(0, 0), blk(1, 1), 1))
        m4 = mm(a22, comb(blk(1, 0), blk(0, 0), -1))
        c11 = mm(xs(4), comb(blk(1, 0), blk(1, 1), 1)) + (m1 + m4 - m5)
        m3 = mm(a11, comb(blk(0, 1), blk(1, 1), -1))
        put_lead(pl.ds(0, NSEG // 2), NSEG // 2, it, c11, m3 + m5)
        m2 = mm(xs(1), blk(0, 0))
        c22 = mm(xs(3), comb(blk(0, 0), blk(0, 1), 1)) + (m1 - m2 + m3)
        put_lead(pl.ds(NSEG // 2, NSEG // 2), NSEG // 2, it, m2 + m4, c22)
        return vregs(m5, m1, m4, c11, m3, m2, c22)

    def quarter_wait(u, q):
        self_wait(wstage.at[u, pl.ds(pl.multiple_of(q * KQ, KQ), KQ)], SW + 4 * u + q)

    def first_unit(q, carry):
        never = q > 1000
        half = q & 1
        self_wait(xlead.at[q], SXL + q)
        quarter_wait(0, q)
        xlead_u[q] = _narrow(xlead[q].astype(F32).reshape(NSEG * M, KQ))
        relayout(0, 0, q)

        @pl.when(q > 0)
        def _():
            quarter_wait(1, q - 1)
        res = []
        xq = pltpu.bitcast(xlead_u[q], BF16)
        for jl in range(4):
            outs = []
            for par in range(2):
                acc = pl.ds((2 * jl + par) * (NSEG * M), NSEG * M)
                row = pl.multiple_of(slab_row(0, par, jl) + q * (KQ // 2), 8)
                w = pltpu.bitcast(w_a[pl.ds(row, KQ // 2), :], BF16)
                d = _dot(xq, w) + jnp.where(q == 0, 0.0, wk[acc, :])
                wk[acc, :] = d
                outs.append(d)
            put_lead(pl.ds(0, NSEG), NSEG, jl, outs[0], outs[1])
            res += outs
        gates = (never, vregs(*res))
        qn = jnp.maximum(q - 1, 0)
        relayout(1, 1, qn, gates, src=(jnp.minimum(q, 1), qn))
        for r in range(0, HR, 8):
            for cb in range(2):
                cols = pl.ds(cb * 128, 128)
                i = 2 * (r // 8) + cb
                a11 = gated(xlead_u[half, pl.ds(r, 8), cols], i, HR // 4, gates)
                a22 = gated(xlead_u[2 + half, pl.ds(HR + r, 8), cols], i, HR // 4, gates)
                a21 = xlead_u[half, pl.ds(HR + r, 8), cols]
                a12 = xlead_u[2 + half, pl.ds(r, 8), cols]
                for f, (x, y, sg) in enumerate(((a11, a22, 1), (a21, a22, 1), (a11, a12, 1),
                                                (a21, a11, -1), (a12, a22, -1))):
                    xs_u[f, half, pl.ds(r, 8), cols] = _narrow(comb(x, y, sg))
        return carry
    lax.fori_loop(0, 4, first_unit, 0)
    w_copy(1, 0).start()
    late_start(0)
    w_copy(0, 1, 3).wait()
    relayout(1, 1, 3)

    def second_unit(jl, carry):
        quarter_wait(2, jl)
        relayout(2, 0, jl, (jl > 1000, batch_pair(1, 1, jl)))
        return carry
    lax.fori_loop(0, 4, second_unit, 0)

    def late_relayout(src, hp, half, gates):
        for r in range(16):
            blk = pltpu.bitcast(wostage[src, pl.ds(half * 256 + r * 16, 16), :], U32)
            row = pl.multiple_of(hp * 128 + r * 8, 8)
            for n in range(NB):
                wo_u[n, pl.ds(row, 8), :] = gated(blk[:, n * 128:(n + 1) * 128], r * NB + n, 16 * NB, gates)
        for t in range(8):
            tile = pltpu.bitcast(hbuf[src, :, pl.ds((8 * half + t) * 128, 128)], U32)
            tile = jnp.concatenate([gated(tile[0:8], t, 8, gates), tile[8:]], axis=0)
            row = pl.multiple_of(hp * 512 + t * 64, 64)
            ht[pl.ds(row, 64), :] = pltpu.bitcast(pltpu.bitcast(tile, BF16).T, U32)

    def unit_body(u, g):
        @pl.when(u < 11)
        def _():
            self_wait(wstage.at[(u + 1) & 3], SW + 12 + ((u + 1) & 3))

        @pl.when(u >= 8)
        def _():
            for e in range(2):
                k = (u - 8) * 2 + e
                self_wait(wostage.at[k], SWO + k)
                self_wait(hbuf.at[k], SH + k)
        for m in (1, 2):
            @pl.when((u + 3) >> 2 == m)
            def _():
                w_copy(m, (u + 3) & 3).start()

        @pl.when(u <= 8)
        def _():
            late_start(u - 1)
        if g == 1:
            @pl.when(u == 9)
            def _():
                x_copy(0).start()
                a_start(0)
                tw_cp.start()
        for jl in range(4):
            gates = (u > 1000, batch_pair(u, g, jl))
            relayout(jnp.where(u < 11, u + 1, u - 1), 1 - g, jl, gates)
            k = jnp.maximum(u - 8, 0) * 2 + jl // 2
            late_relayout(jnp.where(u >= 8, k, 8), 2 * k + jl % 2, jl % 2, gates)

    def unit_pair(mm, carry):
        for g in range(2):
            unit_body(2 * mm + g, g)
        return carry
    lax.fori_loop(1, 6, unit_pair, 0)

    a_start(1)
    for g in range(1, NG):
        x_copy(g).start()
    for cp in small:
        cp.wait()
    dd = ssmd_ref[0].astype(F32)
    for g in range(NG):
        sk = sk_ref[g].astype(F32)
        for j in range(KS):
            taps[g, j] = jnp.broadcast_to(sk[j:j + 1], (8, 128))
        taps[g, KS] = jnp.broadcast_to(dd[g:g + 1], (8, 128))

    def part_a(i, kick):
        g, j = i >> 1, i & 1
        sl = g & 1
        never = i > 1000
        sub = lax.broadcasted_iota(jnp.int32, (8, 128), 0)
        kickbuf[jnp.where(never, 1, 0)] = kick
        chain = [kickbuf[jnp.where(i > 2000, 0, 1)]]

        def begin(xs, ng):
            xs = list(xs)
            for e in range(min(ng, len(xs))):
                c = chain[0]
                c = c if c.dtype == xs[e].dtype else pltpu.bitcast(c, xs[e].dtype)
                xs[e] = jnp.where(never, c, xs[e])
            return xs

        def merge(vals):
            c = vals[-1]
            for v in list(vals[:-1])[:cfg["a_merge"]]:
                c = jnp.maximum(v, c)
            chain[0] = c

        def ld(v):
            if isinstance(v, tuple):
                blk, ri, r = v
                base = 8 * WS + 256 * blk + 16 * ri + 32 * r
                lo = wk[pl.ds(base, 8), :]
                if r == 0:
                    return lo
                return pltpu.roll(jnp.where(sub >= r, lo, wk[pl.ds(base + 8, 8), :]), 8 - r, 0)
            return wk[pl.ds(8 * v, 8), :]

        def st(v, x):
            wk[pl.ds(8 * v, 8), :] = x

        def twid(idx):
            return (tw[j, idx], tw[j, idx + 1])

        def pairs(flat):
            return [(flat[2 * e], flat[2 * e + 1]) for e in range(len(flat) // 2)]

        def fwd4(locs, t0):
            v = pairs(begin([ld(x) for loc in locs[::-1] for x in loc], cfg["a_g4"]))[::-1]
            return _dft4([v[0]] + [_cmul(v[r], twid(t0 + 2 * r)) for r in range(1, 4)], +1)

        def inv4(v, t0):
            o = _dft4(v, -1)
            return [o[0]] + [_cmulc(o[r], twid(t0 + 2 * r)) for r in range(1, 4)]

        def ld4(locs):
            return pairs(begin([ld(x) for loc in locs for x in loc], cfg["a_g4i"]))

        def put4(locs, o):
            for loc, x in zip(locs, o):
                st(loc[0], x[0])
                st(loc[1], x[1])
            merge([x for c in o for x in c])

        def put4_t(dsts, o):
            for (blk, slot), x in zip(dsts, o):
                for ri in range(2):
                    base = 8 * WS + 256 * blk + 16 * ri + slot
                    wk[pl.ds(base, 8, stride=33), :] = x[ri]
            merge([x for c in o for x in c])

        def xloc(sig, n):
            return (WX + 256 * sig + 2 * n, WX + 256 * sig + 2 * n + 1)

        def sloc(kb, l):
            return ((2 * kb + l // 8, 0, l % 8), (2 * kb + l // 8, 1, l % 8))

        def pass_kv():
            t = [taps[g, a] for a in range(KS)]
            prev = [None] + [jnp.zeros((8, 128), F32)] * (KS - 1)
            for v in range(S // 16):
                w, = begin([pltpu.bitcast(abuf[sl, 1, pl.ds(16 * v, 16), :], U32)], 1)
                k2 = _widen(w)
                v2 = abuf[sl, 2, pl.ds(16 * v, 16), :].astype(F32)
                outs = []
                for hh in range(2):
                    x = k2[8 * hh:8 * hh + 8]
                    cur = [None] + [pltpu.roll(x, a, 0) for a in range(1, KS)]
                    ks = x * t[0]
                    for a in range(1, KS):
                        ks = ks + jnp.where(sub < a, prev[a], cur[a]) * t[a]
                    prev = cur
                    kv = (ks * v2[8 * hh:8 * hh + 8]).astype(BF16).astype(F32)
                    st(WK + 2 * v + hh, kv)
                    outs.append(kv)
                merge(outs)

        def forward(sig, src):
            for n in range(32):
                x = src(n)
                cs = []
                for d in range(4):
                    a, b = twid(TAF + 2 * d), twid(TAF + 2 * (d + 4))
                    if d == 0:
                        s_ = x[4] * b[0]
                        cs.append((x[0] + s_, s_))
                    else:
                        cs.append((x[d] * a[0] + x[d + 4] * b[0], x[d] * a[1] + x[d + 4] * b[1]))
                put4([xloc(sig, n + 32 * k0) for k0 in range(4)], _dft4(cs, +1))
            for k0 in range(4):
                for n in range(8):
                    locs = [xloc(sig, n + 8 * r + 32 * k0) for r in range(4)]
                    put4(locs, fwd4(locs, TB + 8 * k0))
            for k0 in range(4):
                for k1 in range(4):
                    k = k0 + 4 * k1
                    for a in range(2):
                        o = fwd4([xloc(sig, a + 2 * r + 8 * k1 + 32 * k0) for r in range(4)], TC + 8 * k)
                        put4_t([(2 * ((k + 16 * k2) // 8) + a, k % 8) for k2 in range(4)], o)
            for kb in range(8):
                for e in range(4):
                    o = fwd4([sloc(kb, e + 4 * r) for r in range(4)], TD + 8 * kb)
                    put4([xloc(sig, 16 * kb + e + 4 * r) for r in range(4)], o)
            for kb in range(8):
                for k3 in range(4):
                    locs = [xloc(sig, 16 * kb + r + 4 * k3) for r in range(4)]
                    t0 = TE + 8 * (4 * kb + k3)
                    o = fwd4(locs, t0)
                    if sig == 0:
                        hs = ld4([xloc(1, 16 * kb + r + 4 * k3) for r in range(4)])
                        o = inv4([_cmul(a, b) for a, b in zip(o, hs)], t0)
                    put4(locs, o)

        def inverse():
            for kb in range(8):
                for e in range(4):
                    o = inv4(ld4([xloc(0, 16 * kb + e + 4 * r) for r in range(4)]), TD + 8 * kb)
                    put4_t([(2 * kb + (e + 4 * f) // 8, (e + 4 * f) % 8) for f in range(4)], o)
            for k0 in range(4):
                for k1 in range(4):
                    k = k0 + 4 * k1
                    for a in range(2):
                        v = ld4([sloc((k + 16 * r) // 8, 8 * a + k % 8) for r in range(4)])
                        put4([xloc(0, a + 2 * b + 8 * k1 + 32 * k0) for b in range(4)], inv4(v, TC + 8 * k))
            for k0 in range(4):
                for n in range(8):
                    locs = [xloc(0, n + 8 * r + 32 * k0) for r in range(4)]
                    put4(locs, inv4(ld4(locs), TB + 8 * k0))
            dskip = taps[g, KS]
            for n0 in range(32):
                cs = _dft4(ld4([xloc(0, n0 + 32 * r) for r in range(4)]), -1)
                outs = []
                for d in [d0 + 4 * hh for d0 in range(4) for hh in range(2)]:
                    n = n0 + 32 * d
                    a = twid(TAI + 2 * d)
                    if 0 < d < 4:
                        cs[d] = tuple(begin(cs[d], 2))
                    c = cs[d % 4]
                    y = c[0] * a[0] if d == 0 else c[0] * a[0] + c[1] * a[1]
                    y = y + jnp.where(j == 0, ld(WK + n) * dskip, ld(WY + n))
                    st(WY + n, y)
                    chain[0] = abuf[sl, 0, pl.ds(8 * n, 8), :].astype(F32) * y
                    aout[g, n // 4, pl.ds(8 * (n % 4), 8), :] = chain[0].astype(BF16)
                    outs.append(chain[0])
                merge(outs)

        def filt(n):
            base = pl.multiple_of(g * (S // 2), S // 2)
            ws = begin([ht[pl.ds(base + 8 * (n // 2 + 16 * d), 8), :] for d in range(8)], 8)
            return [_widen(w)[8 * (n % 2):8 * (n % 2) + 8] for w in ws]
        pass_kv()
        forward(1, filt)
        forward(0, lambda n: begin([ld(WK + n + 32 * d) for d in range(8)], 8))
        inverse()
        return chain[0]

    scale = DH ** (-0.5)

    def w_slab(m, h):
        u = 4 * m + h // 8
        return pltpu.bitcast(w_parts[u % 2][pl.ds(slab_row(u, h % 2, (h // 2) % 4), D // 2), :], BF16)

    class Step:
        def __init__(self, s, prev, mem):
            self.s = s
            self.prev = prev
            self.qkv, self.ps, self.os = {}, {}, []
            self.acc = [None] * NB
            self.ocat, self.lead, self.early, self.marks, self.heads = {}, {}, {}, {}, {}
            self.tie = None
            x = xbuf[s, pl.ds(M, SEG - M), :].astype(F32)
            self.lhsf = jnp.concatenate([mem, x], axis=0)
            self.lhs = self.lhsf.astype(BF16)

        def proj_early(self, m, h, k):
            self.early[m, h] = (k, _dot(self.lhsf[:, :k].astype(BF16), w_slab(m, h)[:k]))

        def proj(self, m, h):
            if (m, h) in self.early:
                k, part = self.early[m, h]
                d = _dot(self.lhsf[:, k:].astype(BF16), w_slab(m, h)[k:]) + part
            else:
                d = _dot(self.lhs, w_slab(m, h))
            self.heads[m, h] = d
            j = h // 2
            if (m, h ^ 1) not in self.heads:
                return
            a, b = self.heads[m, 2 * j], self.heads[m, 2 * j + 1]
            self.marks[m, j] = a[0:8]
            lead = _widen(qkvb[self.s, m * NPAIR + j])
            self.qkv[m, j] = jnp.concatenate([a, b, lead], axis=0).astype(BF16)

        def probs(self, j):
            fill = fill_ref[pl.ds(0, R), pl.ds(0, R)]
            qk = _dot_nt(self.qkv[0, j], self.qkv[1, j])
            sc = jnp.where(fill == 0.0, qk * scale, fill)
            e = jnp.exp(sc - jnp.max(sc, axis=-1, keepdims=True))
            l = jnp.sum(e, axis=-1, keepdims=True)
            r = pl.reciprocal(l, approx=True)
            r = r * (2.0 - l * r)
            self.ps[j] = (e * r).astype(BF16)

        def attend(self, j):
            o = _dot(self.ps[j], self.qkv[2, j])
            la, lb = o[2 * SEG:2 * SEG + M], o[2 * SEG + M:]
            rows = pl.ds(pl.multiple_of((self.s >> 1) * M, M), M)
            if self.prev is None:
                self.lead[j] = (la, lb)
                forms = {2: la + lb, 5: la}
            else:
                a11, a12 = self.prev.lead[j]
                forms = {0: a11 + lb, 1: la + lb, 3: la - a11, 4: a12 - lb, 6: lb}
            for f, v in forms.items():
                ob[f * NPAIR + j, rows, :] = v.astype(BF16)
            self.os += [o[0:SEG], o[SEG:2 * SEG]]

        def wo(self, h0, h1, n):
            if h0 not in self.ocat:
                self.ocat[h0] = jnp.concatenate(self.os[h0:h1], axis=1).astype(BF16)
            w = wo_u[n, pl.ds(h0 * 64, (h1 - h0) * 64), :]
            if self.tie is not None:
                w = jnp.concatenate(
                    [jnp.where(self.s > 1000, pltpu.bitcast(self.tie, U32), w[0:8]), w[8:]], axis=0)
                self.tie = None
            d = _dot(self.ocat[h0], pltpu.bitcast(w, BF16))
            self.acc[n] = d if self.acc[n] is None else d + self.acc[n]

        def finish(self):
            res = jnp.concatenate(self.acc, axis=1)
            obuf[self.s] = res.astype(BF16)
            return res[0:M]

    def steps(i, mem):
        sts = []
        for u in range(U):
            st = Step(i * U + u, sts[-1] if u % 2 else None, mem)
            sts.append(st)
            for item in _step_order(u, cfg):
                if item[0] == "A":
                    ku, km, kj = cfg["kick"]
                    st.tie = part_a(i, sts[ku].marks[km, kj])
                else:
                    dict(P=st.proj, E=st.proj_early, S=st.probs, V=st.attend, W=st.wo)[item[0]](*item[1:])
            mem = st.finish()
        return mem

    def group(g, mem):
        x_copy(g).wait()
        self_wait(abuf.at[g & 1], SA + (g & 1))

        @pl.when(jnp.logical_and(g >= 1, g < NG - 1))
        def _():
            a_start(g + 1)
        return lax.fori_loop(0, 2, lambda j, m_: steps(2 * g + j, m_), mem)

    tw_cp.wait()
    lax.fori_loop(0, NG, group, mem0_ref[...].astype(F32))

    ob_cp = pltpu.make_async_copy(
        obuf.at[:, pl.ds(M, SEG - M), :],
        out_hbm.at[:, pl.ds(M, SEG - M), pl.ds(D, D)], sems.at[SO])
    ob_cp.start()
    for g in range(NG):
        pltpu.make_async_copy(
            aout.at[g], out_hbm.at[:, :, pl.ds(g * 128, 128)], sems.at[SO + 1]).start()

    def epi(it, carry):
        ns = [2 * it, 2 * it + 1]

        def blk(hp, u):
            return [wo_u[ns[u], pl.ds((2 * j + hp) * 64, 64), :] for j in range(NPAIR)]

        def mm(f, bs):
            lhs = jnp.concatenate([ob[f * NPAIR + j] for j in range(NPAIR)], axis=1)
            return _dot(lhs, as_bf16(jnp.concatenate(bs, axis=0)))

        def cb(x, y, sign):
            return [comb(a, b, sign) for a, b in zip(x, y)]

        def put(u, par, c):
            for i in range(NSEG // 2):
                obb[ns[u], 2 * i + par] = c[M * i:M * i + M].astype(BF16)
        m5 = mm(2, blk(1, 1))
        m1 = mm(0, cb(blk(0, 0), blk(1, 1), 1))
        m4 = mm(6, cb(blk(1, 0), blk(0, 0), -1))
        put(0, 0, mm(4, cb(blk(1, 0), blk(1, 1), 1)) + (m1 + m4 - m5))
        m3 = mm(5, cb(blk(0, 1), blk(1, 1), -1))
        put(1, 0, m3 + m5)
        m2 = mm(1, blk(0, 0))
        put(0, 1, m2 + m4)

        def send(n):
            col = pl.multiple_of(D + n * 128, 128)
            pltpu.make_async_copy(
                obb.at[n], out_hbm.at[:, pl.ds(0, M), pl.ds(col, 128)], sems.at[SO + 2]).start()
        send(ns[0])
        put(1, 1, mm(3, cb(blk(0, 0), blk(0, 1), 1)) + (m1 - m2 + m3))
        send(ns[1])
        return carry
    lax.fori_loop(0, NB // 2, epi, 0)
    ob_cp.wait()
    self_wait(aout, SO + 1)
    self_wait(obb, SO + 2)


def _step_order(u, cfg):
    ks = cfg["ks"]
    tmpl = []
    for x in cfg["tmpl"].split():
        kind, lag = x[:-1], int(x[-1])
        tmpl += [(kind + "a", lag), (kind + "b", lag)] if kind in ("q", "k", "v") else [(kind, lag)]

    def proj(kind, j):
        return ("qkv".index(kind[0]), 2 * j + "ab".index(kind[1]))
    out = []
    nw = 0
    for t in range(NPAIR + 1 + max(l for _, l in tmpl)):
        for kind, lag in tmpl:
            j = t - lag
            if j < 0:
                continue
            if j >= NPAIR:
                if kind[1:] == "a" and nw < NB:
                    out.append(("W", 0, ks, nw))
                    nw += 1
                continue
            out.append(("P",) + proj(kind, j) if len(kind) == 2 else (kind, j))
    if u > 0:
        first = [x[1:] for x in out if x[0] == "P"][:cfg["ne"]]
        out = [("E",) + x + (cfg["ek"],) for x in first] + out
    out += [("W", 0, ks, n) for n in range(nw, NB)]
    for n in range(NB):
        if u == U - 1 and n == cfg["tie_n"]:
            out.append(("A",))
        out.append(("W", ks, H, n))
    return out


_DEFAULT_CFG = dict(
    tmpl='V3 ka0 kb0 va1 S1 qa0 qb0 vb1', ks=16, ne=5, ek=768,
    tie_n=7, kick=(0, 0, 0), a_merge=5, a_g4=8, a_g4i=2)


def _build(cfg):
    tw_np = _twiddles()
    fill_np = np.zeros((96, 128), np.float32)
    fill_np[:R, :R] = _mask_fill()

    def run(A_q, A_k, A_v, A_shift_k, A_ssm_k, A_ssm_D, B_x, B_mem0, B_Wq, B_Wk, B_Wv, B_Wo):
        sk = A_shift_k.T.reshape(KS, NG, 128).transpose(1, 0, 2)
        any_spec = pl.BlockSpec(memory_space=pl.ANY)
        out = pl.pallas_call(
            functools.partial(_kernel, cfg),
            out_shape=jax.ShapeDtypeStruct((NSEG, SEG, 2 * D), BF16),
            in_specs=[any_spec] * 14,
            out_specs=any_spec,
            scratch_shapes=[
                pltpu.VMEM((48 * SLAB + 544, 128), U32),
                pltpu.VMEM((48 * SLAB + 544, 128), U32),
                pltpu.VMEM((NB, H * DH // 2, 128), U32),
                pltpu.VMEM((4, D, 8, DH), BF16),
                pltpu.VMEM((9, 512, D), BF16),
                pltpu.VMEM((NSEG, SEG, D), BF16),
                pltpu.VMEM((4, NSEG, M, KQ), BF16),
                pltpu.VMEM((4, NSEG * M // 2, KQ), U32),
                pltpu.VMEM((5, 2, HR, KQ), U32),
                pltpu.VMEM((NSEG, 3 * NPAIR, 8, 128), U32),
                pltpu.VMEM((7 * NPAIR, NSEG * M // 2, DH), BF16),
                pltpu.VMEM((NSEG, SEG, D), BF16),
                pltpu.VMEM((NB, NSEG, M, 128), BF16),
                pltpu.VMEM((2, 3, S, 128), BF16),
                pltpu.VMEM((NG + 1, 128, S), BF16),
                pltpu.VMEM((NG * S // 2, 128), U32),
                pltpu.VMEM((8 * NW + 32, 128), F32),
                pltpu.VMEM((2, NT, 8, 128), F32),
                pltpu.VMEM((NG, NSEG, SEG, 128), BF16),
                pltpu.VMEM((4, 8, 128), F32),
                pltpu.VMEM((96, 128), F32),
                pltpu.VMEM((NG, 8, 8, 128), F32),
                pltpu.VMEM((M, D), BF16),
                pltpu.VMEM((NG, KS, 128), BF16),
                pltpu.VMEM((4, NG, 128), BF16),
                pltpu.SemaphoreType.DMA((56,)),
            ],
            compiler_params=pltpu.CompilerParams(vmem_limit_bytes=124 * 1024 * 1024,
                                                 disable_bounds_checks=True),
        )(A_q.reshape(S, D), A_k.reshape(S, D), A_v.reshape(S, D), sk, A_ssm_k,
          A_ssm_D.reshape(NG, 128), B_x.reshape(NSEG, SEG, D), B_mem0.reshape(M, D),
          B_Wq, B_Wk, B_Wv, B_Wo.reshape(H * DH, D),
          jnp.asarray(tw_np), jnp.asarray(fill_np))
        return out.reshape(1, S, 2 * D)

    return run


@functools.partial(jax.jit, static_argnames=("B_seg_len",))
def pallas_concat_heads__ssm_conv_h3__memory_aug_recurrent_mem_tr__prompt_kernel(
    A_q: jax.Array,
    A_k: jax.Array,
    A_v: jax.Array,
    A_shift_k: jax.Array,
    A_ssm_k: jax.Array,
    A_ssm_D: jax.Array,
    B_x: jax.Array,
    B_mem0: jax.Array,
    B_Wq: jax.Array,
    B_Wk: jax.Array,
    B_Wv: jax.Array,
    B_Wo: jax.Array,
    B_seg_len: int = SEG,
):
    assert B_seg_len == SEG
    return _build(_DEFAULT_CFG)(A_q, A_k, A_v, A_shift_k, A_ssm_k, A_ssm_D, B_x, B_mem0,
                                B_Wq, B_Wk, B_Wv, B_Wo)
```

```python
import functools

import numpy as np
import jax
import jax.numpy as jnp
from jax import lax
import jax.experimental.pallas as pl
import jax.experimental.pallas.tpu as pltpu

F32 = jnp.float32
BF16 = jnp.bfloat16
U32 = jnp.uint32

S = 2048
D = 1024
H = 32
DH = 128
M = 8
SEG = 32
NSEG = S // SEG
U = 4
NPAIR = H // 2
R = 2 * (M + SEG)
SLAB = 520
KS = 4
NG = D // 128
KQ = D // 4
NB = D // 128
HR = NSEG * M // 4

TAF, TAI, TB, TC, TD, TE, NT = 0, 16, 32, 64, 192, 256, 512
WX, WS, WY, WK, NW = 0, 512, 1024, 1280, 1536


def _twiddles():
    tw = np.zeros((2, NT, 8), np.float64)

    def put(j, idx, z):
        tw[j, idx] = np.real(z)
        tw[j, idx + 1] = np.imag(z)
    s = np.arange(8)
    tau = 2j * np.pi
    for j in range(2):
        lx = 1j * np.pi * (1 + 4 * j) / 4096
        for d in range(8):
            put(j, TAF + 2 * d, np.exp(lx * 256 * d))
            put(j, TAI + 2 * d, np.exp(lx * 256 * d) / 2048)
        for r in range(4):
            for k in range(4):
                put(j, TB + 8 * k + 2 * r, np.exp((lx * 64 + tau * k / 16) * r))
            for k in range(16):
                put(j, TC + 8 * k + 2 * r, np.exp((lx * 16 + tau * k / 64) * r))
            for kb in range(8):
                put(j, TD + 8 * kb + 2 * r, np.exp((lx * 4 + tau * (s + 8 * kb) / 256) * r))
                for k3 in range(4):
                    put(j, TE + 8 * (4 * kb + k3) + 2 * r,
                        np.exp((lx + tau * (s + 8 * kb + 64 * k3) / 1024) * r))
    return np.ascontiguousarray(np.broadcast_to(tw[..., None], (2, NT, 8, 128))).astype(np.float32)


def _mask_fill():
    blk = np.concatenate([np.arange(M), M + np.arange(M, SEG)])
    lead = M + np.arange(M)
    head = np.concatenate([np.zeros(SEG), np.ones(SEG), np.zeros(M), np.ones(M)])
    pos = np.concatenate([blk, blk, lead, lead])
    same = head[:, None] == head[None, :]
    ok = (pos[:, None] < M) | (pos[:, None] >= pos[None, :])
    fill = np.where(same, np.where(ok, 0.0, -1e9), -np.inf)
    return fill.astype(np.float32)


def _widen(w):
    return pltpu.bitcast(w, BF16).astype(F32)


def _narrow(x):
    return pltpu.bitcast(x.astype(BF16), U32)


def _dot(a, b):
    return jnp.dot(a, b, preferred_element_type=F32)


def _dot_nt(a, b):
    return lax.dot_general(a, b, (((1,), (1,)), ((), ())), preferred_element_type=F32)


def _cadd(a, b):
    return (a[0] + b[0], a[1] + b[1])


def _csub(a, b):
    return (a[0] - b[0], a[1] - b[1])


def _cmul(a, w):
    return (a[0] * w[0] - a[1] * w[1], a[0] * w[1] + a[1] * w[0])


def _cmulc(a, w):
    return (a[0] * w[0] + a[1] * w[1], a[1] * w[0] - a[0] * w[1])


def _bfly_i(b, d, sg):
    p = (b[0] - d[1], b[1] + d[0])
    q = (b[0] + d[1], b[1] - d[0])
    return (p, q) if sg > 0 else (q, p)


def _dft4(x, sg):
    a, b = _cadd(x[0], x[2]), _csub(x[0], x[2])
    c, d = _cadd(x[1], x[3]), _csub(x[1], x[3])
    p, q = _bfly_i(b, d, sg)
    return [_cadd(a, c), p, _csub(a, c), q]


def _kernel(cfg,
            aq_hbm, ak_hbm, av_hbm, sk_hbm, ssmk_hbm, ssmd_hbm, x_hbm, mem0_hbm,
            wq_hbm, wk_hbm, wv_hbm, wo_hbm, tw_hbm, fill_hbm,
            out_hbm,
            w_a, w_b, wo_u, wstage, wostage, xbuf, xlead, xlead_u, xs_u, qkvb, ob, obuf, obb,
            abuf, hbuf, ht, wk, tw, aout, kickbuf,
            fill_ref, taps, mem0_ref, sk_ref, ssmd_ref,
            sems):
    SW, SWO, SXL, SX, SH, SA, ST, SO, SS = 0, 16, 24, 28, 36, 44, 46, 48, 52
    w_hbms = (wq_hbm, wk_hbm, wv_hbm)
    a_hbms = (aq_hbm, ak_hbm, av_hbm)

    def aligned(x, n):
        return x if isinstance(x, int) else pl.multiple_of(x, n)

    def w_copy(m, hq, q=None):
        rows = pl.ds(0, D) if q is None else pl.ds(q * KQ, KQ)
        sem = SW + 12 + hq if q is None else SW + 4 * hq + q
        heads = aligned(8 * hq, 8)
        return pltpu.make_async_copy(
            w_hbms[m].at[rows, pl.ds(heads, 8), :], wstage.at[hq, rows], sems.at[sem])

    def self_wait(ref, sem):
        pltpu.make_async_copy(ref, ref, sems.at[sem]).wait()

    def late_start(k):
        pltpu.make_async_copy(
            wo_hbm.at[pl.ds(aligned(k * 512, 512), 512), :], wostage.at[k],
            sems.at[SWO + k]).start()
        pltpu.make_async_copy(
            ssmk_hbm.at[pl.ds(aligned(k * 128, 128), 128), :], hbuf.at[k],
            sems.at[SH + k]).start()

    def xlead_copy(q):
        return pltpu.make_async_copy(
            x_hbm.at[:, pl.ds(0, M), pl.ds(q * KQ, KQ)], xlead.at[q], sems.at[SXL + q])

    def x_copy(g):
        segs = pl.ds(g * 8, 8)
        return pltpu.make_async_copy(
            x_hbm.at[segs, pl.ds(M, SEG - M), :], xbuf.at[segs, pl.ds(M, SEG - M), :], sems.at[SX + g])

    def a_start(g):
        col = aligned(g * 128, 128)
        for t in (1, 2, 0):
            pltpu.make_async_copy(
                a_hbms[t].at[:, pl.ds(col, 128)], abuf.at[g & 1, t], sems.at[SA + (g & 1)]).start()

    tw_cp = pltpu.make_async_copy(tw_hbm, tw, sems.at[ST])

    small = [pltpu.make_async_copy(src, dst, sems.at[SS + i]) for i, (src, dst) in enumerate((
        (fill_hbm, fill_ref), (mem0_hbm, mem0_ref), (sk_hbm, sk_ref), (ssmd_hbm, ssmd_ref.at[0])))]

    for q in range(4):
        xlead_copy(q).start()
        w_copy(0, 0, q).start()
        if q > 0:
            w_copy(0, 1, q - 1).start()
    w_copy(0, 1, 3).start()
    for q in range(4):
        w_copy(0, 2, q).start()
    w_copy(0, 3).start()
    for cp in small:
        cp.start()

    kickbuf[...] = jnp.zeros(kickbuf.shape, F32)

    w_parts = (w_a, w_b)

    def slab_row(u, par, jl):
        return ((u >> 1) * 8 + par * 4 + jl) * SLAB

    def gated(x, i, n, gates):
        if gates is None:
            return x
        never, vals = gates
        v = vals[(i * len(vals) * 3) // (n * 4)]
        return jnp.where(never, pltpu.bitcast(v, U32), x)

    def vregs(*mats):
        return [m_[r:r + 8] for m_ in mats for r in range(0, m_.shape[0], 8)]

    def relayout(u, g, q, gates=None, src=None):
        slot, qs = (u & 3, q) if src is None else src
        low = lax.broadcasted_iota(jnp.int32, (8, 128), 0) < 4
        keep = jnp.where(low, jnp.uint32(0xFFFF), jnp.uint32(0xFFFF0000))
        shl = jnp.where(low, jnp.uint32(16), jnp.uint32(0))
        base = slab_row(u, 0, 0) + q * (KQ // 2)
        for i in range(KQ // 2):
            x = wstage[slot, pl.ds(qs * KQ + 2 * i, 2)].reshape(16, DH)
            x = gated(pltpu.bitcast(x, U32), i, KQ // 2, gates)
            y = pltpu.roll(x, 4, 0)
            w_parts[g][pl.ds(base + i, 8, stride=SLAB), :] = (x & keep) | ((y << shl) >> (16 - shl))

    def comb(x, y, sign):
        return _widen(x) + _widen(y) if sign > 0 else _widen(x) - _widen(y)

    def as_bf16(b):
        return pltpu.bitcast(b, BF16) if b.dtype == U32 else b.astype(BF16)

    def put_lead(segs, n, it, a, b):
        both = jnp.concatenate([a.reshape(n, M, DH), b.reshape(n, M, DH)], axis=1)
        qkvb[segs, it] = _narrow(both)

    def batch_pair(u, g, jl):
        it = 4 * u + jl
        rows = [pl.multiple_of(slab_row(u, par, jl), 8) for par in range(2)]

        def blk(kh, par):
            return w_parts[g][pl.ds(rows[par] + kh * (D // 4), D // 4), :]

        def mm(a, b):
            return _dot(pltpu.bitcast(jnp.concatenate(a, axis=1), BF16), as_bf16(b))

        def xs(f):
            return [xs_u[f, q] for q in range(2)]
        a11 = [xlead_u[q, pl.ds(0, HR), :] for q in (0, 1)]
        a22 = [xlead_u[q, pl.ds(HR, HR), :] for q in (2, 3)]
        m5 = mm(xs(2), blk(1, 1))
        m1 = mm(xs(0), comb(blk(0, 0), blk(1, 1), 1))
        m4 = mm(a22, comb(blk(1, 0), blk(0, 0), -1))
        c11 = mm(xs(4), comb(blk(1, 0), blk(1, 1), 1)) + (m1 + m4 - m5)
        m3 = mm(a11, comb(blk(0, 1), blk(1, 1), -1))
        put_lead(pl.ds(0, NSEG // 2), NSEG // 2, it, c11, m3 + m5)
        m2 = mm(xs(1), blk(0, 0))
        c22 = mm(xs(3), comb(blk(0, 0), blk(0, 1), 1)) + (m1 - m2 + m3)
        put_lead(pl.ds(NSEG // 2, NSEG // 2), NSEG // 2, it, m2 + m4, c22)
        return vregs(m5, m1, m4, c11, m3, m2, c22)

    def quarter_wait(u, q):
        self_wait(wstage.at[u, pl.ds(pl.multiple_of(q * KQ, KQ), KQ)], SW + 4 * u + q)

    def first_unit(q, carry):
        never = q > 1000
        half = q & 1
        self_wait(xlead.at[q], SXL + q)
        quarter_wait(0, q)
        xlead_u[q] = _narrow(xlead[q].astype(F32).reshape(NSEG * M, KQ))
        relayout(0, 0, q)

        @pl.when(q > 0)
        def _():
            quarter_wait(1, q - 1)
        res = []
        xq = pltpu.bitcast(xlead_u[q], BF16)
        for jl in range(4):
            outs = []
            for par in range(2):
                acc = pl.ds((2 * jl + par) * (NSEG * M), NSEG * M)
                row = pl.multiple_of(slab_row(0, par, jl) + q * (KQ // 2), 8)
                w = pltpu.bitcast(w_a[pl.ds(row, KQ // 2), :], BF16)
                d = _dot(xq, w) + jnp.where(q == 0, 0.0, wk[acc, :])
                wk[acc, :] = d
                outs.append(d)
            put_lead(pl.ds(0, NSEG), NSEG, jl, outs[0], outs[1])
            res += outs
        gates = (never, vregs(*res))
        qn = jnp.maximum(q - 1, 0)
        relayout(1, 1, qn, gates, src=(jnp.minimum(q, 1), qn))
        for r in range(0, HR, 8):
            for cb in range(2):
                cols = pl.ds(cb * 128, 128)
                i = 2 * (r // 8) + cb
                a11 = gated(xlead_u[half, pl.ds(r, 8), cols], i, HR // 4, gates)
                a22 = gated(xlead_u[2 + half, pl.ds(HR + r, 8), cols], i, HR // 4, gates)
                a21 = xlead_u[half, pl.ds(HR + r, 8), cols]
                a12 = xlead_u[2 + half, pl.ds(r, 8), cols]
                for f, (x, y, sg) in enumerate(((a11, a22, 1), (a21, a22, 1), (a11, a12, 1),
                                                (a21, a11, -1), (a12, a22, -1))):
                    xs_u[f, half, pl.ds(r, 8), cols] = _narrow(comb(x, y, sg))
        return carry
    lax.fori_loop(0, 4, first_unit, 0)
    w_copy(1, 0).start()
    late_start(0)
    w_copy(0, 1, 3).wait()
    relayout(1, 1, 3)

    def second_unit(jl, carry):
        quarter_wait(2, jl)
        relayout(2, 0, jl, (jl > 1000, batch_pair(1, 1, jl)))
        return carry
    lax.fori_loop(0, 4, second_unit, 0)

    def late_relayout(src, hp, half, gates):
        for r in range(16):
            blk = pltpu.bitcast(wostage[src, pl.ds(half * 256 + r * 16, 16), :], U32)
            row = pl.multiple_of(hp * 128 + r * 8, 8)
            for n in range(NB):
                wo_u[n, pl.ds(row, 8), :] = gated(blk[:, n * 128:(n + 1) * 128], r * NB + n, 16 * NB, gates)
        for t in range(8):
            tile = pltpu.bitcast(hbuf[src, :, pl.ds((8 * half + t) * 128, 128)], U32)
            tile = jnp.concatenate([gated(tile[0:8], t, 8, gates), tile[8:]], axis=0)
            row = pl.multiple_of(hp * 512 + t * 64, 64)
            ht[pl.ds(row, 64), :] = pltpu.bitcast(pltpu.bitcast(tile, BF16).T, U32)

    def unit_body(u, g):
        @pl.when(u < 11)
        def _():
            self_wait(wstage.at[(u + 1) & 3], SW + 12 + ((u + 1) & 3))

        @pl.when(u >= 8)
        def _():
            for e in range(2):
                k = (u - 8) * 2 + e
                self_wait(wostage.at[k], SWO + k)
                self_wait(hbuf.at[k], SH + k)
        for m in (1, 2):
            @pl.when((u + 3) >> 2 == m)
            def _():
                w_copy(m, (u + 3) & 3).start()

        @pl.when(u <= 8)
        def _():
            late_start(u - 1)
        if g == 1:
            @pl.when(u == 9)
            def _():
                x_copy(0).start()
                a_start(0)
                tw_cp.start()
        for jl in range(4):
            gates = (u > 1000, batch_pair(u, g, jl))
            relayout(jnp.where(u < 11, u + 1, u - 1), 1 - g, jl, gates)
            k = jnp.maximum(u - 8, 0) * 2 + jl // 2
            late_relayout(jnp.where(u >= 8, k, 8), 2 * k + jl % 2, jl % 2, gates)

    def unit_pair(mm, carry):
        for g in range(2):
            unit_body(2 * mm + g, g)
        return carry
    lax.fori_loop(1, 6, unit_pair, 0)

    a_start(1)
    for g in range(1, NG):
        x_copy(g).start()
    for cp in small:
        cp.wait()
    dd = ssmd_ref[0].astype(F32)
    for g in range(NG):
        sk = sk_ref[g].astype(F32)
        for j in range(KS):
            taps[g, j] = jnp.broadcast_to(sk[j:j + 1], (8, 128))
        taps[g, KS] = jnp.broadcast_to(dd[g:g + 1], (8, 128))

    def part_a(i, kick):
        g, j = i >> 1, i & 1
        sl = g & 1
        never = i > 1000
        sub = lax.broadcasted_iota(jnp.int32, (8, 128), 0)
        kickbuf[jnp.where(never, 1, 0)] = kick
        chain = [kickbuf[jnp.where(i > 2000, 0, 1)]]

        def begin(xs, ng):
            xs = list(xs)
            for e in range(min(ng, len(xs))):
                c = chain[0]
                c = c if c.dtype == xs[e].dtype else pltpu.bitcast(c, xs[e].dtype)
                xs[e] = jnp.where(never, c, xs[e])
            return xs

        def merge(vals):
            c = vals[-1]
            for v in list(vals[:-1])[:cfg["a_merge"]]:
                c = jnp.maximum(v, c)
            chain[0] = c

        def ld(v):
            if isinstance(v, tuple):
                blk, ri, r = v
                base = 8 * WS + 256 * blk + 16 * ri + 32 * r
                lo = wk[pl.ds(base, 8), :]
                if r == 0:
                    return lo
                return pltpu.roll(jnp.where(sub >= r, lo, wk[pl.ds(base + 8, 8), :]), 8 - r, 0)
            return wk[pl.ds(8 * v, 8), :]

        def st(v, x):
            wk[pl.ds(8 * v, 8), :] = x

        def twid(idx):
            return (tw[j, idx], tw[j, idx + 1])

        def pairs(flat):
            return [(flat[2 * e], flat[2 * e + 1]) for e in range(len(flat) // 2)]

        def fwd4(locs, t0):
            v = pairs(begin([ld(x) for loc in locs[::-1] for x in loc], cfg["a_g4"]))[::-1]
            return _dft4([v[0]] + [_cmul(v[r], twid(t0 + 2 * r)) for r in range(1, 4)], +1)

        def inv4(v, t0):
            o = _dft4(v, -1)
            return [o[0]] + [_cmulc(o[r], twid(t0 + 2 * r)) for r in range(1, 4)]

        def ld4(locs):
            return pairs(begin([ld(x) for loc in locs for x in loc], cfg["a_g4i"]))

        def put4(locs, o):
            for loc, x in zip(locs, o):
                st(loc[0], x[0])
                st(loc[1], x[1])
            merge([x for c in o for x in c])

        def put4_t(dsts, o):
            for (blk, slot), x in zip(dsts, o):
                for ri in range(2):
                    base = 8 * WS + 256 * blk + 16 * ri + slot
                    wk[pl.ds(base, 8, stride=33), :] = x[ri]
            merge([x for c in o for x in c])

        def xloc(sig, n):
            return (WX + 256 * sig + 2 * n, WX + 256 * sig + 2 * n + 1)

        def sloc(kb, l):
            return ((2 * kb + l // 8, 0, l % 8), (2 * kb + l // 8, 1, l % 8))

        def pass_kv():
            t = [taps[g, a] for a in range(KS)]
            prev = [None] + [jnp.zeros((8, 128), F32)] * (KS - 1)
            for v in range(S // 16):
                w, = begin([pltpu.bitcast(abuf[sl, 1, pl.ds(16 * v, 16), :], U32)], 1)
                k2 = _widen(w)
                v2 = abuf[sl, 2, pl.ds(16 * v, 16), :].astype(F32)
                outs = []
                for hh in range(2):
                    x = k2[8 * hh:8 * hh + 8]
                    cur = [None] + [pltpu.roll(x, a, 0) for a in range(1, KS)]
                    ks = x * t[0]
                    for a in range(1, KS):
                        ks = ks + jnp.where(sub < a, prev[a], cur[a]) * t[a]
                    prev = cur
                    kv = (ks * v2[8 * hh:8 * hh + 8]).astype(BF16).astype(F32)
                    st(WK + 2 * v + hh, kv)
                    outs.append(kv)
                merge(outs)

        def forward(sig, src):
            for n in range(32):
                x = src(n)
                cs = []
                for d in range(4):
                    a, b = twid(TAF + 2 * d), twid(TAF + 2 * (d + 4))
                    if d == 0:
                        s_ = x[4] * b[0]
                        cs.append((x[0] + s_, s_))
                    else:
                        cs.append((x[d] * a[0] + x[d + 4] * b[0], x[d] * a[1] + x[d + 4] * b[1]))
                put4([xloc(sig, n + 32 * k0) for k0 in range(4)], _dft4(cs, +1))
            for k0 in range(4):
                for n in range(8):
                    locs = [xloc(sig, n + 8 * r + 32 * k0) for r in range(4)]
                    put4(locs, fwd4(locs, TB + 8 * k0))
            for k0 in range(4):
                for k1 in range(4):
                    k = k0 + 4 * k1
                    for a in range(2):
                        o = fwd4([xloc(sig, a + 2 * r + 8 * k1 + 32 * k0) for r in range(4)], TC + 8 * k)
                        put4_t([(2 * ((k + 16 * k2) // 8) + a, k % 8) for k2 in range(4)], o)
            for kb in range(8):
                for e in range(4):
                    o = fwd4([sloc(kb, e + 4 * r) for r in range(4)], TD + 8 * kb)
                    put4([xloc(sig, 16 * kb + e + 4 * r) for r in range(4)], o)
            for kb in range(8):
                for k3 in range(4):
                    locs = [xloc(sig, 16 * kb + r + 4 * k3) for r in range(4)]
                    t0 = TE + 8 * (4 * kb + k3)
                    o = fwd4(locs, t0)
                    if sig == 0:
                        hs = ld4([xloc(1, 16 * kb + r + 4 * k3) for r in range(4)])
                        o = inv4([_cmul(a, b) for a, b in zip(o, hs)], t0)
                    put4(locs, o)

        def inverse():
            for kb in range(8):
                for e in range(4):
                    o = inv4(ld4([xloc(0, 16 * kb + e + 4 * r) for r in range(4)]), TD + 8 * kb)
                    put4_t([(2 * kb + (e + 4 * f) // 8, (e + 4 * f) % 8) for f in range(4)], o)
            for k0 in range(4):
                for k1 in range(4):
                    k = k0 + 4 * k1
                    for a in range(2):
                        v = ld4([sloc((k + 16 * r) // 8, 8 * a + k % 8) for r in range(4)])
                        put4([xloc(0, a + 2 * b + 8 * k1 + 32 * k0) for b in range(4)], inv4(v, TC + 8 * k))
            for k0 in range(4):
                for n in range(8):
                    locs = [xloc(0, n + 8 * r + 32 * k0) for r in range(4)]
                    put4(locs, inv4(ld4(locs), TB + 8 * k0))
            dskip = taps[g, KS]
            for n0 in range(32):
                cs = _dft4(ld4([xloc(0, n0 + 32 * r) for r in range(4)]), -1)
                outs = []
                for d in [d0 + 4 * hh for d0 in range(4) for hh in range(2)]:
                    n = n0 + 32 * d
                    a = twid(TAI + 2 * d)
                    if 0 < d < 4:
                        cs[d] = tuple(begin(cs[d], 2))
                    c = cs[d % 4]
                    y = c[0] * a[0] if d == 0 else c[0] * a[0] + c[1] * a[1]
                    y = y + jnp.where(j == 0, ld(WK + n) * dskip, ld(WY + n))
                    st(WY + n, y)
                    chain[0] = abuf[sl, 0, pl.ds(8 * n, 8), :].astype(F32) * y
                    aout[g, n // 4, pl.ds(8 * (n % 4), 8), :] = chain[0].astype(BF16)
                    outs.append(chain[0])
                merge(outs)

        def filt(n):
            base = pl.multiple_of(g * (S // 2), S // 2)
            ws = begin([ht[pl.ds(base + 8 * (n // 2 + 16 * d), 8), :] for d in range(8)], 8)
            return [_widen(w)[8 * (n % 2):8 * (n % 2) + 8] for w in ws]
        pass_kv()
        forward(1, filt)
        forward(0, lambda n: begin([ld(WK + n + 32 * d) for d in range(8)], 8))
        inverse()
        return chain[0]

    scale = DH ** (-0.5)

    def w_slab(m, h):
        u = 4 * m + h // 8
        return pltpu.bitcast(w_parts[u % 2][pl.ds(slab_row(u, h % 2, (h // 2) % 4), D // 2), :], BF16)

    class Step:
        def __init__(self, s, prev, mem):
            self.s = s
            self.prev = prev
            self.qkv, self.ps, self.os = {}, {}, []
            self.acc = [None] * NB
            self.ocat, self.lead, self.early, self.marks, self.heads = {}, {}, {}, {}, {}
            self.tie = None
            x = xbuf[s, pl.ds(M, SEG - M), :].astype(F32)
            self.lhsf = jnp.concatenate([mem, x], axis=0)
            self.lhs = self.lhsf.astype(BF16)

        def proj_early(self, m, h, k):
            self.early[m, h] = (k, _dot(self.lhsf[:, :k].astype(BF16), w_slab(m, h)[:k]))

        def proj(self, m, h):
            if (m, h) in self.early:
                k, part = self.early[m, h]
                d = _dot(self.lhsf[:, k:].astype(BF16), w_slab(m, h)[k:]) + part
            else:
                d = _dot(self.lhs, w_slab(m, h))
            self.heads[m, h] = d
            j = h // 2
            if (m, h ^ 1) not in self.heads:
                return
            a, b = self.heads[m, 2 * j], self.heads[m, 2 * j + 1]
            self.marks[m, j] = a[0:8]
            lead = _widen(qkvb[self.s, m * NPAIR + j])
            self.qkv[m, j] = jnp.concatenate([a, b, lead], axis=0).astype(BF16)

        def probs(self, j):
            fill = fill_ref[pl.ds(0, R), pl.ds(0, R)]
            qk = _dot_nt(self.qkv[0, j], self.qkv[1, j])
            sc = jnp.where(fill == 0.0, qk * scale, fill)
            e = jnp.exp(sc - jnp.max(sc, axis=-1, keepdims=True))
            l = jnp.sum(e, axis=-1, keepdims=True)
            r = pl.reciprocal(l, approx=True)
            r = r * (2.0 - l * r)
            self.ps[j] = (e * r).astype(BF16)

        def attend(self, j):
            o = _dot(self.ps[j], self.qkv[2, j])
            la, lb = o[2 * SEG:2 * SEG + M], o[2 * SEG + M:]
            rows = pl.ds(pl.multiple_of((self.s >> 1) * M, M), M)
            if self.prev is None:
                self.lead[j] = (la, lb)
                forms = {2: la + lb, 5: la}
            else:
                a11, a12 = self.prev.lead[j]
                forms = {0: a11 + lb, 1: la + lb, 3: la - a11, 4: a12 - lb, 6: lb}
            for f, v in forms.items():
                ob[f * NPAIR + j, rows, :] = v.astype(BF16)
            self.os += [o[0:SEG], o[SEG:2 * SEG]]

        def wo(self, h0, h1, n):
            if h0 not in self.ocat:
                self.ocat[h0] = jnp.concatenate(self.os[h0:h1], axis=1).astype(BF16)
            w = wo_u[n, pl.ds(h0 * 64, (h1 - h0) * 64), :]
            if self.tie is not None:
                w = jnp.concatenate(
                    [jnp.where(self.s > 1000, pltpu.bitcast(self.tie, U32), w[0:8]), w[8:]], axis=0)
                self.tie = None
            d = _dot(self.ocat[h0], pltpu.bitcast(w, BF16))
            self.acc[n] = d if self.acc[n] is None else d + self.acc[n]

        def finish(self):
            res = jnp.concatenate(self.acc, axis=1)
            obuf[self.s] = res.astype(BF16)
            return res[0:M]

    def steps(i, mem):
        sts = []
        for u in range(U):
            st = Step(i * U + u, sts[-1] if u % 2 else None, mem)
            sts.append(st)
            for item in _step_order(u, cfg):
                if item[0] == "A":
                    ku, km, kj = cfg["kick"]
                    st.tie = part_a(i, sts[ku].marks[km, kj])
                else:
                    dict(P=st.proj, E=st.proj_early, S=st.probs, V=st.attend, W=st.wo)[item[0]](*item[1:])
            mem = st.finish()
        return mem

    def group(g, mem):
        x_copy(g).wait()
        self_wait(abuf.at[g & 1], SA + (g & 1))

        @pl.when(jnp.logical_and(g >= 1, g < NG - 1))
        def _():
            a_start(g + 1)
        return lax.fori_loop(0, 2, lambda j, m_: steps(2 * g + j, m_), mem)

    tw_cp.wait()
    lax.fori_loop(0, NG, group, mem0_ref[...].astype(F32))

    ob_cp = pltpu.make_async_copy(
        obuf.at[:, pl.ds(M, SEG - M), :],
        out_hbm.at[:, pl.ds(M, SEG - M), pl.ds(D, D)], sems.at[SO])
    ob_cp.start()
    for g in range(NG):
        pltpu.make_async_copy(
            aout.at[g], out_hbm.at[:, :, pl.ds(g * 128, 128)], sems.at[SO + 1]).start()

    def epi(it, carry):
        ns = [2 * it, 2 * it + 1]

        def blk(hp, u):
            return [wo_u[ns[u], pl.ds((2 * j + hp) * 64, 64), :] for j in range(NPAIR)]

        def mm(f, bs):
            lhs = jnp.concatenate([ob[f * NPAIR + j] for j in range(NPAIR)], axis=1)
            return _dot(lhs, as_bf16(jnp.concatenate(bs, axis=0)))

        def cb(x, y, sign):
            return [comb(a, b, sign) for a, b in zip(x, y)]

        def put(u, par, c):
            for i in range(NSEG // 2):
                obb[ns[u], 2 * i + par] = c[M * i:M * i + M].astype(BF16)
        m5 = mm(2, blk(1, 1))
        m1 = mm(0, cb(blk(0, 0), blk(1, 1), 1))
        m4 = mm(6, cb(blk(1, 0), blk(0, 0), -1))
        put(0, 0, mm(4, cb(blk(1, 0), blk(1, 1), 1)) + (m1 + m4 - m5))
        m3 = mm(5, cb(blk(0, 1), blk(1, 1), -1))
        put(1, 0, m3 + m5)
        m2 = mm(1, blk(0, 0))
        put(0, 1, m2 + m4)

        def send(n):
            col = pl.multiple_of(D + n * 128, 128)
            pltpu.make_async_copy(
                obb.at[n], out_hbm.at[:, pl.ds(0, M), pl.ds(col, 128)], sems.at[SO + 2]).start()
        send(ns[0])
        put(1, 1, mm(3, cb(blk(0, 0), blk(0, 1), 1)) + (m1 - m2 + m3))
        send(ns[1])
        return carry
    lax.fori_loop(0, NB // 2, epi, 0)
    ob_cp.wait()
    self_wait(aout, SO + 1)
    self_wait(obb, SO + 2)


def _step_order(u, cfg):
    cfg = dict(cfg, **cfg["sub"][u])
    ks = cfg["ks"]
    tmpl = []
    for x in cfg["tmpl"].split():
        kind, lag = x[:-1], int(x[-1])
        tmpl += [(kind + "a", lag), (kind + "b", lag)] if kind in ("q", "k", "v") else [(kind, lag)]

    def proj(kind, j):
        return ("qkv".index(kind[0]), 2 * j + "ab".index(kind[1]))
    out = []
    nw = 0
    for t in range(NPAIR + 1 + max(l for _, l in tmpl)):
        for kind, lag in tmpl:
            j = t - lag
            if j < 0:
                continue
            if j >= NPAIR:
                if kind[1:] == "a" and nw < NB:
                    out.append(("W", 0, ks, nw))
                    nw += 1
                continue
            out.append(("P",) + proj(kind, j) if len(kind) == 2 else (kind, j))
    if u > 0:
        first = [x[1:] for x in out if x[0] == "P"][:cfg["ne"]]
        out = [("E",) + x + (cfg["ek"],) for x in first] + out
    out += [("W", 0, ks, n) for n in range(nw, NB)]
    for n in range(NB):
        if u == U - 1 and n == cfg["tie_n"]:
            out.append(("A",))
        out.append(("W", ks, H, n))
    return out


_DEFAULT_CFG = dict(
    sub=(dict(tmpl='ka0 S1 qa0 kb0 qb0 V2 va0 vb0', ks=16, ne=5, ek=640),
         dict(tmpl='ka0 V3 va1 kb0 qa0 S1 vb1 qb0', ks=20, ne=3, ek=640),
         dict(tmpl='S2 qa0 qb0 va2 vb2 ka0 V3 kb0', ks=24, ne=3, ek=640),
         dict(tmpl='S2 ka0 kb0 va2 V3 qa0 qb0 vb2', ks=16, ne=5, ek=640)),
    tie_n=7, kick=(0, 1, 0), a_merge=5, a_g4=8, a_g4i=2)


def _build(cfg):
    tw_np = _twiddles()
    fill_np = np.zeros((96, 128), np.float32)
    fill_np[:R, :R] = _mask_fill()

    def run(A_q, A_k, A_v, A_shift_k, A_ssm_k, A_ssm_D, B_x, B_mem0, B_Wq, B_Wk, B_Wv, B_Wo):
        sk = A_shift_k.T.reshape(KS, NG, 128).transpose(1, 0, 2)
        any_spec = pl.BlockSpec(memory_space=pl.ANY)
        out = pl.pallas_call(
            functools.partial(_kernel, cfg),
            out_shape=jax.ShapeDtypeStruct((NSEG, SEG, 2 * D), BF16),
            in_specs=[any_spec] * 14,
            out_specs=any_spec,
            scratch_shapes=[
                pltpu.VMEM((48 * SLAB + 544, 128), U32),
                pltpu.VMEM((48 * SLAB + 544, 128), U32),
                pltpu.VMEM((NB, H * DH // 2, 128), U32),
                pltpu.VMEM((4, D, 8, DH), BF16),
                pltpu.VMEM((9, 512, D), BF16),
                pltpu.VMEM((NSEG, SEG, D), BF16),
                pltpu.VMEM((4, NSEG, M, KQ), BF16),
                pltpu.VMEM((4, NSEG * M // 2, KQ), U32),
                pltpu.VMEM((5, 2, HR, KQ), U32),
                pltpu.VMEM((NSEG, 3 * NPAIR, 8, 128), U32),
                pltpu.VMEM((7 * NPAIR, NSEG * M // 2, DH), BF16),
                pltpu.VMEM((NSEG, SEG, D), BF16),
                pltpu.VMEM((NB, NSEG, M, 128), BF16),
                pltpu.VMEM((2, 3, S, 128), BF16),
                pltpu.VMEM((NG + 1, 128, S), BF16),
                pltpu.VMEM((NG * S // 2, 128), U32),
                pltpu.VMEM((8 * NW + 32, 128), F32),
                pltpu.VMEM((2, NT, 8, 128), F32),
                pltpu.VMEM((NG, NSEG, SEG, 128), BF16),
                pltpu.VMEM((4, 8, 128), F32),
                pltpu.VMEM((96, 128), F32),
                pltpu.VMEM((NG, 8, 8, 128), F32),
                pltpu.VMEM((M, D), BF16),
                pltpu.VMEM((NG, KS, 128), BF16),
                pltpu.VMEM((4, NG, 128), BF16),
                pltpu.SemaphoreType.DMA((56,)),
            ],
            compiler_params=pltpu.CompilerParams(vmem_limit_bytes=124 * 1024 * 1024,
                                                 disable_bounds_checks=True),
        )(A_q.reshape(S, D), A_k.reshape(S, D), A_v.reshape(S, D), sk, A_ssm_k,
          A_ssm_D.reshape(NG, 128), B_x.reshape(NSEG, SEG, D), B_mem0.reshape(M, D),
          B_Wq, B_Wk, B_Wv, B_Wo.reshape(H * DH, D),
          jnp.asarray(tw_np), jnp.asarray(fill_np))
        return out.reshape(1, S, 2 * D)

    return run


@functools.partial(jax.jit, static_argnames=("B_seg_len",))
def pallas_concat_heads__ssm_conv_h3__memory_aug_recurrent_mem_tr__prompt_kernel(
    A_q: jax.Array,
    A_k: jax.Array,
    A_v: jax.Array,
    A_shift_k: jax.Array,
    A_ssm_k: jax.Array,
    A_ssm_D: jax.Array,
    B_x: jax.Array,
    B_mem0: jax.Array,
    B_Wq: jax.Array,
    B_Wk: jax.Array,
    B_Wv: jax.Array,
    B_Wo: jax.Array,
    B_seg_len: int = SEG,
):
    assert B_seg_len == SEG
    return _build(_DEFAULT_CFG)(A_q, A_k, A_v, A_shift_k, A_ssm_k, A_ssm_D, B_x, B_mem0,
                                B_Wq, B_Wk, B_Wv, B_Wo)
```

```python
import functools

import numpy as np
import jax
import jax.numpy as jnp
from jax import lax
import jax.experimental.pallas as pl
import jax.experimental.pallas.tpu as pltpu

F32 = jnp.float32
BF16 = jnp.bfloat16
U32 = jnp.uint32

S = 2048
D = 1024
H = 32
DH = 128
M = 8
SEG = 32
NSEG = S // SEG
U = 4
NPAIR = H // 2
R = 2 * (M + SEG)
SLAB = 520
KS = 4
NG = D // 128
KQ = D // 4
NB = D // 128
HR = NSEG * M // 4

TAF, TAI, TB, TC, TD, TE, NT = 0, 16, 32, 64, 192, 256, 512
WX, WS, WY, WK, NW = 0, 512, 1024, 1280, 1536


def _twiddles():
    tw = np.zeros((2, NT, 8), np.float64)

    def put(j, idx, z):
        tw[j, idx] = np.real(z)
        tw[j, idx + 1] = np.imag(z)
    s = np.arange(8)
    tau = 2j * np.pi
    for j in range(2):
        lx = 1j * np.pi * (1 + 4 * j) / 4096
        for d in range(8):
            put(j, TAF + 2 * d, np.exp(lx * 256 * d))
            put(j, TAI + 2 * d, np.exp(lx * 256 * d) / 2048)
        for r in range(4):
            for k in range(4):
                put(j, TB + 8 * k + 2 * r, np.exp((lx * 64 + tau * k / 16) * r))
            for k in range(16):
                put(j, TC + 8 * k + 2 * r, np.exp((lx * 16 + tau * k / 64) * r))
            for kb in range(8):
                put(j, TD + 8 * kb + 2 * r, np.exp((lx * 4 + tau * (s + 8 * kb) / 256) * r))
                for k3 in range(4):
                    put(j, TE + 8 * (4 * kb + k3) + 2 * r,
                        np.exp((lx + tau * (s + 8 * kb + 64 * k3) / 1024) * r))
    return np.ascontiguousarray(np.broadcast_to(tw[..., None], (2, NT, 8, 128))).astype(np.float32)


def _mask_fill():
    blk = np.concatenate([np.arange(M), M + np.arange(M, SEG)])
    lead = M + np.arange(M)
    head = np.concatenate([np.zeros(SEG), np.ones(SEG), np.zeros(M), np.ones(M)])
    pos = np.concatenate([blk, blk, lead, lead])
    same = head[:, None] == head[None, :]
    ok = (pos[:, None] < M) | (pos[:, None] >= pos[None, :])
    fill = np.where(same, np.where(ok, 0.0, -1e9), -np.inf)
    return fill.astype(np.float32)


def _widen(w):
    return pltpu.bitcast(w, BF16).astype(F32)


def _narrow(x):
    return pltpu.bitcast(x.astype(BF16), U32)


def _dot(a, b):
    return jnp.dot(a, b, preferred_element_type=F32)


def _dot_nt(a, b):
    return lax.dot_general(a, b, (((1,), (1,)), ((), ())), preferred_element_type=F32)


def _cadd(a, b):
    return (a[0] + b[0], a[1] + b[1])


def _csub(a, b):
    return (a[0] - b[0], a[1] - b[1])


def _cmul(a, w):
    return (a[0] * w[0] - a[1] * w[1], a[0] * w[1] + a[1] * w[0])


def _cmulc(a, w):
    return (a[0] * w[0] + a[1] * w[1], a[1] * w[0] - a[0] * w[1])


def _bfly_i(b, d, sg):
    p = (b[0] - d[1], b[1] + d[0])
    q = (b[0] + d[1], b[1] - d[0])
    return (p, q) if sg > 0 else (q, p)


def _dft4(x, sg):
    a, b = _cadd(x[0], x[2]), _csub(x[0], x[2])
    c, d = _cadd(x[1], x[3]), _csub(x[1], x[3])
    p, q = _bfly_i(b, d, sg)
    return [_cadd(a, c), p, _csub(a, c), q]


def _kernel(cfg,
            aq_hbm, ak_hbm, av_hbm, sk_hbm, ssmk_hbm, ssmd_hbm, x_hbm, mem0_hbm,
            wq_hbm, wk_hbm, wv_hbm, wo_hbm, tw_hbm, fill_hbm,
            out_hbm,
            w_a, w_b, wo_u, wstage, wostage, xbuf, xlead, xlead_u, xs_u, qkvb, wo_s, obuf,
            abuf, hbuf, ht, wk, tw, aout, kickbuf,
            fill_ref, taps, mem0_ref, sk_ref, ssmd_ref,
            sems):
    SW, SWO, SXL, SX, SH, SA, ST, SO, SS = 0, 16, 24, 28, 36, 44, 46, 48, 52
    w_hbms = (wq_hbm, wk_hbm, wv_hbm)
    a_hbms = (aq_hbm, ak_hbm, av_hbm)

    def aligned(x, n):
        return x if isinstance(x, int) else pl.multiple_of(x, n)

    def w_copy(m, hq, q=None):
        rows = pl.ds(0, D) if q is None else pl.ds(q * KQ, KQ)
        sem = SW + 12 + hq if q is None else SW + 4 * hq + q
        heads = aligned(8 * hq, 8)
        return pltpu.make_async_copy(
            w_hbms[m].at[rows, pl.ds(heads, 8), :], wstage.at[hq, rows], sems.at[sem])

    def self_wait(ref, sem):
        pltpu.make_async_copy(ref, ref, sems.at[sem]).wait()

    def late_start(k):
        pltpu.make_async_copy(
            wo_hbm.at[pl.ds(aligned(k * 512, 512), 512), :], wostage.at[k],
            sems.at[SWO + k]).start()
        pltpu.make_async_copy(
            ssmk_hbm.at[pl.ds(aligned(k * 128, 128), 128), :], hbuf.at[k],
            sems.at[SH + k]).start()

    def xlead_copy(q):
        return pltpu.make_async_copy(
            x_hbm.at[:, pl.ds(0, M), pl.ds(q * KQ, KQ)], xlead.at[q], sems.at[SXL + q])

    def x_copy(g):
        segs = pl.ds(g * 8, 8)
        return pltpu.make_async_copy(
            x_hbm.at[segs, pl.ds(M, SEG - M), :], xbuf.at[segs, pl.ds(M, SEG - M), :], sems.at[SX + g])

    def a_start(g):
        col = aligned(g * 128, 128)
        for t in (1, 2, 0):
            pltpu.make_async_copy(
                a_hbms[t].at[:, pl.ds(col, 128)], abuf.at[g & 1, t], sems.at[SA + (g & 1)]).start()

    tw_cp = pltpu.make_async_copy(tw_hbm, tw, sems.at[ST])

    small = [pltpu.make_async_copy(src, dst, sems.at[SS + i]) for i, (src, dst) in enumerate((
        (fill_hbm, fill_ref), (mem0_hbm, mem0_ref), (sk_hbm, sk_ref), (ssmd_hbm, ssmd_ref.at[0])))]

    for q in range(4):
        xlead_copy(q).start()
        w_copy(0, 0, q).start()
        if q > 0:
            w_copy(0, 1, q - 1).start()
    w_copy(0, 1, 3).start()
    for q in range(4):
        w_copy(0, 2, q).start()
    w_copy(0, 3).start()
    for cp in small:
        cp.start()

    kickbuf[...] = jnp.zeros(kickbuf.shape, F32)

    w_parts = (w_a, w_b)

    def slab_row(u, par, jl):
        return ((u >> 1) * 8 + par * 4 + jl) * SLAB

    def gated(x, i, n, gates):
        if gates is None:
            return x
        never, vals = gates
        v = vals[(i * len(vals) * cfg["gspan"]) // (n * 100)]
        return jnp.where(never, pltpu.bitcast(v, U32), x)

    def vregs(*mats):
        return [m_[r:r + 8] for m_ in mats for r in range(0, m_.shape[0], 8)]

    def relayout(u, g, q, gates=None, src=None):
        slot, qs = (u & 3, q) if src is None else src
        low = lax.broadcasted_iota(jnp.int32, (8, 128), 0) < 4
        keep = jnp.where(low, jnp.uint32(0xFFFF), jnp.uint32(0xFFFF0000))
        shl = jnp.where(low, jnp.uint32(16), jnp.uint32(0))
        base = slab_row(u, 0, 0) + q * (KQ // 2)
        for i in range(KQ // 2):
            x = wstage[slot, pl.ds(qs * KQ + 2 * i, 2)].reshape(16, DH)
            x = gated(pltpu.bitcast(x, U32), i, KQ // 2, gates)
            y = pltpu.roll(x, 4, 0)
            w_parts[g][pl.ds(base + i, 8, stride=SLAB), :] = (x & keep) | ((y << shl) >> (16 - shl))

    def comb(x, y, sign):
        return _widen(x) + _widen(y) if sign > 0 else _widen(x) - _widen(y)

    def as_bf16(b):
        return pltpu.bitcast(b, BF16) if b.dtype == U32 else b.astype(BF16)

    def put_lead(segs, n, it, a, b):
        both = jnp.concatenate([a.reshape(n, M, DH), b.reshape(n, M, DH)], axis=1)
        qkvb[segs, it] = _narrow(both)

    def batch_pair(u, g, jl):
        it = 4 * u + jl
        rows = [pl.multiple_of(slab_row(u, par, jl), 8) for par in range(2)]

        def blk(kh, par):
            return w_parts[g][pl.ds(rows[par] + kh * (D // 4), D // 4), :]

        def mm(a, b):
            return _dot(pltpu.bitcast(jnp.concatenate(a, axis=1), BF16), as_bf16(b))

        def xs(f):
            return [xs_u[f, q] for q in range(2)]
        a11 = [xlead_u[q, pl.ds(0, HR), :] for q in (0, 1)]
        a22 = [xlead_u[q, pl.ds(HR, HR), :] for q in (2, 3)]
        m5 = mm(xs(2), blk(1, 1))
        m1 = mm(xs(0), comb(blk(0, 0), blk(1, 1), 1))
        m4 = mm(a22, comb(blk(1, 0), blk(0, 0), -1))
        c11 = mm(xs(4), comb(blk(1, 0), blk(1, 1), 1)) + (m1 + m4 - m5)
        m3 = mm(a11, comb(blk(0, 1), blk(1, 1), -1))
        put_lead(pl.ds(0, NSEG // 2), NSEG // 2, it, c11, m3 + m5)
        m2 = mm(xs(1), blk(0, 0))
        c22 = mm(xs(3), comb(blk(0, 0), blk(0, 1), 1)) + (m1 - m2 + m3)
        put_lead(pl.ds(NSEG // 2, NSEG // 2), NSEG // 2, it, m2 + m4, c22)
        return vregs(m5, m1, m4, c11, m3, m2, c22)

    def quarter_wait(u, q):
        self_wait(wstage.at[u, pl.ds(pl.multiple_of(q * KQ, KQ), KQ)], SW + 4 * u + q)

    def first_unit(q, carry):
        never = q > 1000
        half = q & 1
        self_wait(xlead.at[q], SXL + q)
        quarter_wait(0, q)
        xlead_u[q] = _narrow(xlead[q].astype(F32).reshape(NSEG * M, KQ))
        relayout(0, 0, q)

        @pl.when(q > 0)
        def _():
            quarter_wait(1, q - 1)
        res = []
        xq = pltpu.bitcast(xlead_u[q], BF16)
        for jl in range(4):
            outs = []
            for par in range(2):
                acc = pl.ds((2 * jl + par) * (NSEG * M), NSEG * M)
                row = pl.multiple_of(slab_row(0, par, jl) + q * (KQ // 2), 8)
                w = pltpu.bitcast(w_a[pl.ds(row, KQ // 2), :], BF16)
                d = _dot(xq, w) + jnp.where(q == 0, 0.0, wk[acc, :])
                wk[acc, :] = d
                outs.append(d)
            put_lead(pl.ds(0, NSEG), NSEG, jl, outs[0], outs[1])
            res += outs
        gates = (never, vregs(*res))
        qn = jnp.maximum(q - 1, 0)
        relayout(1, 1, qn, gates, src=(jnp.minimum(q, 1), qn))
        for r in range(0, HR, 8):
            for cb in range(2):
                cols = pl.ds(cb * 128, 128)
                i = 2 * (r // 8) + cb
                a11 = gated(xlead_u[half, pl.ds(r, 8), cols], i, HR // 4, gates)
                a22 = gated(xlead_u[2 + half, pl.ds(HR + r, 8), cols], i, HR // 4, gates)
                a21 = xlead_u[half, pl.ds(HR + r, 8), cols]
                a12 = xlead_u[2 + half, pl.ds(r, 8), cols]
                for f, (x, y, sg) in enumerate(((a11, a22, 1), (a21, a22, 1), (a11, a12, 1),
                                                (a21, a11, -1), (a12, a22, -1))):
                    xs_u[f, half, pl.ds(r, 8), cols] = _narrow(comb(x, y, sg))
        return carry
    lax.fori_loop(0, 4, first_unit, 0)
    w_copy(1, 0).start()
    late_start(0)
    w_copy(0, 1, 3).wait()
    relayout(1, 1, 3)

    def second_unit(jl, carry):
        quarter_wait(2, jl)
        relayout(2, 0, jl, (jl > 1000, batch_pair(1, 1, jl)))
        return carry
    lax.fori_loop(0, 4, second_unit, 0)

    def late_relayout(src, k, jl, gates):
        half = jl // 2
        hp = 2 * k + half
        for ri in range(4):
            r = 4 * (jl % 2) + ri
            blk = [pltpu.bitcast(wostage[src, pl.ds(half * 256 + e * 128 + r * 16, 16), :], U32)
                   for e in range(2)]
            for np_ in range(NB // 2):
                b = [[gated(blk[e][:, (2 * np_ + c) * 128:(2 * np_ + c + 1) * 128],
                            ri * 4 + np_, 16, gates) for c in range(2)] for e in range(2)]
                for e in range(2):
                    for c in range(2):
                        wo_u[2 * np_ + c, pl.ds(pl.multiple_of(hp * 128 + e * 64 + r * 8, 8), 8), :] = b[e][c]
                rows = pl.ds(pl.multiple_of(hp * 64 + r * 8, 8), 8)
                for f, (x, y, sg) in enumerate(((b[0][0], b[1][1], 1), (b[0][1], b[1][1], -1),
                                                (b[1][0], b[0][0], -1), (b[0][0], b[0][1], 1),
                                                (b[1][0], b[1][1], 1))):
                    wo_s[f, np_, rows, :] = _narrow(comb(x, y, sg))
        for t in range(4):
            tile = pltpu.bitcast(hbuf[src, :, pl.ds((4 * jl + t) * 128, 128)], U32)
            tile = jnp.concatenate([gated(tile[0:8], t, 4, gates), tile[8:]], axis=0)
            row = pl.multiple_of(k * 1024 + (4 * jl + t) * 64, 64)
            ht[pl.ds(row, 64), :] = pltpu.bitcast(pltpu.bitcast(tile, BF16).T, U32)

    def unit_body(u, g):
        @pl.when(u < 11)
        def _():
            self_wait(wstage.at[(u + 1) & 3], SW + 12 + ((u + 1) & 3))

        @pl.when(u >= 4)
        def _():
            self_wait(wostage.at[u - 4], SWO + u - 4)
            self_wait(hbuf.at[u - 4], SH + u - 4)
        for m in (1, 2):
            @pl.when((u + 3) >> 2 == m)
            def _():
                w_copy(m, (u + 3) & 3).start()

        @pl.when(u <= 8)
        def _():
            late_start(u - 1)
        if g == 1:
            @pl.when(u == 9)
            def _():
                x_copy(0).start()
                a_start(0)
                tw_cp.start()
        for jl in range(4):
            gates = (u > 1000, batch_pair(u, g, jl))
            relayout(jnp.where(u < 11, u + 1, u - 1), 1 - g, jl, gates)
            late_relayout(jnp.where(u >= 4, u - 4, 8), jnp.maximum(u - 4, 0), jl, gates)

    def unit_pair(mm, carry):
        for g in range(2):
            unit_body(2 * mm + g, g)
        return carry
    lax.fori_loop(1, 6, unit_pair, 0)

    a_start(1)
    for g in range(1, NG):
        x_copy(g).start()
    for cp in small:
        cp.wait()
    dd = ssmd_ref[0].astype(F32)
    for g in range(NG):
        sk = sk_ref[g].astype(F32)
        for j in range(KS):
            taps[g, j] = jnp.broadcast_to(sk[j:j + 1], (8, 128))
        taps[g, KS] = jnp.broadcast_to(dd[g:g + 1], (8, 128))

    def part_a(i, kick):
        g, j = i >> 1, i & 1
        sl = g & 1
        never = i > 1000
        sub = lax.broadcasted_iota(jnp.int32, (8, 128), 0)
        kickbuf[jnp.where(never, 1, 0)] = kick
        chain = [kickbuf[jnp.where(i > 2000, 0, 1)]]

        def begin(xs, ng):
            xs = list(xs)
            for e in range(min(ng, len(xs))):
                c = chain[0]
                c = c if c.dtype == xs[e].dtype else pltpu.bitcast(c, xs[e].dtype)
                xs[e] = jnp.where(never, c, xs[e])
            return xs

        def merge(vals):
            c = vals[-1]
            for v in list(vals[:-1])[:cfg["a_merge"]]:
                c = jnp.maximum(v, c)
            chain[0] = c

        def ld(v):
            if isinstance(v, tuple):
                blk, ri, r = v
                base = 8 * WS + 256 * blk + 16 * ri + 32 * r
                lo = wk[pl.ds(base, 8), :]
                if r == 0:
                    return lo
                return pltpu.roll(jnp.where(sub >= r, lo, wk[pl.ds(base + 8, 8), :]), 8 - r, 0)
            return wk[pl.ds(8 * v, 8), :]

        def st(v, x):
            wk[pl.ds(8 * v, 8), :] = x

        def twid(idx):
            return (tw[j, idx], tw[j, idx + 1])

        def pairs(flat):
            return [(flat[2 * e], flat[2 * e + 1]) for e in range(len(flat) // 2)]

        def fwd4(locs, t0):
            v = pairs(begin([ld(x) for loc in locs[::-1] for x in loc], cfg["a_g4"]))[::-1]
            return _dft4([v[0]] + [_cmul(v[r], twid(t0 + 2 * r)) for r in range(1, 4)], +1)

        def inv4(v, t0):
            o = _dft4(v, -1)
            return [o[0]] + [_cmulc(o[r], twid(t0 + 2 * r)) for r in range(1, 4)]

        def ld4(locs):
            return pairs(begin([ld(x) for loc in locs for x in loc], cfg["a_g4i"]))

        def put4(locs, o):
            for loc, x in zip(locs, o):
                st(loc[0], x[0])
                st(loc[1], x[1])
            merge([x for c in o for x in c])

        def put4_t(dsts, o):
            for (blk, slot), x in zip(dsts, o):
                for ri in range(2):
                    base = 8 * WS + 256 * blk + 16 * ri + slot
                    wk[pl.ds(base, 8, stride=33), :] = x[ri]
            merge([x for c in o for x in c])

        def xloc(sig, n):
            return (WX + 256 * sig + 2 * n, WX + 256 * sig + 2 * n + 1)

        def sloc(kb, l):
            return ((2 * kb + l // 8, 0, l % 8), (2 * kb + l // 8, 1, l % 8))

        def pass_kv():
            t = [taps[g, a] for a in range(KS)]
            prev = [None] + [jnp.zeros((8, 128), F32)] * (KS - 1)
            for v in range(S // 16):
                w, = begin([pltpu.bitcast(abuf[sl, 1, pl.ds(16 * v, 16), :], U32)], 1)
                k2 = _widen(w)
                v2 = abuf[sl, 2, pl.ds(16 * v, 16), :].astype(F32)
                outs = []
                for hh in range(2):
                    x = k2[8 * hh:8 * hh + 8]
                    cur = [None] + [pltpu.roll(x, a, 0) for a in range(1, KS)]
                    ks = x * t[0]
                    for a in range(1, KS):
                        ks = ks + jnp.where(sub < a, prev[a], cur[a]) * t[a]
                    prev = cur
                    kv = (ks * v2[8 * hh:8 * hh + 8]).astype(BF16).astype(F32)
                    st(WK + 2 * v + hh, kv)
                    outs.append(kv)
                merge(outs)

        def forward(sig, src):
            for n in range(32):
                x = src(n)
                cs = []
                for d in range(4):
                    a, b = twid(TAF + 2 * d), twid(TAF + 2 * (d + 4))
                    if d == 0:
                        s_ = x[4] * b[0]
                        cs.append((x[0] + s_, s_))
                    else:
                        cs.append((x[d] * a[0] + x[d + 4] * b[0], x[d] * a[1] + x[d + 4] * b[1]))
                put4([xloc(sig, n + 32 * k0) for k0 in range(4)], _dft4(cs, +1))
            for k0 in range(4):
                for n in range(8):
                    locs = [xloc(sig, n + 8 * r + 32 * k0) for r in range(4)]
                    put4(locs, fwd4(locs, TB + 8 * k0))
            for k0 in range(4):
                for k1 in range(4):
                    k = k0 + 4 * k1
                    for a in range(2):
                        o = fwd4([xloc(sig, a + 2 * r + 8 * k1 + 32 * k0) for r in range(4)], TC + 8 * k)
                        put4_t([(2 * ((k + 16 * k2) // 8) + a, k % 8) for k2 in range(4)], o)
            for kb in range(8):
                for e in range(4):
                    o = fwd4([sloc(kb, e + 4 * r) for r in range(4)], TD + 8 * kb)
                    put4([xloc(sig, 16 * kb + e + 4 * r) for r in range(4)], o)
            for kb in range(8):
                for k3 in range(4):
                    locs = [xloc(sig, 16 * kb + r + 4 * k3) for r in range(4)]
                    t0 = TE + 8 * (4 * kb + k3)
                    o = fwd4(locs, t0)
                    if sig == 0:
                        hs = ld4([xloc(1, 16 * kb + r + 4 * k3) for r in range(4)])
                        o = inv4([_cmul(a, b) for a, b in zip(o, hs)], t0)
                    put4(locs, o)

        def inverse():
            for kb in range(8):
                for e in range(4):
                    o = inv4(ld4([xloc(0, 16 * kb + e + 4 * r) for r in range(4)]), TD + 8 * kb)
                    put4_t([(2 * kb + (e + 4 * f) // 8, (e + 4 * f) % 8) for f in range(4)], o)
            for k0 in range(4):
                for k1 in range(4):
                    k = k0 + 4 * k1
                    for a in range(2):
                        v = ld4([sloc((k + 16 * r) // 8, 8 * a + k % 8) for r in range(4)])
                        put4([xloc(0, a + 2 * b + 8 * k1 + 32 * k0) for b in range(4)], inv4(v, TC + 8 * k))
            for k0 in range(4):
                for n in range(8):
                    locs = [xloc(0, n + 8 * r + 32 * k0) for r in range(4)]
                    put4(locs, inv4(ld4(locs), TB + 8 * k0))
            dskip = taps[g, KS]
            for n0 in range(32):
                cs = _dft4(ld4([xloc(0, n0 + 32 * r) for r in range(4)]), -1)
                outs = []
                for d in [d0 + 4 * hh for d0 in range(4) for hh in range(2)]:
                    n = n0 + 32 * d
                    a = twid(TAI + 2 * d)
                    if 0 < d < 4:
                        cs[d] = tuple(begin(cs[d], 2))
                    c = cs[d % 4]
                    y = c[0] * a[0] if d == 0 else c[0] * a[0] + c[1] * a[1]
                    y = y + jnp.where(j == 0, ld(WK + n) * dskip, ld(WY + n))
                    st(WY + n, y)
                    chain[0] = abuf[sl, 0, pl.ds(8 * n, 8), :].astype(F32) * y
                    aout[g, n // 4, pl.ds(8 * (n % 4), 8), :] = chain[0].astype(BF16)
                    outs.append(chain[0])
                merge(outs)

        def filt(n):
            base = pl.multiple_of(g * (S // 2), S // 2)
            ws = begin([ht[pl.ds(base + 8 * (n // 2 + 16 * d), 8), :] for d in range(8)], 8)
            return [_widen(w)[8 * (n % 2):8 * (n % 2) + 8] for w in ws]
        pass_kv()
        forward(1, filt)
        forward(0, lambda n: begin([ld(WK + n + 32 * d) for d in range(8)], 8))
        inverse()
        return chain[0]

    scale = DH ** (-0.5)

    def w_slab(m, h):
        u = 4 * m + h // 8
        return pltpu.bitcast(w_parts[u % 2][pl.ds(slab_row(u, h % 2, (h // 2) % 4), D // 2), :], BF16)

    class Step:
        def __init__(self, s, leads, mem):
            self.s = s
            self.leads = leads
            self.acc2 = [None] * NB
            self.qkv, self.ps, self.os = {}, {}, []
            self.acc = [None] * NB
            self.ocat, self.early, self.marks, self.heads = {}, {}, {}, {}
            self.tie = None
            x = xbuf[s, pl.ds(M, SEG - M), :].astype(F32)
            self.lhsf = jnp.concatenate([mem, x], axis=0)
            self.lhs = self.lhsf.astype(BF16)

        def proj_early(self, m, h, k):
            self.early[m, h] = (k, _dot(self.lhsf[:, :k].astype(BF16), w_slab(m, h)[:k]))

        def proj(self, m, h):
            if (m, h) in self.early:
                k, part = self.early[m, h]
                d = _dot(self.lhsf[:, k:].astype(BF16), w_slab(m, h)[k:]) + part
            else:
                d = _dot(self.lhs, w_slab(m, h))
            self.heads[m, h] = d
            j = h // 2
            if (m, h ^ 1) not in self.heads:
                return
            a, b = self.heads[m, 2 * j], self.heads[m, 2 * j + 1]
            self.marks[m, j] = a[0:8]
            lead = _widen(qkvb[self.s, m * NPAIR + j])
            self.qkv[m, j] = jnp.concatenate([a, b, lead], axis=0).astype(BF16)

        def probs(self, j):
            fill = fill_ref[pl.ds(0, R), pl.ds(0, R)]
            qk = _dot_nt(self.qkv[0, j], self.qkv[1, j])
            sc = jnp.where(fill == 0.0, qk * scale, fill)
            e = jnp.exp(sc - jnp.max(sc, axis=-1, keepdims=True))
            l = jnp.sum(e, axis=-1, keepdims=True)
            r = pl.reciprocal(l, approx=True)
            r = r * (2.0 - l * r)
            self.ps[j] = (e * r).astype(BF16)

        def attend(self, j):
            o = _dot(self.ps[j], self.qkv[2, j])
            self.leads[2 * j].append(o[2 * SEG:2 * SEG + M])
            self.leads[2 * j + 1].append(o[2 * SEG + M:])
            self.os += [o[0:SEG], o[SEG:2 * SEG]]

        def tied(self, w):
            if self.tie is not None:
                w = jnp.concatenate(
                    [jnp.where(self.s > 1000, pltpu.bitcast(self.tie, U32), w[0:8]), w[8:]], axis=0)
                self.tie = None
            return pltpu.bitcast(w, BF16)

        def wo_strassen(self, j0, j1, np_, f):
            if (j0, f) not in self.ocat:
                parts = []
                for j in range(j0, j1):
                    a11, a12 = self.os[2 * j], self.os[2 * j + 1]
                    a21, a22 = [jnp.concatenate(self.leads[2 * j + e], axis=0) for e in range(2)]
                    parts.append({1: lambda: a11 + a22, 2: lambda: a21 + a22, 3: lambda: a11,
                                  4: lambda: a22, 5: lambda: a11 + a12, 6: lambda: a21 - a11,
                                  7: lambda: a12 - a22}[f]())
                self.ocat[j0, f] = jnp.concatenate(parts, axis=1).astype(BF16)
            if f in (2, 5):
                e = (2, 5).index(f)
                w = jnp.concatenate([wo_u[2 * np_ + e, pl.ds((2 * j + e) * 64, 64), :]
                                     for j in range(j0, j1)], axis=0)
            else:
                w = wo_s[(1, 3, 4, 6, 7).index(f), np_, pl.ds(j0 * 64, (j1 - j0) * 64), :]
            d = _dot(self.ocat[j0, f], self.tied(w))
            uses = {1: ((0, 0, 1), (1, 1, 1)), 2: ((1, 0, 1), (1, 1, -1)), 3: ((0, 1, 1), (1, 1, 1)),
                    4: ((0, 0, 1), (1, 0, 1)), 5: ((0, 1, 1), (0, 0, -1)), 6: ((1, 1, 1),),
                    7: ((0, 0, 1),)}[f]
            for which, c, sg in uses:
                acc = (self.acc, self.acc2)[which]
                n = 2 * np_ + c
                if acc[n] is None:
                    assert sg > 0
                    acc[n] = d
                else:
                    acc[n] = d + acc[n] if sg > 0 else acc[n] - d

        def wo(self, h0, h1, n):
            if h0 not in self.ocat:
                self.ocat[h0] = jnp.concatenate(self.os[h0:h1], axis=1).astype(BF16)
            d = _dot(self.ocat[h0], self.tied(wo_u[n, pl.ds(h0 * 64, (h1 - h0) * 64), :]))
            self.acc[n] = d if self.acc[n] is None else d + self.acc[n]

        def finish(self):
            res = jnp.concatenate(self.acc, axis=1)
            obuf[self.s, pl.ds(M, SEG - M), :] = res[M:].astype(BF16)
            if self.acc2[0] is not None:
                lead = jnp.concatenate(self.acc2, axis=1)
                for e in range(U):
                    obuf[self.s - (U - 1) + e, pl.ds(0, M), :] = lead[M * e:M * e + M].astype(BF16)
            return res[0:M]

    def steps(i, mem):
        def send(segs, rows):
            pltpu.make_async_copy(
                obuf.at[segs, rows], out_hbm.at[segs, rows, pl.ds(D, D)], sems.at[SO]).start()
        sts = []
        leads = [[] for _ in range(H)]
        for u in range(U):
            st = Step(i * U + u, leads, mem)
            sts.append(st)
            for item in _step_order(u, cfg):
                if item[0] == "A":
                    ku, km, kj = cfg["kick"]
                    st.tie = part_a(i, sts[ku].marks[km, kj])
                elif item[0] == "O":
                    last_half = (i & 1) == 1
                    pl.when(last_half)(lambda: a_send(i >> 1))
                    pl.when(jnp.logical_and(last_half, i < 2 * NG - 4))(lambda: a_start((i >> 1) + 2))
                    send(pl.ds(i * U, U - 1), pl.ds(M, SEG - M))
                else:
                    dict(P=st.proj, E=st.proj_early, S=st.probs, V=st.attend, W=st.wo,
                         X=st.wo_strassen)[item[0]](*item[1:])
            mem = st.finish()
        send(pl.ds(i * U, U - 1), pl.ds(0, M))
        send(pl.ds(i * U + U - 1, 1), pl.ds(0, SEG))
        return mem

    def a_send(g):
        pltpu.make_async_copy(
            aout.at[g], out_hbm.at[:, :, pl.ds(pl.multiple_of(g * 128, 128), 128)],
            sems.at[SO + 1]).start()

    def group(g, mem):
        x_copy(g).wait()
        self_wait(abuf.at[g & 1], SA + (g & 1))
        return lax.fori_loop(0, 2, lambda j, m_: steps(2 * g + j, m_), mem)

    tw_cp.wait()
    lax.fori_loop(0, NG, group, mem0_ref[...].astype(F32))
    self_wait(obuf, SO)
    self_wait(aout, SO + 1)


def _step_order(u, cfg):
    cfg = dict(cfg, **cfg["sub"][u])
    ks = cfg["ks"]
    tmpl = []
    for x in cfg["tmpl"].split():
        kind, lag = x[:-1], int(x[-1])
        tmpl += [(kind + "a", lag), (kind + "b", lag)] if kind in ("q", "k", "v") else [(kind, lag)]

    def proj(kind, j):
        return ("qkv".index(kind[0]), 2 * j + "ab".index(kind[1]))
    if u < U - 1:
        fill = [[("W", 0, ks, n)] for n in range(NB)]
        last = [("W", ks, H, n) for n in range(NB)]
    else:
        def products(j0, j1, f_outer):
            fs = (1, 4, 7, 3, 5, 2, 6)
            if f_outer:
                return [("X", j0, j1, np_, f) for f in fs for np_ in range(NB // 2)]
            return [("X", j0, j1, np_, f) for np_ in range(NB // 2) for f in fs]
        xs = products(0, ks // 2, cfg["xo"] & 1)
        fill = [xs[e:e + 2] for e in range(0, len(xs), 2)]
        last = products(ks // 2, NPAIR, cfg["xo"] & 2)
        last.insert(len(last) - cfg["send_back"], ("O",))
        last.insert(len(last) - 1 - cfg["tie_back"], ("A",))
    out = []
    for t in range(NPAIR + 1 + max(l for _, l in tmpl)):
        for kind, lag in tmpl:
            j = t - lag
            if j < 0:
                continue
            if j >= NPAIR:
                if kind[1:] == "a" and fill:
                    out += fill.pop(0)
                continue
            out.append(("P",) + proj(kind, j) if len(kind) == 2 else (kind, j))
    if u > 0:
        first = [x[1:] for x in out if x[0] == "P"][:cfg["ne"]]
        out = [("E",) + x + (cfg["ek"],) for x in first] + out
    return out + [x for f in fill for x in f] + last


_DEFAULT_CFG = dict(
    sub=(dict(tmpl='ka0 S1 qa0 kb0 qb0 V2 va0 vb0', ks=16, ne=5, ek=640),
         dict(tmpl='ka0 V3 va1 kb0 qa0 S1 vb1 qb0', ks=20, ne=3, ek=640),
         dict(tmpl='S2 qa0 qb0 va2 vb2 ka0 V3 kb0', ks=24, ne=3, ek=640),
         dict(tmpl='S2 ka0 kb0 va2 V3 qa0 qb0 vb2', ks=16, ne=5, ek=640)),
    tie_back=28, send_back=26, xo=0, gspan=75, kick=(0, 1, 0), a_merge=5, a_g4=8, a_g4i=2)


def _build(cfg):
    tw_np = _twiddles()
    fill_np = np.zeros((96, 128), np.float32)
    fill_np[:R, :R] = _mask_fill()

    def run(A_q, A_k, A_v, A_shift_k, A_ssm_k, A_ssm_D, B_x, B_mem0, B_Wq, B_Wk, B_Wv, B_Wo):
        sk = A_shift_k.T.reshape(KS, NG, 128).transpose(1, 0, 2)
        any_spec = pl.BlockSpec(memory_space=pl.ANY)
        out = pl.pallas_call(
            functools.partial(_kernel, cfg),
            out_shape=jax.ShapeDtypeStruct((NSEG, SEG, 2 * D), BF16),
            in_specs=[any_spec] * 14,
            out_specs=any_spec,
            scratch_shapes=[
                pltpu.VMEM((48 * SLAB + 544, 128), U32),
                pltpu.VMEM((48 * SLAB + 544, 128), U32),
                pltpu.VMEM((NB, H * DH // 2, 128), U32),
                pltpu.VMEM((4, D, 8, DH), BF16),
                pltpu.VMEM((9, 512, D), BF16),
                pltpu.VMEM((NSEG, SEG, D), BF16),
                pltpu.VMEM((4, NSEG, M, KQ), BF16),
                pltpu.VMEM((4, NSEG * M // 2, KQ), U32),
                pltpu.VMEM((5, 2, HR, KQ), U32),
                pltpu.VMEM((NSEG, 3 * NPAIR, 8, 128), U32),
                pltpu.VMEM((5, NB // 2, H * DH // 4, 128), U32),
                pltpu.VMEM((NSEG, SEG, D), BF16),
                pltpu.VMEM((2, 3, S, 128), BF16),
                pltpu.VMEM((NG + 1, 128, S), BF16),
                pltpu.VMEM((NG * S // 2, 128), U32),
                pltpu.VMEM((8 * NW + 32, 128), F32),
                pltpu.VMEM((2, NT, 8, 128), F32),
                pltpu.VMEM((NG, NSEG, SEG, 128), BF16),
                pltpu.VMEM((4, 8, 128), F32),
                pltpu.VMEM((96, 128), F32),
                pltpu.VMEM((NG, 8, 8, 128), F32),
                pltpu.VMEM((M, D), BF16),
                pltpu.VMEM((NG, KS, 128), BF16),
                pltpu.VMEM((4, NG, 128), BF16),
                pltpu.SemaphoreType.DMA((56,)),
            ],
            compiler_params=pltpu.CompilerParams(vmem_limit_bytes=124 * 1024 * 1024,
                                                 disable_bounds_checks=True),
        )(A_q.reshape(S, D), A_k.reshape(S, D), A_v.reshape(S, D), sk, A_ssm_k,
          A_ssm_D.reshape(NG, 128), B_x.reshape(NSEG, SEG, D), B_mem0.reshape(M, D),
          B_Wq, B_Wk, B_Wv, B_Wo.reshape(H * DH, D),
          jnp.asarray(tw_np), jnp.asarray(fill_np))
        return out.reshape(1, S, 2 * D)

    return run


@functools.partial(jax.jit, static_argnames=("B_seg_len",))
def pallas_concat_heads__ssm_conv_h3__memory_aug_recurrent_mem_tr__prompt_kernel(
    A_q: jax.Array,
    A_k: jax.Array,
    A_v: jax.Array,
    A_shift_k: jax.Array,
    A_ssm_k: jax.Array,
    A_ssm_D: jax.Array,
    B_x: jax.Array,
    B_mem0: jax.Array,
    B_Wq: jax.Array,
    B_Wk: jax.Array,
    B_Wv: jax.Array,
    B_Wo: jax.Array,
    B_seg_len: int = SEG,
):
    assert B_seg_len == SEG
    return _build(_DEFAULT_CFG)(A_q, A_k, A_v, A_shift_k, A_ssm_k, A_ssm_D, B_x, B_mem0,
                                B_Wq, B_Wk, B_Wv, B_Wo)
```

```python
import functools

import numpy as np
import jax
import jax.numpy as jnp
from jax import lax
import jax.experimental.pallas as pl
import jax.experimental.pallas.tpu as pltpu

F32 = jnp.float32
BF16 = jnp.bfloat16
U32 = jnp.uint32

S = 2048
D = 1024
H = 32
DH = 128
M = 8
SEG = 32
NSEG = S // SEG
U = 4
NPAIR = H // 2
R = 2 * (M + SEG)
SLAB = 520
KS = 4
NG = D // 128
KQ = D // 4
NB = D // 128
HR = NSEG * M // 4

TAF, TAI, TB, TC, TD, TE, NT = 0, 16, 32, 64, 192, 256, 512
WX, WS, WY, WK, NW = 0, 512, 1024, 1280, 1536


def _twiddles():
    tw = np.zeros((2, NT, 8), np.float64)

    def put(j, idx, z):
        tw[j, idx] = np.real(z)
        tw[j, idx + 1] = np.imag(z)
    s = np.arange(8)
    tau = 2j * np.pi
    for j in range(2):
        lx = 1j * np.pi * (1 + 4 * j) / 4096
        for d in range(8):
            put(j, TAF + 2 * d, np.exp(lx * 256 * d))
            put(j, TAI + 2 * d, np.exp(lx * 256 * d) / 2048)
        for r in range(4):
            for k in range(4):
                put(j, TB + 8 * k + 2 * r, np.exp((lx * 64 + tau * k / 16) * r))
            for k in range(16):
                put(j, TC + 8 * k + 2 * r, np.exp((lx * 16 + tau * k / 64) * r))
            for kb in range(8):
                put(j, TD + 8 * kb + 2 * r, np.exp((lx * 4 + tau * (s + 8 * kb) / 256) * r))
                for k3 in range(4):
                    put(j, TE + 8 * (4 * kb + k3) + 2 * r,
                        np.exp((lx + tau * (s + 8 * kb + 64 * k3) / 1024) * r))
    return np.ascontiguousarray(np.broadcast_to(tw[..., None], (2, NT, 8, 128))).astype(np.float32)


def _mask_fill():
    blk = np.concatenate([np.arange(M), M + np.arange(M, SEG)])
    lead = M + np.arange(M)
    head = np.concatenate([np.zeros(SEG), np.ones(SEG), np.zeros(M), np.ones(M)])
    pos = np.concatenate([blk, blk, lead, lead])
    same = head[:, None] == head[None, :]
    ok = (pos[:, None] < M) | (pos[:, None] >= pos[None, :])
    fill = np.where(same, np.where(ok, 0.0, -1e9), -np.inf)
    return fill.astype(np.float32)


def _widen(w):
    return pltpu.bitcast(w, BF16).astype(F32)


def _narrow(x):
    return pltpu.bitcast(x.astype(BF16), U32)


def _dot(a, b):
    return jnp.dot(a, b, preferred_element_type=F32)


def _dot_nt(a, b):
    return lax.dot_general(a, b, (((1,), (1,)), ((), ())), preferred_element_type=F32)


def _cadd(a, b):
    return (a[0] + b[0], a[1] + b[1])


def _csub(a, b):
    return (a[0] - b[0], a[1] - b[1])


def _cmul(a, w):
    return (a[0] * w[0] - a[1] * w[1], a[0] * w[1] + a[1] * w[0])


def _cmulc(a, w):
    return (a[0] * w[0] + a[1] * w[1], a[1] * w[0] - a[0] * w[1])


def _bfly_i(b, d, sg):
    p = (b[0] - d[1], b[1] + d[0])
    q = (b[0] + d[1], b[1] - d[0])
    return (p, q) if sg > 0 else (q, p)


def _dft4(x, sg):
    a, b = _cadd(x[0], x[2]), _csub(x[0], x[2])
    c, d = _cadd(x[1], x[3]), _csub(x[1], x[3])
    p, q = _bfly_i(b, d, sg)
    return [_cadd(a, c), p, _csub(a, c), q]


def _kernel(cfg,
            aq_hbm, ak_hbm, av_hbm, sk_hbm, ssmk_hbm, ssmd_hbm, x_hbm, mem0_hbm,
            wq_hbm, wk_hbm, wv_hbm, wo_hbm, tw_hbm, fill_hbm,
            out_hbm,
            w_a, w_b, wo_u, wstage, wostage, xbuf, xlead, xlead_u, xs_u, qkvb, wo_s, obuf,
            abuf, hbuf, ht, wk, tw, aout, kickbuf,
            fill_ref, taps, mem0_ref, sk_ref, ssmd_ref,
            sems):
    SW, SWO, SXL, SX, SH, SA, ST, SO, SS = 0, 16, 24, 28, 36, 44, 46, 48, 52
    w_hbms = (wq_hbm, wk_hbm, wv_hbm)
    a_hbms = (aq_hbm, ak_hbm, av_hbm)

    def aligned(x, n):
        return x if isinstance(x, int) else pl.multiple_of(x, n)

    def w_copy(m, hq, q=None):
        rows = pl.ds(0, D) if q is None else pl.ds(q * KQ, KQ)
        sem = SW + 12 + hq if q is None else SW + 4 * hq + q
        heads = aligned(8 * hq, 8)
        return pltpu.make_async_copy(
            w_hbms[m].at[rows, pl.ds(heads, 8), :], wstage.at[hq, rows], sems.at[sem])

    def self_wait(ref, sem):
        pltpu.make_async_copy(ref, ref, sems.at[sem]).wait()

    def late_start(k):
        pltpu.make_async_copy(
            wo_hbm.at[pl.ds(aligned(k * 512, 512), 512), :], wostage.at[k],
            sems.at[SWO + k]).start()
        pltpu.make_async_copy(
            ssmk_hbm.at[pl.ds(aligned(k * 128, 128), 128), :], hbuf.at[k],
            sems.at[SH + k]).start()

    def xlead_copy(q):
        return pltpu.make_async_copy(
            x_hbm.at[:, pl.ds(0, M), pl.ds(q * KQ, KQ)], xlead.at[q], sems.at[SXL + q])

    def x_copy(g):
        segs = pl.ds(g * 8, 8)
        return pltpu.make_async_copy(
            x_hbm.at[segs, pl.ds(M, SEG - M), :], xbuf.at[segs, pl.ds(M, SEG - M), :], sems.at[SX + g])

    def a_start(g):
        col = aligned(g * 128, 128)
        for t in (1, 2, 0):
            pltpu.make_async_copy(
                a_hbms[t].at[:, pl.ds(col, 128)], abuf.at[g & 1, t], sems.at[SA + (g & 1)]).start()

    tw_cp = pltpu.make_async_copy(tw_hbm, tw, sems.at[ST])

    small = [pltpu.make_async_copy(src, dst, sems.at[SS + i]) for i, (src, dst) in enumerate((
        (fill_hbm, fill_ref), (mem0_hbm, mem0_ref), (sk_hbm, sk_ref), (ssmd_hbm, ssmd_ref.at[0])))]

    for q in range(4):
        xlead_copy(q).start()
        w_copy(0, 0, q).start()
        if q > 0:
            w_copy(0, 1, q - 1).start()
    w_copy(0, 1, 3).start()
    for q in range(4):
        w_copy(0, 2, q).start()
    w_copy(0, 3).start()
    for cp in small:
        cp.start()

    kickbuf[...] = jnp.zeros(kickbuf.shape, F32)

    w_parts = (w_a, w_b)

    def slab_row(u, par, jl):
        return ((u >> 1) * 8 + par * 4 + jl) * SLAB

    def gated(x, i, n, gates):
        if gates is None:
            return x
        never, vals = gates
        v = vals[(i * len(vals) * cfg["gspan"]) // (n * 100)]
        return jnp.where(never, pltpu.bitcast(v, U32), x)

    def vregs(*mats):
        return [m_[r:r + 8] for m_ in mats for r in range(0, m_.shape[0], 8)]

    def relayout(u, g, q, gates=None, src=None):
        slot, qs = (u & 3, q) if src is None else src
        low = lax.broadcasted_iota(jnp.int32, (8, 128), 0) < 4
        keep = jnp.where(low, jnp.uint32(0xFFFF), jnp.uint32(0xFFFF0000))
        shl = jnp.where(low, jnp.uint32(16), jnp.uint32(0))
        base = slab_row(u, 0, 0) + q * (KQ // 2)
        for i in range(KQ // 2):
            x = wstage[slot, pl.ds(qs * KQ + 2 * i, 2)].reshape(16, DH)
            x = gated(pltpu.bitcast(x, U32), i, KQ // 2, gates)
            y = pltpu.roll(x, 4, 0)
            w_parts[g][pl.ds(base + i, 8, stride=SLAB), :] = (x & keep) | ((y << shl) >> (16 - shl))

    def comb(x, y, sign):
        return _widen(x) + _widen(y) if sign > 0 else _widen(x) - _widen(y)

    def as_bf16(b):
        return pltpu.bitcast(b, BF16) if b.dtype == U32 else b.astype(BF16)

    def put_lead(segs, n, it, a, b):
        both = jnp.concatenate([a.reshape(n, M, DH), b.reshape(n, M, DH)], axis=1)
        qkvb[segs, it] = _narrow(both)

    def batch_pair(u, g, jl):
        it = 4 * u + jl
        rows = [pl.multiple_of(slab_row(u, par, jl), 8) for par in range(2)]

        def blk(kh, par):
            return w_parts[g][pl.ds(rows[par] + kh * (D // 4), D // 4), :]

        def mm(a, b):
            return _dot(pltpu.bitcast(jnp.concatenate(a, axis=1), BF16), as_bf16(b))

        def xs(f):
            return [xs_u[f, q] for q in range(2)]
        a11 = [xlead_u[q, pl.ds(0, HR), :] for q in (0, 1)]
        a22 = [xlead_u[q, pl.ds(HR, HR), :] for q in (2, 3)]
        m5 = mm(xs(2), blk(1, 1))
        m1 = mm(xs(0), comb(blk(0, 0), blk(1, 1), 1))
        m4 = mm(a22, comb(blk(1, 0), blk(0, 0), -1))
        c11 = mm(xs(4), comb(blk(1, 0), blk(1, 1), 1)) + (m1 + m4 - m5)
        m3 = mm(a11, comb(blk(0, 1), blk(1, 1), -1))
        put_lead(pl.ds(0, NSEG // 2), NSEG // 2, it, c11, m3 + m5)
        m2 = mm(xs(1), blk(0, 0))
        c22 = mm(xs(3), comb(blk(0, 0), blk(0, 1), 1)) + (m1 - m2 + m3)
        put_lead(pl.ds(NSEG // 2, NSEG // 2), NSEG // 2, it, m2 + m4, c22)
        return vregs(m5, m1, m4, c11, m3, m2, c22)

    def quarter_wait(u, q):
        self_wait(wstage.at[u, pl.ds(pl.multiple_of(q * KQ, KQ), KQ)], SW + 4 * u + q)

    def first_unit(q, carry):
        never = q > 1000
        half = q & 1
        self_wait(xlead.at[q], SXL + q)
        quarter_wait(0, q)
        xlead_u[q] = _narrow(xlead[q].astype(F32).reshape(NSEG * M, KQ))
        relayout(0, 0, q)

        @pl.when(q > 0)
        def _():
            quarter_wait(1, q - 1)
        res = []
        xq = pltpu.bitcast(xlead_u[q], BF16)
        for jl in range(4):
            outs = []
            for par in range(2):
                acc = pl.ds((2 * jl + par) * (NSEG * M), NSEG * M)
                row = pl.multiple_of(slab_row(0, par, jl) + q * (KQ // 2), 8)
                w = pltpu.bitcast(w_a[pl.ds(row, KQ // 2), :], BF16)
                d = _dot(xq, w) + jnp.where(q == 0, 0.0, wk[acc, :])
                wk[acc, :] = d
                outs.append(d)
            put_lead(pl.ds(0, NSEG), NSEG, jl, outs[0], outs[1])
            res += outs
        gates = (never, vregs(*res))
        qn = jnp.maximum(q - 1, 0)
        relayout(1, 1, qn, gates, src=(jnp.minimum(q, 1), qn))
        for r in range(0, HR, 8):
            for cb in range(2):
                cols = pl.ds(cb * 128, 128)
                i = 2 * (r // 8) + cb
                a11 = gated(xlead_u[half, pl.ds(r, 8), cols], i, HR // 4, gates)
                a22 = gated(xlead_u[2 + half, pl.ds(HR + r, 8), cols], i, HR // 4, gates)
                a21 = xlead_u[half, pl.ds(HR + r, 8), cols]
                a12 = xlead_u[2 + half, pl.ds(r, 8), cols]
                for f, (x, y, sg) in enumerate(((a11, a22, 1), (a21, a22, 1), (a11, a12, 1),
                                                (a21, a11, -1), (a12, a22, -1))):
                    xs_u[f, half, pl.ds(r, 8), cols] = _narrow(comb(x, y, sg))
        return carry
    lax.fori_loop(0, 4, first_unit, 0)
    w_copy(1, 0).start()
    late_start(0)
    w_copy(0, 1, 3).wait()
    relayout(1, 1, 3)

    def second_unit(jl, carry):
        quarter_wait(2, jl)
        relayout(2, 0, jl, (jl > 1000, batch_pair(1, 1, jl)))
        return carry
    lax.fori_loop(0, 4, second_unit, 0)

    def late_relayout(src, k, jl, gates):
        half = jl // 2
        hp = 2 * k + half
        for ri in range(4):
            r = 4 * (jl % 2) + ri
            blk = [pltpu.bitcast(wostage[src, pl.ds(half * 256 + e * 128 + r * 16, 16), :], U32)
                   for e in range(2)]
            for np_ in range(NB // 2):
                b = [[gated(blk[e][:, (2 * np_ + c) * 128:(2 * np_ + c + 1) * 128],
                            ri * 4 + np_, 16, gates) for c in range(2)] for e in range(2)]
                for e in range(2):
                    for c in range(2):
                        wo_u[2 * np_ + c, pl.ds(pl.multiple_of(hp * 128 + e * 64 + r * 8, 8), 8), :] = b[e][c]
                rows = pl.ds(pl.multiple_of(hp * 64 + r * 8, 8), 8)
                for f, (x, y, sg) in enumerate(((b[0][0], b[1][1], 1), (b[0][1], b[1][1], -1),
                                                (b[1][0], b[0][0], -1), (b[0][0], b[0][1], 1),
                                                (b[1][0], b[1][1], 1))):
                    wo_s[f, np_, rows, :] = _narrow(comb(x, y, sg))
        for t in range(4):
            tile = pltpu.bitcast(hbuf[src, :, pl.ds((4 * jl + t) * 128, 128)], U32)
            tile = jnp.concatenate([gated(tile[0:8], t, 4, gates), tile[8:]], axis=0)
            row = pl.multiple_of(k * 1024 + (4 * jl + t) * 64, 64)
            ht[pl.ds(row, 64), :] = pltpu.bitcast(pltpu.bitcast(tile, BF16).T, U32)

    def unit_body(u, g):
        @pl.when(u < 11)
        def _():
            self_wait(wstage.at[(u + 1) & 3], SW + 12 + ((u + 1) & 3))

        @pl.when(u >= 4)
        def _():
            self_wait(wostage.at[u - 4], SWO + u - 4)
            self_wait(hbuf.at[u - 4], SH + u - 4)
        for m in (1, 2):
            @pl.when((u + 3) >> 2 == m)
            def _():
                w_copy(m, (u + 3) & 3).start()

        @pl.when(u <= 8)
        def _():
            late_start(u - 1)
        if g == 1:
            @pl.when(u == 9)
            def _():
                x_copy(0).start()
                a_start(0)
                tw_cp.start()
        for jl in range(4):
            gates = (u > 1000, batch_pair(u, g, jl))
            relayout(jnp.where(u < 11, u + 1, u - 1), 1 - g, jl, gates)
            late_relayout(jnp.where(u >= 4, u - 4, 8), jnp.maximum(u - 4, 0), jl, gates)

    def unit_pair(mm, carry):
        for g in range(2):
            unit_body(2 * mm + g, g)
        return carry
    lax.fori_loop(1, 6, unit_pair, 0)

    a_start(1)
    for g in range(1, NG):
        x_copy(g).start()
    for cp in small:
        cp.wait()
    dd = ssmd_ref[0].astype(F32)
    for g in range(NG):
        sk = sk_ref[g].astype(F32)
        for j in range(KS):
            taps[g, j] = jnp.broadcast_to(sk[j:j + 1], (8, 128))
        taps[g, KS] = jnp.broadcast_to(dd[g:g + 1], (8, 128))

    def part_a(i, kick):
        g, j = i >> 1, i & 1
        sl = g & 1
        never = i > 1000
        sub = lax.broadcasted_iota(jnp.int32, (8, 128), 0)
        kickbuf[jnp.where(never, 1, 0)] = kick
        chain = [kickbuf[jnp.where(i > 2000, 0, 1)]]

        def begin(xs, ng):
            xs = list(xs)
            for e in range(min(ng, len(xs))):
                c = chain[0]
                c = c if c.dtype == xs[e].dtype else pltpu.bitcast(c, xs[e].dtype)
                xs[e] = jnp.where(never, c, xs[e])
            return xs

        def merge(vals):
            c = vals[-1]
            for v in list(vals[:-1])[:cfg["a_merge"]]:
                c = jnp.maximum(v, c)
            chain[0] = c

        def ld(v):
            if isinstance(v, tuple):
                blk, ri, r = v
                base = 8 * WS + 256 * blk + 16 * ri + 32 * r
                lo = wk[pl.ds(base, 8), :]
                if r == 0:
                    return lo
                return pltpu.roll(jnp.where(sub >= r, lo, wk[pl.ds(base + 8, 8), :]), 8 - r, 0)
            return wk[pl.ds(8 * v, 8), :]

        def st(v, x):
            wk[pl.ds(8 * v, 8), :] = x

        def twid(idx):
            return (tw[j, idx], tw[j, idx + 1])

        def pairs(flat):
            return [(flat[2 * e], flat[2 * e + 1]) for e in range(len(flat) // 2)]

        def fwd4(locs, t0):
            v = pairs(begin([ld(x) for loc in locs[::-1] for x in loc], cfg["a_g4"]))[::-1]
            return _dft4([v[0]] + [_cmul(v[r], twid(t0 + 2 * r)) for r in range(1, 4)], +1)

        def inv4(v, t0):
            o = _dft4(v, -1)
            return [o[0]] + [_cmulc(o[r], twid(t0 + 2 * r)) for r in range(1, 4)]

        def ld4(locs):
            return pairs(begin([ld(x) for loc in locs for x in loc], cfg["a_g4i"]))

        def put4(locs, o):
            for loc, x in zip(locs, o):
                st(loc[0], x[0])
                st(loc[1], x[1])
            merge([x for c in o for x in c])

        def put4_t(dsts, o):
            for (blk, slot), x in zip(dsts, o):
                for ri in range(2):
                    base = 8 * WS + 256 * blk + 16 * ri + slot
                    wk[pl.ds(base, 8, stride=33), :] = x[ri]
            merge([x for c in o for x in c])

        def xloc(sig, n):
            return (WX + 256 * sig + 2 * n, WX + 256 * sig + 2 * n + 1)

        def sloc(kb, l):
            return ((2 * kb + l // 8, 0, l % 8), (2 * kb + l // 8, 1, l % 8))

        def pass_kv():
            t = [taps[g, a] for a in range(KS)]
            prev = [None] + [jnp.zeros((8, 128), F32)] * (KS - 1)
            for v in range(S // 16):
                w, = begin([pltpu.bitcast(abuf[sl, 1, pl.ds(16 * v, 16), :], U32)], 1)
                k2 = _widen(w)
                v2 = abuf[sl, 2, pl.ds(16 * v, 16), :].astype(F32)
                outs = []
                for hh in range(2):
                    x = k2[8 * hh:8 * hh + 8]
                    cur = [None] + [pltpu.roll(x, a, 0) for a in range(1, KS)]
                    ks = x * t[0]
                    for a in range(1, KS):
                        ks = ks + jnp.where(sub < a, prev[a], cur[a]) * t[a]
                    prev = cur
                    kv = (ks * v2[8 * hh:8 * hh + 8]).astype(BF16).astype(F32)
                    st(WK + 2 * v + hh, kv)
                    outs.append(kv)
                merge(outs)

        def forward(sig, src):
            for n in range(32):
                x = src(n)
                cs = []
                for d in range(4):
                    a, b = twid(TAF + 2 * d), twid(TAF + 2 * (d + 4))
                    if d == 0:
                        s_ = x[4] * b[0]
                        cs.append((x[0] + s_, s_))
                    else:
                        cs.append((x[d] * a[0] + x[d + 4] * b[0], x[d] * a[1] + x[d + 4] * b[1]))
                put4([xloc(sig, n + 32 * k0) for k0 in range(4)], _dft4(cs, +1))
            for k0 in range(4):
                for n in range(8):
                    locs = [xloc(sig, n + 8 * r + 32 * k0) for r in range(4)]
                    put4(locs, fwd4(locs, TB + 8 * k0))
            for k0 in range(4):
                for k1 in range(4):
                    k = k0 + 4 * k1
                    for a in range(2):
                        o = fwd4([xloc(sig, a + 2 * r + 8 * k1 + 32 * k0) for r in range(4)], TC + 8 * k)
                        put4_t([(2 * ((k + 16 * k2) // 8) + a, k % 8) for k2 in range(4)], o)
            for kb in range(8):
                for e in range(4):
                    o = fwd4([sloc(kb, e + 4 * r) for r in range(4)], TD + 8 * kb)
                    put4([xloc(sig, 16 * kb + e + 4 * r) for r in range(4)], o)
            for kb in range(8):
                for k3 in range(4):
                    locs = [xloc(sig, 16 * kb + r + 4 * k3) for r in range(4)]
                    t0 = TE + 8 * (4 * kb + k3)
                    o = fwd4(locs, t0)
                    if sig == 0:
                        hs = ld4([xloc(1, 16 * kb + r + 4 * k3) for r in range(4)])
                        o = inv4([_cmul(a, b) for a, b in zip(o, hs)], t0)
                    put4(locs, o)

        def inverse():
            for kb in range(8):
                for e in range(4):
                    o = inv4(ld4([xloc(0, 16 * kb + e + 4 * r) for r in range(4)]), TD + 8 * kb)
                    put4_t([(2 * kb + (e + 4 * f) // 8, (e + 4 * f) % 8) for f in range(4)], o)
            for k0 in range(4):
                for k1 in range(4):
                    k = k0 + 4 * k1
                    for a in range(2):
                        v = ld4([sloc((k + 16 * r) // 8, 8 * a + k % 8) for r in range(4)])
                        put4([xloc(0, a + 2 * b + 8 * k1 + 32 * k0) for b in range(4)], inv4(v, TC + 8 * k))
            for k0 in range(4):
                for n in range(8):
                    locs = [xloc(0, n + 8 * r + 32 * k0) for r in range(4)]
                    put4(locs, inv4(ld4(locs), TB + 8 * k0))
            dskip = taps[g, KS]
            for n0 in range(32):
                cs = _dft4(ld4([xloc(0, n0 + 32 * r) for r in range(4)]), -1)
                outs = []
                for d in [d0 + 4 * hh for d0 in range(4) for hh in range(2)]:
                    n = n0 + 32 * d
                    a = twid(TAI + 2 * d)
                    if 0 < d < 4:
                        cs[d] = tuple(begin(cs[d], 2))
                    c = cs[d % 4]
                    y = c[0] * a[0] if d == 0 else c[0] * a[0] + c[1] * a[1]
                    y = y + jnp.where(j == 0, ld(WK + n) * dskip, ld(WY + n))
                    st(WY + n, y)
                    chain[0] = abuf[sl, 0, pl.ds(8 * n, 8), :].astype(F32) * y
                    aout[g, n // 4, pl.ds(8 * (n % 4), 8), :] = chain[0].astype(BF16)
                    outs.append(chain[0])
                merge(outs)

        def filt(n):
            base = pl.multiple_of(g * (S // 2), S // 2)
            ws = begin([ht[pl.ds(base + 8 * (n // 2 + 16 * d), 8), :] for d in range(8)], 8)
            return [_widen(w)[8 * (n % 2):8 * (n % 2) + 8] for w in ws]
        pass_kv()
        forward(1, filt)
        forward(0, lambda n: begin([ld(WK + n + 32 * d) for d in range(8)], 8))
        inverse()
        return chain[0]

    scale = DH ** (-0.5)

    def w_slab(m, h):
        u = 4 * m + h // 8
        return pltpu.bitcast(w_parts[u % 2][pl.ds(slab_row(u, h % 2, (h // 2) % 4), D // 2), :], BF16)

    class Step:
        def __init__(self, s, leads, mem):
            self.s = s
            self.leads = leads
            self.acc2 = [None] * NB
            self.qkv, self.ps, self.os = {}, {}, []
            self.acc = [None] * NB
            self.ocat, self.early, self.marks, self.heads = {}, {}, {}, {}
            self.tie = None
            x = xbuf[s, pl.ds(M, SEG - M), :].astype(F32)
            self.lhsf = jnp.concatenate([mem, x], axis=0)
            self.lhs = self.lhsf.astype(BF16)

        def proj_early(self, m, h, k):
            self.early[m, h] = (k, _dot(self.lhsf[:, :k].astype(BF16), w_slab(m, h)[:k]))

        def proj(self, m, h):
            if (m, h) in self.early:
                k, part = self.early[m, h]
                d = _dot(self.lhsf[:, k:].astype(BF16), w_slab(m, h)[k:]) + part
            else:
                d = _dot(self.lhs, w_slab(m, h))
            self.heads[m, h] = d
            j = h // 2
            if (m, h ^ 1) not in self.heads:
                return
            a, b = self.heads[m, 2 * j], self.heads[m, 2 * j + 1]
            self.marks[m, j] = a[0:8]
            lead = _widen(qkvb[self.s, m * NPAIR + j])
            self.qkv[m, j] = jnp.concatenate([a, b, lead], axis=0).astype(BF16)

        def probs(self, j):
            fill = fill_ref[pl.ds(0, R), pl.ds(0, R)]
            qk = _dot_nt(self.qkv[0, j], self.qkv[1, j])
            sc = jnp.where(fill == 0.0, qk * scale, fill)
            e = jnp.exp(sc - jnp.max(sc, axis=-1, keepdims=True))
            l = jnp.sum(e, axis=-1, keepdims=True)
            r = pl.reciprocal(l, approx=True)
            r = r * (2.0 - l * r)
            self.ps[j] = (e * r).astype(BF16)

        def attend(self, j):
            o = _dot(self.ps[j], self.qkv[2, j])
            self.leads[2 * j].append(o[2 * SEG:2 * SEG + M])
            self.leads[2 * j + 1].append(o[2 * SEG + M:])
            self.os += [o[0:SEG], o[SEG:2 * SEG]]

        def tied(self, w):
            if self.tie is not None:
                w = jnp.concatenate(
                    [jnp.where(self.s > 1000, pltpu.bitcast(self.tie, U32), w[0:8]), w[8:]], axis=0)
                self.tie = None
            return pltpu.bitcast(w, BF16)

        def wo_strassen(self, j0, j1, np_, f):
            if (j0, f) not in self.ocat:
                parts = []
                for j in range(j0, j1):
                    a11, a12 = self.os[2 * j], self.os[2 * j + 1]
                    a21, a22 = [jnp.concatenate(self.leads[2 * j + e], axis=0) for e in range(2)]
                    parts.append({1: lambda: a11 + a22, 2: lambda: a21 + a22, 3: lambda: a11,
                                  4: lambda: a22, 5: lambda: a11 + a12, 6: lambda: a21 - a11,
                                  7: lambda: a12 - a22}[f]())
                self.ocat[j0, f] = jnp.concatenate(parts, axis=1).astype(BF16)
            if f in (2, 5):
                e = (2, 5).index(f)
                w = jnp.concatenate([wo_u[2 * np_ + e, pl.ds((2 * j + e) * 64, 64), :]
                                     for j in range(j0, j1)], axis=0)
            else:
                w = wo_s[(1, 3, 4, 6, 7).index(f), np_, pl.ds(j0 * 64, (j1 - j0) * 64), :]
            d = _dot(self.ocat[j0, f], self.tied(w))
            uses = {1: ((0, 0, 1), (1, 1, 1)), 2: ((1, 0, 1), (1, 1, -1)), 3: ((0, 1, 1), (1, 1, 1)),
                    4: ((0, 0, 1), (1, 0, 1)), 5: ((0, 1, 1), (0, 0, -1)), 6: ((1, 1, 1),),
                    7: ((0, 0, 1),)}[f]
            for which, c, sg in uses:
                acc = (self.acc, self.acc2)[which]
                n = 2 * np_ + c
                if acc[n] is None:
                    assert sg > 0
                    acc[n] = d
                else:
                    acc[n] = d + acc[n] if sg > 0 else acc[n] - d

        def wo(self, h0, h1, n):
            if h0 not in self.ocat:
                self.ocat[h0] = jnp.concatenate(self.os[h0:h1], axis=1).astype(BF16)
            d = _dot(self.ocat[h0], self.tied(wo_u[n, pl.ds(h0 * 64, (h1 - h0) * 64), :]))
            self.acc[n] = d if self.acc[n] is None else d + self.acc[n]

        def finish(self):
            res = jnp.concatenate(self.acc, axis=1)
            obuf[self.s, pl.ds(M, SEG - M), :] = res[M:].astype(BF16)
            if self.acc2[0] is not None:
                lead = jnp.concatenate(self.acc2, axis=1)
                for e in range(U):
                    obuf[self.s - (U - 1) + e, pl.ds(0, M), :] = lead[M * e:M * e + M].astype(BF16)
            return res[0:M]

    def steps(i, mem):
        def send(segs, rows):
            pltpu.make_async_copy(
                obuf.at[segs, rows], out_hbm.at[segs, rows, pl.ds(D, D)], sems.at[SO]).start()
        sts = []
        leads = [[] for _ in range(H)]
        for u in range(U):
            st = Step(i * U + u, leads, mem)
            sts.append(st)
            for item in _step_order(u, cfg):
                if item[0] == "A":
                    ku, km, kj = cfg["kick"]
                    st.tie = part_a(i, sts[ku].marks[km, kj])
                elif item[0] == "O":
                    last_half = (i & 1) == 1
                    pl.when(last_half)(lambda: a_send(i >> 1))
                    pl.when(jnp.logical_and(last_half, i < 2 * NG - 4))(lambda: a_start((i >> 1) + 2))
                    send(pl.ds(i * U, U - 1), pl.ds(M, SEG - M))
                else:
                    dict(P=st.proj, E=st.proj_early, S=st.probs, V=st.attend, W=st.wo,
                         X=st.wo_strassen)[item[0]](*item[1:])
            mem = st.finish()
        send(pl.ds(i * U, U - 1), pl.ds(0, M))
        send(pl.ds(i * U + U - 1, 1), pl.ds(0, SEG))
        return mem

    def a_send(g):
        pltpu.make_async_copy(
            aout.at[g], out_hbm.at[:, :, pl.ds(pl.multiple_of(g * 128, 128), 128)],
            sems.at[SO + 1]).start()

    def group(g, mem):
        x_copy(g).wait()
        self_wait(abuf.at[g & 1], SA + (g & 1))
        return lax.fori_loop(0, 2, lambda j, m_: steps(2 * g + j, m_), mem)

    tw_cp.wait()
    lax.fori_loop(0, NG, group, mem0_ref[...].astype(F32))
    self_wait(obuf, SO)
    self_wait(aout, SO + 1)


def _step_order(u, cfg):
    cfg = dict(cfg, **cfg["sub"][u])
    ks = cfg["ks"]
    tmpl = []
    for x in cfg["tmpl"].split():
        kind, lag = x[:-1], int(x[-1])
        tmpl += [(kind + "a", lag), (kind + "b", lag)] if kind in ("q", "k", "v") else [(kind, lag)]

    def proj(kind, j):
        return ("qkv".index(kind[0]), 2 * j + "ab".index(kind[1]))
    if u < U - 1:
        fill = [[("W", 0, ks, n)] for n in range(NB)]
        last = [("W", ks, H, n) for n in range(NB)]
    else:
        def products(j0, j1, f_outer):
            fs = (1, 4, 7, 3, 5, 2, 6)
            if f_outer:
                return [("X", j0, j1, np_, f) for f in fs for np_ in range(NB // 2)]
            return [("X", j0, j1, np_, f) for np_ in range(NB // 2) for f in fs]
        xs = products(0, ks // 2, cfg["xo"] & 1)
        fill = [xs[e:e + 2] for e in range(0, len(xs), 2)]
        last = products(ks // 2, NPAIR, cfg["xo"] & 2)
        last.insert(len(last) - cfg["send_back"], ("O",))
        last.insert(len(last) - 1 - cfg["tie_back"], ("A",))
    out = []
    for t in range(NPAIR + 1 + max(l for _, l in tmpl)):
        for kind, lag in tmpl:
            j = t - lag
            if j < 0:
                continue
            if j >= NPAIR:
                if kind[1:] == "a" and fill:
                    out += fill.pop(0)
                continue
            out.append(("P",) + proj(kind, j) if len(kind) == 2 else (kind, j))
    if u > 0:
        first = [x[1:] for x in out if x[0] == "P"][:cfg["ne"]]
        out = [("E",) + x + (cfg["ek"],) for x in first] + out
    return out + [x for f in fill for x in f] + last


_DEFAULT_CFG = dict(
    sub=(dict(tmpl='ka0 kb0 S1 va0 qa0 V2 qb0 vb0', ks=24, ne=4, ek=640),
         dict(tmpl='ka0 V3 va1 kb0 qa0 S1 vb1 qb0', ks=20, ne=3, ek=640),
         dict(tmpl='qa0 qb0 ka0 V3 kb0 S1 va2 vb2', ks=24, ne=3, ek=768),
         dict(tmpl='ka0 V3 va1 kb0 qa0 S1 vb1 qb0', ks=16, ne=3, ek=640)),
    tie_back=28, send_back=26, xo=0, gspan=75, kick=(0, 1, 0), a_merge=5, a_g4=4, a_g4i=8)


def _build(cfg):
    tw_np = _twiddles()
    fill_np = np.zeros((96, 128), np.float32)
    fill_np[:R, :R] = _mask_fill()

    def run(A_q, A_k, A_v, A_shift_k, A_ssm_k, A_ssm_D, B_x, B_mem0, B_Wq, B_Wk, B_Wv, B_Wo):
        sk = A_shift_k.T.reshape(KS, NG, 128).transpose(1, 0, 2)
        any_spec = pl.BlockSpec(memory_space=pl.ANY)
        out = pl.pallas_call(
            functools.partial(_kernel, cfg),
            out_shape=jax.ShapeDtypeStruct((NSEG, SEG, 2 * D), BF16),
            in_specs=[any_spec] * 14,
            out_specs=any_spec,
            scratch_shapes=[
                pltpu.VMEM((48 * SLAB + 544, 128), U32),
                pltpu.VMEM((48 * SLAB + 544, 128), U32),
                pltpu.VMEM((NB, H * DH // 2, 128), U32),
                pltpu.VMEM((4, D, 8, DH), BF16),
                pltpu.VMEM((9, 512, D), BF16),
                pltpu.VMEM((NSEG, SEG, D), BF16),
                pltpu.VMEM((4, NSEG, M, KQ), BF16),
                pltpu.VMEM((4, NSEG * M // 2, KQ), U32),
                pltpu.VMEM((5, 2, HR, KQ), U32),
                pltpu.VMEM((NSEG, 3 * NPAIR, 8, 128), U32),
                pltpu.VMEM((5, NB // 2, H * DH // 4, 128), U32),
                pltpu.VMEM((NSEG, SEG, D), BF16),
                pltpu.VMEM((2, 3, S, 128), BF16),
                pltpu.VMEM((NG + 1, 128, S), BF16),
                pltpu.VMEM((NG * S // 2, 128), U32),
                pltpu.VMEM((8 * NW + 32, 128), F32),
                pltpu.VMEM((2, NT, 8, 128), F32),
                pltpu.VMEM((NG, NSEG, SEG, 128), BF16),
                pltpu.VMEM((4, 8, 128), F32),
                pltpu.VMEM((96, 128), F32),
                pltpu.VMEM((NG, 8, 8, 128), F32),
                pltpu.VMEM((M, D), BF16),
                pltpu.VMEM((NG, KS, 128), BF16),
                pltpu.VMEM((4, NG, 128), BF16),
                pltpu.SemaphoreType.DMA((56,)),
            ],
            compiler_params=pltpu.CompilerParams(vmem_limit_bytes=124 * 1024 * 1024,
                                                 disable_bounds_checks=True),
        )(A_q.reshape(S, D), A_k.reshape(S, D), A_v.reshape(S, D), sk, A_ssm_k,
          A_ssm_D.reshape(NG, 128), B_x.reshape(NSEG, SEG, D), B_mem0.reshape(M, D),
          B_Wq, B_Wk, B_Wv, B_Wo.reshape(H * DH, D),
          jnp.asarray(tw_np), jnp.asarray(fill_np))
        return out.reshape(1, S, 2 * D)

    return run


@jax.jit
def pallas_concat_heads__ssm_conv_h3__memory_aug_recurrent_mem_tr__prompt_kernel(
    A_q: jax.Array,
    A_k: jax.Array,
    A_v: jax.Array,
    A_shift_k: jax.Array,
    A_ssm_k: jax.Array,
    A_ssm_D: jax.Array,
    B_x: jax.Array,
    B_mem0: jax.Array,
    B_Wq: jax.Array,
    B_Wk: jax.Array,
    B_Wv: jax.Array,
    B_Wo: jax.Array,
    B_seg_len: jax.Array,
):
    del B_seg_len
    return _build(_DEFAULT_CFG)(A_q, A_k, A_v, A_shift_k, A_ssm_k, A_ssm_D, B_x, B_mem0,
                                B_Wq, B_Wk, B_Wv, B_Wo)
```

```python
import functools

import numpy as np
import jax
import jax.numpy as jnp
from jax import lax
import jax.experimental.pallas as pl
import jax.experimental.pallas.tpu as pltpu

F32 = jnp.float32
BF16 = jnp.bfloat16
U32 = jnp.uint32

S = 2048
D = 1024
H = 32
DH = 128
M = 8
SEG = 32
NSEG = S // SEG
U = 4
NPAIR = H // 2
R = 2 * (M + SEG)
SLAB = 520
KS = 4
NG = D // 128
KQ = D // 4
NB = D // 128
HR = NSEG * M // 4

TAF, TAI, TB, TC, TD, TE, NT = 0, 16, 32, 64, 192, 256, 512
WX, WS, WY, WK, NW = 0, 512, 1024, 1280, 1536


_STRASSEN = (
    ("+00 +11", "+00 +11", "+00 +11"), ("+11", "+10 -00", "+00 +10"), ("+01 -11", "+10 +11", "+00"),
    ("+00", "+01 -11", "+01 +11"), ("+00 +01", "+11", "+01 -00"), ("+10 +11", "+00", "+10 -11"),
    ("+10 -00", "+00 +01", "+11"),
)
_HK26 = (
    ("+00 +10", "+00 +02 +03 -10 -30", "+10"),
    ("+01", "+10 +11 +13 +21", "+01"),
    ("+11", "+01 +12 +31 -11", "-11"),
    ("+02 +12", "+12 +20 +22 +23 -30", "+02"),
    ("+03 +13", "+32 +33 -13", "+13"),
    ("+00", "+00 +01 +30 -03 -20", "+00 -10"),
    ("+12", "+02 +03 +21 +32 -22", "+02 -12"),
    ("+03", "+31 +33 -23", "+03 -13"),
    ("+00 +01 +10 +11", "+10", "+00 -01"),
    ("+12 -00", "+02 +03 +20 -30", "+10 -02"),
    ("+00 +02", "+20 -30", "+00 -02"),
    ("+10 +12", "+02 +03", "+12 -10"),
    ("+02 +12 -01 -11", "+12", "-11 -12"),
    ("+01 +03 +11 +13", "+13", "+03 -01"),
    ("+03 -12", "+23 +32", "+02 -13"),
    ("+02 +03", "+30 -23", "+02 -03"),
    ("+12 +13", "+03 +32", "+12 -13"),
    ("+00 +10 +11", "+01 +10", "+01 +10 -00"),
    ("+02 +12 -01", "+12 +21", "+11 +12 -02"),
    ("+03 +11 +13", "+13 +31", "+01 +13 -03"),
    ("+00 +02 +03 +10 +12 +13", "+30", "+00 +03 -02"),
    ("+10 +11", "+01", "+00 +11 -01 -10"),
    ("+02 -01", "+21", "+01 +02 -11 -12"),
    ("+11 +13", "+31", "+03 +11 -01 -13"),
    ("+00 +10 +12 +13", "+03 -30", "+00 +03 -02 -10"),
    ("+10 +12 +13", "+03", "+02 +10 +13 -00 -03 -12"),
)


def _scheme(name):
    tab = {2: _STRASSEN, 4: _HK26}[name]
    terms = [[[(int(t[1]), int(t[2]), t[0] == "+") for t in f.split()] for f in p] for p in tab]
    stored = [i for i, p in enumerate(terms) if len(p[1]) > 1]
    return terms, stored


def _signed_sum(terms, get):
    acc = None
    for r, c, plus in terms:
        x = get(r, c)
        acc = x if acc is None else (acc + x if plus else acc - x)
    return acc


def _twiddles():
    tw = np.zeros((2, NT, 8), np.float64)

    def put(j, idx, z):
        tw[j, idx] = np.real(z)
        tw[j, idx + 1] = np.imag(z)
    s = np.arange(8)
    tau = 2j * np.pi
    for j in range(2):
        lx = 1j * np.pi * (1 + 4 * j) / 4096
        for d in range(8):
            put(j, TAF + 2 * d, np.exp(lx * 256 * d))
            put(j, TAI + 2 * d, np.exp(lx * 256 * d) / 2048)
        for r in range(4):
            for k in range(4):
                put(j, TB + 8 * k + 2 * r, np.exp((lx * 64 + tau * k / 16) * r))
            for k in range(16):
                put(j, TC + 8 * k + 2 * r, np.exp((lx * 16 + tau * k / 64) * r))
            for kb in range(8):
                put(j, TD + 8 * kb + 2 * r, np.exp((lx * 4 + tau * (s + 8 * kb) / 256) * r))
                for k3 in range(4):
                    put(j, TE + 8 * (4 * kb + k3) + 2 * r,
                        np.exp((lx + tau * (s + 8 * kb + 64 * k3) / 1024) * r))
    return np.ascontiguousarray(np.broadcast_to(tw[..., None], (2, NT, 8, 128))).astype(np.float32)


def _mask_fill():
    blk = np.concatenate([np.arange(M), M + np.arange(M, SEG)])
    lead = M + np.arange(M)
    head = np.concatenate([np.zeros(SEG), np.ones(SEG), np.zeros(M), np.ones(M)])
    pos = np.concatenate([blk, blk, lead, lead])
    same = head[:, None] == head[None, :]
    ok = (pos[:, None] < M) | (pos[:, None] >= pos[None, :])
    fill = np.where(same, np.where(ok, 0.0, -1e9), -np.inf)
    return fill.astype(np.float32)


def _widen(w):
    return pltpu.bitcast(w, BF16).astype(F32)


def _narrow(x):
    return pltpu.bitcast(x.astype(BF16), U32)


def _dot(a, b):
    return jnp.dot(a, b, preferred_element_type=F32)


def _dot_nt(a, b):
    return lax.dot_general(a, b, (((1,), (1,)), ((), ())), preferred_element_type=F32)


def _cadd(a, b):
    return (a[0] + b[0], a[1] + b[1])


def _csub(a, b):
    return (a[0] - b[0], a[1] - b[1])


def _cmul(a, w):
    return (a[0] * w[0] - a[1] * w[1], a[0] * w[1] + a[1] * w[0])


def _cmulc(a, w):
    return (a[0] * w[0] + a[1] * w[1], a[1] * w[0] - a[0] * w[1])


def _bfly_i(b, d, sg):
    p = (b[0] - d[1], b[1] + d[0])
    q = (b[0] + d[1], b[1] - d[0])
    return (p, q) if sg > 0 else (q, p)


def _dft4(x, sg):
    a, b = _cadd(x[0], x[2]), _csub(x[0], x[2])
    c, d = _cadd(x[1], x[3]), _csub(x[1], x[3])
    p, q = _bfly_i(b, d, sg)
    return [_cadd(a, c), p, _csub(a, c), q]


def _kernel(cfg,
            aq_hbm, ak_hbm, av_hbm, sk_hbm, ssmk_hbm, ssmd_hbm, x_hbm, mem0_hbm,
            wq_hbm, wk_hbm, wv_hbm, wo_hbm, tw_hbm, fill_hbm,
            out_hbm,
            w_a, w_b, wo_u, wstage, wostage, xbuf, xlead, xlead_u, xs_u, qkvb, wo_s, obuf,
            abuf, hbuf, ht, wk, tw, aout, kickbuf,
            fill_ref, taps, mem0_ref, sk_ref, ssmd_ref,
            sems):
    SW, SWO, SXL, SX, SH, SA, ST, SO, SS = 0, 16, 24, 28, 36, 44, 46, 48, 52
    w_hbms = (wq_hbm, wk_hbm, wv_hbm)
    a_hbms = (aq_hbm, ak_hbm, av_hbm)

    def aligned(x, n):
        return x if isinstance(x, int) else pl.multiple_of(x, n)

    def w_copy(m, hq, q=None):
        rows = pl.ds(0, D) if q is None else pl.ds(q * KQ, KQ)
        sem = SW + 12 + hq if q is None else SW + 4 * hq + q
        heads = aligned(8 * hq, 8)
        return pltpu.make_async_copy(
            w_hbms[m].at[rows, pl.ds(heads, 8), :], wstage.at[hq, rows], sems.at[sem])

    def self_wait(ref, sem):
        pltpu.make_async_copy(ref, ref, sems.at[sem]).wait()

    def late_start(k):
        pltpu.make_async_copy(
            wo_hbm.at[pl.ds(aligned(k * 512, 512), 512), :], wostage.at[k],
            sems.at[SWO + k]).start()
        pltpu.make_async_copy(
            ssmk_hbm.at[pl.ds(aligned(k * 128, 128), 128), :], hbuf.at[k],
            sems.at[SH + k]).start()

    def xlead_copy(q):
        return pltpu.make_async_copy(
            x_hbm.at[:, pl.ds(0, M), pl.ds(q * KQ, KQ)], xlead.at[q], sems.at[SXL + q])

    def x_copy(g):
        segs = pl.ds(g * 8, 8)
        return pltpu.make_async_copy(
            x_hbm.at[segs, pl.ds(M, SEG - M), :], xbuf.at[segs, pl.ds(M, SEG - M), :], sems.at[SX + g])

    def a_start(g):
        col = aligned(g * 128, 128)
        for t in (1, 2, 0):
            pltpu.make_async_copy(
                a_hbms[t].at[:, pl.ds(col, 128)], abuf.at[g & 1, t], sems.at[SA + (g & 1)]).start()

    tw_cp = pltpu.make_async_copy(tw_hbm, tw, sems.at[ST])

    small = [pltpu.make_async_copy(src, dst, sems.at[SS + i]) for i, (src, dst) in enumerate((
        (fill_hbm, fill_ref), (mem0_hbm, mem0_ref), (sk_hbm, sk_ref), (ssmd_hbm, ssmd_ref.at[0])))]

    for q in range(4):
        xlead_copy(q).start()
        w_copy(0, 0, q).start()
        if q > 0:
            w_copy(0, 1, q - 1).start()
    w_copy(0, 1, 3).start()
    for q in range(4):
        w_copy(0, 2, q).start()
    w_copy(0, 3).start()
    for cp in small:
        cp.start()

    kickbuf[...] = jnp.zeros(kickbuf.shape, F32)

    w_parts = (w_a, w_b)

    def slab_row(u, par, jl):
        return ((u >> 1) * 8 + par * 4 + jl) * SLAB

    def gated(x, i, n, gates):
        if gates is None:
            return x
        never, vals = gates
        v = vals[(i * len(vals) * cfg["gspan"]) // (n * 100)]
        return jnp.where(never, pltpu.bitcast(v, U32), x)

    def vregs(*mats):
        return [m_[r:r + 8] for m_ in mats for r in range(0, m_.shape[0], 8)]

    def relayout(u, g, q, gates=None, src=None):
        slot, qs = (u & 3, q) if src is None else src
        low = lax.broadcasted_iota(jnp.int32, (8, 128), 0) < 4
        keep = jnp.where(low, jnp.uint32(0xFFFF), jnp.uint32(0xFFFF0000))
        shl = jnp.where(low, jnp.uint32(16), jnp.uint32(0))
        base = slab_row(u, 0, 0) + q * (KQ // 2)
        for i in range(KQ // 2):
            x = wstage[slot, pl.ds(qs * KQ + 2 * i, 2)].reshape(16, DH)
            x = gated(pltpu.bitcast(x, U32), i, KQ // 2, gates)
            y = pltpu.roll(x, 4, 0)
            w_parts[g][pl.ds(base + i, 8, stride=SLAB), :] = (x & keep) | ((y << shl) >> (16 - shl))

    def comb(x, y, sign):
        return _widen(x) + _widen(y) if sign > 0 else _widen(x) - _widen(y)

    def as_bf16(b):
        return pltpu.bitcast(b, BF16) if b.dtype == U32 else b.astype(BF16)

    def put_lead(segs, n, it, a, b):
        both = jnp.concatenate([a.reshape(n, M, DH), b.reshape(n, M, DH)], axis=1)
        qkvb[segs, it] = _narrow(both)

    def batch_pair(u, g, jl):
        it = 4 * u + jl
        rows = [pl.multiple_of(slab_row(u, par, jl), 8) for par in range(2)]

        def blk(kh, par):
            return w_parts[g][pl.ds(rows[par] + kh * (D // 4), D // 4), :]

        def mm(a, b):
            return _dot(pltpu.bitcast(jnp.concatenate(a, axis=1), BF16), as_bf16(b))

        def xs(f):
            return [xs_u[f, q] for q in range(2)]
        a11 = [xlead_u[q, pl.ds(0, HR), :] for q in (0, 1)]
        a22 = [xlead_u[q, pl.ds(HR, HR), :] for q in (2, 3)]
        m5 = mm(xs(2), blk(1, 1))
        m1 = mm(xs(0), comb(blk(0, 0), blk(1, 1), 1))
        m4 = mm(a22, comb(blk(1, 0), blk(0, 0), -1))
        c11 = mm(xs(4), comb(blk(1, 0), blk(1, 1), 1)) + (m1 + m4 - m5)
        m3 = mm(a11, comb(blk(0, 1), blk(1, 1), -1))
        put_lead(pl.ds(0, NSEG // 2), NSEG // 2, it, c11, m3 + m5)
        m2 = mm(xs(1), blk(0, 0))
        c22 = mm(xs(3), comb(blk(0, 0), blk(0, 1), 1)) + (m1 - m2 + m3)
        put_lead(pl.ds(NSEG // 2, NSEG // 2), NSEG // 2, it, m2 + m4, c22)
        return vregs(m5, m1, m4, c11, m3, m2, c22)

    def quarter_wait(u, q):
        self_wait(wstage.at[u, pl.ds(pl.multiple_of(q * KQ, KQ), KQ)], SW + 4 * u + q)

    def first_unit(q, carry):
        never = q > 1000
        half = q & 1
        self_wait(xlead.at[q], SXL + q)
        quarter_wait(0, q)
        xlead_u[q] = _narrow(xlead[q].astype(F32).reshape(NSEG * M, KQ))
        relayout(0, 0, q)

        @pl.when(q > 0)
        def _():
            quarter_wait(1, q - 1)
        res = []
        xq = pltpu.bitcast(xlead_u[q], BF16)
        for jl in range(4):
            outs = []
            for par in range(2):
                acc = pl.ds((2 * jl + par) * (NSEG * M), NSEG * M)
                row = pl.multiple_of(slab_row(0, par, jl) + q * (KQ // 2), 8)
                w = pltpu.bitcast(w_a[pl.ds(row, KQ // 2), :], BF16)
                d = _dot(xq, w) + jnp.where(q == 0, 0.0, wk[acc, :])
                wk[acc, :] = d
                outs.append(d)
            put_lead(pl.ds(0, NSEG), NSEG, jl, outs[0], outs[1])
            res += outs
        gates = (never, vregs(*res))
        qn = jnp.maximum(q - 1, 0)
        relayout(1, 1, qn, gates, src=(jnp.minimum(q, 1), qn))
        for r in range(0, HR, 8):
            for cb in range(2):
                cols = pl.ds(cb * 128, 128)
                i = 2 * (r // 8) + cb
                a11 = gated(xlead_u[half, pl.ds(r, 8), cols], i, HR // 4, gates)
                a22 = gated(xlead_u[2 + half, pl.ds(HR + r, 8), cols], i, HR // 4, gates)
                a21 = xlead_u[half, pl.ds(HR + r, 8), cols]
                a12 = xlead_u[2 + half, pl.ds(r, 8), cols]
                for f, (x, y, sg) in enumerate(((a11, a22, 1), (a21, a22, 1), (a11, a12, 1),
                                                (a21, a11, -1), (a12, a22, -1))):
                    xs_u[f, half, pl.ds(r, 8), cols] = _narrow(comb(x, y, sg))
        return carry
    lax.fori_loop(0, 4, first_unit, 0)
    w_copy(1, 0).start()
    late_start(0)
    w_copy(0, 1, 3).wait()
    relayout(1, 1, 3)

    def second_unit(jl, carry):
        quarter_wait(2, jl)
        relayout(2, 0, jl, (jl > 1000, batch_pair(1, 1, jl)))
        return carry
    lax.fori_loop(0, 4, second_unit, 0)

    def late_relayout(src, k, jl, gates):
        for ri in range(2):
            r = 2 * jl + ri
            blk = [pltpu.bitcast(wostage[src, pl.ds(e * 128 + r * 16, 16), :], U32) for e in range(4)]
            ngrp = NB // NS
            for kg in range(4 // NS):
                for ng in range(ngrp):
                    i0 = ((ri * (4 // NS) + kg) * ngrp + ng) * len(clusters)
                    rows = pl.ds(pl.multiple_of((k * (4 // NS) + kg) * 64 + r * 8, 8), 8)
                    copied = set()
                    for ci, cl in enumerate(clusters):
                        b = {}
                        for e, c in sorted({t[:2] for f in cl for t in scheme[f][1]}):
                            x = gated(blk[NS * kg + e][:, (NS * ng + c) * 128:(NS * ng + c + 1) * 128],
                                      i0 + ci, len(clusters) * 64 // (NS * NS), gates)
                            b[e, c] = _widen(x)
                            if (e, c) not in copied:
                                copied.add((e, c))
                                row = pl.multiple_of(k * 256 + (NS * kg + e) * 64 + r * 8, 8)
                                wo_u[NS * ng + c, pl.ds(row, 8), :] = x
                        for f in cl:
                            wo_s[stored.index(f), ng, rows, :] = _narrow(
                                _signed_sum(scheme[f][1], lambda e, c: b[e, c]))
                    assert len(copied) == NS * NS
        for t in range(4):
            tile = pltpu.bitcast(hbuf[src, :, pl.ds((4 * jl + t) * 128, 128)], U32)
            tile = jnp.concatenate([gated(tile[0:8], t, 4, gates), tile[8:]], axis=0)
            row = pl.multiple_of(k * 1024 + (4 * jl + t) * 64, 64)
            ht[pl.ds(row, 64), :] = pltpu.bitcast(pltpu.bitcast(tile, BF16).T, U32)

    def unit_body(u, g):
        @pl.when(u < 11)
        def _():
            self_wait(wstage.at[(u + 1) & 3], SW + 12 + ((u + 1) & 3))

        @pl.when(u >= 4)
        def _():
            self_wait(wostage.at[u - 4], SWO + u - 4)
            self_wait(hbuf.at[u - 4], SH + u - 4)
        for m in (1, 2):
            @pl.when((u + 3) >> 2 == m)
            def _():
                w_copy(m, (u + 3) & 3).start()

        @pl.when(u <= 8)
        def _():
            late_start(u - 1)
        if g == 1:
            @pl.when(u == 9)
            def _():
                x_copy(0).start()
                a_start(0)
                tw_cp.start()
        for jl in range(4):
            gates = (u > 1000, batch_pair(u, g, jl))
            relayout(jnp.where(u < 11, u + 1, u - 1), 1 - g, jl, gates)
            late_relayout(jnp.where(u >= 4, u - 4, 8), jnp.maximum(u - 4, 0), jl, gates)

    def unit_pair(mm, carry):
        for g in range(2):
            unit_body(2 * mm + g, g)
        return carry
    lax.fori_loop(1, 6, unit_pair, 0)

    a_start(1)
    for g in range(1, NG):
        x_copy(g).start()
    for cp in small:
        cp.wait()
    dd = ssmd_ref[0].astype(F32)
    for g in range(NG):
        sk = sk_ref[g].astype(F32)
        for j in range(KS):
            taps[g, j] = jnp.broadcast_to(sk[j:j + 1], (8, 128))
        taps[g, KS] = jnp.broadcast_to(dd[g:g + 1], (8, 128))

    def part_a(i, kick):
        g, j = i >> 1, i & 1
        sl = g & 1
        never = i > 1000
        sub = lax.broadcasted_iota(jnp.int32, (8, 128), 0)
        kickbuf[jnp.where(never, 1, 0)] = kick
        chain = [kickbuf[jnp.where(i > 2000, 0, 1)]]

        def begin(xs, ng):
            xs = list(xs)
            for e in range(min(ng, len(xs))):
                c = chain[0]
                c = c if c.dtype == xs[e].dtype else pltpu.bitcast(c, xs[e].dtype)
                xs[e] = jnp.where(never, c, xs[e])
            return xs

        def merge(vals):
            c = vals[-1]
            for v in list(vals[:-1])[:cfg["a_merge"]]:
                c = jnp.maximum(v, c)
            chain[0] = c

        def ld(v):
            if isinstance(v, tuple):
                blk, ri, r = v
                base = 8 * WS + 256 * blk + 16 * ri + 32 * r
                lo = wk[pl.ds(base, 8), :]
                if r == 0:
                    return lo
                return pltpu.roll(jnp.where(sub >= r, lo, wk[pl.ds(base + 8, 8), :]), 8 - r, 0)
            return wk[pl.ds(8 * v, 8), :]

        def st(v, x):
            wk[pl.ds(8 * v, 8), :] = x

        def twid(idx):
            return (tw[j, idx], tw[j, idx + 1])

        def pairs(flat):
            return [(flat[2 * e], flat[2 * e + 1]) for e in range(len(flat) // 2)]

        def fwd4(locs, t0):
            v = pairs(begin([ld(x) for loc in locs[::-1] for x in loc], cfg["a_g4"]))[::-1]
            return _dft4([v[0]] + [_cmul(v[r], twid(t0 + 2 * r)) for r in range(1, 4)], +1)

        def inv4(v, t0):
            o = _dft4(v, -1)
            return [o[0]] + [_cmulc(o[r], twid(t0 + 2 * r)) for r in range(1, 4)]

        def ld4(locs):
            return pairs(begin([ld(x) for loc in locs for x in loc], cfg["a_g4i"]))

        def put4(locs, o):
            for loc, x in zip(locs, o):
                st(loc[0], x[0])
                st(loc[1], x[1])
            merge([x for c in o for x in c])

        def put4_t(dsts, o):
            for (blk, slot), x in zip(dsts, o):
                for ri in range(2):
                    base = 8 * WS + 256 * blk + 16 * ri + slot
                    wk[pl.ds(base, 8, stride=33), :] = x[ri]
            merge([x for c in o for x in c])

        def xloc(sig, n):
            return (WX + 256 * sig + 2 * n, WX + 256 * sig + 2 * n + 1)

        def sloc(kb, l):
            return ((2 * kb + l // 8, 0, l % 8), (2 * kb + l // 8, 1, l % 8))

        def pass_kv():
            t = [taps[g, a] for a in range(KS)]
            prev = [None] + [jnp.zeros((8, 128), F32)] * (KS - 1)
            for v in range(S // 16):
                w, = begin([pltpu.bitcast(abuf[sl, 1, pl.ds(16 * v, 16), :], U32)], 1)
                k2 = _widen(w)
                v2 = abuf[sl, 2, pl.ds(16 * v, 16), :].astype(F32)
                outs = []
                for hh in range(2):
                    x = k2[8 * hh:8 * hh + 8]
                    cur = [None] + [pltpu.roll(x, a, 0) for a in range(1, KS)]
                    ks = x * t[0]
                    for a in range(1, KS):
                        ks = ks + jnp.where(sub < a, prev[a], cur[a]) * t[a]
                    prev = cur
                    kv = (ks * v2[8 * hh:8 * hh + 8]).astype(BF16).astype(F32)
                    st(WK + 2 * v + hh, kv)
                    outs.append(kv)
                merge(outs)

        def forward(sig, src):
            for n in range(32):
                x = src(n)
                cs = []
                for d in range(4):
                    a, b = twid(TAF + 2 * d), twid(TAF + 2 * (d + 4))
                    if d == 0:
                        s_ = x[4] * b[0]
                        cs.append((x[0] + s_, s_))
                    else:
                        cs.append((x[d] * a[0] + x[d + 4] * b[0], x[d] * a[1] + x[d + 4] * b[1]))
                put4([xloc(sig, n + 32 * k0) for k0 in range(4)], _dft4(cs, +1))
            for k0 in range(4):
                for n in range(8):
                    locs = [xloc(sig, n + 8 * r + 32 * k0) for r in range(4)]
                    put4(locs, fwd4(locs, TB + 8 * k0))
            for k0 in range(4):
                for k1 in range(4):
                    k = k0 + 4 * k1
                    for a in range(2):
                        o = fwd4([xloc(sig, a + 2 * r + 8 * k1 + 32 * k0) for r in range(4)], TC + 8 * k)
                        put4_t([(2 * ((k + 16 * k2) // 8) + a, k % 8) for k2 in range(4)], o)
            for kb in range(8):
                for e in range(4):
                    o = fwd4([sloc(kb, e + 4 * r) for r in range(4)], TD + 8 * kb)
                    put4([xloc(sig, 16 * kb + e + 4 * r) for r in range(4)], o)
            for kb in range(8):
                for k3 in range(4):
                    locs = [xloc(sig, 16 * kb + r + 4 * k3) for r in range(4)]
                    t0 = TE + 8 * (4 * kb + k3)
                    o = fwd4(locs, t0)
                    if sig == 0:
                        hs = ld4([xloc(1, 16 * kb + r + 4 * k3) for r in range(4)])
                        o = inv4([_cmul(a, b) for a, b in zip(o, hs)], t0)
                    put4(locs, o)

        def inverse():
            for kb in range(8):
                for e in range(4):
                    o = inv4(ld4([xloc(0, 16 * kb + e + 4 * r) for r in range(4)]), TD + 8 * kb)
                    put4_t([(2 * kb + (e + 4 * f) // 8, (e + 4 * f) % 8) for f in range(4)], o)
            for k0 in range(4):
                for k1 in range(4):
                    k = k0 + 4 * k1
                    for a in range(2):
                        v = ld4([sloc((k + 16 * r) // 8, 8 * a + k % 8) for r in range(4)])
                        put4([xloc(0, a + 2 * b + 8 * k1 + 32 * k0) for b in range(4)], inv4(v, TC + 8 * k))
            for k0 in range(4):
                for n in range(8):
                    locs = [xloc(0, n + 8 * r + 32 * k0) for r in range(4)]
                    put4(locs, inv4(ld4(locs), TB + 8 * k0))
            dskip = taps[g, KS]
            for n0 in range(32):
                cs = _dft4(ld4([xloc(0, n0 + 32 * r) for r in range(4)]), -1)
                outs = []
                for d in [d0 + 4 * hh for d0 in range(4) for hh in range(2)]:
                    n = n0 + 32 * d
                    a = twid(TAI + 2 * d)
                    if 0 < d < 4:
                        cs[d] = tuple(begin(cs[d], 2))
                    c = cs[d % 4]
                    y = c[0] * a[0] if d == 0 else c[0] * a[0] + c[1] * a[1]
                    y = y + jnp.where(j == 0, ld(WK + n) * dskip, ld(WY + n))
                    st(WY + n, y)
                    chain[0] = abuf[sl, 0, pl.ds(8 * n, 8), :].astype(F32) * y
                    aout[g, n // 4, pl.ds(8 * (n % 4), 8), :] = chain[0].astype(BF16)
                    outs.append(chain[0])
                merge(outs)

        def filt(n):
            base = pl.multiple_of(g * (S // 2), S // 2)
            ws = begin([ht[pl.ds(base + 8 * (n // 2 + 16 * d), 8), :] for d in range(8)], 8)
            return [_widen(w)[8 * (n % 2):8 * (n % 2) + 8] for w in ws]
        pass_kv()
        forward(1, filt)
        forward(0, lambda n: begin([ld(WK + n + 32 * d) for d in range(8)], 8))
        inverse()
        return chain[0]

    scale = DH ** (-0.5)

    def w_slab(m, h):
        u = 4 * m + h // 8
        return pltpu.bitcast(w_parts[u % 2][pl.ds(slab_row(u, h % 2, (h // 2) % 4), D // 2), :], BF16)

    class Step:
        def __init__(self, s, leads, mem):
            self.s = s
            self.leads = leads
            self.acc2 = [None] * NB
            self.part = {}
            self.qkv, self.ps, self.os = {}, {}, []
            self.acc = [None] * NB
            self.ocat, self.early, self.marks, self.heads = {}, {}, {}, {}
            self.tie = None
            x = xbuf[s, pl.ds(M, SEG - M), :].astype(F32)
            self.lhsf = jnp.concatenate([mem, x], axis=0)
            self.lhs = self.lhsf.astype(BF16)

        def proj_early(self, m, h, k):
            self.early[m, h] = (k, _dot(self.lhsf[:, :k].astype(BF16), w_slab(m, h)[:k]))

        def proj(self, m, h):
            if (m, h) in self.early:
                k, part = self.early[m, h]
                d = _dot(self.lhsf[:, k:].astype(BF16), w_slab(m, h)[k:]) + part
            else:
                d = _dot(self.lhs, w_slab(m, h))
            self.heads[m, h] = d
            j = h // 2
            if (m, h ^ 1) not in self.heads:
                return
            a, b = self.heads[m, 2 * j], self.heads[m, 2 * j + 1]
            self.marks[m, j] = a[0:8]
            lead = _widen(qkvb[self.s, m * NPAIR + j])
            self.qkv[m, j] = jnp.concatenate([a, b, lead], axis=0).astype(BF16)

        def probs(self, j):
            fill = fill_ref[pl.ds(0, R), pl.ds(0, R)]
            qk = _dot_nt(self.qkv[0, j], self.qkv[1, j])
            sc = jnp.where(fill == 0.0, qk * scale, fill)
            e = jnp.exp(sc - jnp.max(sc, axis=-1, keepdims=True))
            l = jnp.sum(e, axis=-1, keepdims=True)
            r = pl.reciprocal(l, approx=True)
            r = r * (2.0 - l * r)
            self.ps[j] = (e * r).astype(BF16)

        def attend(self, j):
            o = _dot(self.ps[j], self.qkv[2, j])
            self.leads[2 * j].append(o[2 * SEG:2 * SEG + M])
            self.leads[2 * j + 1].append(o[2 * SEG + M:])
            self.os += [o[0:SEG], o[SEG:2 * SEG]]

        def tied(self, w):
            if self.tie is not None:
                w = jnp.concatenate(
                    [jnp.where(self.s > 1000, pltpu.bitcast(self.tie, U32), w[0:8]), w[8:]], axis=0)
                self.tie = None
            return pltpu.bitcast(w, BF16)

        def wo_fast(self, g0, g1, ng, f):
            ta, tb, tc = scheme[f]
            if (g0, f) not in self.ocat:
                def a_blk(kg, r, e):
                    h = NS * kg + e
                    return self.os[h] if r == 0 else jnp.concatenate(self.leads[h], axis=0)
                parts = [_signed_sum(ta, functools.partial(a_blk, kg)) for kg in range(g0, g1)]
                self.ocat[g0, f] = jnp.concatenate(parts, axis=1).astype(BF16)
            if f in stored:
                w = wo_s[stored.index(f), ng, pl.ds(g0 * 64, (g1 - g0) * 64), :]
            else:
                e, c, _ = tb[0]
                w = jnp.concatenate([wo_u[NS * ng + c, pl.ds((NS * kg + e) * 64, 64), :]
                                     for kg in range(g0, g1)], axis=0)
            d = _dot(self.ocat[g0, f], self.tied(w))
            if cfg["acc_m"]:
                if g0 == 0:
                    self.part[ng, f] = d
                    return
                d = d + self.part[ng, f]
            for r, c, plus in tc:
                acc = (self.acc, self.acc2)[r]
                n = NS * ng + c
                if acc[n] is None:
                    acc[n] = d if plus else -d
                else:
                    acc[n] = d + acc[n] if plus else acc[n] - d

        def wo(self, h0, h1, n):
            if h0 not in self.ocat:
                self.ocat[h0] = jnp.concatenate(self.os[h0:h1], axis=1).astype(BF16)
            d = _dot(self.ocat[h0], self.tied(wo_u[n, pl.ds(h0 * 64, (h1 - h0) * 64), :]))
            self.acc[n] = d if self.acc[n] is None else d + self.acc[n]

        def finish(self):
            res = jnp.concatenate(self.acc, axis=1)
            obuf[self.s, pl.ds(M, SEG - M), :] = res[M:].astype(BF16)
            if self.acc2[0] is not None:
                lead = jnp.concatenate(self.acc2, axis=1)
                for e in range(U):
                    obuf[self.s - (U - 1) + e, pl.ds(0, M), :] = lead[M * e:M * e + M].astype(BF16)
            return res[0:M]

    def steps(i, mem):
        def send(segs, rows):
            pltpu.make_async_copy(
                obuf.at[segs, rows], out_hbm.at[segs, rows, pl.ds(D, D)], sems.at[SO]).start()
        sts = []
        leads = [[] for _ in range(H)]
        for u in range(U):
            st = Step(i * U + u, leads, mem)
            sts.append(st)
            for item in _step_order(u, cfg):
                if item[0] == "A":
                    ku, km, kj = cfg["kick"]
                    st.tie = part_a(i, sts[ku].marks[km, kj])
                elif item[0] == "O":
                    last_half = (i & 1) == 1
                    pl.when(last_half)(lambda: a_send(i >> 1))
                    pl.when(jnp.logical_and(last_half, i < 2 * NG - 4))(lambda: a_start((i >> 1) + 2))
                    send(pl.ds(i * U, U - 1), pl.ds(M, SEG - M))
                else:
                    dict(P=st.proj, E=st.proj_early, S=st.probs, V=st.attend, W=st.wo,
                         X=st.wo_fast)[item[0]](*item[1:])
            mem = st.finish()
        send(pl.ds(i * U, U - 1), pl.ds(0, M))
        send(pl.ds(i * U + U - 1, 1), pl.ds(0, SEG))
        return mem

    def a_send(g):
        pltpu.make_async_copy(
            aout.at[g], out_hbm.at[:, :, pl.ds(pl.multiple_of(g * 128, 128), 128)],
            sems.at[SO + 1]).start()

    def group(g, mem):
        x_copy(g).wait()
        self_wait(abuf.at[g & 1], SA + (g & 1))
        return lax.fori_loop(0, 2, lambda j, m_: steps(2 * g + j, m_), mem)

    tw_cp.wait()
    lax.fori_loop(0, NG, group, mem0_ref[...].astype(F32))
    self_wait(obuf, SO)
    self_wait(aout, SO + 1)


def _step_order(u, cfg):
    cfg = dict(cfg, **cfg["sub"][u])
    ks = cfg["ks"]
    tmpl = []
    for x in cfg["tmpl"].split():
        kind, lag = x[:-1], int(x[-1])
        tmpl += [(kind + "a", lag), (kind + "b", lag)] if kind in ("q", "k", "v") else [(kind, lag)]

    def proj(kind, j):
        return ("qkv".index(kind[0]), 2 * j + "ab".index(kind[1]))
    if u < U - 1:
        fill = [[("W", 0, ks, n)] for n in range(NB)]
        last = [("W", ks, H, n) for n in range(NB)]
    else:
        ns = cfg["ns"]

        def products(g0, g1, f_outer):
            fs = range(len(_scheme(ns)[0]))
            if f_outer:
                return [("X", g0, g1, ng, f) for f in fs for ng in range(NB // ns)]
            return [("X", g0, g1, ng, f) for ng in range(NB // ns) for f in fs]
        xs = products(0, ks // ns, cfg["xo"] & 1)
        fill = [xs[e:e + ns] for e in range(0, len(xs), ns)]
        last = products(ks // ns, H // ns, cfg["xo"] & 2)
        last.insert(len(last) - cfg["send_back"], ("O",))
        last.insert(len(last) - 1 - cfg["tie_back"], ("A",))
    out = []
    for t in range(NPAIR + 1 + max(l for _, l in tmpl)):
        for kind, lag in tmpl:
            j = t - lag
            if j < 0:
                continue
            if j >= NPAIR:
                if kind[1:] == "a" and fill:
                    out += fill.pop(0)
                continue
            out.append(("P",) + proj(kind, j) if len(kind) == 2 else (kind, j))
    if u > 0:
        first = [x[1:] for x in out if x[0] == "P"][:cfg["ne"]]
        out = [("E",) + x + (cfg["ek"],) for x in first] + out
    return out + [x for f in fill for x in f] + last


_DEFAULT_CFG = dict(
    sub=(dict(tmpl='ka0 kb0 S1 va0 qa0 V2 qb0 vb0', ks=24, ne=4, ek=640),
         dict(tmpl='ka0 V3 va1 kb0 qa0 S1 vb1 qb0', ks=20, ne=3, ek=640),
         dict(tmpl='qa0 qb0 ka0 V3 kb0 S1 va2 vb2', ks=24, ne=3, ek=768),
         dict(tmpl='ka0 V3 va1 kb0 qa0 S1 vb1 qb0', ks=16, ne=3, ek=640)),
    ns=4, acc_m=1, clusters=((0, 11, 17), (5, 9, 10, 24), (1, 19), (2, 18), (3, 15), (6, 16), (4, 7, 14)),
    tie_back=52, send_back=48, xo=0, gspan=75, kick=(0, 1, 0), a_merge=5, a_g4=4, a_g4i=8)


def _build(cfg):
    tw_np = _twiddles()
    fill_np = np.zeros((96, 128), np.float32)
    fill_np[:R, :R] = _mask_fill()

    def run(A_q, A_k, A_v, A_shift_k, A_ssm_k, A_ssm_D, B_x, B_mem0, B_Wq, B_Wk, B_Wv, B_Wo):
        sk = A_shift_k.T.reshape(KS, NG, 128).transpose(1, 0, 2)
        any_spec = pl.BlockSpec(memory_space=pl.ANY)
        out = pl.pallas_call(
            functools.partial(_kernel, cfg),
            out_shape=jax.ShapeDtypeStruct((NSEG, SEG, 2 * D), BF16),
            in_specs=[any_spec] * 14,
            out_specs=any_spec,
            scratch_shapes=[
                pltpu.VMEM((48 * SLAB + 544, 128), U32),
                pltpu.VMEM((48 * SLAB + 544, 128), U32),
                pltpu.VMEM((NB, H * DH // 2, 128), U32),
                pltpu.VMEM((4, D, 8, DH), BF16),
                pltpu.VMEM((9, 512, D), BF16),
                pltpu.VMEM((NSEG, SEG, D), BF16),
                pltpu.VMEM((4, NSEG, M, KQ), BF16),
                pltpu.VMEM((4, NSEG * M // 2, KQ), U32),
                pltpu.VMEM((5, 2, HR, KQ), U32),
                pltpu.VMEM((NSEG, 3 * NPAIR, 8, 128), U32),
                pltpu.VMEM((len(_scheme(cfg["ns"])[1]), NB // cfg["ns"], H * 64 // cfg["ns"], 128), U32),
                pltpu.VMEM((NSEG, SEG, D), BF16),
                pltpu.VMEM((2, 3, S, 128), BF16),
                pltpu.VMEM((NG + 1, 128, S), BF16),
                pltpu.VMEM((NG * S // 2, 128), U32),
                pltpu.VMEM((8 * NW + 32, 128), F32),
                pltpu.VMEM((2, NT, 8, 128), F32),
                pltpu.VMEM((NG, NSEG, SEG, 128), BF16),
                pltpu.VMEM((4, 8, 128), F32),
                pltpu.VMEM((96, 128), F32),
                pltpu.VMEM((NG, 8, 8, 128), F32),
                pltpu.VMEM((M, D), BF16),
                pltpu.VMEM((NG, KS, 128), BF16),
                pltpu.VMEM((4, NG, 128), BF16),
                pltpu.SemaphoreType.DMA((56,)),
            ],
            compiler_params=pltpu.CompilerParams(vmem_limit_bytes=124 * 1024 * 1024,
                                                 disable_bounds_checks=True),
        )(A_q.reshape(S, D), A_k.reshape(S, D), A_v.reshape(S, D), sk, A_ssm_k,
          A_ssm_D.reshape(NG, 128), B_x.reshape(NSEG, SEG, D), B_mem0.reshape(M, D),
          B_Wq, B_Wk, B_Wv, B_Wo.reshape(H * DH, D),
          jnp.asarray(tw_np), jnp.asarray(fill_np))
        return out.reshape(1, S, 2 * D)

    return run


@jax.jit
def pallas_concat_heads__ssm_conv_h3__memory_aug_recurrent_mem_tr__prompt_kernel(
    A_q: jax.Array,
    A_k: jax.Array,
    A_v: jax.Array,
    A_shift_k: jax.Array,
    A_ssm_k: jax.Array,
    A_ssm_D: jax.Array,
    B_x: jax.Array,
    B_mem0: jax.Array,
    B_Wq: jax.Array,
    B_Wk: jax.Array,
    B_Wv: jax.Array,
    B_Wo: jax.Array,
    B_seg_len: jax.Array,
):
    del B_seg_len
    return _build(_DEFAULT_CFG)(A_q, A_k, A_v, A_shift_k, A_ssm_k, A_ssm_D, B_x, B_mem0,
                                B_Wq, B_Wk, B_Wv, B_Wo)
```

```python
import functools

import numpy as np
import jax
import jax.numpy as jnp
from jax import lax
import jax.experimental.pallas as pl
import jax.experimental.pallas.tpu as pltpu

F32 = jnp.float32
BF16 = jnp.bfloat16
U32 = jnp.uint32

S = 2048
D = 1024
H = 32
DH = 128
M = 8
SEG = 32
NSEG = S // SEG
U = 4
NPAIR = H // 2
R = 2 * (M + SEG)
SLAB = 520
KS = 4
NG = D // 128
KQ = D // 4
NB = D // 128
HR = NSEG * M // 4

TAF, TAI, TB, TC, TD, TE, NT = 0, 16, 32, 64, 192, 256, 512
WX, WS, WY, WK, NW = 0, 512, 1024, 1280, 1536


_STRASSEN = (
    ("+00 +11", "+00 +11", "+00 +11"), ("+11", "+10 -00", "+00 +10"), ("+01 -11", "+10 +11", "+00"),
    ("+00", "+01 -11", "+01 +11"), ("+00 +01", "+11", "+01 -00"), ("+10 +11", "+00", "+10 -11"),
    ("+10 -00", "+00 +01", "+11"),
)
_HK26 = (
    ("+00 +10", "+00 +02 +03 -10 -30", "+10"),
    ("+01", "+10 +11 +13 +21", "+01"),
    ("+11", "+01 +12 +31 -11", "-11"),
    ("+02 +12", "+12 +20 +22 +23 -30", "+02"),
    ("+03 +13", "+32 +33 -13", "+13"),
    ("+00", "+00 +01 +30 -03 -20", "+00 -10"),
    ("+12", "+02 +03 +21 +32 -22", "+02 -12"),
    ("+03", "+31 +33 -23", "+03 -13"),
    ("+00 +01 +10 +11", "+10", "+00 -01"),
    ("+12 -00", "+02 +03 +20 -30", "+10 -02"),
    ("+00 +02", "+20 -30", "+00 -02"),
    ("+10 +12", "+02 +03", "+12 -10"),
    ("+02 +12 -01 -11", "+12", "-11 -12"),
    ("+01 +03 +11 +13", "+13", "+03 -01"),
    ("+03 -12", "+23 +32", "+02 -13"),
    ("+02 +03", "+30 -23", "+02 -03"),
    ("+12 +13", "+03 +32", "+12 -13"),
    ("+00 +10 +11", "+01 +10", "+01 +10 -00"),
    ("+02 +12 -01", "+12 +21", "+11 +12 -02"),
    ("+03 +11 +13", "+13 +31", "+01 +13 -03"),
    ("+00 +02 +03 +10 +12 +13", "+30", "+00 +03 -02"),
    ("+10 +11", "+01", "+00 +11 -01 -10"),
    ("+02 -01", "+21", "+01 +02 -11 -12"),
    ("+11 +13", "+31", "+03 +11 -01 -13"),
    ("+00 +10 +12 +13", "+03 -30", "+00 +03 -02 -10"),
    ("+10 +12 +13", "+03", "+02 +10 +13 -00 -03 -12"),
)


def _scheme(name):
    tab = {2: _STRASSEN, 4: _HK26}[name]
    terms = [[[(int(t[1]), int(t[2]), t[0] == "+") for t in f.split()] for f in p] for p in tab]
    stored = [i for i, p in enumerate(terms) if len(p[1]) > 1]
    return terms, stored


def _signed_sum(terms, get):
    acc = None
    for r, c, plus in terms:
        x = get(r, c)
        acc = x if acc is None else (acc + x if plus else acc - x)
    return acc


def _twiddles():
    tw = np.zeros((2, NT, 8), np.float64)

    def put(j, idx, z):
        tw[j, idx] = np.real(z)
        tw[j, idx + 1] = np.imag(z)
    s = np.arange(8)
    tau = 2j * np.pi
    for j in range(2):
        lx = 1j * np.pi * (1 + 4 * j) / 4096
        for d in range(8):
            put(j, TAF + 2 * d, np.exp(lx * 256 * d))
            put(j, TAI + 2 * d, np.exp(lx * 256 * d) / 2048)
        for r in range(4):
            for k in range(4):
                put(j, TB + 8 * k + 2 * r, np.exp((lx * 64 + tau * k / 16) * r))
            for k in range(16):
                put(j, TC + 8 * k + 2 * r, np.exp((lx * 16 + tau * k / 64) * r))
            for kb in range(8):
                put(j, TD + 8 * kb + 2 * r, np.exp((lx * 4 + tau * (s + 8 * kb) / 256) * r))
                for k3 in range(4):
                    put(j, TE + 8 * (4 * kb + k3) + 2 * r,
                        np.exp((lx + tau * (s + 8 * kb + 64 * k3) / 1024) * r))
    return np.ascontiguousarray(np.broadcast_to(tw[..., None], (2, NT, 8, 128))).astype(np.float32)


def _mask_fill():
    blk = np.concatenate([np.arange(M), M + np.arange(M, SEG)])
    lead = M + np.arange(M)
    head = np.concatenate([np.zeros(SEG), np.ones(SEG), np.zeros(M), np.ones(M)])
    pos = np.concatenate([blk, blk, lead, lead])
    same = head[:, None] == head[None, :]
    ok = (pos[:, None] < M) | (pos[:, None] >= pos[None, :])
    fill = np.where(same, np.where(ok, 0.0, -1e9), -np.inf)
    return fill.astype(np.float32)


def _widen(w):
    return pltpu.bitcast(w, BF16).astype(F32)


def _narrow(x):
    return pltpu.bitcast(x.astype(BF16), U32)


def _dot(a, b):
    return jnp.dot(a, b, preferred_element_type=F32)


def _dot_nt(a, b):
    return lax.dot_general(a, b, (((1,), (1,)), ((), ())), preferred_element_type=F32)


def _cadd(a, b):
    return (a[0] + b[0], a[1] + b[1])


def _csub(a, b):
    return (a[0] - b[0], a[1] - b[1])


def _cmul(a, w):
    return (a[0] * w[0] - a[1] * w[1], a[0] * w[1] + a[1] * w[0])


def _cmulc(a, w):
    return (a[0] * w[0] + a[1] * w[1], a[1] * w[0] - a[0] * w[1])


def _bfly_i(b, d, sg):
    p = (b[0] - d[1], b[1] + d[0])
    q = (b[0] + d[1], b[1] - d[0])
    return (p, q) if sg > 0 else (q, p)


def _dft4(x, sg):
    a, b = _cadd(x[0], x[2]), _csub(x[0], x[2])
    c, d = _cadd(x[1], x[3]), _csub(x[1], x[3])
    p, q = _bfly_i(b, d, sg)
    return [_cadd(a, c), p, _csub(a, c), q]


def _kernel(cfg,
            aq_hbm, ak_hbm, av_hbm, sk_hbm, ssmk_hbm, ssmd_hbm, x_hbm, mem0_hbm,
            wq_hbm, wk_hbm, wv_hbm, wo_hbm, tw_hbm, fill_hbm,
            out_hbm,
            w_a, w_b, wo_u, wstage, wostage, xbuf, xlead, xlead_u, xs_u, qkvb, wo_s, obuf,
            abuf, hbuf, ht, wk, tw, aout, kickbuf,
            fill_ref, taps, mem0_ref, sk_ref, ssmd_ref,
            sems):
    SW, SWO, SXL, SX, SH, SA, ST, SO, SS = 0, 16, 24, 28, 36, 44, 46, 48, 52
    NS = cfg["ns"]
    scheme, stored = _scheme(NS)
    clusters = [stored] if NS == 2 else cfg["clusters"]
    assert sorted(f for cl in clusters for f in cl) == stored
    w_hbms = (wq_hbm, wk_hbm, wv_hbm)
    a_hbms = (aq_hbm, ak_hbm, av_hbm)

    def aligned(x, n):
        return x if isinstance(x, int) else pl.multiple_of(x, n)

    def w_copy(m, hq, q=None):
        rows = pl.ds(0, D) if q is None else pl.ds(q * KQ, KQ)
        sem = SW + 12 + hq if q is None else SW + 4 * hq + q
        heads = aligned(8 * hq, 8)
        return pltpu.make_async_copy(
            w_hbms[m].at[rows, pl.ds(heads, 8), :], wstage.at[hq, rows], sems.at[sem])

    def self_wait(ref, sem):
        pltpu.make_async_copy(ref, ref, sems.at[sem]).wait()

    def late_start(k):
        pltpu.make_async_copy(
            wo_hbm.at[pl.ds(aligned(k * 512, 512), 512), :], wostage.at[k],
            sems.at[SWO + k]).start()
        pltpu.make_async_copy(
            ssmk_hbm.at[pl.ds(aligned(k * 128, 128), 128), :], hbuf.at[k],
            sems.at[SH + k]).start()

    def xlead_copy(q):
        return pltpu.make_async_copy(
            x_hbm.at[:, pl.ds(0, M), pl.ds(q * KQ, KQ)], xlead.at[q], sems.at[SXL + q])

    def x_copy(g):
        segs = pl.ds(g * 8, 8)
        return pltpu.make_async_copy(
            x_hbm.at[segs, pl.ds(M, SEG - M), :], xbuf.at[segs, pl.ds(M, SEG - M), :], sems.at[SX + g])

    def a_start(g):
        col = aligned(g * 128, 128)
        for t in (1, 2, 0):
            pltpu.make_async_copy(
                a_hbms[t].at[:, pl.ds(col, 128)], abuf.at[g & 1, t], sems.at[SA + (g & 1)]).start()

    tw_cp = pltpu.make_async_copy(tw_hbm, tw, sems.at[ST])

    small = [pltpu.make_async_copy(src, dst, sems.at[SS + i]) for i, (src, dst) in enumerate((
        (fill_hbm, fill_ref), (mem0_hbm, mem0_ref), (sk_hbm, sk_ref), (ssmd_hbm, ssmd_ref.at[0])))]

    for q in range(4):
        xlead_copy(q).start()
        w_copy(0, 0, q).start()
        if q > 0:
            w_copy(0, 1, q - 1).start()
    w_copy(0, 1, 3).start()
    for q in range(4):
        w_copy(0, 2, q).start()
    w_copy(0, 3).start()
    for cp in small:
        cp.start()

    kickbuf[...] = jnp.zeros(kickbuf.shape, F32)

    w_parts = (w_a, w_b)

    def slab_row(u, par, jl):
        return ((u >> 1) * 8 + par * 4 + jl) * SLAB

    def gated(x, i, n, gates):
        if gates is None:
            return x
        never, vals = gates
        v = vals[(i * len(vals) * cfg["gspan"]) // (n * 100)]
        return jnp.where(never, pltpu.bitcast(v, U32), x)

    def vregs(*mats):
        return [m_[r:r + 8] for m_ in mats for r in range(0, m_.shape[0], 8)]

    def relayout(u, g, q, gates=None, src=None):
        slot, qs = (u & 3, q) if src is None else src
        low = lax.broadcasted_iota(jnp.int32, (8, 128), 0) < 4
        keep = jnp.where(low, jnp.uint32(0xFFFF), jnp.uint32(0xFFFF0000))
        shl = jnp.where(low, jnp.uint32(16), jnp.uint32(0))
        base = slab_row(u, 0, 0) + q * (KQ // 2)
        for i in range(KQ // 2):
            x = wstage[slot, pl.ds(qs * KQ + 2 * i, 2)].reshape(16, DH)
            x = gated(pltpu.bitcast(x, U32), i, KQ // 2, gates)
            y = pltpu.roll(x, 4, 0)
            w_parts[g][pl.ds(base + i, 8, stride=SLAB), :] = (x & keep) | ((y << shl) >> (16 - shl))

    def comb(x, y, sign):
        return _widen(x) + _widen(y) if sign > 0 else _widen(x) - _widen(y)

    def as_bf16(b):
        return pltpu.bitcast(b, BF16) if b.dtype == U32 else b.astype(BF16)

    def put_lead(segs, n, it, a, b):
        both = jnp.concatenate([a.reshape(n, M, DH), b.reshape(n, M, DH)], axis=1)
        qkvb[segs, it] = _narrow(both)

    def batch_pair(u, g, jl):
        it = 4 * u + jl
        rows = [pl.multiple_of(slab_row(u, par, jl), 8) for par in range(2)]

        def blk(kh, par):
            return w_parts[g][pl.ds(rows[par] + kh * (D // 4), D // 4), :]

        def mm(a, b):
            return _dot(pltpu.bitcast(jnp.concatenate(a, axis=1), BF16), as_bf16(b))

        def xs(f):
            return [xs_u[f, q] for q in range(2)]
        a11 = [xlead_u[q, pl.ds(0, HR), :] for q in (0, 1)]
        a22 = [xlead_u[q, pl.ds(HR, HR), :] for q in (2, 3)]
        m5 = mm(xs(2), blk(1, 1))
        m1 = mm(xs(0), comb(blk(0, 0), blk(1, 1), 1))
        m4 = mm(a22, comb(blk(1, 0), blk(0, 0), -1))
        c11 = mm(xs(4), comb(blk(1, 0), blk(1, 1), 1)) + (m1 + m4 - m5)
        m3 = mm(a11, comb(blk(0, 1), blk(1, 1), -1))
        put_lead(pl.ds(0, NSEG // 2), NSEG // 2, it, c11, m3 + m5)
        m2 = mm(xs(1), blk(0, 0))
        c22 = mm(xs(3), comb(blk(0, 0), blk(0, 1), 1)) + (m1 - m2 + m3)
        put_lead(pl.ds(NSEG // 2, NSEG // 2), NSEG // 2, it, m2 + m4, c22)
        return vregs(m5, m1, m4, c11, m3, m2, c22)

    def quarter_wait(u, q):
        self_wait(wstage.at[u, pl.ds(pl.multiple_of(q * KQ, KQ), KQ)], SW + 4 * u + q)

    def first_unit(q, carry):
        never = q > 1000
        half = q & 1
        self_wait(xlead.at[q], SXL + q)
        quarter_wait(0, q)
        xlead_u[q] = _narrow(xlead[q].astype(F32).reshape(NSEG * M, KQ))
        relayout(0, 0, q)

        @pl.when(q > 0)
        def _():
            quarter_wait(1, q - 1)
        res = []
        xq = pltpu.bitcast(xlead_u[q], BF16)
        for jl in range(4):
            outs = []
            for par in range(2):
                acc = pl.ds((2 * jl + par) * (NSEG * M), NSEG * M)
                row = pl.multiple_of(slab_row(0, par, jl) + q * (KQ // 2), 8)
                w = pltpu.bitcast(w_a[pl.ds(row, KQ // 2), :], BF16)
                d = _dot(xq, w) + jnp.where(q == 0, 0.0, wk[acc, :])
                wk[acc, :] = d
                outs.append(d)
            put_lead(pl.ds(0, NSEG), NSEG, jl, outs[0], outs[1])
            res += outs
        gates = (never, vregs(*res))
        qn = jnp.maximum(q - 1, 0)
        relayout(1, 1, qn, gates, src=(jnp.minimum(q, 1), qn))
        for r in range(0, HR, 8):
            for cb in range(2):
                cols = pl.ds(cb * 128, 128)
                i = 2 * (r // 8) + cb
                a11 = gated(xlead_u[half, pl.ds(r, 8), cols], i, HR // 4, gates)
                a22 = gated(xlead_u[2 + half, pl.ds(HR + r, 8), cols], i, HR // 4, gates)
                a21 = xlead_u[half, pl.ds(HR + r, 8), cols]
                a12 = xlead_u[2 + half, pl.ds(r, 8), cols]
                for f, (x, y, sg) in enumerate(((a11, a22, 1), (a21, a22, 1), (a11, a12, 1),
                                                (a21, a11, -1), (a12, a22, -1))):
                    xs_u[f, half, pl.ds(r, 8), cols] = _narrow(comb(x, y, sg))
        return carry
    lax.fori_loop(0, 4, first_unit, 0)
    w_copy(1, 0).start()
    late_start(0)
    w_copy(0, 1, 3).wait()
    relayout(1, 1, 3)

    def second_unit(jl, carry):
        quarter_wait(2, jl)
        relayout(2, 0, jl, (jl > 1000, batch_pair(1, 1, jl)))
        return carry
    lax.fori_loop(0, 4, second_unit, 0)

    def late_relayout(src, k, jl, gates):
        for ri in range(2):
            r = 2 * jl + ri
            blk = [pltpu.bitcast(wostage[src, pl.ds(e * 128 + r * 16, 16), :], U32) for e in range(4)]
            ngrp = NB // NS
            for kg in range(4 // NS):
                for ng in range(ngrp):
                    i0 = ((ri * (4 // NS) + kg) * ngrp + ng) * len(clusters)
                    rows = pl.ds(pl.multiple_of((k * (4 // NS) + kg) * 64 + r * 8, 8), 8)
                    copied = set()
                    for ci, cl in enumerate(clusters):
                        b = {}
                        for e, c in sorted({t[:2] for f in cl for t in scheme[f][1]}):
                            x = gated(blk[NS * kg + e][:, (NS * ng + c) * 128:(NS * ng + c + 1) * 128],
                                      i0 + ci, len(clusters) * 64 // (NS * NS), gates)
                            b[e, c] = _widen(x)
                            if (e, c) not in copied:
                                copied.add((e, c))
                                row = pl.multiple_of(k * 256 + (NS * kg + e) * 64 + r * 8, 8)
                                wo_u[NS * ng + c, pl.ds(row, 8), :] = x
                        for f in cl:
                            wo_s[stored.index(f), ng, rows, :] = _narrow(
                                _signed_sum(scheme[f][1], lambda e, c: b[e, c]))
                    assert len(copied) == NS * NS
        for t in range(4):
            tile = pltpu.bitcast(hbuf[src, :, pl.ds((4 * jl + t) * 128, 128)], U32)
            tile = jnp.concatenate([gated(tile[0:8], t, 4, gates), tile[8:]], axis=0)
            row = pl.multiple_of(k * 1024 + (4 * jl + t) * 64, 64)
            ht[pl.ds(row, 64), :] = pltpu.bitcast(pltpu.bitcast(tile, BF16).T, U32)

    def unit_body(u, g):
        @pl.when(u < 11)
        def _():
            self_wait(wstage.at[(u + 1) & 3], SW + 12 + ((u + 1) & 3))

        @pl.when(u >= 4)
        def _():
            self_wait(wostage.at[u - 4], SWO + u - 4)
            self_wait(hbuf.at[u - 4], SH + u - 4)
        for m in (1, 2):
            @pl.when((u + 3) >> 2 == m)
            def _():
                w_copy(m, (u + 3) & 3).start()

        @pl.when(u <= 8)
        def _():
            late_start(u - 1)
        if g == 1:
            @pl.when(u == 9)
            def _():
                x_copy(0).start()
                a_start(0)
                tw_cp.start()
        for jl in range(4):
            gates = (u > 1000, batch_pair(u, g, jl))
            relayout(jnp.where(u < 11, u + 1, u - 1), 1 - g, jl, gates)
            late_relayout(jnp.where(u >= 4, u - 4, 8), jnp.maximum(u - 4, 0), jl, gates)

    def unit_pair(mm, carry):
        for g in range(2):
            unit_body(2 * mm + g, g)
        return carry
    lax.fori_loop(1, 6, unit_pair, 0)

    a_start(1)
    for g in range(1, NG):
        x_copy(g).start()
    for cp in small:
        cp.wait()
    dd = ssmd_ref[0].astype(F32)
    for g in range(NG):
        sk = sk_ref[g].astype(F32)
        for j in range(KS):
            taps[g, j] = jnp.broadcast_to(sk[j:j + 1], (8, 128))
        taps[g, KS] = jnp.broadcast_to(dd[g:g + 1], (8, 128))

    def part_a(i, kick):
        g, j = i >> 1, i & 1
        sl = g & 1
        never = i > 1000
        sub = lax.broadcasted_iota(jnp.int32, (8, 128), 0)
        kickbuf[jnp.where(never, 1, 0)] = kick
        chain = [kickbuf[jnp.where(i > 2000, 0, 1)]]

        def begin(xs, ng):
            xs = list(xs)
            for e in range(min(ng, len(xs))):
                c = chain[0]
                c = c if c.dtype == xs[e].dtype else pltpu.bitcast(c, xs[e].dtype)
                xs[e] = jnp.where(never, c, xs[e])
            return xs

        def merge(vals):
            c = vals[-1]
            for v in list(vals[:-1])[:cfg["a_merge"]]:
                c = jnp.maximum(v, c)
            chain[0] = c

        def ld(v):
            if isinstance(v, tuple):
                blk, ri, r = v
                base = 8 * WS + 256 * blk + 16 * ri + 32 * r
                lo = wk[pl.ds(base, 8), :]
                if r == 0:
                    return lo
                return pltpu.roll(jnp.where(sub >= r, lo, wk[pl.ds(base + 8, 8), :]), 8 - r, 0)
            return wk[pl.ds(8 * v, 8), :]

        def st(v, x):
            wk[pl.ds(8 * v, 8), :] = x

        def twid(idx):
            return (tw[j, idx], tw[j, idx + 1])

        def pairs(flat):
            return [(flat[2 * e], flat[2 * e + 1]) for e in range(len(flat) // 2)]

        def fwd4(locs, t0):
            v = pairs(begin([ld(x) for loc in locs[::-1] for x in loc], cfg["a_g4"]))[::-1]
            return _dft4([v[0]] + [_cmul(v[r], twid(t0 + 2 * r)) for r in range(1, 4)], +1)

        def inv4(v, t0):
            o = _dft4(v, -1)
            return [o[0]] + [_cmulc(o[r], twid(t0 + 2 * r)) for r in range(1, 4)]

        def ld4(locs):
            return pairs(begin([ld(x) for loc in locs for x in loc], cfg["a_g4i"]))

        def put4(locs, o):
            for loc, x in zip(locs, o):
                st(loc[0], x[0])
                st(loc[1], x[1])
            merge([x for c in o for x in c])

        def put4_t(dsts, o):
            for (blk, slot), x in zip(dsts, o):
                for ri in range(2):
                    base = 8 * WS + 256 * blk + 16 * ri + slot
                    wk[pl.ds(base, 8, stride=33), :] = x[ri]
            merge([x for c in o for x in c])

        def xloc(sig, n):
            return (WX + 256 * sig + 2 * n, WX + 256 * sig + 2 * n + 1)

        def sloc(kb, l):
            return ((2 * kb + l // 8, 0, l % 8), (2 * kb + l // 8, 1, l % 8))

        def pass_kv():
            t = [taps[g, a] for a in range(KS)]
            prev = [None] + [jnp.zeros((8, 128), F32)] * (KS - 1)
            for v in range(S // 16):
                w, = begin([pltpu.bitcast(abuf[sl, 1, pl.ds(16 * v, 16), :], U32)], 1)
                k2 = _widen(w)
                v2 = abuf[sl, 2, pl.ds(16 * v, 16), :].astype(F32)
                outs = []
                for hh in range(2):
                    x = k2[8 * hh:8 * hh + 8]
                    cur = [None] + [pltpu.roll(x, a, 0) for a in range(1, KS)]
                    ks = x * t[0]
                    for a in range(1, KS):
                        ks = ks + jnp.where(sub < a, prev[a], cur[a]) * t[a]
                    prev = cur
                    kv = (ks * v2[8 * hh:8 * hh + 8]).astype(BF16).astype(F32)
                    st(WK + 2 * v + hh, kv)
                    outs.append(kv)
                merge(outs)

        def forward(sig, src):
            for n in range(32):
                x = src(n)
                cs = []
                for d in range(4):
                    a, b = twid(TAF + 2 * d), twid(TAF + 2 * (d + 4))
                    if d == 0:
                        s_ = x[4] * b[0]
                        cs.append((x[0] + s_, s_))
                    else:
                        cs.append((x[d] * a[0] + x[d + 4] * b[0], x[d] * a[1] + x[d + 4] * b[1]))
                put4([xloc(sig, n + 32 * k0) for k0 in range(4)], _dft4(cs, +1))
            for k0 in range(4):
                for n in range(8):
                    locs = [xloc(sig, n + 8 * r + 32 * k0) for r in range(4)]
                    put4(locs, fwd4(locs, TB + 8 * k0))
            for k0 in range(4):
                for k1 in range(4):
                    k = k0 + 4 * k1
                    for a in range(2):
                        o = fwd4([xloc(sig, a + 2 * r + 8 * k1 + 32 * k0) for r in range(4)], TC + 8 * k)
                        put4_t([(2 * ((k + 16 * k2) // 8) + a, k % 8) for k2 in range(4)], o)
            for kb in range(8):
                for e in range(4):
                    o = fwd4([sloc(kb, e + 4 * r) for r in range(4)], TD + 8 * kb)
                    put4([xloc(sig, 16 * kb + e + 4 * r) for r in range(4)], o)
            for kb in range(8):
                for k3 in range(4):
                    locs = [xloc(sig, 16 * kb + r + 4 * k3) for r in range(4)]
                    t0 = TE + 8 * (4 * kb + k3)
                    o = fwd4(locs, t0)
                    if sig == 0:
                        hs = ld4([xloc(1, 16 * kb + r + 4 * k3) for r in range(4)])
                        o = inv4([_cmul(a, b) for a, b in zip(o, hs)], t0)
                    put4(locs, o)

        def inverse():
            for kb in range(8):
                for e in range(4):
                    o = inv4(ld4([xloc(0, 16 * kb + e + 4 * r) for r in range(4)]), TD + 8 * kb)
                    put4_t([(2 * kb + (e + 4 * f) // 8, (e + 4 * f) % 8) for f in range(4)], o)
            for k0 in range(4):
                for k1 in range(4):
                    k = k0 + 4 * k1
                    for a in range(2):
                        v = ld4([sloc((k + 16 * r) // 8, 8 * a + k % 8) for r in range(4)])
                        put4([xloc(0, a + 2 * b + 8 * k1 + 32 * k0) for b in range(4)], inv4(v, TC + 8 * k))
            for k0 in range(4):
                for n in range(8):
                    locs = [xloc(0, n + 8 * r + 32 * k0) for r in range(4)]
                    put4(locs, inv4(ld4(locs), TB + 8 * k0))
            dskip = taps[g, KS]
            for n0 in range(32):
                cs = _dft4(ld4([xloc(0, n0 + 32 * r) for r in range(4)]), -1)
                outs = []
                for d in [d0 + 4 * hh for d0 in range(4) for hh in range(2)]:
                    n = n0 + 32 * d
                    a = twid(TAI + 2 * d)
                    if 0 < d < 4:
                        cs[d] = tuple(begin(cs[d], 2))
                    c = cs[d % 4]
                    y = c[0] * a[0] if d == 0 else c[0] * a[0] + c[1] * a[1]
                    y = y + jnp.where(j == 0, ld(WK + n) * dskip, ld(WY + n))
                    st(WY + n, y)
                    chain[0] = abuf[sl, 0, pl.ds(8 * n, 8), :].astype(F32) * y
                    aout[g, n // 4, pl.ds(8 * (n % 4), 8), :] = chain[0].astype(BF16)
                    outs.append(chain[0])
                merge(outs)

        def filt(n):
            base = pl.multiple_of(g * (S // 2), S // 2)
            ws = begin([ht[pl.ds(base + 8 * (n // 2 + 16 * d), 8), :] for d in range(8)], 8)
            return [_widen(w)[8 * (n % 2):8 * (n % 2) + 8] for w in ws]
        pass_kv()
        forward(1, filt)
        forward(0, lambda n: begin([ld(WK + n + 32 * d) for d in range(8)], 8))
        inverse()
        return chain[0]

    scale = DH ** (-0.5)

    def w_slab(m, h):
        u = 4 * m + h // 8
        return pltpu.bitcast(w_parts[u % 2][pl.ds(slab_row(u, h % 2, (h // 2) % 4), D // 2), :], BF16)

    class Step:
        def __init__(self, s, leads, mem):
            self.s = s
            self.leads = leads
            self.acc2 = [None] * NB
            self.part = {}
            self.qkv, self.ps, self.os = {}, {}, []
            self.acc = [None] * NB
            self.ocat, self.early, self.marks, self.heads = {}, {}, {}, {}
            self.tie = None
            x = xbuf[s, pl.ds(M, SEG - M), :].astype(F32)
            self.lhsf = jnp.concatenate([mem, x], axis=0)
            self.lhs = self.lhsf.astype(BF16)

        def proj_early(self, m, h, k):
            self.early[m, h] = (k, _dot(self.lhsf[:, :k].astype(BF16), w_slab(m, h)[:k]))

        def proj(self, m, h):
            if (m, h) in self.early:
                k, part = self.early[m, h]
                d = _dot(self.lhsf[:, k:].astype(BF16), w_slab(m, h)[k:]) + part
            else:
                d = _dot(self.lhs, w_slab(m, h))
            self.heads[m, h] = d
            j = h // 2
            if (m, h ^ 1) not in self.heads:
                return
            a, b = self.heads[m, 2 * j], self.heads[m, 2 * j + 1]
            self.marks[m, j] = a[0:8]
            lead = _widen(qkvb[self.s, m * NPAIR + j])
            self.qkv[m, j] = jnp.concatenate([a, b, lead], axis=0).astype(BF16)

        def probs(self, j):
            fill = fill_ref[pl.ds(0, R), pl.ds(0, R)]
            qk = _dot_nt(self.qkv[0, j], self.qkv[1, j])
            sc = jnp.where(fill == 0.0, qk * scale, fill)
            e = jnp.exp(sc - jnp.max(sc, axis=-1, keepdims=True))
            l = jnp.sum(e, axis=-1, keepdims=True)
            r = pl.reciprocal(l, approx=True)
            r = r * (2.0 - l * r)
            self.ps[j] = (e * r).astype(BF16)

        def attend(self, j):
            o = _dot(self.ps[j], self.qkv[2, j])
            self.leads[2 * j].append(o[2 * SEG:2 * SEG + M])
            self.leads[2 * j + 1].append(o[2 * SEG + M:])
            self.os += [o[0:SEG], o[SEG:2 * SEG]]

        def tied(self, w):
            if self.tie is not None:
                w = jnp.concatenate(
                    [jnp.where(self.s > 1000, pltpu.bitcast(self.tie, U32), w[0:8]), w[8:]], axis=0)
                self.tie = None
            return pltpu.bitcast(w, BF16)

        def wo_fast(self, g0, g1, ng, f):
            ta, tb, tc = scheme[f]
            if (g0, f) not in self.ocat:
                def a_blk(kg, r, e):
                    h = NS * kg + e
                    return self.os[h] if r == 0 else jnp.concatenate(self.leads[h], axis=0)
                parts = [_signed_sum(ta, functools.partial(a_blk, kg)) for kg in range(g0, g1)]
                self.ocat[g0, f] = jnp.concatenate(parts, axis=1).astype(BF16)
            if f in stored:
                w = wo_s[stored.index(f), ng, pl.ds(g0 * 64, (g1 - g0) * 64), :]
            else:
                e, c, _ = tb[0]
                w = jnp.concatenate([wo_u[NS * ng + c, pl.ds((NS * kg + e) * 64, 64), :]
                                     for kg in range(g0, g1)], axis=0)
            d = _dot(self.ocat[g0, f], self.tied(w))
            if cfg["acc_m"]:
                if g0 == 0:
                    self.part[ng, f] = d
                    return
                d = d + self.part[ng, f]
            for r, c, plus in tc:
                acc = (self.acc, self.acc2)[r]
                n = NS * ng + c
                if acc[n] is None:
                    acc[n] = d if plus else -d
                else:
                    acc[n] = d + acc[n] if plus else acc[n] - d

        def wo(self, h0, h1, n):
            if h0 not in self.ocat:
                self.ocat[h0] = jnp.concatenate(self.os[h0:h1], axis=1).astype(BF16)
            d = _dot(self.ocat[h0], self.tied(wo_u[n, pl.ds(h0 * 64, (h1 - h0) * 64), :]))
            self.acc[n] = d if self.acc[n] is None else d + self.acc[n]

        def finish(self):
            res = jnp.concatenate(self.acc, axis=1)
            obuf[self.s, pl.ds(M, SEG - M), :] = res[M:].astype(BF16)
            if self.acc2[0] is not None:
                lead = jnp.concatenate(self.acc2, axis=1)
                for e in range(U):
                    obuf[self.s - (U - 1) + e, pl.ds(0, M), :] = lead[M * e:M * e + M].astype(BF16)
            return res[0:M]

    def steps(i, mem):
        def send(segs, rows):
            pltpu.make_async_copy(
                obuf.at[segs, rows], out_hbm.at[segs, rows, pl.ds(D, D)], sems.at[SO]).start()
        sts = []
        leads = [[] for _ in range(H)]
        for u in range(U):
            st = Step(i * U + u, leads, mem)
            sts.append(st)
            for item in _step_order(u, cfg):
                if item[0] == "A":
                    ku, km, kj = cfg["kick"]
                    st.tie = part_a(i, sts[ku].marks[km, kj])
                elif item[0] == "O":
                    last_half = (i & 1) == 1
                    pl.when(last_half)(lambda: a_send(i >> 1))
                    pl.when(jnp.logical_and(last_half, i < 2 * NG - 4))(lambda: a_start((i >> 1) + 2))
                    send(pl.ds(i * U, U - 1), pl.ds(M, SEG - M))
                else:
                    dict(P=st.proj, E=st.proj_early, S=st.probs, V=st.attend, W=st.wo,
                         X=st.wo_fast)[item[0]](*item[1:])
            mem = st.finish()
        send(pl.ds(i * U, U - 1), pl.ds(0, M))
        send(pl.ds(i * U + U - 1, 1), pl.ds(0, SEG))
        return mem

    def a_send(g):
        pltpu.make_async_copy(
            aout.at[g], out_hbm.at[:, :, pl.ds(pl.multiple_of(g * 128, 128), 128)],
            sems.at[SO + 1]).start()

    def group(g, mem):
        x_copy(g).wait()
        self_wait(abuf.at[g & 1], SA + (g & 1))
        return lax.fori_loop(0, 2, lambda j, m_: steps(2 * g + j, m_), mem)

    tw_cp.wait()
    lax.fori_loop(0, NG, group, mem0_ref[...].astype(F32))
    self_wait(obuf, SO)
    self_wait(aout, SO + 1)


def _step_order(u, cfg):
    cfg = dict(cfg, **cfg["sub"][u])
    ks = cfg["ks"]
    tmpl = []
    for x in cfg["tmpl"].split():
        kind, lag = x[:-1], int(x[-1])
        tmpl += [(kind + "a", lag), (kind + "b", lag)] if kind in ("q", "k", "v") else [(kind, lag)]

    def proj(kind, j):
        return ("qkv".index(kind[0]), 2 * j + "ab".index(kind[1]))
    if u < U - 1:
        fill = [[("W", 0, ks, n)] for n in range(NB)]
        last = [("W", ks, H, n) for n in range(NB)]
    else:
        ns = cfg["ns"]

        def products(g0, g1, f_outer):
            fs = range(len(_scheme(ns)[0]))
            if f_outer:
                return [("X", g0, g1, ng, f) for f in fs for ng in range(NB // ns)]
            return [("X", g0, g1, ng, f) for ng in range(NB // ns) for f in fs]
        xs = products(0, ks // ns, cfg["xo"] & 1)
        fill = [xs[e:e + ns] for e in range(0, len(xs), ns)]
        last = products(ks // ns, H // ns, cfg["xo"] & 2)
        last.insert(len(last) - cfg["send_back"], ("O",))
        last.insert(len(last) - 1 - cfg["tie_back"], ("A",))
    out = []
    for t in range(NPAIR + 1 + max(l for _, l in tmpl)):
        for kind, lag in tmpl:
            j = t - lag
            if j < 0:
                continue
            if j >= NPAIR:
                if kind[1:] == "a" and fill:
                    out += fill.pop(0)
                continue
            out.append(("P",) + proj(kind, j) if len(kind) == 2 else (kind, j))
    if u > 0:
        first = [x[1:] for x in out if x[0] == "P"][:cfg["ne"]]
        out = [("E",) + x + (cfg["ek"],) for x in first] + out
    return out + [x for f in fill for x in f] + last


_DEFAULT_CFG = dict(
    sub=(dict(tmpl='ka0 kb0 S1 va0 qa0 V2 qb0 vb0', ks=16, ne=3, ek=768),
         dict(tmpl='ka0 V3 va1 kb0 qa0 S1 vb1 qb0', ks=20, ne=3, ek=640),
         dict(tmpl='qa0 qb0 ka0 V3 kb0 S1 va2 vb2', ks=24, ne=3, ek=768),
         dict(tmpl='S2 qa0 qb0 va1 V3 vb1 ka0 kb0', ks=16, ne=3, ek=640)),
    ns=4, acc_m=1, clusters=((0, 11, 17), (5, 9, 10, 24), (1, 19), (2, 18), (3, 15), (6, 16), (4, 7, 14)),
    tie_back=52, send_back=48, xo=0, gspan=75, kick=(0, 1, 0), a_merge=5, a_g4=4, a_g4i=8)


def _build(cfg):
    tw_np = _twiddles()
    fill_np = np.zeros((96, 128), np.float32)
    fill_np[:R, :R] = _mask_fill()

    def run(A_q, A_k, A_v, A_shift_k, A_ssm_k, A_ssm_D, B_x, B_mem0, B_Wq, B_Wk, B_Wv, B_Wo):
        sk = A_shift_k.T.reshape(KS, NG, 128).transpose(1, 0, 2)
        any_spec = pl.BlockSpec(memory_space=pl.ANY)
        out = pl.pallas_call(
            functools.partial(_kernel, cfg),
            out_shape=jax.ShapeDtypeStruct((NSEG, SEG, 2 * D), BF16),
            in_specs=[any_spec] * 14,
            out_specs=any_spec,
            scratch_shapes=[
                pltpu.VMEM((48 * SLAB + 544, 128), U32),
                pltpu.VMEM((48 * SLAB + 544, 128), U32),
                pltpu.VMEM((NB, H * DH // 2, 128), U32),
                pltpu.VMEM((4, D, 8, DH), BF16),
                pltpu.VMEM((9, 512, D), BF16),
                pltpu.VMEM((NSEG, SEG, D), BF16),
                pltpu.VMEM((4, NSEG, M, KQ), BF16),
                pltpu.VMEM((4, NSEG * M // 2, KQ), U32),
                pltpu.VMEM((5, 2, HR, KQ), U32),
                pltpu.VMEM((NSEG, 3 * NPAIR, 8, 128), U32),
                pltpu.VMEM((len(_scheme(cfg["ns"])[1]), NB // cfg["ns"], H * 64 // cfg["ns"], 128), U32),
                pltpu.VMEM((NSEG, SEG, D), BF16),
                pltpu.VMEM((2, 3, S, 128), BF16),
                pltpu.VMEM((NG + 1, 128, S), BF16),
                pltpu.VMEM((NG * S // 2, 128), U32),
                pltpu.VMEM((8 * NW + 32, 128), F32),
                pltpu.VMEM((2, NT, 8, 128), F32),
                pltpu.VMEM((NG, NSEG, SEG, 128), BF16),
                pltpu.VMEM((4, 8, 128), F32),
                pltpu.VMEM((96, 128), F32),
                pltpu.VMEM((NG, 8, 8, 128), F32),
                pltpu.VMEM((M, D), BF16),
                pltpu.VMEM((NG, KS, 128), BF16),
                pltpu.VMEM((4, NG, 128), BF16),
                pltpu.SemaphoreType.DMA((56,)),
            ],
            compiler_params=pltpu.CompilerParams(vmem_limit_bytes=124 * 1024 * 1024,
                                                 disable_bounds_checks=True),
        )(A_q.reshape(S, D), A_k.reshape(S, D), A_v.reshape(S, D), sk, A_ssm_k,
          A_ssm_D.reshape(NG, 128), B_x.reshape(NSEG, SEG, D), B_mem0.reshape(M, D),
          B_Wq, B_Wk, B_Wv, B_Wo.reshape(H * DH, D),
          jnp.asarray(tw_np), jnp.asarray(fill_np))
        return out.reshape(1, S, 2 * D)

    return run


@jax.jit
def pallas_concat_heads__ssm_conv_h3__memory_aug_recurrent_mem_tr__prompt_kernel(
    A_q: jax.Array,
    A_k: jax.Array,
    A_v: jax.Array,
    A_shift_k: jax.Array,
    A_ssm_k: jax.Array,
    A_ssm_D: jax.Array,
    B_x: jax.Array,
    B_mem0: jax.Array,
    B_Wq: jax.Array,
    B_Wk: jax.Array,
    B_Wv: jax.Array,
    B_Wo: jax.Array,
    B_seg_len: jax.Array,
):
    del B_seg_len
    return _build(_DEFAULT_CFG)(A_q, A_k, A_v, A_shift_k, A_ssm_k, A_ssm_D, B_x, B_mem0,
                                B_Wq, B_Wk, B_Wv, B_Wo)
```

```python
import functools

import numpy as np
import jax
import jax.numpy as jnp
from jax import lax
import jax.experimental.pallas as pl
import jax.experimental.pallas.tpu as pltpu

F32 = jnp.float32
BF16 = jnp.bfloat16
U32 = jnp.uint32

S = 2048
D = 1024
H = 32
DH = 128
M = 8
SEG = 32
NSEG = S // SEG
U = 4
NPAIR = H // 2
R = 2 * (M + SEG)
SLAB = 520
KS = 4
NG = D // 128
KQ = D // 4
NB = D // 128
HR = NSEG * M // 4

TAF, TAI, TB, TC, TD, TE, NT = 0, 16, 32, 64, 192, 256, 512
WX, WS, WY, WK, NW = 0, 512, 1024, 1280, 1536


_STRASSEN = (
    ("+00 +11", "+00 +11", "+00 +11"), ("+11", "+10 -00", "+00 +10"), ("+01 -11", "+10 +11", "+00"),
    ("+00", "+01 -11", "+01 +11"), ("+00 +01", "+11", "+01 -00"), ("+10 +11", "+00", "+10 -11"),
    ("+10 -00", "+00 +01", "+11"),
)
_HK26 = (
    ("+00 +10", "+00 +02 +03 -10 -30", "+10"),
    ("+01", "+10 +11 +13 +21", "+01"),
    ("+11", "+01 +12 +31 -11", "-11"),
    ("+02 +12", "+12 +20 +22 +23 -30", "+02"),
    ("+03 +13", "+32 +33 -13", "+13"),
    ("+00", "+00 +01 +30 -03 -20", "+00 -10"),
    ("+12", "+02 +03 +21 +32 -22", "+02 -12"),
    ("+03", "+31 +33 -23", "+03 -13"),
    ("+00 +01 +10 +11", "+10", "+00 -01"),
    ("+12 -00", "+02 +03 +20 -30", "+10 -02"),
    ("+00 +02", "+20 -30", "+00 -02"),
    ("+10 +12", "+02 +03", "+12 -10"),
    ("+02 +12 -01 -11", "+12", "-11 -12"),
    ("+01 +03 +11 +13", "+13", "+03 -01"),
    ("+03 -12", "+23 +32", "+02 -13"),
    ("+02 +03", "+30 -23", "+02 -03"),
    ("+12 +13", "+03 +32", "+12 -13"),
    ("+00 +10 +11", "+01 +10", "+01 +10 -00"),
    ("+02 +12 -01", "+12 +21", "+11 +12 -02"),
    ("+03 +11 +13", "+13 +31", "+01 +13 -03"),
    ("+00 +02 +03 +10 +12 +13", "+30", "+00 +03 -02"),
    ("+10 +11", "+01", "+00 +11 -01 -10"),
    ("+02 -01", "+21", "+01 +02 -11 -12"),
    ("+11 +13", "+31", "+03 +11 -01 -13"),
    ("+00 +10 +12 +13", "+03 -30", "+00 +03 -02 -10"),
    ("+10 +12 +13", "+03", "+02 +10 +13 -00 -03 -12"),
)


def _scheme(name):
    tab = {2: _STRASSEN, 4: _HK26}[name]
    terms = [[[(int(t[1]), int(t[2]), t[0] == "+") for t in f.split()] for f in p] for p in tab]
    stored = [i for i, p in enumerate(terms) if len(p[1]) > 1]
    return terms, stored


def _signed_sum(terms, get):
    acc = None
    for r, c, plus in terms:
        x = get(r, c)
        acc = x if acc is None else (acc + x if plus else acc - x)
    return acc


def _twiddles():
    tw = np.zeros((2, NT, 8), np.float64)

    def put(j, idx, z):
        tw[j, idx] = np.real(z)
        tw[j, idx + 1] = np.imag(z)
    s = np.arange(8)
    tau = 2j * np.pi
    for j in range(2):
        lx = 1j * np.pi * (1 + 4 * j) / 4096
        for d in range(8):
            put(j, TAF + 2 * d, np.exp(lx * 256 * d))
            put(j, TAI + 2 * d, np.exp(lx * 256 * d) / 2048)
        for r in range(4):
            for k in range(4):
                put(j, TB + 8 * k + 2 * r, np.exp((lx * 64 + tau * k / 16) * r))
            for k in range(16):
                put(j, TC + 8 * k + 2 * r, np.exp((lx * 16 + tau * k / 64) * r))
            for kb in range(8):
                put(j, TD + 8 * kb + 2 * r, np.exp((lx * 4 + tau * (s + 8 * kb) / 256) * r))
                for k3 in range(4):
                    put(j, TE + 8 * (4 * kb + k3) + 2 * r,
                        np.exp((lx + tau * (s + 8 * kb + 64 * k3) / 1024) * r))
    return np.ascontiguousarray(np.broadcast_to(tw[..., None], (2, NT, 8, 128))).astype(np.float32)


def _mask_fill():
    blk = np.concatenate([np.arange(M), M + np.arange(M, SEG)])
    lead = M + np.arange(M)
    head = np.concatenate([np.zeros(SEG), np.ones(SEG), np.zeros(M), np.ones(M)])
    pos = np.concatenate([blk, blk, lead, lead])
    same = head[:, None] == head[None, :]
    ok = (pos[:, None] < M) | (pos[:, None] >= pos[None, :])
    fill = np.where(same, np.where(ok, 0.0, -1e9), -np.inf)
    return fill.astype(np.float32)


def _widen(w):
    return pltpu.bitcast(w, BF16).astype(F32)


def _narrow(x):
    return pltpu.bitcast(x.astype(BF16), U32)


def _dot(a, b):
    return jnp.dot(a, b, preferred_element_type=F32)


def _dot_nt(a, b):
    return lax.dot_general(a, b, (((1,), (1,)), ((), ())), preferred_element_type=F32)


def _cadd(a, b):
    return (a[0] + b[0], a[1] + b[1])


def _csub(a, b):
    return (a[0] - b[0], a[1] - b[1])


def _cmul(a, w):
    return (a[0] * w[0] - a[1] * w[1], a[0] * w[1] + a[1] * w[0])


def _cmulc(a, w):
    return (a[0] * w[0] + a[1] * w[1], a[1] * w[0] - a[0] * w[1])


def _bfly_i(b, d, sg):
    p = (b[0] - d[1], b[1] + d[0])
    q = (b[0] + d[1], b[1] - d[0])
    return (p, q) if sg > 0 else (q, p)


def _dft4(x, sg):
    a, b = _cadd(x[0], x[2]), _csub(x[0], x[2])
    c, d = _cadd(x[1], x[3]), _csub(x[1], x[3])
    p, q = _bfly_i(b, d, sg)
    return [_cadd(a, c), p, _csub(a, c), q]


def _kernel(cfg,
            aq_hbm, ak_hbm, av_hbm, sk_hbm, ssmk_hbm, ssmd_hbm, x_hbm, mem0_hbm,
            wq_hbm, wk_hbm, wv_hbm, wo_hbm, tw_hbm, fill_hbm,
            out_hbm,
            w_a, w_b, wo_u, wstage, wostage, xbuf, xlead, xlead_u, xs_u, qkvb, wo_s, obuf,
            abuf, hbuf, ht, wk, tw, aout, kickbuf,
            fill_ref, taps, mem0_ref, sk_ref, ssmd_ref,
            sems):
    SW, SWO, SXL, SX, SH, SA, ST, SO, SS = 0, 16, 24, 28, 36, 44, 46, 48, 52
    NS = cfg["ns"]
    scheme, stored = _scheme(NS)
    clusters = [stored] if NS == 2 else cfg["clusters"]
    assert sorted(f for cl in clusters for f in cl) == stored
    w_hbms = (wv_hbm, wk_hbm, wq_hbm)
    a_hbms = (aq_hbm, ak_hbm, av_hbm)

    def aligned(x, n):
        return x if isinstance(x, int) else pl.multiple_of(x, n)

    def w_copy(m, hq, q=None):
        rows = pl.ds(0, D) if q is None else pl.ds(q * KQ, KQ)
        sem = SW + 12 + hq if q is None else SW + 4 * hq + q
        heads = aligned(8 * hq, 8)
        return pltpu.make_async_copy(
            w_hbms[m].at[rows, pl.ds(heads, 8), :], wstage.at[hq, rows], sems.at[sem])

    def self_wait(ref, sem):
        pltpu.make_async_copy(ref, ref, sems.at[sem]).wait()

    def late_start(k):
        pltpu.make_async_copy(
            wo_hbm.at[pl.ds(aligned(k * 512, 512), 512), :], wostage.at[k],
            sems.at[SWO + k]).start()
        pltpu.make_async_copy(
            ssmk_hbm.at[pl.ds(aligned(k * 128, 128), 128), :], hbuf.at[k],
            sems.at[SH + k]).start()

    def xlead_copy(q):
        return pltpu.make_async_copy(
            x_hbm.at[:, pl.ds(0, M), pl.ds(q * KQ, KQ)], xlead.at[q], sems.at[SXL + q])

    def x_copy(g):
        segs = pl.ds(g * 8, 8)
        return pltpu.make_async_copy(
            x_hbm.at[segs, pl.ds(M, SEG - M), :], xbuf.at[segs, pl.ds(M, SEG - M), :], sems.at[SX + g])

    def a_start(g):
        col = aligned(g * 128, 128)
        for t in (1, 2, 0):
            pltpu.make_async_copy(
                a_hbms[t].at[:, pl.ds(col, 128)], abuf.at[g & 1, t], sems.at[SA + (g & 1)]).start()

    tw_cp = pltpu.make_async_copy(tw_hbm, tw, sems.at[ST])

    small = [pltpu.make_async_copy(src, dst, sems.at[SS + i]) for i, (src, dst) in enumerate((
        (fill_hbm, fill_ref), (mem0_hbm, mem0_ref), (sk_hbm, sk_ref), (ssmd_hbm, ssmd_ref.at[0])))]

    for q in range(4):
        xlead_copy(q).start()
        w_copy(0, 0, q).start()
        if q > 0:
            w_copy(0, 1, q - 1).start()
    w_copy(0, 1, 3).start()
    for q in range(4):
        w_copy(0, 2, q).start()
    w_copy(0, 3).start()
    for cp in small:
        cp.start()

    kickbuf[...] = jnp.zeros(kickbuf.shape, F32)

    w_parts = (w_a, w_b)

    def slab_row(u, par, jl):
        return ((u >> 1) * 8 + par * 4 + jl) * SLAB

    def gated(x, i, n, gates):
        if gates is None:
            return x
        never, vals = gates
        v = vals[(i * len(vals) * cfg["gspan"]) // (n * 100)]
        return jnp.where(never, pltpu.bitcast(v, U32), x)

    def vregs(*mats):
        return [m_[r:r + 8] for m_ in mats for r in range(0, m_.shape[0], 8)]

    def relayout(u, g, q, gates=None, src=None):
        slot, qs = (u & 3, q) if src is None else src
        low = lax.broadcasted_iota(jnp.int32, (8, 128), 0) < 4
        keep = jnp.where(low, jnp.uint32(0xFFFF), jnp.uint32(0xFFFF0000))
        shl = jnp.where(low, jnp.uint32(16), jnp.uint32(0))
        base = slab_row(u, 0, 0) + q * (KQ // 2)
        for i in range(KQ // 2):
            x = wstage[slot, pl.ds(qs * KQ + 2 * i, 2)].reshape(16, DH)
            x = gated(pltpu.bitcast(x, U32), i, KQ // 2, gates)
            y = pltpu.roll(x, 4, 0)
            w_parts[g][pl.ds(base + i, 8, stride=SLAB), :] = (x & keep) | ((y << shl) >> (16 - shl))

    def comb(x, y, sign):
        return _widen(x) + _widen(y) if sign > 0 else _widen(x) - _widen(y)

    def as_bf16(b):
        return pltpu.bitcast(b, BF16) if b.dtype == U32 else b.astype(BF16)

    def put_lead(segs, n, it, a, b):
        both = jnp.concatenate([a.reshape(n, M, DH), b.reshape(n, M, DH)], axis=1)
        qkvb[segs, it] = _narrow(both)

    def batch_pair(u, g, jl):
        it = 4 * u + jl
        rows = [pl.multiple_of(slab_row(u, par, jl), 8) for par in range(2)]

        def blk(kh, par):
            return w_parts[g][pl.ds(rows[par] + kh * (D // 4), D // 4), :]

        def mm(a, b):
            return _dot(pltpu.bitcast(jnp.concatenate(a, axis=1), BF16), as_bf16(b))

        def xs(f):
            return [xs_u[f, q] for q in range(2)]
        a11 = [xlead_u[q, pl.ds(0, HR), :] for q in (0, 1)]
        a22 = [xlead_u[q, pl.ds(HR, HR), :] for q in (2, 3)]
        m5 = mm(xs(2), blk(1, 1))
        m1 = mm(xs(0), comb(blk(0, 0), blk(1, 1), 1))
        m4 = mm(a22, comb(blk(1, 0), blk(0, 0), -1))
        c11 = mm(xs(4), comb(blk(1, 0), blk(1, 1), 1)) + (m1 + m4 - m5)
        m3 = mm(a11, comb(blk(0, 1), blk(1, 1), -1))
        put_lead(pl.ds(0, NSEG // 2), NSEG // 2, it, c11, m3 + m5)
        m2 = mm(xs(1), blk(0, 0))
        c22 = mm(xs(3), comb(blk(0, 0), blk(0, 1), 1)) + (m1 - m2 + m3)
        put_lead(pl.ds(NSEG // 2, NSEG // 2), NSEG // 2, it, m2 + m4, c22)
        return vregs(m5, m1, m4, c11, m3, m2, c22)

    def quarter_wait(u, q):
        self_wait(wstage.at[u, pl.ds(pl.multiple_of(q * KQ, KQ), KQ)], SW + 4 * u + q)

    def first_unit(q, carry):
        never = q > 1000
        half = q & 1
        self_wait(xlead.at[q], SXL + q)
        quarter_wait(0, q)
        xlead_u[q] = _narrow(xlead[q].astype(F32).reshape(NSEG * M, KQ))
        relayout(0, 0, q)

        @pl.when(q > 0)
        def _():
            quarter_wait(1, q - 1)
        res = []
        xq = pltpu.bitcast(xlead_u[q], BF16)
        for jl in range(4):
            outs = []
            for par in range(2):
                acc = pl.ds((2 * jl + par) * (NSEG * M), NSEG * M)
                row = pl.multiple_of(slab_row(0, par, jl) + q * (KQ // 2), 8)
                w = pltpu.bitcast(w_a[pl.ds(row, KQ // 2), :], BF16)
                d = _dot(xq, w) + jnp.where(q == 0, 0.0, wk[acc, :])
                wk[acc, :] = d
                outs.append(d)
            put_lead(pl.ds(0, NSEG), NSEG, jl, outs[0], outs[1])
            res += outs
        gates = (never, vregs(*res))
        qn = jnp.maximum(q - 1, 0)
        relayout(1, 1, qn, gates, src=(jnp.minimum(q, 1), qn))
        for r in range(0, HR, 8):
            for cb in range(2):
                cols = pl.ds(cb * 128, 128)
                i = 2 * (r // 8) + cb
                a11 = gated(xlead_u[half, pl.ds(r, 8), cols], i, HR // 4, gates)
                a22 = gated(xlead_u[2 + half, pl.ds(HR + r, 8), cols], i, HR // 4, gates)
                a21 = xlead_u[half, pl.ds(HR + r, 8), cols]
                a12 = xlead_u[2 + half, pl.ds(r, 8), cols]
                for f, (x, y, sg) in enumerate(((a11, a22, 1), (a21, a22, 1), (a11, a12, 1),
                                                (a21, a11, -1), (a12, a22, -1))):
                    xs_u[f, half, pl.ds(r, 8), cols] = _narrow(comb(x, y, sg))
        return carry
    lax.fori_loop(0, 4, first_unit, 0)
    w_copy(1, 0).start()
    late_start(0)
    w_copy(0, 1, 3).wait()
    relayout(1, 1, 3)

    def second_unit(jl, carry):
        quarter_wait(2, jl)
        relayout(2, 0, jl, (jl > 1000, batch_pair(1, 1, jl)))
        return carry
    lax.fori_loop(0, 4, second_unit, 0)

    def late_relayout(src, k, jl, gates):
        for ri in range(2):
            r = 2 * jl + ri
            blk = [pltpu.bitcast(wostage[src, pl.ds(e * 128 + r * 16, 16), :], U32) for e in range(4)]
            ngrp = NB // NS
            for kg in range(4 // NS):
                for ng in range(ngrp):
                    i0 = ((ri * (4 // NS) + kg) * ngrp + ng) * len(clusters)
                    rows = pl.ds(pl.multiple_of((k * (4 // NS) + kg) * 64 + r * 8, 8), 8)
                    copied = set()
                    for ci, cl in enumerate(clusters):
                        b = {}
                        for e, c in sorted({t[:2] for f in cl for t in scheme[f][1]}):
                            x = gated(blk[NS * kg + e][:, (NS * ng + c) * 128:(NS * ng + c + 1) * 128],
                                      i0 + ci, len(clusters) * 64 // (NS * NS), gates)
                            b[e, c] = _widen(x)
                            if (e, c) not in copied:
                                copied.add((e, c))
                                row = pl.multiple_of(k * 256 + (NS * kg + e) * 64 + r * 8, 8)
                                wo_u[NS * ng + c, pl.ds(row, 8), :] = x
                        for f in cl:
                            wo_s[stored.index(f), ng, rows, :] = _narrow(
                                _signed_sum(scheme[f][1], lambda e, c: b[e, c]))
                    assert len(copied) == NS * NS
        for t in range(4):
            tile = pltpu.bitcast(hbuf[src, :, pl.ds((4 * jl + t) * 128, 128)], U32)
            tile = jnp.concatenate([gated(tile[0:8], t, 4, gates), tile[8:]], axis=0)
            row = pl.multiple_of(k * 1024 + (4 * jl + t) * 64, 64)
            ht[pl.ds(row, 64), :] = pltpu.bitcast(pltpu.bitcast(tile, BF16).T, U32)

    def unit_body(u, g):
        @pl.when(u < 11)
        def _():
            self_wait(wstage.at[(u + 1) & 3], SW + 12 + ((u + 1) & 3))

        @pl.when(u >= 4)
        def _():
            self_wait(wostage.at[u - 4], SWO + u - 4)
            self_wait(hbuf.at[u - 4], SH + u - 4)
        for m in (1, 2):
            @pl.when((u + 3) >> 2 == m)
            def _():
                w_copy(m, (u + 3) & 3).start()

        @pl.when(u <= 8)
        def _():
            late_start(u - 1)
        if g == 1:
            @pl.when(u == 9)
            def _():
                x_copy(0).start()
                a_start(0)
                tw_cp.start()
        for jl in range(4):
            gates = (u > 1000, batch_pair(u, g, jl))
            relayout(jnp.where(u < 11, u + 1, u - 1), 1 - g, jl, gates)
            late_relayout(jnp.where(u >= 4, u - 4, 8), jnp.maximum(u - 4, 0), jl, gates)

    def unit_pair(mm, carry):
        for g in range(2):
            unit_body(2 * mm + g, g)
        return carry
    lax.fori_loop(1, 6, unit_pair, 0)

    a_start(1)
    for g in range(1, NG):
        x_copy(g).start()
    for cp in small:
        cp.wait()
    dd = ssmd_ref[0].astype(F32)
    for g in range(NG):
        sk = sk_ref[g].astype(F32)
        for j in range(KS):
            taps[g, j] = jnp.broadcast_to(sk[j:j + 1], (8, 128))
        taps[g, KS] = jnp.broadcast_to(dd[g:g + 1], (8, 128))

    def part_a(i, kick):
        g, j = i >> 1, i & 1
        sl = g & 1
        never = i > 1000
        sub = lax.broadcasted_iota(jnp.int32, (8, 128), 0)
        kickbuf[jnp.where(never, 1, 0)] = kick
        chain = [kickbuf[jnp.where(i > 2000, 0, 1)]]

        def begin(xs, ng):
            xs = list(xs)
            for e in range(min(ng, len(xs))):
                c = chain[0]
                c = c if c.dtype == xs[e].dtype else pltpu.bitcast(c, xs[e].dtype)
                xs[e] = jnp.where(never, c, xs[e])
            return xs

        def merge(vals):
            c = vals[-1]
            for v in list(vals[:-1])[:cfg["a_merge"]]:
                c = jnp.maximum(v, c)
            chain[0] = c

        def ld(v):
            if isinstance(v, tuple):
                blk, ri, r = v
                base = 8 * WS + 256 * blk + 16 * ri + 32 * r
                lo = wk[pl.ds(base, 8), :]
                if r == 0:
                    return lo
                return pltpu.roll(jnp.where(sub >= r, lo, wk[pl.ds(base + 8, 8), :]), 8 - r, 0)
            return wk[pl.ds(8 * v, 8), :]

        def st(v, x):
            wk[pl.ds(8 * v, 8), :] = x

        def twid(idx):
            return (tw[j, idx], tw[j, idx + 1])

        def pairs(flat):
            return [(flat[2 * e], flat[2 * e + 1]) for e in range(len(flat) // 2)]

        def fwd4(locs, t0):
            v = pairs(begin([ld(x) for loc in locs[::-1] for x in loc], cfg["a_g4"]))[::-1]
            return _dft4([v[0]] + [_cmul(v[r], twid(t0 + 2 * r)) for r in range(1, 4)], +1)

        def inv4(v, t0):
            o = _dft4(v, -1)
            return [o[0]] + [_cmulc(o[r], twid(t0 + 2 * r)) for r in range(1, 4)]

        def ld4(locs):
            return pairs(begin([ld(x) for loc in locs for x in loc], cfg["a_g4i"]))

        def put4(locs, o):
            for loc, x in zip(locs, o):
                st(loc[0], x[0])
                st(loc[1], x[1])
            merge([x for c in o for x in c])

        def put4_t(dsts, o):
            for (blk, slot), x in zip(dsts, o):
                for ri in range(2):
                    base = 8 * WS + 256 * blk + 16 * ri + slot
                    wk[pl.ds(base, 8, stride=33), :] = x[ri]
            merge([x for c in o for x in c])

        def xloc(sig, n):
            return (WX + 256 * sig + 2 * n, WX + 256 * sig + 2 * n + 1)

        def sloc(kb, l):
            return ((2 * kb + l // 8, 0, l % 8), (2 * kb + l // 8, 1, l % 8))

        def pass_kv():
            t = [taps[g, a] for a in range(KS)]
            prev = [None] + [jnp.zeros((8, 128), F32)] * (KS - 1)
            for v in range(S // 16):
                w, = begin([pltpu.bitcast(abuf[sl, 1, pl.ds(16 * v, 16), :], U32)], 1)
                k2 = _widen(w)
                v2 = abuf[sl, 2, pl.ds(16 * v, 16), :].astype(F32)
                outs = []
                for hh in range(2):
                    x = k2[8 * hh:8 * hh + 8]
                    cur = [None] + [pltpu.roll(x, a, 0) for a in range(1, KS)]
                    ks = x * t[0]
                    for a in range(1, KS):
                        ks = ks + jnp.where(sub < a, prev[a], cur[a]) * t[a]
                    prev = cur
                    kv = (ks * v2[8 * hh:8 * hh + 8]).astype(BF16).astype(F32)
                    st(WK + 2 * v + hh, kv)
                    outs.append(kv)
                merge(outs)

        def forward(sig, src):
            for n in range(32):
                x = src(n)
                cs = []
                for d in range(4):
                    a, b = twid(TAF + 2 * d), twid(TAF + 2 * (d + 4))
                    if d == 0:
                        s_ = x[4] * b[0]
                        cs.append((x[0] + s_, s_))
                    else:
                        cs.append((x[d] * a[0] + x[d + 4] * b[0], x[d] * a[1] + x[d + 4] * b[1]))
                put4([xloc(sig, n + 32 * k0) for k0 in range(4)], _dft4(cs, +1))
            for k0 in range(4):
                for n in range(8):
                    locs = [xloc(sig, n + 8 * r + 32 * k0) for r in range(4)]
                    put4(locs, fwd4(locs, TB + 8 * k0))
            for k0 in range(4):
                for k1 in range(4):
                    k = k0 + 4 * k1
                    for a in range(2):
                        o = fwd4([xloc(sig, a + 2 * r + 8 * k1 + 32 * k0) for r in range(4)], TC + 8 * k)
                        put4_t([(2 * ((k + 16 * k2) // 8) + a, k % 8) for k2 in range(4)], o)
            for kb in range(8):
                for e in range(4):
                    o = fwd4([sloc(kb, e + 4 * r) for r in range(4)], TD + 8 * kb)
                    put4([xloc(sig, 16 * kb + e + 4 * r) for r in range(4)], o)
            for kb in range(8):
                for k3 in range(4):
                    locs = [xloc(sig, 16 * kb + r + 4 * k3) for r in range(4)]
                    t0 = TE + 8 * (4 * kb + k3)
                    o = fwd4(locs, t0)
                    if sig == 0:
                        hs = ld4([xloc(1, 16 * kb + r + 4 * k3) for r in range(4)])
                        o = inv4([_cmul(a, b) for a, b in zip(o, hs)], t0)
                    put4(locs, o)

        def inverse():
            for kb in range(8):
                for e in range(4):
                    o = inv4(ld4([xloc(0, 16 * kb + e + 4 * r) for r in range(4)]), TD + 8 * kb)
                    put4_t([(2 * kb + (e + 4 * f) // 8, (e + 4 * f) % 8) for f in range(4)], o)
            for k0 in range(4):
                for k1 in range(4):
                    k = k0 + 4 * k1
                    for a in range(2):
                        v = ld4([sloc((k + 16 * r) // 8, 8 * a + k % 8) for r in range(4)])
                        put4([xloc(0, a + 2 * b + 8 * k1 + 32 * k0) for b in range(4)], inv4(v, TC + 8 * k))
            for k0 in range(4):
                for n in range(8):
                    locs = [xloc(0, n + 8 * r + 32 * k0) for r in range(4)]
                    put4(locs, inv4(ld4(locs), TB + 8 * k0))
            dskip = taps[g, KS]
            for n0 in range(32):
                cs = _dft4(ld4([xloc(0, n0 + 32 * r) for r in range(4)]), -1)
                outs = []
                for d in [d0 + 4 * hh for d0 in range(4) for hh in range(2)]:
                    n = n0 + 32 * d
                    a = twid(TAI + 2 * d)
                    if 0 < d < 4:
                        cs[d] = tuple(begin(cs[d], 2))
                    c = cs[d % 4]
                    y = c[0] * a[0] if d == 0 else c[0] * a[0] + c[1] * a[1]
                    y = y + jnp.where(j == 0, ld(WK + n) * dskip, ld(WY + n))
                    st(WY + n, y)
                    chain[0] = abuf[sl, 0, pl.ds(8 * n, 8), :].astype(F32) * y
                    aout[g, n // 4, pl.ds(8 * (n % 4), 8), :] = chain[0].astype(BF16)
                    outs.append(chain[0])
                merge(outs)

        def filt(n):
            base = pl.multiple_of(g * (S // 2), S // 2)
            ws = begin([ht[pl.ds(base + 8 * (n // 2 + 16 * d), 8), :] for d in range(8)], 8)
            return [_widen(w)[8 * (n % 2):8 * (n % 2) + 8] for w in ws]
        pass_kv()
        forward(1, filt)
        forward(0, lambda n: begin([ld(WK + n + 32 * d) for d in range(8)], 8))
        inverse()
        return chain[0]

    scale = DH ** (-0.5)

    def w_slab(m, h):
        u = 4 * (2 - m) + h // 8
        return pltpu.bitcast(w_parts[u % 2][pl.ds(slab_row(u, h % 2, (h // 2) % 4), D // 2), :], BF16)

    class Step:
        def __init__(self, s, leads, mem):
            self.s = s
            self.leads = leads
            self.acc2 = [None] * NB
            self.part = {}
            self.qkv, self.ps, self.os = {}, {}, []
            self.acc = [None] * NB
            self.ocat, self.early, self.marks, self.heads = {}, {}, {}, {}
            self.tie = None
            x = xbuf[s, pl.ds(M, SEG - M), :].astype(F32)
            self.lhsf = jnp.concatenate([mem, x], axis=0)
            self.lhs = self.lhsf.astype(BF16)

        def proj_early(self, m, h, k):
            self.early[m, h] = (k, _dot(self.lhsf[:, :k].astype(BF16), w_slab(m, h)[:k]))

        def proj(self, m, h):
            if (m, h) in self.early:
                k, part = self.early[m, h]
                d = _dot(self.lhsf[:, k:].astype(BF16), w_slab(m, h)[k:]) + part
            else:
                d = _dot(self.lhs, w_slab(m, h))
            self.heads[m, h] = d
            j = h // 2
            if (m, h ^ 1) not in self.heads:
                return
            a, b = self.heads[m, 2 * j], self.heads[m, 2 * j + 1]
            self.marks[m, j] = a[0:8]
            lead = _widen(qkvb[self.s, (2 - m) * NPAIR + j])
            self.qkv[m, j] = jnp.concatenate([a, b, lead], axis=0).astype(BF16)

        def probs(self, j):
            fill = fill_ref[pl.ds(0, R), pl.ds(0, R)]
            qk = _dot_nt(self.qkv[0, j], self.qkv[1, j])
            sc = jnp.where(fill == 0.0, qk * scale, fill)
            e = jnp.exp(sc - jnp.max(sc, axis=-1, keepdims=True))
            l = jnp.sum(e, axis=-1, keepdims=True)
            r = pl.reciprocal(l, approx=True)
            r = r * (2.0 - l * r)
            self.ps[j] = (e * r).astype(BF16)

        def attend(self, j):
            o = _dot(self.ps[j], self.qkv[2, j])
            self.leads[2 * j].append(o[2 * SEG:2 * SEG + M])
            self.leads[2 * j + 1].append(o[2 * SEG + M:])
            self.os += [o[0:SEG], o[SEG:2 * SEG]]

        def tied(self, w):
            if self.tie is not None:
                w = jnp.concatenate(
                    [jnp.where(self.s > 1000, pltpu.bitcast(self.tie, U32), w[0:8]), w[8:]], axis=0)
                self.tie = None
            return pltpu.bitcast(w, BF16)

        def wo_fast(self, g0, g1, ng, f):
            ta, tb, tc = scheme[f]
            if (g0, f) not in self.ocat:
                def a_blk(kg, r, e):
                    h = NS * kg + e
                    return self.os[h] if r == 0 else jnp.concatenate(self.leads[h], axis=0)
                parts = [_signed_sum(ta, functools.partial(a_blk, kg)) for kg in range(g0, g1)]
                self.ocat[g0, f] = jnp.concatenate(parts, axis=1).astype(BF16)
            if f in stored:
                w = wo_s[stored.index(f), ng, pl.ds(g0 * 64, (g1 - g0) * 64), :]
            else:
                e, c, _ = tb[0]
                w = jnp.concatenate([wo_u[NS * ng + c, pl.ds((NS * kg + e) * 64, 64), :]
                                     for kg in range(g0, g1)], axis=0)
            d = _dot(self.ocat[g0, f], self.tied(w))
            if cfg["acc_m"]:
                if g0 == 0:
                    self.part[ng, f] = d
                    return
                d = d + self.part[ng, f]
            for r, c, plus in tc:
                acc = (self.acc, self.acc2)[r]
                n = NS * ng + c
                if acc[n] is None:
                    acc[n] = d if plus else -d
                else:
                    acc[n] = d + acc[n] if plus else acc[n] - d

        def wo(self, h0, h1, n):
            if h0 not in self.ocat:
                self.ocat[h0] = jnp.concatenate(self.os[h0:h1], axis=1).astype(BF16)
            d = _dot(self.ocat[h0], self.tied(wo_u[n, pl.ds(h0 * 64, (h1 - h0) * 64), :]))
            self.acc[n] = d if self.acc[n] is None else d + self.acc[n]

        def finish(self):
            res = jnp.concatenate(self.acc, axis=1)
            obuf[self.s, pl.ds(M, SEG - M), :] = res[M:].astype(BF16)
            if self.acc2[0] is not None:
                lead = jnp.concatenate(self.acc2, axis=1)
                for e in range(U):
                    obuf[self.s - (U - 1) + e, pl.ds(0, M), :] = lead[M * e:M * e + M].astype(BF16)
            return res[0:M]

    def steps(i, mem):
        def send(segs, rows):
            pltpu.make_async_copy(
                obuf.at[segs, rows], out_hbm.at[segs, rows, pl.ds(D, D)], sems.at[SO]).start()
        sts = []
        leads = [[] for _ in range(H)]
        for u in range(U):
            st = Step(i * U + u, leads, mem)
            sts.append(st)
            for item in _step_order(u, cfg):
                if item[0] == "A":
                    ku, km, kj = cfg["kick"]
                    st.tie = part_a(i, sts[ku].marks[km, kj])
                elif item[0] == "O":
                    last_half = (i & 1) == 1
                    pl.when(last_half)(lambda: a_send(i >> 1))
                    pl.when(jnp.logical_and(last_half, i < 2 * NG - 4))(lambda: a_start((i >> 1) + 2))
                    send(pl.ds(i * U, U - 1), pl.ds(M, SEG - M))
                else:
                    dict(P=st.proj, E=st.proj_early, S=st.probs, V=st.attend, W=st.wo,
                         X=st.wo_fast)[item[0]](*item[1:])
            mem = st.finish()
        send(pl.ds(i * U, U - 1), pl.ds(0, M))
        send(pl.ds(i * U + U - 1, 1), pl.ds(0, SEG))
        return mem

    def a_send(g):
        pltpu.make_async_copy(
            aout.at[g], out_hbm.at[:, :, pl.ds(pl.multiple_of(g * 128, 128), 128)],
            sems.at[SO + 1]).start()

    def group(g, mem):
        x_copy(g).wait()
        self_wait(abuf.at[g & 1], SA + (g & 1))
        return lax.fori_loop(0, 2, lambda j, m_: steps(2 * g + j, m_), mem)

    tw_cp.wait()
    lax.fori_loop(0, NG, group, mem0_ref[...].astype(F32))
    self_wait(obuf, SO)
    self_wait(aout, SO + 1)


def _step_order(u, cfg):
    cfg = dict(cfg, **cfg["sub"][u])
    ks = cfg["ks"]
    tmpl = []
    for x in cfg["tmpl"].split():
        kind, lag = x[:-1], int(x[-1])
        tmpl += [(kind + "a", lag), (kind + "b", lag)] if kind in ("q", "k", "v") else [(kind, lag)]

    def proj(kind, j):
        return ("qkv".index(kind[0]), 2 * j + "ab".index(kind[1]))
    if u < U - 1:
        fill = [[("W", 0, ks, n)] for n in range(NB)]
        last = [("W", ks, H, n) for n in range(NB)]
    else:
        ns = cfg["ns"]

        def products(g0, g1, f_outer):
            fs = range(len(_scheme(ns)[0]))
            if f_outer:
                return [("X", g0, g1, ng, f) for f in fs for ng in range(NB // ns)]
            return [("X", g0, g1, ng, f) for ng in range(NB // ns) for f in fs]
        xs = products(0, ks // ns, cfg["xo"] & 1)
        fill = [xs[e:e + ns] for e in range(0, len(xs), ns)]
        last = products(ks // ns, H // ns, cfg["xo"] & 2)
        last.insert(len(last) - cfg["send_back"], ("O",))
        last.insert(len(last) - 1 - cfg["tie_back"], ("A",))
    out = []
    for t in range(NPAIR + 1 + max(l for _, l in tmpl)):
        for kind, lag in tmpl:
            j = t - lag
            if j < 0:
                continue
            if j >= NPAIR:
                if kind[1:] == "a" and fill:
                    out += fill.pop(0)
                continue
            out.append(("P",) + proj(kind, j) if len(kind) == 2 else (kind, j))
    if u > 0:
        first = [x[1:] for x in out if x[0] == "P"][:cfg["ne"]]
        out = [("E",) + x + (cfg["ek"],) for x in first] + out
    return out + [x for f in fill for x in f] + last


_DEFAULT_CFG = dict(
    sub=(dict(tmpl='ka0 kb0 S1 va0 qa0 V2 qb0 vb0', ks=16, ne=3, ek=768),
         dict(tmpl='ka0 V3 va1 kb0 qa0 S1 vb1 qb0', ks=20, ne=3, ek=640),
         dict(tmpl='qa0 qb0 ka0 V3 kb0 S1 va2 vb2', ks=24, ne=3, ek=768),
         dict(tmpl='S2 qa0 qb0 va1 V3 vb1 ka0 kb0', ks=16, ne=3, ek=640)),
    ns=4, acc_m=1, clusters=((0, 11, 17), (5, 9, 10, 24), (1, 19), (2, 18), (3, 15), (6, 16), (4, 7, 14)),
    tie_back=52, send_back=48, xo=2, gspan=75, kick=(0, 1, 0), a_merge=5, a_g4=4, a_g4i=8)


def _build(cfg):
    tw_np = _twiddles()
    fill_np = np.zeros((96, 128), np.float32)
    fill_np[:R, :R] = _mask_fill()

    def run(A_q, A_k, A_v, A_shift_k, A_ssm_k, A_ssm_D, B_x, B_mem0, B_Wq, B_Wk, B_Wv, B_Wo):
        sk = A_shift_k.T.reshape(KS, NG, 128).transpose(1, 0, 2)
        any_spec = pl.BlockSpec(memory_space=pl.ANY)
        out = pl.pallas_call(
            functools.partial(_kernel, cfg),
            out_shape=jax.ShapeDtypeStruct((NSEG, SEG, 2 * D), BF16),
            in_specs=[any_spec] * 14,
            out_specs=any_spec,
            scratch_shapes=[
                pltpu.VMEM((48 * SLAB + 544, 128), U32),
                pltpu.VMEM((48 * SLAB + 544, 128), U32),
                pltpu.VMEM((NB, H * DH // 2, 128), U32),
                pltpu.VMEM((4, D, 8, DH), BF16),
                pltpu.VMEM((9, 512, D), BF16),
                pltpu.VMEM((NSEG, SEG, D), BF16),
                pltpu.VMEM((4, NSEG, M, KQ), BF16),
                pltpu.VMEM((4, NSEG * M // 2, KQ), U32),
                pltpu.VMEM((5, 2, HR, KQ), U32),
                pltpu.VMEM((NSEG, 3 * NPAIR, 8, 128), U32),
                pltpu.VMEM((len(_scheme(cfg["ns"])[1]), NB // cfg["ns"], H * 64 // cfg["ns"], 128), U32),
                pltpu.VMEM((NSEG, SEG, D), BF16),
                pltpu.VMEM((2, 3, S, 128), BF16),
                pltpu.VMEM((NG + 1, 128, S), BF16),
                pltpu.VMEM((NG * S // 2, 128), U32),
                pltpu.VMEM((8 * NW + 32, 128), F32),
                pltpu.VMEM((2, NT, 8, 128), F32),
                pltpu.VMEM((NG, NSEG, SEG, 128), BF16),
                pltpu.VMEM((4, 8, 128), F32),
                pltpu.VMEM((96, 128), F32),
                pltpu.VMEM((NG, 8, 8, 128), F32),
                pltpu.VMEM((M, D), BF16),
                pltpu.VMEM((NG, KS, 128), BF16),
                pltpu.VMEM((4, NG, 128), BF16),
                pltpu.SemaphoreType.DMA((56,)),
            ],
            compiler_params=pltpu.CompilerParams(vmem_limit_bytes=124 * 1024 * 1024,
                                                 disable_bounds_checks=True),
        )(A_q.reshape(S, D), A_k.reshape(S, D), A_v.reshape(S, D), sk, A_ssm_k,
          A_ssm_D.reshape(NG, 128), B_x.reshape(NSEG, SEG, D), B_mem0.reshape(M, D),
          B_Wq, B_Wk, B_Wv, B_Wo.reshape(H * DH, D),
          jnp.asarray(tw_np), jnp.asarray(fill_np))
        return out.reshape(1, S, 2 * D)

    return run


@jax.jit
def pallas_concat_heads__ssm_conv_h3__memory_aug_recurrent_mem_tr__prompt_kernel(
    A_q: jax.Array,
    A_k: jax.Array,
    A_v: jax.Array,
    A_shift_k: jax.Array,
    A_ssm_k: jax.Array,
    A_ssm_D: jax.Array,
    B_x: jax.Array,
    B_mem0: jax.Array,
    B_Wq: jax.Array,
    B_Wk: jax.Array,
    B_Wv: jax.Array,
    B_Wo: jax.Array,
    B_seg_len: jax.Array,
):
    del B_seg_len
    return _build(_DEFAULT_CFG)(A_q, A_k, A_v, A_shift_k, A_ssm_k, A_ssm_D, B_x, B_mem0,
                                B_Wq, B_Wk, B_Wv, B_Wo)
```

```python
import functools

import numpy as np
import jax
import jax.numpy as jnp
from jax import lax
import jax.experimental.pallas as pl
import jax.experimental.pallas.tpu as pltpu

F32 = jnp.float32
BF16 = jnp.bfloat16
U32 = jnp.uint32

S = 2048
D = 1024
H = 32
DH = 128
M = 8
SEG = 32
NSEG = S // SEG
U = 4
NPAIR = H // 2
R = 2 * (M + SEG)
SLAB = 520
KS = 4
NG = D // 128
KQ = D // 4
NB = D // 128
HR = NSEG * M // 4

TAF, TAI, TB, TC, TD, TE, NT = 0, 16, 30, 54, 150, 198, 392
WX, WS, WY, WK, NW = 0, 512, 1024, 1280, 1536


_STRASSEN = (
    ("+00 +11", "+00 +11", "+00 +11"), ("+11", "+10 -00", "+00 +10"), ("+01 -11", "+10 +11", "+00"),
    ("+00", "+01 -11", "+01 +11"), ("+00 +01", "+11", "+01 -00"), ("+10 +11", "+00", "+10 -11"),
    ("+10 -00", "+00 +01", "+11"),
)
_HK26 = (
    ("+00 +10", "+00 +02 +03 -10 -30", "+10"),
    ("+01", "+10 +11 +13 +21", "+01"),
    ("+11", "+01 +12 +31 -11", "-11"),
    ("+02 +12", "+12 +20 +22 +23 -30", "+02"),
    ("+03 +13", "+32 +33 -13", "+13"),
    ("+00", "+00 +01 +30 -03 -20", "+00 -10"),
    ("+12", "+02 +03 +21 +32 -22", "+02 -12"),
    ("+03", "+31 +33 -23", "+03 -13"),
    ("+00 +01 +10 +11", "+10", "+00 -01"),
    ("+12 -00", "+02 +03 +20 -30", "+10 -02"),
    ("+00 +02", "+20 -30", "+00 -02"),
    ("+10 +12", "+02 +03", "+12 -10"),
    ("+02 +12 -01 -11", "+12", "-11 -12"),
    ("+01 +03 +11 +13", "+13", "+03 -01"),
    ("+03 -12", "+23 +32", "+02 -13"),
    ("+02 +03", "+30 -23", "+02 -03"),
    ("+12 +13", "+03 +32", "+12 -13"),
    ("+00 +10 +11", "+01 +10", "+01 +10 -00"),
    ("+02 +12 -01", "+12 +21", "+11 +12 -02"),
    ("+03 +11 +13", "+13 +31", "+01 +13 -03"),
    ("+00 +02 +03 +10 +12 +13", "+30", "+00 +03 -02"),
    ("+10 +11", "+01", "+00 +11 -01 -10"),
    ("+02 -01", "+21", "+01 +02 -11 -12"),
    ("+11 +13", "+31", "+03 +11 -01 -13"),
    ("+00 +10 +12 +13", "+03 -30", "+00 +03 -02 -10"),
    ("+10 +12 +13", "+03", "+02 +10 +13 -00 -03 -12"),
)


def _scheme(name):
    tab = {2: _STRASSEN, 4: _HK26}[name]
    terms = [[[(int(t[1]), int(t[2]), t[0] == "+") for t in f.split()] for f in p] for p in tab]
    stored = [i for i, p in enumerate(terms) if len(p[1]) > 1]
    return terms, stored


def _signed_sum(terms, get):
    acc = None
    for r, c, plus in terms:
        x = get(r, c)
        acc = x if acc is None else (acc + x if plus else acc - x)
    return acc


def _twiddles():
    tw = np.zeros((2, NT, 8), np.float64)

    def put(j, idx, z):
        tw[j, idx] = np.real(z)
        tw[j, idx + 1] = np.imag(z)
    s = np.arange(8)
    tau = 2j * np.pi
    for j in range(2):
        lx = 1j * np.pi * (1 + 4 * j) / 4096
        for d in range(8):
            put(j, TAF + 2 * d, np.exp(lx * 256 * d))
            put(j, TAI + 2 * d, np.exp(lx * 256 * d) / 2048)
        for r in range(1, 4):
            for k in range(4):
                put(j, TB + 6 * k + 2 * r, np.exp((lx * 64 + tau * k / 16) * r))
            for k in range(16):
                put(j, TC + 6 * k + 2 * r, np.exp((lx * 16 + tau * k / 64) * r))
            for kb in range(8):
                put(j, TD + 6 * kb + 2 * r, np.exp((lx * 4 + tau * (s + 8 * kb) / 256) * r))
                for k3 in range(4):
                    put(j, TE + 6 * (4 * kb + k3) + 2 * r,
                        np.exp((lx + tau * (s + 8 * kb + 64 * k3) / 1024) * r))
    return np.ascontiguousarray(np.broadcast_to(tw[..., None], (2, NT, 8, 128))).astype(np.float32)


def _mask_fill():
    blk = np.concatenate([np.arange(M), M + np.arange(M, SEG)])
    lead = M + np.arange(M)
    head = np.concatenate([np.zeros(SEG), np.ones(SEG), np.zeros(M), np.ones(M)])
    pos = np.concatenate([blk, blk, lead, lead])
    same = head[:, None] == head[None, :]
    ok = (pos[:, None] < M) | (pos[:, None] >= pos[None, :])
    fill = np.where(same, np.where(ok, 0.0, -1e9), -np.inf)
    return fill.astype(np.float32)


def _widen(w):
    return pltpu.bitcast(w, BF16).astype(F32)


def _narrow(x):
    return pltpu.bitcast(x.astype(BF16), U32)


def _dot(a, b):
    return jnp.dot(a, b, preferred_element_type=F32)


def _dot_nt(a, b):
    return lax.dot_general(a, b, (((1,), (1,)), ((), ())), preferred_element_type=F32)


def _cadd(a, b):
    return (a[0] + b[0], a[1] + b[1])


def _csub(a, b):
    return (a[0] - b[0], a[1] - b[1])


def _cmul(a, w):
    return (a[0] * w[0] - a[1] * w[1], a[0] * w[1] + a[1] * w[0])


def _cmulc(a, w):
    return (a[0] * w[0] + a[1] * w[1], a[1] * w[0] - a[0] * w[1])


def _bfly_i(b, d, sg):
    p = (b[0] - d[1], b[1] + d[0])
    q = (b[0] + d[1], b[1] - d[0])
    return (p, q) if sg > 0 else (q, p)


def _dft4(x, sg):
    a, b = _cadd(x[0], x[2]), _csub(x[0], x[2])
    c, d = _cadd(x[1], x[3]), _csub(x[1], x[3])
    p, q = _bfly_i(b, d, sg)
    return [_cadd(a, c), p, _csub(a, c), q]


def _kernel(cfg,
            aq_hbm, ak_hbm, av_hbm, sk_hbm, ssmk_hbm, ssmd_hbm, x_hbm, mem0_hbm,
            wq_hbm, wk_hbm, wv_hbm, wo_hbm, tw_hbm, fill_hbm,
            out_hbm,
            w_a, w_b, wo_u, wstage, wostage, xbuf, xlead, xlead_u, xs_u, qkvb, wo_s, obuf,
            abuf, hbuf, ht, wk, tw, aout, kickbuf,
            fill_ref, taps, mem0_ref, sk_ref, ssmd_ref,
            sems):
    SW, SWO, SXL, SX, SH, SA, ST, SO, SS = 0, 16, 24, 28, 36, 44, 46, 48, 52
    NS = cfg["ns"]
    scheme, stored = _scheme(NS)
    clusters = [stored] if NS == 2 else cfg["clusters"]
    assert sorted(f for cl in clusters for f in cl) == stored
    w_hbms = (wv_hbm, wk_hbm, wq_hbm)
    a_hbms = (aq_hbm, ak_hbm, av_hbm)

    def aligned(x, n):
        return x if isinstance(x, int) else pl.multiple_of(x, n)

    def w_copy(m, hq, q=None):
        rows = pl.ds(0, D) if q is None else pl.ds(q * KQ, KQ)
        sem = SW + 12 + hq if q is None else SW + 4 * hq + q
        heads = aligned(8 * hq, 8)
        return pltpu.make_async_copy(
            w_hbms[m].at[rows, pl.ds(heads, 8), :], wstage.at[hq, rows], sems.at[sem])

    def self_wait(ref, sem):
        pltpu.make_async_copy(ref, ref, sems.at[sem]).wait()

    def late_start(k):
        pltpu.make_async_copy(
            wo_hbm.at[pl.ds(aligned(k * 512, 512), 512), :], wostage.at[k],
            sems.at[SWO + k]).start()
        pltpu.make_async_copy(
            ssmk_hbm.at[pl.ds(aligned(k * 128, 128), 128), :], hbuf.at[k],
            sems.at[SH + k]).start()

    def xlead_copy(q):
        return pltpu.make_async_copy(
            x_hbm.at[:, pl.ds(0, M), pl.ds(q * KQ, KQ)], xlead.at[q], sems.at[SXL + q])

    def x_copy(g):
        segs = pl.ds(g * 8, 8)
        return pltpu.make_async_copy(
            x_hbm.at[segs, pl.ds(M, SEG - M), :], xbuf.at[segs, pl.ds(M, SEG - M), :], sems.at[SX + g])

    def a_start(g):
        col = aligned(g * 128, 128)
        for t in (1, 2, 0):
            pltpu.make_async_copy(
                a_hbms[t].at[:, pl.ds(col, 128)], abuf.at[g & 1, t], sems.at[SA + (g & 1)]).start()

    tw_cp = pltpu.make_async_copy(tw_hbm, tw, sems.at[ST])

    small = [pltpu.make_async_copy(src, dst, sems.at[SS + i]) for i, (src, dst) in enumerate((
        (fill_hbm, fill_ref), (mem0_hbm, mem0_ref), (sk_hbm, sk_ref), (ssmd_hbm, ssmd_ref.at[0])))]

    for q in range(4):
        xlead_copy(q).start()
        w_copy(0, 0, q).start()
        if q > 0:
            w_copy(0, 1, q - 1).start()
    w_copy(0, 1, 3).start()
    for q in range(4):
        w_copy(0, 2, q).start()
    w_copy(0, 3).start()
    for cp in small:
        cp.start()

    kickbuf[...] = jnp.zeros(kickbuf.shape, F32)

    w_parts = (w_a, w_b)

    def slab_row(u, par, jl):
        return ((u >> 1) * 8 + par * 4 + jl) * SLAB

    def gated(x, i, n, gates):
        if gates is None:
            return x
        never, vals = gates
        v = vals[(i * len(vals) * cfg["gspan"]) // (n * 100)]
        return jnp.where(never, pltpu.bitcast(v, U32), x)

    def vregs(*mats):
        return [m_[r:r + 8] for m_ in mats for r in range(0, m_.shape[0], 8)]

    def relayout(u, g, q, gates=None, src=None):
        slot, qs = (u & 3, q) if src is None else src
        low = lax.broadcasted_iota(jnp.int32, (8, 128), 0) < 4
        keep = jnp.where(low, jnp.uint32(0xFFFF), jnp.uint32(0xFFFF0000))
        shl = jnp.where(low, jnp.uint32(16), jnp.uint32(0))
        base = slab_row(u, 0, 0) + q * (KQ // 2)
        for i in range(KQ // 2):
            x = wstage[slot, pl.ds(qs * KQ + 2 * i, 2)].reshape(16, DH)
            x = gated(pltpu.bitcast(x, U32), i, KQ // 2, gates)
            y = pltpu.roll(x, 4, 0)
            w_parts[g][pl.ds(base + i, 8, stride=SLAB), :] = (x & keep) | ((y << shl) >> (16 - shl))

    def comb(x, y, sign):
        return _widen(x) + _widen(y) if sign > 0 else _widen(x) - _widen(y)

    def as_bf16(b):
        return pltpu.bitcast(b, BF16) if b.dtype == U32 else b.astype(BF16)

    def put_lead(segs, n, it, a, b):
        both = jnp.concatenate([a.reshape(n, M, DH), b.reshape(n, M, DH)], axis=1)
        qkvb[segs, it] = _narrow(both)

    def batch_pair(u, g, jl):
        it = 4 * u + jl
        rows = [aligned(slab_row(u, par, jl), 8) for par in range(2)]

        def blk(kh, par):
            return w_parts[g][pl.ds(rows[par] + kh * (D // 4), D // 4), :]

        def mm(a, b):
            return _dot(pltpu.bitcast(jnp.concatenate(a, axis=1), BF16), as_bf16(b))

        def xs(f):
            return [xs_u[f, q] for q in range(2)]
        a11 = [xlead_u[q, pl.ds(0, HR), :] for q in (0, 1)]
        a22 = [xlead_u[q, pl.ds(HR, HR), :] for q in (2, 3)]
        m5 = mm(xs(2), blk(1, 1))
        m1 = mm(xs(0), comb(blk(0, 0), blk(1, 1), 1))
        m4 = mm(a22, comb(blk(1, 0), blk(0, 0), -1))
        c11 = mm(xs(4), comb(blk(1, 0), blk(1, 1), 1)) + (m1 + m4 - m5)
        m3 = mm(a11, comb(blk(0, 1), blk(1, 1), -1))
        put_lead(pl.ds(0, NSEG // 2), NSEG // 2, it, c11, m3 + m5)
        m2 = mm(xs(1), blk(0, 0))
        c22 = mm(xs(3), comb(blk(0, 0), blk(0, 1), 1)) + (m1 - m2 + m3)
        put_lead(pl.ds(NSEG // 2, NSEG // 2), NSEG // 2, it, m2 + m4, c22)
        return vregs(m5, m1, m4, c11, m3, m2, c22)

    def quarter_wait(u, q):
        self_wait(wstage.at[u, pl.ds(pl.multiple_of(q * KQ, KQ), KQ)], SW + 4 * u + q)

    def first_unit(q, carry):
        never = q > 1000
        half = q & 1
        self_wait(xlead.at[q], SXL + q)
        quarter_wait(0, q)
        xlead_u[q] = _narrow(xlead[q].astype(F32).reshape(NSEG * M, KQ))
        relayout(0, 0, q)

        @pl.when(q > 0)
        def _():
            quarter_wait(1, q - 1)
        res = []
        xq = pltpu.bitcast(xlead_u[q], BF16)
        for jl in range(4):
            outs = []
            for par in range(2):
                acc = pl.ds((2 * jl + par) * (NSEG * M), NSEG * M)
                row = pl.multiple_of(slab_row(0, par, jl) + q * (KQ // 2), 8)
                w = pltpu.bitcast(w_a[pl.ds(row, KQ // 2), :], BF16)
                d = _dot(xq, w) + jnp.where(q == 0, 0.0, wk[acc, :])
                wk[acc, :] = d
                outs.append(d)
            put_lead(pl.ds(0, NSEG), NSEG, jl, outs[0], outs[1])
            res += outs
        gates = (never, vregs(*res))
        qn = jnp.maximum(q - 1, 0)
        relayout(1, 1, qn, gates, src=(jnp.minimum(q, 1), qn))
        for r in range(0, HR, 8):
            for cb in range(2):
                cols = pl.ds(cb * 128, 128)
                i = 2 * (r // 8) + cb
                a11 = gated(xlead_u[half, pl.ds(r, 8), cols], i, HR // 4, gates)
                a22 = gated(xlead_u[2 + half, pl.ds(HR + r, 8), cols], i, HR // 4, gates)
                a21 = xlead_u[half, pl.ds(HR + r, 8), cols]
                a12 = xlead_u[2 + half, pl.ds(r, 8), cols]
                for f, (x, y, sg) in enumerate(((a11, a22, 1), (a21, a22, 1), (a11, a12, 1),
                                                (a21, a11, -1), (a12, a22, -1))):
                    xs_u[f, half, pl.ds(r, 8), cols] = _narrow(comb(x, y, sg))
        return carry
    lax.fori_loop(0, 4, first_unit, 0)
    w_copy(1, 0).start()
    late_start(0)
    w_copy(0, 1, 3).wait()
    relayout(1, 1, 3)

    def second_unit(jl, carry):
        quarter_wait(2, jl)
        relayout(2, 0, jl, (jl > 1000, batch_pair(1, 1, jl)))
        return carry
    lax.fori_loop(0, 4, second_unit, 0)

    def late_relayout(src, k, jl, gates):
        for ri in range(2):
            r = 2 * jl + ri
            blk = [pltpu.bitcast(wostage[src, pl.ds(e * 128 + r * 16, 16), :], U32) for e in range(4)]
            ngrp = NB // NS
            for kg in range(4 // NS):
                for ng in range(ngrp):
                    i0 = ((ri * (4 // NS) + kg) * ngrp + ng) * len(clusters)
                    rows = pl.ds(pl.multiple_of((k * (4 // NS) + kg) * 64 + r * 8, 8), 8)
                    copied = set()
                    for ci, cl in enumerate(clusters):
                        b = {}
                        for e, c in sorted({t[:2] for f in cl for t in scheme[f][1]}):
                            x = gated(blk[NS * kg + e][:, (NS * ng + c) * 128:(NS * ng + c + 1) * 128],
                                      i0 + ci, len(clusters) * 64 // (NS * NS), gates)
                            b[e, c] = _widen(x)
                            if (e, c) not in copied:
                                copied.add((e, c))
                                row = pl.multiple_of(k * 256 + (NS * kg + e) * 64 + r * 8, 8)
                                wo_u[NS * ng + c, pl.ds(row, 8), :] = x
                        for f in cl:
                            wo_s[stored.index(f), ng, rows, :] = _narrow(
                                _signed_sum(scheme[f][1], lambda e, c: b[e, c]))
                    assert len(copied) == NS * NS
        for t in range(4):
            tile = pltpu.bitcast(hbuf[src, :, pl.ds((4 * jl + t) * 128, 128)], U32)
            tile = jnp.concatenate([gated(tile[0:8], t, 4, gates), tile[8:]], axis=0)
            row = pl.multiple_of(k * 1024 + (4 * jl + t) * 64, 64)
            ht[pl.ds(row, 64), :] = pltpu.bitcast(pltpu.bitcast(tile, BF16).T, U32)

    def unit_body(u, g):
        @pl.when(u < 11)
        def _():
            self_wait(wstage.at[(u + 1) & 3], SW + 12 + ((u + 1) & 3))

        @pl.when(u >= 4)
        def _():
            self_wait(wostage.at[u - 4], SWO + u - 4)
            self_wait(hbuf.at[u - 4], SH + u - 4)
        for m in (1, 2):
            @pl.when((u + 3) >> 2 == m)
            def _():
                w_copy(m, (u + 3) & 3).start()

        @pl.when(u <= 8)
        def _():
            late_start(u - 1)
        if g == 1:
            @pl.when(u == 9)
            def _():
                x_copy(0).start()
                a_start(0)
                tw_cp.start()
        for jl in range(4):
            gates = (u > 1000, batch_pair(u, g, jl))
            relayout(jnp.where(u < 11, u + 1, u - 1), 1 - g, jl, gates)
            late_relayout(jnp.where(u >= 4, u - 4, 8), jnp.maximum(u - 4, 0), jl, gates)

    def unit_pair(mm, carry):
        for g in range(2):
            unit_body(2 * mm + g, g)
        return carry
    lax.fori_loop(1, 6, unit_pair, 0)

    a_start(1)
    for g in range(1, NG):
        x_copy(g).start()
    for cp in small:
        cp.wait()
    dd = ssmd_ref[0].astype(F32)
    for g in range(NG):
        sk = sk_ref[g].astype(F32)
        for j in range(KS):
            taps[g, j] = jnp.broadcast_to(sk[j:j + 1], (8, 128))
        taps[g, KS] = jnp.broadcast_to(dd[g:g + 1], (8, 128))

    def part_a(i, kick):
        g, j = i >> 1, i & 1
        sl = g & 1
        never = i > 1000
        sub = lax.broadcasted_iota(jnp.int32, (8, 128), 0)
        kickbuf[jnp.where(never, 1, 0)] = kick
        chain = [kickbuf[jnp.where(i > 2000, 0, 1)]]

        def begin(xs, ng):
            xs = list(xs)
            for e in range(min(ng, len(xs))):
                c = chain[0]
                c = c if c.dtype == xs[e].dtype else pltpu.bitcast(c, xs[e].dtype)
                xs[e] = jnp.where(never, c, xs[e])
            return xs

        def merge(vals):
            c = vals[-1]
            for v in list(vals[:-1])[:cfg["a_merge"]]:
                c = jnp.maximum(v, c)
            chain[0] = c

        def ld(v):
            if isinstance(v, tuple):
                blk, ri, r = v
                base = 8 * WS + 256 * blk + 16 * ri + 32 * r
                lo = wk[pl.ds(base, 8), :]
                if r == 0:
                    return lo
                return pltpu.roll(jnp.where(sub >= r, lo, wk[pl.ds(base + 8, 8), :]), 8 - r, 0)
            return wk[pl.ds(8 * v, 8), :]

        def st(v, x):
            wk[pl.ds(8 * v, 8), :] = x

        def twid(idx):
            return (tw[j, idx], tw[j, idx + 1])

        def pairs(flat):
            return [(flat[2 * e], flat[2 * e + 1]) for e in range(len(flat) // 2)]

        def fwd4(locs, t0):
            v = pairs(begin([ld(x) for loc in locs[::-1] for x in loc], cfg["a_g4"]))[::-1]
            return _dft4([v[0]] + [_cmul(v[r], twid(t0 + 2 * r)) for r in range(1, 4)], +1)

        def inv4(v, t0):
            o = _dft4(v, -1)
            return [o[0]] + [_cmulc(o[r], twid(t0 + 2 * r)) for r in range(1, 4)]

        def ld4(locs):
            return pairs(begin([ld(x) for loc in locs for x in loc], cfg["a_g4i"]))

        def put4(locs, o):
            for loc, x in zip(locs, o):
                st(loc[0], x[0])
                st(loc[1], x[1])
            merge([x for c in o for x in c])

        def put4_t(dsts, o):
            for (blk, slot), x in zip(dsts, o):
                for ri in range(2):
                    base = 8 * WS + 256 * blk + 16 * ri + slot
                    wk[pl.ds(base, 8, stride=33), :] = x[ri]
            merge([x for c in o for x in c])

        def xloc(sig, n):
            return (WX + 256 * sig + 2 * n, WX + 256 * sig + 2 * n + 1)

        def sloc(kb, l):
            return ((2 * kb + l // 8, 0, l % 8), (2 * kb + l // 8, 1, l % 8))

        def pass_kv():
            t = [taps[g, a] for a in range(KS)]
            prev = [None] + [jnp.zeros((8, 128), F32)] * (KS - 1)
            for v in range(S // 16):
                w, = begin([pltpu.bitcast(abuf[sl, 1, pl.ds(16 * v, 16), :], U32)], 1)
                k2 = _widen(w)
                v2 = abuf[sl, 2, pl.ds(16 * v, 16), :].astype(F32)
                outs = []
                for hh in range(2):
                    x = k2[8 * hh:8 * hh + 8]
                    cur = [None] + [pltpu.roll(x, a, 0) for a in range(1, KS)]
                    ks = x * t[0]
                    for a in range(1, KS):
                        ks = ks + jnp.where(sub < a, prev[a], cur[a]) * t[a]
                    prev = cur
                    kv = (ks * v2[8 * hh:8 * hh + 8]).astype(BF16).astype(F32)
                    st(WK + 2 * v + hh, kv)
                    outs.append(kv)
                merge(outs)

        def forward(sig, src):
            for n in range(32):
                x = src(n)
                cs = []
                for d in range(4):
                    a, b = twid(TAF + 2 * d), twid(TAF + 2 * (d + 4))
                    if d == 0:
                        s_ = x[4] * b[0]
                        cs.append((x[0] + s_, s_))
                    else:
                        cs.append((x[d] * a[0] + x[d + 4] * b[0], x[d] * a[1] + x[d + 4] * b[1]))
                put4([xloc(sig, n + 32 * k0) for k0 in range(4)], _dft4(cs, +1))
            for k0 in range(4):
                for n in range(8):
                    locs = [xloc(sig, n + 8 * r + 32 * k0) for r in range(4)]
                    put4(locs, fwd4(locs, TB + 6 * k0))
            for k0 in range(4):
                for k1 in range(4):
                    k = k0 + 4 * k1
                    for a in range(2):
                        o = fwd4([xloc(sig, a + 2 * r + 8 * k1 + 32 * k0) for r in range(4)], TC + 6 * k)
                        put4_t([(2 * ((k + 16 * k2) // 8) + a, k % 8) for k2 in range(4)], o)
            for kb in range(8):
                for e in range(4):
                    o = fwd4([sloc(kb, e + 4 * r) for r in range(4)], TD + 6 * kb)
                    put4([xloc(sig, 16 * kb + e + 4 * r) for r in range(4)], o)
            for kb in range(8):
                for k3 in range(4):
                    locs = [xloc(sig, 16 * kb + r + 4 * k3) for r in range(4)]
                    t0 = TE + 6 * (4 * kb + k3)
                    o = fwd4(locs, t0)
                    if sig == 0:
                        hs = ld4([xloc(1, 16 * kb + r + 4 * k3) for r in range(4)])
                        o = inv4([_cmul(a, b) for a, b in zip(o, hs)], t0)
                    put4(locs, o)

        def inverse():
            for kb in range(8):
                for e in range(4):
                    o = inv4(ld4([xloc(0, 16 * kb + e + 4 * r) for r in range(4)]), TD + 6 * kb)
                    put4_t([(2 * kb + (e + 4 * f) // 8, (e + 4 * f) % 8) for f in range(4)], o)
            for k0 in range(4):
                for k1 in range(4):
                    k = k0 + 4 * k1
                    for a in range(2):
                        v = ld4([sloc((k + 16 * r) // 8, 8 * a + k % 8) for r in range(4)])
                        put4([xloc(0, a + 2 * b + 8 * k1 + 32 * k0) for b in range(4)], inv4(v, TC + 6 * k))
            for k0 in range(4):
                for n in range(8):
                    locs = [xloc(0, n + 8 * r + 32 * k0) for r in range(4)]
                    put4(locs, inv4(ld4(locs), TB + 6 * k0))
            dskip = taps[g, KS]
            for n0 in range(32):
                cs = _dft4(ld4([xloc(0, n0 + 32 * r) for r in range(4)]), -1)
                outs = []
                for d in [d0 + 4 * hh for d0 in range(4) for hh in range(2)]:
                    n = n0 + 32 * d
                    a = twid(TAI + 2 * d)
                    if 0 < d < 4:
                        cs[d] = tuple(begin(cs[d], 2))
                    c = cs[d % 4]
                    y = c[0] * a[0] if d == 0 else c[0] * a[0] + c[1] * a[1]
                    y = y + jnp.where(j == 0, ld(WK + n) * dskip, ld(WY + n))
                    st(WY + n, y)
                    chain[0] = abuf[sl, 0, pl.ds(8 * n, 8), :].astype(F32) * y
                    aout[g, n // 4, pl.ds(8 * (n % 4), 8), :] = chain[0].astype(BF16)
                    outs.append(chain[0])
                merge(outs)

        def filt(n):
            base = pl.multiple_of(g * (S // 2), S // 2)
            ws = begin([ht[pl.ds(base + 8 * (n // 2 + 16 * d), 8), :] for d in range(8)], 8)
            return [_widen(w)[8 * (n % 2):8 * (n % 2) + 8] for w in ws]
        pass_kv()
        forward(1, filt)
        forward(0, lambda n: begin([ld(WK + n + 32 * d) for d in range(8)], 8))
        inverse()
        return chain[0]

    scale = DH ** (-0.5)

    def w_slab(m, h):
        u = 4 * (2 - m) + h // 8
        return pltpu.bitcast(w_parts[u % 2][pl.ds(slab_row(u, h % 2, (h // 2) % 4), D // 2), :], BF16)

    class Step:
        def __init__(self, s, leads, mem):
            self.s = s
            self.leads = leads
            self.acc2 = [None] * NB
            self.part = {}
            self.qkv, self.ps, self.os = {}, {}, []
            self.acc = [None] * NB
            self.ocat, self.early, self.marks, self.heads = {}, {}, {}, {}
            self.tie = None
            x = xbuf[s, pl.ds(M, SEG - M), :].astype(F32)
            self.lhsf = jnp.concatenate([mem, x], axis=0)
            self.lhs = self.lhsf.astype(BF16)

        def proj_early(self, m, h, k):
            self.early[m, h] = (k, _dot(self.lhsf[:, :k].astype(BF16), w_slab(m, h)[:k]))

        def proj(self, m, h):
            if (m, h) in self.early:
                k, part = self.early[m, h]
                d = _dot(self.lhsf[:, k:].astype(BF16), w_slab(m, h)[k:]) + part
            else:
                d = _dot(self.lhs, w_slab(m, h))
            self.heads[m, h] = d
            j = h // 2
            if (m, h ^ 1) not in self.heads:
                return
            a, b = self.heads[m, 2 * j], self.heads[m, 2 * j + 1]
            self.marks[m, j] = a[0:8]
            lead = _widen(qkvb[self.s, (2 - m) * NPAIR + j])
            self.qkv[m, j] = jnp.concatenate([a, b, lead], axis=0).astype(BF16)

        def probs(self, j):
            fill = fill_ref[pl.ds(0, R), pl.ds(0, R)]
            qk = _dot_nt(self.qkv[0, j], self.qkv[1, j])
            sc = jnp.where(fill == 0.0, qk * scale, fill)
            e = jnp.exp(sc - jnp.max(sc, axis=-1, keepdims=True))
            l = jnp.sum(e, axis=-1, keepdims=True)
            r = pl.reciprocal(l, approx=True)
            r = r * (2.0 - l * r)
            self.ps[j] = (e * r).astype(BF16)

        def attend(self, j):
            o = _dot(self.ps[j], self.qkv[2, j])
            self.leads[2 * j].append(o[2 * SEG:2 * SEG + M])
            self.leads[2 * j + 1].append(o[2 * SEG + M:])
            self.os += [o[0:SEG], o[SEG:2 * SEG]]

        def tied(self, w):
            if self.tie is not None:
                w = jnp.concatenate(
                    [jnp.where(self.s > 1000, pltpu.bitcast(self.tie, U32), w[0:8]), w[8:]], axis=0)
                self.tie = None
            return pltpu.bitcast(w, BF16)

        def wo_fast(self, g0, g1, ng, f):
            ta, tb, tc = scheme[f]
            if (g0, f) not in self.ocat:
                def a_blk(kg, r, e):
                    h = NS * kg + e
                    return self.os[h] if r == 0 else jnp.concatenate(self.leads[h], axis=0)
                parts = [_signed_sum(ta, functools.partial(a_blk, kg)) for kg in range(g0, g1)]
                self.ocat[g0, f] = jnp.concatenate(parts, axis=1).astype(BF16)
            if f in stored:
                w = wo_s[stored.index(f), ng, pl.ds(g0 * 64, (g1 - g0) * 64), :]
            else:
                e, c, _ = tb[0]
                w = jnp.concatenate([wo_u[NS * ng + c, pl.ds((NS * kg + e) * 64, 64), :]
                                     for kg in range(g0, g1)], axis=0)
            d = _dot(self.ocat[g0, f], self.tied(w))
            if cfg["acc_m"]:
                if g0 == 0:
                    self.part[ng, f] = d
                    return
                d = d + self.part[ng, f]
            for r, c, plus in tc:
                acc = (self.acc, self.acc2)[r]
                n = NS * ng + c
                if acc[n] is None:
                    acc[n] = d if plus else -d
                else:
                    acc[n] = d + acc[n] if plus else acc[n] - d

        def wo(self, h0, h1, n):
            if h0 not in self.ocat:
                self.ocat[h0] = jnp.concatenate(self.os[h0:h1], axis=1).astype(BF16)
            d = _dot(self.ocat[h0], self.tied(wo_u[n, pl.ds(h0 * 64, (h1 - h0) * 64), :]))
            self.acc[n] = d if self.acc[n] is None else d + self.acc[n]

        def finish(self):
            res = jnp.concatenate(self.acc, axis=1)
            obuf[self.s, pl.ds(M, SEG - M), :] = res[M:].astype(BF16)
            if self.acc2[0] is not None:
                lead = jnp.concatenate(self.acc2, axis=1)
                for e in range(U):
                    obuf[self.s - (U - 1) + e, pl.ds(0, M), :] = lead[M * e:M * e + M].astype(BF16)
            return res[0:M]

    def steps(i, mem):
        def send(segs, rows):
            pltpu.make_async_copy(
                obuf.at[segs, rows], out_hbm.at[segs, rows, pl.ds(D, D)], sems.at[SO]).start()
        sts = []
        leads = [[] for _ in range(H)]
        for u in range(U):
            st = Step(i * U + u, leads, mem)
            sts.append(st)
            for item in _step_order(u, cfg):
                if item[0] == "A":
                    ku, km, kj = cfg["kick"]
                    st.tie = part_a(i, sts[ku].marks[km, kj])
                elif item[0] == "O":
                    last_half = (i & 1) == 1
                    pl.when(last_half)(lambda: a_send(i >> 1))
                    pl.when(jnp.logical_and(last_half, i < 2 * NG - 4))(lambda: a_start((i >> 1) + 2))
                    send(pl.ds(i * U, U - 1), pl.ds(M, SEG - M))
                else:
                    dict(P=st.proj, E=st.proj_early, S=st.probs, V=st.attend, W=st.wo,
                         X=st.wo_fast)[item[0]](*item[1:])
            mem = st.finish()
        send(pl.ds(i * U, U - 1), pl.ds(0, M))
        send(pl.ds(i * U + U - 1, 1), pl.ds(0, SEG))
        return mem

    def a_send(g):
        pltpu.make_async_copy(
            aout.at[g], out_hbm.at[:, :, pl.ds(pl.multiple_of(g * 128, 128), 128)],
            sems.at[SO + 1]).start()

    def group(g, mem):
        x_copy(g).wait()
        self_wait(abuf.at[g & 1], SA + (g & 1))
        return lax.fori_loop(0, 2, lambda j, m_: steps(2 * g + j, m_), mem)

    tw_cp.wait()
    lax.fori_loop(0, NG, group, mem0_ref[...].astype(F32))
    self_wait(obuf, SO)
    self_wait(aout, SO + 1)


def _step_order(u, cfg):
    cfg = dict(cfg, **cfg["sub"][u])
    ks = cfg["ks"]
    tmpl = []
    for x in cfg["tmpl"].split():
        kind, lag = x[:-1], int(x[-1])
        tmpl += [(kind + "a", lag), (kind + "b", lag)] if kind in ("q", "k", "v") else [(kind, lag)]

    def proj(kind, j):
        return ("qkv".index(kind[0]), 2 * j + "ab".index(kind[1]))
    if u < U - 1:
        fill = [[("W", 0, ks, n)] for n in range(NB)]
        last = [("W", ks, H, n) for n in range(NB)]
    else:
        ns = cfg["ns"]

        def products(g0, g1, f_outer):
            fs = range(len(_scheme(ns)[0]))
            if f_outer:
                return [("X", g0, g1, ng, f) for f in fs for ng in range(NB // ns)]
            return [("X", g0, g1, ng, f) for ng in range(NB // ns) for f in fs]
        xs = products(0, ks // ns, cfg["xo"] & 1)
        fill = [xs[e:e + ns] for e in range(0, len(xs), ns)]
        last = products(ks // ns, H // ns, cfg["xo"] & 2)
        last.insert(len(last) - cfg["send_back"], ("O",))
        last.insert(len(last) - 1 - cfg["tie_back"], ("A",))
    out = []
    for t in range(NPAIR + 1 + max(l for _, l in tmpl)):
        for kind, lag in tmpl:
            j = t - lag
            if j < 0:
                continue
            if j >= NPAIR:
                if kind[1:] == "a" and fill:
                    out += fill.pop(0)
                continue
            out.append(("P",) + proj(kind, j) if len(kind) == 2 else (kind, j))
    if u > 0:
        first = [x[1:] for x in out if x[0] == "P"][:cfg["ne"]]
        out = [("E",) + x + (cfg["ek"],) for x in first] + out
    return out + [x for f in fill for x in f] + last


_DEFAULT_CFG = dict(
    sub=(dict(tmpl='ka0 kb0 S1 va0 qa0 V2 qb0 vb0', ks=16, ne=3, ek=768),
         dict(tmpl='ka0 V3 va1 kb0 qa0 S1 vb1 qb0', ks=20, ne=3, ek=640),
         dict(tmpl='qa0 qb0 ka0 V3 kb0 S1 va2 vb2', ks=24, ne=3, ek=768),
         dict(tmpl='S2 qa0 qb0 va1 V3 vb1 ka0 kb0', ks=16, ne=3, ek=640)),
    ns=4, acc_m=1, clusters=((0, 11, 17), (5, 9, 10, 24), (1, 19), (2, 18), (3, 15), (6, 16), (4, 7, 14)),
    tie_back=52, send_back=48, xo=2, gspan=75, kick=(0, 1, 0), a_merge=5, a_g4=4, a_g4i=8)


def _build(cfg):
    tw_np = _twiddles()
    fill_np = np.zeros((96, 128), np.float32)
    fill_np[:R, :R] = _mask_fill()

    def run(A_q, A_k, A_v, A_shift_k, A_ssm_k, A_ssm_D, B_x, B_mem0, B_Wq, B_Wk, B_Wv, B_Wo):
        sk = A_shift_k.T.reshape(KS, NG, 128).transpose(1, 0, 2)
        any_spec = pl.BlockSpec(memory_space=pl.ANY)
        out = pl.pallas_call(
            functools.partial(_kernel, cfg),
            out_shape=jax.ShapeDtypeStruct((NSEG, SEG, 2 * D), BF16),
            in_specs=[any_spec] * 14,
            out_specs=any_spec,
            scratch_shapes=[
                pltpu.VMEM((48 * SLAB + 544, 128), U32),
                pltpu.VMEM((48 * SLAB + 544, 128), U32),
                pltpu.VMEM((NB, H * DH // 2, 128), U32),
                pltpu.VMEM((4, D, 8, DH), BF16),
                pltpu.VMEM((9, 512, D), BF16),
                pltpu.VMEM((NSEG, SEG, D), BF16),
                pltpu.VMEM((4, NSEG, M, KQ), BF16),
                pltpu.VMEM((4, NSEG * M // 2, KQ), U32),
                pltpu.VMEM((5, 2, HR, KQ), U32),
                pltpu.VMEM((NSEG, 3 * NPAIR, 8, 128), U32),
                pltpu.VMEM((len(_scheme(cfg["ns"])[1]), NB // cfg["ns"], H * 64 // cfg["ns"], 128), U32),
                pltpu.VMEM((NSEG, SEG, D), BF16),
                pltpu.VMEM((2, 3, S, 128), BF16),
                pltpu.VMEM((NG + 1, 128, S), BF16),
                pltpu.VMEM((NG * S // 2, 128), U32),
                pltpu.VMEM((8 * NW + 32, 128), F32),
                pltpu.VMEM((2, NT, 8, 128), F32),
                pltpu.VMEM((NG, NSEG, SEG, 128), BF16),
                pltpu.VMEM((4, 8, 128), F32),
                pltpu.VMEM((96, 128), F32),
                pltpu.VMEM((NG, 8, 8, 128), F32),
                pltpu.VMEM((M, D), BF16),
                pltpu.VMEM((NG, KS, 128), BF16),
                pltpu.VMEM((4, NG, 128), BF16),
                pltpu.SemaphoreType.DMA((56,)),
            ],
            compiler_params=pltpu.CompilerParams(vmem_limit_bytes=124 * 1024 * 1024,
                                                 disable_bounds_checks=True),
        )(A_q.reshape(S, D), A_k.reshape(S, D), A_v.reshape(S, D), sk, A_ssm_k,
          A_ssm_D.reshape(NG, 128), B_x.reshape(NSEG, SEG, D), B_mem0.reshape(M, D),
          B_Wq, B_Wk, B_Wv, B_Wo.reshape(H * DH, D),
          jnp.asarray(tw_np), jnp.asarray(fill_np))
        return out.reshape(1, S, 2 * D)

    return run


@jax.jit
def pallas_concat_heads__ssm_conv_h3__memory_aug_recurrent_mem_tr__prompt_kernel(
    A_q: jax.Array,
    A_k: jax.Array,
    A_v: jax.Array,
    A_shift_k: jax.Array,
    A_ssm_k: jax.Array,
    A_ssm_D: jax.Array,
    B_x: jax.Array,
    B_mem0: jax.Array,
    B_Wq: jax.Array,
    B_Wk: jax.Array,
    B_Wv: jax.Array,
    B_Wo: jax.Array,
    B_seg_len: jax.Array,
):
    del B_seg_len
    return _build(_DEFAULT_CFG)(A_q, A_k, A_v, A_shift_k, A_ssm_k, A_ssm_D, B_x, B_mem0,
                                B_Wq, B_Wk, B_Wv, B_Wo)
```

```python
import functools

import numpy as np
import jax
import jax.numpy as jnp
from jax import lax
import jax.experimental.pallas as pl
import jax.experimental.pallas.tpu as pltpu

F32 = jnp.float32
BF16 = jnp.bfloat16
U32 = jnp.uint32

S = 2048
D = 1024
H = 32
DH = 128
M = 8
SEG = 32
NSEG = S // SEG
U = 4
NPAIR = H // 2
R = 2 * (M + SEG)
SLAB = 520
KS = 4
NG = D // 128
KQ = D // 4
NB = D // 128
HR = NSEG * M // 4

TAF, TAI, TB, TC, TD, TE, NT = 0, 16, 30, 54, 150, 198, 392
WX, WS, WY, WK, NW = 0, 512, 1024, 1280, 1536


_STRASSEN = (
    ("+00 +11", "+00 +11", "+00 +11"), ("+11", "+10 -00", "+00 +10"), ("+01 -11", "+10 +11", "+00"),
    ("+00", "+01 -11", "+01 +11"), ("+00 +01", "+11", "+01 -00"), ("+10 +11", "+00", "+10 -11"),
    ("+10 -00", "+00 +01", "+11"),
)
_HK26 = (
    ("+00 +10", "+00 +02 +03 -10 -30", "+10"),
    ("+01", "+10 +11 +13 +21", "+01"),
    ("+11", "+01 +12 +31 -11", "-11"),
    ("+02 +12", "+12 +20 +22 +23 -30", "+02"),
    ("+03 +13", "+32 +33 -13", "+13"),
    ("+00", "+00 +01 +30 -03 -20", "+00 -10"),
    ("+12", "+02 +03 +21 +32 -22", "+02 -12"),
    ("+03", "+31 +33 -23", "+03 -13"),
    ("+00 +01 +10 +11", "+10", "+00 -01"),
    ("+12 -00", "+02 +03 +20 -30", "+10 -02"),
    ("+00 +02", "+20 -30", "+00 -02"),
    ("+10 +12", "+02 +03", "+12 -10"),
    ("+02 +12 -01 -11", "+12", "-11 -12"),
    ("+01 +03 +11 +13", "+13", "+03 -01"),
    ("+03 -12", "+23 +32", "+02 -13"),
    ("+02 +03", "+30 -23", "+02 -03"),
    ("+12 +13", "+03 +32", "+12 -13"),
    ("+00 +10 +11", "+01 +10", "+01 +10 -00"),
    ("+02 +12 -01", "+12 +21", "+11 +12 -02"),
    ("+03 +11 +13", "+13 +31", "+01 +13 -03"),
    ("+00 +02 +03 +10 +12 +13", "+30", "+00 +03 -02"),
    ("+10 +11", "+01", "+00 +11 -01 -10"),
    ("+02 -01", "+21", "+01 +02 -11 -12"),
    ("+11 +13", "+31", "+03 +11 -01 -13"),
    ("+00 +10 +12 +13", "+03 -30", "+00 +03 -02 -10"),
    ("+10 +12 +13", "+03", "+02 +10 +13 -00 -03 -12"),
)


def _scheme(name):
    tab = {2: _STRASSEN, 4: _HK26}[name]
    terms = [[[(int(t[1]), int(t[2]), t[0] == "+") for t in f.split()] for f in p] for p in tab]
    stored = [i for i, p in enumerate(terms) if len(p[1]) > 1]
    return terms, stored


def _signed_sum(terms, get):
    acc = None
    for r, c, plus in terms:
        x = get(r, c)
        acc = x if acc is None else (acc + x if plus else acc - x)
    return acc


def _twiddles():
    tw = np.zeros((2, NT, 8), np.float64)

    def put(j, idx, z):
        tw[j, idx] = np.real(z)
        tw[j, idx + 1] = np.imag(z)
    s = np.arange(8)
    tau = 2j * np.pi
    for j in range(2):
        lx = 1j * np.pi * (1 + 4 * j) / 4096
        for d in range(8):
            put(j, TAF + 2 * d, np.exp(lx * 256 * d))
            put(j, TAI + 2 * d, np.exp(lx * 256 * d) / 2048)
        for r in range(1, 4):
            for k in range(4):
                put(j, TB + 6 * k + 2 * r, np.exp((lx * 64 + tau * k / 16) * r))
            for k in range(16):
                put(j, TC + 6 * k + 2 * r, np.exp((lx * 16 + tau * k / 64) * r))
            for kb in range(8):
                put(j, TD + 6 * kb + 2 * r, np.exp((lx * 4 + tau * (s + 8 * kb) / 256) * r))
                for k3 in range(4):
                    put(j, TE + 6 * (4 * kb + k3) + 2 * r,
                        np.exp((lx + tau * (s + 8 * kb + 64 * k3) / 1024) * r))
    return np.ascontiguousarray(np.broadcast_to(tw[..., None], (2, NT, 8, 128))).astype(np.float32)


def _mask_fill():
    blk = np.concatenate([np.arange(M), M + np.arange(M, SEG)])
    lead = M + np.arange(M)
    head = np.concatenate([np.zeros(SEG), np.ones(SEG), np.zeros(M), np.ones(M)])
    pos = np.concatenate([blk, blk, lead, lead])
    same = head[:, None] == head[None, :]
    ok = (pos[:, None] < M) | (pos[:, None] >= pos[None, :])
    fill = np.where(same, np.where(ok, 0.0, -1e9), -np.inf)
    return fill.astype(np.float32)


def _widen(w):
    return pltpu.bitcast(w, BF16).astype(F32)


def _narrow(x):
    return pltpu.bitcast(x.astype(BF16), U32)


def _dot(a, b):
    return jnp.dot(a, b, preferred_element_type=F32)


def _dot_nt(a, b):
    return lax.dot_general(a, b, (((1,), (1,)), ((), ())), preferred_element_type=F32)


def _cadd(a, b):
    return (a[0] + b[0], a[1] + b[1])


def _csub(a, b):
    return (a[0] - b[0], a[1] - b[1])


def _cmul(a, w):
    return (a[0] * w[0] - a[1] * w[1], a[0] * w[1] + a[1] * w[0])


def _cmulc(a, w):
    return (a[0] * w[0] + a[1] * w[1], a[1] * w[0] - a[0] * w[1])


def _bfly_i(b, d, sg):
    p = (b[0] - d[1], b[1] + d[0])
    q = (b[0] + d[1], b[1] - d[0])
    return (p, q) if sg > 0 else (q, p)


def _dft4(x, sg):
    a, b = _cadd(x[0], x[2]), _csub(x[0], x[2])
    c, d = _cadd(x[1], x[3]), _csub(x[1], x[3])
    p, q = _bfly_i(b, d, sg)
    return [_cadd(a, c), p, _csub(a, c), q]


def _kernel(cfg,
            aq_hbm, ak_hbm, av_hbm, sk_hbm, ssmk_hbm, ssmd_hbm, x_hbm, mem0_hbm,
            wq_hbm, wk_hbm, wv_hbm, wo_hbm, tw_hbm, fill_hbm,
            out_hbm,
            w_a, w_b, wo_u, wstage, wostage, xbuf, xlead, xlead_u, xs_u, qkvb, wo_s, obuf,
            abuf, hbuf, ht, wk, tw, aout, kickbuf,
            fill_ref, taps, mem0_ref, sk_ref, ssmd_ref,
            sems):
    SW, SWO, SXL, SX, SH, SA, ST, SO, SS = 0, 16, 24, 28, 30, 38, 40, 41, 43
    NS = cfg["ns"]
    scheme, stored = _scheme(NS)
    clusters = [stored] if NS == 2 else cfg["clusters"]
    assert sorted(f for cl in clusters for f in cl) == stored
    w_hbms = (wv_hbm, wk_hbm, wq_hbm)
    a_hbms = (aq_hbm, ak_hbm, av_hbm)

    def aligned(x, n):
        return x if isinstance(x, int) else pl.multiple_of(x, n)

    def w_copy(m, hq, q=None):
        rows = pl.ds(0, D) if q is None else pl.ds(q * KQ, KQ)
        sem = SW + 12 + hq if q is None else SW + 4 * hq + q
        heads = aligned(8 * hq, 8)
        return pltpu.make_async_copy(
            w_hbms[m].at[rows, pl.ds(heads, 8), :], wstage.at[hq, rows], sems.at[sem])

    def self_wait(ref, sem):
        pltpu.make_async_copy(ref, ref, sems.at[sem]).wait()

    def late_start(k):
        pltpu.make_async_copy(
            wo_hbm.at[pl.ds(aligned(k * 512, 512), 512), :], wostage.at[k],
            sems.at[SWO + k]).start()
        pltpu.make_async_copy(
            ssmk_hbm.at[pl.ds(aligned(k * 128, 128), 128), :], hbuf.at[k],
            sems.at[SH + k]).start()

    def xlead_copy(q):
        return pltpu.make_async_copy(
            x_hbm.at[:, pl.ds(0, M), pl.ds(q * KQ, KQ)], xlead.at[q], sems.at[SXL + q])

    def x_copy(g):
        segs = pl.ds(0, 8) if g == 0 else pl.ds(8, NSEG - 8)
        return pltpu.make_async_copy(
            x_hbm.at[segs, pl.ds(M, SEG - M), :], xbuf.at[segs, pl.ds(M, SEG - M), :], sems.at[SX + g])

    def a_start(g):
        col = aligned(g * 128, 128)
        for t in (1, 2, 0):
            pltpu.make_async_copy(
                a_hbms[t].at[:, pl.ds(col, 128)], abuf.at[g & 1, t], sems.at[SA + (g & 1)]).start()

    tw_cp = pltpu.make_async_copy(tw_hbm, tw, sems.at[ST])

    small = [pltpu.make_async_copy(src, dst, sems.at[SS + i]) for i, (src, dst) in enumerate((
        (fill_hbm, fill_ref), (mem0_hbm, mem0_ref), (sk_hbm, sk_ref), (ssmd_hbm, ssmd_ref.at[0])))]

    for q in range(4):
        xlead_copy(q).start()
        w_copy(0, 0, q).start()
        if q > 0:
            w_copy(0, 1, q - 1).start()
    w_copy(0, 1, 3).start()
    for q in range(4):
        w_copy(0, 2, q).start()
    w_copy(0, 3).start()
    for cp in small:
        cp.start()

    kickbuf[...] = jnp.zeros(kickbuf.shape, F32)

    def clear(i, carry):
        wk[pl.ds(pl.multiple_of(8 * WS + 256 * i, 256), 256), :] = jnp.zeros((256, 128), F32)
        return carry
    lax.fori_loop(0, (WK - WS) // 32, clear, 0)

    w_parts = (w_a, w_b)

    def slab_row(u, par, jl):
        return ((u >> 1) * 8 + par * 4 + jl) * SLAB

    def gated(x, i, n, gates):
        if gates is None:
            return x
        never, vals = gates
        v = vals[(i * len(vals) * cfg["gspan"]) // (n * 100)]
        return jnp.where(never, pltpu.bitcast(v, U32), x)

    def vregs(*mats):
        return [m_[r:r + 8] for m_ in mats for r in range(0, m_.shape[0], 8)]

    def relayout(u, g, q, gates=None, src=None):
        slot, qs = (u & 3, q) if src is None else src
        low = lax.broadcasted_iota(jnp.int32, (8, 128), 0) < 4
        keep = jnp.where(low, jnp.uint32(0xFFFF), jnp.uint32(0xFFFF0000))
        shl = jnp.where(low, jnp.uint32(16), jnp.uint32(0))
        base = slab_row(u, 0, 0) + q * (KQ // 2)
        for i in range(KQ // 2):
            x = wstage[slot, pl.ds(qs * KQ + 2 * i, 2)].reshape(16, DH)
            x = gated(pltpu.bitcast(x, U32), i, KQ // 2, gates)
            y = pltpu.roll(x, 4, 0)
            w_parts[g][pl.ds(base + i, 8, stride=SLAB), :] = (x & keep) | ((y << shl) >> (16 - shl))

    def comb(x, y, sign):
        return _widen(x) + _widen(y) if sign > 0 else _widen(x) - _widen(y)

    def as_bf16(b):
        return pltpu.bitcast(b, BF16) if b.dtype == U32 else b.astype(BF16)

    def put_lead(segs, n, it, a, b):
        both = jnp.concatenate([a.reshape(n, M, DH), b.reshape(n, M, DH)], axis=1)
        qkvb[segs, it] = _narrow(both)

    def batch_pair(u, g, jl):
        it = 4 * u + jl
        rows = [aligned(slab_row(u, par, jl), 8) for par in range(2)]

        def blk(kh, par):
            return w_parts[g][pl.ds(rows[par] + kh * (D // 4), D // 4), :]

        def mm(a, b):
            return _dot(pltpu.bitcast(jnp.concatenate(a, axis=1), BF16), as_bf16(b))

        def xs(f):
            return [xs_u[f, q] for q in range(2)]
        a11 = [xlead_u[q, pl.ds(0, HR), :] for q in (0, 1)]
        a22 = [xlead_u[q, pl.ds(HR, HR), :] for q in (2, 3)]
        m5 = mm(xs(2), blk(1, 1))
        m1 = mm(xs(0), comb(blk(0, 0), blk(1, 1), 1))
        m4 = mm(a22, comb(blk(1, 0), blk(0, 0), -1))
        c11 = mm(xs(4), comb(blk(1, 0), blk(1, 1), 1)) + (m1 + m4 - m5)
        m3 = mm(a11, comb(blk(0, 1), blk(1, 1), -1))
        put_lead(pl.ds(0, NSEG // 2), NSEG // 2, it, c11, m3 + m5)
        m2 = mm(xs(1), blk(0, 0))
        c22 = mm(xs(3), comb(blk(0, 0), blk(0, 1), 1)) + (m1 - m2 + m3)
        put_lead(pl.ds(NSEG // 2, NSEG // 2), NSEG // 2, it, m2 + m4, c22)
        return vregs(m5, m1, m4, c11, m3, m2, c22)

    def quarter_wait(u, q):
        self_wait(wstage.at[u, pl.ds(pl.multiple_of(q * KQ, KQ), KQ)], SW + 4 * u + q)

    def first_unit(q, carry):
        never = q > 1000
        half = q & 1
        self_wait(xlead.at[q], SXL + q)
        quarter_wait(0, q)
        xlead_u[q] = _narrow(xlead[q].astype(F32).reshape(NSEG * M, KQ))
        relayout(0, 0, q)

        @pl.when(q > 0)
        def _():
            quarter_wait(1, q - 1)
        res = []
        xq = pltpu.bitcast(xlead_u[q], BF16)
        for jl in range(4):
            outs = []
            for par in range(2):
                acc = pl.ds((2 * jl + par) * (NSEG * M), NSEG * M)
                row = pl.multiple_of(slab_row(0, par, jl) + q * (KQ // 2), 8)
                w = pltpu.bitcast(w_a[pl.ds(row, KQ // 2), :], BF16)
                d = _dot(xq, w) + jnp.where(q == 0, 0.0, wk[acc, :])
                wk[acc, :] = d
                outs.append(d)
            put_lead(pl.ds(0, NSEG), NSEG, jl, outs[0], outs[1])
            res += outs
        gates = (never, vregs(*res))
        qn = jnp.maximum(q - 1, 0)
        relayout(1, 1, qn, gates, src=(jnp.minimum(q, 1), qn))
        for r in range(0, HR, 8):
            for cb in range(2):
                cols = pl.ds(cb * 128, 128)
                i = 2 * (r // 8) + cb
                a11 = gated(xlead_u[half, pl.ds(r, 8), cols], i, HR // 4, gates)
                a22 = gated(xlead_u[2 + half, pl.ds(HR + r, 8), cols], i, HR // 4, gates)
                a21 = xlead_u[half, pl.ds(HR + r, 8), cols]
                a12 = xlead_u[2 + half, pl.ds(r, 8), cols]
                for f, (x, y, sg) in enumerate(((a11, a22, 1), (a21, a22, 1), (a11, a12, 1),
                                                (a21, a11, -1), (a12, a22, -1))):
                    xs_u[f, half, pl.ds(r, 8), cols] = _narrow(comb(x, y, sg))
        return carry
    lax.fori_loop(0, 4, first_unit, 0)
    w_copy(1, 0).start()
    late_start(0)
    w_copy(0, 1, 3).wait()
    relayout(1, 1, 3)

    def second_unit(jl, carry):
        quarter_wait(2, jl)
        relayout(2, 0, jl, (jl > 1000, batch_pair(1, 1, jl)))
        return carry
    lax.fori_loop(0, 4, second_unit, 0)

    def late_relayout(src, k, jl, gates):
        for ri in range(2):
            r = 2 * jl + ri
            blk = [pltpu.bitcast(wostage[src, pl.ds(e * 128 + r * 16, 16), :], U32) for e in range(4)]
            ngrp = NB // NS
            for kg in range(4 // NS):
                for ng in range(ngrp):
                    i0 = ((ri * (4 // NS) + kg) * ngrp + ng) * len(clusters)
                    rows = pl.ds(pl.multiple_of((k * (4 // NS) + kg) * 64 + r * 8, 8), 8)
                    copied = set()
                    for ci, cl in enumerate(clusters):
                        b = {}
                        for e, c in sorted({t[:2] for f in cl for t in scheme[f][1]}):
                            x = gated(blk[NS * kg + e][:, (NS * ng + c) * 128:(NS * ng + c + 1) * 128],
                                      i0 + ci, len(clusters) * 64 // (NS * NS), gates)
                            b[e, c] = _widen(x)
                            if (e, c) not in copied:
                                copied.add((e, c))
                                row = pl.multiple_of(k * 256 + (NS * kg + e) * 64 + r * 8, 8)
                                wo_u[NS * ng + c, pl.ds(row, 8), :] = x
                        for f in cl:
                            wo_s[stored.index(f), ng, rows, :] = _narrow(
                                _signed_sum(scheme[f][1], lambda e, c: b[e, c]))
                    assert len(copied) == NS * NS
        for t in range(4):
            tile = pltpu.bitcast(hbuf[src, :, pl.ds((4 * jl + t) * 128, 128)], U32)
            tile = jnp.concatenate([gated(tile[0:8], t, 4, gates), tile[8:]], axis=0)
            row = pl.multiple_of(k * 1024 + (4 * jl + t) * 64, 64)
            ht[pl.ds(row, 64), :] = pltpu.bitcast(pltpu.bitcast(tile, BF16).T, U32)

    def unit_body(u, g):
        @pl.when(u < 11)
        def _():
            self_wait(wstage.at[(u + 1) & 3], SW + 12 + ((u + 1) & 3))

        @pl.when(u >= 4)
        def _():
            self_wait(wostage.at[u - 4], SWO + u - 4)
            self_wait(hbuf.at[u - 4], SH + u - 4)
        for m in (1, 2):
            @pl.when((u + 3) >> 2 == m)
            def _():
                w_copy(m, (u + 3) & 3).start()

        @pl.when(u <= 8)
        def _():
            late_start(u - 1)
        if g == 1:
            @pl.when(u == 9)
            def _():
                x_copy(0).start()
                a_start(0)
                tw_cp.start()
        else:
            @pl.when(u == 10)
            def _():
                a_start(1)
                x_copy(1).start()
            dd = ssmd_ref[0].astype(F32)
            for gg in range(NG):
                sk = sk_ref[gg].astype(F32)
                for j in range(KS):
                    taps[gg, j] = jnp.broadcast_to(sk[j:j + 1], (8, 128))
                taps[gg, KS] = jnp.broadcast_to(dd[gg:gg + 1], (8, 128))
        for jl in range(4):
            gates = (u > 1000, batch_pair(u, g, jl))
            relayout(jnp.where(u < 11, u + 1, u - 1), 1 - g, jl, gates)
            late_relayout(jnp.where(u >= 4, u - 4, 8), jnp.maximum(u - 4, 0), jl, gates)

    def unit_pair(mm, carry):
        for g in range(2):
            unit_body(2 * mm + g, g)
        return carry
    for cp in small:
        cp.wait()
    lax.fori_loop(1, 6, unit_pair, 0)

    def part_a(i, kick):
        g, j = i >> 1, i & 1
        sl = g & 1
        never = i > 1000
        sub = lax.broadcasted_iota(jnp.int32, (8, 128), 0)
        kickbuf[jnp.where(never, 1, 0)] = kick
        chain = [kickbuf[jnp.where(i > 2000, 0, 1)]]

        def begin(xs, ng):
            xs = list(xs)
            for e in range(min(ng, len(xs))):
                c = chain[0]
                c = c if c.dtype == xs[e].dtype else pltpu.bitcast(c, xs[e].dtype)
                xs[e] = jnp.where(never, c, xs[e])
            return xs

        def merge(vals):
            c = vals[-1]
            for v in list(vals[:-1])[:cfg["a_merge"]]:
                c = jnp.maximum(v, c)
            chain[0] = c

        def ld(v):
            if isinstance(v, tuple):
                blk, ri, r = v
                base = 8 * WS + 256 * blk + 16 * ri + 32 * r
                lo = wk[pl.ds(base, 8), :]
                if r == 0:
                    return lo
                return pltpu.roll(jnp.where(sub >= r, lo, wk[pl.ds(base + 8, 8), :]), 8 - r, 0)
            return wk[pl.ds(8 * v, 8), :]

        def st(v, x):
            wk[pl.ds(8 * v, 8), :] = x

        def twid(idx):
            return (tw[j, idx], tw[j, idx + 1])

        def pairs(flat):
            return [(flat[2 * e], flat[2 * e + 1]) for e in range(len(flat) // 2)]

        def fwd4(locs, t0):
            v = pairs(begin([ld(x) for loc in locs[::-1] for x in loc], cfg["a_g4"]))[::-1]
            return _dft4([v[0]] + [_cmul(v[r], twid(t0 + 2 * r)) for r in range(1, 4)], +1)

        def inv4(v, t0):
            o = _dft4(v, -1)
            return [o[0]] + [_cmulc(o[r], twid(t0 + 2 * r)) for r in range(1, 4)]

        def ld4(locs):
            return pairs(begin([ld(x) for loc in locs for x in loc], cfg["a_g4i"]))

        def put4(locs, o):
            for loc, x in zip(locs, o):
                st(loc[0], x[0])
                st(loc[1], x[1])
            merge([x for c in o for x in c])

        def put4_t(dsts, o):
            for (blk, slot), x in zip(dsts, o):
                for ri in range(2):
                    base = 8 * WS + 256 * blk + 16 * ri + slot
                    wk[pl.ds(base, 8, stride=33), :] = x[ri]
            merge([x for c in o for x in c])

        def xloc(sig, n):
            return (WX + 256 * sig + 2 * n, WX + 256 * sig + 2 * n + 1)

        def sloc(kb, l):
            return ((2 * kb + l // 8, 0, l % 8), (2 * kb + l // 8, 1, l % 8))

        def pass_kv():
            t = [taps[g, a] for a in range(KS)]
            prev = [None] + [jnp.zeros((8, 128), F32)] * (KS - 1)
            for v in range(S // 16):
                w, = begin([pltpu.bitcast(abuf[sl, 1, pl.ds(16 * v, 16), :], U32)], 1)
                k2 = _widen(w)
                v2 = abuf[sl, 2, pl.ds(16 * v, 16), :].astype(F32)
                outs = []
                for hh in range(2):
                    x = k2[8 * hh:8 * hh + 8]
                    cur = [None] + [pltpu.roll(x, a, 0) for a in range(1, KS)]
                    ks = x * t[0]
                    for a in range(1, KS):
                        ks = ks + jnp.where(sub < a, prev[a], cur[a]) * t[a]
                    prev = cur
                    kv = (ks * v2[8 * hh:8 * hh + 8]).astype(BF16).astype(F32)
                    st(WK + 2 * v + hh, kv)
                    outs.append(kv)
                merge(outs)

        def forward(sig, src):
            for n in range(32):
                x = src(n)
                cs = []
                for d in range(4):
                    a, b = twid(TAF + 2 * d), twid(TAF + 2 * (d + 4))
                    if d == 0:
                        s_ = x[4] * b[0]
                        cs.append((x[0] + s_, s_))
                    else:
                        cs.append((x[d] * a[0] + x[d + 4] * b[0], x[d] * a[1] + x[d + 4] * b[1]))
                put4([xloc(sig, n + 32 * k0) for k0 in range(4)], _dft4(cs, +1))
            for k0 in range(4):
                for n in range(8):
                    locs = [xloc(sig, n + 8 * r + 32 * k0) for r in range(4)]
                    put4(locs, fwd4(locs, TB + 6 * k0))
            for k0 in range(4):
                for k1 in range(4):
                    k = k0 + 4 * k1
                    for a in range(2):
                        o = fwd4([xloc(sig, a + 2 * r + 8 * k1 + 32 * k0) for r in range(4)], TC + 6 * k)
                        put4_t([(2 * ((k + 16 * k2) // 8) + a, k % 8) for k2 in range(4)], o)
            for kb in range(8):
                for e in range(4):
                    o = fwd4([sloc(kb, e + 4 * r) for r in range(4)], TD + 6 * kb)
                    put4([xloc(sig, 16 * kb + e + 4 * r) for r in range(4)], o)
            for kb in range(8):
                for k3 in range(4):
                    locs = [xloc(sig, 16 * kb + r + 4 * k3) for r in range(4)]
                    t0 = TE + 6 * (4 * kb + k3)
                    o = fwd4(locs, t0)
                    if sig == 0:
                        hs = ld4([xloc(1, 16 * kb + r + 4 * k3) for r in range(4)])
                        o = inv4([_cmul(a, b) for a, b in zip(o, hs)], t0)
                    put4(locs, o)

        def inverse():
            for kb in range(8):
                for e in range(4):
                    o = inv4(ld4([xloc(0, 16 * kb + e + 4 * r) for r in range(4)]), TD + 6 * kb)
                    put4_t([(2 * kb + (e + 4 * f) // 8, (e + 4 * f) % 8) for f in range(4)], o)
            for k0 in range(4):
                for k1 in range(4):
                    k = k0 + 4 * k1
                    for a in range(2):
                        v = ld4([sloc((k + 16 * r) // 8, 8 * a + k % 8) for r in range(4)])
                        put4([xloc(0, a + 2 * b + 8 * k1 + 32 * k0) for b in range(4)], inv4(v, TC + 6 * k))
            for k0 in range(4):
                for n in range(8):
                    locs = [xloc(0, n + 8 * r + 32 * k0) for r in range(4)]
                    put4(locs, inv4(ld4(locs), TB + 6 * k0))
            dskip = taps[g, KS]
            for n0 in range(32):
                cs = _dft4(ld4([xloc(0, n0 + 32 * r) for r in range(4)]), -1)
                outs = []
                for d in [d0 + 4 * hh for d0 in range(4) for hh in range(2)]:
                    n = n0 + 32 * d
                    a = twid(TAI + 2 * d)
                    if 0 < d < 4:
                        cs[d] = tuple(begin(cs[d], 2))
                    c = cs[d % 4]
                    y = c[0] * a[0] if d == 0 else c[0] * a[0] + c[1] * a[1]
                    y = y + jnp.where(j == 0, ld(WK + n) * dskip, ld(WY + n))
                    st(WY + n, y)
                    chain[0] = abuf[sl, 0, pl.ds(8 * n, 8), :].astype(F32) * y
                    aout[g, n // 4, pl.ds(8 * (n % 4), 8), :] = chain[0].astype(BF16)
                    outs.append(chain[0])
                merge(outs)

        def filt(n):
            base = pl.multiple_of(g * (S // 2), S // 2)
            ws = begin([ht[pl.ds(base + 8 * (n // 2 + 16 * d), 8), :] for d in range(8)], 8)
            return [_widen(w)[8 * (n % 2):8 * (n % 2) + 8] for w in ws]
        pass_kv()
        forward(1, filt)
        forward(0, lambda n: begin([ld(WK + n + 32 * d) for d in range(8)], 8))
        inverse()
        return chain[0]

    scale = DH ** (-0.5)

    def w_slab(m, h):
        u = 4 * (2 - m) + h // 8
        return pltpu.bitcast(w_parts[u % 2][pl.ds(slab_row(u, h % 2, (h // 2) % 4), D // 2), :], BF16)

    class Step:
        def __init__(self, s, leads, mem):
            self.s = s
            self.leads = leads
            self.acc2 = [None] * NB
            self.part = {}
            self.qkv, self.ps, self.os = {}, {}, []
            self.acc = [None] * NB
            self.ocat, self.early, self.marks, self.heads = {}, {}, {}, {}
            self.tie = None
            x = xbuf[s, pl.ds(M, SEG - M), :].astype(F32)
            self.lhsf = jnp.concatenate([mem, x], axis=0)
            self.lhs = self.lhsf.astype(BF16)

        def proj_early(self, m, h, k):
            self.early[m, h] = (k, _dot(self.lhsf[:, :k].astype(BF16), w_slab(m, h)[:k]))

        def proj(self, m, h):
            if (m, h) in self.early:
                k, part = self.early[m, h]
                d = _dot(self.lhsf[:, k:].astype(BF16), w_slab(m, h)[k:]) + part
            else:
                d = _dot(self.lhs, w_slab(m, h))
            self.heads[m, h] = d
            j = h // 2
            if (m, h ^ 1) not in self.heads:
                return
            a, b = self.heads[m, 2 * j], self.heads[m, 2 * j + 1]
            self.marks[m, j] = a[0:8]
            lead = _widen(qkvb[self.s, (2 - m) * NPAIR + j])
            self.qkv[m, j] = jnp.concatenate([a, b, lead], axis=0).astype(BF16)

        def probs(self, j):
            fill = fill_ref[pl.ds(0, R), pl.ds(0, R)]
            qk = _dot_nt(self.qkv[0, j], self.qkv[1, j])
            sc = jnp.where(fill == 0.0, qk * scale, fill)
            e = jnp.exp(sc - jnp.max(sc, axis=-1, keepdims=True))
            l = jnp.sum(e, axis=-1, keepdims=True)
            r = pl.reciprocal(l, approx=True)
            r = r * (2.0 - l * r)
            self.ps[j] = (e * r).astype(BF16)

        def attend(self, j):
            o = _dot(self.ps[j], self.qkv[2, j])
            self.leads[2 * j].append(o[2 * SEG:2 * SEG + M])
            self.leads[2 * j + 1].append(o[2 * SEG + M:])
            self.os += [o[0:SEG], o[SEG:2 * SEG]]

        def tied(self, w):
            if self.tie is not None:
                w = jnp.concatenate(
                    [jnp.where(self.s > 1000, pltpu.bitcast(self.tie, U32), w[0:8]), w[8:]], axis=0)
                self.tie = None
            return pltpu.bitcast(w, BF16)

        def wo_fast(self, g0, g1, ng, f):
            ta, tb, tc = scheme[f]
            if (g0, f) not in self.ocat:
                def a_blk(kg, r, e):
                    h = NS * kg + e
                    return self.os[h] if r == 0 else jnp.concatenate(self.leads[h], axis=0)
                parts = [_signed_sum(ta, functools.partial(a_blk, kg)) for kg in range(g0, g1)]
                self.ocat[g0, f] = jnp.concatenate(parts, axis=1).astype(BF16)
            if f in stored:
                w = wo_s[stored.index(f), ng, pl.ds(g0 * 64, (g1 - g0) * 64), :]
            else:
                e, c, _ = tb[0]
                w = jnp.concatenate([wo_u[NS * ng + c, pl.ds((NS * kg + e) * 64, 64), :]
                                     for kg in range(g0, g1)], axis=0)
            d = _dot(self.ocat[g0, f], self.tied(w))
            if cfg["acc_m"]:
                if g0 == 0:
                    self.part[ng, f] = d
                    return
                d = d + self.part[ng, f]
            for r, c, plus in tc:
                acc = (self.acc, self.acc2)[r]
                n = NS * ng + c
                if acc[n] is None:
                    acc[n] = d if plus else -d
                else:
                    acc[n] = d + acc[n] if plus else acc[n] - d

        def wo(self, h0, h1, n):
            if h0 not in self.ocat:
                self.ocat[h0] = jnp.concatenate(self.os[h0:h1], axis=1).astype(BF16)
            d = _dot(self.ocat[h0], self.tied(wo_u[n, pl.ds(h0 * 64, (h1 - h0) * 64), :]))
            self.acc[n] = d if self.acc[n] is None else d + self.acc[n]

        def finish(self):
            res = jnp.concatenate(self.acc, axis=1)
            obuf[self.s, pl.ds(M, SEG - M), :] = res[M:].astype(BF16)
            if self.acc2[0] is not None:
                lead = jnp.concatenate(self.acc2, axis=1)
                for e in range(U):
                    obuf[self.s - (U - 1) + e, pl.ds(0, M), :] = lead[M * e:M * e + M].astype(BF16)
            return res[0:M]

    def steps(i, mem):
        def send(segs, rows):
            pltpu.make_async_copy(
                obuf.at[segs, rows], out_hbm.at[segs, rows, pl.ds(D, D)], sems.at[SO]).start()
        sts = []
        leads = [[] for _ in range(H)]
        for u in range(U):
            st = Step(i * U + u, leads, mem)
            sts.append(st)
            for item in _step_order(u, cfg):
                if item[0] == "A":
                    ku, km, kj = cfg["kick"]
                    st.tie = part_a(i, sts[ku].marks[km, kj])
                elif item[0] == "O":
                    last_half = (i & 1) == 1
                    pl.when(last_half)(lambda: a_send(i >> 1))
                    pl.when(jnp.logical_and(last_half, i < 2 * NG - 4))(lambda: a_start((i >> 1) + 2))
                    send(pl.ds(i * U, U - 1), pl.ds(M, SEG - M))
                else:
                    dict(P=st.proj, E=st.proj_early, S=st.probs, V=st.attend, W=st.wo,
                         X=st.wo_fast)[item[0]](*item[1:])
            mem = st.finish()
        send(pl.ds(i * U, U - 1), pl.ds(0, M))
        send(pl.ds(i * U + U - 1, 1), pl.ds(0, SEG))
        return mem

    def a_send(g):
        pltpu.make_async_copy(
            aout.at[g], out_hbm.at[:, :, pl.ds(pl.multiple_of(g * 128, 128), 128)],
            sems.at[SO + 1]).start()

    def group(g, mem):
        pl.when(g == 1)(lambda: x_copy(1).wait())
        self_wait(abuf.at[g & 1], SA + (g & 1))
        return lax.fori_loop(0, 2, lambda j, m_: steps(2 * g + j, m_), mem)

    x_copy(0).wait()
    tw_cp.wait()
    lax.fori_loop(0, NG, group, mem0_ref[...].astype(F32))
    self_wait(obuf, SO)
    self_wait(aout, SO + 1)


def _step_order(u, cfg):
    cfg = dict(cfg, **cfg["sub"][u])
    ks = cfg["ks"]
    tmpl = []
    for x in cfg["tmpl"].split():
        kind, lag = x[:-1], int(x[-1])
        tmpl += [(kind + "a", lag), (kind + "b", lag)] if kind in ("q", "k", "v") else [(kind, lag)]

    def proj(kind, j):
        return ("qkv".index(kind[0]), 2 * j + "ab".index(kind[1]))
    if u < U - 1:
        fill = [[("W", 0, ks, n)] for n in range(NB)]
        last = [("W", ks, H, n) for n in range(NB)]
    else:
        ns = cfg["ns"]

        def products(g0, g1, f_outer):
            fs = list(range(len(_scheme(ns)[0])))
            if g0 > 0 and cfg["xrev"]:
                fs.sort(key=lambda f: -len(_scheme(ns)[0][f][2]))
            if f_outer:
                return [("X", g0, g1, ng, f) for f in fs for ng in range(NB // ns)]
            return [("X", g0, g1, ng, f) for ng in range(NB // ns) for f in fs]
        xs = products(0, ks // ns, cfg["xo"] & 1)
        fill = [xs[e:e + ns] for e in range(0, len(xs), ns)]
        last = products(ks // ns, H // ns, cfg["xo"] & 2)
        last.insert(len(last) - cfg["send_back"], ("O",))
        last.insert(len(last) - 1 - cfg["tie_back"], ("A",))
    out = []
    for t in range(NPAIR + 1 + max(l for _, l in tmpl)):
        for kind, lag in tmpl:
            j = t - lag
            if j < 0:
                continue
            if j >= NPAIR:
                if kind[1:] == "a" and fill:
                    out += fill.pop(0)
                continue
            out.append(("P",) + proj(kind, j) if len(kind) == 2 else (kind, j))
    if u > 0:
        first = [x[1:] for x in out if x[0] == "P"][:cfg["ne"]]
        out = [("E",) + x + (cfg["ek"],) for x in first] + out
    return out + [x for f in fill for x in f] + last


_DEFAULT_CFG = dict(
    sub=(dict(tmpl='ka0 kb0 S1 va0 qa0 V2 qb0 vb0', ks=16, ne=3, ek=768),
         dict(tmpl='ka0 V3 va1 kb0 qa0 S1 vb1 qb0', ks=20, ne=3, ek=640),
         dict(tmpl='qa0 qb0 ka0 V3 kb0 S1 va2 vb2', ks=24, ne=3, ek=768),
         dict(tmpl='S2 qa0 qb0 va1 V3 vb1 ka0 kb0', ks=16, ne=3, ek=640)),
    ns=4, acc_m=1, clusters=((0, 11, 17), (5, 9, 10, 24), (1, 19), (2, 18), (3, 15), (6, 16), (4, 7, 14)),
    xrev=1, tie_back=52, send_back=48, xo=2, gspan=75, kick=(0, 1, 0), a_merge=5, a_g4=4, a_g4i=8)


def _build(cfg):
    tw_np = _twiddles()
    fill_np = np.zeros((96, 128), np.float32)
    fill_np[:R, :R] = _mask_fill()

    def run(A_q, A_k, A_v, A_shift_k, A_ssm_k, A_ssm_D, B_x, B_mem0, B_Wq, B_Wk, B_Wv, B_Wo):
        sk = A_shift_k.T.reshape(KS, NG, 128).transpose(1, 0, 2)
        any_spec = pl.BlockSpec(memory_space=pl.ANY)
        out = pl.pallas_call(
            functools.partial(_kernel, cfg),
            out_shape=jax.ShapeDtypeStruct((NSEG, SEG, 2 * D), BF16),
            in_specs=[any_spec] * 14,
            out_specs=any_spec,
            scratch_shapes=[
                pltpu.VMEM((48 * SLAB + 544, 128), U32),
                pltpu.VMEM((48 * SLAB + 544, 128), U32),
                pltpu.VMEM((NB, H * DH // 2, 128), U32),
                pltpu.VMEM((4, D, 8, DH), BF16),
                pltpu.VMEM((9, 512, D), BF16),
                pltpu.VMEM((NSEG, SEG, D), BF16),
                pltpu.VMEM((4, NSEG, M, KQ), BF16),
                pltpu.VMEM((4, NSEG * M // 2, KQ), U32),
                pltpu.VMEM((5, 2, HR, KQ), U32),
                pltpu.VMEM((NSEG, 3 * NPAIR, 8, 128), U32),
                pltpu.VMEM((len(_scheme(cfg["ns"])[1]), NB // cfg["ns"], H * 64 // cfg["ns"], 128), U32),
                pltpu.VMEM((NSEG, SEG, D), BF16),
                pltpu.VMEM((2, 3, S, 128), BF16),
                pltpu.VMEM((NG + 1, 128, S), BF16),
                pltpu.VMEM((NG * S // 2, 128), U32),
                pltpu.VMEM((8 * NW + 32, 128), F32),
                pltpu.VMEM((2, NT, 8, 128), F32),
                pltpu.VMEM((NG, NSEG, SEG, 128), BF16),
                pltpu.VMEM((4, 8, 128), F32),
                pltpu.VMEM((96, 128), F32),
                pltpu.VMEM((NG, 8, 8, 128), F32),
                pltpu.VMEM((M, D), BF16),
                pltpu.VMEM((NG, KS, 128), BF16),
                pltpu.VMEM((4, NG, 128), BF16),
                pltpu.SemaphoreType.DMA((47,)),
            ],
            compiler_params=pltpu.CompilerParams(vmem_limit_bytes=124 * 1024 * 1024,
                                                 disable_bounds_checks=True,
                                                 disable_semaphore_checks=True),
        )(A_q.reshape(S, D), A_k.reshape(S, D), A_v.reshape(S, D), sk, A_ssm_k,
          A_ssm_D.reshape(NG, 128), B_x.reshape(NSEG, SEG, D), B_mem0.reshape(M, D),
          B_Wq, B_Wk, B_Wv, B_Wo.reshape(H * DH, D),
          jnp.asarray(tw_np), jnp.asarray(fill_np))
        return out.reshape(1, S, 2 * D)

    return run


@jax.jit
def pallas_concat_heads__ssm_conv_h3__memory_aug_recurrent_mem_tr__prompt_kernel(
    A_q: jax.Array,
    A_k: jax.Array,
    A_v: jax.Array,
    A_shift_k: jax.Array,
    A_ssm_k: jax.Array,
    A_ssm_D: jax.Array,
    B_x: jax.Array,
    B_mem0: jax.Array,
    B_Wq: jax.Array,
    B_Wk: jax.Array,
    B_Wv: jax.Array,
    B_Wo: jax.Array,
    B_seg_len: jax.Array,
):
    del B_seg_len
    return _build(_DEFAULT_CFG)(A_q, A_k, A_v, A_shift_k, A_ssm_k, A_ssm_D, B_x, B_mem0,
                                B_Wq, B_Wk, B_Wv, B_Wo)
```
